```python
import jax
import jax.numpy as jnp

def _softmax(x, axis=-1):
    return jax.nn.softmax(x, axis=axis)

def _gelu(x):
    return jax.nn.gelu(x, approximate=True)

def _silu(x):
    return jax.nn.silu(x)

def _sigmoid(x):
    return jax.nn.sigmoid(x)

def _layernorm(x, axis=-1, eps=1e-05):
    m = jnp.mean(x, axis=axis, keepdims=True)
    v = jnp.var(x, axis=axis, keepdims=True)
    return (x - m) / jnp.sqrt(v + eps)

def _scatter_add(tgt, idx, src, axis=0):
    return tgt.at[idx].add(src)

def _segment_sum(src, seg, n):
    return jax.ops.segment_sum(src, seg, n)

class _Rng:

    def __init__(self, key):
        self._k = key

    def _next(self):
        self._k, sub = jax.random.split(self._k)
        return sub

    def normal(self, shape):
        return jax.random.normal(self._next(), shape, dtype=jnp.bfloat16)

    def randint(self, lo, hi, shape):
        return jax.random.randint(self._next(), shape, lo, hi, dtype=jnp.int32)

    def uniform(self, shape, lo=0.0, hi=1.0):
        return jax.random.uniform(self._next(), shape, jnp.bfloat16, lo, hi)

    def permutation(self, n):
        return jax.random.permutation(self._next(), n)
kernel_name = 'adaLN_cond__compressed_kv_cla__mixer_s_mlp__prompt'

def setup_inputs():
    _rng = _Rng(jax.random.key(int.from_bytes(__import__("os").urandom(4), "little")))
    _w = lambda a: (lambda t: t.astype(jnp.bfloat16) if jnp.issubdtype(t.dtype, jnp.floating) else t)(jnp.asarray(a))

    def _A_setup():
        B, H, Sq, Sk, D, M = (1, 32, 2048, 2048, 128, 640)
        Dc = 4 * D
        return {'x': _w((lambda *s: _rng.normal(s) * 0.05)(B, Sq, M)), 'c_kv': _w((lambda *s: _rng.normal(s) * 0.05)(B, Sk, Dc)), 'w_q': _w((lambda *s: _rng.normal(s) * 0.05)(M, H, D) * M ** (-0.5)), 'w_uk': _w((lambda *s: _rng.normal(s) * 0.05)(Dc, H, D) * Dc ** (-0.5)), 'w_uv': _w((lambda *s: _rng.normal(s) * 0.05)(Dc, H, D) * Dc ** (-0.5)), 'w_o': _w((lambda *s: _rng.normal(s) * 0.05)(H, D, M) * (H * D) ** (-0.5))}
    _A_in = _A_setup()

    def _B_setup():
        B, S, D, F = (1, 2048, 640, 1728)
        return {'x': _w((lambda *s: _rng.normal(s) * 0.05)(B, S, D)), 'w1': _w((lambda *s: _rng.normal(s) * 0.05)(D, D) * D ** (-0.5)), 'w2': _w((lambda *s: _rng.normal(s) * 0.05)(D, D) * D ** (-0.5)), 'w3': _w((lambda *s: _rng.normal(s) * 0.05)(D, F) * D ** (-0.5)), 'w4': _w((lambda *s: _rng.normal(s) * 0.05)(F, D) * F ** (-0.5))}
    _B_in = _B_setup()
    return {'A_x': _A_in['x'], 'A_c_kv': _A_in['c_kv'], 'A_w_q': _A_in['w_q'], 'A_w_uk': _A_in['w_uk'], 'A_w_uv': _A_in['w_uv'], 'A_w_o': _A_in['w_o'], 'B_x': _B_in['x'], 'B_w1': _B_in['w1'], 'B_w2': _B_in['w2'], 'B_w3': _B_in['w3'], 'B_w4': _B_in['w4'], 'c': _w((lambda *s: _rng.normal(s) * 0.05)(1, 640)), 'w_mod': _w((lambda *s: _rng.normal(s) * 0.05)(640, 6 * 640) * 640 ** (-0.5))}

def reference(A_x, A_c_kv, A_w_q, A_w_uk, A_w_uv, A_w_o, B_x, B_w1, B_w2, B_w3, B_w4, c, w_mod):

    def _A_ref(x, c_kv, w_q, w_uk, w_uv, w_o):
        B, Sq, M = (x.shape[0], x.shape[1], x.shape[2])
        Sk = c_kv.shape[1]
        H, D = (w_q.shape[1], w_q.shape[2])
        q = jnp.einsum('bqm,mhd->bhqd', x, w_q)
        k = jnp.einsum('bkc,chd->bhkd', c_kv, w_uk)
        v = jnp.einsum('bkc,chd->bhkd', c_kv, w_uv)
        scores = jnp.einsum('bhqd,bhkd->bhqk', q, k) * D ** (-0.5)
        off = Sk - Sq
        qi = jnp.arange(Sq)[:, None]
        kj = jnp.arange(Sk)[None, :]
        cmask = kj <= qi + off
        scores = jnp.where(cmask[None, None], scores, -1000000000.0)
        p = _softmax(scores, axis=-1)
        ctx = jnp.einsum('bhqk,bhkd->bhqd', p, v)
        return jnp.einsum('bhqd,hdm->bqm', ctx, w_o)

    def _B_ref(x, w1, w2, w3, w4):
        B, S, D = x.shape
        h = _gelu(_layernorm(x, axis=-1) @ w1)
        c = D // 4
        g0 = jnp.pad(h[:, :, 0 * c:1 * c], ((0, 0), (1, 0), (0, 0)))[:, :S, :]
        g1 = jnp.pad(h[:, :, 1 * c:2 * c], ((0, 0), (0, 1), (0, 0)))[:, 1:, :]
        g2 = jnp.pad(h[:, :, 2 * c:3 * c], ((0, 0), (2, 0), (0, 0)))[:, :S, :]
        g3 = jnp.pad(h[:, :, 3 * c:], ((0, 0), (0, 2), (0, 0)))[:, 2:, :]
        hs = jnp.concatenate([g0, g1, g2, g3], axis=-1) @ w2
        x1 = x + hs
        h2 = _gelu(_layernorm(x1, axis=-1) @ w3) @ w4
        return x1 + h2
    x = A_x
    mod = (_silu(c) @ w_mod).reshape(c.shape[0], 6, 1, -1)
    sa, ca, ga, sb, cb, gb = (mod[:, 0].copy(), mod[:, 1].copy(), mod[:, 2].copy(), mod[:, 3].copy(), mod[:, 4].copy(), mod[:, 5].copy())
    h = _layernorm(x, axis=-1) * (1 + ca) + sa
    x = x + ga * _A_ref(h, A_c_kv, A_w_q, A_w_uk, A_w_uv, A_w_o)
    h = _layernorm(x, axis=-1) * (1 + cb) + sb
    x = x + gb * _B_ref(h, B_w1, B_w2, B_w3, B_w4)
    return x
```

```python
import math

import jax
import jax.numpy as jnp
import jax.experimental.pallas as pl
import jax.experimental.pallas.tpu as pltpu

F32 = jnp.float32
BF16 = jnp.bfloat16
U32 = jnp.uint32
NT = (((1,), (1,)), ((), ()))
T = 128
EPS = 1e-5
LOG2E = math.log2(math.e)

GRP = 4
LEAD = 10
PROW = 3
RES = 32
LAT_A = 16
LAT_B = 20
ALEAD = 32
MID = 40
SD0, SDS, SDN, SDJ = 158, 2, 20, 30
QT = 0
ONV, OEND = 0.5, 24
SIDE, SLAG = 1, 4
L_LO, L_HI, L_RATIO = 2.0 ** -24, 2.0 ** 24, 4.0
RB = 256
PC = 32
P0, PSTEP, PD = 440, 30, 52
NLN, LN0, LNS = 4, 4, 5
LP = 16
PROLOGUE = ('|kva|Z; |b|; kva|wc|K0123; bw|xdn|C0@56 N0123@52 K4567; cx|mq|N4567@52 K89ab; '
            'd|y|C1@56 Kcdef; nmq|zo|M H01 H234567@30 Q0123; y||H89ab@30 Q4567; '
            'zo||L Hcdef@30 Q89ab S01 Qcdef')


def _dot(a, b):
    return jnp.dot(a, b, preferred_element_type=F32)


def _dot_nt(a, b):
    return jax.lax.dot_general(a, b, NT, preferred_element_type=F32)


def _ln(x):
    m = jnp.mean(x, axis=-1, keepdims=True)
    xc = x - m
    v = jnp.mean(xc * xc, axis=-1, keepdims=True)
    return xc * jnp.exp2(jnp.log(v + EPS) * (-0.5 * LOG2E))


def _rows(v, n):
    return jnp.broadcast_to(v[None], (n // 8, 8, v.shape[1])).reshape(n, v.shape[1])


def _gelu(x):
    c0 = math.sqrt(2.0 / math.pi)
    return 0.5 * x * (1.0 + jnp.tanh(c0 * (x + 0.044715 * (x * x * x))))


def _after(x, dep):
    return jnp.where(dep > jnp.inf, dep, x)


def _tie(x, dep):
    xu = pltpu.bitcast(x, U32)
    first = jnp.where(dep > jnp.inf, jnp.uint32(0), xu[:8])
    return pltpu.bitcast(jnp.concatenate([first, xu[8:]], axis=0), BF16)


def _tile(j):
    return slice(j * T, (j + 1) * T)


def _ld(ref, *idx):
    return pltpu.bitcast(ref[idx], BF16)


def _ldb(ref, *idx):
    return pltpu.bitcast(ref.bitcast(U32)[idx], BF16)


def _pk(x):
    return pltpu.bitcast(x, U32)


def _a_ops(a11, a12, a21, a22):
    return [a11 + a22, a21 + a22, a11, a22, a11 + a12, a21 - a11, a12 - a22]


def _b_ops(b11, b12, b21, b22):
    return [b11 + b22, b11, b12 - b22, b21 - b11, b22, b11 + b12, b21 + b22]


def _strassen(prod, col1=None, col2=None):
    m4 = prod(3)
    m2 = prod(1)
    c21 = m2 + m4
    if col1 is not None:
        e11, e21 = col1()
        m4, c21 = m4 + e11, c21 + e21
    m3 = prod(2)
    m5 = prod(4)
    c12 = m3 + m5
    if col2 is not None:
        e12, e22 = col2()
        c12, m3 = c12 + e12, m3 + e22
    m1 = prod(0)
    c11 = prod(6) + (m1 + (m4 - m5))
    c22 = prod(5) + (m1 + (m3 - m2))
    return c11, c12, c21, c22


def _group(rows, cols, pairs):
    xs, ys = dict.fromkeys(x for x, _ in pairs), dict.fromkeys(y for _, y in pairs)
    used = set(xs) | set(ys) | {(x[0], y[1]) for x, y in pairs} | {(y[0], x[1]) for x, y in pairs}
    prods = []
    for n, r in enumerate(rows):
        for i, k in [x for x in xs if x[0] == r]:
            mates = [y for x, y in pairs if x == (i, k)]
            prods.append((((1, i, k),) + tuple((1, i, k2) for _, k2 in mates), ((1, k, 0),),
                          ((1, i, 0), (-1, i, 1))))
            prods.append((((1, i, k),) + tuple((-1, i2, k) for i2, _ in mates), ((1, k, 0), (1, k, 1)),
                          ((1, i, 1),)))
        for i2, k2 in [y for y in ys if y[0] == r]:
            mates = [x for x, y in pairs if y == (i2, k2)]
            prods.append((((1, i2, k2),) + tuple((1, i2, k) for _, k in mates), ((1, k2, 1),),
                          ((1, i2, 1), (-1, i2, 0))))
            prods.append((((1, i2, k2),) + tuple((-1, i, k2) for i, _ in mates), ((1, k2, 0), (1, k2, 1)),
                          ((1, i2, 0),)))
        prods += [(((1, r, k),), ((1, k, h),), ((1, r, h),)) for k in cols if (r, k) not in used for h in (0, 1)]
        for (i, k), (i2, k2) in pairs:
            if r in (i, i2) and i + i2 - r in rows[n + 1:]:
                prods.append((((1, i, k2),), ((1, k2, 0), (-1, k, 0)), ((1, i2, 0), (1, i, 0))))
                prods.append((((1, i2, k), (1, i, k2)), ((1, k, 0), (1, k2, 1)), ((1, i2, 0), (1, i, 1))))
                prods.append((((1, i2, k),), ((1, k, 1), (-1, k2, 1)), ((1, i2, 1), (1, i, 1))))
    return prods


def _all_pairs(xrows, yrows):
    return [((x, a), (y, b)) for a, x in enumerate(xrows) for b, y in enumerate(yrows) if a != b]


_PAIRS65 = [((x[0] + 10, x[1]), (y[0] + 10, y[1])) for x, y in (
    ((0, 1), (1, 0)), ((0, 1), (5, 2)), ((2, 3), (1, 0)), ((2, 3), (3, 1)), ((2, 3), (5, 2)), ((3, 2), (1, 0)),
    ((4, 4), (0, 3)), ((4, 4), (1, 0)), ((4, 4), (3, 1)), ((4, 4), (5, 2)))]
_C_GROUPS = [_group(range(r, r + 8), range(4), _all_pairs(range(r, r + 4), range(r + 4, r + 8))) for r in (0, 8)]
_H_GROUPS = [_group(range(10), range(5), _all_pairs(range(5), range(5, 10))),
             _group(range(10, 16), range(5), _PAIRS65)]
_sum_index = lambda groups: {f: n for n, f in enumerate(
    dict.fromkeys(t[0] for g in groups for t in g if len(t[0]) > 1))}
_C_SUMS, _H_SUMS = _sum_index(_C_GROUPS), _sum_index(_H_GROUPS)


def _form(form, get):
    acc = None
    for sign, i, j in form:
        v = get(i, j)
        acc = v if acc is None else (acc + v if sign > 0 else acc - v)
    return acc


def _gap_items(bufs, gap_scr):
    items = []
    for n, buf in enumerate(bufs):
        acc = []

        def part(r0, buf=buf, acc=acc):
            def fn(dep):
                wu = jnp.concatenate([buf[r:r + 8, :] for r in range(r0, r0 + T, 32)])
                mask = jnp.full((8, T), 0x7FFF0000, U32)
                if dep is not None:
                    mask = jnp.where(dep > jnp.inf, jnp.uint32(0), mask)
                mask = _rows(mask, 32)
                new = [jnp.sum(pltpu.bitcast(v & mask, F32).reshape(4, 8, T), axis=0) for v in (wu << 16, wu)]
                acc[:] = [u + v for u, v in zip(acc, new)] if acc else new
            return fn

        def last(_, n=n, acc=acc):
            bits = []
            for v in acc:
                l1 = jnp.sum(jnp.sum(v, axis=1, keepdims=True), axis=0, keepdims=True)
                bits.append(pltpu.bitcast(jnp.broadcast_to(l1, (8, T)), jnp.int32) >> 8)
            gap_scr[n] = jnp.clip((bits[0] - bits[1] + (1 << 14)) >> 15, -8, 8) << 23

        items += [part(r0) for r0 in range(0, buf.shape[0], T)] + [last]
    return items


class _PairWeights:
    def __init__(self, w_ref, transpose=False, shift=None):
        self.base = {}
        if shift is not None:
            fac = _rows(pltpu.bitcast(0x3F800000 + shift, F32), T)
            self.inv = pltpu.bitcast(0x3F800000 - shift, F32)
        for j in range(w_ref.shape[0] // T):
            wu = w_ref[_tile(j), :]
            if transpose:
                wu = wu.T
            hi = pltpu.bitcast(wu & jnp.uint32(0xFFFF0000), F32)
            self.base[j, 0] = pltpu.bitcast(wu << 16, F32)
            self.base[j, 1] = hi if shift is None else hi * fac
        self.cache = {}

    def __call__(self, form):
        sign = 1
        if form[-1][0] < 0 and form[0][1:] > form[1][1:]:
            sign, form = -1, ((1,) + form[1][1:], (-1,) + form[0][1:])
        if form not in self.cache:
            self.cache[form] = _form(form, lambda k, h: self.base[k, h]).astype(BF16)
        return sign, self.cache[form]


def _run_group(jobs, prods, a_get, w, transposed, finish):
    left = {}
    for _, _, outs in prods:
        for _, i, h in outs:
            left[i, h] = left.get((i, h), 0) + 1
    acc = {}
    for af, bf, outs in prods:
        sign, wt = w(bf)
        m = jobs.mm([wt], [a_get(af)], _dot_nt) if transposed else jobs.mm([a_get(af)], [wt], _dot)
        for s_, i, h in outs:
            if (i, h) not in acc:
                acc[i, h] = (s_ * sign, m)
            else:
                s0, v = acc[i, h]
                acc[i, h] = (s0, v + m if s0 == s_ * sign else v - m) if s0 > 0 or s_ * sign < 0 else (1, m - v)
            left[i, h] -= 1
            if not left[i, h]:
                s0, v = acc.pop((i, h))
                assert s0 > 0
                finish(2 * i + h, v)


class _Jobs:
    def __init__(self, side=()):
        self.res = []
        self.side = list(side)

    def mm(self, lhs, wt, dot):
        acc = None
        for x, w in zip(lhs, wt):
            v = dot(x, w)
            self.res.append(v)
            acc = v if acc is None else v + acc
            rel = 4 * (len(self.res) % 4)
            while self.side and self.side[0][0] <= len(self.res):
                self.side.pop(0)[1](v[8 * rel:8 * rel + 8, :])
                rel = (rel + 2) % 16
        return acc


def _proj_step(h_scr, hs_scr, c_ref, cs_scr, wq_ref, wuk_ref, wuv_ref, q_scr, k_scr, v_scr, scale, shifts, side):
    wk, wvT, wq = [_PairWeights(w, n == 1, shifts[n]) for n, w in enumerate((wuk_ref, wuv_ref, wq_ref))]
    c_get = lambda f: cs_scr[_C_SUMS[f]] if len(f) > 1 else c_ref[_tile(f[0][1]), _tile(f[0][2])]
    h_get = lambda f: hs_scr[_H_SUMS[f]] if len(f) > 1 else h_scr[f[0][1], f[0][2]]

    def put(dst, w, mul=None):
        muls = [mul, _rows(w.inv if mul is None else w.inv * mul, T)]

        def fn(u, v):
            v = (v if muls[u % 2] is None else v * muls[u % 2]).astype(BF16)
            dst[u] = _pk(v.T if mul is not None and u < QT else v)
        return fn

    jobs = _Jobs(side)
    for groups, get, w, transposed, fin in ((_C_GROUPS, c_get, wk, False, put(k_scr, wk)),
                                            (_C_GROUPS, c_get, wvT, True, put(v_scr, wvT)),
                                            (_H_GROUPS, h_get, wq, False, put(q_scr, wq, scale))):
        for prods in groups:
            _run_group(jobs, prods, get, w, transposed, fin)
    assert not jobs.side


def _inner_group(rows, cols, pairs):
    xs, ys = dict.fromkeys(x for x, _ in pairs), dict.fromkeys(y for _, y in pairs)
    used = set(xs) | set(ys) | {(x[0], y[1]) for x, y in pairs} | {(y[0], x[1]) for x, y in pairs}
    prods = []
    for i, j in xs:
        mates = [y for x, y in pairs if x == (i, j)]
        prods.append((((1, i, 0),), ((1, 0, j), (-1, 1, j)), ((1, i, j),) + tuple((1, i2, j) for i2, _ in mates)))
        prods.append((((1, i, 0), (1, i, 1)), ((1, 1, j),), ((1, i, j),) + tuple((-1, i, j2) for _, j2 in mates)))
    for i2, j2 in ys:
        mates = [x for x, y in pairs if y == (i2, j2)]
        prods.append((((1, i2, 0), (1, i2, 1)), ((1, 0, j2),),
                      ((1, i2, j2),) + tuple((-1, i2, j) for _, j in mates)))
        prods.append((((1, i2, 1),), ((1, 0, j2), (-1, 1, j2)),
                      ((-1, i2, j2),) + tuple((-1, i, j2) for i, _ in mates)))
    prods += [(((1, i, h),), ((1, h, j),), ((1, i, j),))
              for i in rows for j in cols if (i, j) not in used for h in (0, 1)]
    for (i, j), (i2, j2) in pairs:
        lo, hi = min(j, j2), max(j, j2)
        prods.append((((1, i2, 0), (-1, i, 0)), ((1, 0, lo), (1, 0, hi)), ((1, i2, j),)))
        prods.append((((1, i, 0), (1, i2, 1)), ((1, 0, j2), (1, 1, j)), ((1, i, j2), (1, i2, j))))
        prods.append((((1, i, 1), (-1, i2, 1)), ((1, 1, lo), (1, 1, hi)), ((1, i, j2),)))
    return prods


def _o_jobs():
    prods = (_inner_group(range(10), range(5), _all_pairs(range(0, 10, 2), range(1, 10, 2)))
             + _inner_group(range(10, 16), range(5), _PAIRS65))
    row = lambda t: max(i for _, i, _ in t[0])
    unit = lambda t: max(2 * i + h for _, i, h in t[0])
    need = lambda t: unit(t) if row(t) == 15 else 2 * row(t) + 1
    return [(need(t), t) for t in sorted(prods, key=need)]


_O_JOBS = _o_jobs()


SB = 4
TS = (-1.125, -0.375, 0.375, 1.125)
_SBP = [(i, j) for i in range(SB) for j in range(i + 1, SB)]
_PF = {f: n for n, f in enumerate([('R', i) for i in range(SB)] + [('C', i) for i in range(SB)]
                                  + [('S', i, j) for i in range(SB) for j in range(SB) if i != j]
                                  + [('A', i, j) for i, j in _SBP])}
_VF = {f: n for n, f in enumerate([('W', i) for i in range(SB)]
                                  + [(q, i, j) for i, j in _SBP for q in ('Q1', 'Q2', 'Q3')])}
_PV = {**{('W', i): ('R', i) for i in range(SB)}, **{('B', i): ('C', i) for i in range(SB)},
       **{('Q1', i, j): ('S', i, j) for i, j in _SBP}, **{('Q2', i, j): ('A', i, j) for i, j in _SBP},
       **{('Q3', i, j): ('S', j, i) for i, j in _SBP}}
_NPF, _NVF = len(_PF), len(_VF)
_DSLOT = (SB - 1) * _NPF
_VSLOT = _DSLOT + SB * (SB + 1) // 2
_FENCE = _VSLOT + (SB - 1) * _NVF // 2


def _job_order(nsb):
    units = [(I, h) for I in range(nsb) for h in range(2)]
    qe, qv = [], []
    for I, h in units:
        qe += [('e', I, h, J, p) for J in range(I) for p in range(SB)]
        qe += [('d', I, h, i, k) for i in range(SB) for k in range(i + 1)]
        for i in range(SB):
            prods = [('W', i), ('B', i)] + [(q, i, j) for j in range(i + 1, SB) for q in ('Q1', 'Q2', 'Q3')]
            qv += [('p', I, h, f, J) for f in prods for J in range(I)]
            qv += [('v', I, h, i, k) for k in range(i + 1)]
    qo = [('o', u, j) for j, (u, _) in enumerate(_O_JOBS)]
    cost = dict(e=8, d=2, p=1, v=2, o=2)
    tot_e, tot_r = sum(cost[j[0]] for j in qe), sum(cost[j[0]] for j in qv + qo)
    order, done = [], {}
    now = [0]
    did_e = did_r = 0

    def emit(q):
        job = q.pop(0)
        order.append(job)
        now[0] += cost[job[0]]
        if job[0] == 'e':
            done['e', job[1], job[2]] = now[0]
        elif job[0] == 'd':
            done[job] = now[0]
        elif job[0] == 'v' and job[4] == job[3]:
            done['u', 2 * (SB * job[1] + job[3]) + job[2]] = now[0]
        return cost[job[0]]

    def v_ready():
        if not qv:
            return False
        key = ('d', qv[0][1], qv[0][2], SB - 1, SB - 1)
        return key in done and done[key] + LAT_A <= now[0]

    def o_ready():
        return bool(qo) and ('u', qo[0][1]) in done and done['u', qo[0][1]] + LAT_B <= now[0]

    def fill(nv, no):
        n = 0
        while nv > 0 or no > 0 or n % 4:
            if no > 0 and n % 2 == 0 and o_ready() and no * ONV >= nv:
                no -= 2
                n += emit(qo)
            elif v_ready() and (nv > 0 or n % 4):
                c = emit(qv)
                nv -= c
                n += c
            elif o_ready() and n % 2 == 0 and (no > 0 or n % 4 or nv > 0) and len(qo) > RES:
                no -= 2
                n += emit(qo)
            else:
                break

    while qe:
        unit = qe[0][1:3]
        ne = 0
        while qe and ne < 8 and (ne == 0 or (qe[0][0] == 'd' and qe[0][1:3] == unit)):
            ne += emit(qe)
        groups = lambda q: sum(cost[j[0]] for j in q) / 8
        old = [j for j in qv if j[1:3] != unit and ('d', j[1], j[2], SB - 1, SB - 1) in done]
        here = [j for j in qe if j[1:3] == unit]
        rest = sum(cost[j[0]] for j in old)
        nv = (rest - (LAT_A if here else 0)) / (groups(here) + 1) if here else min(rest, LAT_A)
        no = 2 * max(len(qo) - RES - OEND, 0) / (groups(qe) + 1)
        fill(int(nv + 0.5), int(no + 0.5))
    while qv or qo:
        if qv and v_ready():
            fill(6, 2)
            if not qv:
                continue
        elif o_ready():
            emit(qo)
        else:
            emit(qv or qo)
    return order


def _softmax_shifts(q_scr, k_scr, m_scr):
    causal = (jax.lax.broadcasted_iota(jnp.int32, (T, T), 0)
              <= jax.lax.broadcasted_iota(jnp.int32, (T, T), 1))

    def unit(u, carry):
        r, hd = u // 2, u % 2

        def block(c, ml):
            s = _dot_nt(_ld(k_scr, 2 * c + hd), _ld(q_scr, u))
            s = jnp.where(jnp.logical_or(causal, c < r), s, -1e9 * LOG2E)
            m = jnp.maximum(ml[0], jnp.max(s, axis=0, keepdims=True))
            return m, ml[1] * jnp.exp2(ml[0] - m) + jnp.sum(jnp.exp2(s - m), axis=0, keepdims=True)

        m, l = jax.lax.fori_loop(0, r + 1, block, (jnp.full((1, T), -jnp.inf, F32), jnp.zeros((1, T), F32)))
        m_scr[u] = jnp.broadcast_to(m + jnp.log(l) * LOG2E, (8, T))
        return carry

    jax.lax.fori_loop(0, q_scr.shape[0], unit, 0)


def _attention_step(q_scr, k_scr, v_scr, m_scr, pf, wo_ref, acc_scr, flag_scr, mid, z):
    causal = (jax.lax.broadcasted_iota(jnp.int32, (T, T), 0)
              <= jax.lax.broadcasted_iota(jnp.int32, (T, T), 1))
    HT = T // 2
    lsum, lrow, acc, fg, dacc, of, lhs = {}, {}, {}, {}, {}, {}, {}
    res = []
    wo, terms = {}, {}
    left = {}
    side = []
    chk = [jnp.zeros((8, T), F32), None]
    for _, t in _O_JOBS:
        for _, i, j in t[2]:
            left[i, j] = left.get((i, j), 0) + 1

    def probs(s, u):
        return jnp.exp2(s.reshape(T // 8, 8, T) - m_scr[u][None]).reshape(T, T)

    def add_l(u, v):
        lsum[u] = v if u not in lsum else lsum[u] + v

    def v_forms(h, J):
        n = 16

        def item(r0, pairs):
            def fn(dep):
                ts = {k: _rows(_after(jnp.full((8, T), TS[k], F32), dep), n) for k in range(SB)}

                def get(k, a):
                    r = (a * HT + r0) // 2
                    return pltpu.bitcast(v_scr[2 * (SB * J + k) + h, r:r + n // 2, :], BF16).astype(F32)

                def put(f, v):
                    f = _VF[f] + J * _NVF
                    pf[h][_VSLOT + f // 2, f % 2 * HT + r0:f % 2 * HT + r0 + n, :] = v.astype(BF16)

                if pairs is None:
                    w = [get(k, 0) + ts[k] * get(k, 1) for k in range(SB)]
                    for k in range(SB):
                        put(('W', k), w[k])
                    for i, j in _SBP:
                        put(('Q2', i, j), w[i] - w[j])
                    return
                b = {(k, a): get(k, a) for k in sorted({k for pr in pairs for k in pr}) for a in range(2)}
                for i, j in pairs:
                    d0, d1 = b[j, 0] - b[i, 0], b[j, 1] - b[i, 1]
                    put(('Q1', i, j), d0 + ts[i] * d1)
                    put(('Q3', i, j), d0 + ts[j] * d1)
            return fn

        return [item(r0, pairs) for r0 in range(0, HT, n)
                for pairs in (None, _SBP[:2], [_SBP[2], _SBP[4]], [_SBP[3], _SBP[5]])]

    def job_e(I, h, J, p):
        if J == 0 and p == 0:
            side.extend(v_forms(h, I - 1))
        ps = []
        for i in range(SB):
            u = 2 * (SB * I + i) + h
            x = jnp.concatenate([k_scr[2 * (SB * J + (t - i) % SB) + h, 8 * g:8 * g + 8, :]
                                 for g in (2 * p, 2 * p + 1) for t in range(SB)], axis=0)
            s = (_dot if u < QT else _dot_nt)(pltpu.bitcast(x, BF16), _ld(q_scr, u))
            res.append(s)
            ps.append(probs(s, u))
        for n, g in enumerate((2 * p, 2 * p + 1)):
            at = lambda i, t: ps[i][16 * (SB * n + t):16 * (SB * n + t) + 16]
            cell = lambda i, k: at(i, (i + k) % SB)

            def put(f, v):
                pf[h][J * _NPF + _PF[f], 16 * g:16 * g + 16, :] = v.astype(BF16)

            for i in range(SB):
                r = ((at(i, 0) + at(i, 1)) + at(i, 2)) + at(i, 3)
                put(('R', i), r)
                add_l(2 * (SB * I + i) + h, r[:8] + r[8:])
                c = None
                for t in range(SB):
                    i2 = (t - i) % SB
                    v = cell(i2, i)
                    if c is None:
                        c = v if i2 == i else -v
                    else:
                        c = c + v if i2 == i else c - v
                put(('C', i), c)
                for j in range(SB):
                    if j != i:
                        put(('S', i, j), cell(i, j))
            for i, j in _SBP:
                put(('A', i, j), cell(i, j) + cell(j, i))

    def job_d(I, h, i, k):
        u = 2 * (SB * I + i) + h
        s = (_dot if u < QT else _dot_nt)(_ld(k_scr, 2 * (SB * I + k) + h), _ld(q_scr, u))
        res.append(s)
        if i == k:
            s = jnp.where(causal, s, -1e9 * LOG2E)
        p = probs(s, u)
        add_l(u, jnp.sum(p.reshape(T // 8, 8, T), axis=0))
        pf[h][_DSLOT + i * (i + 1) // 2 + k] = p.astype(BF16)
        if i == k:
            lrow[u] = jnp.sum(lsum.pop(u), axis=0, keepdims=True)
            if i == SB - 1:
                while side:
                    side.pop(0)(res[-1][0:8, :])
                pf[h][_FENCE + z, 0:16, :] = jnp.zeros((16, T), BF16)
                ls = [lrow[2 * (SB * I + a) + h] for a in range(SB)]
                lo = jnp.minimum(jnp.minimum(ls[0], ls[1]), jnp.minimum(ls[2], ls[3]))
                hi = jnp.maximum(jnp.maximum(ls[0], ls[1]), jnp.maximum(ls[2], ls[3]))
                ok = jnp.logical_and(lo >= L_LO, hi <= L_HI)
                if I:
                    ok = jnp.logical_and(ok, hi <= L_RATIO * lo)
                bad = jnp.where(ok, 0.0, 1.0)
                chk[1] = bad if chk[1] is None else jnp.maximum(chk[1], bad)

    def job_p(I, h, f, J):
        n = J * _NVF + _VF.get(f, 0)
        x = (pltpu.bitcast(v_scr[2 * (SB * J + f[1]) + h, HT // 2:, :], BF16) if f[0] == 'B'
             else pltpu.bitcast(pf[h].bitcast(U32)[_VSLOT + n // 2, n % 2 * HT // 2:(n % 2 + 1) * HT // 2, :], BF16))
        v = _dot(x, _ldb(pf[h], J * _NPF + _PF[_PV[f]]))
        res.append(v)
        acc[f] = v if J == 0 else acc[f] + v
        if J < I - 1:
            return

        def add(key, v, sign=1):
            fg[key] = (v if sign > 0 else -v) if key not in fg else (fg[key] + v if sign > 0 else fg[key] - v)

        if f[0] == 'W':
            add(('F', f[1]), acc.pop(f))
        elif f[0] == 'B':
            add(('G', f[1]), acc.pop(f))
        elif f[0] == 'Q3':
            _, i, j = f
            q1, q2, q3 = (acc.pop((q, i, j)) for q in ('Q1', 'Q2', 'Q3'))
            t = ((q1 + q2) + q3) * (1.0 / (TS[i] - TS[j]))
            add(('G', i), t)
            add(('G', j), t)
            add(('F', i), q1)
            add(('F', j), q3, -1)

    def job_v(I, h, i, k):
        u = 2 * (SB * I + i) + h
        v = _dot(_ld(v_scr, 2 * (SB * I + k) + h), _ldb(pf[h], _DSLOT + i * (i + 1) // 2 + k))
        res.append(v)
        dacc[u] = v if u not in dacc else dacc[u] + v
        if k == i:
            o = dacc.pop(u)
            if I:
                f, g = fg.pop(('F', i)), fg.pop(('G', i))
                o = o + jnp.concatenate([f - TS[i] * g, g], axis=0)
            o = o * (1.0 / lrow[u])
            of[u] = o
            chk[0] = chk[0] + jnp.sum(o.reshape(T // 8, 8, T), axis=0)

    def job_o(_, n):
        af, bf, outs = _O_JOBS[n][1]
        if af not in lhs:
            v = _form(af, lambda i, h: of[2 * i + h])
            lhs[af] = _tie(v.astype(BF16).T, v[0:8, :])
        if bf not in wo:
            wo[bf] = (wo_ref[_tile(bf[0][1]), _tile(bf[0][2])] if len(bf) == 1 else
                      _form(bf, lambda h, j: wo_ref[_tile(h), _tile(j)].astype(F32)).astype(BF16))
        v = _dot(lhs[af], wo[bf])
        res.append(v)
        for sign, i, j in outs:
            terms.setdefault((i, j), []).append((sign, v))
            if len(terms[i, j]) == left[i, j]:
                tot = acc_scr[_tile(i), _tile(j)]
                for sg, m in terms.pop((i, j)):
                    tot = tot + m if sg > 0 else tot - m
                acc_scr[_tile(i), _tile(j)] = tot

    fns = dict(e=job_e, d=job_d, p=job_p, v=job_v, o=job_o)
    for n, job in enumerate(_job_order(q_scr.shape[0] // (2 * SB))):
        if n == MID:
            mid()
        fns[job[0]](*job[1:])
        if side and n % SIDE == 0:
            side.pop(0)(res[-1 - SLAG][8 * (n % 4):8 * (n % 4) + 8, :])
    fine = jnp.abs(chk[0]) < jnp.inf
    flag_scr[...] = jnp.maximum(flag_scr[...], jnp.where(fine, chk[1], 1.0))


def _kernel(x_hbm, c_hbm, wq_hbm, wuk_hbm, wuv_hbm, wo_hbm, w1_hbm, w2_hbm, w3_hbm, w4_hbm,
            cond_hbm, wmod_hbm, out_hbm,
            x_ref, c_ref, cond_ref, wma_ref, wmb_ref, w1_ref, w2_ref, w3_ref, w4_ref,
            wq_buf, wk_buf, wv_buf, wo_buf, out_buf, sem, wsem, osem,
            mod_scr, h_scr, cs_scr, hs_scr, w_scr, q_scr, k_scr, v_scr, acc_scr, xn_scr, xh_scr, a1_scr, t_scr,
            ws12, ws3, ws4, pq_buf, pk_buf, pv_buf, gap_scr, st_in, m_scr, pf_scr, vf_scr, flag_scr, redo):
    S, M = x_hbm.shape
    D = wq_hbm.shape[2]
    nattn = wo_hbm.shape[0]
    Fd = w4_hbm.shape[0]
    scale = float(D) ** -0.5 * LOG2E
    nb, nrb = S // T, S // RB
    km, kc = M // T, c_hbm.shape[1] // T
    NX = 4
    XR = S // NX
    CB = XR // T

    work, probe = (wk_buf, wv_buf, wq_buf), (pk_buf, pv_buf, pq_buf)

    def pcopies(g, bufs=work, s0=0):
        return [pltpu.make_async_copy(src.bitcast(U32).at[:, g, :], dst, wsem.at[s0 + j])
                for j, (src, dst) in enumerate(zip((wuk_hbm, wuv_hbm, wq_hbm), bufs))]

    def ocopy(g):
        return pltpu.make_async_copy(wo_hbm.at[g], wo_buf, wsem.at[3])

    def chunk_copy(src, dst, i, s0):
        rows = slice(i * XR, (i + 1) * XR)
        return pltpu.make_async_copy(src.at[rows, :], dst.at[rows, :], sem.at[s0 + i])

    cp_cond = pltpu.make_async_copy(cond_hbm, cond_ref, sem.at[0])
    cp_wma = pltpu.make_async_copy(wmod_hbm.at[:, 0:2 * M], wma_ref, sem.at[1])
    cp_late = [pltpu.make_async_copy(src, dst, sem.at[2 + j]) for j, (src, dst) in enumerate((
        (wmod_hbm.at[:, 2 * M:6 * M], wmb_ref), (w1_hbm, w1_ref), (w2_hbm, w2_ref),
        (w3_hbm, w3_ref), (w4_hbm, w4_ref)))]
    cp_x = [chunk_copy(x_hbm, x_ref, i, 7) for i in range(NX)]
    cp_c = [chunk_copy(c_hbm, c_ref, i, 7 + NX) for i in range(NX)]

    def silu_cond():
        cf = cond_ref[...].astype(F32)
        return jnp.broadcast_to((cf * jax.nn.sigmoid(cf)).astype(BF16), (8, M))

    cp_wk, cp_wv, cp_wq = pcopies(0)
    named = dict(k=cp_wk, v=cp_wv, q=cp_wq, o=ocopy(0), n=cp_cond, m=cp_wma)
    named.update(zip('abcd', cp_c))
    named.update(zip('wxyz', cp_x))
    started, arrived, did = set(), set(), set()

    def zero(r, carry):
        acc_scr[pl.ds(pl.multiple_of(r * T, T), T), :] = jnp.zeros((T, M), F32)
        return carry

    def x_rows(rows, dep):
        xf = x_ref[rows, :].astype(F32)
        if dep is None:
            return xf
        return jnp.concatenate([_after(xf[:, :T], _rows(dep, xf.shape[0])), xf[:, T:]], axis=1)

    def n_item(r, i):
        def fn(dep):
            rows = slice(r * T + i * LP, r * T + (i + 1) * LP)
            xn_scr[rows, :] = _ln(x_rows(rows, dep))
        return fn

    def h_item(r, i, normed):
        def fn(dep):
            rows = slice(i * LP, (i + 1) * LP)
            grows = slice(r * T + i * LP, r * T + (i + 1) * LP)
            sa = mod_scr[:, 0:M]
            if normed and dep is not None:
                sa = jnp.concatenate([_after(sa[:, _tile(j)], dep) for j in range(km)], axis=1)
            hf = ((xn_scr[grows, :] if normed else _ln(x_rows(grows, dep))) * _rows(mod_scr[:, M:2 * M], LP)
                  + _rows(sa, LP))
            for j in range(km):
                h_scr[r, j, rows, :] = hf[:, _tile(j)].astype(BF16)
            for f, n in _H_SUMS.items():
                if all(t[1] == r for t in f):
                    hs_scr[n, rows, :] = _form(f, lambda _, k: hf[:, _tile(k)]).astype(BF16)
            did.add(('h', r, i))
        return fn

    def release(jobs, span, items):
        if span and items:
            jobs.side += [(len(jobs.res) + 1 + i * span // len(items), fn) for i, fn in enumerate(items)]
            jobs.side.sort(key=lambda e: e[0])
        else:
            for fn in items:
                fn(None)

    def sum_items(n, group, index, dst, get, skip_rows):
        forms = [f for f in dict.fromkeys(t[0] for t in group)
                 if len(f) > 1 and not (skip_rows and len({t[1] for t in f}) == 1)]

        def item(f, rows):
            def fn(dep):
                def term(r, k):
                    v = get(r, k, rows).astype(F32)
                    return v if dep is None or (r, k) != f[0][1:] else _after(v, _rows(dep, v.shape[0]))
                dst[index[f], rows, :] = _form(f, term).astype(BF16)
            return fn

        return [item(f, slice(i, i + n)) for i in range(0, T, n) for f in forms]

    h_sums = lambda n, gi: sum_items(n, _H_GROUPS[gi], _H_SUMS, hs_scr,
                                     lambda r_, k, rows: h_scr[r_, k, rows, :], True)

    def stash(key, buf, j0, transpose=False):
        n = buf.shape[0] // T
        if key not in did:
            assert key in arrived
            did.add(key)
            w = _PairWeights(buf, transpose)
            for j in range(n):
                for hd in range(2):
                    w_scr[hd, j0 + j] = _pk(w(((1, j, hd),))[1])
        return lambda hd: [_ld(w_scr, hd, j0 + j) for j in range(n)]

    def kv_tile(jobs, r):
        wk, wvT = stash('k', wk_buf, 0), stash('v', wv_buf, kc, True)
        ct = [c_ref[_tile(r), _tile(j)] for j in range(kc)]
        for hd in range(2):
            k_scr[2 * r + hd] = _pk(jobs.mm(ct, wk(hd), _dot).astype(BF16))
        for hd in range(2):
            v_scr[2 * r + hd] = _pk(jobs.mm(wvT(hd), ct, _dot_nt).astype(BF16))

    def q_tile(jobs, r):
        wq = stash('q', wq_buf, 2 * kc)
        ht = [h_scr[r, j] for j in range(km)]
        for hd in range(2):
            v = (jobs.mm(ht, wq(hd), _dot) * scale).astype(BF16)
            q_scr[2 * r + hd] = _pk(v.T if 2 * r + hd < QT else v)

    for blk in PROLOGUE.split(';'):
        waits, starts, acts = blk.split('|')
        for ch in waits.strip():
            assert ch in started and ch not in arrived
            arrived.add(ch)
            named[ch].wait()
        for ch in starts.strip():
            assert ch not in started
            started.add(ch)
            named[ch].start()
        jobs = _Jobs()
        for act in acts.split():
            if act == 'Z':
                jax.lax.fori_loop(0, nb, zero, 0)
                acc_scr[S:, :] = jnp.zeros((acc_scr.shape[0] - S, M), F32)
                x_ref[S:, :] = jnp.zeros((x_ref.shape[0] - S, M), BF16)
                m_scr[...] = jnp.zeros(m_scr.shape, F32)
                flag_scr[...] = jnp.zeros(flag_scr.shape, F32)
                redo[0] = 0
            elif act == 'L':
                did.add('L')
                for cp in cp_late:
                    cp.start()
            elif act == 'M':
                assert arrived >= set('nm')
                mod = _dot(silu_cond(), wma_ref[...])
                mod_scr[:, 0:M] = mod[:, 0:M]
                mod_scr[:, M:2 * M] = 1.0 + mod[:, M:2 * M]
                did.add('M')
            else:
                act, _, span = act.partition('@')
                span = int(span or 0)
                items = []
                for r in [int(ch, 16) for ch in act[1:]]:
                    did.add((act[0], r))
                    if act[0] == 'K':
                        assert 'abcd'[r // CB] in arrived
                        kv_tile(jobs, r)
                    elif act[0] == 'H':
                        assert 'wxyz'[r // CB] in arrived and 'M' in did
                        items += [h_item(r, i, ('N', r) in did) for i in range(T // LP)]
                    elif act[0] == 'N':
                        assert 'wxyz'[r // CB] in arrived
                        items += [n_item(r, i) for i in range(T // LP)]
                    elif act[0] == 'Q':
                        assert all(('h', r, i) in did for i in range(T // LP))
                        q_tile(jobs, r)
                    elif act[0] == 'C':
                        assert all('abcd'[t[1] // CB] in arrived for p_ in _C_GROUPS[r] for t in p_[0])
                        items += sum_items(
                            32, _C_GROUPS[r], _C_SUMS, cs_scr,
                            lambda r_, k, rows: c_ref[r_ * T + rows.start:r_ * T + rows.stop, _tile(k)], False)
                    else:
                        assert act[0] == 'S' and all(('h', t[1], T // LP - 1) in did for p_ in _H_GROUPS[r] for t in p_[0])
                        items += h_sums(32 if span else 16, r)
                release(jobs, span, items)
        assert not jobs.side
    assert arrived == set(named) and all((k_, r) in did for k_ in 'KHQ' for r in range(nb))
    assert all((k_, r) in did for k_ in 'CS' for r in range(2)) and 'L' in did

    FH = ws3.shape[0] * T
    assert nattn - 1 >= FH // 64

    slices = ((w1_hbm, 32, 2 * T, 0), (w2_hbm, 32, 2 * T, 64), (w4_hbm, 64, FH, 128), (w3_hbm, T, FH, 256))
    slice_of = lambda g, n, half: jnp.minimum(g, half // n - 1)

    def prep_in(g):
        return [pltpu.make_async_copy(
            w.at[pl.ds(pl.multiple_of(slice_of(g, n, half) * n + x * half, n), n), 0:4 * T],
            st_in.at[r0 + x * n:r0 + (x + 1) * n, :], wsem.at[7]) for w, n, half, r0 in slices for x in range(2)]

    def mixer_prep(g):
        def blocks(r0, n, half, c0, c1, dep):
            get = lambda x, c: st_in[r0 + x * half:r0 + x * half + n, _tile(c)].astype(F32)
            return [_after(get(0, c0), _rows(dep, n)), get(0, c1), get(1, c0), _after(get(1, c1), _rows(dep, n))]

        def rows_item(dst, per, half, r0, c, o, n=16):
            def fn(dep):
                rows = pl.ds(pl.multiple_of(slice_of(g, per, half) * (per // 2), per // 2) + o // 2, n // 2)
                for i, v in enumerate(_b_ops(*blocks(r0 + o, n, per, c, c + 2, dep))):
                    dst[i, c, rows, :] = _pk(v.astype(BF16))
            return fn

        def w3_item(k, i):
            def fn(dep):
                b11, b21, b12, b22 = blocks(slices[3][3], T, T, k, k + 2, dep)
                ws3[slice_of(g, T, FH), i, k] = _pk(_b_ops(b11, b12, b21, b22)[i].astype(BF16).T)
            return fn

        return ([rows_item(dst, *sl[1:], c, o) for dst, sl in zip((ws12.at[0], ws12.at[1], ws4), slices)
                 for c in range(2) for o in range(0, sl[1], 16)]
                + [w3_item(k, i) for k in range(2) for i in range(7)])

    def attn_body(g, exact):
        gw = jnp.maximum(g, 0)
        copies = pcopies(jnp.minimum(g + 1, nattn - 1)) + pcopies(jnp.minimum(g + 2, nattn - 1), probe, 4)

        def mid():
            for cp in copies + prep_in(gw):
                cp.start()

        @pl.when(g >= 0)
        def _():
            pl.when(exact > 0)(lambda: _softmax_shifts(q_scr, k_scr, m_scr))
            bufs = (q_scr, k_scr, v_scr, m_scr, (pf_scr, vf_scr), wo_buf, acc_scr, flag_scr)
            _attention_step(*bufs, mid, g >> 16)

        pl.when(g < 0)(mid)
        for cp in copies:
            cp.wait()
        pltpu.make_async_copy(st_in, st_in, wsem.at[7]).wait()

        @pl.when(g == -exact)
        def _():
            for fn in _gap_items(work, gap_scr):
                fn(None)

        @pl.when(g + 1 < nattn)
        def _():
            ocopy(g + 1).start()
            side = mixer_prep(gw) + _gap_items(probe, gap_scr)
            side = [(SD0 + i * SDS + (SDJ if i >= SDN else 0), fn) for i, fn in enumerate(side)]
            bufs = (h_scr, hs_scr, c_ref, cs_scr, wq_buf, wk_buf, wv_buf, q_scr, k_scr, v_scr)
            _proj_step(*bufs, scale, gap_scr, side)
            ocopy(g + 1).wait()

        return exact

    def attn_pass(exact, carry):
        @pl.when(jnp.logical_or(exact == 0, redo[0] > 0))
        def _():
            @pl.when(exact > 0)
            def _():
                jax.lax.fori_loop(0, nb, zero, 0)


            jax.lax.fori_loop(-exact, nattn, attn_body, exact)

        @pl.when(exact == 0)
        def _():
            redo[0] = (jnp.max(flag_scr[...]) > 0).astype(jnp.int32)

        return carry

    jax.lax.fori_loop(0, 2, attn_pass, 0)

    for cp in cp_late:
        cp.wait()
    mod = _dot(silu_cond(), wmb_ref[...])
    mod_scr[:, 2 * M:4 * M] = mod[:, 0:2 * M]
    mod_scr[:, 4 * M:5 * M] = 1.0 + mod[:, 2 * M:3 * M]
    mod_scr[:, 5 * M:6 * M] = mod[:, 3 * M:4 * M]
    ftiles = [(f, min(f + T, Fd)) for f in range(0, Fd, T)]
    OFF = x_ref.shape[0] - S
    CAR = t_scr.shape[0] - RB

    def p1(r0, l0, n, dep=None):
        ga = mod_scr[:, 2 * M:3 * M]
        if dep is not None:
            ga = jnp.concatenate([_after(ga[:, 0:T], dep), ga[:, T:]], axis=1)
        rows = pl.ds(r0, n)
        x1 = x_ref[rows, :].astype(F32) + _rows(ga, n) * acc_scr[rows, :]
        xh_scr[0, l0:l0 + n, :] = x1
        hb = _ln(x1) * _rows(mod_scr[:, 4 * M:5 * M], n) + _rows(mod_scr[:, 3 * M:4 * M], n)
        xh_scr[1, l0:l0 + n, :] = hb
        return _ln(hb)

    HT = T // 2

    def p1_store(r0, c, dep=None):
        v = p1(r0 + c * PC, OFF + c * PC, PC, dep)
        a1_scr[c * PC:(c + 1) * PC, :] = v
        return jnp.max(v[:, M - T:].reshape(PC // 8, 8, T), axis=0)

    t_scr[RB:RB + CAR - OFF, :] = jnp.zeros((CAR - OFF, M), F32)
    t_scr[RB + CAR - OFF:RB + CAR, :] = _gelu(_dot(p1(0, 0, OFF).astype(BF16), w1_ref[...]))
    for c in range(RB // PC):
        p1_store(OFF, c)

    def out_copy(i):
        rows = pl.ds(i * T if isinstance(i, int) else pl.multiple_of(i * T, T), T)
        return pltpu.make_async_copy(out_buf.at[rows, :], out_hbm.at[rows, :], osem.at[i])

    def b_body(r, carry):
        gb = _rows(mod_scr[:, 5 * M:6 * M], T)
        r0 = pl.multiple_of(r * RB, RB)
        n0 = pl.multiple_of(jnp.minimum(r0 + RB, S - RB) + OFF, OFF)
        nh = RB // T
        now = [0]
        due = []
        pace = []

        def p1_item(c):
            return lambda dep: due.append((now[0] + PD, p1_store(n0, c, dep)))

        pace += [(P0 + i * PSTEP, p1_item(i)) for i in range(RB // PC)]
        wt = lambda ref, f0, f1, n: ref[f0:f1, _tile(n)]

        def mm(lhs, wts, dot=_dot):
            acc = None
            for x, w in zip(lhs, wts):
                if due and due[0][0] <= now[0]:
                    w = _tie(w, due.pop(0)[1])
                v = dot(x, w)
                now[0] += x.shape[0] // HT
                acc = v if acc is None else v + acc
                if pace and pace[0][0] <= now[0]:
                    pace.pop(0)[1](v[0:8, :])
            return acc

        def split_ops(lo, hi):
            return [v.astype(BF16) for v in _a_ops(lo[:HT], hi[:HT], lo[HT:], hi[HT:])]

        def two_tiles(aops, wsel, rest):
            def col(w):
                v = mm(rest[0], w, rest[3])
                return v[:HT], v[HT:]

            c11, c12, c21, c22 = _strassen(
                lambda i: mm([a[i] for a in aops], [wsel(i, k) for k in range(len(aops))]),
                lambda: col(rest[1]), lambda: col(rest[2]))
            return jnp.concatenate([c11, c21], axis=0), jnp.concatenate([c12, c22], axis=0)

        def square(full, aops, w_ref, ws_ref):
            out = {}
            for n in range(2):
                out[n], out[n + 2] = two_tiles(
                    aops, lambda i, k: _ld(ws_ref, i, n, slice(k * HT, (k + 1) * HT)),
                    (full[4:], [wt(w_ref, 4 * T, M, n)], [wt(w_ref, 4 * T, M, n + 2)], _dot))
            out[4] = mm(full, [wt(w_ref, j * T, (j + 1) * T, 4) for j in range(km)])
            return out

        t_scr[0:CAR, :] = t_scr[RB:RB + CAR, :]
        for hf in range(nh):
            a1 = [a1_scr[_tile(hf), _tile(j)] for j in range(km)]
            full = [v.astype(BF16) for v in a1]
            aops = [split_ops(a1[k], a1[2 + k]) for k in range(2)]
            for n, v in square(full, aops, w1_ref, ws12.at[0]).items():
                t = _gelu(v)
                if hf == nh - 1:
                    t = jnp.concatenate([t[:T - OFF], jnp.where(r < nrb - 1, t[T - OFF:], 0.0)], axis=0)
                t_scr[CAR + hf * T:CAR + (hf + 1) * T, _tile(n)] = t
        cq = M // 4
        shifts = (-1, 1, -2, 2)
        lane = jax.lax.broadcasted_iota(jnp.int32, (T, T), 1)
        y1, z, a3 = [], [], []
        for hf in range(nh):
            base = CAR - OFF + hf * T
            sh = []
            for j in range(km):
                g_lo, g_hi = (j * T) // cq, ((j + 1) * T - 1) // cq
                assert g_hi - g_lo <= 1
                v = t_scr[base + shifts[g_lo]:base + shifts[g_lo] + T, _tile(j)]
                if g_hi != g_lo:
                    v2 = t_scr[base + shifts[g_hi]:base + shifts[g_hi] + T, _tile(j)]
                    v = jnp.where(lane < g_hi * cq - j * T, v, v2)
                sh.append(v)
            hs = square([v.astype(BF16) for v in sh], [split_ops(sh[k], sh[2 + k]) for k in range(2)],
                        w2_ref, ws12.at[1])
            hs = jnp.concatenate([hs[n] for n in range(km)], axis=1)
            y1.append(hs + xh_scr[1, _tile(hf), :])
            z.append(xh_scr[0, _tile(hf), :] + gb * y1[hf])
            a3.append({})

            def ln_item(hf, c):
                def item(dep):
                    n = HT // NLN
                    for d in (0, HT):
                        v = y1[hf][d + c * n:d + (c + 1) * n]
                        if dep is not None:
                            v = jnp.concatenate([_after(v[:, :T], _rows(dep, n)), v[:, T:]], axis=1)
                        a3[hf][d + c * n] = _ln(v)
                return item

            ln_item(hf, 0)(None)
            pace += [(now[0] + LN0 + (c - 1) * LNS * (1 + hf), ln_item(hf, c)) for c in range(1, NLN)]
            pace.sort(key=lambda e: e[0])
        xh_scr[:, 0:OFF, :] = xh_scr[:, RB:RB + OFF, :]
        nf = FH // T
        h3, h3ops = [], []
        for hf in range(nh):
            assert len(a3[hf]) == 2 * NLN
            af = jnp.concatenate([a3[hf][key] for key in sorted(a3[hf])], axis=0)
            full = [af[:, _tile(j)].astype(BF16) for j in range(km)]
            aops = [split_ops(af[:, _tile(k)], af[:, _tile(2 + k)]) for k in range(2)]
            row, ops = {}, []
            narrow = None
            for n in range(nf):
                lo, hi = two_tiles(aops, lambda i, k: _ld(ws3, n, i, k),
                                   (full[4:], [wt(w3_ref, *ftiles[n], 4)],
                                    [wt(w3_ref, *ftiles[nf + n], 4)], _dot_nt))
                lo, hi = _gelu(lo), _gelu(hi)
                row[n], row[nf + n] = lo.astype(BF16), hi.astype(BF16)
                ops.append(split_ops(lo, hi))
                if n < km:
                    v = mm([wt(w3_ref, *ftiles[-1], n)], [full[n]], _dot_nt)
                    narrow = v if narrow is None else v + narrow
            row[2 * nf] = _gelu(mm(full, [wt(w3_ref, *ftiles[2 * nf], j) for j in range(km)],
                                   _dot_nt)).astype(BF16)
            fw = Fd - ftiles[-1][0]
            gT = jnp.concatenate([_gelu(narrow), jnp.zeros((T - fw, T), F32)], axis=0)
            row[2 * nf + 1] = _tie(gT.astype(BF16).T, gT[0:8, :])[:, :fw]
            h3.append([row[i] for i in range(len(ftiles))])
            h3ops.append(ops)
        for hf in range(nh):
            rows = pl.ds(pl.multiple_of(r0 + hf * T, T), T)

            def finish(n, v):
                out_buf[rows, _tile(n)] = (z[hf][:, _tile(n)] + gb[:, _tile(n)] * v).astype(out_buf.dtype)

            w4t = lambda n, f_: [wt(w4_ref, f0, f1, n) for f0, f1 in f_]
            finish(4, mm(h3[hf], w4t(4, ftiles)))
            for n in range(2):
                lo, hi = two_tiles(h3ops[hf], lambda i, k: _ld(ws4, i, n, slice(k * HT, (k + 1) * HT)),
                                   (h3[hf][2 * nf:], w4t(n, ftiles[2 * nf:]), w4t(n + 2, ftiles[2 * nf:]), _dot))
                finish(n, lo)
                finish(n + 2, hi)
            out_copy(r * nh + hf).start()
        assert not pace
        return carry

    jax.lax.fori_loop(0, nrb, b_body, 0)
    for i in range(nb):
        out_copy(i).wait()


@jax.jit
def pallas_adaLN_cond__compressed_kv_cla__mixer_s_mlp__prompt_kernel(
    A_x: jax.Array,
    A_c_kv: jax.Array,
    A_w_q: jax.Array,
    A_w_uk: jax.Array,
    A_w_uv: jax.Array,
    A_w_o: jax.Array,
    B_x: jax.Array,
    B_w1: jax.Array,
    B_w2: jax.Array,
    B_w3: jax.Array,
    B_w4: jax.Array,
    c: jax.Array,
    w_mod: jax.Array,
):
    _, S, M = A_x.shape
    Dc = A_c_kv.shape[2]
    H, D = A_w_q.shape[1], A_w_q.shape[2]
    Fd = B_w3.shape[1]
    assert D == T and A_c_kv.shape[1] == S and Dc == 4 * T and M == 5 * T and 13 * T < Fd < 14 * T and S == 16 * T
    vmem = pltpu.VMEM
    packed = lambda *lead: vmem(lead + (T // 2, T), U32)
    out = pl.pallas_call(
        _kernel,
        in_specs=[pl.BlockSpec(memory_space=pltpu.HBM)] * 12,
        out_specs=pl.BlockSpec(memory_space=pltpu.HBM),
        out_shape=jax.ShapeDtypeStruct((S, M), A_x.dtype),
        scratch_shapes=[
            vmem((S + 16, M), BF16),
            vmem((S, Dc), BF16),
            vmem((1, M), BF16),
            vmem((M, 2 * M), BF16),
            vmem((M, 4 * M), BF16),
            vmem((M, M), BF16),
            vmem((M, M), BF16),
            vmem((Fd, M), BF16),
            vmem((Fd, M), BF16),
            vmem((M, D), U32),
            vmem((Dc, D), U32),
            vmem((Dc, D), U32),
            vmem((2 * D, M), BF16),
            vmem((S, M), A_x.dtype),
            pltpu.SemaphoreType.DMA((15,)),
            pltpu.SemaphoreType.DMA((8,)),
            pltpu.SemaphoreType.DMA((S // T,)),
            vmem((8, 6 * M), F32),
            vmem((S // T, M // T, T, T), BF16),
            vmem((len(_C_SUMS), T, T), BF16),
            vmem((len(_H_SUMS), T, T), BF16),
            packed(2, M // T + 2 * (Dc // T)),
            packed(2 * S // T),
            packed(2 * S // T),
            packed(2 * S // T),
            vmem((S + 16, M), F32),
            vmem((S, M), F32),
            vmem((2, RB + 16, M), F32),
            vmem((RB, M), F32),
            vmem((RB + 32, M), F32),
            vmem((2, 7, 2, T, T), U32),
            packed(6, 7, 2),
            vmem((7, 2, 3 * T, T), U32),
            vmem((M, D), U32),
            vmem((Dc, D), U32),
            vmem((Dc, D), U32),
            vmem((3, 8, T), jnp.int32),
            vmem((4 * T, 4 * T), BF16),
            vmem((2 * S // T, 8, T), F32),
            vmem((_FENCE + 1, T, T), BF16),
            vmem((_FENCE + 1, T, T), BF16),
            vmem((8, T), F32),
            pltpu.SMEM((1,), jnp.int32),
        ],
        compiler_params=pltpu.CompilerParams(
            vmem_limit_bytes=100 * 1024 * 1024,
            disable_bounds_checks=True,
        ),
    )(
        A_x.reshape(S, M), A_c_kv.reshape(S, Dc),
        A_w_q, A_w_uk, A_w_uv,
        A_w_o.reshape(H // 2, 2 * D, M),
        B_w1, B_w2, B_w3.T, B_w4, c, w_mod,
    )
    return out.reshape(1, S, M)
```

```python
import math

import jax
import jax.numpy as jnp
import jax.experimental.pallas as pl
import jax.experimental.pallas.tpu as pltpu

F32 = jnp.float32
BF16 = jnp.bfloat16
U32 = jnp.uint32
NT = (((1,), (1,)), ((), ()))
T = 128
EPS = 1e-5
LOG2E = math.log2(math.e)

GRP = 4
LEAD = 10
PROW = 3
RES = 32
LAT_A = 16
LAT_B = 20
ALEAD = 32
SD0, SDS, SDN, SDJ = 158, 2, 20, 30
QT = 0
ONV, OEND = 0.5, 24
SIDE, SLAG = 1, 4
L_LO, L_HI, L_RATIO = 2.0 ** -24, 2.0 ** 24, 4.0
RB = 256
PC = 32
P0, PSTEP, PD = 440, 30, 52
NLN, LN0, LNS = 4, 4, 5
LP = 16
PROLOGUE = ('|kva|Z; |b|; kva|wc|K0123; bw|xdn|C0@56 N0123@52 K4567; cx|mq|N4567@52 K89ab; '
            'd|y|C1@56 Kcdef; nmq|zo|M H01 H234567@30 Q0123; y||H89ab@30 Q4567; '
            'zo||L Hcdef@30 Q89ab S01 Qcdef')


def _dot(a, b):
    return jnp.dot(a, b, preferred_element_type=F32)


def _dot_nt(a, b):
    return jax.lax.dot_general(a, b, NT, preferred_element_type=F32)


def _ln(x):
    m = jnp.mean(x, axis=-1, keepdims=True)
    xc = x - m
    v = jnp.mean(xc * xc, axis=-1, keepdims=True)
    return xc * jnp.exp2(jnp.log(v + EPS) * (-0.5 * LOG2E))


def _rows(v, n):
    return jnp.broadcast_to(v[None], (n // 8, 8, v.shape[1])).reshape(n, v.shape[1])


def _gelu(x):
    c0 = math.sqrt(2.0 / math.pi)
    return 0.5 * x * (1.0 + jnp.tanh(c0 * (x + 0.044715 * (x * x * x))))


def _after(x, dep):
    return jnp.where(dep > jnp.inf, dep, x)


def _tie(x, dep):
    xu = pltpu.bitcast(x, U32)
    first = jnp.where(dep > jnp.inf, jnp.uint32(0), xu[:8])
    return pltpu.bitcast(jnp.concatenate([first, xu[8:]], axis=0), BF16)


def _tile(j):
    return slice(j * T, (j + 1) * T)


def _ld(ref, *idx):
    return pltpu.bitcast(ref.bitcast(U32)[idx], BF16)


def _a_ops(a11, a12, a21, a22):
    return [a11 + a22, a21 + a22, a11, a22, a11 + a12, a21 - a11, a12 - a22]


def _b_ops(b11, b12, b21, b22):
    return [b11 + b22, b11, b12 - b22, b21 - b11, b22, b11 + b12, b21 + b22]


def _strassen(prod, col1=None, col2=None):
    m4 = prod(3)
    m2 = prod(1)
    c21 = m2 + m4
    if col1 is not None:
        e11, e21 = col1()
        m4, c21 = m4 + e11, c21 + e21
    m3 = prod(2)
    m5 = prod(4)
    c12 = m3 + m5
    if col2 is not None:
        e12, e22 = col2()
        c12, m3 = c12 + e12, m3 + e22
    m1 = prod(0)
    c11 = prod(6) + (m1 + (m4 - m5))
    c22 = prod(5) + (m1 + (m3 - m2))
    return c11, c12, c21, c22


def _group(rows, cols, pairs):
    xs, ys = dict.fromkeys(x for x, _ in pairs), dict.fromkeys(y for _, y in pairs)
    used = set(xs) | set(ys) | {(x[0], y[1]) for x, y in pairs} | {(y[0], x[1]) for x, y in pairs}
    prods = []
    for n, r in enumerate(rows):
        for i, k in [x for x in xs if x[0] == r]:
            mates = [y for x, y in pairs if x == (i, k)]
            prods.append((((1, i, k),) + tuple((1, i, k2) for _, k2 in mates), ((1, k, 0),),
                          ((1, i, 0), (-1, i, 1))))
            prods.append((((1, i, k),) + tuple((-1, i2, k) for i2, _ in mates), ((1, k, 0), (1, k, 1)),
                          ((1, i, 1),)))
        for i2, k2 in [y for y in ys if y[0] == r]:
            mates = [x for x, y in pairs if y == (i2, k2)]
            prods.append((((1, i2, k2),) + tuple((1, i2, k) for _, k in mates), ((1, k2, 1),),
                          ((1, i2, 1), (-1, i2, 0))))
            prods.append((((1, i2, k2),) + tuple((-1, i, k2) for i, _ in mates), ((1, k2, 0), (1, k2, 1)),
                          ((1, i2, 0),)))
        prods += [(((1, r, k),), ((1, k, h),), ((1, r, h),)) for k in cols if (r, k) not in used for h in (0, 1)]
        for (i, k), (i2, k2) in pairs:
            if r in (i, i2) and i + i2 - r in rows[n + 1:]:
                prods.append((((1, i, k2),), ((1, k2, 0), (-1, k, 0)), ((1, i2, 0), (1, i, 0))))
                prods.append((((1, i2, k), (1, i, k2)), ((1, k, 0), (1, k2, 1)), ((1, i2, 0), (1, i, 1))))
                prods.append((((1, i2, k),), ((1, k, 1), (-1, k2, 1)), ((1, i2, 1), (1, i, 1))))
    return prods


def _all_pairs(xrows, yrows):
    return [((x, a), (y, b)) for a, x in enumerate(xrows) for b, y in enumerate(yrows) if a != b]


_PAIRS65 = [((x[0] + 10, x[1]), (y[0] + 10, y[1])) for x, y in (
    ((0, 1), (1, 0)), ((0, 1), (5, 2)), ((2, 3), (1, 0)), ((2, 3), (3, 1)), ((2, 3), (5, 2)), ((3, 2), (1, 0)),
    ((4, 4), (0, 3)), ((4, 4), (1, 0)), ((4, 4), (3, 1)), ((4, 4), (5, 2)))]
_C_GROUPS = [_group(range(r, r + 8), range(4), _all_pairs(range(r, r + 4), range(r + 4, r + 8))) for r in (0, 8)]
_H_GROUPS = [_group(range(10), range(5), _all_pairs(range(5), range(5, 10))),
             _group(range(10, 16), range(5), _PAIRS65)]
_sum_index = lambda groups: {f: n for n, f in enumerate(
    dict.fromkeys(t[0] for g in groups for t in g if len(t[0]) > 1))}
_C_SUMS, _H_SUMS = _sum_index(_C_GROUPS), _sum_index(_H_GROUPS)


def _form(form, get):
    acc = None
    for sign, i, j in form:
        v = get(i, j)
        acc = v if acc is None else (acc + v if sign > 0 else acc - v)
    return acc


def _gap_items(bufs, gap_scr):
    items = []
    for n, buf in enumerate(bufs):
        acc = []

        def part(r0, buf=buf, acc=acc):
            def fn(dep):
                wu = jnp.concatenate([buf[r:r + 8, :] for r in range(r0, r0 + T, 32)])
                mask = jnp.full((8, T), 0x7FFF0000, U32)
                if dep is not None:
                    mask = jnp.where(dep > jnp.inf, jnp.uint32(0), mask)
                mask = _rows(mask, 32)
                new = [jnp.sum(pltpu.bitcast(v & mask, F32).reshape(4, 8, T), axis=0) for v in (wu << 16, wu)]
                acc[:] = [u + v for u, v in zip(acc, new)] if acc else new
            return fn

        def last(_, n=n, acc=acc):
            bits = []
            for v in acc:
                l1 = jnp.sum(jnp.sum(v, axis=1, keepdims=True), axis=0, keepdims=True)
                bits.append(pltpu.bitcast(jnp.broadcast_to(l1, (8, T)), jnp.int32) >> 8)
            gap_scr[n] = jnp.clip((bits[0] - bits[1] + (1 << 14)) >> 15, -8, 8) << 23

        items += [part(r0) for r0 in range(0, buf.shape[0], T)] + [last]
    return items


class _PairWeights:
    def __init__(self, w_ref, transpose=False, shift=None):
        self.base = {}
        if shift is not None:
            fac = _rows(pltpu.bitcast(0x3F800000 + shift, F32), T)
            self.inv = pltpu.bitcast(0x3F800000 - shift, F32)
        for j in range(w_ref.shape[0] // T):
            wu = w_ref[_tile(j), :]
            if transpose:
                wu = wu.T
            hi = pltpu.bitcast(wu & jnp.uint32(0xFFFF0000), F32)
            self.base[j, 0] = pltpu.bitcast(wu << 16, F32)
            self.base[j, 1] = hi if shift is None else hi * fac
        self.cache = {}

    def __call__(self, form):
        sign = 1
        if form[-1][0] < 0 and form[0][1:] > form[1][1:]:
            sign, form = -1, ((1,) + form[1][1:], (-1,) + form[0][1:])
        if form not in self.cache:
            self.cache[form] = _form(form, lambda k, h: self.base[k, h]).astype(BF16)
        return sign, self.cache[form]


def _run_group(jobs, prods, a_get, w, transposed, finish):
    left = {}
    for _, _, outs in prods:
        for _, i, h in outs:
            left[i, h] = left.get((i, h), 0) + 1
    acc = {}
    for af, bf, outs in prods:
        sign, wt = w(bf)
        m = jobs.mm([wt], [a_get(af)], _dot_nt) if transposed else jobs.mm([a_get(af)], [wt], _dot)
        for s_, i, h in outs:
            if (i, h) not in acc:
                acc[i, h] = (s_ * sign, m)
            else:
                s0, v = acc[i, h]
                acc[i, h] = (s0, v + m if s0 == s_ * sign else v - m) if s0 > 0 or s_ * sign < 0 else (1, m - v)
            left[i, h] -= 1
            if not left[i, h]:
                s0, v = acc.pop((i, h))
                assert s0 > 0
                finish(2 * i + h, v)


class _Jobs:
    def __init__(self, side=()):
        self.res = []
        self.side = list(side)

    def mm(self, lhs, wt, dot):
        acc = None
        for x, w in zip(lhs, wt):
            v = dot(x, w)
            self.res.append(v)
            acc = v if acc is None else v + acc
            rel = 4 * (len(self.res) % 4)
            while self.side and self.side[0][0] <= len(self.res):
                self.side.pop(0)[1](v[8 * rel:8 * rel + 8, :])
                rel = (rel + 2) % 16
        return acc


def _proj_step(h_scr, hs_scr, c_ref, cs_scr, wq_ref, wuk_ref, wuv_ref, q_scr, k_scr, v_scr, scale, shifts, side):
    wk, wvT, wq = [_PairWeights(w, n == 1, shifts[n]) for n, w in enumerate((wuk_ref, wuv_ref, wq_ref))]
    c_get = lambda f: _ld(cs_scr, _C_SUMS[f]) if len(f) > 1 else c_ref[_tile(f[0][1]), _tile(f[0][2])]
    h_get = lambda f: _ld(hs_scr, _H_SUMS[f]) if len(f) > 1 else _ld(h_scr, f[0][1], f[0][2])

    def put(dst, w, mul=None):
        muls = [mul, _rows(w.inv if mul is None else w.inv * mul, T)]

        def fn(u, v):
            v = (v if muls[u % 2] is None else v * muls[u % 2]).astype(BF16)
            dst[u] = v.T if mul is not None and u < QT else v
        return fn

    jobs = _Jobs(side)
    for groups, get, w, transposed, fin in ((_C_GROUPS, c_get, wk, False, put(k_scr, wk)),
                                            (_C_GROUPS, c_get, wvT, True, put(v_scr, wvT)),
                                            (_H_GROUPS, h_get, wq, False, put(q_scr, wq, scale))):
        for prods in groups:
            _run_group(jobs, prods, get, w, transposed, fin)
    assert not jobs.side


def _inner_group(rows, cols, pairs):
    xs, ys = dict.fromkeys(x for x, _ in pairs), dict.fromkeys(y for _, y in pairs)
    used = set(xs) | set(ys) | {(x[0], y[1]) for x, y in pairs} | {(y[0], x[1]) for x, y in pairs}
    prods = []
    for i, j in xs:
        mates = [y for x, y in pairs if x == (i, j)]
        prods.append((((1, i, 0),), ((1, 0, j), (-1, 1, j)), ((1, i, j),) + tuple((1, i2, j) for i2, _ in mates)))
        prods.append((((1, i, 0), (1, i, 1)), ((1, 1, j),), ((1, i, j),) + tuple((-1, i, j2) for _, j2 in mates)))
    for i2, j2 in ys:
        mates = [x for x, y in pairs if y == (i2, j2)]
        prods.append((((1, i2, 0), (1, i2, 1)), ((1, 0, j2),),
                      ((1, i2, j2),) + tuple((-1, i2, j) for _, j in mates)))
        prods.append((((1, i2, 1),), ((1, 0, j2), (-1, 1, j2)),
                      ((-1, i2, j2),) + tuple((-1, i, j2) for i, _ in mates)))
    prods += [(((1, i, h),), ((1, h, j),), ((1, i, j),))
              for i in rows for j in cols if (i, j) not in used for h in (0, 1)]
    for (i, j), (i2, j2) in pairs:
        lo, hi = min(j, j2), max(j, j2)
        prods.append((((1, i2, 0), (-1, i, 0)), ((1, 0, lo), (1, 0, hi)), ((1, i2, j),)))
        prods.append((((1, i, 0), (1, i2, 1)), ((1, 0, j2), (1, 1, j)), ((1, i, j2), (1, i2, j))))
        prods.append((((1, i, 1), (-1, i2, 1)), ((1, 1, lo), (1, 1, hi)), ((1, i, j2),)))
    return prods


def _o_jobs():
    prods = (_inner_group(range(10), range(5), _all_pairs(range(0, 10, 2), range(1, 10, 2)))
             + _inner_group(range(10, 16), range(5), _PAIRS65))
    row = lambda t: max(i for _, i, _ in t[0])
    unit = lambda t: max(2 * i + h for _, i, h in t[0])
    need = lambda t: unit(t) if row(t) == 15 else 2 * row(t) + 1
    return [(need(t), t) for t in sorted(prods, key=need)]


_O_JOBS = _o_jobs()


SB = 4
TS = (-1.125, -0.375, 0.375, 1.125)
_SBP = [(i, j) for i in range(SB) for j in range(i + 1, SB)]
_PF = {f: n for n, f in enumerate([('R', i) for i in range(SB)] + [('C', i) for i in range(SB)]
                                  + [('S', i, j) for i in range(SB) for j in range(SB) if i != j]
                                  + [('A', i, j) for i, j in _SBP])}
_VF = {f: n for n, f in enumerate([('W', i) for i in range(SB)]
                                  + [(q, i, j) for i, j in _SBP for q in ('Q1', 'Q2', 'Q3')])}
_PV = {**{('W', i): ('R', i) for i in range(SB)}, **{('B', i): ('C', i) for i in range(SB)},
       **{('Q1', i, j): ('S', i, j) for i, j in _SBP}, **{('Q2', i, j): ('A', i, j) for i, j in _SBP},
       **{('Q3', i, j): ('S', j, i) for i, j in _SBP}}
_NPF, _NVF = len(_PF), len(_VF)
_DSLOT = (SB - 1) * _NPF
_VSLOT = _DSLOT + SB * (SB + 1) // 2
_FENCE = _VSLOT + (SB - 1) * _NVF // 2


def _job_order(nsb):
    units = [(I, h) for I in range(nsb) for h in range(2)]
    qe, qv = [], []
    for I, h in units:
        qe += [('e', I, h, J, p) for J in range(I) for p in range(SB)]
        qe += [('d', I, h, i, k) for i in range(SB) for k in range(i + 1)]
        for i in range(SB):
            prods = [('W', i), ('B', i)] + [(q, i, j) for j in range(i + 1, SB) for q in ('Q1', 'Q2', 'Q3')]
            qv += [('p', I, h, f, J) for f in prods for J in range(I)]
            qv += [('v', I, h, i, k) for k in range(i + 1)]
    qo = [('o', u, j) for j, (u, _) in enumerate(_O_JOBS)]
    cost = dict(e=8, d=2, p=1, v=2, o=2)
    tot_e, tot_r = sum(cost[j[0]] for j in qe), sum(cost[j[0]] for j in qv + qo)
    order, done = [], {}
    now = [0]
    did_e = did_r = 0

    def emit(q):
        job = q.pop(0)
        order.append(job)
        now[0] += cost[job[0]]
        if job[0] == 'e':
            done['e', job[1], job[2]] = now[0]
        elif job[0] == 'd':
            done[job] = now[0]
        elif job[0] == 'v' and job[4] == job[3]:
            done['u', 2 * (SB * job[1] + job[3]) + job[2]] = now[0]
        return cost[job[0]]

    def v_ready():
        if not qv:
            return False
        key = ('d', qv[0][1], qv[0][2], SB - 1, SB - 1)
        return key in done and done[key] + LAT_A <= now[0]

    def o_ready():
        return bool(qo) and ('u', qo[0][1]) in done and done['u', qo[0][1]] + LAT_B <= now[0]

    def fill(nv, no):
        n = 0
        while nv > 0 or no > 0 or n % 4:
            if no > 0 and n % 2 == 0 and o_ready() and no * ONV >= nv:
                no -= 2
                n += emit(qo)
            elif v_ready() and (nv > 0 or n % 4):
                c = emit(qv)
                nv -= c
                n += c
            elif o_ready() and n % 2 == 0 and (no > 0 or n % 4 or nv > 0) and len(qo) > RES:
                no -= 2
                n += emit(qo)
            else:
                break

    while qe:
        unit = qe[0][1:3]
        ne = 0
        while qe and ne < 8 and (ne == 0 or (qe[0][0] == 'd' and qe[0][1:3] == unit)):
            ne += emit(qe)
        groups = lambda q: sum(cost[j[0]] for j in q) / 8
        old = [j for j in qv if j[1:3] != unit and ('d', j[1], j[2], SB - 1, SB - 1) in done]
        here = [j for j in qe if j[1:3] == unit]
        rest = sum(cost[j[0]] for j in old)
        nv = (rest - (LAT_A if here else 0)) / (groups(here) + 1) if here else min(rest, LAT_A)
        no = 2 * max(len(qo) - RES - OEND, 0) / (groups(qe) + 1)
        fill(int(nv + 0.5), int(no + 0.5))
    while qv or qo:
        if qv and v_ready():
            fill(6, 2)
            if not qv:
                continue
        elif o_ready():
            emit(qo)
        else:
            emit(qv or qo)
    return order


def _softmax_shifts(q_scr, k_scr, m_scr):
    causal = (jax.lax.broadcasted_iota(jnp.int32, (T, T), 0)
              <= jax.lax.broadcasted_iota(jnp.int32, (T, T), 1))

    def unit(u, carry):
        r, hd = u // 2, u % 2

        def block(c, ml):
            s = _dot_nt(_ld(k_scr, 2 * c + hd), _ld(q_scr, u))
            s = jnp.where(jnp.logical_or(causal, c < r), s, -1e9 * LOG2E)
            m = jnp.maximum(ml[0], jnp.max(s, axis=0, keepdims=True))
            return m, ml[1] * jnp.exp2(ml[0] - m) + jnp.sum(jnp.exp2(s - m), axis=0, keepdims=True)

        m, l = jax.lax.fori_loop(0, r + 1, block, (jnp.full((1, T), -jnp.inf, F32), jnp.zeros((1, T), F32)))
        m_scr[u] = jnp.broadcast_to(m + jnp.log(l) * LOG2E, (8, T))
        return carry

    jax.lax.fori_loop(0, q_scr.shape[0], unit, 0)


def _attention_step(q_scr, k_scr, v_scr, m_scr, pf, wo_ref, acc_scr, flag_scr, z):
    causal = (jax.lax.broadcasted_iota(jnp.int32, (T, T), 0)
              <= jax.lax.broadcasted_iota(jnp.int32, (T, T), 1))
    HT = T // 2
    lsum, lrow, acc, fg, dacc, of, lhs = {}, {}, {}, {}, {}, {}, {}
    res = []
    wo, terms = {}, {}
    left = {}
    side = []
    chk = [jnp.zeros((8, T), F32), None]
    for _, t in _O_JOBS:
        for _, i, j in t[2]:
            left[i, j] = left.get((i, j), 0) + 1

    def probs(s, u):
        return jnp.exp2(s.reshape(T // 8, 8, T) - m_scr[u][None]).reshape(T, T)

    def add_l(u, v):
        lsum[u] = v if u not in lsum else lsum[u] + v

    def v_forms(h, J):
        n = 16

        def item(r0, pairs):
            def fn(dep):
                ts = {k: _rows(_after(jnp.full((8, T), TS[k], F32), dep), n) for k in range(SB)}

                def get(k, a):
                    r = (a * HT + r0) // 2
                    return _ld(v_scr, 2 * (SB * J + k) + h, slice(r, r + n // 2)).astype(F32)

                def put(f, v):
                    f = _VF[f] + J * _NVF
                    pf[h][_VSLOT + f // 2, f % 2 * HT + r0:f % 2 * HT + r0 + n, :] = v.astype(BF16)

                if pairs is None:
                    w = [get(k, 0) + ts[k] * get(k, 1) for k in range(SB)]
                    for k in range(SB):
                        put(('W', k), w[k])
                    for i, j in _SBP:
                        put(('Q2', i, j), w[i] - w[j])
                    return
                b = {(k, a): get(k, a) for k in sorted({k for pr in pairs for k in pr}) for a in range(2)}
                for i, j in pairs:
                    d0, d1 = b[j, 0] - b[i, 0], b[j, 1] - b[i, 1]
                    put(('Q1', i, j), d0 + ts[i] * d1)
                    put(('Q3', i, j), d0 + ts[j] * d1)
            return fn

        return [item(r0, pairs) for r0 in range(0, HT, n)
                for pairs in (None, _SBP[:2], [_SBP[2], _SBP[4]], [_SBP[3], _SBP[5]])]

    def job_e(I, h, J, p):
        if J == 0 and p == 0:
            side.extend(v_forms(h, I - 1))
        ps = []
        for i in range(SB):
            u = 2 * (SB * I + i) + h
            x = jnp.concatenate([k_scr.bitcast(U32)[2 * (SB * J + (t - i) % SB) + h, 8 * g:8 * g + 8, :]
                                 for g in (2 * p, 2 * p + 1) for t in range(SB)], axis=0)
            s = (_dot if u < QT else _dot_nt)(pltpu.bitcast(x, BF16), _ld(q_scr, u))
            res.append(s)
            ps.append(probs(s, u))
        for n, g in enumerate((2 * p, 2 * p + 1)):
            at = lambda i, t: ps[i][16 * (SB * n + t):16 * (SB * n + t) + 16]
            cell = lambda i, k: at(i, (i + k) % SB)

            def put(f, v):
                pf[h][J * _NPF + _PF[f], 16 * g:16 * g + 16, :] = v.astype(BF16)

            for i in range(SB):
                r = ((at(i, 0) + at(i, 1)) + at(i, 2)) + at(i, 3)
                put(('R', i), r)
                add_l(2 * (SB * I + i) + h, r[:8] + r[8:])
                c = None
                for t in range(SB):
                    i2 = (t - i) % SB
                    v = cell(i2, i)
                    if c is None:
                        c = v if i2 == i else -v
                    else:
                        c = c + v if i2 == i else c - v
                put(('C', i), c)
                for j in range(SB):
                    if j != i:
                        put(('S', i, j), cell(i, j))
            for i, j in _SBP:
                put(('A', i, j), cell(i, j) + cell(j, i))

    def job_d(I, h, i, k):
        u = 2 * (SB * I + i) + h
        s = (_dot if u < QT else _dot_nt)(_ld(k_scr, 2 * (SB * I + k) + h), _ld(q_scr, u))
        res.append(s)
        if i == k:
            s = jnp.where(causal, s, -1e9 * LOG2E)
        p = probs(s, u)
        add_l(u, jnp.sum(p.reshape(T // 8, 8, T), axis=0))
        pf[h][_DSLOT + i * (i + 1) // 2 + k] = p.astype(BF16)
        if i == k:
            lrow[u] = jnp.sum(lsum.pop(u), axis=0, keepdims=True)
            if i == SB - 1:
                while side:
                    side.pop(0)(res[-1][0:8, :])
                pf[h][_FENCE + z, 0:16, :] = jnp.zeros((16, T), BF16)
                ls = [lrow[2 * (SB * I + a) + h] for a in range(SB)]
                lo = jnp.minimum(jnp.minimum(ls[0], ls[1]), jnp.minimum(ls[2], ls[3]))
                hi = jnp.maximum(jnp.maximum(ls[0], ls[1]), jnp.maximum(ls[2], ls[3]))
                ok = jnp.logical_and(lo >= L_LO, hi <= L_HI)
                if I:
                    ok = jnp.logical_and(ok, hi <= L_RATIO * lo)
                bad = jnp.where(ok, 0.0, 1.0)
                chk[1] = bad if chk[1] is None else jnp.maximum(chk[1], bad)

    def job_p(I, h, f, J):
        n = J * _NVF + _VF.get(f, 0)
        x = (_ld(v_scr, 2 * (SB * J + f[1]) + h, slice(HT // 2, HT)) if f[0] == 'B'
             else _ld(pf[h], _VSLOT + n // 2, slice(n % 2 * HT // 2, (n % 2 + 1) * HT // 2)))
        v = _dot(x, _ld(pf[h], J * _NPF + _PF[_PV[f]]))
        res.append(v)
        acc[f] = v if J == 0 else acc[f] + v
        if J < I - 1:
            return

        def add(key, v, sign=1):
            fg[key] = (v if sign > 0 else -v) if key not in fg else (fg[key] + v if sign > 0 else fg[key] - v)

        if f[0] == 'W':
            add(('F', f[1]), acc.pop(f))
        elif f[0] == 'B':
            add(('G', f[1]), acc.pop(f))
        elif f[0] == 'Q3':
            _, i, j = f
            q1, q2, q3 = (acc.pop((q, i, j)) for q in ('Q1', 'Q2', 'Q3'))
            t = ((q1 + q2) + q3) * (1.0 / (TS[i] - TS[j]))
            add(('G', i), t)
            add(('G', j), t)
            add(('F', i), q1)
            add(('F', j), q3, -1)

    def job_v(I, h, i, k):
        u = 2 * (SB * I + i) + h
        v = _dot(_ld(v_scr, 2 * (SB * I + k) + h), _ld(pf[h], _DSLOT + i * (i + 1) // 2 + k))
        res.append(v)
        dacc[u] = v if u not in dacc else dacc[u] + v
        if k == i:
            o = dacc.pop(u)
            if I:
                f, g = fg.pop(('F', i)), fg.pop(('G', i))
                o = o + jnp.concatenate([f - TS[i] * g, g], axis=0)
            o = o * (1.0 / lrow[u])
            of[u] = o
            chk[0] = chk[0] + jnp.sum(o.reshape(T // 8, 8, T), axis=0)

    def job_o(_, n):
        af, bf, outs = _O_JOBS[n][1]
        if af not in lhs:
            v = _form(af, lambda i, h: of[2 * i + h])
            lhs[af] = _tie(v.astype(BF16).T, v[0:8, :])
        if bf not in wo:
            wo[bf] = (wo_ref[_tile(bf[0][1]), _tile(bf[0][2])] if len(bf) == 1 else
                      _form(bf, lambda h, j: wo_ref[_tile(h), _tile(j)].astype(F32)).astype(BF16))
        v = _dot(lhs[af], wo[bf])
        res.append(v)
        for sign, i, j in outs:
            terms.setdefault((i, j), []).append((sign, v))
            if len(terms[i, j]) == left[i, j]:
                tot = acc_scr[_tile(i), _tile(j)]
                for sg, m in terms.pop((i, j)):
                    tot = tot + m if sg > 0 else tot - m
                acc_scr[_tile(i), _tile(j)] = tot

    fns = dict(e=job_e, d=job_d, p=job_p, v=job_v, o=job_o)
    for n, job in enumerate(_job_order(q_scr.shape[0] // (2 * SB))):
        fns[job[0]](*job[1:])
        if side and n % SIDE == 0:
            side.pop(0)(res[-1 - SLAG][8 * (n % 4):8 * (n % 4) + 8, :])
    fine = jnp.abs(chk[0]) < jnp.inf
    flag_scr[...] = jnp.maximum(flag_scr[...], jnp.where(fine, chk[1], 1.0))


def _kernel(x_hbm, c_hbm, wq_hbm, wuk_hbm, wuv_hbm, wo_hbm, w1_hbm, w2_hbm, w3_hbm, w4_hbm,
            cond_hbm, wmod_hbm, out_hbm,
            x_ref, c_ref, cond_ref, wma_ref, wmb_ref, w1_ref, w2_ref, w3_ref, w4_ref,
            wq_buf, wk_buf, wv_buf, wo_buf, out_buf, sem, wsem, osem,
            mod_scr, h_scr, cs_scr, hs_scr, w_scr, q_scr, k_scr, v_scr, acc_scr, xn_scr, xh_scr, a1_scr, t_scr,
            ws12, ws3, ws4, pq_buf, pk_buf, pv_buf, gap_scr, st_in, m_scr, pf_scr, vf_scr, flag_scr, redo):
    S, M = x_hbm.shape
    D = wq_hbm.shape[2]
    nattn = wo_hbm.shape[0]
    Fd = w4_hbm.shape[0]
    scale = float(D) ** -0.5 * LOG2E
    nb, nrb = S // T, S // RB
    km, kc = M // T, c_hbm.shape[1] // T
    NX = 4
    XR = S // NX
    CB = XR // T

    work, probe = (wk_buf, wv_buf, wq_buf), (pk_buf, pv_buf, pq_buf)

    def pcopies(g, bufs=work, s0=0):
        return [pltpu.make_async_copy(src.bitcast(U32).at[:, g, :], dst, wsem.at[s0 + j])
                for j, (src, dst) in enumerate(zip((wuk_hbm, wuv_hbm, wq_hbm), bufs))]

    def ocopy(g):
        return pltpu.make_async_copy(wo_hbm.at[g], wo_buf, wsem.at[3])

    def chunk_copy(src, dst, i, s0):
        rows = slice(i * XR, (i + 1) * XR)
        return pltpu.make_async_copy(src.at[rows, :], dst.at[rows, :], sem.at[s0 + i])

    cp_cond = pltpu.make_async_copy(cond_hbm, cond_ref, sem.at[0])
    cp_wma = pltpu.make_async_copy(wmod_hbm.at[:, 0:2 * M], wma_ref, sem.at[1])
    cp_late = [pltpu.make_async_copy(src, dst, sem.at[2 + j]) for j, (src, dst) in enumerate((
        (wmod_hbm.at[:, 2 * M:6 * M], wmb_ref), (w1_hbm, w1_ref), (w2_hbm, w2_ref),
        (w3_hbm, w3_ref), (w4_hbm, w4_ref)))]
    cp_x = [chunk_copy(x_hbm, x_ref, i, 7) for i in range(NX)]
    cp_c = [chunk_copy(c_hbm, c_ref, i, 7 + NX) for i in range(NX)]

    def silu_cond():
        cf = cond_ref[...].astype(F32)
        return jnp.broadcast_to((cf * jax.nn.sigmoid(cf)).astype(BF16), (8, M))

    cp_wk, cp_wv, cp_wq = pcopies(0)
    named = dict(k=cp_wk, v=cp_wv, q=cp_wq, o=ocopy(0), n=cp_cond, m=cp_wma)
    named.update(zip('abcd', cp_c))
    named.update(zip('wxyz', cp_x))
    started, arrived, did = set(), set(), set()

    def zero(r, carry):
        acc_scr[pl.ds(pl.multiple_of(r * T, T), T), :] = jnp.zeros((T, M), F32)
        return carry

    def x_rows(rows, dep):
        xf = x_ref[rows, :].astype(F32)
        if dep is None:
            return xf
        return jnp.concatenate([_after(xf[:, :T], _rows(dep, xf.shape[0])), xf[:, T:]], axis=1)

    def n_item(r, i):
        def fn(dep):
            rows = slice(r * T + i * LP, r * T + (i + 1) * LP)
            xn_scr[rows, :] = _ln(x_rows(rows, dep))
        return fn

    def h_item(r, i, normed):
        def fn(dep):
            rows = slice(i * LP, (i + 1) * LP)
            grows = slice(r * T + i * LP, r * T + (i + 1) * LP)
            sa = mod_scr[:, 0:M]
            if normed and dep is not None:
                sa = jnp.concatenate([_after(sa[:, _tile(j)], dep) for j in range(km)], axis=1)
            hf = ((xn_scr[grows, :] if normed else _ln(x_rows(grows, dep))) * _rows(mod_scr[:, M:2 * M], LP)
                  + _rows(sa, LP))
            for j in range(km):
                h_scr[r, j, rows, :] = hf[:, _tile(j)].astype(BF16)
            for f, n in _H_SUMS.items():
                if all(t[1] == r for t in f):
                    hs_scr[n, rows, :] = _form(f, lambda _, k: hf[:, _tile(k)]).astype(BF16)
            did.add(('h', r, i))
        return fn

    def release(jobs, span, items):
        if span and items:
            jobs.side += [(len(jobs.res) + 1 + i * span // len(items), fn) for i, fn in enumerate(items)]
            jobs.side.sort(key=lambda e: e[0])
        else:
            for fn in items:
                fn(None)

    def sum_items(n, group, index, dst, get, skip_rows):
        forms = [f for f in dict.fromkeys(t[0] for t in group)
                 if len(f) > 1 and not (skip_rows and len({t[1] for t in f}) == 1)]

        def item(f, rows):
            def fn(dep):
                def term(r, k):
                    v = get(r, k, rows).astype(F32)
                    return v if dep is None or (r, k) != f[0][1:] else _after(v, _rows(dep, v.shape[0]))
                dst[index[f], rows, :] = _form(f, term).astype(BF16)
            return fn

        return [item(f, slice(i, i + n)) for i in range(0, T, n) for f in forms]

    h_sums = lambda n, gi: sum_items(n, _H_GROUPS[gi], _H_SUMS, hs_scr,
                                     lambda r_, k, rows: h_scr[r_, k, rows, :], True)

    def stash(key, buf, j0, transpose=False):
        n = buf.shape[0] // T
        if key not in did:
            assert key in arrived
            did.add(key)
            w = _PairWeights(buf, transpose)
            for j in range(n):
                for hd in range(2):
                    w_scr[hd, j0 + j] = w(((1, j, hd),))[1]
        return lambda hd: [_ld(w_scr, hd, j0 + j) for j in range(n)]

    def kv_tile(jobs, r):
        wk, wvT = stash('k', wk_buf, 0), stash('v', wv_buf, kc, True)
        ct = [c_ref[_tile(r), _tile(j)] for j in range(kc)]
        for hd in range(2):
            k_scr[2 * r + hd] = jobs.mm(ct, wk(hd), _dot).astype(BF16)
        for hd in range(2):
            v_scr[2 * r + hd] = jobs.mm(wvT(hd), ct, _dot_nt).astype(BF16)

    def q_tile(jobs, r):
        wq = stash('q', wq_buf, 2 * kc)
        ht = [_ld(h_scr, r, j) for j in range(km)]
        for hd in range(2):
            v = (jobs.mm(ht, wq(hd), _dot) * scale).astype(BF16)
            q_scr[2 * r + hd] = v.T if 2 * r + hd < QT else v

    for blk in PROLOGUE.split(';'):
        waits, starts, acts = blk.split('|')
        for ch in waits.strip():
            assert ch in started and ch not in arrived
            arrived.add(ch)
            named[ch].wait()
        for ch in starts.strip():
            assert ch not in started
            started.add(ch)
            named[ch].start()
        jobs = _Jobs()
        for act in acts.split():
            if act == 'Z':
                jax.lax.fori_loop(0, nb, zero, 0)
                acc_scr[S:, :] = jnp.zeros((acc_scr.shape[0] - S, M), F32)
                x_ref[S:, :] = jnp.zeros((x_ref.shape[0] - S, M), BF16)
                m_scr[...] = jnp.zeros(m_scr.shape, F32)
                flag_scr[...] = jnp.zeros(flag_scr.shape, F32)
                redo[0] = 0
            elif act == 'L':
                did.add('L')
                for cp in cp_late:
                    cp.start()
            elif act == 'M':
                assert arrived >= set('nm')
                mod = _dot(silu_cond(), wma_ref[...])
                mod_scr[:, 0:M] = mod[:, 0:M]
                mod_scr[:, M:2 * M] = 1.0 + mod[:, M:2 * M]
                did.add('M')
            else:
                act, _, span = act.partition('@')
                span = int(span or 0)
                items = []
                for r in [int(ch, 16) for ch in act[1:]]:
                    did.add((act[0], r))
                    if act[0] == 'K':
                        assert 'abcd'[r // CB] in arrived
                        kv_tile(jobs, r)
                    elif act[0] == 'H':
                        assert 'wxyz'[r // CB] in arrived and 'M' in did
                        items += [h_item(r, i, ('N', r) in did) for i in range(T // LP)]
                    elif act[0] == 'N':
                        assert 'wxyz'[r // CB] in arrived
                        items += [n_item(r, i) for i in range(T // LP)]
                    elif act[0] == 'Q':
                        assert all(('h', r, i) in did for i in range(T // LP))
                        q_tile(jobs, r)
                    elif act[0] == 'C':
                        assert all('abcd'[t[1] // CB] in arrived for p_ in _C_GROUPS[r] for t in p_[0])
                        items += sum_items(
                            32, _C_GROUPS[r], _C_SUMS, cs_scr,
                            lambda r_, k, rows: c_ref[r_ * T + rows.start:r_ * T + rows.stop, _tile(k)], False)
                    else:
                        assert act[0] == 'S' and all(('h', t[1], T // LP - 1) in did for p_ in _H_GROUPS[r] for t in p_[0])
                        items += h_sums(32 if span else 16, r)
                release(jobs, span, items)
        assert not jobs.side
    assert arrived == set(named) and all((k_, r) in did for k_ in 'KHQ' for r in range(nb))
    assert all((k_, r) in did for k_ in 'CS' for r in range(2)) and 'L' in did

    FH = ws3.shape[0] * T
    assert nattn - 1 >= FH // 64

    slices = ((w1_hbm, 32, 2 * T, 0), (w2_hbm, 32, 2 * T, 64), (w4_hbm, 64, FH, 128), (w3_hbm, T, FH, 256))
    slice_of = lambda g, n, half: jnp.minimum(g, half // n - 1)

    def prep_in(g):
        return [pltpu.make_async_copy(
            w.at[pl.ds(pl.multiple_of(slice_of(g, n, half) * n + x * half, n), n), 0:4 * T],
            st_in.at[r0 + x * n:r0 + (x + 1) * n, :], wsem.at[7]) for w, n, half, r0 in slices for x in range(2)]

    def mixer_prep(g):
        def blocks(r0, n, half, c0, c1, dep):
            get = lambda x, c: st_in[r0 + x * half:r0 + x * half + n, _tile(c)].astype(F32)
            return [_after(get(0, c0), _rows(dep, n)), get(0, c1), get(1, c0), _after(get(1, c1), _rows(dep, n))]

        def rows_item(dst, per, half, r0, c, o, n=16):
            def fn(dep):
                rows = pl.ds(pl.multiple_of(slice_of(g, per, half) * per, per) + o, n)
                for i, v in enumerate(_b_ops(*blocks(r0 + o, n, per, c, c + 2, dep))):
                    dst[i, c, rows, :] = v.astype(BF16)
            return fn

        def w3_item(k, i):
            def fn(dep):
                b11, b21, b12, b22 = blocks(slices[3][3], T, T, k, k + 2, dep)
                ws3[slice_of(g, T, FH), i, k] = _b_ops(b11, b12, b21, b22)[i].astype(BF16).T
            return fn

        return ([rows_item(dst, *sl[1:], c, o) for dst, sl in zip((ws12.at[0], ws12.at[1], ws4), slices)
                 for c in range(2) for o in range(0, sl[1], 16)]
                + [w3_item(k, i) for k in range(2) for i in range(7)])

    def next_copies(g):
        return pcopies(jnp.minimum(g + 1, nattn - 1)) + pcopies(jnp.minimum(g + 2, nattn - 1), probe, 4)

    def start_copies(g):
        for cp in next_copies(g) + prep_in(jnp.maximum(g, 0)):
            cp.start()

    def attn_body(g, exact):
        gw = jnp.maximum(g, 0)
        copies = next_copies(g)

        @pl.when(g >= 0)
        def _():
            pl.when(exact > 0)(lambda: _softmax_shifts(q_scr, k_scr, m_scr))
            bufs = (q_scr, k_scr, v_scr, m_scr, (pf_scr, vf_scr), wo_buf, acc_scr, flag_scr)
            _attention_step(*bufs, g >> 16)

        for cp in copies:
            cp.wait()
        pltpu.make_async_copy(st_in, st_in, wsem.at[7]).wait()

        @pl.when(g == -exact)
        def _():
            for fn in _gap_items(work, gap_scr):
                fn(None)

        @pl.when(g + 1 < nattn)
        def _():
            ocopy(g + 1).start()
            side = mixer_prep(gw) + _gap_items(probe, gap_scr)
            side = [(SD0 + i * SDS + (SDJ if i >= SDN else 0), fn) for i, fn in enumerate(side)]
            bufs = (h_scr, hs_scr, c_ref, cs_scr, wq_buf, wk_buf, wv_buf, q_scr, k_scr, v_scr)
            _proj_step(*bufs, scale, gap_scr, side)
            start_copies(g + 1)
            ocopy(g + 1).wait()

        return exact

    def attn_pass(exact, carry):
        @pl.when(jnp.logical_or(exact == 0, redo[0] > 0))
        def _():
            @pl.when(exact > 0)
            def _():
                jax.lax.fori_loop(0, nb, zero, 0)

            start_copies(-exact)
            jax.lax.fori_loop(-exact, nattn, attn_body, exact)

        @pl.when(exact == 0)
        def _():
            redo[0] = (jnp.max(flag_scr[...]) > 0).astype(jnp.int32)

        return carry

    jax.lax.fori_loop(0, 2, attn_pass, 0)

    for cp in cp_late:
        cp.wait()
    mod = _dot(silu_cond(), wmb_ref[...])
    mod_scr[:, 2 * M:4 * M] = mod[:, 0:2 * M]
    mod_scr[:, 4 * M:5 * M] = 1.0 + mod[:, 2 * M:3 * M]
    mod_scr[:, 5 * M:6 * M] = mod[:, 3 * M:4 * M]
    ftiles = [(f, min(f + T, Fd)) for f in range(0, Fd, T)]
    OFF = x_ref.shape[0] - S
    CAR = t_scr.shape[0] - RB

    def p1(r0, l0, n, dep=None):
        ga = mod_scr[:, 2 * M:3 * M]
        if dep is not None:
            ga = jnp.concatenate([_after(ga[:, 0:T], dep), ga[:, T:]], axis=1)
        rows = pl.ds(r0, n)
        x1 = x_ref[rows, :].astype(F32) + _rows(ga, n) * acc_scr[rows, :]
        xh_scr[0, l0:l0 + n, :] = x1
        hb = _ln(x1) * _rows(mod_scr[:, 4 * M:5 * M], n) + _rows(mod_scr[:, 3 * M:4 * M], n)
        xh_scr[1, l0:l0 + n, :] = hb
        return _ln(hb)

    HT = T // 2

    def p1_store(r0, c, dep=None):
        v = p1(r0 + c * PC, OFF + c * PC, PC, dep)
        a1_scr[c * PC:(c + 1) * PC, :] = v
        return jnp.max(v[:, M - T:].reshape(PC // 8, 8, T), axis=0)

    t_scr[RB:RB + CAR - OFF, :] = jnp.zeros((CAR - OFF, M), F32)
    t_scr[RB + CAR - OFF:RB + CAR, :] = _gelu(_dot(p1(0, 0, OFF).astype(BF16), w1_ref[...]))
    for c in range(RB // PC):
        p1_store(OFF, c)

    def out_copy(i):
        rows = pl.ds(i * T if isinstance(i, int) else pl.multiple_of(i * T, T), T)
        return pltpu.make_async_copy(out_buf.at[rows, :], out_hbm.at[rows, :], osem.at[i])

    def b_body(r, carry):
        gb = _rows(mod_scr[:, 5 * M:6 * M], T)
        r0 = pl.multiple_of(r * RB, RB)
        n0 = pl.multiple_of(jnp.minimum(r0 + RB, S - RB) + OFF, OFF)
        nh = RB // T
        now = [0]
        due = []
        pace = []

        def p1_item(c):
            return lambda dep: due.append((now[0] + PD, p1_store(n0, c, dep)))

        pace += [(P0 + i * PSTEP, p1_item(i)) for i in range(RB // PC)]
        wt = lambda ref, f0, f1, n: ref[f0:f1, _tile(n)]

        def mm(lhs, wts, dot=_dot):
            acc = None
            for x, w in zip(lhs, wts):
                if due and due[0][0] <= now[0]:
                    w = _tie(w, due.pop(0)[1])
                v = dot(x, w)
                now[0] += x.shape[0] // HT
                acc = v if acc is None else v + acc
                if pace and pace[0][0] <= now[0]:
                    pace.pop(0)[1](v[0:8, :])
            return acc

        def split_ops(lo, hi):
            return [v.astype(BF16) for v in _a_ops(lo[:HT], hi[:HT], lo[HT:], hi[HT:])]

        def two_tiles(aops, wsel, rest):
            def col(w):
                v = mm(rest[0], w, rest[3])
                return v[:HT], v[HT:]

            c11, c12, c21, c22 = _strassen(
                lambda i: mm([a[i] for a in aops], [wsel(i, k) for k in range(len(aops))]),
                lambda: col(rest[1]), lambda: col(rest[2]))
            return jnp.concatenate([c11, c21], axis=0), jnp.concatenate([c12, c22], axis=0)

        def square(full, aops, w_ref, ws_ref):
            out = {}
            for n in range(2):
                out[n], out[n + 2] = two_tiles(
                    aops, lambda i, k: _ld(ws_ref, i, n, slice(k * HT, (k + 1) * HT)),
                    (full[4:], [wt(w_ref, 4 * T, M, n)], [wt(w_ref, 4 * T, M, n + 2)], _dot))
            out[4] = mm(full, [wt(w_ref, j * T, (j + 1) * T, 4) for j in range(km)])
            return out

        t_scr[0:CAR, :] = t_scr[RB:RB + CAR, :]
        for hf in range(nh):
            a1 = [a1_scr[_tile(hf), _tile(j)] for j in range(km)]
            full = [v.astype(BF16) for v in a1]
            aops = [split_ops(a1[k], a1[2 + k]) for k in range(2)]
            for n, v in square(full, aops, w1_ref, ws12.at[0]).items():
                t = _gelu(v)
                if hf == nh - 1:
                    t = jnp.concatenate([t[:T - OFF], jnp.where(r < nrb - 1, t[T - OFF:], 0.0)], axis=0)
                t_scr[CAR + hf * T:CAR + (hf + 1) * T, _tile(n)] = t
        cq = M // 4
        shifts = (-1, 1, -2, 2)
        lane = jax.lax.broadcasted_iota(jnp.int32, (T, T), 1)
        y1, z, a3 = [], [], []
        for hf in range(nh):
            base = CAR - OFF + hf * T
            sh = []
            for j in range(km):
                g_lo, g_hi = (j * T) // cq, ((j + 1) * T - 1) // cq
                assert g_hi - g_lo <= 1
                v = t_scr[base + shifts[g_lo]:base + shifts[g_lo] + T, _tile(j)]
                if g_hi != g_lo:
                    v2 = t_scr[base + shifts[g_hi]:base + shifts[g_hi] + T, _tile(j)]
                    v = jnp.where(lane < g_hi * cq - j * T, v, v2)
                sh.append(v)
            hs = square([v.astype(BF16) for v in sh], [split_ops(sh[k], sh[2 + k]) for k in range(2)],
                        w2_ref, ws12.at[1])
            hs = jnp.concatenate([hs[n] for n in range(km)], axis=1)
            y1.append(hs + xh_scr[1, _tile(hf), :])
            z.append(xh_scr[0, _tile(hf), :] + gb * y1[hf])
            a3.append({})

            def ln_item(hf, c):
                def item(dep):
                    n = HT // NLN
                    for d in (0, HT):
                        v = y1[hf][d + c * n:d + (c + 1) * n]
                        if dep is not None:
                            v = jnp.concatenate([_after(v[:, :T], _rows(dep, n)), v[:, T:]], axis=1)
                        a3[hf][d + c * n] = _ln(v)
                return item

            ln_item(hf, 0)(None)
            pace += [(now[0] + LN0 + (c - 1) * LNS * (1 + hf), ln_item(hf, c)) for c in range(1, NLN)]
            pace.sort(key=lambda e: e[0])
        xh_scr[:, 0:OFF, :] = xh_scr[:, RB:RB + OFF, :]
        nf = FH // T
        h3, h3ops = [], []
        for hf in range(nh):
            assert len(a3[hf]) == 2 * NLN
            af = jnp.concatenate([a3[hf][key] for key in sorted(a3[hf])], axis=0)
            full = [af[:, _tile(j)].astype(BF16) for j in range(km)]
            aops = [split_ops(af[:, _tile(k)], af[:, _tile(2 + k)]) for k in range(2)]
            row, ops = {}, []
            narrow = None
            for n in range(nf):
                lo, hi = two_tiles(aops, lambda i, k: _ld(ws3, n, i, k),
                                   (full[4:], [wt(w3_ref, *ftiles[n], 4)],
                                    [wt(w3_ref, *ftiles[nf + n], 4)], _dot_nt))
                lo, hi = _gelu(lo), _gelu(hi)
                row[n], row[nf + n] = lo.astype(BF16), hi.astype(BF16)
                ops.append(split_ops(lo, hi))
                if n < km:
                    v = mm([wt(w3_ref, *ftiles[-1], n)], [full[n]], _dot_nt)
                    narrow = v if narrow is None else v + narrow
            row[2 * nf] = _gelu(mm(full, [wt(w3_ref, *ftiles[2 * nf], j) for j in range(km)],
                                   _dot_nt)).astype(BF16)
            fw = Fd - ftiles[-1][0]
            gT = jnp.concatenate([_gelu(narrow), jnp.zeros((T - fw, T), F32)], axis=0)
            row[2 * nf + 1] = _tie(gT.astype(BF16).T, gT[0:8, :])[:, :fw]
            h3.append([row[i] for i in range(len(ftiles))])
            h3ops.append(ops)
        for hf in range(nh):
            rows = pl.ds(pl.multiple_of(r0 + hf * T, T), T)

            def finish(n, v):
                out_buf[rows, _tile(n)] = (z[hf][:, _tile(n)] + gb[:, _tile(n)] * v).astype(out_buf.dtype)

            w4t = lambda n, f_: [wt(w4_ref, f0, f1, n) for f0, f1 in f_]
            finish(4, mm(h3[hf], w4t(4, ftiles)))
            for n in range(2):
                lo, hi = two_tiles(h3ops[hf], lambda i, k: _ld(ws4, i, n, slice(k * HT, (k + 1) * HT)),
                                   (h3[hf][2 * nf:], w4t(n, ftiles[2 * nf:]), w4t(n + 2, ftiles[2 * nf:]), _dot))
                finish(n, lo)
                finish(n + 2, hi)
            out_copy(r * nh + hf).start()
        assert not pace
        return carry

    jax.lax.fori_loop(0, nrb, b_body, 0)
    for i in range(nb):
        out_copy(i).wait()


@jax.jit
def pallas_adaLN_cond__compressed_kv_cla__mixer_s_mlp__prompt_kernel(
    A_x: jax.Array,
    A_c_kv: jax.Array,
    A_w_q: jax.Array,
    A_w_uk: jax.Array,
    A_w_uv: jax.Array,
    A_w_o: jax.Array,
    B_x: jax.Array,
    B_w1: jax.Array,
    B_w2: jax.Array,
    B_w3: jax.Array,
    B_w4: jax.Array,
    c: jax.Array,
    w_mod: jax.Array,
):
    _, S, M = A_x.shape
    Dc = A_c_kv.shape[2]
    H, D = A_w_q.shape[1], A_w_q.shape[2]
    Fd = B_w3.shape[1]
    assert D == T and A_c_kv.shape[1] == S and Dc == 4 * T and M == 5 * T and 13 * T < Fd < 14 * T and S == 16 * T
    vmem = pltpu.VMEM
    packed = lambda *lead: vmem(lead + (T, T), BF16)
    out = pl.pallas_call(
        _kernel,
        in_specs=[pl.BlockSpec(memory_space=pltpu.HBM)] * 12,
        out_specs=pl.BlockSpec(memory_space=pltpu.HBM),
        out_shape=jax.ShapeDtypeStruct((S, M), A_x.dtype),
        scratch_shapes=[
            vmem((S + 16, M), BF16),
            vmem((S, Dc), BF16),
            vmem((1, M), BF16),
            vmem((M, 2 * M), BF16),
            vmem((M, 4 * M), BF16),
            vmem((M, M), BF16),
            vmem((M, M), BF16),
            vmem((Fd, M), BF16),
            vmem((Fd, M), BF16),
            vmem((M, D), U32),
            vmem((Dc, D), U32),
            vmem((Dc, D), U32),
            vmem((2 * D, M), BF16),
            vmem((S, M), A_x.dtype),
            pltpu.SemaphoreType.DMA((15,)),
            pltpu.SemaphoreType.DMA((8,)),
            pltpu.SemaphoreType.DMA((S // T,)),
            vmem((8, 6 * M), F32),
            vmem((S // T, M // T, T, T), BF16),
            vmem((len(_C_SUMS), T, T), BF16),
            vmem((len(_H_SUMS), T, T), BF16),
            packed(2, M // T + 2 * (Dc // T)),
            packed(2 * S // T),
            packed(2 * S // T),
            packed(2 * S // T),
            vmem((S + 16, M), F32),
            vmem((S, M), F32),
            vmem((2, RB + 16, M), F32),
            vmem((RB, M), F32),
            vmem((RB + 32, M), F32),
            vmem((2, 7, 2, 2 * T, T), BF16),
            packed(6, 7, 2),
            vmem((7, 2, 6 * T, T), BF16),
            vmem((M, D), U32),
            vmem((Dc, D), U32),
            vmem((Dc, D), U32),
            vmem((3, 8, T), jnp.int32),
            vmem((4 * T, 4 * T), BF16),
            vmem((2 * S // T, 8, T), F32),
            vmem((_FENCE + 1, T, T), BF16),
            vmem((_FENCE + 1, T, T), BF16),
            vmem((8, T), F32),
            pltpu.SMEM((1,), jnp.int32),
        ],
        compiler_params=pltpu.CompilerParams(
            vmem_limit_bytes=100 * 1024 * 1024,
            disable_bounds_checks=True,
        ),
    )(
        A_x.reshape(S, M), A_c_kv.reshape(S, Dc),
        A_w_q, A_w_uk, A_w_uv,
        A_w_o.reshape(H // 2, 2 * D, M),
        B_w1, B_w2, B_w3.T, B_w4, c, w_mod,
    )
    return out.reshape(1, S, M)
```

```python
import math

import jax
import jax.numpy as jnp
import jax.experimental.pallas as pl
import jax.experimental.pallas.tpu as pltpu

F32 = jnp.float32
BF16 = jnp.bfloat16
U32 = jnp.uint32
NT = (((1,), (1,)), ((), ()))
T = 128
EPS = 1e-5
LOG2E = math.log2(math.e)

GRP = 4
LEAD = 10
PROW = 3
RES = 32
LAT_0 = 24
LAT_A = 16
LAT_B = 20
ALEAD = 32
SD0, SDS, SDN, SDJ = 158, 2, 20, 30
QT = 0
ONV, OEND = 0.5, 24
SIDE, SLAG = 3, 4
L_LO, L_HI, L_RATIO = 2.0 ** -24, 2.0 ** 24, 4.0
RB = 256
PC = 32
P0, PSTEP, PD = 440, 30, 52
NLN, LN0, LNS = 4, 4, 5
LP = 16
PROLOGUE = ('|kva|Z; |b|; kva|wc|K0123; bw|xdn|C0@56 N0123@52 K4567; cx|mq|N4567@52 K89ab; '
            'd|y|C1@56 Kcdef; nmq|zo|M H01 H234567@30 Q0123; y||H89ab@30 Q4567; '
            'zo||L Hcdef@30 Q89ab S01 Qcdef')


def _dot(a, b):
    return jnp.dot(a, b, preferred_element_type=F32)


def _dot_nt(a, b):
    return jax.lax.dot_general(a, b, NT, preferred_element_type=F32)


def _ln(x):
    m = jnp.mean(x, axis=-1, keepdims=True)
    xc = x - m
    v = jnp.mean(xc * xc, axis=-1, keepdims=True)
    return xc * jnp.exp2(jnp.log(v + EPS) * (-0.5 * LOG2E))


def _rows(v, n):
    return jnp.broadcast_to(v[None], (n // 8, 8, v.shape[1])).reshape(n, v.shape[1])


def _gelu(x):
    c0 = math.sqrt(2.0 / math.pi)
    return 0.5 * x * (1.0 + jnp.tanh(c0 * (x + 0.044715 * (x * x * x))))


def _after(x, dep):
    return jnp.where(dep > jnp.inf, dep, x)


def _tie(x, dep):
    xu = pltpu.bitcast(x, U32)
    first = jnp.where(dep > jnp.inf, jnp.uint32(0), xu[:8])
    return pltpu.bitcast(jnp.concatenate([first, xu[8:]], axis=0), BF16)


def _tile(j):
    return slice(j * T, (j + 1) * T)


def _ld(ref, *idx):
    return pltpu.bitcast(ref.bitcast(U32)[idx], BF16)


def _a_ops(a11, a12, a21, a22):
    return [a11 + a22, a21 + a22, a11, a22, a11 + a12, a21 - a11, a12 - a22]


def _b_ops(b11, b12, b21, b22):
    return [b11 + b22, b11, b12 - b22, b21 - b11, b22, b11 + b12, b21 + b22]


def _strassen(prod, col1=None, col2=None):
    m4 = prod(3)
    m2 = prod(1)
    c21 = m2 + m4
    if col1 is not None:
        e11, e21 = col1()
        m4, c21 = m4 + e11, c21 + e21
    m3 = prod(2)
    m5 = prod(4)
    c12 = m3 + m5
    if col2 is not None:
        e12, e22 = col2()
        c12, m3 = c12 + e12, m3 + e22
    m1 = prod(0)
    c11 = prod(6) + (m1 + (m4 - m5))
    c22 = prod(5) + (m1 + (m3 - m2))
    return c11, c12, c21, c22


def _group(rows, cols, pairs):
    xs, ys = dict.fromkeys(x for x, _ in pairs), dict.fromkeys(y for _, y in pairs)
    used = set(xs) | set(ys) | {(x[0], y[1]) for x, y in pairs} | {(y[0], x[1]) for x, y in pairs}
    prods = []
    for n, r in enumerate(rows):
        for i, k in [x for x in xs if x[0] == r]:
            mates = [y for x, y in pairs if x == (i, k)]
            prods.append((((1, i, k),) + tuple((1, i, k2) for _, k2 in mates), ((1, k, 0),),
                          ((1, i, 0), (-1, i, 1))))
            prods.append((((1, i, k),) + tuple((-1, i2, k) for i2, _ in mates), ((1, k, 0), (1, k, 1)),
                          ((1, i, 1),)))
        for i2, k2 in [y for y in ys if y[0] == r]:
            mates = [x for x, y in pairs if y == (i2, k2)]
            prods.append((((1, i2, k2),) + tuple((1, i2, k) for _, k in mates), ((1, k2, 1),),
                          ((1, i2, 1), (-1, i2, 0))))
            prods.append((((1, i2, k2),) + tuple((-1, i, k2) for i, _ in mates), ((1, k2, 0), (1, k2, 1)),
                          ((1, i2, 0),)))
        prods += [(((1, r, k),), ((1, k, h),), ((1, r, h),)) for k in cols if (r, k) not in used for h in (0, 1)]
        for (i, k), (i2, k2) in pairs:
            if r in (i, i2) and i + i2 - r in rows[n + 1:]:
                prods.append((((1, i, k2),), ((1, k2, 0), (-1, k, 0)), ((1, i2, 0), (1, i, 0))))
                prods.append((((1, i2, k), (1, i, k2)), ((1, k, 0), (1, k2, 1)), ((1, i2, 0), (1, i, 1))))
                prods.append((((1, i2, k),), ((1, k, 1), (-1, k2, 1)), ((1, i2, 1), (1, i, 1))))
    return prods


def _all_pairs(xrows, yrows):
    return [((x, a), (y, b)) for a, x in enumerate(xrows) for b, y in enumerate(yrows) if a != b]


_PAIRS65 = [((x[0] + 10, x[1]), (y[0] + 10, y[1])) for x, y in (
    ((0, 1), (1, 0)), ((0, 1), (5, 2)), ((2, 3), (1, 0)), ((2, 3), (3, 1)), ((2, 3), (5, 2)), ((3, 2), (1, 0)),
    ((4, 4), (0, 3)), ((4, 4), (1, 0)), ((4, 4), (3, 1)), ((4, 4), (5, 2)))]
_C_GROUPS = [_group(range(r, r + 8), range(4), _all_pairs(range(r, r + 4), range(r + 4, r + 8))) for r in (0, 8)]
_H_GROUPS = [_group(range(10), range(5), _all_pairs(range(5), range(5, 10))),
             _group(range(10, 16), range(5), _PAIRS65)]
_sum_index = lambda groups: {f: n for n, f in enumerate(
    dict.fromkeys(t[0] for g in groups for t in g if len(t[0]) > 1))}
_C_SUMS, _H_SUMS = _sum_index(_C_GROUPS), _sum_index(_H_GROUPS)


def _form(form, get):
    acc = None
    for sign, i, j in form:
        v = get(i, j)
        acc = v if acc is None else (acc + v if sign > 0 else acc - v)
    return acc


def _gap_items(bufs, gap_scr):
    items = []
    for n, buf in enumerate(bufs):
        acc = []

        def part(r0, buf=buf, acc=acc):
            def fn(dep):
                wu = jnp.concatenate([buf[r:r + 8, :] for r in range(r0, r0 + T, 32)])
                mask = jnp.full((8, T), 0x7FFF0000, U32)
                if dep is not None:
                    mask = jnp.where(dep > jnp.inf, jnp.uint32(0), mask)
                mask = _rows(mask, 32)
                new = [jnp.sum(pltpu.bitcast(v & mask, F32).reshape(4, 8, T), axis=0) for v in (wu << 16, wu)]
                acc[:] = [u + v for u, v in zip(acc, new)] if acc else new
            return fn

        def last(_, n=n, acc=acc):
            bits = []
            for v in acc:
                l1 = jnp.sum(jnp.sum(v, axis=1, keepdims=True), axis=0, keepdims=True)
                bits.append(pltpu.bitcast(jnp.broadcast_to(l1, (8, T)), jnp.int32) >> 8)
            gap_scr[n] = jnp.clip((bits[0] - bits[1] + (1 << 14)) >> 15, -8, 8) << 23

        items += [part(r0) for r0 in range(0, buf.shape[0], T)] + [last]
    return items


class _PairWeights:
    def __init__(self, w_ref, transpose=False, shift=None):
        self.base = {}
        if shift is not None:
            fac = _rows(pltpu.bitcast(0x3F800000 + shift, F32), T)
            self.inv = pltpu.bitcast(0x3F800000 - shift, F32)
        for j in range(w_ref.shape[0] // T):
            wu = w_ref[_tile(j), :]
            if transpose:
                wu = wu.T
            hi = pltpu.bitcast(wu & jnp.uint32(0xFFFF0000), F32)
            self.base[j, 0] = pltpu.bitcast(wu << 16, F32)
            self.base[j, 1] = hi if shift is None else hi * fac
        self.cache = {}

    def __call__(self, form):
        sign = 1
        if form[-1][0] < 0 and form[0][1:] > form[1][1:]:
            sign, form = -1, ((1,) + form[1][1:], (-1,) + form[0][1:])
        if form not in self.cache:
            self.cache[form] = _form(form, lambda k, h: self.base[k, h]).astype(BF16)
        return sign, self.cache[form]


def _run_group(jobs, prods, a_get, w, transposed, finish):
    left = {}
    for _, _, outs in prods:
        for _, i, h in outs:
            left[i, h] = left.get((i, h), 0) + 1
    acc = {}
    for af, bf, outs in prods:
        sign, wt = w(bf)
        m = jobs.mm([wt], [a_get(af)], _dot_nt) if transposed else jobs.mm([a_get(af)], [wt], _dot)
        for s_, i, h in outs:
            if (i, h) not in acc:
                acc[i, h] = (s_ * sign, m)
            else:
                s0, v = acc[i, h]
                acc[i, h] = (s0, v + m if s0 == s_ * sign else v - m) if s0 > 0 or s_ * sign < 0 else (1, m - v)
            left[i, h] -= 1
            if not left[i, h]:
                s0, v = acc.pop((i, h))
                assert s0 > 0
                finish(2 * i + h, v)


class _Jobs:
    def __init__(self, side=()):
        self.res = []
        self.side = list(side)

    def mm(self, lhs, wt, dot):
        acc = None
        for x, w in zip(lhs, wt):
            v = dot(x, w)
            self.res.append(v)
            acc = v if acc is None else v + acc
            rel = 4 * (len(self.res) % 4)
            while self.side and self.side[0][0] <= len(self.res):
                self.side.pop(0)[1](v[8 * rel:8 * rel + 8, :])
                rel = (rel + 2) % 16
        return acc


def _proj_step(h_scr, hs_scr, c_ref, cs_scr, wq_ref, wuk_ref, wuv_ref, q_scr, k_scr, v_scr, scale, shifts, side):
    wk, wvT, wq = [_PairWeights(w, n == 1, shifts[n]) for n, w in enumerate((wuk_ref, wuv_ref, wq_ref))]
    c_get = lambda f: _ld(cs_scr, _C_SUMS[f]) if len(f) > 1 else c_ref[_tile(f[0][1]), _tile(f[0][2])]
    h_get = lambda f: _ld(hs_scr, _H_SUMS[f]) if len(f) > 1 else _ld(h_scr, f[0][1], f[0][2])

    def put(dst, w, mul=None):
        muls = [mul, _rows(w.inv if mul is None else w.inv * mul, T)]

        def fn(u, v):
            v = (v if muls[u % 2] is None else v * muls[u % 2]).astype(BF16)
            dst[u] = v.T if mul is not None and u < QT else v
        return fn

    jobs = _Jobs(side)
    for groups, get, w, transposed, fin in ((_C_GROUPS, c_get, wk, False, put(k_scr, wk)),
                                            (_C_GROUPS, c_get, wvT, True, put(v_scr, wvT)),
                                            (_H_GROUPS, h_get, wq, False, put(q_scr, wq, scale))):
        for prods in groups:
            _run_group(jobs, prods, get, w, transposed, fin)
    assert not jobs.side


def _inner_group(rows, cols, pairs):
    xs, ys = dict.fromkeys(x for x, _ in pairs), dict.fromkeys(y for _, y in pairs)
    used = set(xs) | set(ys) | {(x[0], y[1]) for x, y in pairs} | {(y[0], x[1]) for x, y in pairs}
    prods = []
    for i, j in xs:
        mates = [y for x, y in pairs if x == (i, j)]
        prods.append((((1, i, 0),), ((1, 0, j), (-1, 1, j)), ((1, i, j),) + tuple((1, i2, j) for i2, _ in mates)))
        prods.append((((1, i, 0), (1, i, 1)), ((1, 1, j),), ((1, i, j),) + tuple((-1, i, j2) for _, j2 in mates)))
    for i2, j2 in ys:
        mates = [x for x, y in pairs if y == (i2, j2)]
        prods.append((((1, i2, 0), (1, i2, 1)), ((1, 0, j2),),
                      ((1, i2, j2),) + tuple((-1, i2, j) for _, j in mates)))
        prods.append((((1, i2, 1),), ((1, 0, j2), (-1, 1, j2)),
                      ((-1, i2, j2),) + tuple((-1, i, j2) for i, _ in mates)))
    prods += [(((1, i, h),), ((1, h, j),), ((1, i, j),))
              for i in rows for j in cols if (i, j) not in used for h in (0, 1)]
    for (i, j), (i2, j2) in pairs:
        lo, hi = min(j, j2), max(j, j2)
        prods.append((((1, i2, 0), (-1, i, 0)), ((1, 0, lo), (1, 0, hi)), ((1, i2, j),)))
        prods.append((((1, i, 0), (1, i2, 1)), ((1, 0, j2), (1, 1, j)), ((1, i, j2), (1, i2, j))))
        prods.append((((1, i, 1), (-1, i2, 1)), ((1, 1, lo), (1, 1, hi)), ((1, i, j2),)))
    return prods


def _o_jobs():
    prods = (_inner_group(range(10), range(5), _all_pairs(range(0, 10, 2), range(1, 10, 2)))
             + _inner_group(range(10, 16), range(5), _PAIRS65))
    row = lambda t: max(i for _, i, _ in t[0])
    unit = lambda t: max(2 * i + h for _, i, h in t[0])
    need = lambda t: unit(t) if row(t) == 15 else 2 * row(t) + 1
    return [(need(t), t) for t in sorted(prods, key=need)]


_O_JOBS = _o_jobs()


SB = 4
TS = (-1.125, -0.375, 0.375, 1.125)
_SBP = [(i, j) for i in range(SB) for j in range(i + 1, SB)]
_PF = {f: n for n, f in enumerate([('R', i) for i in range(SB)] + [('C', i) for i in range(SB)]
                                  + [('S', i, j) for i in range(SB) for j in range(SB) if i != j]
                                  + [('A', i, j) for i, j in _SBP])}
_VF = {f: n for n, f in enumerate([('W', i) for i in range(SB)]
                                  + [(q, i, j) for i, j in _SBP for q in ('Q1', 'Q2', 'Q3')])}
_PV = {**{('W', i): ('R', i) for i in range(SB)}, **{('B', i): ('C', i) for i in range(SB)},
       **{('Q1', i, j): ('S', i, j) for i, j in _SBP}, **{('Q2', i, j): ('A', i, j) for i, j in _SBP},
       **{('Q3', i, j): ('S', j, i) for i, j in _SBP}}
_NPF, _NVF = len(_PF), len(_VF)
_DSLOT = (SB - 1) * _NPF
_VSLOT = _DSLOT + SB * (SB + 1) // 2
_FENCE = _VSLOT + (SB - 1) * _NVF // 2


def _job_order(nsb):
    units = [(I, h) for I in range(nsb) for h in range(2)]
    qe, qv = [], []
    for I, h in units:
        qe += [('e', I, h, J, p) for J in range(I) for p in range(SB)]
        qe += [('d', I, h, i, k) for i in range(SB) for k in range(i + 1)]
        for i in range(SB):
            prods = [('W', i), ('B', i)] + [(q, i, j) for j in range(i + 1, SB) for q in ('Q1', 'Q2', 'Q3')]
            qv += [('p', I, h, f, J) for f in prods for J in range(I)]
            qv += [('v', I, h, i, k) for k in range(i + 1)]
    qo = [('o', u, j) for j, (u, _) in enumerate(_O_JOBS)]
    cost = dict(e=8, d=2, p=1, v=2, o=2)
    tot_e, tot_r = sum(cost[j[0]] for j in qe), sum(cost[j[0]] for j in qv + qo)
    order, done = [], {}
    now = [0]
    did_e = did_r = 0

    def emit(q):
        job = q.pop(0)
        order.append(job)
        now[0] += cost[job[0]]
        if job[0] == 'e':
            done['e', job[1], job[2]] = now[0]
        elif job[0] == 'd':
            done[job] = now[0]
        elif job[0] == 'v' and job[4] == job[3]:
            done['u', 2 * (SB * job[1] + job[3]) + job[2]] = now[0]
        return cost[job[0]]

    def v_ready():
        if not qv:
            return False
        key = ('d', qv[0][1], qv[0][2], SB - 1, SB - 1)
        return key in done and done[key] + (LAT_0 if qv[0][1:3] == (0, 0) else LAT_A) <= now[0]

    def o_ready():
        return bool(qo) and ('u', qo[0][1]) in done and done['u', qo[0][1]] + LAT_B <= now[0]

    def fill(nv, no):
        n = 0
        while nv > 0 or no > 0 or n % 4:
            if no > 0 and n % 2 == 0 and o_ready() and no * ONV >= nv:
                no -= 2
                n += emit(qo)
            elif v_ready() and (nv > 0 or n % 4):
                c = emit(qv)
                nv -= c
                n += c
            elif o_ready() and n % 2 == 0 and (no > 0 or n % 4 or nv > 0) and len(qo) > RES:
                no -= 2
                n += emit(qo)
            else:
                break

    while qe:
        unit = qe[0][1:3]
        ne = 0
        while qe and ne < 8 and (ne == 0 or (qe[0][0] == 'd' and qe[0][1:3] == unit)):
            ne += emit(qe)
        groups = lambda q: sum(cost[j[0]] for j in q) / 8
        old = [j for j in qv if j[1:3] != unit and ('d', j[1], j[2], SB - 1, SB - 1) in done]
        here = [j for j in qe if j[1:3] == unit]
        rest = sum(cost[j[0]] for j in old)
        nv = (rest - (LAT_A if here else 0)) / (groups(here) + 1) if here else min(rest, LAT_A)
        no = 2 * max(len(qo) - RES - OEND, 0) / (groups(qe) + 1)
        fill(int(nv + 0.5), int(no + 0.5))
    while qv or qo:
        if qv and v_ready():
            fill(6, 2)
            if not qv:
                continue
        elif o_ready():
            emit(qo)
        else:
            emit(qv or qo)
    return order


def _softmax_shifts(q_scr, k_scr, m_scr):
    causal = (jax.lax.broadcasted_iota(jnp.int32, (T, T), 0)
              <= jax.lax.broadcasted_iota(jnp.int32, (T, T), 1))

    def unit(u, carry):
        r, hd = u // 2, u % 2

        def block(c, ml):
            s = _dot_nt(_ld(k_scr, 2 * c + hd), _ld(q_scr, u))
            s = jnp.where(jnp.logical_or(causal, c < r), s, -1e9 * LOG2E)
            m = jnp.maximum(ml[0], jnp.max(s, axis=0, keepdims=True))
            return m, ml[1] * jnp.exp2(ml[0] - m) + jnp.sum(jnp.exp2(s - m), axis=0, keepdims=True)

        m, l = jax.lax.fori_loop(0, r + 1, block, (jnp.full((1, T), -jnp.inf, F32), jnp.zeros((1, T), F32)))
        m_scr[u] = jnp.broadcast_to(m + jnp.log(l) * LOG2E, (8, T))
        return carry

    jax.lax.fori_loop(0, q_scr.shape[0], unit, 0)


def _attention_step(q_scr, k_scr, v_scr, m_scr, pf, wo_ref, acc_scr, flag_scr, z):
    causal = (jax.lax.broadcasted_iota(jnp.int32, (T, T), 0)
              <= jax.lax.broadcasted_iota(jnp.int32, (T, T), 1))
    HT = T // 2
    lsum, lrow, acc, fg, dacc, of, lhs = {}, {}, {}, {}, {}, {}, {}
    res = []
    wo, terms = {}, {}
    left = {}
    side = []
    chk = [jnp.zeros((8, T), F32), None]
    for _, t in _O_JOBS:
        for _, i, j in t[2]:
            left[i, j] = left.get((i, j), 0) + 1

    def probs(s, u):
        return jnp.exp2(s.reshape(T // 8, 8, T) - m_scr[u][None]).reshape(T, T)

    def add_l(u, v):
        lsum[u] = v if u not in lsum else lsum[u] + v

    def v_forms(h, J):
        n = 16

        def item(r0, pairs):
            def fn(dep):
                ts = {k: _rows(_after(jnp.full((8, T), TS[k], F32), dep), n) for k in range(SB)}

                def get(k, a):
                    r = (a * HT + r0) // 2
                    return _ld(v_scr, 2 * (SB * J + k) + h, slice(r, r + n // 2)).astype(F32)

                def put(f, v):
                    f = _VF[f] + J * _NVF
                    pf[h][_VSLOT + f // 2, f % 2 * HT + r0:f % 2 * HT + r0 + n, :] = v.astype(BF16)

                if pairs is None:
                    w = [get(k, 0) + ts[k] * get(k, 1) for k in range(SB)]
                    for k in range(SB):
                        put(('W', k), w[k])
                    for i, j in _SBP:
                        put(('Q2', i, j), w[i] - w[j])
                    return
                b = {(k, a): get(k, a) for k in sorted({k for pr in pairs for k in pr}) for a in range(2)}
                for i, j in pairs:
                    d0, d1 = b[j, 0] - b[i, 0], b[j, 1] - b[i, 1]
                    put(('Q1', i, j), d0 + ts[i] * d1)
                    put(('Q3', i, j), d0 + ts[j] * d1)
            return fn

        return [item(r0, pairs) for r0 in range(0, HT, n)
                for pairs in (None, _SBP[:2], [_SBP[2], _SBP[4]], [_SBP[3], _SBP[5]])]

    def job_e(I, h, J, p):
        ps = []
        for i in range(SB):
            u = 2 * (SB * I + i) + h
            x = jnp.concatenate([k_scr.bitcast(U32)[2 * (SB * J + (t - i) % SB) + h, 8 * g:8 * g + 8, :]
                                 for g in (2 * p, 2 * p + 1) for t in range(SB)], axis=0)
            s = (_dot if u < QT else _dot_nt)(pltpu.bitcast(x, BF16), _ld(q_scr, u))
            res.append(s)
            ps.append(probs(s, u))
        for n, g in enumerate((2 * p, 2 * p + 1)):
            at = lambda i, t: ps[i][16 * (SB * n + t):16 * (SB * n + t) + 16]
            cell = lambda i, k: at(i, (i + k) % SB)

            def put(f, v):
                pf[h][J * _NPF + _PF[f], 16 * g:16 * g + 16, :] = v.astype(BF16)

            for i in range(SB):
                r = ((at(i, 0) + at(i, 1)) + at(i, 2)) + at(i, 3)
                put(('R', i), r)
                add_l(2 * (SB * I + i) + h, r[:8] + r[8:])
                c = None
                for t in range(SB):
                    i2 = (t - i) % SB
                    v = cell(i2, i)
                    if c is None:
                        c = v if i2 == i else -v
                    else:
                        c = c + v if i2 == i else c - v
                put(('C', i), c)
                for j in range(SB):
                    if j != i:
                        put(('S', i, j), cell(i, j))
            for i, j in _SBP:
                put(('A', i, j), cell(i, j) + cell(j, i))

    def job_d(I, h, i, k):
        u = 2 * (SB * I + i) + h
        s = (_dot if u < QT else _dot_nt)(_ld(k_scr, 2 * (SB * I + k) + h), _ld(q_scr, u))
        res.append(s)
        if i == k:
            s = jnp.where(causal, s, -1e9 * LOG2E)
        p = probs(s, u)
        add_l(u, jnp.sum(p.reshape(T // 8, 8, T), axis=0))
        pf[h][_DSLOT + i * (i + 1) // 2 + k] = p.astype(BF16)
        if i == k:
            lrow[u] = jnp.sum(lsum.pop(u), axis=0, keepdims=True)
            if i == SB - 1:
                while side and side[0][0] <= (I - 1, h):
                    side.pop(0)[1](res[-1][0:8, :])
                pf[h][_FENCE + z, 0:16, :] = jnp.zeros((16, T), BF16)
                ls = [lrow[2 * (SB * I + a) + h] for a in range(SB)]
                lo = jnp.minimum(jnp.minimum(ls[0], ls[1]), jnp.minimum(ls[2], ls[3]))
                hi = jnp.maximum(jnp.maximum(ls[0], ls[1]), jnp.maximum(ls[2], ls[3]))
                ok = jnp.logical_and(lo >= L_LO, hi <= L_HI)
                if I:
                    ok = jnp.logical_and(ok, hi <= L_RATIO * lo)
                bad = jnp.where(ok, 0.0, 1.0)
                chk[1] = bad if chk[1] is None else jnp.maximum(chk[1], bad)

    def job_p(I, h, f, J):
        n = J * _NVF + _VF.get(f, 0)
        x = (_ld(v_scr, 2 * (SB * J + f[1]) + h, slice(HT // 2, HT)) if f[0] == 'B'
             else _ld(pf[h], _VSLOT + n // 2, slice(n % 2 * HT // 2, (n % 2 + 1) * HT // 2)))
        v = _dot(x, _ld(pf[h], J * _NPF + _PF[_PV[f]]))
        res.append(v)
        acc[f] = v if J == 0 else acc[f] + v
        if J < I - 1:
            return

        def add(key, v, sign=1):
            fg[key] = (v if sign > 0 else -v) if key not in fg else (fg[key] + v if sign > 0 else fg[key] - v)

        if f[0] == 'W':
            add(('F', f[1]), acc.pop(f))
        elif f[0] == 'B':
            add(('G', f[1]), acc.pop(f))
        elif f[0] == 'Q3':
            _, i, j = f
            q1, q2, q3 = (acc.pop((q, i, j)) for q in ('Q1', 'Q2', 'Q3'))
            t = ((q1 + q2) + q3) * (1.0 / (TS[i] - TS[j]))
            add(('G', i), t)
            add(('G', j), t)
            add(('F', i), q1)
            add(('F', j), q3, -1)

    def job_v(I, h, i, k):
        u = 2 * (SB * I + i) + h
        v = _dot(_ld(v_scr, 2 * (SB * I + k) + h), _ld(pf[h], _DSLOT + i * (i + 1) // 2 + k))
        res.append(v)
        dacc[u] = v if u not in dacc else dacc[u] + v
        if k == i:
            o = dacc.pop(u)
            if I:
                f, g = fg.pop(('F', i)), fg.pop(('G', i))
                o = o + jnp.concatenate([f - TS[i] * g, g], axis=0)
            o = o * (1.0 / lrow[u])
            of[u] = o
            chk[0] = chk[0] + jnp.sum(o.reshape(T // 8, 8, T), axis=0)

    def job_o(_, n):
        af, bf, outs = _O_JOBS[n][1]
        if af not in lhs:
            v = _form(af, lambda i, h: of[2 * i + h])
            lhs[af] = _tie(v.astype(BF16).T, v[0:8, :])
        if bf not in wo:
            wo[bf] = (wo_ref[_tile(bf[0][1]), _tile(bf[0][2])] if len(bf) == 1 else
                      _form(bf, lambda h, j: wo_ref[_tile(h), _tile(j)].astype(F32)).astype(BF16))
        v = _dot(lhs[af], wo[bf])
        res.append(v)
        for sign, i, j in outs:
            terms.setdefault((i, j), []).append((sign, v))
            if len(terms[i, j]) == left[i, j]:
                tot = acc_scr[_tile(i), _tile(j)]
                for sg, m in terms.pop((i, j)):
                    tot = tot + m if sg > 0 else tot - m
                acc_scr[_tile(i), _tile(j)] = tot

    side += [((J, h), fn) for J in range(SB - 1) for h in range(2) for fn in v_forms(h, J)]
    fns = dict(e=job_e, d=job_d, p=job_p, v=job_v, o=job_o)
    for n, job in enumerate(_job_order(q_scr.shape[0] // (2 * SB))):
        fns[job[0]](*job[1:])
        if side and n % SIDE == 0 and n >= SLAG:
            side.pop(0)[1](res[-1 - SLAG][8 * (n % 4):8 * (n % 4) + 8, :])
    fine = jnp.abs(chk[0]) < jnp.inf
    flag_scr[...] = jnp.maximum(flag_scr[...], jnp.where(fine, chk[1], 1.0))


def _kernel(x_hbm, c_hbm, wq_hbm, wuk_hbm, wuv_hbm, wo_hbm, w1_hbm, w2_hbm, w3_hbm, w4_hbm,
            cond_hbm, wmod_hbm, out_hbm,
            x_ref, c_ref, cond_ref, wma_ref, wmb_ref, w1_ref, w2_ref, w3_ref, w4_ref,
            wq_buf, wk_buf, wv_buf, wo_buf, out_buf, sem, wsem, osem,
            mod_scr, h_scr, cs_scr, hs_scr, w_scr, q_scr, k_scr, v_scr, acc_scr, xn_scr, xh_scr, a1_scr, t_scr,
            ws12, ws3, ws4, pq_buf, pk_buf, pv_buf, gap_scr, st_in, m_scr, pf_scr, vf_scr, flag_scr, redo):
    S, M = x_hbm.shape
    D = wq_hbm.shape[2]
    nattn = wo_hbm.shape[0]
    Fd = w4_hbm.shape[0]
    scale = float(D) ** -0.5 * LOG2E
    nb, nrb = S // T, S // RB
    km, kc = M // T, c_hbm.shape[1] // T
    NX = 4
    XR = S // NX
    CB = XR // T

    work, probe = (wk_buf, wv_buf, wq_buf), (pk_buf, pv_buf, pq_buf)

    def pcopies(g, bufs=work, s0=0):
        return [pltpu.make_async_copy(src.bitcast(U32).at[:, g, :], dst, wsem.at[s0 + j])
                for j, (src, dst) in enumerate(zip((wuk_hbm, wuv_hbm, wq_hbm), bufs))]

    def ocopy(g):
        return pltpu.make_async_copy(wo_hbm.at[g], wo_buf, wsem.at[3])

    def chunk_copy(src, dst, i, s0):
        rows = slice(i * XR, (i + 1) * XR)
        return pltpu.make_async_copy(src.at[rows, :], dst.at[rows, :], sem.at[s0 + i])

    cp_cond = pltpu.make_async_copy(cond_hbm, cond_ref, sem.at[0])
    cp_wma = pltpu.make_async_copy(wmod_hbm.at[:, 0:2 * M], wma_ref, sem.at[1])
    cp_late = [pltpu.make_async_copy(src, dst, sem.at[2 + j]) for j, (src, dst) in enumerate((
        (wmod_hbm.at[:, 2 * M:6 * M], wmb_ref), (w1_hbm, w1_ref), (w2_hbm, w2_ref),
        (w3_hbm, w3_ref), (w4_hbm, w4_ref)))]
    cp_x = [chunk_copy(x_hbm, x_ref, i, 7) for i in range(NX)]
    cp_c = [chunk_copy(c_hbm, c_ref, i, 7 + NX) for i in range(NX)]

    def silu_cond():
        cf = cond_ref[...].astype(F32)
        return jnp.broadcast_to((cf * jax.nn.sigmoid(cf)).astype(BF16), (8, M))

    cp_wk, cp_wv, cp_wq = pcopies(0)
    named = dict(k=cp_wk, v=cp_wv, q=cp_wq, o=ocopy(0), n=cp_cond, m=cp_wma)
    named.update(zip('abcd', cp_c))
    named.update(zip('wxyz', cp_x))
    started, arrived, did = set(), set(), set()

    def zero(r, carry):
        acc_scr[pl.ds(pl.multiple_of(r * T, T), T), :] = jnp.zeros((T, M), F32)
        return carry

    def x_rows(rows, dep):
        xf = x_ref[rows, :].astype(F32)
        if dep is None:
            return xf
        return jnp.concatenate([_after(xf[:, :T], _rows(dep, xf.shape[0])), xf[:, T:]], axis=1)

    def n_item(r, i):
        def fn(dep):
            rows = slice(r * T + i * LP, r * T + (i + 1) * LP)
            xn_scr[rows, :] = _ln(x_rows(rows, dep))
        return fn

    def h_item(r, i, normed):
        def fn(dep):
            rows = slice(i * LP, (i + 1) * LP)
            grows = slice(r * T + i * LP, r * T + (i + 1) * LP)
            sa = mod_scr[:, 0:M]
            if normed and dep is not None:
                sa = jnp.concatenate([_after(sa[:, _tile(j)], dep) for j in range(km)], axis=1)
            hf = ((xn_scr[grows, :] if normed else _ln(x_rows(grows, dep))) * _rows(mod_scr[:, M:2 * M], LP)
                  + _rows(sa, LP))
            for j in range(km):
                h_scr[r, j, rows, :] = hf[:, _tile(j)].astype(BF16)
            for f, n in _H_SUMS.items():
                if all(t[1] == r for t in f):
                    hs_scr[n, rows, :] = _form(f, lambda _, k: hf[:, _tile(k)]).astype(BF16)
            did.add(('h', r, i))
        return fn

    def release(jobs, span, items):
        if span and items:
            jobs.side += [(len(jobs.res) + 1 + i * span // len(items), fn) for i, fn in enumerate(items)]
            jobs.side.sort(key=lambda e: e[0])
        else:
            for fn in items:
                fn(None)

    def sum_items(n, group, index, dst, get, skip_rows):
        forms = [f for f in dict.fromkeys(t[0] for t in group)
                 if len(f) > 1 and not (skip_rows and len({t[1] for t in f}) == 1)]

        def item(f, rows):
            def fn(dep):
                def term(r, k):
                    v = get(r, k, rows).astype(F32)
                    return v if dep is None or (r, k) != f[0][1:] else _after(v, _rows(dep, v.shape[0]))
                dst[index[f], rows, :] = _form(f, term).astype(BF16)
            return fn

        return [item(f, slice(i, i + n)) for i in range(0, T, n) for f in forms]

    h_sums = lambda n, gi: sum_items(n, _H_GROUPS[gi], _H_SUMS, hs_scr,
                                     lambda r_, k, rows: h_scr[r_, k, rows, :], True)

    def stash(key, buf, j0, transpose=False):
        n = buf.shape[0] // T
        if key not in did:
            assert key in arrived
            did.add(key)
            w = _PairWeights(buf, transpose)
            for j in range(n):
                for hd in range(2):
                    w_scr[hd, j0 + j] = w(((1, j, hd),))[1]
        return lambda hd: [_ld(w_scr, hd, j0 + j) for j in range(n)]

    def kv_tile(jobs, r):
        wk, wvT = stash('k', wk_buf, 0), stash('v', wv_buf, kc, True)
        ct = [c_ref[_tile(r), _tile(j)] for j in range(kc)]
        for hd in range(2):
            k_scr[2 * r + hd] = jobs.mm(ct, wk(hd), _dot).astype(BF16)
        for hd in range(2):
            v_scr[2 * r + hd] = jobs.mm(wvT(hd), ct, _dot_nt).astype(BF16)

    def q_tile(jobs, r):
        wq = stash('q', wq_buf, 2 * kc)
        ht = [_ld(h_scr, r, j) for j in range(km)]
        for hd in range(2):
            v = (jobs.mm(ht, wq(hd), _dot) * scale).astype(BF16)
            q_scr[2 * r + hd] = v.T if 2 * r + hd < QT else v

    for blk in PROLOGUE.split(';'):
        waits, starts, acts = blk.split('|')
        for ch in waits.strip():
            assert ch in started and ch not in arrived
            arrived.add(ch)
            named[ch].wait()
        for ch in starts.strip():
            assert ch not in started
            started.add(ch)
            named[ch].start()
        jobs = _Jobs()
        for act in acts.split():
            if act == 'Z':
                jax.lax.fori_loop(0, nb, zero, 0)
                acc_scr[S:, :] = jnp.zeros((acc_scr.shape[0] - S, M), F32)
                x_ref[S:, :] = jnp.zeros((x_ref.shape[0] - S, M), BF16)
                m_scr[...] = jnp.zeros(m_scr.shape, F32)
                flag_scr[...] = jnp.zeros(flag_scr.shape, F32)
                redo[0] = 0
            elif act == 'L':
                did.add('L')
                for cp in cp_late:
                    cp.start()
            elif act == 'M':
                assert arrived >= set('nm')
                mod = _dot(silu_cond(), wma_ref[...])
                mod_scr[:, 0:M] = mod[:, 0:M]
                mod_scr[:, M:2 * M] = 1.0 + mod[:, M:2 * M]
                did.add('M')
            else:
                act, _, span = act.partition('@')
                span = int(span or 0)
                items = []
                for r in [int(ch, 16) for ch in act[1:]]:
                    did.add((act[0], r))
                    if act[0] == 'K':
                        assert 'abcd'[r // CB] in arrived
                        kv_tile(jobs, r)
                    elif act[0] == 'H':
                        assert 'wxyz'[r // CB] in arrived and 'M' in did
                        items += [h_item(r, i, ('N', r) in did) for i in range(T // LP)]
                    elif act[0] == 'N':
                        assert 'wxyz'[r // CB] in arrived
                        items += [n_item(r, i) for i in range(T // LP)]
                    elif act[0] == 'Q':
                        assert all(('h', r, i) in did for i in range(T // LP))
                        q_tile(jobs, r)
                    elif act[0] == 'C':
                        assert all('abcd'[t[1] // CB] in arrived for p_ in _C_GROUPS[r] for t in p_[0])
                        items += sum_items(
                            32, _C_GROUPS[r], _C_SUMS, cs_scr,
                            lambda r_, k, rows: c_ref[r_ * T + rows.start:r_ * T + rows.stop, _tile(k)], False)
                    else:
                        assert act[0] == 'S' and all(('h', t[1], T // LP - 1) in did for p_ in _H_GROUPS[r] for t in p_[0])
                        items += h_sums(32 if span else 16, r)
                release(jobs, span, items)
        assert not jobs.side
    assert arrived == set(named) and all((k_, r) in did for k_ in 'KHQ' for r in range(nb))
    assert all((k_, r) in did for k_ in 'CS' for r in range(2)) and 'L' in did

    FH = ws3.shape[0] * T
    assert nattn - 1 >= FH // 64

    slices = ((w1_hbm, 32, 2 * T, 0), (w2_hbm, 32, 2 * T, 64), (w4_hbm, 64, FH, 128), (w3_hbm, T, FH, 256))
    slice_of = lambda g, n, half: jnp.minimum(g, half // n - 1)

    def prep_in(g):
        return [pltpu.make_async_copy(
            w.at[pl.ds(pl.multiple_of(slice_of(g, n, half) * n + x * half, n), n), 0:4 * T],
            st_in.at[r0 + x * n:r0 + (x + 1) * n, :], wsem.at[7]) for w, n, half, r0 in slices for x in range(2)]

    def mixer_prep(g):
        def blocks(r0, n, half, c0, c1, dep):
            get = lambda x, c: st_in[r0 + x * half:r0 + x * half + n, _tile(c)].astype(F32)
            return [_after(get(0, c0), _rows(dep, n)), get(0, c1), get(1, c0), _after(get(1, c1), _rows(dep, n))]

        def rows_item(dst, per, half, r0, c, o, n=16):
            def fn(dep):
                rows = pl.ds(pl.multiple_of(slice_of(g, per, half) * per, per) + o, n)
                for i, v in enumerate(_b_ops(*blocks(r0 + o, n, per, c, c + 2, dep))):
                    dst[i, c, rows, :] = v.astype(BF16)
            return fn

        def w3_item(k, i):
            def fn(dep):
                b11, b21, b12, b22 = blocks(slices[3][3], T, T, k, k + 2, dep)
                ws3[slice_of(g, T, FH), i, k] = _b_ops(b11, b12, b21, b22)[i].astype(BF16).T
            return fn

        return ([rows_item(dst, *sl[1:], c, o) for dst, sl in zip((ws12.at[0], ws12.at[1], ws4), slices)
                 for c in range(2) for o in range(0, sl[1], 16)]
                + [w3_item(k, i) for k in range(2) for i in range(7)])

    def next_copies(g):
        return pcopies(jnp.minimum(g + 1, nattn - 1)) + pcopies(jnp.minimum(g + 2, nattn - 1), probe, 4)

    def start_copies(g):
        for cp in next_copies(g) + prep_in(jnp.maximum(g, 0)):
            cp.start()

    def attn_body(g, exact):
        gw = jnp.maximum(g, 0)
        copies = next_copies(g)

        @pl.when(g >= 0)
        def _():
            pl.when(exact > 0)(lambda: _softmax_shifts(q_scr, k_scr, m_scr))
            bufs = (q_scr, k_scr, v_scr, m_scr, (pf_scr, vf_scr), wo_buf, acc_scr, flag_scr)
            _attention_step(*bufs, g >> 16)

        for cp in copies:
            cp.wait()
        pltpu.make_async_copy(st_in, st_in, wsem.at[7]).wait()

        @pl.when(g == -exact)
        def _():
            for fn in _gap_items(work, gap_scr):
                fn(None)

        @pl.when(g + 1 < nattn)
        def _():
            ocopy(g + 1).start()
            side = mixer_prep(gw) + _gap_items(probe, gap_scr)
            side = [(SD0 + i * SDS + (SDJ if i >= SDN else 0), fn) for i, fn in enumerate(side)]
            bufs = (h_scr, hs_scr, c_ref, cs_scr, wq_buf, wk_buf, wv_buf, q_scr, k_scr, v_scr)
            _proj_step(*bufs, scale, gap_scr, side)
            start_copies(g + 1)
            ocopy(g + 1).wait()

        return exact

    def attn_pass(exact, carry):
        @pl.when(jnp.logical_or(exact == 0, redo[0] > 0))
        def _():
            @pl.when(exact > 0)
            def _():
                jax.lax.fori_loop(0, nb, zero, 0)

            start_copies(-exact)
            jax.lax.fori_loop(-exact, nattn, attn_body, exact)

        @pl.when(exact == 0)
        def _():
            redo[0] = (jnp.max(flag_scr[...]) > 0).astype(jnp.int32)

        return carry

    jax.lax.fori_loop(0, 2, attn_pass, 0)

    for cp in cp_late:
        cp.wait()
    mod = _dot(silu_cond(), wmb_ref[...])
    mod_scr[:, 2 * M:4 * M] = mod[:, 0:2 * M]
    mod_scr[:, 4 * M:5 * M] = 1.0 + mod[:, 2 * M:3 * M]
    mod_scr[:, 5 * M:6 * M] = mod[:, 3 * M:4 * M]
    ftiles = [(f, min(f + T, Fd)) for f in range(0, Fd, T)]
    OFF = x_ref.shape[0] - S
    CAR = t_scr.shape[0] - RB

    def p1(r0, l0, n, dep=None):
        ga = mod_scr[:, 2 * M:3 * M]
        if dep is not None:
            ga = jnp.concatenate([_after(ga[:, 0:T], dep), ga[:, T:]], axis=1)
        rows = pl.ds(r0, n)
        x1 = x_ref[rows, :].astype(F32) + _rows(ga, n) * acc_scr[rows, :]
        xh_scr[0, l0:l0 + n, :] = x1
        hb = _ln(x1) * _rows(mod_scr[:, 4 * M:5 * M], n) + _rows(mod_scr[:, 3 * M:4 * M], n)
        xh_scr[1, l0:l0 + n, :] = hb
        return _ln(hb)

    HT = T // 2

    def p1_store(r0, c, dep=None):
        v = p1(r0 + c * PC, OFF + c * PC, PC, dep)
        a1_scr[c * PC:(c + 1) * PC, :] = v
        return jnp.max(v[:, M - T:].reshape(PC // 8, 8, T), axis=0)

    t_scr[RB:RB + CAR - OFF, :] = jnp.zeros((CAR - OFF, M), F32)
    t_scr[RB + CAR - OFF:RB + CAR, :] = _gelu(_dot(p1(0, 0, OFF).astype(BF16), w1_ref[...]))
    for c in range(RB // PC):
        p1_store(OFF, c)

    def out_copy(i):
        rows = pl.ds(i * T if isinstance(i, int) else pl.multiple_of(i * T, T), T)
        return pltpu.make_async_copy(out_buf.at[rows, :], out_hbm.at[rows, :], osem.at[i])

    def b_body(r, carry):
        gb = _rows(mod_scr[:, 5 * M:6 * M], T)
        r0 = pl.multiple_of(r * RB, RB)
        n0 = pl.multiple_of(jnp.minimum(r0 + RB, S - RB) + OFF, OFF)
        nh = RB // T
        now = [0]
        due = []
        pace = []

        def p1_item(c):
            return lambda dep: due.append((now[0] + PD, p1_store(n0, c, dep)))

        pace += [(P0 + i * PSTEP, p1_item(i)) for i in range(RB // PC)]
        wt = lambda ref, f0, f1, n: ref[f0:f1, _tile(n)]

        def mm(lhs, wts, dot=_dot):
            acc = None
            for x, w in zip(lhs, wts):
                if due and due[0][0] <= now[0]:
                    w = _tie(w, due.pop(0)[1])
                v = dot(x, w)
                now[0] += x.shape[0] // HT
                acc = v if acc is None else v + acc
                if pace and pace[0][0] <= now[0]:
                    pace.pop(0)[1](v[0:8, :])
            return acc

        def split_ops(lo, hi):
            return [v.astype(BF16) for v in _a_ops(lo[:HT], hi[:HT], lo[HT:], hi[HT:])]

        def two_tiles(aops, wsel, rest):
            def col(w):
                v = mm(rest[0], w, rest[3])
                return v[:HT], v[HT:]

            c11, c12, c21, c22 = _strassen(
                lambda i: mm([a[i] for a in aops], [wsel(i, k) for k in range(len(aops))]),
                lambda: col(rest[1]), lambda: col(rest[2]))
            return jnp.concatenate([c11, c21], axis=0), jnp.concatenate([c12, c22], axis=0)

        def square(full, aops, w_ref, ws_ref):
            out = {}
            for n in range(2):
                out[n], out[n + 2] = two_tiles(
                    aops, lambda i, k: _ld(ws_ref, i, n, slice(k * HT, (k + 1) * HT)),
                    (full[4:], [wt(w_ref, 4 * T, M, n)], [wt(w_ref, 4 * T, M, n + 2)], _dot))
            out[4] = mm(full, [wt(w_ref, j * T, (j + 1) * T, 4) for j in range(km)])
            return out

        t_scr[0:CAR, :] = t_scr[RB:RB + CAR, :]
        for hf in range(nh):
            a1 = [a1_scr[_tile(hf), _tile(j)] for j in range(km)]
            full = [v.astype(BF16) for v in a1]
            aops = [split_ops(a1[k], a1[2 + k]) for k in range(2)]
            for n, v in square(full, aops, w1_ref, ws12.at[0]).items():
                t = _gelu(v)
                if hf == nh - 1:
                    t = jnp.concatenate([t[:T - OFF], jnp.where(r < nrb - 1, t[T - OFF:], 0.0)], axis=0)
                t_scr[CAR + hf * T:CAR + (hf + 1) * T, _tile(n)] = t
        cq = M // 4
        shifts = (-1, 1, -2, 2)
        lane = jax.lax.broadcasted_iota(jnp.int32, (T, T), 1)
        y1, z, a3 = [], [], []
        for hf in range(nh):
            base = CAR - OFF + hf * T
            sh = []
            for j in range(km):
                g_lo, g_hi = (j * T) // cq, ((j + 1) * T - 1) // cq
                assert g_hi - g_lo <= 1
                v = t_scr[base + shifts[g_lo]:base + shifts[g_lo] + T, _tile(j)]
                if g_hi != g_lo:
                    v2 = t_scr[base + shifts[g_hi]:base + shifts[g_hi] + T, _tile(j)]
                    v = jnp.where(lane < g_hi * cq - j * T, v, v2)
                sh.append(v)
            hs = square([v.astype(BF16) for v in sh], [split_ops(sh[k], sh[2 + k]) for k in range(2)],
                        w2_ref, ws12.at[1])
            hs = jnp.concatenate([hs[n] for n in range(km)], axis=1)
            y1.append(hs + xh_scr[1, _tile(hf), :])
            z.append(xh_scr[0, _tile(hf), :] + gb * y1[hf])
            a3.append({})

            def ln_item(hf, c):
                def item(dep):
                    n = HT // NLN
                    for d in (0, HT):
                        v = y1[hf][d + c * n:d + (c + 1) * n]
                        if dep is not None:
                            v = jnp.concatenate([_after(v[:, :T], _rows(dep, n)), v[:, T:]], axis=1)
                        a3[hf][d + c * n] = _ln(v)
                return item

            ln_item(hf, 0)(None)
            pace += [(now[0] + LN0 + (c - 1) * LNS * (1 + hf), ln_item(hf, c)) for c in range(1, NLN)]
            pace.sort(key=lambda e: e[0])
        xh_scr[:, 0:OFF, :] = xh_scr[:, RB:RB + OFF, :]
        nf = FH // T
        h3, h3ops = [], []
        for hf in range(nh):
            assert len(a3[hf]) == 2 * NLN
            af = jnp.concatenate([a3[hf][key] for key in sorted(a3[hf])], axis=0)
            full = [af[:, _tile(j)].astype(BF16) for j in range(km)]
            aops = [split_ops(af[:, _tile(k)], af[:, _tile(2 + k)]) for k in range(2)]
            row, ops = {}, []
            narrow = None
            for n in range(nf):
                lo, hi = two_tiles(aops, lambda i, k: _ld(ws3, n, i, k),
                                   (full[4:], [wt(w3_ref, *ftiles[n], 4)],
                                    [wt(w3_ref, *ftiles[nf + n], 4)], _dot_nt))
                lo, hi = _gelu(lo), _gelu(hi)
                row[n], row[nf + n] = lo.astype(BF16), hi.astype(BF16)
                ops.append(split_ops(lo, hi))
                if n < km:
                    v = mm([wt(w3_ref, *ftiles[-1], n)], [full[n]], _dot_nt)
                    narrow = v if narrow is None else v + narrow
            row[2 * nf] = _gelu(mm(full, [wt(w3_ref, *ftiles[2 * nf], j) for j in range(km)],
                                   _dot_nt)).astype(BF16)
            fw = Fd - ftiles[-1][0]
            gT = jnp.concatenate([_gelu(narrow), jnp.zeros((T - fw, T), F32)], axis=0)
            row[2 * nf + 1] = _tie(gT.astype(BF16).T, gT[0:8, :])[:, :fw]
            h3.append([row[i] for i in range(len(ftiles))])
            h3ops.append(ops)
        for hf in range(nh):
            rows = pl.ds(pl.multiple_of(r0 + hf * T, T), T)

            def finish(n, v):
                out_buf[rows, _tile(n)] = (z[hf][:, _tile(n)] + gb[:, _tile(n)] * v).astype(out_buf.dtype)

            w4t = lambda n, f_: [wt(w4_ref, f0, f1, n) for f0, f1 in f_]
            finish(4, mm(h3[hf], w4t(4, ftiles)))
            for n in range(2):
                lo, hi = two_tiles(h3ops[hf], lambda i, k: _ld(ws4, i, n, slice(k * HT, (k + 1) * HT)),
                                   (h3[hf][2 * nf:], w4t(n, ftiles[2 * nf:]), w4t(n + 2, ftiles[2 * nf:]), _dot))
                finish(n, lo)
                finish(n + 2, hi)
            out_copy(r * nh + hf).start()
        assert not pace
        return carry

    jax.lax.fori_loop(0, nrb, b_body, 0)
    for i in range(nb):
        out_copy(i).wait()


@jax.jit
def pallas_adaLN_cond__compressed_kv_cla__mixer_s_mlp__prompt_kernel(
    A_x: jax.Array,
    A_c_kv: jax.Array,
    A_w_q: jax.Array,
    A_w_uk: jax.Array,
    A_w_uv: jax.Array,
    A_w_o: jax.Array,
    B_x: jax.Array,
    B_w1: jax.Array,
    B_w2: jax.Array,
    B_w3: jax.Array,
    B_w4: jax.Array,
    c: jax.Array,
    w_mod: jax.Array,
):
    _, S, M = A_x.shape
    Dc = A_c_kv.shape[2]
    H, D = A_w_q.shape[1], A_w_q.shape[2]
    Fd = B_w3.shape[1]
    assert D == T and A_c_kv.shape[1] == S and Dc == 4 * T and M == 5 * T and 13 * T < Fd < 14 * T and S == 16 * T
    vmem = pltpu.VMEM
    packed = lambda *lead: vmem(lead + (T, T), BF16)
    out = pl.pallas_call(
        _kernel,
        in_specs=[pl.BlockSpec(memory_space=pltpu.HBM)] * 12,
        out_specs=pl.BlockSpec(memory_space=pltpu.HBM),
        out_shape=jax.ShapeDtypeStruct((S, M), A_x.dtype),
        scratch_shapes=[
            vmem((S + 16, M), BF16),
            vmem((S, Dc), BF16),
            vmem((1, M), BF16),
            vmem((M, 2 * M), BF16),
            vmem((M, 4 * M), BF16),
            vmem((M, M), BF16),
            vmem((M, M), BF16),
            vmem((Fd, M), BF16),
            vmem((Fd, M), BF16),
            vmem((M, D), U32),
            vmem((Dc, D), U32),
            vmem((Dc, D), U32),
            vmem((2 * D, M), BF16),
            vmem((S, M), A_x.dtype),
            pltpu.SemaphoreType.DMA((15,)),
            pltpu.SemaphoreType.DMA((8,)),
            pltpu.SemaphoreType.DMA((S // T,)),
            vmem((8, 6 * M), F32),
            vmem((S // T, M // T, T, T), BF16),
            vmem((len(_C_SUMS), T, T), BF16),
            vmem((len(_H_SUMS), T, T), BF16),
            packed(2, M // T + 2 * (Dc // T)),
            packed(2 * S // T),
            packed(2 * S // T),
            packed(2 * S // T),
            vmem((S + 16, M), F32),
            vmem((S, M), F32),
            vmem((2, RB + 16, M), F32),
            vmem((RB, M), F32),
            vmem((RB + 32, M), F32),
            vmem((2, 7, 2, 2 * T, T), BF16),
            packed(6, 7, 2),
            vmem((7, 2, 6 * T, T), BF16),
            vmem((M, D), U32),
            vmem((Dc, D), U32),
            vmem((Dc, D), U32),
            vmem((3, 8, T), jnp.int32),
            vmem((4 * T, 4 * T), BF16),
            vmem((2 * S // T, 8, T), F32),
            vmem((_FENCE + 1, T, T), BF16),
            vmem((_FENCE + 1, T, T), BF16),
            vmem((8, T), F32),
            pltpu.SMEM((1,), jnp.int32),
        ],
        compiler_params=pltpu.CompilerParams(
            vmem_limit_bytes=100 * 1024 * 1024,
            disable_bounds_checks=True,
        ),
    )(
        A_x.reshape(S, M), A_c_kv.reshape(S, Dc),
        A_w_q, A_w_uk, A_w_uv,
        A_w_o.reshape(H // 2, 2 * D, M),
        B_w1, B_w2, B_w3.T, B_w4, c, w_mod,
    )
    return out.reshape(1, S, M)
```

```python
import functools
import math

import jax
import jax.numpy as jnp
import jax.experimental.pallas as pl
import jax.experimental.pallas.tpu as pltpu

F32 = jnp.float32
BF16 = jnp.bfloat16
U32 = jnp.uint32
NT = (((1,), (1,)), ((), ()))
T = 128
EPS = 1e-5
LOG2E = math.log2(math.e)

GRP = 4
LEAD = 10
PROW = 3
RES = 32
LAT_0 = 32
LAT_A = 16
LAT_B = 20
ALEAD = 32
SD0, SDS, SDN, SDJ = 20, 2, 20, 30
QT = 0
ONV, OEND = 0.5, 24
FPOS, DPOS = 0, 0
VF0, VFS = 4, 1.7
L_LO, L_HI, L_RATIO = 2.0 ** -24, 2.0 ** 24, 4.0
RB = 256
PC = 32
P0, PSTEP, PD = 440, 30, 52
NLN, LN0, LNS = 4, 4, 5
LP = 16
PROLOGUE = ('|kva|Z; |b|; kva|wc|K0123; bw|xdn|C0@56 N0123@52 K4567; cx|mq|N4567@52 F0@56 K89ab; '
            'd|y|C1@56 F1@56 Kcdef; nmq|zo|M H01 H234567@30 F2@36 Q0123; y||H89ab@30 F3@36 Q4567; '
            'zo||L Hcdef@30 Q89ab S01 Qcdef')


def _dot(a, b):
    return jnp.dot(a, b, preferred_element_type=F32)


def _dot_nt(a, b):
    return jax.lax.dot_general(a, b, NT, preferred_element_type=F32)


def _ln(x):
    m = jnp.mean(x, axis=-1, keepdims=True)
    xc = x - m
    v = jnp.mean(xc * xc, axis=-1, keepdims=True)
    return xc * jnp.exp2(jnp.log(v + EPS) * (-0.5 * LOG2E))


def _rows(v, n):
    return jnp.broadcast_to(v[None], (n // 8, 8, v.shape[1])).reshape(n, v.shape[1])


def _gelu(x):
    c0 = math.sqrt(2.0 / math.pi)
    return 0.5 * x * (1.0 + jnp.tanh(c0 * (x + 0.044715 * (x * x * x))))


def _after(x, dep):
    return jnp.where(dep > jnp.inf, dep, x)


def _tie(x, dep):
    xu = pltpu.bitcast(x, U32)
    first = jnp.where(dep > jnp.inf, jnp.uint32(0), xu[:8])
    return pltpu.bitcast(jnp.concatenate([first, xu[8:]], axis=0), BF16)


def _tile(j):
    return slice(j * T, (j + 1) * T)


def _ld(ref, *idx):
    return pltpu.bitcast(ref.bitcast(U32)[idx], BF16)


def _a_ops(a11, a12, a21, a22):
    return [a11 + a22, a21 + a22, a11, a22, a11 + a12, a21 - a11, a12 - a22]


def _b_ops(b11, b12, b21, b22):
    return [b11 + b22, b11, b12 - b22, b21 - b11, b22, b11 + b12, b21 + b22]


def _strassen(prod, col1=None, col2=None):
    m4 = prod(3)
    m2 = prod(1)
    c21 = m2 + m4
    if col1 is not None:
        e11, e21 = col1()
        m4, c21 = m4 + e11, c21 + e21
    m3 = prod(2)
    m5 = prod(4)
    c12 = m3 + m5
    if col2 is not None:
        e12, e22 = col2()
        c12, m3 = c12 + e12, m3 + e22
    m1 = prod(0)
    c11 = prod(6) + (m1 + (m4 - m5))
    c22 = prod(5) + (m1 + (m3 - m2))
    return c11, c12, c21, c22


def _group(rows, cols, pairs):
    xs, ys = dict.fromkeys(x for x, _ in pairs), dict.fromkeys(y for _, y in pairs)
    used = set(xs) | set(ys) | {(x[0], y[1]) for x, y in pairs} | {(y[0], x[1]) for x, y in pairs}
    prods = []
    for n, r in enumerate(rows):
        for i, k in [x for x in xs if x[0] == r]:
            mates = [y for x, y in pairs if x == (i, k)]
            prods.append((((1, i, k),) + tuple((1, i, k2) for _, k2 in mates), ((1, k, 0),),
                          ((1, i, 0), (-1, i, 1))))
            prods.append((((1, i, k),) + tuple((-1, i2, k) for i2, _ in mates), ((1, k, 0), (1, k, 1)),
                          ((1, i, 1),)))
        for i2, k2 in [y for y in ys if y[0] == r]:
            mates = [x for x, y in pairs if y == (i2, k2)]
            prods.append((((1, i2, k2),) + tuple((1, i2, k) for _, k in mates), ((1, k2, 1),),
                          ((1, i2, 1), (-1, i2, 0))))
            prods.append((((1, i2, k2),) + tuple((-1, i, k2) for i, _ in mates), ((1, k2, 0), (1, k2, 1)),
                          ((1, i2, 0),)))
        prods += [(((1, r, k),), ((1, k, h),), ((1, r, h),)) for k in cols if (r, k) not in used for h in (0, 1)]
        for (i, k), (i2, k2) in pairs:
            if r in (i, i2) and i + i2 - r in rows[n + 1:]:
                prods.append((((1, i, k2),), ((1, k2, 0), (-1, k, 0)), ((1, i2, 0), (1, i, 0))))
                prods.append((((1, i2, k), (1, i, k2)), ((1, k, 0), (1, k2, 1)), ((1, i2, 0), (1, i, 1))))
                prods.append((((1, i2, k),), ((1, k, 1), (-1, k2, 1)), ((1, i2, 1), (1, i, 1))))
    return prods


def _all_pairs(xrows, yrows):
    return [((x, a), (y, b)) for a, x in enumerate(xrows) for b, y in enumerate(yrows) if a != b]


_PAIRS65 = [((x[0] + 10, x[1]), (y[0] + 10, y[1])) for x, y in (
    ((0, 1), (1, 0)), ((0, 1), (5, 2)), ((2, 3), (1, 0)), ((2, 3), (3, 1)), ((2, 3), (5, 2)), ((3, 2), (1, 0)),
    ((4, 4), (0, 3)), ((4, 4), (1, 0)), ((4, 4), (3, 1)), ((4, 4), (5, 2)))]
_C_GROUPS = [_group(range(r, r + 8), range(4), _all_pairs(range(r, r + 4), range(r + 4, r + 8))) for r in (0, 8)]
_H_GROUPS = [_group(range(10), range(5), _all_pairs(range(5), range(5, 10))),
             _group(range(10, 16), range(5), _PAIRS65)]
_sum_index = lambda groups: {f: n for n, f in enumerate(
    dict.fromkeys(t[0] for g in groups for t in g if len(t[0]) > 1))}
_C_SUMS, _H_SUMS = _sum_index(_C_GROUPS), _sum_index(_H_GROUPS)


def _form(form, get):
    acc = None
    for sign, i, j in form:
        v = get(i, j)
        acc = v if acc is None else (acc + v if sign > 0 else acc - v)
    return acc


def _gap_items(bufs, gap_scr):
    items = []
    for n, buf in enumerate(bufs):
        acc = []

        def part(r0, buf=buf, acc=acc):
            def fn(dep):
                wu = jnp.concatenate([buf[r:r + 8, :] for r in range(r0, r0 + T, 32)])
                mask = jnp.full((8, T), 0x7FFF0000, U32)
                if dep is not None:
                    mask = jnp.where(dep > jnp.inf, jnp.uint32(0), mask)
                mask = _rows(mask, 32)
                new = [jnp.sum(pltpu.bitcast(v & mask, F32).reshape(4, 8, T), axis=0) for v in (wu << 16, wu)]
                acc[:] = [u + v for u, v in zip(acc, new)] if acc else new
            return fn

        def last(_, n=n, acc=acc):
            bits = []
            for v in acc:
                l1 = jnp.sum(jnp.sum(v, axis=1, keepdims=True), axis=0, keepdims=True)
                bits.append(pltpu.bitcast(jnp.broadcast_to(l1, (8, T)), jnp.int32) >> 8)
            gap_scr[n] = jnp.clip((bits[0] - bits[1] + (1 << 14)) >> 15, -8, 8) << 23

        items += [part(r0) for r0 in range(0, buf.shape[0], T)] + [last]
    return items


class _PairWeights:
    def __init__(self, w_ref, transpose=False, shift=None):
        self.base = {}
        if shift is not None:
            fac = _rows(pltpu.bitcast(0x3F800000 + shift, F32), T)
            self.inv = pltpu.bitcast(0x3F800000 - shift, F32)
        for j in range(w_ref.shape[0] // T):
            wu = w_ref[_tile(j), :]
            if transpose:
                wu = wu.T
            hi = pltpu.bitcast(wu & jnp.uint32(0xFFFF0000), F32)
            self.base[j, 0] = pltpu.bitcast(wu << 16, F32)
            self.base[j, 1] = hi if shift is None else hi * fac
        self.cache = {}

    def __call__(self, form):
        sign = 1
        if form[-1][0] < 0 and form[0][1:] > form[1][1:]:
            sign, form = -1, ((1,) + form[1][1:], (-1,) + form[0][1:])
        if form not in self.cache:
            self.cache[form] = _form(form, lambda k, h: self.base[k, h]).astype(BF16)
        return sign, self.cache[form]


def _run_group(jobs, prods, a_get, w, transposed, finish):
    left = {}
    for _, _, outs in prods:
        for _, i, h in outs:
            left[i, h] = left.get((i, h), 0) + 1
    acc = {}
    for af, bf, outs in prods:
        sign, wt = w(bf)
        m = jobs.mm([wt], [a_get(af)], _dot_nt) if transposed else jobs.mm([a_get(af)], [wt], _dot)
        for s_, i, h in outs:
            if (i, h) not in acc:
                acc[i, h] = (s_ * sign, m)
            else:
                s0, v = acc[i, h]
                acc[i, h] = (s0, v + m if s0 == s_ * sign else v - m) if s0 > 0 or s_ * sign < 0 else (1, m - v)
            left[i, h] -= 1
            if not left[i, h]:
                s0, v = acc.pop((i, h))
                assert s0 > 0
                finish(2 * i + h, v)


class _Jobs:
    def __init__(self, side=()):
        self.res = []
        self.side = list(side)

    def mm(self, lhs, wt, dot):
        acc = None
        for x, w in zip(lhs, wt):
            v = dot(x, w)
            self.res.append(v)
            acc = v if acc is None else v + acc
            rel = 4 * (len(self.res) % 4)
            while self.side and self.side[0][0] <= len(self.res):
                self.side.pop(0)[1](v[8 * rel:8 * rel + 8, :])
                rel = (rel + 2) % 16
        return acc


def _proj_step(h_scr, hs_scr, c_ref, cs_scr, wq_ref, wuk_ref, wuv_ref, q_scr, k_scr, v_scr, pf, scale, shifts, side):
    wk, wvT, wq = [_PairWeights(w, n == 1, shifts[n]) for n, w in enumerate((wuk_ref, wuv_ref, wq_ref))]
    c_get = lambda f: _ld(cs_scr, _C_SUMS[f]) if len(f) > 1 else c_ref[_tile(f[0][1]), _tile(f[0][2])]
    h_get = lambda f: _ld(hs_scr, _H_SUMS[f]) if len(f) > 1 else _ld(h_scr, f[0][1], f[0][2])

    def put(dst, w, mul=None):
        muls = [mul, _rows(w.inv if mul is None else w.inv * mul, T)]

        def fn(u, v):
            v = (v if muls[u % 2] is None else v * muls[u % 2]).astype(BF16)
            dst[u] = v.T if mul is not None and u < QT else v
        return fn

    jobs = _Jobs(side)
    put_v, stored = put(v_scr, wvT), set()
    nxt = [0]

    def fin_v(u, v):
        put_v(u, v)
        stored.add(u)
        for J in range(SB):
            if all(2 * (SB * J + k) + h in stored for k in range(SB) for h in range(2)) and ('J', J) not in stored:
                stored.add(('J', J))
                for fn in _v_form_items(v_scr, pf, J):
                    nxt[0] = max(nxt[0] + VFS, len(jobs.res) + VF0)
                    jobs.side.append((int(nxt[0]), fn))
                jobs.side.sort(key=lambda e: e[0])

    kk, vv, qq = ((c_get, wk, False, put(k_scr, wk)), (c_get, wvT, True, fin_v),
                  (h_get, wq, False, put(q_scr, wq, scale)))
    for prods, args in ((_C_GROUPS[0], kk), (_C_GROUPS[0], vv), (_C_GROUPS[1], vv), (_C_GROUPS[1], kk),
                        (_H_GROUPS[0], qq), (_H_GROUPS[1], qq)):
        _run_group(jobs, prods, *args)
    assert not jobs.side


def _inner_group(rows, cols, pairs):
    xs, ys = dict.fromkeys(x for x, _ in pairs), dict.fromkeys(y for _, y in pairs)
    used = set(xs) | set(ys) | {(x[0], y[1]) for x, y in pairs} | {(y[0], x[1]) for x, y in pairs}
    prods = []
    for i, j in xs:
        mates = [y for x, y in pairs if x == (i, j)]
        prods.append((((1, i, 0),), ((1, 0, j), (-1, 1, j)), ((1, i, j),) + tuple((1, i2, j) for i2, _ in mates)))
        prods.append((((1, i, 0), (1, i, 1)), ((1, 1, j),), ((1, i, j),) + tuple((-1, i, j2) for _, j2 in mates)))
    for i2, j2 in ys:
        mates = [x for x, y in pairs if y == (i2, j2)]
        prods.append((((1, i2, 0), (1, i2, 1)), ((1, 0, j2),),
                      ((1, i2, j2),) + tuple((-1, i2, j) for _, j in mates)))
        prods.append((((1, i2, 1),), ((1, 0, j2), (-1, 1, j2)),
                      ((-1, i2, j2),) + tuple((-1, i, j2) for i, _ in mates)))
    prods += [(((1, i, h),), ((1, h, j),), ((1, i, j),))
              for i in rows for j in cols if (i, j) not in used for h in (0, 1)]
    for (i, j), (i2, j2) in pairs:
        lo, hi = min(j, j2), max(j, j2)
        prods.append((((1, i2, 0), (-1, i, 0)), ((1, 0, lo), (1, 0, hi)), ((1, i2, j),)))
        prods.append((((1, i, 0), (1, i2, 1)), ((1, 0, j2), (1, 1, j)), ((1, i, j2), (1, i2, j))))
        prods.append((((1, i, 1), (-1, i2, 1)), ((1, 1, lo), (1, 1, hi)), ((1, i, j2),)))
    return prods


def _o_jobs():
    prods = (_inner_group(range(10), range(5), _all_pairs(range(0, 10, 2), range(1, 10, 2)))
             + _inner_group(range(10, 16), range(5), _PAIRS65))
    row = lambda t: max(i for _, i, _ in t[0])
    unit = lambda t: max(2 * i + h for _, i, h in t[0])
    need = lambda t: unit(t) if row(t) == 15 else 2 * row(t) + 1
    return [(need(t), t) for t in sorted(prods, key=need)]


_O_JOBS = _o_jobs()


SB = 4


class _Star:
    def __init__(self, ts):
        self.ts, self.n = ts, len(ts)
        rn = range(self.n)
        self.pairs = [(i, j) for i in rn for j in rn if i < j]
        self.pf = {f: m for m, f in enumerate([('R', i) for i in rn] + [('C', i) for i in rn]
                                              + [('S', i, j) for i in rn for j in rn if i != j]
                                              + [('A', i, j) for i, j in self.pairs])}
        self.vf = {f: m for m, f in enumerate([('W', i) for i in rn]
                                              + [(q, i, j) for i, j in self.pairs for q in ('Q1', 'Q2', 'Q3')])}
        self.pv = {**{('W', i): ('R', i) for i in rn}, **{('B', i): ('C', i) for i in rn},
                   **{('Q1', i, j): ('S', i, j) for i, j in self.pairs},
                   **{('Q2', i, j): ('A', i, j) for i, j in self.pairs},
                   **{('Q3', i, j): ('S', j, i) for i, j in self.pairs}}

    def products(self, i):
        return [('W', i), ('B', i)] + [(q, i, j) for j in range(i + 1, self.n) for q in ('Q1', 'Q2', 'Q3')]


_FULL = _Star((-1.125, -0.375, 0.375, 1.125))
_HALF = _Star((-0.75, 0.75))
_DCELLS = [(0, 0), (1, 0), (1, 1), (2, 2), (3, 2), (3, 3)]
_HSLOT = (SB - 1) * len(_FULL.pf)
_DSLOT = _HSLOT + len(_HALF.pf)
_VSLOT = _DSLOT + len(_DCELLS)
_VHALF = (SB - 1) * len(_FULL.vf)
_FENCE = _VSLOT + (_VHALF + SB * len(_HALF.vf) + 1) // 2


def _v_slot(star, J, f):
    m = star.vf[f] + J * len(star.vf) + (0 if star is _FULL else _VHALF)
    return _VSLOT + m // 2, m % 2 * (T // 2)


def _v_form_items(v_scr, pf, J):
    n, HT = 16, T // 2

    def item(star, h, r0, pairs):
        def fn(dep):
            ts = [jnp.full((8, T), t, F32) for t in star.ts]
            ts = [_rows(t if dep is None else _after(t, dep), n) for t in ts]

            def get(k, a):
                r = (a * HT + r0) // 2
                return _ld(v_scr, 2 * (SB * J + k) + h, slice(r, r + n // 2)).astype(F32)

            def put(f, v):
                slot, r = _v_slot(star, J, f)
                pf[h][slot, r + r0:r + r0 + n, :] = v.astype(BF16)

            b = {(k, a): get(k, a) for k in sorted({k for pr in pairs or star.pairs for k in pr})
                 for a in range(2)}
            if pairs is None or star.n == 2:
                w = [b[k, 0] + ts[k] * b[k, 1] for k in range(star.n)]
                for k in range(star.n):
                    put(('W', k), w[k])
                for i, j in star.pairs:
                    put(('Q2', i, j), w[i] - w[j])
            for i, j in pairs or ():
                d0, d1 = b[j, 0] - b[i, 0], b[j, 1] - b[i, 1]
                put(('Q1', i, j), d0 + ts[i] * d1)
                put(('Q3', i, j), d0 + ts[j] * d1)
        return fn

    pr = _FULL.pairs
    parts = [(_HALF, _HALF.pairs)]
    if J < SB - 1:
        parts += [(_FULL, x) for x in (None, pr[:2], [pr[2], pr[4]], [pr[3], pr[5]])]
    return [item(star, h, r0, pairs) for h in range(2) for r0 in range(0, HT, n) for star, pairs in parts]


def _job_order(nsb):
    units = [(I, h) for I in range(nsb) for h in range(2)]
    qe, qv = [], []
    for I, h in units:
        es = [('e', I, h, J, p) for J in range(I) for p in range(SB)]
        ds = [('d', I, h) + c for c in _DCELLS]
        es.insert(max(len(es) - FPOS, 0), ('f', I, h))
        qe += es + ds if I or FPOS < 9 else ds[:DPOS] + es + ds[DPOS:]
        for i in range(SB):
            qv += [('p', I, h, f, J) for f in _FULL.products(i) for J in range(I)]
            if i >= 2:
                qv += [('p', I, h, f, None) for f in _HALF.products(i - 2)]
            qv += [('v', I, h) + c for c in _DCELLS if c[0] == i]
    qo = [('o', u, j) for j, (u, _) in enumerate(_O_JOBS)]
    cost = dict(e=8, f=8, d=2, p=1, v=2, o=2)
    order, done = [], {}
    now = [0]

    def emit(q):
        job = q.pop(0)
        order.append(job)
        now[0] += cost[job[0]]
        if job[0] == 'd':
            done[job] = now[0]
        elif job[0] == 'v' and job[4] == job[3]:
            done['u', 2 * (SB * job[1] + job[3]) + job[2]] = now[0]
        return cost[job[0]]

    def v_ready():
        if not qv:
            return False
        key = ('d', qv[0][1], qv[0][2], SB - 1, SB - 1)
        return key in done and done[key] + (LAT_0 if qv[0][1:3] == (0, 0) else LAT_A) <= now[0]

    def o_ready():
        return bool(qo) and ('u', qo[0][1]) in done and done['u', qo[0][1]] + LAT_B <= now[0]

    def fill(nv, no):
        n = 0
        while nv > 0 or no > 0 or n % 4:
            if no > 0 and n % 2 == 0 and o_ready() and no * ONV >= nv:
                no -= 2
                n += emit(qo)
            elif v_ready() and (nv > 0 or n % 4):
                c = emit(qv)
                nv -= c
                n += c
            elif o_ready() and n % 2 == 0 and (no > 0 or n % 4 or nv > 0) and len(qo) > RES:
                no -= 2
                n += emit(qo)
            else:
                break

    while qe:
        unit = qe[0][1:3]
        while qv and qv[0][2] == unit[1] and qv[0][1] < unit[0]:
            emit(qv)
        ne = 0
        while qe and ne < 8 and (ne == 0 or (qe[0][0] == 'd' and qe[0][1:3] == unit and ne + 2 <= 8)):
            ne += emit(qe)
        groups = lambda q: sum(cost[j[0]] for j in q) / 8
        old = [j for j in qv if j[1:3] != unit and ('d', j[1], j[2], SB - 1, SB - 1) in done]
        here = [j for j in qe if j[1:3] == unit]
        rest = sum(cost[j[0]] for j in old)
        nv = (rest - LAT_A) / (groups(here) + 1) if here else rest
        no = 2 * max(len(qo) - RES - OEND, 0) / (groups(qe) + 1)
        fill(int(nv + 0.5), int(no + 0.5))
    while qv or qo:
        if qv and v_ready():
            fill(6, 2)
            if not qv:
                continue
        elif o_ready():
            emit(qo)
        else:
            emit(qv or qo)
    return order


def _attention_safe(q_scr, k_scr, v_scr, wo_ref, acc_scr):
    causal = (jax.lax.broadcasted_iota(jnp.int32, (T, T), 0)
              <= jax.lax.broadcasted_iota(jnp.int32, (T, T), 1))

    def unit(u, carry):
        r, hd = u // 2, u % 2

        def block(c, mlo):
            m0, l, o = mlo
            s = _dot_nt(_ld(k_scr, 2 * c + hd), _ld(q_scr, u))
            s = jnp.where(jnp.logical_or(causal, c < r), s, -1e9 * LOG2E)
            m = jnp.maximum(m0, jnp.max(s, axis=0, keepdims=True))
            a = jnp.exp2(m0 - m)
            p = jnp.exp2(s - m)
            return (m, l * a + jnp.sum(p, axis=0, keepdims=True),
                    o * a + _dot(_ld(v_scr, 2 * c + hd), p.astype(BF16)))

        _, l, o = jax.lax.fori_loop(0, r + 1, block, (jnp.full((1, T), -jnp.inf, F32), jnp.zeros((1, T), F32),
                                                      jnp.zeros((T, T), F32)))
        rows = pl.ds(pl.multiple_of(r * T, T), T)
        acc_scr[rows, :] += _dot((o * (1.0 / l)).astype(BF16).T, wo_ref[pl.ds(pl.multiple_of(hd * T, T), T), :])
        return carry

    jax.lax.fori_loop(0, q_scr.shape[0], unit, 0)


def _attention_step(q_scr, k_scr, v_scr, pf, wo_ref, acc_scr, flag_scr, z):
    causal = (jax.lax.broadcasted_iota(jnp.int32, (T, T), 0)
              <= jax.lax.broadcasted_iota(jnp.int32, (T, T), 1))
    HT = T // 2
    lsum, lrow, acc, fg, dacc, of, lhs = {}, {}, {}, {}, {}, {}, {}
    res = []
    wo, terms = {}, {}
    left = {}
    chk = [jnp.zeros((8, T), F32), None]
    for _, t in _O_JOBS:
        for _, i, j in t[2]:
            left[i, j] = left.get((i, j), 0) + 1

    def add_l(u, v):
        lsum[u] = v if u not in lsum else lsum[u] + v

    csign = {}

    def p_forms(star, h, slot0, g, tiles, cell, when):
        n = star.n

        def put(f, v):
            pf[h][slot0 + star.pf[f], 16 * g:16 * g + 16, :] = v.astype(BF16)

        for i in range(n):
            row = [cell(i, k) for k in sorted(range(n), key=lambda k: when(i, k))]
            r = functools.reduce(lambda x, y: x + y, row)
            put(('R', i), r)
            add_l(tiles[i], r[:8] + r[8:])
            col = sorted(range(n), key=lambda i2: (when(i2, i), i2 != i))
            sign = csign[n, i] = 1 if col[0] == i else -1
            c = cell(col[0], i)
            for i2 in col[1:]:
                c = c + cell(i2, i) if (1 if i2 == i else -1) == sign else c - cell(i2, i)
            put(('C', i), c)
            for j in range(n):
                if j != i:
                    put(('S', i, j), cell(i, j))
        for i, j in star.pairs:
            put(('A', i, j), cell(i, j) + cell(j, i))

    def scores(x, u):
        s = (_dot if u < QT else _dot_nt)(x, _ld(q_scr, u))
        res.append(s)
        return s

    def job_e(I, h, J, p):
        tiles = [2 * (SB * I + i) + h for i in range(SB)]
        ps = []
        for i, u in enumerate(tiles):
            x = jnp.concatenate([k_scr.bitcast(U32)[2 * (SB * J + (t - i) % SB) + h, 8 * g:8 * g + 8, :]
                                 for g in (2 * p, 2 * p + 1) for t in range(SB)], axis=0)
            ps.append(jnp.exp2(scores(pltpu.bitcast(x, BF16), u)))
        when = lambda i, k: (i + k) % SB
        for n, g in enumerate((2 * p, 2 * p + 1)):
            cell = lambda i, k: ps[i][16 * (SB * n + when(i, k)):16 * (SB * n + when(i, k)) + 16]
            p_forms(_FULL, h, J * len(_FULL.pf), g, tiles, cell, when)

    def job_f(I, h):
        tiles = [2 * (SB * I + 2 + i) + h for i in range(2)]
        ps = {(i, k): jnp.exp2(scores(_ld(k_scr, 2 * (SB * I + k) + h), u))
              for i, u in enumerate(tiles) for k in range(2)}
        for g in range(T // 16):
            p_forms(_HALF, h, _HSLOT, g, tiles, lambda i, k: ps[i, k][16 * g:16 * g + 16], lambda i, k: 0)

    def job_d(I, h, i, k):
        u = 2 * (SB * I + i) + h
        s = scores(_ld(k_scr, 2 * (SB * I + k) + h), u)
        if i == k:
            s = jnp.where(causal, s, -1e9 * LOG2E)
        p = jnp.exp2(s)
        add_l(u, jnp.sum(p.reshape(T // 8, 8, T), axis=0))
        pf[h][_DSLOT + _DCELLS.index((i, k))] = p.astype(BF16)
        if (i, k) == _DCELLS[-1]:
            pf[h][_FENCE + z, 0:16, :] = jnp.zeros((16, T), BF16)
            for u in [2 * (SB * I + a) + h for a in range(SB)]:
                lrow[u] = jnp.sum(lsum.pop(u), axis=0, keepdims=True)
            ls = [lrow[2 * (SB * I + a) + h] for a in range(SB)]
            lo = jnp.minimum(jnp.minimum(ls[0], ls[1]), jnp.minimum(ls[2], ls[3]))
            hi = jnp.maximum(jnp.maximum(ls[0], ls[1]), jnp.maximum(ls[2], ls[3]))
            ok = jnp.logical_and(lo >= L_LO, hi <= L_HI)
            ok = jnp.logical_and(ok, (hi if I else jnp.maximum(ls[2], ls[3]))
                                 <= L_RATIO * (lo if I else jnp.minimum(ls[2], ls[3])))
            bad = jnp.where(ok, 0.0, 1.0)
            chk[1] = bad if chk[1] is None else jnp.maximum(chk[1], bad)

    def job_p(I, h, f, J):
        star, last = (_HALF, True) if J is None else (_FULL, J == I - 1)
        blk = I if J is None else J
        if f[0] == 'B':
            x = _ld(v_scr, 2 * (SB * blk + f[1]) + h, slice(HT // 2, HT))
        else:
            slot, r = _v_slot(star, blk, f)
            x = _ld(pf[h], slot, slice(r // 2, (r + HT) // 2))
        v = _dot(x, _ld(pf[h], (_HSLOT if J is None else J * len(_FULL.pf)) + star.pf[star.pv[f]]))
        res.append(v)
        key = (star.n,) + f
        acc[key] = v if key not in acc else acc[key] + v
        if not last:
            return

        def add(which, i, v, sign=1):
            k_ = (star.n, which, i)
            if k_ not in fg:
                fg[k_] = v if sign > 0 else -v
            else:
                fg[k_] = fg[k_] + v if sign > 0 else fg[k_] - v

        if f[0] == 'W':
            add('F', f[1], acc.pop(key))
        elif f[0] == 'B':
            add('G', f[1], acc.pop(key), csign[star.n, f[1]])
        elif f[0] == 'Q3':
            _, i, j = f
            q1, q2, q3 = (acc.pop((star.n, q, i, j)) for q in ('Q1', 'Q2', 'Q3'))
            t = ((q1 + q2) + q3) * (1.0 / (star.ts[i] - star.ts[j]))
            add('G', i, t)
            add('G', j, t)
            add('F', i, q1)
            add('F', j, q3, -1)

    def job_v(I, h, i, k):
        u = 2 * (SB * I + i) + h
        v = _dot(_ld(v_scr, 2 * (SB * I + k) + h), _ld(pf[h], _DSLOT + _DCELLS.index((i, k))))
        res.append(v)
        dacc[u] = v if u not in dacc else dacc[u] + v
        if k == i:
            o = dacc.pop(u)
            for star, a in ([(_FULL, i)] if I else []) + ([(_HALF, i - 2)] if i >= 2 else []):
                f, g = fg.pop((star.n, 'F', a)), fg.pop((star.n, 'G', a))
                o = o + jnp.concatenate([f - star.ts[a] * g, g], axis=0)
            o = o * (1.0 / lrow[u])
            of[u] = o
            chk[0] = chk[0] + jnp.sum(o.reshape(T // 8, 8, T), axis=0)

    def job_o(_, n):
        af, bf, outs = _O_JOBS[n][1]
        if af not in lhs:
            v = _form(af, lambda i, h: of[2 * i + h])
            lhs[af] = _tie(v.astype(BF16).T, v[0:8, :])
        if bf not in wo:
            wo[bf] = (wo_ref[_tile(bf[0][1]), _tile(bf[0][2])] if len(bf) == 1 else
                      _form(bf, lambda h, j: wo_ref[_tile(h), _tile(j)].astype(F32)).astype(BF16))
        v = _dot(lhs[af], wo[bf])
        res.append(v)
        for sign, i, j in outs:
            terms.setdefault((i, j), []).append((sign, v))
            if len(terms[i, j]) == left[i, j]:
                tot = acc_scr[_tile(i), _tile(j)]
                for sg, m in terms.pop((i, j)):
                    tot = tot + m if sg > 0 else tot - m
                acc_scr[_tile(i), _tile(j)] = tot

    fns = dict(e=job_e, f=job_f, d=job_d, p=job_p, v=job_v, o=job_o)
    order = _job_order(q_scr.shape[0] // (2 * SB))
    for n, job in enumerate(order):
        assert job[0] not in 'efd' or not any(j[0] in 'pv' and j[2] == job[2] and j[1] < job[1] for j in order[n:])
    for job in order:
        fns[job[0]](*job[1:])
    fine = jnp.abs(chk[0]) < jnp.inf
    flag_scr[...] = jnp.maximum(flag_scr[...], jnp.where(fine, chk[1], 1.0))


def _kernel(x_hbm, c_hbm, wq_hbm, wuk_hbm, wuv_hbm, wo_hbm, w1_hbm, w2_hbm, w3_hbm, w4_hbm,
            cond_hbm, wmod_hbm, out_hbm,
            x_ref, c_ref, cond_ref, wma_ref, wmb_ref, w1_ref, w2_ref, w3_ref, w4_ref,
            wq_buf, wk_buf, wv_buf, wo_buf, out_buf, sem, wsem, osem,
            mod_scr, h_scr, cs_scr, hs_scr, w_scr, q_scr, k_scr, v_scr, acc_scr, xn_scr, xh_scr, a1_scr, t_scr,
            ws12, ws3, ws4, pq_buf, pk_buf, pv_buf, gap_scr, st_in, pf_scr, vf_scr, flag_scr, redo):
    S, M = x_hbm.shape
    D = wq_hbm.shape[2]
    nattn = wo_hbm.shape[0]
    Fd = w4_hbm.shape[0]
    scale = float(D) ** -0.5 * LOG2E
    nb, nrb = S // T, S // RB
    km, kc = M // T, c_hbm.shape[1] // T
    NX = 4
    XR = S // NX
    CB = XR // T

    work, probe = (wk_buf, wv_buf, wq_buf), (pk_buf, pv_buf, pq_buf)

    def pcopies(g, bufs=work, s0=0):
        return [pltpu.make_async_copy(src.bitcast(U32).at[:, g, :], dst, wsem.at[s0 + j])
                for j, (src, dst) in enumerate(zip((wuk_hbm, wuv_hbm, wq_hbm), bufs))]

    def ocopy(g):
        return pltpu.make_async_copy(wo_hbm.at[g], wo_buf, wsem.at[3])

    def chunk_copy(src, dst, i, s0):
        rows = slice(i * XR, (i + 1) * XR)
        return pltpu.make_async_copy(src.at[rows, :], dst.at[rows, :], sem.at[s0 + i])

    cp_cond = pltpu.make_async_copy(cond_hbm, cond_ref, sem.at[0])
    cp_wma = pltpu.make_async_copy(wmod_hbm.at[:, 0:2 * M], wma_ref, sem.at[1])
    cp_late = [pltpu.make_async_copy(src, dst, sem.at[2 + j]) for j, (src, dst) in enumerate((
        (wmod_hbm.at[:, 2 * M:6 * M], wmb_ref), (w1_hbm, w1_ref), (w2_hbm, w2_ref),
        (w3_hbm, w3_ref), (w4_hbm, w4_ref)))]
    cp_x = [chunk_copy(x_hbm, x_ref, i, 7) for i in range(NX)]
    cp_c = [chunk_copy(c_hbm, c_ref, i, 7 + NX) for i in range(NX)]

    def silu_cond():
        cf = cond_ref[...].astype(F32)
        return jnp.broadcast_to((cf * jax.nn.sigmoid(cf)).astype(BF16), (8, M))

    cp_wk, cp_wv, cp_wq = pcopies(0)
    named = dict(k=cp_wk, v=cp_wv, q=cp_wq, o=ocopy(0), n=cp_cond, m=cp_wma)
    named.update(zip('abcd', cp_c))
    named.update(zip('wxyz', cp_x))
    started, arrived, did = set(), set(), set()

    def zero(r, carry):
        acc_scr[pl.ds(pl.multiple_of(r * T, T), T), :] = jnp.zeros((T, M), F32)
        return carry

    def x_rows(rows, dep):
        xf = x_ref[rows, :].astype(F32)
        if dep is None:
            return xf
        return jnp.concatenate([_after(xf[:, :T], _rows(dep, xf.shape[0])), xf[:, T:]], axis=1)

    def n_item(r, i):
        def fn(dep):
            rows = slice(r * T + i * LP, r * T + (i + 1) * LP)
            xn_scr[rows, :] = _ln(x_rows(rows, dep))
        return fn

    def h_item(r, i, normed):
        def fn(dep):
            rows = slice(i * LP, (i + 1) * LP)
            grows = slice(r * T + i * LP, r * T + (i + 1) * LP)
            sa = mod_scr[:, 0:M]
            if normed and dep is not None:
                sa = jnp.concatenate([_after(sa[:, _tile(j)], dep) for j in range(km)], axis=1)
            hf = ((xn_scr[grows, :] if normed else _ln(x_rows(grows, dep))) * _rows(mod_scr[:, M:2 * M], LP)
                  + _rows(sa, LP))
            for j in range(km):
                h_scr[r, j, rows, :] = hf[:, _tile(j)].astype(BF16)
            for f, n in _H_SUMS.items():
                if all(t[1] == r for t in f):
                    hs_scr[n, rows, :] = _form(f, lambda _, k: hf[:, _tile(k)]).astype(BF16)
            did.add(('h', r, i))
        return fn

    def release(jobs, span, items):
        if span and items:
            jobs.side += [(len(jobs.res) + 1 + i * span // len(items), fn) for i, fn in enumerate(items)]
            jobs.side.sort(key=lambda e: e[0])
        else:
            for fn in items:
                fn(None)

    def sum_items(n, group, index, dst, get, skip_rows):
        forms = [f for f in dict.fromkeys(t[0] for t in group)
                 if len(f) > 1 and not (skip_rows and len({t[1] for t in f}) == 1)]

        def item(f, rows):
            def fn(dep):
                def term(r, k):
                    v = get(r, k, rows).astype(F32)
                    return v if dep is None or (r, k) != f[0][1:] else _after(v, _rows(dep, v.shape[0]))
                dst[index[f], rows, :] = _form(f, term).astype(BF16)
            return fn

        return [item(f, slice(i, i + n)) for i in range(0, T, n) for f in forms]

    h_sums = lambda n, gi: sum_items(n, _H_GROUPS[gi], _H_SUMS, hs_scr,
                                     lambda r_, k, rows: h_scr[r_, k, rows, :], True)

    def stash(key, buf, j0, transpose=False):
        n = buf.shape[0] // T
        if key not in did:
            assert key in arrived
            did.add(key)
            w = _PairWeights(buf, transpose)
            for j in range(n):
                for hd in range(2):
                    w_scr[hd, j0 + j] = w(((1, j, hd),))[1]
        return lambda hd: [_ld(w_scr, hd, j0 + j) for j in range(n)]

    def kv_tile(jobs, r):
        wk, wvT = stash('k', wk_buf, 0), stash('v', wv_buf, kc, True)
        ct = [c_ref[_tile(r), _tile(j)] for j in range(kc)]
        for hd in range(2):
            k_scr[2 * r + hd] = jobs.mm(ct, wk(hd), _dot).astype(BF16)
        for hd in range(2):
            v_scr[2 * r + hd] = jobs.mm(wvT(hd), ct, _dot_nt).astype(BF16)

    def q_tile(jobs, r):
        wq = stash('q', wq_buf, 2 * kc)
        ht = [_ld(h_scr, r, j) for j in range(km)]
        for hd in range(2):
            v = (jobs.mm(ht, wq(hd), _dot) * scale).astype(BF16)
            q_scr[2 * r + hd] = v.T if 2 * r + hd < QT else v

    for blk in PROLOGUE.split(';'):
        waits, starts, acts = blk.split('|')
        for ch in waits.strip():
            assert ch in started and ch not in arrived
            arrived.add(ch)
            named[ch].wait()
        for ch in starts.strip():
            assert ch not in started
            started.add(ch)
            named[ch].start()
        jobs = _Jobs()
        for act in acts.split():
            if act == 'Z':
                jax.lax.fori_loop(0, nb, zero, 0)
                acc_scr[S:, :] = jnp.zeros((acc_scr.shape[0] - S, M), F32)
                x_ref[S:, :] = jnp.zeros((x_ref.shape[0] - S, M), BF16)
                flag_scr[...] = jnp.zeros(flag_scr.shape, F32)
                redo[0] = 0
            elif act == 'L':
                did.add('L')
                for cp in cp_late:
                    cp.start()
            elif act == 'M':
                assert arrived >= set('nm')
                mod = _dot(silu_cond(), wma_ref[...])
                mod_scr[:, 0:M] = mod[:, 0:M]
                mod_scr[:, M:2 * M] = 1.0 + mod[:, M:2 * M]
                did.add('M')
            else:
                act, _, span = act.partition('@')
                span = int(span or 0)
                items = []
                for r in [int(ch, 16) for ch in act[1:]]:
                    did.add((act[0], r))
                    if act[0] == 'K':
                        assert 'abcd'[r // CB] in arrived
                        kv_tile(jobs, r)
                    elif act[0] == 'H':
                        assert 'wxyz'[r // CB] in arrived and 'M' in did
                        items += [h_item(r, i, ('N', r) in did) for i in range(T // LP)]
                    elif act[0] == 'N':
                        assert 'wxyz'[r // CB] in arrived
                        items += [n_item(r, i) for i in range(T // LP)]
                    elif act[0] == 'Q':
                        assert all(('h', r, i) in did for i in range(T // LP))
                        q_tile(jobs, r)
                    elif act[0] == 'F':
                        assert all(('K', SB * r + k_) in did for k_ in range(SB))
                        items += _v_form_items(v_scr, (pf_scr, vf_scr), r)
                    elif act[0] == 'C':
                        assert all('abcd'[t[1] // CB] in arrived for p_ in _C_GROUPS[r] for t in p_[0])
                        items += sum_items(
                            32, _C_GROUPS[r], _C_SUMS, cs_scr,
                            lambda r_, k, rows: c_ref[r_ * T + rows.start:r_ * T + rows.stop, _tile(k)], False)
                    else:
                        assert act[0] == 'S' and all(('h', t[1], T // LP - 1) in did for p_ in _H_GROUPS[r] for t in p_[0])
                        items += h_sums(32 if span else 16, r)
                release(jobs, span, items)
        assert not jobs.side
    assert arrived == set(named) and all((k_, r) in did for k_ in 'KHQ' for r in range(nb))
    assert all((k_, r) in did for k_ in 'CS' for r in range(2)) and 'L' in did
    assert all(('F', r) in did for r in range(SB))

    FH = ws3.shape[0] * T
    assert nattn - 1 >= FH // 64

    slices = ((w1_hbm, 32, 2 * T, 0), (w2_hbm, 32, 2 * T, 64), (w4_hbm, 64, FH, 128), (w3_hbm, T, FH, 256))
    slice_of = lambda g, n, half: jnp.minimum(g, half // n - 1)

    def prep_in(g):
        return [pltpu.make_async_copy(
            w.at[pl.ds(pl.multiple_of(slice_of(g, n, half) * n + x * half, n), n), 0:4 * T],
            st_in.at[r0 + x * n:r0 + (x + 1) * n, :], wsem.at[7]) for w, n, half, r0 in slices for x in range(2)]

    def mixer_prep(g):
        def blocks(r0, n, half, c0, c1, dep):
            get = lambda x, c: st_in[r0 + x * half:r0 + x * half + n, _tile(c)].astype(F32)
            return [_after(get(0, c0), _rows(dep, n)), get(0, c1), get(1, c0), _after(get(1, c1), _rows(dep, n))]

        def rows_item(dst, per, half, r0, c, o, n=16):
            def fn(dep):
                rows = pl.ds(pl.multiple_of(slice_of(g, per, half) * per, per) + o, n)
                for i, v in enumerate(_b_ops(*blocks(r0 + o, n, per, c, c + 2, dep))):
                    dst[i, c, rows, :] = v.astype(BF16)
            return fn

        def w3_item(k, i):
            def fn(dep):
                b11, b21, b12, b22 = blocks(slices[3][3], T, T, k, k + 2, dep)
                ws3[slice_of(g, T, FH), i, k] = _b_ops(b11, b12, b21, b22)[i].astype(BF16).T
            return fn

        return ([rows_item(dst, *sl[1:], c, o) for dst, sl in zip((ws12.at[0], ws12.at[1], ws4), slices)
                 for c in range(2) for o in range(0, sl[1], 16)]
                + [w3_item(k, i) for k in range(2) for i in range(7)])

    def next_copies(g):
        return pcopies(jnp.minimum(g + 1, nattn - 1)) + pcopies(jnp.minimum(g + 2, nattn - 1), probe, 4)

    def start_copies(g):
        for cp in next_copies(g) + prep_in(jnp.maximum(g, 0)):
            cp.start()

    def attn_body(g, exact):
        gw = jnp.maximum(g, 0)
        copies = next_copies(g)

        @pl.when(exact == 0)
        def _():
            bufs = (q_scr, k_scr, v_scr, (pf_scr, vf_scr), wo_buf, acc_scr, flag_scr)
            _attention_step(*bufs, g >> 16)

        @pl.when(jnp.logical_and(exact > 0, g >= 0))
        def _():
            _attention_safe(q_scr, k_scr, v_scr, wo_buf, acc_scr)

        for cp in copies:
            cp.wait()
        pltpu.make_async_copy(st_in, st_in, wsem.at[7]).wait()

        @pl.when(g == -exact)
        def _():
            for fn in _gap_items(work, gap_scr):
                fn(None)

        @pl.when(g + 1 < nattn)
        def _():
            ocopy(g + 1).start()
            side = mixer_prep(gw) + _gap_items(probe, gap_scr)
            side = [(SD0 + i * SDS + (SDJ if i >= SDN else 0), fn) for i, fn in enumerate(side)]
            bufs = (h_scr, hs_scr, c_ref, cs_scr, wq_buf, wk_buf, wv_buf, q_scr, k_scr, v_scr, (pf_scr, vf_scr))
            _proj_step(*bufs, scale, gap_scr, side)
            start_copies(g + 1)
            ocopy(g + 1).wait()

        return exact

    def attn_pass(exact, carry):
        @pl.when(jnp.logical_or(exact == 0, redo[0] > 0))
        def _():
            @pl.when(exact > 0)
            def _():
                jax.lax.fori_loop(0, nb, zero, 0)

            start_copies(-exact)
            jax.lax.fori_loop(-exact, nattn, attn_body, exact)

        @pl.when(exact == 0)
        def _():
            redo[0] = (jnp.max(flag_scr[...]) > 0).astype(jnp.int32)

        return carry

    jax.lax.fori_loop(0, 2, attn_pass, 0)

    for cp in cp_late:
        cp.wait()
    mod = _dot(silu_cond(), wmb_ref[...])
    mod_scr[:, 2 * M:4 * M] = mod[:, 0:2 * M]
    mod_scr[:, 4 * M:5 * M] = 1.0 + mod[:, 2 * M:3 * M]
    mod_scr[:, 5 * M:6 * M] = mod[:, 3 * M:4 * M]
    ftiles = [(f, min(f + T, Fd)) for f in range(0, Fd, T)]
    OFF = x_ref.shape[0] - S
    CAR = t_scr.shape[0] - RB

    def p1(r0, l0, n, dep=None):
        ga = mod_scr[:, 2 * M:3 * M]
        if dep is not None:
            ga = jnp.concatenate([_after(ga[:, 0:T], dep), ga[:, T:]], axis=1)
        rows = pl.ds(r0, n)
        x1 = x_ref[rows, :].astype(F32) + _rows(ga, n) * acc_scr[rows, :]
        xh_scr[0, l0:l0 + n, :] = x1
        hb = _ln(x1) * _rows(mod_scr[:, 4 * M:5 * M], n) + _rows(mod_scr[:, 3 * M:4 * M], n)
        xh_scr[1, l0:l0 + n, :] = hb
        return _ln(hb)

    HT = T // 2

    def p1_store(r0, c, dep=None):
        v = p1(r0 + c * PC, OFF + c * PC, PC, dep)
        a1_scr[c * PC:(c + 1) * PC, :] = v
        return jnp.max(v[:, M - T:].reshape(PC // 8, 8, T), axis=0)

    t_scr[RB:RB + CAR - OFF, :] = jnp.zeros((CAR - OFF, M), F32)
    t_scr[RB + CAR - OFF:RB + CAR, :] = _gelu(_dot(p1(0, 0, OFF).astype(BF16), w1_ref[...]))
    for c in range(RB // PC):
        p1_store(OFF, c)

    def out_copy(i):
        rows = pl.ds(i * T if isinstance(i, int) else pl.multiple_of(i * T, T), T)
        return pltpu.make_async_copy(out_buf.at[rows, :], out_hbm.at[rows, :], osem.at[i])

    def b_body(r, carry):
        gb = _rows(mod_scr[:, 5 * M:6 * M], T)
        r0 = pl.multiple_of(r * RB, RB)
        n0 = pl.multiple_of(jnp.minimum(r0 + RB, S - RB) + OFF, OFF)
        nh = RB // T
        now = [0]
        due = []
        pace = []

        def p1_item(c):
            return lambda dep: due.append((now[0] + PD, p1_store(n0, c, dep)))

        pace += [(P0 + i * PSTEP, p1_item(i)) for i in range(RB // PC)]
        wt = lambda ref, f0, f1, n: ref[f0:f1, _tile(n)]

        def mm(lhs, wts, dot=_dot):
            acc = None
            for x, w in zip(lhs, wts):
                if due and due[0][0] <= now[0]:
                    w = _tie(w, due.pop(0)[1])
                v = dot(x, w)
                now[0] += x.shape[0] // HT
                acc = v if acc is None else v + acc
                if pace and pace[0][0] <= now[0]:
                    pace.pop(0)[1](v[0:8, :])
            return acc

        def split_ops(lo, hi):
            return [v.astype(BF16) for v in _a_ops(lo[:HT], hi[:HT], lo[HT:], hi[HT:])]

        def two_tiles(aops, wsel, rest):
            def col(w):
                v = mm(rest[0], w, rest[3])
                return v[:HT], v[HT:]

            c11, c12, c21, c22 = _strassen(
                lambda i: mm([a[i] for a in aops], [wsel(i, k) for k in range(len(aops))]),
                lambda: col(rest[1]), lambda: col(rest[2]))
            return jnp.concatenate([c11, c21], axis=0), jnp.concatenate([c12, c22], axis=0)

        def square(full, aops, w_ref, ws_ref):
            out = {}
            for n in range(2):
                out[n], out[n + 2] = two_tiles(
                    aops, lambda i, k: _ld(ws_ref, i, n, slice(k * HT, (k + 1) * HT)),
                    (full[4:], [wt(w_ref, 4 * T, M, n)], [wt(w_ref, 4 * T, M, n + 2)], _dot))
            out[4] = mm(full, [wt(w_ref, j * T, (j + 1) * T, 4) for j in range(km)])
            return out

        t_scr[0:CAR, :] = t_scr[RB:RB + CAR, :]
        for hf in range(nh):
            a1 = [a1_scr[_tile(hf), _tile(j)] for j in range(km)]
            full = [v.astype(BF16) for v in a1]
            aops = [split_ops(a1[k], a1[2 + k]) for k in range(2)]
            for n, v in square(full, aops, w1_ref, ws12.at[0]).items():
                t = _gelu(v)
                if hf == nh - 1:
                    t = jnp.concatenate([t[:T - OFF], jnp.where(r < nrb - 1, t[T - OFF:], 0.0)], axis=0)
                t_scr[CAR + hf * T:CAR + (hf + 1) * T, _tile(n)] = t
        cq = M // 4
        shifts = (-1, 1, -2, 2)
        lane = jax.lax.broadcasted_iota(jnp.int32, (T, T), 1)
        y1, z, a3 = [], [], []
        for hf in range(nh):
            base = CAR - OFF + hf * T
            sh = []
            for j in range(km):
                g_lo, g_hi = (j * T) // cq, ((j + 1) * T - 1) // cq
                assert g_hi - g_lo <= 1
                v = t_scr[base + shifts[g_lo]:base + shifts[g_lo] + T, _tile(j)]
                if g_hi != g_lo:
                    v2 = t_scr[base + shifts[g_hi]:base + shifts[g_hi] + T, _tile(j)]
                    v = jnp.where(lane < g_hi * cq - j * T, v, v2)
                sh.append(v)
            hs = square([v.astype(BF16) for v in sh], [split_ops(sh[k], sh[2 + k]) for k in range(2)],
                        w2_ref, ws12.at[1])
            hs = jnp.concatenate([hs[n] for n in range(km)], axis=1)
            y1.append(hs + xh_scr[1, _tile(hf), :])
            z.append(xh_scr[0, _tile(hf), :] + gb * y1[hf])
            a3.append({})

            def ln_item(hf, c):
                def item(dep):
                    n = HT // NLN
                    for d in (0, HT):
                        v = y1[hf][d + c * n:d + (c + 1) * n]
                        if dep is not None:
                            v = jnp.concatenate([_after(v[:, :T], _rows(dep, n)), v[:, T:]], axis=1)
                        a3[hf][d + c * n] = _ln(v)
                return item

            ln_item(hf, 0)(None)
            pace += [(now[0] + LN0 + (c - 1) * LNS * (1 + hf), ln_item(hf, c)) for c in range(1, NLN)]
            pace.sort(key=lambda e: e[0])
        xh_scr[:, 0:OFF, :] = xh_scr[:, RB:RB + OFF, :]
        nf = FH // T
        h3, h3ops = [], []
        for hf in range(nh):
            assert len(a3[hf]) == 2 * NLN
            af = jnp.concatenate([a3[hf][key] for key in sorted(a3[hf])], axis=0)
            full = [af[:, _tile(j)].astype(BF16) for j in range(km)]
            aops = [split_ops(af[:, _tile(k)], af[:, _tile(2 + k)]) for k in range(2)]
            row, ops = {}, []
            narrow = None
            for n in range(nf):
                lo, hi = two_tiles(aops, lambda i, k: _ld(ws3, n, i, k),
                                   (full[4:], [wt(w3_ref, *ftiles[n], 4)],
                                    [wt(w3_ref, *ftiles[nf + n], 4)], _dot_nt))
                lo, hi = _gelu(lo), _gelu(hi)
                row[n], row[nf + n] = lo.astype(BF16), hi.astype(BF16)
                ops.append(split_ops(lo, hi))
                if n < km:
                    v = mm([wt(w3_ref, *ftiles[-1], n)], [full[n]], _dot_nt)
                    narrow = v if narrow is None else v + narrow
            row[2 * nf] = _gelu(mm(full, [wt(w3_ref, *ftiles[2 * nf], j) for j in range(km)],
                                   _dot_nt)).astype(BF16)
            fw = Fd - ftiles[-1][0]
            gT = jnp.concatenate([_gelu(narrow), jnp.zeros((T - fw, T), F32)], axis=0)
            row[2 * nf + 1] = _tie(gT.astype(BF16).T, gT[0:8, :])[:, :fw]
            h3.append([row[i] for i in range(len(ftiles))])
            h3ops.append(ops)
        for hf in range(nh):
            rows = pl.ds(pl.multiple_of(r0 + hf * T, T), T)

            def finish(n, v):
                out_buf[rows, _tile(n)] = (z[hf][:, _tile(n)] + gb[:, _tile(n)] * v).astype(out_buf.dtype)

            w4t = lambda n, f_: [wt(w4_ref, f0, f1, n) for f0, f1 in f_]
            finish(4, mm(h3[hf], w4t(4, ftiles)))
            for n in range(2):
                lo, hi = two_tiles(h3ops[hf], lambda i, k: _ld(ws4, i, n, slice(k * HT, (k + 1) * HT)),
                                   (h3[hf][2 * nf:], w4t(n, ftiles[2 * nf:]), w4t(n + 2, ftiles[2 * nf:]), _dot))
                finish(n, lo)
                finish(n + 2, hi)
            out_copy(r * nh + hf).start()
        assert not pace
        return carry

    jax.lax.fori_loop(0, nrb, b_body, 0)
    for i in range(nb):
        out_copy(i).wait()


@jax.jit
def pallas_adaLN_cond__compressed_kv_cla__mixer_s_mlp__prompt_kernel(
    A_x: jax.Array,
    A_c_kv: jax.Array,
    A_w_q: jax.Array,
    A_w_uk: jax.Array,
    A_w_uv: jax.Array,
    A_w_o: jax.Array,
    B_x: jax.Array,
    B_w1: jax.Array,
    B_w2: jax.Array,
    B_w3: jax.Array,
    B_w4: jax.Array,
    c: jax.Array,
    w_mod: jax.Array,
):
    _, S, M = A_x.shape
    Dc = A_c_kv.shape[2]
    H, D = A_w_q.shape[1], A_w_q.shape[2]
    Fd = B_w3.shape[1]
    assert D == T and A_c_kv.shape[1] == S and Dc == 4 * T and M == 5 * T and 13 * T < Fd < 14 * T and S == 16 * T
    vmem = pltpu.VMEM
    packed = lambda *lead: vmem(lead + (T, T), BF16)
    out = pl.pallas_call(
        _kernel,
        in_specs=[pl.BlockSpec(memory_space=pltpu.HBM)] * 12,
        out_specs=pl.BlockSpec(memory_space=pltpu.HBM),
        out_shape=jax.ShapeDtypeStruct((S, M), A_x.dtype),
        scratch_shapes=[
            vmem((S + 16, M), BF16),
            vmem((S, Dc), BF16),
            vmem((1, M), BF16),
            vmem((M, 2 * M), BF16),
            vmem((M, 4 * M), BF16),
            vmem((M, M), BF16),
            vmem((M, M), BF16),
            vmem((Fd, M), BF16),
            vmem((Fd, M), BF16),
            vmem((M, D), U32),
            vmem((Dc, D), U32),
            vmem((Dc, D), U32),
            vmem((2 * D, M), BF16),
            vmem((S, M), A_x.dtype),
            pltpu.SemaphoreType.DMA((15,)),
            pltpu.SemaphoreType.DMA((8,)),
            pltpu.SemaphoreType.DMA((S // T,)),
            vmem((8, 6 * M), F32),
            vmem((S // T, M // T, T, T), BF16),
            vmem((len(_C_SUMS), T, T), BF16),
            vmem((len(_H_SUMS), T, T), BF16),
            packed(2, M // T + 2 * (Dc // T)),
            packed(2 * S // T),
            packed(2 * S // T),
            packed(2 * S // T),
            vmem((S + 16, M), F32),
            vmem((S, M), F32),
            vmem((2, RB + 16, M), F32),
            vmem((RB, M), F32),
            vmem((RB + 32, M), F32),
            vmem((2, 7, 2, 2 * T, T), BF16),
            packed(6, 7, 2),
            vmem((7, 2, 6 * T, T), BF16),
            vmem((M, D), U32),
            vmem((Dc, D), U32),
            vmem((Dc, D), U32),
            vmem((3, 8, T), jnp.int32),
            vmem((4 * T, 4 * T), BF16),
            vmem((_FENCE + 1, T, T), BF16),
            vmem((_FENCE + 1, T, T), BF16),
            vmem((8, T), F32),
            pltpu.SMEM((1,), jnp.int32),
        ],
        compiler_params=pltpu.CompilerParams(
            vmem_limit_bytes=100 * 1024 * 1024,
            disable_bounds_checks=True,
        ),
    )(
        A_x.reshape(S, M), A_c_kv.reshape(S, Dc),
        A_w_q, A_w_uk, A_w_uv,
        A_w_o.reshape(H // 2, 2 * D, M),
        B_w1, B_w2, B_w3.T, B_w4, c, w_mod,
    )
    return out.reshape(1, S, M)
```

```python
import functools
import math

import jax
import jax.numpy as jnp
import jax.experimental.pallas as pl
import jax.experimental.pallas.tpu as pltpu

F32 = jnp.float32
BF16 = jnp.bfloat16
U32 = jnp.uint32
NT = (((1,), (1,)), ((), ()))
T = 128
EPS = 1e-5
LOG2E = math.log2(math.e)

GRP = 4
LEAD = 10
PROW = 3
RES = 32
LAT_0 = 32
LAT_A = 16
LAT_B = 20
ALEAD = 32
SD0, SDS, SDN, SDJ = 20, 2, 20, 30
QT = 0
ONV, OEND = 0.5, 24
FPOS, DPOS = 0, 0
VF0, VFS = 4, 1.7
L_LO, L_HI, L_RATIO = 2.0 ** -24, 2.0 ** 24, 4.0
RB = 256
PC = 32
P0, PSTEP, PD = 440, 30, 52
NLN, LN0, LNS = 4, 4, 5
LP = 16
SP0, SP1 = 76, 38
_prologue = lambda: ('|kva|Z; |b|; kva|wc|K0123; bw|xdn|C0@56 N0123@52 K4567; cx|mq|N4567@52 F0@56 K89ab; '
            'd|y|C1@56 F1@56 Kcdef; nmq|zo|M H01 H234567@30 F2@36 Q0123; y||H89ab@30 F3@36 Q4567; '
            'zo||L Hcdef@30 S0@%d Q89ab S1@%d Qcdef' % (SP0, SP1))


def _dot(a, b):
    return jnp.dot(a, b, preferred_element_type=F32)


def _dot_nt(a, b):
    return jax.lax.dot_general(a, b, NT, preferred_element_type=F32)


def _ln(x):
    m = jnp.mean(x, axis=-1, keepdims=True)
    xc = x - m
    v = jnp.mean(xc * xc, axis=-1, keepdims=True)
    return xc * jnp.exp2(jnp.log(v + EPS) * (-0.5 * LOG2E))


def _rows(v, n):
    return jnp.broadcast_to(v[None], (n // 8, 8, v.shape[1])).reshape(n, v.shape[1])


def _gelu(x):
    c0 = math.sqrt(2.0 / math.pi)
    return 0.5 * x * (1.0 + jnp.tanh(c0 * (x + 0.044715 * (x * x * x))))


def _after(x, dep):
    return jnp.where(dep > jnp.inf, dep, x)


def _tie(x, dep):
    xu = pltpu.bitcast(x, U32)
    first = jnp.where(dep > jnp.inf, jnp.uint32(0), xu[:8])
    return pltpu.bitcast(jnp.concatenate([first, xu[8:]], axis=0), BF16)


def _tile(j):
    return slice(j * T, (j + 1) * T)


def _ld(ref, *idx):
    return pltpu.bitcast(ref.bitcast(U32)[idx], BF16)


def _a_ops(a11, a12, a21, a22):
    return [a11 + a22, a21 + a22, a11, a22, a11 + a12, a21 - a11, a12 - a22]


def _b_ops(b11, b12, b21, b22):
    return [b11 + b22, b11, b12 - b22, b21 - b11, b22, b11 + b12, b21 + b22]


def _strassen(prod, col1=None, col2=None):
    m4 = prod(3)
    m2 = prod(1)
    c21 = m2 + m4
    if col1 is not None:
        e11, e21 = col1()
        m4, c21 = m4 + e11, c21 + e21
    m3 = prod(2)
    m5 = prod(4)
    c12 = m3 + m5
    if col2 is not None:
        e12, e22 = col2()
        c12, m3 = c12 + e12, m3 + e22
    m1 = prod(0)
    c11 = prod(6) + (m1 + (m4 - m5))
    c22 = prod(5) + (m1 + (m3 - m2))
    return c11, c12, c21, c22


def _group(rows, cols, pairs):
    xs, ys = dict.fromkeys(x for x, _ in pairs), dict.fromkeys(y for _, y in pairs)
    used = set(xs) | set(ys) | {(x[0], y[1]) for x, y in pairs} | {(y[0], x[1]) for x, y in pairs}
    prods = []
    for n, r in enumerate(rows):
        for i, k in [x for x in xs if x[0] == r]:
            mates = [y for x, y in pairs if x == (i, k)]
            prods.append((((1, i, k),) + tuple((1, i, k2) for _, k2 in mates), ((1, k, 0),),
                          ((1, i, 0), (-1, i, 1))))
            prods.append((((1, i, k),) + tuple((-1, i2, k) for i2, _ in mates), ((1, k, 0), (1, k, 1)),
                          ((1, i, 1),)))
        for i2, k2 in [y for y in ys if y[0] == r]:
            mates = [x for x, y in pairs if y == (i2, k2)]
            prods.append((((1, i2, k2),) + tuple((1, i2, k) for _, k in mates), ((1, k2, 1),),
                          ((1, i2, 1), (-1, i2, 0))))
            prods.append((((1, i2, k2),) + tuple((-1, i, k2) for i, _ in mates), ((1, k2, 0), (1, k2, 1)),
                          ((1, i2, 0),)))
        prods += [(((1, r, k),), ((1, k, h),), ((1, r, h),)) for k in cols if (r, k) not in used for h in (0, 1)]
        for (i, k), (i2, k2) in pairs:
            if r in (i, i2) and i + i2 - r in rows[n + 1:]:
                prods.append((((1, i, k2),), ((1, k2, 0), (-1, k, 0)), ((1, i2, 0), (1, i, 0))))
                prods.append((((1, i2, k), (1, i, k2)), ((1, k, 0), (1, k2, 1)), ((1, i2, 0), (1, i, 1))))
                prods.append((((1, i2, k),), ((1, k, 1), (-1, k2, 1)), ((1, i2, 1), (1, i, 1))))
    return prods


def _all_pairs(xrows, yrows):
    return [((x, a), (y, b)) for a, x in enumerate(xrows) for b, y in enumerate(yrows) if a != b]


_PAIRS65 = [((x[0] + 10, x[1]), (y[0] + 10, y[1])) for x, y in (
    ((0, 1), (1, 0)), ((0, 1), (5, 2)), ((2, 3), (1, 0)), ((2, 3), (3, 1)), ((2, 3), (5, 2)), ((3, 2), (1, 0)),
    ((4, 4), (0, 3)), ((4, 4), (1, 0)), ((4, 4), (3, 1)), ((4, 4), (5, 2)))]
_C_GROUPS = [_group(range(r, r + 8), range(4), _all_pairs(range(r, r + 4), range(r + 4, r + 8))) for r in (0, 8)]
_H_GROUPS = [_group(range(10), range(5), _all_pairs(range(5), range(5, 10))),
             _group(range(10, 16), range(5), _PAIRS65)]
_sum_index = lambda groups: {f: n for n, f in enumerate(
    dict.fromkeys(t[0] for g in groups for t in g if len(t[0]) > 1))}
_C_SUMS, _H_SUMS = _sum_index(_C_GROUPS), _sum_index(_H_GROUPS)


def _form(form, get):
    acc = None
    for sign, i, j in form:
        v = get(i, j)
        acc = v if acc is None else (acc + v if sign > 0 else acc - v)
    return acc


def _gap_items(bufs, gap_scr):
    items = []
    for n, buf in enumerate(bufs):
        acc = []

        def part(r0, buf=buf, acc=acc):
            def fn(dep):
                wu = jnp.concatenate([buf[r:r + 8, :] for r in range(r0, r0 + T, 32)])
                mask = jnp.full((8, T), 0x7FFF0000, U32)
                if dep is not None:
                    mask = jnp.where(dep > jnp.inf, jnp.uint32(0), mask)
                mask = _rows(mask, 32)
                new = [jnp.sum(pltpu.bitcast(v & mask, F32).reshape(4, 8, T), axis=0) for v in (wu << 16, wu)]
                acc[:] = [u + v for u, v in zip(acc, new)] if acc else new
            return fn

        def last(_, n=n, acc=acc):
            bits = []
            for v in acc:
                l1 = jnp.sum(jnp.sum(v, axis=1, keepdims=True), axis=0, keepdims=True)
                bits.append(pltpu.bitcast(jnp.broadcast_to(l1, (8, T)), jnp.int32) >> 8)
            gap_scr[n] = jnp.clip((bits[0] - bits[1] + (1 << 14)) >> 15, -8, 8) << 23

        items += [part(r0) for r0 in range(0, buf.shape[0], T)] + [last]
    return items


class _PairWeights:
    def __init__(self, w_ref, transpose=False, shift=None):
        self.base = {}
        if shift is not None:
            fac = _rows(pltpu.bitcast(0x3F800000 + shift, F32), T)
            self.inv = pltpu.bitcast(0x3F800000 - shift, F32)
        for j in range(w_ref.shape[0] // T):
            wu = w_ref[_tile(j), :]
            if transpose:
                wu = wu.T
            hi = pltpu.bitcast(wu & jnp.uint32(0xFFFF0000), F32)
            self.base[j, 0] = pltpu.bitcast(wu << 16, F32)
            self.base[j, 1] = hi if shift is None else hi * fac
        self.cache = {}

    def __call__(self, form):
        sign = 1
        if form[-1][0] < 0 and form[0][1:] > form[1][1:]:
            sign, form = -1, ((1,) + form[1][1:], (-1,) + form[0][1:])
        if form not in self.cache:
            self.cache[form] = _form(form, lambda k, h: self.base[k, h]).astype(BF16)
        return sign, self.cache[form]


def _run_group(jobs, prods, a_get, w, transposed, finish):
    left = {}
    for _, _, outs in prods:
        for _, i, h in outs:
            left[i, h] = left.get((i, h), 0) + 1
    acc = {}
    for af, bf, outs in prods:
        sign, wt = w(bf)
        m = jobs.mm([wt], [a_get(af)], _dot_nt) if transposed else jobs.mm([a_get(af)], [wt], _dot)
        for s_, i, h in outs:
            if (i, h) not in acc:
                acc[i, h] = (s_ * sign, m)
            else:
                s0, v = acc[i, h]
                acc[i, h] = (s0, v + m if s0 == s_ * sign else v - m) if s0 > 0 or s_ * sign < 0 else (1, m - v)
            left[i, h] -= 1
            if not left[i, h]:
                s0, v = acc.pop((i, h))
                assert s0 > 0
                finish(2 * i + h, v)


class _Jobs:
    def __init__(self, side=()):
        self.res = []
        self.side = list(side)

    def mm(self, lhs, wt, dot):
        acc = None
        for x, w in zip(lhs, wt):
            v = dot(x, w)
            self.res.append(v)
            acc = v if acc is None else v + acc
            rel = 4 * (len(self.res) % 4)
            while self.side and self.side[0][0] <= len(self.res):
                self.side.pop(0)[1](v[8 * rel:8 * rel + 8, :])
                rel = (rel + 2) % 16
        return acc


def _proj_step(h_scr, hs_scr, c_ref, cs_scr, wq_ref, wuk_ref, wuv_ref, q_scr, k_scr, v_scr, pf, scale, shifts, side):
    wk, wvT, wq = [_PairWeights(w, n == 1, shifts[n]) for n, w in enumerate((wuk_ref, wuv_ref, wq_ref))]
    c_get = lambda f: _ld(cs_scr, _C_SUMS[f]) if len(f) > 1 else c_ref[_tile(f[0][1]), _tile(f[0][2])]
    h_get = lambda f: _ld(hs_scr, _H_SUMS[f]) if len(f) > 1 else _ld(h_scr, f[0][1], f[0][2])

    def put(dst, w, mul=None):
        muls = [mul, _rows(w.inv if mul is None else w.inv * mul, T)]

        def fn(u, v):
            v = (v if muls[u % 2] is None else v * muls[u % 2]).astype(BF16)
            dst[u] = v.T if mul is not None and u < QT else v
        return fn

    jobs = _Jobs(side)
    put_v, stored = put(v_scr, wvT), set()
    nxt = [0]

    def fin_v(u, v):
        put_v(u, v)
        stored.add(u)
        for J in range(SB):
            if all(2 * (SB * J + k) + h in stored for k in range(SB) for h in range(2)) and ('J', J) not in stored:
                stored.add(('J', J))
                for fn in _v_form_items(v_scr, pf, J):
                    nxt[0] = max(nxt[0] + VFS, len(jobs.res) + VF0)
                    jobs.side.append((int(nxt[0]), fn))
                jobs.side.sort(key=lambda e: e[0])

    kk, vv, qq = ((c_get, wk, False, put(k_scr, wk)), (c_get, wvT, True, fin_v),
                  (h_get, wq, False, put(q_scr, wq, scale)))
    for prods, args in ((_C_GROUPS[0], kk), (_C_GROUPS[0], vv), (_C_GROUPS[1], vv), (_C_GROUPS[1], kk),
                        (_H_GROUPS[0], qq), (_H_GROUPS[1], qq)):
        _run_group(jobs, prods, *args)
    assert not jobs.side


def _inner_group(rows, cols, pairs):
    xs, ys = dict.fromkeys(x for x, _ in pairs), dict.fromkeys(y for _, y in pairs)
    used = set(xs) | set(ys) | {(x[0], y[1]) for x, y in pairs} | {(y[0], x[1]) for x, y in pairs}
    prods = []
    for i, j in xs:
        mates = [y for x, y in pairs if x == (i, j)]
        prods.append((((1, i, 0),), ((1, 0, j), (-1, 1, j)), ((1, i, j),) + tuple((1, i2, j) for i2, _ in mates)))
        prods.append((((1, i, 0), (1, i, 1)), ((1, 1, j),), ((1, i, j),) + tuple((-1, i, j2) for _, j2 in mates)))
    for i2, j2 in ys:
        mates = [x for x, y in pairs if y == (i2, j2)]
        prods.append((((1, i2, 0), (1, i2, 1)), ((1, 0, j2),),
                      ((1, i2, j2),) + tuple((-1, i2, j) for _, j in mates)))
        prods.append((((1, i2, 1),), ((1, 0, j2), (-1, 1, j2)),
                      ((-1, i2, j2),) + tuple((-1, i, j2) for i, _ in mates)))
    prods += [(((1, i, h),), ((1, h, j),), ((1, i, j),))
              for i in rows for j in cols if (i, j) not in used for h in (0, 1)]
    for (i, j), (i2, j2) in pairs:
        lo, hi = min(j, j2), max(j, j2)
        prods.append((((1, i2, 0), (-1, i, 0)), ((1, 0, lo), (1, 0, hi)), ((1, i2, j),)))
        prods.append((((1, i, 0), (1, i2, 1)), ((1, 0, j2), (1, 1, j)), ((1, i, j2), (1, i2, j))))
        prods.append((((1, i, 1), (-1, i2, 1)), ((1, 1, lo), (1, 1, hi)), ((1, i, j2),)))
    return prods


def _o_jobs():
    prods = (_inner_group(range(10), range(5), _all_pairs(range(0, 10, 2), range(1, 10, 2)))
             + _inner_group(range(10, 16), range(5), _PAIRS65))
    row = lambda t: max(i for _, i, _ in t[0])
    unit = lambda t: max(2 * i + h for _, i, h in t[0])
    need = lambda t: unit(t) if row(t) == 15 else 2 * row(t) + 1
    return [(need(t), t) for t in sorted(prods, key=need)]


_O_JOBS = _o_jobs()


SB = 4


class _Star:
    def __init__(self, ts):
        self.ts, self.n = ts, len(ts)
        rn = range(self.n)
        self.pairs = [(i, j) for i in rn for j in rn if i < j]
        self.pf = {f: m for m, f in enumerate([('R', i) for i in rn] + [('C', i) for i in rn]
                                              + [('S', i, j) for i in rn for j in rn if i != j]
                                              + [('A', i, j) for i, j in self.pairs])}
        self.vf = {f: m for m, f in enumerate([('W', i) for i in rn]
                                              + [(q, i, j) for i, j in self.pairs for q in ('Q1', 'Q2', 'Q3')])}
        self.pv = {**{('W', i): ('R', i) for i in rn}, **{('B', i): ('C', i) for i in rn},
                   **{('Q1', i, j): ('S', i, j) for i, j in self.pairs},
                   **{('Q2', i, j): ('A', i, j) for i, j in self.pairs},
                   **{('Q3', i, j): ('S', j, i) for i, j in self.pairs}}

    def products(self, i):
        return [('W', i), ('B', i)] + [(q, i, j) for j in range(i + 1, self.n) for q in ('Q1', 'Q2', 'Q3')]


_FULL = _Star((-1.125, -0.375, 0.375, 1.125))
_HALF = _Star((-0.75, 0.75))
_DCELLS = [(0, 0), (1, 0), (1, 1), (2, 2), (3, 2), (3, 3)]
_HSLOT = (SB - 1) * len(_FULL.pf)
_DSLOT = _HSLOT + len(_HALF.pf)
_VSLOT = _DSLOT + len(_DCELLS)
_VHALF = (SB - 1) * len(_FULL.vf)
_FENCE = _VSLOT + (_VHALF + SB * len(_HALF.vf) + 1) // 2


def _v_slot(star, J, f):
    m = star.vf[f] + J * len(star.vf) + (0 if star is _FULL else _VHALF)
    return _VSLOT + m // 2, m % 2 * (T // 2)


def _v_form_items(v_scr, pf, J):
    n, HT = 16, T // 2

    def item(star, h, r0, pairs):
        def fn(dep):
            ts = [jnp.full((8, T), t, F32) for t in star.ts]
            ts = [_rows(t if dep is None else _after(t, dep), n) for t in ts]

            def get(k, a):
                r = (a * HT + r0) // 2
                return _ld(v_scr, 2 * (SB * J + k) + h, slice(r, r + n // 2)).astype(F32)

            def put(f, v):
                slot, r = _v_slot(star, J, f)
                pf[h][slot, r + r0:r + r0 + n, :] = v.astype(BF16)

            b = {(k, a): get(k, a) for k in sorted({k for pr in pairs or star.pairs for k in pr})
                 for a in range(2)}
            if pairs is None or star.n == 2:
                w = [b[k, 0] + ts[k] * b[k, 1] for k in range(star.n)]
                for k in range(star.n):
                    put(('W', k), w[k])
                for i, j in star.pairs:
                    put(('Q2', i, j), w[i] - w[j])
            for i, j in pairs or ():
                d0, d1 = b[j, 0] - b[i, 0], b[j, 1] - b[i, 1]
                put(('Q1', i, j), d0 + ts[i] * d1)
                put(('Q3', i, j), d0 + ts[j] * d1)
        return fn

    pr = _FULL.pairs
    parts = [(_HALF, _HALF.pairs)]
    if J < SB - 1:
        parts += [(_FULL, x) for x in (None, pr[:2], [pr[2], pr[4]], [pr[3], pr[5]])]
    return [item(star, h, r0, pairs) for h in range(2) for r0 in range(0, HT, n) for star, pairs in parts]


def _job_order(nsb):
    units = [(I, h) for I in range(nsb) for h in range(2)]
    qe, qv = [], []
    for I, h in units:
        es = [('e', I, h, J, p) for J in range(I) for p in range(SB)]
        ds = [('d', I, h) + c for c in _DCELLS]
        es.insert(max(len(es) - FPOS, 0), ('f', I, h))
        qe += es + ds if I or FPOS < 9 else ds[:DPOS] + es + ds[DPOS:]
        for i in range(SB):
            qv += [('p', I, h, f, J) for f in _FULL.products(i) for J in range(I)]
            if i >= 2:
                qv += [('p', I, h, f, None) for f in _HALF.products(i - 2)]
            qv += [('v', I, h) + c for c in _DCELLS if c[0] == i]
    qo = [('o', u, j) for j, (u, _) in enumerate(_O_JOBS)]
    cost = dict(e=8, f=8, d=2, p=1, v=2, o=2)
    order, done = [], {}
    now = [0]

    def emit(q):
        job = q.pop(0)
        order.append(job)
        now[0] += cost[job[0]]
        if job[0] == 'd':
            done[job] = now[0]
        elif job[0] == 'v' and job[4] == job[3]:
            done['u', 2 * (SB * job[1] + job[3]) + job[2]] = now[0]
        return cost[job[0]]

    def v_ready():
        if not qv:
            return False
        key = ('d', qv[0][1], qv[0][2], SB - 1, SB - 1)
        return key in done and done[key] + (LAT_0 if qv[0][1:3] == (0, 0) else LAT_A) <= now[0]

    def o_ready():
        return bool(qo) and ('u', qo[0][1]) in done and done['u', qo[0][1]] + LAT_B <= now[0]

    def fill(nv, no):
        n = 0
        while nv > 0 or no > 0 or n % 4:
            if no > 0 and n % 2 == 0 and o_ready() and no * ONV >= nv:
                no -= 2
                n += emit(qo)
            elif v_ready() and (nv > 0 or n % 4):
                c = emit(qv)
                nv -= c
                n += c
            elif o_ready() and n % 2 == 0 and (no > 0 or n % 4 or nv > 0) and len(qo) > RES:
                no -= 2
                n += emit(qo)
            else:
                break

    while qe:
        unit = qe[0][1:3]
        while qv and qv[0][2] == unit[1] and qv[0][1] < unit[0]:
            emit(qv)
        ne = 0
        while qe and ne < 8 and (ne == 0 or (qe[0][0] == 'd' and qe[0][1:3] == unit and ne + 2 <= 8)):
            ne += emit(qe)
        groups = lambda q: sum(cost[j[0]] for j in q) / 8
        old = [j for j in qv if j[1:3] != unit and ('d', j[1], j[2], SB - 1, SB - 1) in done]
        here = [j for j in qe if j[1:3] == unit]
        rest = sum(cost[j[0]] for j in old)
        nv = (rest - LAT_A) / (groups(here) + 1) if here else rest
        no = 2 * max(len(qo) - RES - OEND, 0) / (groups(qe) + 1)
        fill(int(nv + 0.5), int(no + 0.5))
    while qv or qo:
        if qv and v_ready():
            fill(6, 2)
            if not qv:
                continue
        elif o_ready():
            emit(qo)
        else:
            emit(qv or qo)
    return order


def _attention_safe(q_scr, k_scr, v_scr, wo_ref, acc_scr):
    causal = (jax.lax.broadcasted_iota(jnp.int32, (T, T), 0)
              <= jax.lax.broadcasted_iota(jnp.int32, (T, T), 1))

    def unit(u, carry):
        r, hd = u // 2, u % 2

        def block(c, mlo):
            m0, l, o = mlo
            s = _dot_nt(_ld(k_scr, 2 * c + hd), _ld(q_scr, u))
            s = jnp.where(jnp.logical_or(causal, c < r), s, -1e9 * LOG2E)
            m = jnp.maximum(m0, jnp.max(s, axis=0, keepdims=True))
            a = jnp.exp2(m0 - m)
            p = jnp.exp2(s - m)
            return (m, l * a + jnp.sum(p, axis=0, keepdims=True),
                    o * a + _dot(_ld(v_scr, 2 * c + hd), p.astype(BF16)))

        _, l, o = jax.lax.fori_loop(0, r + 1, block, (jnp.full((1, T), -jnp.inf, F32), jnp.zeros((1, T), F32),
                                                      jnp.zeros((T, T), F32)))
        rows = pl.ds(pl.multiple_of(r * T, T), T)
        acc_scr[rows, :] += _dot((o * (1.0 / l)).astype(BF16).T, wo_ref[pl.ds(pl.multiple_of(hd * T, T), T), :])
        return carry

    jax.lax.fori_loop(0, q_scr.shape[0], unit, 0)


def _attention_step(q_scr, k_scr, v_scr, pf, wo_ref, acc_scr, flag_scr, z):
    causal = (jax.lax.broadcasted_iota(jnp.int32, (T, T), 0)
              <= jax.lax.broadcasted_iota(jnp.int32, (T, T), 1))
    HT = T // 2
    lsum, lrow, acc, fg, dacc, of, lhs = {}, {}, {}, {}, {}, {}, {}
    res = []
    wo, terms = {}, {}
    left = {}
    chk = [jnp.zeros((8, T), F32), None]
    for _, t in _O_JOBS:
        for _, i, j in t[2]:
            left[i, j] = left.get((i, j), 0) + 1

    def add_l(u, v):
        lsum[u] = v if u not in lsum else lsum[u] + v

    csign = {}

    def p_forms(star, h, slot0, g, tiles, cell, when):
        n = star.n

        def put(f, v):
            pf[h][slot0 + star.pf[f], 16 * g:16 * g + 16, :] = v.astype(BF16)

        for i in range(n):
            row = [cell(i, k) for k in sorted(range(n), key=lambda k: when(i, k))]
            r = functools.reduce(lambda x, y: x + y, row)
            put(('R', i), r)
            add_l(tiles[i], r[:8] + r[8:])
            col = sorted(range(n), key=lambda i2: (when(i2, i), i2 != i))
            sign = csign[n, i] = 1 if col[0] == i else -1
            c = cell(col[0], i)
            for i2 in col[1:]:
                c = c + cell(i2, i) if (1 if i2 == i else -1) == sign else c - cell(i2, i)
            put(('C', i), c)
            for j in range(n):
                if j != i:
                    put(('S', i, j), cell(i, j))
        for i, j in star.pairs:
            put(('A', i, j), cell(i, j) + cell(j, i))

    def scores(x, u):
        s = (_dot if u < QT else _dot_nt)(x, _ld(q_scr, u))
        res.append(s)
        return s

    def job_e(I, h, J, p):
        tiles = [2 * (SB * I + i) + h for i in range(SB)]
        ps = []
        for i, u in enumerate(tiles):
            x = jnp.concatenate([k_scr.bitcast(U32)[2 * (SB * J + (t - i) % SB) + h, 8 * g:8 * g + 8, :]
                                 for g in (2 * p, 2 * p + 1) for t in range(SB)], axis=0)
            ps.append(jnp.exp2(scores(pltpu.bitcast(x, BF16), u)))
        when = lambda i, k: (i + k) % SB
        for n, g in enumerate((2 * p, 2 * p + 1)):
            cell = lambda i, k: ps[i][16 * (SB * n + when(i, k)):16 * (SB * n + when(i, k)) + 16]
            p_forms(_FULL, h, J * len(_FULL.pf), g, tiles, cell, when)

    def job_f(I, h):
        tiles = [2 * (SB * I + 2 + i) + h for i in range(2)]
        ps = {(i, k): jnp.exp2(scores(_ld(k_scr, 2 * (SB * I + k) + h), u))
              for i, u in enumerate(tiles) for k in range(2)}
        for g in range(T // 16):
            p_forms(_HALF, h, _HSLOT, g, tiles, lambda i, k: ps[i, k][16 * g:16 * g + 16], lambda i, k: 0)

    def job_d(I, h, i, k):
        u = 2 * (SB * I + i) + h
        s = scores(_ld(k_scr, 2 * (SB * I + k) + h), u)
        if i == k:
            s = jnp.where(causal, s, -1e9 * LOG2E)
        p = jnp.exp2(s)
        add_l(u, jnp.sum(p.reshape(T // 8, 8, T), axis=0))
        pf[h][_DSLOT + _DCELLS.index((i, k))] = p.astype(BF16)
        if (i, k) == _DCELLS[-1]:
            pf[h][_FENCE + z, 0:16, :] = jnp.zeros((16, T), BF16)
            for u in [2 * (SB * I + a) + h for a in range(SB)]:
                lrow[u] = jnp.sum(lsum.pop(u), axis=0, keepdims=True)
            ls = [lrow[2 * (SB * I + a) + h] for a in range(SB)]
            lo = jnp.minimum(jnp.minimum(ls[0], ls[1]), jnp.minimum(ls[2], ls[3]))
            hi = jnp.maximum(jnp.maximum(ls[0], ls[1]), jnp.maximum(ls[2], ls[3]))
            ok = jnp.logical_and(lo >= L_LO, hi <= L_HI)
            ok = jnp.logical_and(ok, (hi if I else jnp.maximum(ls[2], ls[3]))
                                 <= L_RATIO * (lo if I else jnp.minimum(ls[2], ls[3])))
            bad = jnp.where(ok, 0.0, 1.0)
            chk[1] = bad if chk[1] is None else jnp.maximum(chk[1], bad)

    def job_p(I, h, f, J):
        star, last = (_HALF, True) if J is None else (_FULL, J == I - 1)
        blk = I if J is None else J
        if f[0] == 'B':
            x = _ld(v_scr, 2 * (SB * blk + f[1]) + h, slice(HT // 2, HT))
        else:
            slot, r = _v_slot(star, blk, f)
            x = _ld(pf[h], slot, slice(r // 2, (r + HT) // 2))
        v = _dot(x, _ld(pf[h], (_HSLOT if J is None else J * len(_FULL.pf)) + star.pf[star.pv[f]]))
        res.append(v)
        key = (star.n,) + f
        acc[key] = v if key not in acc else acc[key] + v
        if not last:
            return

        def add(which, i, v, sign=1):
            k_ = (star.n, which, i)
            if k_ not in fg:
                fg[k_] = v if sign > 0 else -v
            else:
                fg[k_] = fg[k_] + v if sign > 0 else fg[k_] - v

        if f[0] == 'W':
            add('F', f[1], acc.pop(key))
        elif f[0] == 'B':
            add('G', f[1], acc.pop(key), csign[star.n, f[1]])
        elif f[0] == 'Q3':
            _, i, j = f
            q1, q2, q3 = (acc.pop((star.n, q, i, j)) for q in ('Q1', 'Q2', 'Q3'))
            t = ((q1 + q2) + q3) * (1.0 / (star.ts[i] - star.ts[j]))
            add('G', i, t)
            add('G', j, t)
            add('F', i, q1)
            add('F', j, q3, -1)

    def job_v(I, h, i, k):
        u = 2 * (SB * I + i) + h
        v = _dot(_ld(v_scr, 2 * (SB * I + k) + h), _ld(pf[h], _DSLOT + _DCELLS.index((i, k))))
        res.append(v)
        dacc[u] = v if u not in dacc else dacc[u] + v
        if k == i:
            o = dacc.pop(u)
            for star, a in ([(_FULL, i)] if I else []) + ([(_HALF, i - 2)] if i >= 2 else []):
                f, g = fg.pop((star.n, 'F', a)), fg.pop((star.n, 'G', a))
                o = o + jnp.concatenate([f - star.ts[a] * g, g], axis=0)
            o = o * (1.0 / lrow[u])
            of[u] = o
            chk[0] = chk[0] + jnp.sum(o.reshape(T // 8, 8, T), axis=0)

    def job_o(_, n):
        af, bf, outs = _O_JOBS[n][1]
        if af not in lhs:
            v = _form(af, lambda i, h: of[2 * i + h])
            lhs[af] = _tie(v.astype(BF16).T, v[0:8, :])
        if bf not in wo:
            wo[bf] = (wo_ref[_tile(bf[0][1]), _tile(bf[0][2])] if len(bf) == 1 else
                      _form(bf, lambda h, j: wo_ref[_tile(h), _tile(j)].astype(F32)).astype(BF16))
        v = _dot(lhs[af], wo[bf])
        res.append(v)
        for sign, i, j in outs:
            terms.setdefault((i, j), []).append((sign, v))
            if len(terms[i, j]) == left[i, j]:
                tot = acc_scr[_tile(i), _tile(j)]
                for sg, m in terms.pop((i, j)):
                    tot = tot + m if sg > 0 else tot - m
                acc_scr[_tile(i), _tile(j)] = tot

    fns = dict(e=job_e, f=job_f, d=job_d, p=job_p, v=job_v, o=job_o)
    order = _job_order(q_scr.shape[0] // (2 * SB))
    for n, job in enumerate(order):
        assert job[0] not in 'efd' or not any(j[0] in 'pv' and j[2] == job[2] and j[1] < job[1] for j in order[n:])
    for job in order:
        fns[job[0]](*job[1:])
    fine = jnp.abs(chk[0]) < jnp.inf
    flag_scr[...] = jnp.maximum(flag_scr[...], jnp.where(fine, chk[1], 1.0))


def _kernel(x_hbm, c_hbm, wq_hbm, wuk_hbm, wuv_hbm, wo_hbm, w1_hbm, w2_hbm, w3_hbm, w4_hbm,
            cond_hbm, wmod_hbm, out_hbm,
            x_ref, c_ref, cond_ref, wma_ref, wmb_ref, w1_ref, w2_ref, w3_ref, w4_ref,
            wq_buf, wk_buf, wv_buf, wo_buf, out_buf, sem, wsem, osem,
            mod_scr, h_scr, cs_scr, hs_scr, w_scr, q_scr, k_scr, v_scr, acc_scr, xn_scr, xh_scr, a1_scr, t_scr,
            ws12, ws3, ws4, pq_buf, pk_buf, pv_buf, gap_scr, st_in, pf_scr, vf_scr, flag_scr, redo):
    S, M = x_hbm.shape
    D = wq_hbm.shape[2]
    nattn = wo_hbm.shape[0]
    Fd = w4_hbm.shape[0]
    scale = float(D) ** -0.5 * LOG2E
    nb, nrb = S // T, S // RB
    km, kc = M // T, c_hbm.shape[1] // T
    NX = 4
    XR = S // NX
    CB = XR // T

    work, probe = (wk_buf, wv_buf, wq_buf), (pk_buf, pv_buf, pq_buf)

    def pcopies(g, bufs=work, s0=0):
        return [pltpu.make_async_copy(src.bitcast(U32).at[:, g, :], dst, wsem.at[s0 + j])
                for j, (src, dst) in enumerate(zip((wuk_hbm, wuv_hbm, wq_hbm), bufs))]

    def ocopy(g):
        return pltpu.make_async_copy(wo_hbm.at[g], wo_buf, wsem.at[3])

    def chunk_copy(src, dst, i, s0):
        rows = slice(i * XR, (i + 1) * XR)
        return pltpu.make_async_copy(src.at[rows, :], dst.at[rows, :], sem.at[s0 + i])

    cp_cond = pltpu.make_async_copy(cond_hbm, cond_ref, sem.at[0])
    cp_wma = pltpu.make_async_copy(wmod_hbm.at[:, 0:2 * M], wma_ref, sem.at[1])
    cp_late = [pltpu.make_async_copy(src, dst, sem.at[2 + j]) for j, (src, dst) in enumerate((
        (wmod_hbm.at[:, 2 * M:6 * M], wmb_ref), (w1_hbm, w1_ref), (w2_hbm, w2_ref),
        (w3_hbm, w3_ref), (w4_hbm, w4_ref)))]
    cp_x = [chunk_copy(x_hbm, x_ref, i, 7) for i in range(NX)]
    cp_c = [chunk_copy(c_hbm, c_ref, i, 7 + NX) for i in range(NX)]

    def silu_cond():
        cf = cond_ref[...].astype(F32)
        return jnp.broadcast_to((cf * jax.nn.sigmoid(cf)).astype(BF16), (8, M))

    cp_wk, cp_wv, cp_wq = pcopies(0)
    named = dict(k=cp_wk, v=cp_wv, q=cp_wq, o=ocopy(0), n=cp_cond, m=cp_wma)
    named.update(zip('abcd', cp_c))
    named.update(zip('wxyz', cp_x))
    started, arrived, did = set(), set(), set()

    def zero(r, carry):
        acc_scr[pl.ds(pl.multiple_of(r * T, T), T), :] = jnp.zeros((T, M), F32)
        return carry

    def x_rows(rows, dep):
        xf = x_ref[rows, :].astype(F32)
        if dep is None:
            return xf
        return jnp.concatenate([_after(xf[:, :T], _rows(dep, xf.shape[0])), xf[:, T:]], axis=1)

    def n_item(r, i):
        def fn(dep):
            rows = slice(r * T + i * LP, r * T + (i + 1) * LP)
            xn_scr[rows, :] = _ln(x_rows(rows, dep))
        return fn

    def h_item(r, i, normed):
        def fn(dep):
            rows = slice(i * LP, (i + 1) * LP)
            grows = slice(r * T + i * LP, r * T + (i + 1) * LP)
            sa = mod_scr[:, 0:M]
            if normed and dep is not None:
                sa = jnp.concatenate([_after(sa[:, _tile(j)], dep) for j in range(km)], axis=1)
            hf = ((xn_scr[grows, :] if normed else _ln(x_rows(grows, dep))) * _rows(mod_scr[:, M:2 * M], LP)
                  + _rows(sa, LP))
            for j in range(km):
                h_scr[r, j, rows, :] = hf[:, _tile(j)].astype(BF16)
            for f, n in _H_SUMS.items():
                if all(t[1] == r for t in f):
                    hs_scr[n, rows, :] = _form(f, lambda _, k: hf[:, _tile(k)]).astype(BF16)
            did.add(('h', r, i))
        return fn

    def release(jobs, span, items):
        if span and items:
            jobs.side += [(len(jobs.res) + 1 + i * span // len(items), fn) for i, fn in enumerate(items)]
            jobs.side.sort(key=lambda e: e[0])
        else:
            for fn in items:
                fn(None)

    def sum_items(n, group, index, dst, get, skip_rows):
        forms = [f for f in dict.fromkeys(t[0] for t in group)
                 if len(f) > 1 and not (skip_rows and len({t[1] for t in f}) == 1)]

        def item(f, rows):
            def fn(dep):
                def term(r, k):
                    v = get(r, k, rows).astype(F32)
                    return v if dep is None or (r, k) != f[0][1:] else _after(v, _rows(dep, v.shape[0]))
                dst[index[f], rows, :] = _form(f, term).astype(BF16)
            return fn

        return [item(f, slice(i, i + n)) for i in range(0, T, n) for f in forms]

    h_sums = lambda n, gi: sum_items(n, _H_GROUPS[gi], _H_SUMS, hs_scr,
                                     lambda r_, k, rows: h_scr[r_, k, rows, :], True)

    def stash(key, buf, j0, transpose=False):
        n = buf.shape[0] // T
        if key not in did:
            assert key in arrived
            did.add(key)
            w = _PairWeights(buf, transpose)
            for j in range(n):
                for hd in range(2):
                    w_scr[hd, j0 + j] = w(((1, j, hd),))[1]
        return lambda hd: [_ld(w_scr, hd, j0 + j) for j in range(n)]

    def kv_tile(jobs, r):
        wk, wvT = stash('k', wk_buf, 0), stash('v', wv_buf, kc, True)
        ct = [c_ref[_tile(r), _tile(j)] for j in range(kc)]
        for hd in range(2):
            k_scr[2 * r + hd] = jobs.mm(ct, wk(hd), _dot).astype(BF16)
        for hd in range(2):
            v_scr[2 * r + hd] = jobs.mm(wvT(hd), ct, _dot_nt).astype(BF16)

    def q_tile(jobs, r):
        wq = stash('q', wq_buf, 2 * kc)
        ht = [_ld(h_scr, r, j) for j in range(km)]
        for hd in range(2):
            v = (jobs.mm(ht, wq(hd), _dot) * scale).astype(BF16)
            q_scr[2 * r + hd] = v.T if 2 * r + hd < QT else v

    for blk in _prologue().split(';'):
        waits, starts, acts = blk.split('|')
        for ch in waits.strip():
            assert ch in started and ch not in arrived
            arrived.add(ch)
            named[ch].wait()
        for ch in starts.strip():
            assert ch not in started
            started.add(ch)
            named[ch].start()
        jobs = _Jobs()
        for act in acts.split():
            if act == 'Z':
                jax.lax.fori_loop(0, nb, zero, 0)
                acc_scr[S:, :] = jnp.zeros((acc_scr.shape[0] - S, M), F32)
                x_ref[S:, :] = jnp.zeros((x_ref.shape[0] - S, M), BF16)
                flag_scr[...] = jnp.zeros(flag_scr.shape, F32)
                redo[0] = 0
            elif act == 'L':
                did.add('L')
                for cp in cp_late:
                    cp.start()
            elif act == 'M':
                assert arrived >= set('nm')
                mod = _dot(silu_cond(), wma_ref[...])
                mod_scr[:, 0:M] = mod[:, 0:M]
                mod_scr[:, M:2 * M] = 1.0 + mod[:, M:2 * M]
                did.add('M')
            else:
                act, _, span = act.partition('@')
                span = int(span or 0)
                items = []
                for r in [int(ch, 16) for ch in act[1:]]:
                    did.add((act[0], r))
                    if act[0] == 'K':
                        assert 'abcd'[r // CB] in arrived
                        kv_tile(jobs, r)
                    elif act[0] == 'H':
                        assert 'wxyz'[r // CB] in arrived and 'M' in did
                        items += [h_item(r, i, ('N', r) in did) for i in range(T // LP)]
                    elif act[0] == 'N':
                        assert 'wxyz'[r // CB] in arrived
                        items += [n_item(r, i) for i in range(T // LP)]
                    elif act[0] == 'Q':
                        assert all(('h', r, i) in did for i in range(T // LP))
                        q_tile(jobs, r)
                    elif act[0] == 'F':
                        assert all(('K', SB * r + k_) in did for k_ in range(SB))
                        items += _v_form_items(v_scr, (pf_scr, vf_scr), r)
                    elif act[0] == 'C':
                        assert all('abcd'[t[1] // CB] in arrived for p_ in _C_GROUPS[r] for t in p_[0])
                        items += sum_items(
                            32, _C_GROUPS[r], _C_SUMS, cs_scr,
                            lambda r_, k, rows: c_ref[r_ * T + rows.start:r_ * T + rows.stop, _tile(k)], False)
                    else:
                        assert act[0] == 'S' and all(('h', t[1], T // LP - 1) in did for p_ in _H_GROUPS[r] for t in p_[0])
                        items += h_sums(32 if span else 16, r)
                release(jobs, span, items)
        assert not jobs.side
    assert arrived == set(named) and all((k_, r) in did for k_ in 'KHQ' for r in range(nb))
    assert all((k_, r) in did for k_ in 'CS' for r in range(2)) and 'L' in did
    assert all(('F', r) in did for r in range(SB))

    FH = ws3.shape[0] * T
    assert nattn - 1 >= FH // 64

    slices = ((w1_hbm, 32, 2 * T, 0), (w2_hbm, 32, 2 * T, 64), (w4_hbm, 64, FH, 128), (w3_hbm, T, FH, 256))
    slice_of = lambda g, n, half: jnp.minimum(g, half // n - 1)

    def prep_in(g):
        return [pltpu.make_async_copy(
            w.at[pl.ds(pl.multiple_of(slice_of(g, n, half) * n + x * half, n), n), 0:4 * T],
            st_in.at[r0 + x * n:r0 + (x + 1) * n, :], wsem.at[7]) for w, n, half, r0 in slices for x in range(2)]

    def mixer_prep(g):
        def blocks(r0, n, half, c0, c1, dep):
            get = lambda x, c: st_in[r0 + x * half:r0 + x * half + n, _tile(c)].astype(F32)
            return [_after(get(0, c0), _rows(dep, n)), get(0, c1), get(1, c0), _after(get(1, c1), _rows(dep, n))]

        def rows_item(dst, per, half, r0, c, o, n=16):
            def fn(dep):
                rows = pl.ds(pl.multiple_of(slice_of(g, per, half) * per, per) + o, n)
                for i, v in enumerate(_b_ops(*blocks(r0 + o, n, per, c, c + 2, dep))):
                    dst[i, c, rows, :] = v.astype(BF16)
            return fn

        def w3_item(k, i):
            def fn(dep):
                b11, b21, b12, b22 = blocks(slices[3][3], T, T, k, k + 2, dep)
                ws3[slice_of(g, T, FH), i, k] = _b_ops(b11, b12, b21, b22)[i].astype(BF16).T
            return fn

        return ([rows_item(dst, *sl[1:], c, o) for dst, sl in zip((ws12.at[0], ws12.at[1], ws4), slices)
                 for c in range(2) for o in range(0, sl[1], 16)]
                + [w3_item(k, i) for k in range(2) for i in range(7)])

    def next_copies(g):
        return pcopies(jnp.minimum(g + 1, nattn - 1)) + pcopies(jnp.minimum(g + 2, nattn - 1), probe, 4)

    def start_copies(g):
        for cp in next_copies(g) + prep_in(jnp.maximum(g, 0)):
            cp.start()

    def attn_body(g, exact):
        gw = jnp.maximum(g, 0)
        copies = next_copies(g)

        @pl.when(exact == 0)
        def _():
            bufs = (q_scr, k_scr, v_scr, (pf_scr, vf_scr), wo_buf, acc_scr, flag_scr)
            _attention_step(*bufs, g >> 16)

        @pl.when(jnp.logical_and(exact > 0, g >= 0))
        def _():
            _attention_safe(q_scr, k_scr, v_scr, wo_buf, acc_scr)

        for cp in copies:
            cp.wait()
        pltpu.make_async_copy(st_in, st_in, wsem.at[7]).wait()

        @pl.when(g == -exact)
        def _():
            for fn in _gap_items(work, gap_scr):
                fn(None)

        @pl.when(g + 1 < nattn)
        def _():
            ocopy(g + 1).start()
            side = mixer_prep(gw) + _gap_items(probe, gap_scr)
            side = [(SD0 + i * SDS + (SDJ if i >= SDN else 0), fn) for i, fn in enumerate(side)]
            bufs = (h_scr, hs_scr, c_ref, cs_scr, wq_buf, wk_buf, wv_buf, q_scr, k_scr, v_scr, (pf_scr, vf_scr))
            _proj_step(*bufs, scale, gap_scr, side)
            start_copies(g + 1)
            ocopy(g + 1).wait()

        return exact

    def attn_pass(exact, carry):
        @pl.when(jnp.logical_or(exact == 0, redo[0] > 0))
        def _():
            @pl.when(exact > 0)
            def _():
                jax.lax.fori_loop(0, nb, zero, 0)

            start_copies(-exact)
            jax.lax.fori_loop(-exact, nattn, attn_body, exact)

        @pl.when(exact == 0)
        def _():
            redo[0] = (jnp.max(flag_scr[...]) > 0).astype(jnp.int32)

        return carry

    jax.lax.fori_loop(0, 2, attn_pass, 0)

    for cp in cp_late:
        cp.wait()
    mod = _dot(silu_cond(), wmb_ref[...])
    mod_scr[:, 2 * M:4 * M] = mod[:, 0:2 * M]
    mod_scr[:, 4 * M:5 * M] = 1.0 + mod[:, 2 * M:3 * M]
    mod_scr[:, 5 * M:6 * M] = mod[:, 3 * M:4 * M]
    ftiles = [(f, min(f + T, Fd)) for f in range(0, Fd, T)]
    OFF = x_ref.shape[0] - S
    CAR = t_scr.shape[0] - RB

    def p1(r0, l0, n, dep=None):
        ga = mod_scr[:, 2 * M:3 * M]
        if dep is not None:
            ga = jnp.concatenate([_after(ga[:, 0:T], dep), ga[:, T:]], axis=1)
        rows = pl.ds(r0, n)
        x1 = x_ref[rows, :].astype(F32) + _rows(ga, n) * acc_scr[rows, :]
        xh_scr[0, l0:l0 + n, :] = x1
        hb = _ln(x1) * _rows(mod_scr[:, 4 * M:5 * M], n) + _rows(mod_scr[:, 3 * M:4 * M], n)
        xh_scr[1, l0:l0 + n, :] = hb
        return _ln(hb)

    HT = T // 2

    def p1_store(r0, c, dep=None):
        v = p1(r0 + c * PC, OFF + c * PC, PC, dep)
        a1_scr[c * PC:(c + 1) * PC, :] = v
        return jnp.max(v[:, M - T:].reshape(PC // 8, 8, T), axis=0)

    t_scr[RB:RB + CAR - OFF, :] = jnp.zeros((CAR - OFF, M), F32)
    t_scr[RB + CAR - OFF:RB + CAR, :] = _gelu(_dot(p1(0, 0, OFF).astype(BF16), w1_ref[...]))
    for c in range(RB // PC):
        p1_store(OFF, c)

    def out_copy(i):
        rows = pl.ds(i * T if isinstance(i, int) else pl.multiple_of(i * T, T), T)
        return pltpu.make_async_copy(out_buf.at[rows, :], out_hbm.at[rows, :], osem.at[i])

    def b_body(r, carry):
        gb = _rows(mod_scr[:, 5 * M:6 * M], T)
        r0 = pl.multiple_of(r * RB, RB)
        n0 = pl.multiple_of(jnp.minimum(r0 + RB, S - RB) + OFF, OFF)
        nh = RB // T
        now = [0]
        due = []
        pace = []

        def p1_item(c):
            return lambda dep: due.append((now[0] + PD, p1_store(n0, c, dep)))

        pace += [(P0 + i * PSTEP, p1_item(i)) for i in range(RB // PC)]
        wt = lambda ref, f0, f1, n: ref[f0:f1, _tile(n)]

        def mm(lhs, wts, dot=_dot):
            acc = None
            for x, w in zip(lhs, wts):
                if due and due[0][0] <= now[0]:
                    w = _tie(w, due.pop(0)[1])
                v = dot(x, w)
                now[0] += x.shape[0] // HT
                acc = v if acc is None else v + acc
                if pace and pace[0][0] <= now[0]:
                    pace.pop(0)[1](v[0:8, :])
            return acc

        def split_ops(lo, hi):
            return [v.astype(BF16) for v in _a_ops(lo[:HT], hi[:HT], lo[HT:], hi[HT:])]

        def two_tiles(aops, wsel, rest):
            def col(w):
                v = mm(rest[0], w, rest[3])
                return v[:HT], v[HT:]

            c11, c12, c21, c22 = _strassen(
                lambda i: mm([a[i] for a in aops], [wsel(i, k) for k in range(len(aops))]),
                lambda: col(rest[1]), lambda: col(rest[2]))
            return jnp.concatenate([c11, c21], axis=0), jnp.concatenate([c12, c22], axis=0)

        def square(full, aops, w_ref, ws_ref):
            out = {}
            for n in range(2):
                out[n], out[n + 2] = two_tiles(
                    aops, lambda i, k: _ld(ws_ref, i, n, slice(k * HT, (k + 1) * HT)),
                    (full[4:], [wt(w_ref, 4 * T, M, n)], [wt(w_ref, 4 * T, M, n + 2)], _dot))
            out[4] = mm(full, [wt(w_ref, j * T, (j + 1) * T, 4) for j in range(km)])
            return out

        t_scr[0:CAR, :] = t_scr[RB:RB + CAR, :]
        for hf in range(nh):
            a1 = [a1_scr[_tile(hf), _tile(j)] for j in range(km)]
            full = [v.astype(BF16) for v in a1]
            aops = [split_ops(a1[k], a1[2 + k]) for k in range(2)]
            for n, v in square(full, aops, w1_ref, ws12.at[0]).items():
                t = _gelu(v)
                if hf == nh - 1:
                    t = jnp.concatenate([t[:T - OFF], jnp.where(r < nrb - 1, t[T - OFF:], 0.0)], axis=0)
                t_scr[CAR + hf * T:CAR + (hf + 1) * T, _tile(n)] = t
        cq = M // 4
        shifts = (-1, 1, -2, 2)
        lane = jax.lax.broadcasted_iota(jnp.int32, (T, T), 1)
        y1, z, a3 = [], [], []
        for hf in range(nh):
            base = CAR - OFF + hf * T
            sh = []
            for j in range(km):
                g_lo, g_hi = (j * T) // cq, ((j + 1) * T - 1) // cq
                assert g_hi - g_lo <= 1
                v = t_scr[base + shifts[g_lo]:base + shifts[g_lo] + T, _tile(j)]
                if g_hi != g_lo:
                    v2 = t_scr[base + shifts[g_hi]:base + shifts[g_hi] + T, _tile(j)]
                    v = jnp.where(lane < g_hi * cq - j * T, v, v2)
                sh.append(v)
            hs = square([v.astype(BF16) for v in sh], [split_ops(sh[k], sh[2 + k]) for k in range(2)],
                        w2_ref, ws12.at[1])
            hs = jnp.concatenate([hs[n] for n in range(km)], axis=1)
            y1.append(hs + xh_scr[1, _tile(hf), :])
            z.append(xh_scr[0, _tile(hf), :] + gb * y1[hf])
            a3.append({})

            def ln_item(hf, c):
                def item(dep):
                    n = HT // NLN
                    for d in (0, HT):
                        v = y1[hf][d + c * n:d + (c + 1) * n]
                        if dep is not None:
                            v = jnp.concatenate([_after(v[:, :T], _rows(dep, n)), v[:, T:]], axis=1)
                        a3[hf][d + c * n] = _ln(v)
                return item

            ln_item(hf, 0)(None)
            pace += [(now[0] + LN0 + (c - 1) * LNS * (1 + hf), ln_item(hf, c)) for c in range(1, NLN)]
            pace.sort(key=lambda e: e[0])
        xh_scr[:, 0:OFF, :] = xh_scr[:, RB:RB + OFF, :]
        nf = FH // T
        h3, h3ops = [], []
        for hf in range(nh):
            assert len(a3[hf]) == 2 * NLN
            af = jnp.concatenate([a3[hf][key] for key in sorted(a3[hf])], axis=0)
            full = [af[:, _tile(j)].astype(BF16) for j in range(km)]
            aops = [split_ops(af[:, _tile(k)], af[:, _tile(2 + k)]) for k in range(2)]
            row, ops = {}, []
            narrow = None
            for n in range(nf):
                lo, hi = two_tiles(aops, lambda i, k: _ld(ws3, n, i, k),
                                   (full[4:], [wt(w3_ref, *ftiles[n], 4)],
                                    [wt(w3_ref, *ftiles[nf + n], 4)], _dot_nt))
                lo, hi = _gelu(lo), _gelu(hi)
                row[n], row[nf + n] = lo.astype(BF16), hi.astype(BF16)
                ops.append(split_ops(lo, hi))
                if n < km:
                    v = mm([wt(w3_ref, *ftiles[-1], n)], [full[n]], _dot_nt)
                    narrow = v if narrow is None else v + narrow
            row[2 * nf] = _gelu(mm(full, [wt(w3_ref, *ftiles[2 * nf], j) for j in range(km)],
                                   _dot_nt)).astype(BF16)
            fw = Fd - ftiles[-1][0]
            gT = jnp.concatenate([_gelu(narrow), jnp.zeros((T - fw, T), F32)], axis=0)
            row[2 * nf + 1] = _tie(gT.astype(BF16).T, gT[0:8, :])[:, :fw]
            h3.append([row[i] for i in range(len(ftiles))])
            h3ops.append(ops)
        for hf in range(nh):
            rows = pl.ds(pl.multiple_of(r0 + hf * T, T), T)

            def finish(n, v):
                out_buf[rows, _tile(n)] = (z[hf][:, _tile(n)] + gb[:, _tile(n)] * v).astype(out_buf.dtype)

            w4t = lambda n, f_: [wt(w4_ref, f0, f1, n) for f0, f1 in f_]
            finish(4, mm(h3[hf], w4t(4, ftiles)))
            for n in range(2):
                lo, hi = two_tiles(h3ops[hf], lambda i, k: _ld(ws4, i, n, slice(k * HT, (k + 1) * HT)),
                                   (h3[hf][2 * nf:], w4t(n, ftiles[2 * nf:]), w4t(n + 2, ftiles[2 * nf:]), _dot))
                finish(n, lo)
                finish(n + 2, hi)
            out_copy(r * nh + hf).start()
        assert not pace
        return carry

    jax.lax.fori_loop(0, nrb, b_body, 0)
    for i in range(nb):
        out_copy(i).wait()


@jax.jit
def pallas_adaLN_cond__compressed_kv_cla__mixer_s_mlp__prompt_kernel(
    A_x: jax.Array,
    A_c_kv: jax.Array,
    A_w_q: jax.Array,
    A_w_uk: jax.Array,
    A_w_uv: jax.Array,
    A_w_o: jax.Array,
    B_x: jax.Array,
    B_w1: jax.Array,
    B_w2: jax.Array,
    B_w3: jax.Array,
    B_w4: jax.Array,
    c: jax.Array,
    w_mod: jax.Array,
):
    _, S, M = A_x.shape
    Dc = A_c_kv.shape[2]
    H, D = A_w_q.shape[1], A_w_q.shape[2]
    Fd = B_w3.shape[1]
    assert D == T and A_c_kv.shape[1] == S and Dc == 4 * T and M == 5 * T and 13 * T < Fd < 14 * T and S == 16 * T
    vmem = pltpu.VMEM
    packed = lambda *lead: vmem(lead + (T, T), BF16)
    out = pl.pallas_call(
        _kernel,
        in_specs=[pl.BlockSpec(memory_space=pltpu.HBM)] * 12,
        out_specs=pl.BlockSpec(memory_space=pltpu.HBM),
        out_shape=jax.ShapeDtypeStruct((S, M), A_x.dtype),
        scratch_shapes=[
            vmem((S + 16, M), BF16),
            vmem((S, Dc), BF16),
            vmem((1, M), BF16),
            vmem((M, 2 * M), BF16),
            vmem((M, 4 * M), BF16),
            vmem((M, M), BF16),
            vmem((M, M), BF16),
            vmem((Fd, M), BF16),
            vmem((Fd, M), BF16),
            vmem((M, D), U32),
            vmem((Dc, D), U32),
            vmem((Dc, D), U32),
            vmem((2 * D, M), BF16),
            vmem((S, M), A_x.dtype),
            pltpu.SemaphoreType.DMA((15,)),
            pltpu.SemaphoreType.DMA((8,)),
            pltpu.SemaphoreType.DMA((S // T,)),
            vmem((8, 6 * M), F32),
            vmem((S // T, M // T, T, T), BF16),
            vmem((len(_C_SUMS), T, T), BF16),
            vmem((len(_H_SUMS), T, T), BF16),
            packed(2, M // T + 2 * (Dc // T)),
            packed(2 * S // T),
            packed(2 * S // T),
            packed(2 * S // T),
            vmem((S + 16, M), F32),
            vmem((S, M), F32),
            vmem((2, RB + 16, M), F32),
            vmem((RB, M), F32),
            vmem((RB + 32, M), F32),
            vmem((2, 7, 2, 2 * T, T), BF16),
            packed(6, 7, 2),
            vmem((7, 2, 6 * T, T), BF16),
            vmem((M, D), U32),
            vmem((Dc, D), U32),
            vmem((Dc, D), U32),
            vmem((3, 8, T), jnp.int32),
            vmem((4 * T, 4 * T), BF16),
            vmem((_FENCE + 1, T, T), BF16),
            vmem((_FENCE + 1, T, T), BF16),
            vmem((8, T), F32),
            pltpu.SMEM((1,), jnp.int32),
        ],
        compiler_params=pltpu.CompilerParams(
            vmem_limit_bytes=100 * 1024 * 1024,
            disable_bounds_checks=True,
        ),
    )(
        A_x.reshape(S, M), A_c_kv.reshape(S, Dc),
        A_w_q, A_w_uk, A_w_uv,
        A_w_o.reshape(H // 2, 2 * D, M),
        B_w1, B_w2, B_w3.T, B_w4, c, w_mod,
    )
    return out.reshape(1, S, M)
```

```python
import functools
import math

import jax
import jax.numpy as jnp
import jax.experimental.pallas as pl
import jax.experimental.pallas.tpu as pltpu

F32 = jnp.float32
BF16 = jnp.bfloat16
U32 = jnp.uint32
NT = (((1,), (1,)), ((), ()))
T = 128
EPS = 1e-5
LOG2E = math.log2(math.e)

GRP = 4
LEAD = 10
PROW = 3
RES = 32
LAT_0 = 32
LAT_A = 16
LAT_B = 20
ALEAD = 32
QT = (4, 6)
ONV, OEND = 0.5, 24
FPOS, DPOS = 0, 0
SIDE0, SIDE1, SLAG, SDUE = 8, 60, 4, 8
SKIND = 'pvo'
HACKWO = 0
SG0, SG1 = 6, 4
SD0, SDS = 10, 2
WFN = (4, 4, 6)
VF0, VFS = 4, 1.7
L_LO, L_HI, L_RATIO = 2.0 ** -24, 2.0 ** 24, 4.0
RB = 256
PC = 32
P0, PSTEP, PD = 440, 30, 52
NLN, LN0, LNS = 4, 4, 5
LP = 16
SP0, SP1 = 76, 38
_prologue = lambda: ('|kva|Z; |b|; kva|wc|K0123; bw|xdn|C0@56 N0123@52 K4567; cx|mq|N4567@52 F0@56 K89ab; '
            'd|y|C1@56 F1@56 Kcdef; nmq|zo|M H01 H234567@30 F2@36 Q0123; y||H89ab@30 F3@36 Q4567; '
            'zo||L Hcdef@30 S0@%d Q89ab S1@%d Qcdef' % (SP0, SP1))


def _dot(a, b):
    return jnp.dot(a, b, preferred_element_type=F32)


def _dot_nt(a, b):
    return jax.lax.dot_general(a, b, NT, preferred_element_type=F32)


def _ln(x):
    m = jnp.mean(x, axis=-1, keepdims=True)
    xc = x - m
    v = jnp.mean(xc * xc, axis=-1, keepdims=True)
    return xc * jnp.exp2(jnp.log(v + EPS) * (-0.5 * LOG2E))


def _rows(v, n):
    return jnp.broadcast_to(v[None], (n // 8, 8, v.shape[1])).reshape(n, v.shape[1])


def _gelu(x):
    c0 = math.sqrt(2.0 / math.pi)
    return 0.5 * x * (1.0 + jnp.tanh(c0 * (x + 0.044715 * (x * x * x))))


def _after(x, dep):
    return jnp.where(dep > jnp.inf, dep, x)


def _tie(x, dep):
    xu = pltpu.bitcast(x, U32)
    first = jnp.where(dep > jnp.inf, jnp.uint32(0), xu[:8])
    return pltpu.bitcast(jnp.concatenate([first, xu[8:]], axis=0), BF16)


def _tile(j):
    return slice(j * T, (j + 1) * T)


def _ld(ref, *idx):
    return pltpu.bitcast(ref.bitcast(U32)[idx], BF16)


def _a_ops(a11, a12, a21, a22):
    return [a11 + a22, a21 + a22, a11, a22, a11 + a12, a21 - a11, a12 - a22]


def _b_ops(b11, b12, b21, b22):
    return [b11 + b22, b11, b12 - b22, b21 - b11, b22, b11 + b12, b21 + b22]


def _strassen(prod, col1=None, col2=None):
    m4 = prod(3)
    m2 = prod(1)
    c21 = m2 + m4
    if col1 is not None:
        e11, e21 = col1()
        m4, c21 = m4 + e11, c21 + e21
    m3 = prod(2)
    m5 = prod(4)
    c12 = m3 + m5
    if col2 is not None:
        e12, e22 = col2()
        c12, m3 = c12 + e12, m3 + e22
    m1 = prod(0)
    c11 = prod(6) + (m1 + (m4 - m5))
    c22 = prod(5) + (m1 + (m3 - m2))
    return c11, c12, c21, c22


def _group(rows, cols, pairs):
    xs, ys = dict.fromkeys(x for x, _ in pairs), dict.fromkeys(y for _, y in pairs)
    used = set(xs) | set(ys) | {(x[0], y[1]) for x, y in pairs} | {(y[0], x[1]) for x, y in pairs}
    prods = []
    for n, r in enumerate(rows):
        for i, k in [x for x in xs if x[0] == r]:
            mates = [y for x, y in pairs if x == (i, k)]
            prods.append((((1, i, k),) + tuple((1, i, k2) for _, k2 in mates), ((1, k, 0),),
                          ((1, i, 0), (-1, i, 1))))
            prods.append((((1, i, k),) + tuple((-1, i2, k) for i2, _ in mates), ((1, k, 0), (1, k, 1)),
                          ((1, i, 1),)))
        for i2, k2 in [y for y in ys if y[0] == r]:
            mates = [x for x, y in pairs if y == (i2, k2)]
            prods.append((((1, i2, k2),) + tuple((1, i2, k) for _, k in mates), ((1, k2, 1),),
                          ((1, i2, 1), (-1, i2, 0))))
            prods.append((((1, i2, k2),) + tuple((-1, i, k2) for i, _ in mates), ((1, k2, 0), (1, k2, 1)),
                          ((1, i2, 0),)))
        prods += [(((1, r, k),), ((1, k, h),), ((1, r, h),)) for k in cols if (r, k) not in used for h in (0, 1)]
        for (i, k), (i2, k2) in pairs:
            if r in (i, i2) and i + i2 - r in rows[n + 1:]:
                prods.append((((1, i, k2),), ((1, k2, 0), (-1, k, 0)), ((1, i2, 0), (1, i, 0))))
                prods.append((((1, i2, k), (1, i, k2)), ((1, k, 0), (1, k2, 1)), ((1, i2, 0), (1, i, 1))))
                prods.append((((1, i2, k),), ((1, k, 1), (-1, k2, 1)), ((1, i2, 1), (1, i, 1))))
    return prods


def _all_pairs(xrows, yrows):
    return [((x, a), (y, b)) for a, x in enumerate(xrows) for b, y in enumerate(yrows) if a != b]


_PAIRS65 = [((x[0] + 10, x[1]), (y[0] + 10, y[1])) for x, y in (
    ((0, 1), (1, 0)), ((0, 1), (5, 2)), ((2, 3), (1, 0)), ((2, 3), (3, 1)), ((2, 3), (5, 2)), ((3, 2), (1, 0)),
    ((4, 4), (0, 3)), ((4, 4), (1, 0)), ((4, 4), (3, 1)), ((4, 4), (5, 2)))]
_C_GROUPS = [_group(range(r, r + 8), range(4), _all_pairs(range(r, r + 4), range(r + 4, r + 8))) for r in (0, 8)]
_H_GROUPS = [_group(range(10), range(5), _all_pairs(range(5), range(5, 10))),
             _group(range(10, 16), range(5), _PAIRS65)]
_sum_index = lambda groups: {f: n for n, f in enumerate(
    dict.fromkeys(t[0] for g in groups for t in g if len(t[0]) > 1))}
_C_SUMS, _H_SUMS = _sum_index(_C_GROUPS), _sum_index(_H_GROUPS)


def _form(form, get):
    acc = None
    for sign, i, j in form:
        v = get(i, j)
        acc = v if acc is None else (acc + v if sign > 0 else acc - v)
    return acc


def _gap_items(bufs, gap_scr):
    items = []
    for n, buf in enumerate(bufs):
        acc = []

        def part(r0, buf=buf, acc=acc):
            def fn(dep):
                wu = jnp.concatenate([buf[r:r + 8, :] for r in range(r0, r0 + T, 32)])
                mask = jnp.full((8, T), 0x7FFF0000, U32)
                if dep is not None:
                    mask = jnp.where(dep > jnp.inf, jnp.uint32(0), mask)
                mask = _rows(mask, 32)
                new = [jnp.sum(pltpu.bitcast(v & mask, F32).reshape(4, 8, T), axis=0) for v in (wu << 16, wu)]
                acc[:] = [u + v for u, v in zip(acc, new)] if acc else new
            return fn

        def last(_, n=n, acc=acc):
            bits = []
            for v in acc:
                l1 = jnp.sum(jnp.sum(v, axis=1, keepdims=True), axis=0, keepdims=True)
                bits.append(pltpu.bitcast(jnp.broadcast_to(l1, (8, T)), jnp.int32) >> 8)
            gap = jnp.clip((bits[0] - bits[1] + (1 << 14)) >> 15, -8, 8) << 23
            gap_scr[n] = gap
            return pltpu.bitcast(gap, F32)

        items += [part(r0) for r0 in range(0, buf.shape[0], T)] + [last]
    return items


def _pair_tiles(w_ref, transpose=False):
    tiles = {}
    for j in range(w_ref.shape[0] // T):
        wu = w_ref[_tile(j), :]
        if transpose:
            wu = wu.T
        tiles[j, 0] = pltpu.bitcast(wu << 16, F32).astype(BF16)
        tiles[j, 1] = pltpu.bitcast(wu & jnp.uint32(0xFFFF0000), F32).astype(BF16)
    return tiles


def _canon(form):
    if form[-1][0] < 0 and form[0][1:] > form[1][1:]:
        return -1, ((1,) + form[1][1:], (-1,) + form[0][1:])
    return 1, form


_w_forms = lambda groups: list(dict.fromkeys(_canon(t[1])[1] for g in groups for t in g))
_WF = {key: n for n, key in enumerate([(m, f) for m, groups in enumerate((_C_GROUPS, _C_GROUPS, _H_GROUPS))
                                       for f in _w_forms(groups)])}


def _weight_form_items(bufs, gap_scr, wt_scr, wf_scr, which):
    n = 16
    items = []

    def flip(j):
        def fn(dep):
            wu = bufs[1][_tile(j), :]
            wu = (wu if dep is None else jnp.where(_rows(dep, T) > jnp.inf, jnp.uint32(0), wu)).T
            wt_scr[j] = wu
            return pltpu.bitcast(wu[T - 8:], F32)
        return fn

    def part(m, r0, forms):
        def fn(dep):
            fac = pltpu.bitcast(0x3F800000 + gap_scr[m], F32)
            mask = jnp.full((8, T), 0xFFFF0000, U32)
            sh = jnp.full((8, T), 16, U32)
            if dep is not None:
                mask = jnp.where(dep > jnp.inf, jnp.uint32(0), mask)
                sh = jnp.where(dep > jnp.inf, jnp.uint32(0), sh)
            fac, mask, sh = _rows(fac, n), _rows(mask, n), _rows(sh, n)
            base = {}

            def get(k, h):
                if (k, h) not in base:
                    wu = wt_scr[k, r0:r0 + n, :] if m == 1 else bufs[m][k * T + r0:k * T + r0 + n, :]
                    base[k, h] = pltpu.bitcast(wu & mask, F32) * fac if h else pltpu.bitcast(wu << sh, F32)
                return base[k, h]

            for f in forms:
                wf_scr[_WF[m, f], r0:r0 + n, :] = _form(f, get).astype(BF16)
        return fn

    for m in which:
        forms = [f for mm, f in _WF if mm == m]
        if m == 1:
            items += [flip(j) for j in range(bufs[1].shape[0] // T)]
        per = -(-len(forms) // WFN[m])
        forms.sort(key=lambda f: sorted({t[1] for t in f}))
        items += [part(m, r0, forms[i:i + per]) for r0 in range(0, T, n) for i in range(0, len(forms), per)]
    return items


def _run_group(jobs, prods, a_get, w, transposed, finish):
    left = {}
    for _, _, outs in prods:
        for _, i, h in outs:
            left[i, h] = left.get((i, h), 0) + 1
    acc = {}
    for af, bf, outs in prods:
        sign, wt = w(bf)
        m = jobs.mm([wt], [a_get(af)], _dot_nt) if transposed else jobs.mm([a_get(af)], [wt], _dot)
        for s_, i, h in outs:
            if (i, h) not in acc:
                acc[i, h] = (s_ * sign, m)
            else:
                s0, v = acc[i, h]
                acc[i, h] = (s0, v + m if s0 == s_ * sign else v - m) if s0 > 0 or s_ * sign < 0 else (1, m - v)
            left[i, h] -= 1
            if not left[i, h]:
                s0, v = acc.pop((i, h))
                assert s0 > 0
                finish(2 * i + h, v)


class _Jobs:
    def __init__(self, side=()):
        self.res = []
        self.side = list(side)

    def mm(self, lhs, wt, dot):
        acc = None
        for x, w in zip(lhs, wt):
            v = dot(x, w)
            self.res.append(v)
            acc = v if acc is None else v + acc
            rel = 4 * (len(self.res) % 4)
            while self.side and self.side[0][0] <= len(self.res):
                self.side.pop(0)[1](v[8 * rel:8 * rel + 8, :])
                rel = (rel + 2) % 16
        return acc


def _proj_step(h_scr, hs_scr, c_ref, cs_scr, wf_scr, q_scr, k_scr, v_scr, pf, scale, shifts, side):
    def weight(m):
        def get(form):
            sign, form = _canon(form)
            return sign, _ld(wf_scr, _WF[m, form])
        get.inv = pltpu.bitcast(0x3F800000 - shifts[m], F32)
        return get

    wk, wvT, wq = weight(0), weight(1), weight(2)
    c_get = lambda f: _ld(cs_scr, _C_SUMS[f]) if len(f) > 1 else c_ref[_tile(f[0][1]), _tile(f[0][2])]
    h_get = lambda f: _ld(hs_scr, _H_SUMS[f]) if len(f) > 1 else _ld(h_scr, f[0][1], f[0][2])

    def put(dst, w, mul=None):
        muls = [mul, _rows(w.inv if mul is None else w.inv * mul, T)]

        def fn(u, v):
            v = (v if muls[u % 2] is None else v * muls[u % 2]).astype(BF16)
            dst[u] = v.T if mul is not None and u in QT else v
        return fn

    jobs = _Jobs(side)
    put_v, stored = put(v_scr, wvT), set()
    nxt = [0]

    def fin_v(u, v):
        put_v(u, v)
        stored.add(u)
        for J in range(SB):
            if all(2 * (SB * J + k) + h in stored for k in range(SB) for h in range(2)) and ('J', J) not in stored:
                stored.add(('J', J))
                for fn in _v_form_items(v_scr, pf, J):
                    nxt[0] = max(nxt[0] + VFS, len(jobs.res) + VF0)
                    jobs.side.append((int(nxt[0]), fn))
                jobs.side.sort(key=lambda e: e[0])

    kk, vv, qq = ((c_get, wk, False, put(k_scr, wk)), (c_get, wvT, True, fin_v),
                  (h_get, wq, False, put(q_scr, wq, scale)))
    for prods, args in ((_C_GROUPS[0], kk), (_C_GROUPS[0], vv), (_C_GROUPS[1], vv), (_C_GROUPS[1], kk),
                        (_H_GROUPS[0], qq), (_H_GROUPS[1], qq)):
        _run_group(jobs, prods, *args)
    assert not jobs.side


def _inner_group(rows, cols, pairs):
    xs, ys = dict.fromkeys(x for x, _ in pairs), dict.fromkeys(y for _, y in pairs)
    used = set(xs) | set(ys) | {(x[0], y[1]) for x, y in pairs} | {(y[0], x[1]) for x, y in pairs}
    prods = []
    for i, j in xs:
        mates = [y for x, y in pairs if x == (i, j)]
        prods.append((((1, i, 0),), ((1, 0, j), (-1, 1, j)), ((1, i, j),) + tuple((1, i2, j) for i2, _ in mates)))
        prods.append((((1, i, 0), (1, i, 1)), ((1, 1, j),), ((1, i, j),) + tuple((-1, i, j2) for _, j2 in mates)))
    for i2, j2 in ys:
        mates = [x for x, y in pairs if y == (i2, j2)]
        prods.append((((1, i2, 0), (1, i2, 1)), ((1, 0, j2),),
                      ((1, i2, j2),) + tuple((-1, i2, j) for _, j in mates)))
        prods.append((((1, i2, 1),), ((1, 0, j2), (-1, 1, j2)),
                      ((-1, i2, j2),) + tuple((-1, i, j2) for i, _ in mates)))
    prods += [(((1, i, h),), ((1, h, j),), ((1, i, j),))
              for i in rows for j in cols if (i, j) not in used for h in (0, 1)]
    for (i, j), (i2, j2) in pairs:
        lo, hi = min(j, j2), max(j, j2)
        prods.append((((1, i2, 0), (-1, i, 0)), ((1, 0, lo), (1, 0, hi)), ((1, i2, j),)))
        prods.append((((1, i, 0), (1, i2, 1)), ((1, 0, j2), (1, 1, j)), ((1, i, j2), (1, i2, j))))
        prods.append((((1, i, 1), (-1, i2, 1)), ((1, 1, lo), (1, 1, hi)), ((1, i, j2),)))
    return prods


def _o_jobs():
    prods = (_inner_group(range(10), range(5), _all_pairs(range(0, 10, 2), range(1, 10, 2)))
             + _inner_group(range(10, 16), range(5), _PAIRS65))
    row = lambda t: max(i for _, i, _ in t[0])
    unit = lambda t: max(2 * i + h for _, i, h in t[0])
    need = lambda t: unit(t) if row(t) == 15 else 2 * row(t) + 1
    return [(need(t), t) for t in sorted(prods, key=need)]


_O_JOBS = _o_jobs()


SB = 4


class _Star:
    def __init__(self, ts):
        self.ts, self.n = ts, len(ts)
        rn = range(self.n)
        self.pairs = [(i, j) for i in rn for j in rn if i < j]
        self.pf = {f: m for m, f in enumerate([('R', i) for i in rn] + [('C', i) for i in rn]
                                              + [('S', i, j) for i in rn for j in rn if i != j]
                                              + [('A', i, j) for i, j in self.pairs])}
        self.vf = {f: m for m, f in enumerate([('W', i) for i in rn]
                                              + [(q, i, j) for i, j in self.pairs for q in ('Q1', 'Q2', 'Q3')])}
        self.pv = {**{('W', i): ('R', i) for i in rn}, **{('B', i): ('C', i) for i in rn},
                   **{('Q1', i, j): ('S', i, j) for i, j in self.pairs},
                   **{('Q2', i, j): ('A', i, j) for i, j in self.pairs},
                   **{('Q3', i, j): ('S', j, i) for i, j in self.pairs}}

    def products(self, i):
        return [('W', i), ('B', i)] + [(q, i, j) for j in range(i + 1, self.n) for q in ('Q1', 'Q2', 'Q3')]


_FULL = _Star((-1.125, -0.375, 0.375, 1.125))
_HALF = _Star((-0.75, 0.75))
_DCELLS = [(0, 0), (1, 0), (1, 1), (2, 2), (3, 2), (3, 3)]
_HSLOT = (SB - 1) * len(_FULL.pf)
_DSLOT = _HSLOT + len(_HALF.pf)
_VSLOT = _DSLOT + len(_DCELLS)
_VHALF = (SB - 1) * len(_FULL.vf)
_FENCE = _VSLOT + (_VHALF + SB * len(_HALF.vf) + 1) // 2


def _v_slot(star, J, f):
    m = star.vf[f] + J * len(star.vf) + (0 if star is _FULL else _VHALF)
    return _VSLOT + m // 2, m % 2 * (T // 2)


def _v_form_items(v_scr, pf, J):
    n, HT = 16, T // 2

    def item(star, h, r0, pairs):
        def fn(dep):
            ts = [jnp.full((8, T), t, F32) for t in star.ts]
            ts = [_rows(t if dep is None else _after(t, dep), n) for t in ts]

            def get(k, a):
                r = (a * HT + r0) // 2
                return _ld(v_scr, 2 * (SB * J + k) + h, slice(r, r + n // 2)).astype(F32)

            def put(f, v):
                slot, r = _v_slot(star, J, f)
                pf[h][slot, r + r0:r + r0 + n, :] = v.astype(BF16)

            b = {(k, a): get(k, a) for k in sorted({k for pr in pairs or star.pairs for k in pr})
                 for a in range(2)}
            if pairs is None or star.n == 2:
                w = [b[k, 0] + ts[k] * b[k, 1] for k in range(star.n)]
                for k in range(star.n):
                    put(('W', k), w[k])
                for i, j in star.pairs:
                    put(('Q2', i, j), w[i] - w[j])
            for i, j in pairs or ():
                d0, d1 = b[j, 0] - b[i, 0], b[j, 1] - b[i, 1]
                put(('Q1', i, j), d0 + ts[i] * d1)
                put(('Q3', i, j), d0 + ts[j] * d1)
        return fn

    pr = _FULL.pairs
    parts = [(_HALF, _HALF.pairs)]
    if J < SB - 1:
        parts += [(_FULL, x) for x in (None, pr[:2], [pr[2], pr[4]], [pr[3], pr[5]])]
    return [item(star, h, r0, pairs) for h in range(2) for r0 in range(0, HT, n) for star, pairs in parts]


def _job_order(nsb):
    units = [(I, h) for I in range(nsb) for h in range(2)]
    qe, qv = [], []
    for I, h in units:
        es = [('e', I, h, J, p) for J in range(I) for p in range(SB)]
        ds = [('d', I, h) + c for c in _DCELLS]
        es.insert(max(len(es) - FPOS, 0), ('f', I, h))
        qe += es + ds if I or FPOS < 9 else ds[:DPOS] + es + ds[DPOS:]
        for i in range(SB):
            qv += [('p', I, h, f, J) for f in _FULL.products(i) for J in range(I)]
            if i >= 2:
                qv += [('p', I, h, f, None) for f in _HALF.products(i - 2)]
            qv += [('v', I, h) + c for c in _DCELLS if c[0] == i]
    qo = [('o', u, j) for j, (u, _) in enumerate(_O_JOBS)]
    cost = dict(e=8, f=8, d=2, p=1, v=2, o=2)
    order, done = [], {}
    now = [0]

    def emit(q):
        job = q.pop(0)
        order.append(job)
        now[0] += cost[job[0]]
        if job[0] == 'd':
            done[job] = now[0]
        elif job[0] == 'v' and job[4] == job[3]:
            done['u', 2 * (SB * job[1] + job[3]) + job[2]] = now[0]
        return cost[job[0]]

    def v_ready():
        if not qv:
            return False
        key = ('d', qv[0][1], qv[0][2], SB - 1, SB - 1)
        return key in done and done[key] + (LAT_0 if qv[0][1:3] == (0, 0) else LAT_A) <= now[0]

    def o_ready():
        return bool(qo) and ('u', qo[0][1]) in done and done['u', qo[0][1]] + LAT_B <= now[0]

    def fill(nv, no):
        n = 0
        while nv > 0 or no > 0 or n % 4:
            if no > 0 and n % 2 == 0 and o_ready() and no * ONV >= nv:
                no -= 2
                n += emit(qo)
            elif v_ready() and (nv > 0 or n % 4):
                c = emit(qv)
                nv -= c
                n += c
            elif o_ready() and n % 2 == 0 and (no > 0 or n % 4 or nv > 0) and len(qo) > RES:
                no -= 2
                n += emit(qo)
            else:
                break

    while qe:
        unit = qe[0][1:3]
        while qv and qv[0][2] == unit[1] and qv[0][1] < unit[0]:
            emit(qv)
        ne = 0
        while qe and ne < 8 and (ne == 0 or (qe[0][0] == 'd' and qe[0][1:3] == unit and ne + 2 <= 8)):
            ne += emit(qe)
        groups = lambda q: sum(cost[j[0]] for j in q) / 8
        old = [j for j in qv if j[1:3] != unit and ('d', j[1], j[2], SB - 1, SB - 1) in done]
        here = [j for j in qe if j[1:3] == unit]
        rest = sum(cost[j[0]] for j in old)
        nv = (rest - LAT_A) / (groups(here) + 1) if here else rest
        no = 2 * max(len(qo) - RES - OEND, 0) / (groups(qe) + 1)
        fill(int(nv + 0.5), int(no + 0.5))
    while qv or qo:
        if qv and v_ready():
            fill(6, 2)
            if not qv:
                continue
        elif o_ready():
            emit(qo)
        else:
            emit(qv or qo)
    return order


def _attention_safe(q_scr, k_scr, v_scr, wo_ref, acc_scr):
    causal = (jax.lax.broadcasted_iota(jnp.int32, (T, T), 0)
              <= jax.lax.broadcasted_iota(jnp.int32, (T, T), 1))

    def unit(u, carry):
        r, hd = u // 2, u % 2

        def block(c, mlo):
            m0, l, o = mlo
            s = _dot_nt(_ld(k_scr, 2 * c + hd), _ld(q_scr, u))
            s = jnp.where(jnp.logical_or(causal, c < r), s, -1e9 * LOG2E)
            m = jnp.maximum(m0, jnp.max(s, axis=0, keepdims=True))
            a = jnp.exp2(m0 - m)
            p = jnp.exp2(s - m)
            return (m, l * a + jnp.sum(p, axis=0, keepdims=True),
                    o * a + _dot(_ld(v_scr, 2 * c + hd), p.astype(BF16)))

        _, l, o = jax.lax.fori_loop(0, r + 1, block, (jnp.full((1, T), -jnp.inf, F32), jnp.zeros((1, T), F32),
                                                      jnp.zeros((T, T), F32)))
        rows = pl.ds(pl.multiple_of(r * T, T), T)
        acc_scr[rows, :] += _dot((o * (1.0 / l)).astype(BF16).T, wo_ref[pl.ds(pl.multiple_of(hd * T, T), T), :])
        return carry

    jax.lax.fori_loop(0, q_scr.shape[0], unit, 0)


def _attention_step(q_scr, k_scr, v_scr, pf, wo_ref, acc_scr, flag_scr, z, side):
    causal = (jax.lax.broadcasted_iota(jnp.int32, (T, T), 0)
              <= jax.lax.broadcasted_iota(jnp.int32, (T, T), 1))
    HT = T // 2
    lsum, lrow, acc, fg, dacc, of, lhs = {}, {}, {}, {}, {}, {}, {}
    res = []
    wo, terms = {}, {}
    left = {}
    done_side = [0, 0]
    chk = [jnp.zeros((8, T), F32), None]
    for _, t in _O_JOBS:
        for _, i, j in t[2]:
            left[i, j] = left.get((i, j), 0) + 1

    def add_l(u, v):
        lsum[u] = v if u not in lsum else lsum[u] + v

    csign = {}

    def p_forms(star, h, slot0, g, tiles, cell, when):
        n = star.n

        def put(f, v):
            pf[h][slot0 + star.pf[f], 16 * g:16 * g + 16, :] = v.astype(BF16)

        for i in range(n):
            row = [cell(i, k) for k in sorted(range(n), key=lambda k: when(i, k))]
            r = functools.reduce(lambda x, y: x + y, row)
            put(('R', i), r)
            add_l(tiles[i], r[:8] + r[8:])
            col = sorted(range(n), key=lambda i2: (when(i2, i), i2 != i))
            sign = csign[n, i] = 1 if col[0] == i else -1
            c = cell(col[0], i)
            for i2 in col[1:]:
                c = c + cell(i2, i) if (1 if i2 == i else -1) == sign else c - cell(i2, i)
            put(('C', i), c)
            for j in range(n):
                if j != i:
                    put(('S', i, j), cell(i, j))
        for i, j in star.pairs:
            put(('A', i, j), cell(i, j) + cell(j, i))

    due = []

    def scores(x, u):
        if due and due[0][0] <= done_side[1]:
            x = _tie(x, due.pop(0)[1])
        s = (_dot if u in QT else _dot_nt)(x, _ld(q_scr, u))
        res.append(s)
        return s

    def job_e(I, h, J, p):
        tiles = [2 * (SB * I + i) + h for i in range(SB)]
        ps = []
        for i, u in enumerate(tiles):
            x = jnp.concatenate([k_scr.bitcast(U32)[2 * (SB * J + (t - i) % SB) + h, 8 * g:8 * g + 8, :]
                                 for g in (2 * p, 2 * p + 1) for t in range(SB)], axis=0)
            ps.append(jnp.exp2(scores(pltpu.bitcast(x, BF16), u)))
        when = lambda i, k: (i + k) % SB
        for n, g in enumerate((2 * p, 2 * p + 1)):
            cell = lambda i, k: ps[i][16 * (SB * n + when(i, k)):16 * (SB * n + when(i, k)) + 16]
            p_forms(_FULL, h, J * len(_FULL.pf), g, tiles, cell, when)

    def job_f(I, h):
        tiles = [2 * (SB * I + 2 + i) + h for i in range(2)]
        ps = {(i, k): jnp.exp2(scores(_ld(k_scr, 2 * (SB * I + k) + h), u))
              for i, u in enumerate(tiles) for k in range(2)}
        for g in range(T // 16):
            p_forms(_HALF, h, _HSLOT, g, tiles, lambda i, k: ps[i, k][16 * g:16 * g + 16], lambda i, k: 0)

    def job_d(I, h, i, k):
        u = 2 * (SB * I + i) + h
        s = scores(_ld(k_scr, 2 * (SB * I + k) + h), u)
        if i == k:
            s = jnp.where(causal, s, -1e9 * LOG2E)
        p = jnp.exp2(s)
        add_l(u, jnp.sum(p.reshape(T // 8, 8, T), axis=0))
        pf[h][_DSLOT + _DCELLS.index((i, k))] = p.astype(BF16)
        if (i, k) == _DCELLS[-1]:
            pf[h][_FENCE + z, 0:16, :] = jnp.zeros((16, T), BF16)
            for u in [2 * (SB * I + a) + h for a in range(SB)]:
                lrow[u] = jnp.sum(lsum.pop(u), axis=0, keepdims=True)
            ls = [lrow[2 * (SB * I + a) + h] for a in range(SB)]
            lo = jnp.minimum(jnp.minimum(ls[0], ls[1]), jnp.minimum(ls[2], ls[3]))
            hi = jnp.maximum(jnp.maximum(ls[0], ls[1]), jnp.maximum(ls[2], ls[3]))
            ok = jnp.logical_and(lo >= L_LO, hi <= L_HI)
            ok = jnp.logical_and(ok, (hi if I else jnp.maximum(ls[2], ls[3]))
                                 <= L_RATIO * (lo if I else jnp.minimum(ls[2], ls[3])))
            bad = jnp.where(ok, 0.0, 1.0)
            chk[1] = bad if chk[1] is None else jnp.maximum(chk[1], bad)

    def job_p(I, h, f, J):
        star, last = (_HALF, True) if J is None else (_FULL, J == I - 1)
        blk = I if J is None else J
        if f[0] == 'B':
            x = _ld(v_scr, 2 * (SB * blk + f[1]) + h, slice(HT // 2, HT))
        else:
            slot, r = _v_slot(star, blk, f)
            x = _ld(pf[h], slot, slice(r // 2, (r + HT) // 2))
        v = _dot(x, _ld(pf[h], (_HSLOT if J is None else J * len(_FULL.pf)) + star.pf[star.pv[f]]))
        res.append(v)
        key = (star.n,) + f
        acc[key] = v if key not in acc else acc[key] + v
        if not last:
            return

        def add(which, i, v, sign=1):
            k_ = (star.n, which, i)
            if k_ not in fg:
                fg[k_] = v if sign > 0 else -v
            else:
                fg[k_] = fg[k_] + v if sign > 0 else fg[k_] - v

        if f[0] == 'W':
            add('F', f[1], acc.pop(key))
        elif f[0] == 'B':
            add('G', f[1], acc.pop(key), csign[star.n, f[1]])
        elif f[0] == 'Q3':
            _, i, j = f
            q1, q2, q3 = (acc.pop((star.n, q, i, j)) for q in ('Q1', 'Q2', 'Q3'))
            t = ((q1 + q2) + q3) * (1.0 / (star.ts[i] - star.ts[j]))
            add('G', i, t)
            add('G', j, t)
            add('F', i, q1)
            add('F', j, q3, -1)

    def job_v(I, h, i, k):
        u = 2 * (SB * I + i) + h
        v = _dot(_ld(v_scr, 2 * (SB * I + k) + h), _ld(pf[h], _DSLOT + _DCELLS.index((i, k))))
        res.append(v)
        dacc[u] = v if u not in dacc else dacc[u] + v
        if k == i:
            o = dacc.pop(u)
            for star, a in ([(_FULL, i)] if I else []) + ([(_HALF, i - 2)] if i >= 2 else []):
                f, g = fg.pop((star.n, 'F', a)), fg.pop((star.n, 'G', a))
                o = o + jnp.concatenate([f - star.ts[a] * g, g], axis=0)
            o = o * (1.0 / lrow[u])
            of[u] = o
            chk[0] = chk[0] + jnp.sum(o.reshape(T // 8, 8, T), axis=0)

    def job_o(_, n):
        af, bf, outs = _O_JOBS[n][1]
        if af not in lhs:
            v = _form(af, lambda i, h: of[2 * i + h])
            lhs[af] = _tie(v.astype(BF16).T, v[0:8, :])
        if bf not in wo:
            wo[bf] = (wo_ref[_tile(bf[0][1]), _tile(bf[0][2])] if len(bf) == 1 else
                      _form(bf, lambda h, j: wo_ref[_tile(h), _tile(j)].astype(F32)).astype(BF16))
            if HACKWO:
                wo[bf] = _ld(q_scr, len(wo) % 32)
        v = _dot(lhs[af], wo[bf])
        res.append(v)
        for sign, i, j in outs:
            terms.setdefault((i, j), []).append((sign, v))
            if len(terms[i, j]) == left[i, j]:
                tot = acc_scr[_tile(i), _tile(j)]
                for sg, m in terms.pop((i, j)):
                    tot = tot + m if sg > 0 else tot - m
                acc_scr[_tile(i), _tile(j)] = tot

    fns = dict(e=job_e, f=job_f, d=job_d, p=job_p, v=job_v, o=job_o)
    order = _job_order(q_scr.shape[0] // (2 * SB))
    for n, job in enumerate(order):
        assert job[0] not in 'efd' or not any(j[0] in 'pv' and j[2] == job[2] and j[1] < job[1] for j in order[n:])
    side = list(side)
    fences = [n for n, job in enumerate(order) if job[0] == 'd' and job[3:] == _DCELLS[-1]]
    step = (len(order) - SIDE0 - SIDE1 - 10) / len(side)
    for n, job in enumerate(order):
        done_side[1] = n
        fns[job[0]](*job[1:])
        last_chance = n >= len(order) - SIDE1
        near = any(-SG1 <= f - n <= SG0 for f in fences)
        if side and n >= SIDE0 + step * done_side[0] and ((job[0] in SKIND and not near) or last_chance):
            done_side[0] += 1
            v = side.pop(0)(res[-1 - SLAG][8 * (n % 4):8 * (n % 4) + 8, :])
            if v is not None:
                due.append((n + SDUE, v))
    assert not side and not due
    fine = jnp.abs(chk[0]) < jnp.inf
    flag_scr[...] = jnp.maximum(flag_scr[...], jnp.where(fine, chk[1], 1.0))


def _kernel(x_hbm, c_hbm, wq_hbm, wuk_hbm, wuv_hbm, wo_hbm, w1_hbm, w2_hbm, w3_hbm, w4_hbm,
            cond_hbm, wmod_hbm, out_hbm,
            x_ref, c_ref, cond_ref, wma_ref, wmb_ref, w1_ref, w2_ref, w3_ref, w4_ref,
            wq_buf, wk_buf, wv_buf, wo_buf, out_buf, sem, wsem, osem,
            mod_scr, h_scr, cs_scr, hs_scr, w_scr, q_scr, k_scr, v_scr, acc_scr, xn_scr, xh_scr, a1_scr, t_scr,
            ws12, ws3, ws4, wt_scr, wf_scr, gap_scr, st_in, pf_scr, vf_scr, flag_scr):
    S, M = x_hbm.shape
    D = wq_hbm.shape[2]
    nattn = wo_hbm.shape[0]
    Fd = w4_hbm.shape[0]
    scale = float(D) ** -0.5 * LOG2E
    nb, nrb = S // T, S // RB
    km, kc = M // T, c_hbm.shape[1] // T
    NX = 4
    XR = S // NX
    CB = XR // T

    work = (wk_buf, wv_buf, wq_buf)

    def pcopies(g, bufs=work, s0=0):
        return [pltpu.make_async_copy(src.bitcast(U32).at[:, g, :], dst, wsem.at[s0 + j])
                for j, (src, dst) in enumerate(zip((wuk_hbm, wuv_hbm, wq_hbm), bufs))]

    def ocopy(g):
        return pltpu.make_async_copy(wo_hbm.at[g], wo_buf, wsem.at[3])

    def chunk_copy(src, dst, i, s0):
        rows = slice(i * XR, (i + 1) * XR)
        return pltpu.make_async_copy(src.at[rows, :], dst.at[rows, :], sem.at[s0 + i])

    FH = ws3.shape[0] * T
    assert nattn - 1 >= FH // 64

    slices = ((w1_hbm, 32, 2 * T, 0), (w2_hbm, 32, 2 * T, 64), (w4_hbm, 64, FH, 128), (w3_hbm, T, FH, 256))
    slice_of = lambda g, n, half: jnp.minimum(g, half // n - 1)

    def prep_in(g):
        return [pltpu.make_async_copy(
            w.at[pl.ds(pl.multiple_of(slice_of(g, n, half) * n + x * half, n), n), 0:4 * T],
            st_in.at[r0 + x * n:r0 + (x + 1) * n, :], wsem.at[7]) for w, n, half, r0 in slices for x in range(2)]

    def stage_in(g):
        return pcopies(jnp.minimum(g + 1, nattn - 1))

    cp_cond = pltpu.make_async_copy(cond_hbm, cond_ref, sem.at[0])
    cp_wma = pltpu.make_async_copy(wmod_hbm.at[:, 0:2 * M], wma_ref, sem.at[1])
    cp_late = [pltpu.make_async_copy(src, dst, sem.at[2 + j]) for j, (src, dst) in enumerate((
        (wmod_hbm.at[:, 2 * M:6 * M], wmb_ref), (w1_hbm, w1_ref), (w2_hbm, w2_ref),
        (w3_hbm, w3_ref), (w4_hbm, w4_ref)))]
    cp_x = [chunk_copy(x_hbm, x_ref, i, 7) for i in range(NX)]
    cp_c = [chunk_copy(c_hbm, c_ref, i, 7 + NX) for i in range(NX)]

    def silu_cond():
        cf = cond_ref[...].astype(F32)
        return jnp.broadcast_to((cf * jax.nn.sigmoid(cf)).astype(BF16), (8, M))

    cp_wk, cp_wv, cp_wq = pcopies(0)
    named = dict(k=cp_wk, v=cp_wv, q=cp_wq, o=ocopy(0), n=cp_cond, m=cp_wma)
    named.update(zip('abcd', cp_c))
    named.update(zip('wxyz', cp_x))
    started, arrived, did = set(), set(), set()

    def zero(r, carry):
        acc_scr[pl.ds(pl.multiple_of(r * T, T), T), :] = jnp.zeros((T, M), F32)
        return carry

    def x_rows(rows, dep):
        xf = x_ref[rows, :].astype(F32)
        if dep is None:
            return xf
        return jnp.concatenate([_after(xf[:, :T], _rows(dep, xf.shape[0])), xf[:, T:]], axis=1)

    def n_item(r, i):
        def fn(dep):
            rows = slice(r * T + i * LP, r * T + (i + 1) * LP)
            xn_scr[rows, :] = _ln(x_rows(rows, dep))
        return fn

    def h_item(r, i, normed):
        def fn(dep):
            rows = slice(i * LP, (i + 1) * LP)
            grows = slice(r * T + i * LP, r * T + (i + 1) * LP)
            sa = mod_scr[:, 0:M]
            if normed and dep is not None:
                sa = jnp.concatenate([_after(sa[:, _tile(j)], dep) for j in range(km)], axis=1)
            hf = ((xn_scr[grows, :] if normed else _ln(x_rows(grows, dep))) * _rows(mod_scr[:, M:2 * M], LP)
                  + _rows(sa, LP))
            for j in range(km):
                h_scr[r, j, rows, :] = hf[:, _tile(j)].astype(BF16)
            for f, n in _H_SUMS.items():
                if all(t[1] == r for t in f):
                    hs_scr[n, rows, :] = _form(f, lambda _, k: hf[:, _tile(k)]).astype(BF16)
            did.add(('h', r, i))
        return fn

    def release(jobs, span, items):
        if span and items:
            jobs.side += [(len(jobs.res) + 1 + i * span // len(items), fn) for i, fn in enumerate(items)]
            jobs.side.sort(key=lambda e: e[0])
        else:
            for fn in items:
                fn(None)

    def sum_items(n, group, index, dst, get, skip_rows):
        forms = [f for f in dict.fromkeys(t[0] for t in group)
                 if len(f) > 1 and not (skip_rows and len({t[1] for t in f}) == 1)]

        def item(f, rows):
            def fn(dep):
                def term(r, k):
                    v = get(r, k, rows).astype(F32)
                    return v if dep is None or (r, k) != f[0][1:] else _after(v, _rows(dep, v.shape[0]))
                dst[index[f], rows, :] = _form(f, term).astype(BF16)
            return fn

        return [item(f, slice(i, i + n)) for i in range(0, T, n) for f in forms]

    h_sums = lambda n, gi: sum_items(n, _H_GROUPS[gi], _H_SUMS, hs_scr,
                                     lambda r_, k, rows: h_scr[r_, k, rows, :], True)

    def stash(key, buf, j0, transpose=False):
        n = buf.shape[0] // T
        if key not in did:
            assert key in arrived
            did.add(key)
            for (j, hd), w in _pair_tiles(buf, transpose).items():
                w_scr[hd, j0 + j] = w
        return lambda hd: [_ld(w_scr, hd, j0 + j) for j in range(n)]

    def kv_tile(jobs, r):
        wk, wvT = stash('k', wk_buf, 0), stash('v', wv_buf, kc, True)
        ct = [c_ref[_tile(r), _tile(j)] for j in range(kc)]
        for hd in range(2):
            k_scr[2 * r + hd] = jobs.mm(ct, wk(hd), _dot).astype(BF16)
        for hd in range(2):
            v_scr[2 * r + hd] = jobs.mm(wvT(hd), ct, _dot_nt).astype(BF16)

    def q_tile(jobs, r):
        wq = stash('q', wq_buf, 2 * kc)
        ht = [_ld(h_scr, r, j) for j in range(km)]
        for hd in range(2):
            v = (jobs.mm(ht, wq(hd), _dot) * scale).astype(BF16)
            q_scr[2 * r + hd] = v.T if 2 * r + hd in QT else v

    for blk in _prologue().split(';'):
        waits, starts, acts = blk.split('|')
        for ch in waits.strip():
            assert ch in started and ch not in arrived
            arrived.add(ch)
            named[ch].wait()
        for ch in starts.strip():
            assert ch not in started
            started.add(ch)
            named[ch].start()
        jobs = _Jobs()
        for act in acts.split():
            if act == 'Z':
                jax.lax.fori_loop(0, nb, zero, 0)
                acc_scr[S:, :] = jnp.zeros((acc_scr.shape[0] - S, M), F32)
                x_ref[S:, :] = jnp.zeros((x_ref.shape[0] - S, M), BF16)
                flag_scr[...] = jnp.zeros(flag_scr.shape, F32)
            elif act == 'L':
                did.add('L')
                assert ('Q', 0) in did
                for cp in stage_in(0) + prep_in(0):
                    cp.start()
            elif act == 'M':
                assert arrived >= set('nm')
                mod = _dot(silu_cond(), wma_ref[...])
                mod_scr[:, 0:M] = mod[:, 0:M]
                mod_scr[:, M:2 * M] = 1.0 + mod[:, M:2 * M]
                did.add('M')
            else:
                act, _, span = act.partition('@')
                span = int(span or 0)
                items = []
                for r in [int(ch, 16) for ch in act[1:]]:
                    did.add((act[0], r))
                    if act[0] == 'K':
                        assert 'abcd'[r // CB] in arrived
                        kv_tile(jobs, r)
                    elif act[0] == 'H':
                        assert 'wxyz'[r // CB] in arrived and 'M' in did
                        items += [h_item(r, i, ('N', r) in did) for i in range(T // LP)]
                    elif act[0] == 'N':
                        assert 'wxyz'[r // CB] in arrived
                        items += [n_item(r, i) for i in range(T // LP)]
                    elif act[0] == 'Q':
                        assert all(('h', r, i) in did for i in range(T // LP))
                        q_tile(jobs, r)
                    elif act[0] == 'F':
                        assert all(('K', SB * r + k_) in did for k_ in range(SB))
                        items += _v_form_items(v_scr, (pf_scr, vf_scr), r)
                    elif act[0] == 'C':
                        assert all('abcd'[t[1] // CB] in arrived for p_ in _C_GROUPS[r] for t in p_[0])
                        items += sum_items(
                            32, _C_GROUPS[r], _C_SUMS, cs_scr,
                            lambda r_, k, rows: c_ref[r_ * T + rows.start:r_ * T + rows.stop, _tile(k)], False)
                    else:
                        assert act[0] == 'S' and all(('h', t[1], T // LP - 1) in did for p_ in _H_GROUPS[r] for t in p_[0])
                        items += h_sums(32 if span else 16, r)
                release(jobs, span, items)
        assert not jobs.side
    assert arrived == set(named) and all((k_, r) in did for k_ in 'KHQ' for r in range(nb))
    assert all((k_, r) in did for k_ in 'CS' for r in range(2)) and 'L' in did
    assert all(('F', r) in did for r in range(SB))

    def mixer_prep(g):
        def blocks(r0, n, half, c0, c1, dep):
            get = lambda x, c: st_in[r0 + x * half:r0 + x * half + n, _tile(c)].astype(F32)
            return [_after(get(0, c0), _rows(dep, n)), get(0, c1), get(1, c0), _after(get(1, c1), _rows(dep, n))]

        def rows_item(dst, per, half, r0, c, o, n=16):
            def fn(dep):
                rows = pl.ds(pl.multiple_of(slice_of(g, per, half) * per, per) + o, n)
                for i, v in enumerate(_b_ops(*blocks(r0 + o, n, per, c, c + 2, dep))):
                    dst[i, c, rows, :] = v.astype(BF16)
            return fn

        def w3_item(k, i):
            def fn(dep):
                b11, b21, b12, b22 = blocks(slices[3][3], T, T, k, k + 2, dep)
                ws3[slice_of(g, T, FH), i, k] = _b_ops(b11, b12, b21, b22)[i].astype(BF16).T
            return fn

        return ([rows_item(dst, *sl[1:], c, o) for dst, sl in zip((ws12.at[0], ws12.at[1], ws4), slices)
                 for c in range(2) for o in range(0, sl[1], 16)]
                + [w3_item(k, i) for k in range(2) for i in range(7)])

    def stage_wait():
        for cp in pcopies(0):
            cp.wait()
        pltpu.make_async_copy(st_in, st_in, wsem.at[7]).wait()

    def attn_body(g, carry):
        side = _gap_items(work, gap_scr) + _weight_form_items(work, gap_scr, wt_scr, wf_scr, (0, 1, 2))
        bufs = (q_scr, k_scr, v_scr, (pf_scr, vf_scr), wo_buf, acc_scr, flag_scr)
        _attention_step(*bufs, g >> 16, side)

        @pl.when(g + 1 < nattn)
        def _():
            copies = stage_in(g + 1) + [ocopy(g + 1)]
            for cp in copies:
                cp.start()
            bufs = (h_scr, hs_scr, c_ref, cs_scr, wf_scr, q_scr, k_scr, v_scr, (pf_scr, vf_scr))
            side = [(SD0 + i * SDS, fn) for i, fn in enumerate(mixer_prep(g))]
            _proj_step(*bufs, scale, gap_scr, side)
            for cp in prep_in(g + 1):
                cp.start()
            stage_wait()
            ocopy(g + 1).wait()

        return carry

    stage_wait()
    for cp in cp_late:
        cp.start()
    jax.lax.fori_loop(0, nattn, attn_body, 0)

    def safe_pair(g, carry):
        copies = pcopies(g) + [ocopy(g)]
        for cp in copies:
            cp.start()
        for cp in copies:
            cp.wait()
        for buf, j0, transpose in ((wk_buf, 0, False), (wv_buf, kc, True), (wq_buf, 2 * kc, False)):
            for (j, hd), w in _pair_tiles(buf, transpose).items():
                w_scr[hd, j0 + j] = w

        def tile(u, carry):
            r, hd = u // 2, u % 2
            rows = pl.ds(pl.multiple_of(r * T, T), T)
            ct = [c_ref[rows, _tile(j)] for j in range(kc)]
            k_scr[u] = sum(_dot(ct[j], _ld(w_scr, hd, j)) for j in range(kc)).astype(BF16)
            v_scr[u] = sum(_dot_nt(_ld(w_scr, hd, kc + j), ct[j]) for j in range(kc)).astype(BF16)
            q = sum(_dot(_ld(h_scr, r, j), _ld(w_scr, hd, 2 * kc + j)) for j in range(km))
            q_scr[u] = (q * scale).astype(BF16)
            return carry

        jax.lax.fori_loop(0, 2 * nb, tile, 0)
        _attention_safe(q_scr, k_scr, v_scr, wo_buf, acc_scr)
        return carry

    @pl.when(jnp.max(flag_scr[...]) > 0)
    def _():
        jax.lax.fori_loop(0, nb, zero, 0)
        jax.lax.fori_loop(0, nattn, safe_pair, 0)

    for cp in cp_late:
        cp.wait()
    mod = _dot(silu_cond(), wmb_ref[...])
    mod_scr[:, 2 * M:4 * M] = mod[:, 0:2 * M]
    mod_scr[:, 4 * M:5 * M] = 1.0 + mod[:, 2 * M:3 * M]
    mod_scr[:, 5 * M:6 * M] = mod[:, 3 * M:4 * M]
    ftiles = [(f, min(f + T, Fd)) for f in range(0, Fd, T)]
    OFF = x_ref.shape[0] - S
    CAR = t_scr.shape[0] - RB

    def p1(r0, l0, n, dep=None):
        ga = mod_scr[:, 2 * M:3 * M]
        if dep is not None:
            ga = jnp.concatenate([_after(ga[:, 0:T], dep), ga[:, T:]], axis=1)
        rows = pl.ds(r0, n)
        x1 = x_ref[rows, :].astype(F32) + _rows(ga, n) * acc_scr[rows, :]
        xh_scr[0, l0:l0 + n, :] = x1
        hb = _ln(x1) * _rows(mod_scr[:, 4 * M:5 * M], n) + _rows(mod_scr[:, 3 * M:4 * M], n)
        xh_scr[1, l0:l0 + n, :] = hb
        return _ln(hb)

    HT = T // 2

    def p1_store(r0, c, dep=None):
        v = p1(r0 + c * PC, OFF + c * PC, PC, dep)
        a1_scr[c * PC:(c + 1) * PC, :] = v
        return jnp.max(v[:, M - T:].reshape(PC // 8, 8, T), axis=0)

    t_scr[RB:RB + CAR - OFF, :] = jnp.zeros((CAR - OFF, M), F32)
    t_scr[RB + CAR - OFF:RB + CAR, :] = _gelu(_dot(p1(0, 0, OFF).astype(BF16), w1_ref[...]))
    for c in range(RB // PC):
        p1_store(OFF, c)

    def out_copy(i):
        rows = pl.ds(i * T if isinstance(i, int) else pl.multiple_of(i * T, T), T)
        return pltpu.make_async_copy(out_buf.at[rows, :], out_hbm.at[rows, :], osem.at[i])

    def b_body(r, carry):
        gb = _rows(mod_scr[:, 5 * M:6 * M], T)
        r0 = pl.multiple_of(r * RB, RB)
        n0 = pl.multiple_of(jnp.minimum(r0 + RB, S - RB) + OFF, OFF)
        nh = RB // T
        now = [0]
        due = []
        pace = []

        def p1_item(c):
            return lambda dep: due.append((now[0] + PD, p1_store(n0, c, dep)))

        pace += [(P0 + i * PSTEP, p1_item(i)) for i in range(RB // PC)]
        wt = lambda ref, f0, f1, n: ref[f0:f1, _tile(n)]

        def mm(lhs, wts, dot=_dot):
            acc = None
            for x, w in zip(lhs, wts):
                if due and due[0][0] <= now[0]:
                    w = _tie(w, due.pop(0)[1])
                v = dot(x, w)
                now[0] += x.shape[0] // HT
                acc = v if acc is None else v + acc
                if pace and pace[0][0] <= now[0]:
                    pace.pop(0)[1](v[0:8, :])
            return acc

        def split_ops(lo, hi):
            return [v.astype(BF16) for v in _a_ops(lo[:HT], hi[:HT], lo[HT:], hi[HT:])]

        def two_tiles(aops, wsel, rest):
            def col(w):
                v = mm(rest[0], w, rest[3])
                return v[:HT], v[HT:]

            c11, c12, c21, c22 = _strassen(
                lambda i: mm([a[i] for a in aops], [wsel(i, k) for k in range(len(aops))]),
                lambda: col(rest[1]), lambda: col(rest[2]))
            return jnp.concatenate([c11, c21], axis=0), jnp.concatenate([c12, c22], axis=0)

        def square(full, aops, w_ref, ws_ref):
            out = {}
            for n in range(2):
                out[n], out[n + 2] = two_tiles(
                    aops, lambda i, k: _ld(ws_ref, i, n, slice(k * HT, (k + 1) * HT)),
                    (full[4:], [wt(w_ref, 4 * T, M, n)], [wt(w_ref, 4 * T, M, n + 2)], _dot))
            out[4] = mm(full, [wt(w_ref, j * T, (j + 1) * T, 4) for j in range(km)])
            return out

        t_scr[0:CAR, :] = t_scr[RB:RB + CAR, :]
        for hf in range(nh):
            a1 = [a1_scr[_tile(hf), _tile(j)] for j in range(km)]
            full = [v.astype(BF16) for v in a1]
            aops = [split_ops(a1[k], a1[2 + k]) for k in range(2)]
            for n, v in square(full, aops, w1_ref, ws12.at[0]).items():
                t = _gelu(v)
                if hf == nh - 1:
                    t = jnp.concatenate([t[:T - OFF], jnp.where(r < nrb - 1, t[T - OFF:], 0.0)], axis=0)
                t_scr[CAR + hf * T:CAR + (hf + 1) * T, _tile(n)] = t
        cq = M // 4
        shifts = (-1, 1, -2, 2)
        lane = jax.lax.broadcasted_iota(jnp.int32, (T, T), 1)
        y1, z, a3 = [], [], []
        for hf in range(nh):
            base = CAR - OFF + hf * T
            sh = []
            for j in range(km):
                g_lo, g_hi = (j * T) // cq, ((j + 1) * T - 1) // cq
                assert g_hi - g_lo <= 1
                v = t_scr[base + shifts[g_lo]:base + shifts[g_lo] + T, _tile(j)]
                if g_hi != g_lo:
                    v2 = t_scr[base + shifts[g_hi]:base + shifts[g_hi] + T, _tile(j)]
                    v = jnp.where(lane < g_hi * cq - j * T, v, v2)
                sh.append(v)
            hs = square([v.astype(BF16) for v in sh], [split_ops(sh[k], sh[2 + k]) for k in range(2)],
                        w2_ref, ws12.at[1])
            hs = jnp.concatenate([hs[n] for n in range(km)], axis=1)
            y1.append(hs + xh_scr[1, _tile(hf), :])
            z.append(xh_scr[0, _tile(hf), :] + gb * y1[hf])
            a3.append({})

            def ln_item(hf, c):
                def item(dep):
                    n = HT // NLN
                    for d in (0, HT):
                        v = y1[hf][d + c * n:d + (c + 1) * n]
                        if dep is not None:
                            v = jnp.concatenate([_after(v[:, :T], _rows(dep, n)), v[:, T:]], axis=1)
                        a3[hf][d + c * n] = _ln(v)
                return item

            ln_item(hf, 0)(None)
            pace += [(now[0] + LN0 + (c - 1) * LNS * (1 + hf), ln_item(hf, c)) for c in range(1, NLN)]
            pace.sort(key=lambda e: e[0])
        xh_scr[:, 0:OFF, :] = xh_scr[:, RB:RB + OFF, :]
        nf = FH // T
        h3, h3ops = [], []
        for hf in range(nh):
            assert len(a3[hf]) == 2 * NLN
            af = jnp.concatenate([a3[hf][key] for key in sorted(a3[hf])], axis=0)
            full = [af[:, _tile(j)].astype(BF16) for j in range(km)]
            aops = [split_ops(af[:, _tile(k)], af[:, _tile(2 + k)]) for k in range(2)]
            row, ops = {}, []
            narrow = None
            for n in range(nf):
                lo, hi = two_tiles(aops, lambda i, k: _ld(ws3, n, i, k),
                                   (full[4:], [wt(w3_ref, *ftiles[n], 4)],
                                    [wt(w3_ref, *ftiles[nf + n], 4)], _dot_nt))
                lo, hi = _gelu(lo), _gelu(hi)
                row[n], row[nf + n] = lo.astype(BF16), hi.astype(BF16)
                ops.append(split_ops(lo, hi))
                if n < km:
                    v = mm([wt(w3_ref, *ftiles[-1], n)], [full[n]], _dot_nt)
                    narrow = v if narrow is None else v + narrow
            row[2 * nf] = _gelu(mm(full, [wt(w3_ref, *ftiles[2 * nf], j) for j in range(km)],
                                   _dot_nt)).astype(BF16)
            fw = Fd - ftiles[-1][0]
            gT = jnp.concatenate([_gelu(narrow), jnp.zeros((T - fw, T), F32)], axis=0)
            row[2 * nf + 1] = _tie(gT.astype(BF16).T, gT[0:8, :])[:, :fw]
            h3.append([row[i] for i in range(len(ftiles))])
            h3ops.append(ops)
        for hf in range(nh):
            rows = pl.ds(pl.multiple_of(r0 + hf * T, T), T)

            def finish(n, v):
                out_buf[rows, _tile(n)] = (z[hf][:, _tile(n)] + gb[:, _tile(n)] * v).astype(out_buf.dtype)

            w4t = lambda n, f_: [wt(w4_ref, f0, f1, n) for f0, f1 in f_]
            finish(4, mm(h3[hf], w4t(4, ftiles)))
            for n in range(2):
                lo, hi = two_tiles(h3ops[hf], lambda i, k: _ld(ws4, i, n, slice(k * HT, (k + 1) * HT)),
                                   (h3[hf][2 * nf:], w4t(n, ftiles[2 * nf:]), w4t(n + 2, ftiles[2 * nf:]), _dot))
                finish(n, lo)
                finish(n + 2, hi)
            out_copy(r * nh + hf).start()
        assert not pace
        return carry

    jax.lax.fori_loop(0, nrb, b_body, 0)
    for i in range(nb):
        out_copy(i).wait()


@jax.jit
def pallas_adaLN_cond__compressed_kv_cla__mixer_s_mlp__prompt_kernel(
    A_x: jax.Array,
    A_c_kv: jax.Array,
    A_w_q: jax.Array,
    A_w_uk: jax.Array,
    A_w_uv: jax.Array,
    A_w_o: jax.Array,
    B_x: jax.Array,
    B_w1: jax.Array,
    B_w2: jax.Array,
    B_w3: jax.Array,
    B_w4: jax.Array,
    c: jax.Array,
    w_mod: jax.Array,
):
    _, S, M = A_x.shape
    Dc = A_c_kv.shape[2]
    H, D = A_w_q.shape[1], A_w_q.shape[2]
    Fd = B_w3.shape[1]
    assert D == T and A_c_kv.shape[1] == S and Dc == 4 * T and M == 5 * T and 13 * T < Fd < 14 * T and S == 16 * T
    vmem = pltpu.VMEM
    packed = lambda *lead: vmem(lead + (T, T), BF16)
    out = pl.pallas_call(
        _kernel,
        in_specs=[pl.BlockSpec(memory_space=pltpu.HBM)] * 12,
        out_specs=pl.BlockSpec(memory_space=pltpu.HBM),
        out_shape=jax.ShapeDtypeStruct((S, M), A_x.dtype),
        scratch_shapes=[
            vmem((S + 16, M), BF16),
            vmem((S, Dc), BF16),
            vmem((1, M), BF16),
            vmem((M, 2 * M), BF16),
            vmem((M, 4 * M), BF16),
            vmem((M, M), BF16),
            vmem((M, M), BF16),
            vmem((Fd, M), BF16),
            vmem((Fd, M), BF16),
            vmem((M, D), U32),
            vmem((Dc, D), U32),
            vmem((Dc, D), U32),
            vmem((2 * D, M), BF16),
            vmem((S, M), A_x.dtype),
            pltpu.SemaphoreType.DMA((15,)),
            pltpu.SemaphoreType.DMA((8,)),
            pltpu.SemaphoreType.DMA((S // T,)),
            vmem((8, 6 * M), F32),
            vmem((S // T, M // T, T, T), BF16),
            vmem((len(_C_SUMS), T, T), BF16),
            vmem((len(_H_SUMS), T, T), BF16),
            packed(2, M // T + 2 * (Dc // T)),
            packed(2 * S // T),
            packed(2 * S // T),
            packed(2 * S // T),
            vmem((S + 16, M), F32),
            vmem((S, M), F32),
            vmem((2, RB + 16, M), F32),
            vmem((RB, M), F32),
            vmem((RB + 32, M), F32),
            vmem((2, 7, 2, 2 * T, T), BF16),
            packed(6, 7, 2),
            vmem((7, 2, 6 * T, T), BF16),
            vmem((Dc // T, T, T), U32),
            vmem((len(_WF), T, T), BF16),
            vmem((3, 8, T), jnp.int32),
            vmem((4 * T, 4 * T), BF16),
            vmem((_FENCE + 1, T, T), BF16),
            vmem((_FENCE + 1, T, T), BF16),
            vmem((8, T), F32),
        ],
        compiler_params=pltpu.CompilerParams(
            vmem_limit_bytes=100 * 1024 * 1024,
            disable_bounds_checks=True,
        ),
    )(
        A_x.reshape(S, M), A_c_kv.reshape(S, Dc),
        A_w_q, A_w_uk, A_w_uv,
        A_w_o.reshape(H // 2, 2 * D, M),
        B_w1, B_w2, B_w3.T, B_w4, c, w_mod,
    )
    return out.reshape(1, S, M)
```

```python
import functools
import math

import jax
import jax.numpy as jnp
import jax.experimental.pallas as pl
import jax.experimental.pallas.tpu as pltpu

F32 = jnp.float32
BF16 = jnp.bfloat16
U32 = jnp.uint32
NT = (((1,), (1,)), ((), ()))
T = 128
EPS = 1e-5
LOG2E = math.log2(math.e)

GRP = 4
LEAD = 10
PROW = 3
RES = 32
LAT_0 = 32
LAT_A = 16
LAT_B = 20
ALEAD = 32
QT = (4, 6)
ONV, OEND = 0.5, 24
FPOS, DPOS = 0, 0
SIDE0, SIDE1, SLAG, SDUE = 8, 60, 4, 8
SKIND = 'pvo'
HACKWO = 0
SG0, SG1 = 6, 4
SD0, SDS = 10, 2.2
WFN = (4, 4, 6)
VF0, VFS = 4, 1.7
L_LO, L_HI, L_RATIO = 2.0 ** -24, 2.0 ** 24, 4.0
RB = 256
PC = 32
P0, PSTEP, PD = 360, 27, 48
GD, NAR0, NARS = 36, 4, 8
MWOPS = 70
NLN, LN0, LNS = 4, 4, 5
LP = 16
SP0, SP1 = 76, 38
_prologue = lambda: ('|kva|Z; |b|; kva|wc|K0123; bw|xdn|C0@56 N0123@52 K4567; cx|mq|N4567@52 F0@56 K89ab; '
            'd|y|C1@56 F1@56 Kcdef; nmq|zo|M H01 H234567@30 F2@36 Q0123; y||H89ab@30 F3@36 Q4567; '
            'zo||L Hcdef@30 S0@%d Q89ab S1@%d Qcdef' % (SP0, SP1))


def _dot(a, b):
    return jnp.dot(a, b, preferred_element_type=F32)


def _dot_nt(a, b):
    return jax.lax.dot_general(a, b, NT, preferred_element_type=F32)


def _ln(x):
    m = jnp.mean(x, axis=-1, keepdims=True)
    xc = x - m
    v = jnp.mean(xc * xc, axis=-1, keepdims=True)
    return xc * jnp.exp2(jnp.log(v + EPS) * (-0.5 * LOG2E))


def _rows(v, n):
    return jnp.broadcast_to(v[None], (n // 8, 8, v.shape[1])).reshape(n, v.shape[1])


def _gelu2(x):
    c0 = math.sqrt(2.0 / math.pi)
    return x + x * jnp.tanh(x * (c0 + (c0 * 0.044715) * (x * x)))


def _after(x, dep):
    return jnp.where(dep > jnp.inf, dep, x)


def _tie(x, dep):
    xu = pltpu.bitcast(x, U32)
    first = jnp.where(dep > jnp.inf, jnp.uint32(0), xu[:8])
    return pltpu.bitcast(jnp.concatenate([first, xu[8:]], axis=0), BF16)


def _tile(j):
    return slice(j * T, (j + 1) * T)


def _ld(ref, *idx):
    return pltpu.bitcast(ref.bitcast(U32)[idx], BF16)


def _a_ops(a11, a12, a21, a22):
    return [a11 + a22, a21 + a22, a11, a22, a11 + a12, a21 - a11, a12 - a22]


def _b_ops(b11, b12, b21, b22):
    return [b11 + b22, b11, b12 - b22, b21 - b11, b22, b11 + b12, b21 + b22]


def _strassen(prod, col1=None, col2=None):
    m4 = prod(3)
    m2 = prod(1)
    c21 = m2 + m4
    if col1 is not None:
        e11, e21 = col1()
        m4, c21 = m4 + e11, c21 + e21
    m3 = prod(2)
    m5 = prod(4)
    c12 = m3 + m5
    if col2 is not None:
        e12, e22 = col2()
        c12, m3 = c12 + e12, m3 + e22
    m1 = prod(0)
    c11 = prod(6) + (m1 + (m4 - m5))
    c22 = prod(5) + (m1 + (m3 - m2))
    return c11, c12, c21, c22


def _group(rows, cols, pairs):
    xs, ys = dict.fromkeys(x for x, _ in pairs), dict.fromkeys(y for _, y in pairs)
    used = set(xs) | set(ys) | {(x[0], y[1]) for x, y in pairs} | {(y[0], x[1]) for x, y in pairs}
    prods = []
    for n, r in enumerate(rows):
        for i, k in [x for x in xs if x[0] == r]:
            mates = [y for x, y in pairs if x == (i, k)]
            prods.append((((1, i, k),) + tuple((1, i, k2) for _, k2 in mates), ((1, k, 0),),
                          ((1, i, 0), (-1, i, 1))))
            prods.append((((1, i, k),) + tuple((-1, i2, k) for i2, _ in mates), ((1, k, 0), (1, k, 1)),
                          ((1, i, 1),)))
        for i2, k2 in [y for y in ys if y[0] == r]:
            mates = [x for x, y in pairs if y == (i2, k2)]
            prods.append((((1, i2, k2),) + tuple((1, i2, k) for _, k in mates), ((1, k2, 1),),
                          ((1, i2, 1), (-1, i2, 0))))
            prods.append((((1, i2, k2),) + tuple((-1, i, k2) for i, _ in mates), ((1, k2, 0), (1, k2, 1)),
                          ((1, i2, 0),)))
        prods += [(((1, r, k),), ((1, k, h),), ((1, r, h),)) for k in cols if (r, k) not in used for h in (0, 1)]
        for (i, k), (i2, k2) in pairs:
            if r in (i, i2) and i + i2 - r in rows[n + 1:]:
                prods.append((((1, i, k2),), ((1, k2, 0), (-1, k, 0)), ((1, i2, 0), (1, i, 0))))
                prods.append((((1, i2, k), (1, i, k2)), ((1, k, 0), (1, k2, 1)), ((1, i2, 0), (1, i, 1))))
                prods.append((((1, i2, k),), ((1, k, 1), (-1, k2, 1)), ((1, i2, 1), (1, i, 1))))
    return prods


def _all_pairs(xrows, yrows):
    return [((x, a), (y, b)) for a, x in enumerate(xrows) for b, y in enumerate(yrows) if a != b]


_PAIRS65 = [((x[0] + 10, x[1]), (y[0] + 10, y[1])) for x, y in (
    ((0, 1), (1, 0)), ((0, 1), (5, 2)), ((2, 3), (1, 0)), ((2, 3), (3, 1)), ((2, 3), (5, 2)), ((3, 2), (1, 0)),
    ((4, 4), (0, 3)), ((4, 4), (1, 0)), ((4, 4), (3, 1)), ((4, 4), (5, 2)))]
_C_GROUPS = [_group(range(r, r + 8), range(4), _all_pairs(range(r, r + 4), range(r + 4, r + 8))) for r in (0, 8)]
_H_GROUPS = [_group(range(10), range(5), _all_pairs(range(5), range(5, 10))),
             _group(range(10, 16), range(5), _PAIRS65)]
_sum_index = lambda groups: {f: n for n, f in enumerate(
    dict.fromkeys(t[0] for g in groups for t in g if len(t[0]) > 1))}
_C_SUMS, _H_SUMS = _sum_index(_C_GROUPS), _sum_index(_H_GROUPS)


def _cells(rows, cols, pairs):
    xs = list(dict.fromkeys(p[0] for p in pairs))
    ys = list(dict.fromkeys(p[1] for p in pairs))
    used = set(xs + ys) | {(x[0], y[1]) for x, y in pairs} | {(y[0], x[1]) for x, y in pairs}

    def home_x(i, k):
        mates = [y for x, y in pairs if x == (i, k)]
        return [(((1, i, k),) + tuple((1, i, k2) for _, k2 in mates), ((1, k, 0),), ((1, i, 0), (-1, i, 1))),
                (((1, i, k),) + tuple((-1, i2, k) for i2, _ in mates), ((1, k, 0), (1, k, 1)), ((1, i, 1),))]

    def home_y(i2, k2):
        mates = [x for x, y in pairs if y == (i2, k2)]
        return [(((1, i2, k2),) + tuple((1, i2, k) for _, k in mates), ((1, k2, 1),), ((1, i2, 1), (-1, i2, 0))),
                (((1, i2, k2),) + tuple((-1, i, k2) for i, _ in mates), ((1, k2, 0), (1, k2, 1)), ((1, i2, 0),))]

    def cross(x, y):
        (i, k), (i2, k2) = x, y
        return [(((1, i, k2),), ((1, k2, 0), (-1, k, 0)), ((1, i2, 0), (1, i, 0))),
                (((1, i2, k), (1, i, k2)), ((1, k, 0), (1, k2, 1)), ((1, i2, 0), (1, i, 1))),
                (((1, i2, k),), ((1, k, 1), (-1, k2, 1)), ((1, i2, 1), (1, i, 1)))]

    direct = lambda i: [(((1, i, k),), None, ((1, i, 0), (1, i, 1))) for k in cols if (i, k) not in used]
    single = lambda i: ([t for x in xs if x[0] == i for t in home_x(*x)]
                        + [t for y in ys if y[0] == i for t in home_y(*y)] + direct(i))
    prods = []
    for n, i in enumerate(rows):
        prods += single(i)
        for i2 in rows[n + 1:]:
            for x, y in pairs:
                if {x[0], y[0]} == {i, i2}:
                    prods += cross(x, y)
    return prods


_square = lambda q: [((a, a), (q + b, b)) for a in range(q) for b in range(q) if a != b]
_shift = lambda pairs, r0: [((x[0] + r0, x[1]), (y[0] + r0, y[1])) for x, y in pairs]
_flip = lambda pairs: [(x[::-1], y[::-1]) for x, y in pairs]
_P35 = [((1, 2), (0, 4)), ((1, 2), (2, 1)), ((2, 3), (0, 4)), ((2, 3), (1, 0))]
_P45 = [((0, 2), (1, 1)), ((2, 4), (0, 3)), ((2, 4), (1, 1)), ((2, 4), (3, 2)), ((3, 0), (0, 3)), ((3, 0), (1, 1))]
_P55 = [((2, 1), (0, 4)), ((2, 1), (1, 0)), ((2, 1), (3, 2)), ((2, 1), (4, 3)), ((3, 3), (0, 4)), ((3, 3), (1, 0)),
        ((4, 2), (0, 4)), ((4, 2), (1, 0))]
_MIX = [_cells(range(5), range(5), _P55), _cells(range(5), range(5), _P55),
        _cells(range(13), range(5), _square(5) + _shift(_P35, 10)),
        _cells(range(5), range(14), _flip(_square(5) + _shift(_P45, 10)))]
_MIXW = {(m, f): n for n, (m, f) in enumerate(dict.fromkeys((m, t[0]) for m in range(4) for t in _MIX[m]))}


def _form(form, get):
    acc = None
    for sign, i, j in form:
        v = get(i, j)
        acc = v if acc is None else (acc + v if sign > 0 else acc - v)
    return acc


def _gap_items(bufs, gap_scr):
    items = []
    for n, buf in enumerate(bufs):
        acc = []

        def part(r0, buf=buf, acc=acc):
            def fn(dep):
                wu = jnp.concatenate([buf[r:r + 8, :] for r in range(r0, r0 + T, 32)])
                mask = jnp.full((8, T), 0x7FFF0000, U32)
                if dep is not None:
                    mask = jnp.where(dep > jnp.inf, jnp.uint32(0), mask)
                mask = _rows(mask, 32)
                new = [jnp.sum(pltpu.bitcast(v & mask, F32).reshape(4, 8, T), axis=0) for v in (wu << 16, wu)]
                acc[:] = [u + v for u, v in zip(acc, new)] if acc else new
            return fn

        def last(_, n=n, acc=acc):
            bits = []
            for v in acc:
                l1 = jnp.sum(jnp.sum(v, axis=1, keepdims=True), axis=0, keepdims=True)
                bits.append(pltpu.bitcast(jnp.broadcast_to(l1, (8, T)), jnp.int32) >> 8)
            gap = jnp.clip((bits[0] - bits[1] + (1 << 14)) >> 15, -8, 8) << 23
            gap_scr[n] = gap
            return pltpu.bitcast(gap, F32)

        items += [part(r0) for r0 in range(0, buf.shape[0], T)] + [last]
    return items


def _pair_tiles(w_ref, transpose=False):
    tiles = {}
    for j in range(w_ref.shape[0] // T):
        wu = w_ref[_tile(j), :]
        if transpose:
            wu = wu.T
        tiles[j, 0] = pltpu.bitcast(wu << 16, F32).astype(BF16)
        tiles[j, 1] = pltpu.bitcast(wu & jnp.uint32(0xFFFF0000), F32).astype(BF16)
    return tiles


def _canon(form):
    if form[-1][0] < 0 and form[0][1:] > form[1][1:]:
        return -1, ((1,) + form[1][1:], (-1,) + form[0][1:])
    return 1, form


_w_forms = lambda groups: list(dict.fromkeys(_canon(t[1])[1] for g in groups for t in g))
_WF = {key: n for n, key in enumerate([(m, f) for m, groups in enumerate((_C_GROUPS, _C_GROUPS, _H_GROUPS))
                                       for f in _w_forms(groups)])}


def _weight_form_items(bufs, gap_scr, wt_scr, wf_scr, which):
    n = 16
    items = []

    def flip(j):
        def fn(dep):
            wu = bufs[1][_tile(j), :]
            wu = (wu if dep is None else jnp.where(_rows(dep, T) > jnp.inf, jnp.uint32(0), wu)).T
            wt_scr[j] = wu
            return pltpu.bitcast(wu[T - 8:], F32)
        return fn

    def part(m, r0, forms):
        def fn(dep):
            fac = pltpu.bitcast(0x3F800000 + gap_scr[m], F32)
            mask = jnp.full((8, T), 0xFFFF0000, U32)
            sh = jnp.full((8, T), 16, U32)
            if dep is not None:
                mask = jnp.where(dep > jnp.inf, jnp.uint32(0), mask)
                sh = jnp.where(dep > jnp.inf, jnp.uint32(0), sh)
            fac, mask, sh = _rows(fac, n), _rows(mask, n), _rows(sh, n)
            base = {}

            def get(k, h):
                if (k, h) not in base:
                    wu = wt_scr[k, r0:r0 + n, :] if m == 1 else bufs[m][k * T + r0:k * T + r0 + n, :]
                    base[k, h] = pltpu.bitcast(wu & mask, F32) * fac if h else pltpu.bitcast(wu << sh, F32)
                return base[k, h]

            for f in forms:
                wf_scr[_WF[m, f], r0:r0 + n, :] = _form(f, get).astype(BF16)
        return fn

    for m in which:
        forms = [f for mm, f in _WF if mm == m]
        if m == 1:
            items += [flip(j) for j in range(bufs[1].shape[0] // T)]
        per = -(-len(forms) // WFN[m])
        forms.sort(key=lambda f: sorted({t[1] for t in f}))
        items += [part(m, r0, forms[i:i + per]) for r0 in range(0, T, n) for i in range(0, len(forms), per)]
    return items


def _run_group(jobs, prods, a_get, w, transposed, finish):
    left = {}
    for _, _, outs in prods:
        for _, i, h in outs:
            left[i, h] = left.get((i, h), 0) + 1
    acc = {}
    for af, bf, outs in prods:
        sign, wt = w(bf)
        m = jobs.mm([wt], [a_get(af)], _dot_nt) if transposed else jobs.mm([a_get(af)], [wt], _dot)
        for s_, i, h in outs:
            if (i, h) not in acc:
                acc[i, h] = (s_ * sign, m)
            else:
                s0, v = acc[i, h]
                acc[i, h] = (s0, v + m if s0 == s_ * sign else v - m) if s0 > 0 or s_ * sign < 0 else (1, m - v)
            left[i, h] -= 1
            if not left[i, h]:
                s0, v = acc.pop((i, h))
                assert s0 > 0
                finish(2 * i + h, v)


class _Jobs:
    def __init__(self, side=()):
        self.res = []
        self.side = list(side)

    def mm(self, lhs, wt, dot):
        acc = None
        for x, w in zip(lhs, wt):
            v = dot(x, w)
            self.res.append(v)
            acc = v if acc is None else v + acc
            rel = 4 * (len(self.res) % 4)
            while self.side and self.side[0][0] <= len(self.res):
                self.side.pop(0)[1](v[8 * rel:8 * rel + 8, :])
                rel = (rel + 2) % 16
        return acc


def _proj_step(h_scr, hs_scr, c_ref, cs_scr, wf_scr, q_scr, k_scr, v_scr, pf, scale, shifts, side):
    def weight(m):
        def get(form):
            sign, form = _canon(form)
            return sign, _ld(wf_scr, _WF[m, form])
        get.inv = pltpu.bitcast(0x3F800000 - shifts[m], F32)
        return get

    wk, wvT, wq = weight(0), weight(1), weight(2)
    c_get = lambda f: _ld(cs_scr, _C_SUMS[f]) if len(f) > 1 else c_ref[_tile(f[0][1]), _tile(f[0][2])]
    h_get = lambda f: _ld(hs_scr, _H_SUMS[f]) if len(f) > 1 else _ld(h_scr, f[0][1], f[0][2])

    def put(dst, w, mul=None):
        muls = [mul, _rows(w.inv if mul is None else w.inv * mul, T)]

        def fn(u, v):
            v = (v if muls[u % 2] is None else v * muls[u % 2]).astype(BF16)
            dst[u] = v.T if mul is not None and u in QT else v
        return fn

    jobs = _Jobs(side)
    put_v, stored = put(v_scr, wvT), set()
    nxt = [0]

    def fin_v(u, v):
        put_v(u, v)
        stored.add(u)
        for J in range(SB):
            if all(2 * (SB * J + k) + h in stored for k in range(SB) for h in range(2)) and ('J', J) not in stored:
                stored.add(('J', J))
                for fn in _v_form_items(v_scr, pf, J):
                    nxt[0] = max(nxt[0] + VFS, len(jobs.res) + VF0)
                    jobs.side.append((int(nxt[0]), fn))
                jobs.side.sort(key=lambda e: e[0])

    kk, vv, qq = ((c_get, wk, False, put(k_scr, wk)), (c_get, wvT, True, fin_v),
                  (h_get, wq, False, put(q_scr, wq, scale)))
    for prods, args in ((_C_GROUPS[0], kk), (_C_GROUPS[0], vv), (_C_GROUPS[1], vv), (_C_GROUPS[1], kk),
                        (_H_GROUPS[0], qq), (_H_GROUPS[1], qq)):
        _run_group(jobs, prods, *args)
    assert not jobs.side


def _inner_group(rows, cols, pairs):
    xs, ys = dict.fromkeys(x for x, _ in pairs), dict.fromkeys(y for _, y in pairs)
    used = set(xs) | set(ys) | {(x[0], y[1]) for x, y in pairs} | {(y[0], x[1]) for x, y in pairs}
    prods = []
    for i, j in xs:
        mates = [y for x, y in pairs if x == (i, j)]
        prods.append((((1, i, 0),), ((1, 0, j), (-1, 1, j)), ((1, i, j),) + tuple((1, i2, j) for i2, _ in mates)))
        prods.append((((1, i, 0), (1, i, 1)), ((1, 1, j),), ((1, i, j),) + tuple((-1, i, j2) for _, j2 in mates)))
    for i2, j2 in ys:
        mates = [x for x, y in pairs if y == (i2, j2)]
        prods.append((((1, i2, 0), (1, i2, 1)), ((1, 0, j2),),
                      ((1, i2, j2),) + tuple((-1, i2, j) for _, j in mates)))
        prods.append((((1, i2, 1),), ((1, 0, j2), (-1, 1, j2)),
                      ((-1, i2, j2),) + tuple((-1, i, j2) for i, _ in mates)))
    prods += [(((1, i, h),), ((1, h, j),), ((1, i, j),))
              for i in rows for j in cols if (i, j) not in used for h in (0, 1)]
    for (i, j), (i2, j2) in pairs:
        lo, hi = min(j, j2), max(j, j2)
        prods.append((((1, i2, 0), (-1, i, 0)), ((1, 0, lo), (1, 0, hi)), ((1, i2, j),)))
        prods.append((((1, i, 0), (1, i2, 1)), ((1, 0, j2), (1, 1, j)), ((1, i, j2), (1, i2, j))))
        prods.append((((1, i, 1), (-1, i2, 1)), ((1, 1, lo), (1, 1, hi)), ((1, i, j2),)))
    return prods


def _o_jobs():
    prods = (_inner_group(range(10), range(5), _all_pairs(range(0, 10, 2), range(1, 10, 2)))
             + _inner_group(range(10, 16), range(5), _PAIRS65))
    row = lambda t: max(i for _, i, _ in t[0])
    unit = lambda t: max(2 * i + h for _, i, h in t[0])
    need = lambda t: unit(t) if row(t) == 15 else 2 * row(t) + 1
    return [(need(t), t) for t in sorted(prods, key=need)]


_O_JOBS = _o_jobs()


SB = 4


class _Star:
    def __init__(self, ts):
        self.ts, self.n = ts, len(ts)
        rn = range(self.n)
        self.pairs = [(i, j) for i in rn for j in rn if i < j]
        self.pf = {f: m for m, f in enumerate([('R', i) for i in rn] + [('C', i) for i in rn]
                                              + [('S', i, j) for i in rn for j in rn if i != j]
                                              + [('A', i, j) for i, j in self.pairs])}
        self.vf = {f: m for m, f in enumerate([('W', i) for i in rn]
                                              + [(q, i, j) for i, j in self.pairs for q in ('Q1', 'Q2', 'Q3')])}
        self.pv = {**{('W', i): ('R', i) for i in rn}, **{('B', i): ('C', i) for i in rn},
                   **{('Q1', i, j): ('S', i, j) for i, j in self.pairs},
                   **{('Q2', i, j): ('A', i, j) for i, j in self.pairs},
                   **{('Q3', i, j): ('S', j, i) for i, j in self.pairs}}

    def products(self, i):
        return [('W', i), ('B', i)] + [(q, i, j) for j in range(i + 1, self.n) for q in ('Q1', 'Q2', 'Q3')]


_FULL = _Star((-1.125, -0.375, 0.375, 1.125))
_HALF = _Star((-0.75, 0.75))
_DCELLS = [(0, 0), (1, 0), (1, 1), (2, 2), (3, 2), (3, 3)]
_HSLOT = (SB - 1) * len(_FULL.pf)
_DSLOT = _HSLOT + len(_HALF.pf)
_VSLOT = _DSLOT + len(_DCELLS)
_VHALF = (SB - 1) * len(_FULL.vf)
_FENCE = _VSLOT + (_VHALF + SB * len(_HALF.vf) + 1) // 2


def _v_slot(star, J, f):
    m = star.vf[f] + J * len(star.vf) + (0 if star is _FULL else _VHALF)
    return _VSLOT + m // 2, m % 2 * (T // 2)


def _v_form_items(v_scr, pf, J):
    n, HT = 16, T // 2

    def item(star, h, r0, pairs):
        def fn(dep):
            ts = [jnp.full((8, T), t, F32) for t in star.ts]
            ts = [_rows(t if dep is None else _after(t, dep), n) for t in ts]

            def get(k, a):
                r = (a * HT + r0) // 2
                return _ld(v_scr, 2 * (SB * J + k) + h, slice(r, r + n // 2)).astype(F32)

            def put(f, v):
                slot, r = _v_slot(star, J, f)
                pf[h][slot, r + r0:r + r0 + n, :] = v.astype(BF16)

            b = {(k, a): get(k, a) for k in sorted({k for pr in pairs or star.pairs for k in pr})
                 for a in range(2)}
            if pairs is None or star.n == 2:
                w = [b[k, 0] + ts[k] * b[k, 1] for k in range(star.n)]
                for k in range(star.n):
                    put(('W', k), w[k])
                for i, j in star.pairs:
                    put(('Q2', i, j), w[i] - w[j])
            for i, j in pairs or ():
                d0, d1 = b[j, 0] - b[i, 0], b[j, 1] - b[i, 1]
                put(('Q1', i, j), d0 + ts[i] * d1)
                put(('Q3', i, j), d0 + ts[j] * d1)
        return fn

    pr = _FULL.pairs
    parts = [(_HALF, _HALF.pairs)]
    if J < SB - 1:
        parts += [(_FULL, x) for x in (None, pr[:2], [pr[2], pr[4]], [pr[3], pr[5]])]
    return [item(star, h, r0, pairs) for h in range(2) for r0 in range(0, HT, n) for star, pairs in parts]


def _job_order(nsb):
    units = [(I, h) for I in range(nsb) for h in range(2)]
    qe, qv = [], []
    for I, h in units:
        es = [('e', I, h, J, p) for J in range(I) for p in range(SB)]
        ds = [('d', I, h) + c for c in _DCELLS]
        es.insert(max(len(es) - FPOS, 0), ('f', I, h))
        qe += es + ds if I or FPOS < 9 else ds[:DPOS] + es + ds[DPOS:]
        for i in range(SB):
            qv += [('p', I, h, f, J) for f in _FULL.products(i) for J in range(I)]
            if i >= 2:
                qv += [('p', I, h, f, None) for f in _HALF.products(i - 2)]
            qv += [('v', I, h) + c for c in _DCELLS if c[0] == i]
    qo = [('o', u, j) for j, (u, _) in enumerate(_O_JOBS)]
    cost = dict(e=8, f=8, d=2, p=1, v=2, o=2)
    order, done = [], {}
    now = [0]

    def emit(q):
        job = q.pop(0)
        order.append(job)
        now[0] += cost[job[0]]
        if job[0] == 'd':
            done[job] = now[0]
        elif job[0] == 'v' and job[4] == job[3]:
            done['u', 2 * (SB * job[1] + job[3]) + job[2]] = now[0]
        return cost[job[0]]

    def v_ready():
        if not qv:
            return False
        key = ('d', qv[0][1], qv[0][2], SB - 1, SB - 1)
        return key in done and done[key] + (LAT_0 if qv[0][1:3] == (0, 0) else LAT_A) <= now[0]

    def o_ready():
        return bool(qo) and ('u', qo[0][1]) in done and done['u', qo[0][1]] + LAT_B <= now[0]

    def fill(nv, no):
        n = 0
        while nv > 0 or no > 0 or n % 4:
            if no > 0 and n % 2 == 0 and o_ready() and no * ONV >= nv:
                no -= 2
                n += emit(qo)
            elif v_ready() and (nv > 0 or n % 4):
                c = emit(qv)
                nv -= c
                n += c
            elif o_ready() and n % 2 == 0 and (no > 0 or n % 4 or nv > 0) and len(qo) > RES:
                no -= 2
                n += emit(qo)
            else:
                break

    while qe:
        unit = qe[0][1:3]
        while qv and qv[0][2] == unit[1] and qv[0][1] < unit[0]:
            emit(qv)
        ne = 0
        while qe and ne < 8 and (ne == 0 or (qe[0][0] == 'd' and qe[0][1:3] == unit and ne + 2 <= 8)):
            ne += emit(qe)
        groups = lambda q: sum(cost[j[0]] for j in q) / 8
        old = [j for j in qv if j[1:3] != unit and ('d', j[1], j[2], SB - 1, SB - 1) in done]
        here = [j for j in qe if j[1:3] == unit]
        rest = sum(cost[j[0]] for j in old)
        nv = (rest - LAT_A) / (groups(here) + 1) if here else rest
        no = 2 * max(len(qo) - RES - OEND, 0) / (groups(qe) + 1)
        fill(int(nv + 0.5), int(no + 0.5))
    while qv or qo:
        if qv and v_ready():
            fill(6, 2)
            if not qv:
                continue
        elif o_ready():
            emit(qo)
        else:
            emit(qv or qo)
    return order


def _attention_safe(q_scr, k_scr, v_scr, wo_ref, acc_scr):
    causal = (jax.lax.broadcasted_iota(jnp.int32, (T, T), 0)
              <= jax.lax.broadcasted_iota(jnp.int32, (T, T), 1))

    def unit(u, carry):
        r, hd = u // 2, u % 2

        def block(c, mlo):
            m0, l, o = mlo
            s = _dot_nt(_ld(k_scr, 2 * c + hd), _ld(q_scr, u))
            s = jnp.where(jnp.logical_or(causal, c < r), s, -1e9 * LOG2E)
            m = jnp.maximum(m0, jnp.max(s, axis=0, keepdims=True))
            a = jnp.exp2(m0 - m)
            p = jnp.exp2(s - m)
            return (m, l * a + jnp.sum(p, axis=0, keepdims=True),
                    o * a + _dot(_ld(v_scr, 2 * c + hd), p.astype(BF16)))

        _, l, o = jax.lax.fori_loop(0, r + 1, block, (jnp.full((1, T), -jnp.inf, F32), jnp.zeros((1, T), F32),
                                                      jnp.zeros((T, T), F32)))
        rows = pl.ds(pl.multiple_of(r * T, T), T)
        acc_scr[rows, :] += _dot((o * (1.0 / l)).astype(BF16).T, wo_ref[pl.ds(pl.multiple_of(hd * T, T), T), :])
        return carry

    jax.lax.fori_loop(0, q_scr.shape[0], unit, 0)


def _attention_step(q_scr, k_scr, v_scr, pf, wo_ref, acc_scr, flag_scr, z, side):
    causal = (jax.lax.broadcasted_iota(jnp.int32, (T, T), 0)
              <= jax.lax.broadcasted_iota(jnp.int32, (T, T), 1))
    HT = T // 2
    lsum, lrow, acc, fg, dacc, of, lhs = {}, {}, {}, {}, {}, {}, {}
    res = []
    wo, terms = {}, {}
    left = {}
    done_side = [0, 0]
    chk = [jnp.zeros((8, T), F32), None]
    for _, t in _O_JOBS:
        for _, i, j in t[2]:
            left[i, j] = left.get((i, j), 0) + 1

    def add_l(u, v):
        lsum[u] = v if u not in lsum else lsum[u] + v

    csign = {}

    def p_forms(star, h, slot0, g, tiles, cell, when):
        n = star.n

        def put(f, v):
            pf[h][slot0 + star.pf[f], 16 * g:16 * g + 16, :] = v.astype(BF16)

        for i in range(n):
            row = [cell(i, k) for k in sorted(range(n), key=lambda k: when(i, k))]
            r = functools.reduce(lambda x, y: x + y, row)
            put(('R', i), r)
            add_l(tiles[i], r[:8] + r[8:])
            col = sorted(range(n), key=lambda i2: (when(i2, i), i2 != i))
            sign = csign[n, i] = 1 if col[0] == i else -1
            c = cell(col[0], i)
            for i2 in col[1:]:
                c = c + cell(i2, i) if (1 if i2 == i else -1) == sign else c - cell(i2, i)
            put(('C', i), c)
            for j in range(n):
                if j != i:
                    put(('S', i, j), cell(i, j))
        for i, j in star.pairs:
            put(('A', i, j), cell(i, j) + cell(j, i))

    due = []

    def scores(x, u):
        if due and due[0][0] <= done_side[1]:
            x = _tie(x, due.pop(0)[1])
        s = (_dot if u in QT else _dot_nt)(x, _ld(q_scr, u))
        res.append(s)
        return s

    def job_e(I, h, J, p):
        tiles = [2 * (SB * I + i) + h for i in range(SB)]
        ps = []
        for i, u in enumerate(tiles):
            x = jnp.concatenate([k_scr.bitcast(U32)[2 * (SB * J + (t - i) % SB) + h, 8 * g:8 * g + 8, :]
                                 for g in (2 * p, 2 * p + 1) for t in range(SB)], axis=0)
            ps.append(jnp.exp2(scores(pltpu.bitcast(x, BF16), u)))
        when = lambda i, k: (i + k) % SB
        for n, g in enumerate((2 * p, 2 * p + 1)):
            cell = lambda i, k: ps[i][16 * (SB * n + when(i, k)):16 * (SB * n + when(i, k)) + 16]
            p_forms(_FULL, h, J * len(_FULL.pf), g, tiles, cell, when)

    def job_f(I, h):
        tiles = [2 * (SB * I + 2 + i) + h for i in range(2)]
        ps = {(i, k): jnp.exp2(scores(_ld(k_scr, 2 * (SB * I + k) + h), u))
              for i, u in enumerate(tiles) for k in range(2)}
        for g in range(T // 16):
            p_forms(_HALF, h, _HSLOT, g, tiles, lambda i, k: ps[i, k][16 * g:16 * g + 16], lambda i, k: 0)

    def job_d(I, h, i, k):
        u = 2 * (SB * I + i) + h
        s = scores(_ld(k_scr, 2 * (SB * I + k) + h), u)
        if i == k:
            s = jnp.where(causal, s, -1e9 * LOG2E)
        p = jnp.exp2(s)
        add_l(u, jnp.sum(p.reshape(T // 8, 8, T), axis=0))
        pf[h][_DSLOT + _DCELLS.index((i, k))] = p.astype(BF16)
        if (i, k) == _DCELLS[-1]:
            pf[h][_FENCE + z, 0:16, :] = jnp.zeros((16, T), BF16)
            for u in [2 * (SB * I + a) + h for a in range(SB)]:
                lrow[u] = jnp.sum(lsum.pop(u), axis=0, keepdims=True)
            ls = [lrow[2 * (SB * I + a) + h] for a in range(SB)]
            lo = jnp.minimum(jnp.minimum(ls[0], ls[1]), jnp.minimum(ls[2], ls[3]))
            hi = jnp.maximum(jnp.maximum(ls[0], ls[1]), jnp.maximum(ls[2], ls[3]))
            ok = jnp.logical_and(lo >= L_LO, hi <= L_HI)
            ok = jnp.logical_and(ok, (hi if I else jnp.maximum(ls[2], ls[3]))
                                 <= L_RATIO * (lo if I else jnp.minimum(ls[2], ls[3])))
            bad = jnp.where(ok, 0.0, 1.0)
            chk[1] = bad if chk[1] is None else jnp.maximum(chk[1], bad)

    def job_p(I, h, f, J):
        star, last = (_HALF, True) if J is None else (_FULL, J == I - 1)
        blk = I if J is None else J
        if f[0] == 'B':
            x = _ld(v_scr, 2 * (SB * blk + f[1]) + h, slice(HT // 2, HT))
        else:
            slot, r = _v_slot(star, blk, f)
            x = _ld(pf[h], slot, slice(r // 2, (r + HT) // 2))
        v = _dot(x, _ld(pf[h], (_HSLOT if J is None else J * len(_FULL.pf)) + star.pf[star.pv[f]]))
        res.append(v)
        key = (star.n,) + f
        acc[key] = v if key not in acc else acc[key] + v
        if not last:
            return

        def add(which, i, v, sign=1):
            k_ = (star.n, which, i)
            if k_ not in fg:
                fg[k_] = v if sign > 0 else -v
            else:
                fg[k_] = fg[k_] + v if sign > 0 else fg[k_] - v

        if f[0] == 'W':
            add('F', f[1], acc.pop(key))
        elif f[0] == 'B':
            add('G', f[1], acc.pop(key), csign[star.n, f[1]])
        elif f[0] == 'Q3':
            _, i, j = f
            q1, q2, q3 = (acc.pop((star.n, q, i, j)) for q in ('Q1', 'Q2', 'Q3'))
            t = ((q1 + q2) + q3) * (1.0 / (star.ts[i] - star.ts[j]))
            add('G', i, t)
            add('G', j, t)
            add('F', i, q1)
            add('F', j, q3, -1)

    def job_v(I, h, i, k):
        u = 2 * (SB * I + i) + h
        v = _dot(_ld(v_scr, 2 * (SB * I + k) + h), _ld(pf[h], _DSLOT + _DCELLS.index((i, k))))
        res.append(v)
        dacc[u] = v if u not in dacc else dacc[u] + v
        if k == i:
            o = dacc.pop(u)
            for star, a in ([(_FULL, i)] if I else []) + ([(_HALF, i - 2)] if i >= 2 else []):
                f, g = fg.pop((star.n, 'F', a)), fg.pop((star.n, 'G', a))
                o = o + jnp.concatenate([f - star.ts[a] * g, g], axis=0)
            o = o * (1.0 / lrow[u])
            of[u] = o
            chk[0] = chk[0] + jnp.sum(o.reshape(T // 8, 8, T), axis=0)

    def job_o(_, n):
        af, bf, outs = _O_JOBS[n][1]
        if af not in lhs:
            v = _form(af, lambda i, h: of[2 * i + h])
            lhs[af] = _tie(v.astype(BF16).T, v[0:8, :])
        if bf not in wo:
            wo[bf] = (wo_ref[_tile(bf[0][1]), _tile(bf[0][2])] if len(bf) == 1 else
                      _form(bf, lambda h, j: wo_ref[_tile(h), _tile(j)].astype(F32)).astype(BF16))
            if HACKWO:
                wo[bf] = _ld(q_scr, len(wo) % 32)
        v = _dot(lhs[af], wo[bf])
        res.append(v)
        for sign, i, j in outs:
            terms.setdefault((i, j), []).append((sign, v))
            if len(terms[i, j]) == left[i, j]:
                tot = acc_scr[_tile(i), _tile(j)]
                for sg, m in terms.pop((i, j)):
                    tot = tot + m if sg > 0 else tot - m
                acc_scr[_tile(i), _tile(j)] = tot

    fns = dict(e=job_e, f=job_f, d=job_d, p=job_p, v=job_v, o=job_o)
    order = _job_order(q_scr.shape[0] // (2 * SB))
    for n, job in enumerate(order):
        assert job[0] not in 'efd' or not any(j[0] in 'pv' and j[2] == job[2] and j[1] < job[1] for j in order[n:])
    side = list(side)
    fences = [n for n, job in enumerate(order) if job[0] == 'd' and job[3:] == _DCELLS[-1]]
    step = (len(order) - SIDE0 - SIDE1 - 10) / len(side)
    for n, job in enumerate(order):
        done_side[1] = n
        fns[job[0]](*job[1:])
        last_chance = n >= len(order) - SIDE1
        near = any(-SG1 <= f - n <= SG0 for f in fences)
        if side and n >= SIDE0 + step * done_side[0] and ((job[0] in SKIND and not near) or last_chance):
            done_side[0] += 1
            v = side.pop(0)(res[-1 - SLAG][8 * (n % 4):8 * (n % 4) + 8, :])
            if v is not None:
                due.append((n + SDUE, v))
    assert not side and not due
    fine = jnp.abs(chk[0]) < jnp.inf
    flag_scr[...] = jnp.maximum(flag_scr[...], jnp.where(fine, chk[1], 1.0))


def _kernel(x_hbm, c_hbm, wq_hbm, wuk_hbm, wuv_hbm, wo_hbm, w1_hbm, w2_hbm, w3_hbm, w4_hbm,
            cond_hbm, wmod_hbm, out_hbm,
            x_ref, c_ref, cond_ref, wma_ref, wmb_ref, w1_ref, w3_ref,
            wq_buf, wk_buf, wv_buf, wo_buf, out_buf, sem, wsem, osem,
            mod_scr, h_scr, cs_scr, hs_scr, w_scr, q_scr, k_scr, v_scr, acc_scr, xn_scr, xh_scr, a1_scr, t_scr,
            mw_scr, wt_scr, wf_scr, gap_scr, st_in, pf_scr, vf_scr, flag_scr):
    S, M = x_hbm.shape
    D = wq_hbm.shape[2]
    nattn = wo_hbm.shape[0]
    Fd = w4_hbm.shape[0]
    scale = float(D) ** -0.5 * LOG2E
    nb, nrb = S // T, S // RB
    km, kc = M // T, c_hbm.shape[1] // T
    NX = 4
    XR = S // NX
    CB = XR // T

    work = (wk_buf, wv_buf, wq_buf)

    def pcopies(g, bufs=work, s0=0):
        return [pltpu.make_async_copy(src.bitcast(U32).at[:, g, :], dst, wsem.at[s0 + j])
                for j, (src, dst) in enumerate(zip((wuk_hbm, wuv_hbm, wq_hbm), bufs))]

    def ocopy(g):
        return pltpu.make_async_copy(wo_hbm.at[g], wo_buf, wsem.at[3])

    def chunk_copy(src, dst, i, s0):
        rows = slice(i * XR, (i + 1) * XR)
        return pltpu.make_async_copy(src.at[rows, :], dst.at[rows, :], sem.at[s0 + i])

    MS = 16
    NSL = T // MS
    assert nattn - 1 >= NSL
    mixw = ((w1_hbm, km, 0), (w2_hbm, km, km * MS), (w3_hbm, Fd // T, 2 * km * MS),
            (w4_hbm, -(-Fd // T), (2 * km + Fd // T) * MS))

    def prep_in(g):
        o = jnp.minimum(g, NSL - 1) * MS
        return [pltpu.make_async_copy(
            w.at[pl.ds(pl.multiple_of(jnp.minimum(b * T + o, w.shape[0] - MS), MS), MS), :],
            st_in.at[r0 + b * MS:r0 + (b + 1) * MS, :], wsem.at[7]) for w, nblk, r0 in mixw for b in range(nblk)]

    def stage_in(g):
        return pcopies(jnp.minimum(g + 1, nattn - 1))

    cp_cond = pltpu.make_async_copy(cond_hbm, cond_ref, sem.at[0])
    cp_wma = pltpu.make_async_copy(wmod_hbm.at[:, 0:2 * M], wma_ref, sem.at[1])
    cp_late = [pltpu.make_async_copy(src, dst, sem.at[2 + j]) for j, (src, dst) in enumerate((
        (wmod_hbm.at[:, 2 * M:6 * M], wmb_ref), (w1_hbm, w1_ref), (w3_hbm.at[Fd // T * T:, :], w3_ref)))]
    cp_x = [chunk_copy(x_hbm, x_ref, i, 7) for i in range(NX)]
    cp_c = [chunk_copy(c_hbm, c_ref, i, 7 + NX) for i in range(NX)]

    def silu_cond():
        cf = cond_ref[...].astype(F32)
        return jnp.broadcast_to((cf * jax.nn.sigmoid(cf)).astype(BF16), (8, M))

    cp_wk, cp_wv, cp_wq = pcopies(0)
    named = dict(k=cp_wk, v=cp_wv, q=cp_wq, o=ocopy(0), n=cp_cond, m=cp_wma)
    named.update(zip('abcd', cp_c))
    named.update(zip('wxyz', cp_x))
    started, arrived, did = set(), set(), set()

    def zero(r, carry):
        acc_scr[pl.ds(pl.multiple_of(r * T, T), T), :] = jnp.zeros((T, M), F32)
        return carry

    def x_rows(rows, dep):
        xf = x_ref[rows, :].astype(F32)
        if dep is None:
            return xf
        return jnp.concatenate([_after(xf[:, :T], _rows(dep, xf.shape[0])), xf[:, T:]], axis=1)

    def n_item(r, i):
        def fn(dep):
            rows = slice(r * T + i * LP, r * T + (i + 1) * LP)
            xn_scr[rows, :] = _ln(x_rows(rows, dep))
        return fn

    def h_item(r, i, normed):
        def fn(dep):
            rows = slice(i * LP, (i + 1) * LP)
            grows = slice(r * T + i * LP, r * T + (i + 1) * LP)
            sa = mod_scr[:, 0:M]
            if normed and dep is not None:
                sa = jnp.concatenate([_after(sa[:, _tile(j)], dep) for j in range(km)], axis=1)
            hf = ((xn_scr[grows, :] if normed else _ln(x_rows(grows, dep))) * _rows(mod_scr[:, M:2 * M], LP)
                  + _rows(sa, LP))
            for j in range(km):
                h_scr[r, j, rows, :] = hf[:, _tile(j)].astype(BF16)
            for f, n in _H_SUMS.items():
                if all(t[1] == r for t in f):
                    hs_scr[n, rows, :] = _form(f, lambda _, k: hf[:, _tile(k)]).astype(BF16)
            did.add(('h', r, i))
        return fn

    def release(jobs, span, items):
        if span and items:
            jobs.side += [(len(jobs.res) + 1 + i * span // len(items), fn) for i, fn in enumerate(items)]
            jobs.side.sort(key=lambda e: e[0])
        else:
            for fn in items:
                fn(None)

    def sum_items(n, group, index, dst, get, skip_rows):
        forms = [f for f in dict.fromkeys(t[0] for t in group)
                 if len(f) > 1 and not (skip_rows and len({t[1] for t in f}) == 1)]

        def item(f, rows):
            def fn(dep):
                def term(r, k):
                    v = get(r, k, rows).astype(F32)
                    return v if dep is None or (r, k) != f[0][1:] else _after(v, _rows(dep, v.shape[0]))
                dst[index[f], rows, :] = _form(f, term).astype(BF16)
            return fn

        return [item(f, slice(i, i + n)) for i in range(0, T, n) for f in forms]

    h_sums = lambda n, gi: sum_items(n, _H_GROUPS[gi], _H_SUMS, hs_scr,
                                     lambda r_, k, rows: h_scr[r_, k, rows, :], True)

    def stash(key, buf, j0, transpose=False):
        n = buf.shape[0] // T
        if key not in did:
            assert key in arrived
            did.add(key)
            for (j, hd), w in _pair_tiles(buf, transpose).items():
                w_scr[hd, j0 + j] = w
        return lambda hd: [_ld(w_scr, hd, j0 + j) for j in range(n)]

    def kv_tile(jobs, r):
        wk, wvT = stash('k', wk_buf, 0), stash('v', wv_buf, kc, True)
        ct = [c_ref[_tile(r), _tile(j)] for j in range(kc)]
        for hd in range(2):
            k_scr[2 * r + hd] = jobs.mm(ct, wk(hd), _dot).astype(BF16)
        for hd in range(2):
            v_scr[2 * r + hd] = jobs.mm(wvT(hd), ct, _dot_nt).astype(BF16)

    def q_tile(jobs, r):
        wq = stash('q', wq_buf, 2 * kc)
        ht = [_ld(h_scr, r, j) for j in range(km)]
        for hd in range(2):
            v = (jobs.mm(ht, wq(hd), _dot) * scale).astype(BF16)
            q_scr[2 * r + hd] = v.T if 2 * r + hd in QT else v

    for blk in _prologue().split(';'):
        waits, starts, acts = blk.split('|')
        for ch in waits.strip():
            assert ch in started and ch not in arrived
            arrived.add(ch)
            named[ch].wait()
        for ch in starts.strip():
            assert ch not in started
            started.add(ch)
            named[ch].start()
        jobs = _Jobs()
        for act in acts.split():
            if act == 'Z':
                jax.lax.fori_loop(0, nb, zero, 0)
                acc_scr[S:, :] = jnp.zeros((acc_scr.shape[0] - S, M), F32)
                x_ref[S:, :] = jnp.zeros((x_ref.shape[0] - S, M), BF16)
                flag_scr[...] = jnp.zeros(flag_scr.shape, F32)
            elif act == 'L':
                did.add('L')
                assert ('Q', 0) in did
                for cp in stage_in(0) + prep_in(0):
                    cp.start()
            elif act == 'M':
                assert arrived >= set('nm')
                mod = _dot(silu_cond(), wma_ref[...])
                mod_scr[:, 0:M] = mod[:, 0:M]
                mod_scr[:, M:2 * M] = 1.0 + mod[:, M:2 * M]
                did.add('M')
            else:
                act, _, span = act.partition('@')
                span = int(span or 0)
                items = []
                for r in [int(ch, 16) for ch in act[1:]]:
                    did.add((act[0], r))
                    if act[0] == 'K':
                        assert 'abcd'[r // CB] in arrived
                        kv_tile(jobs, r)
                    elif act[0] == 'H':
                        assert 'wxyz'[r // CB] in arrived and 'M' in did
                        items += [h_item(r, i, ('N', r) in did) for i in range(T // LP)]
                    elif act[0] == 'N':
                        assert 'wxyz'[r // CB] in arrived
                        items += [n_item(r, i) for i in range(T // LP)]
                    elif act[0] == 'Q':
                        assert all(('h', r, i) in did for i in range(T // LP))
                        q_tile(jobs, r)
                    elif act[0] == 'F':
                        assert all(('K', SB * r + k_) in did for k_ in range(SB))
                        items += _v_form_items(v_scr, (pf_scr, vf_scr), r)
                    elif act[0] == 'C':
                        assert all('abcd'[t[1] // CB] in arrived for p_ in _C_GROUPS[r] for t in p_[0])
                        items += sum_items(
                            32, _C_GROUPS[r], _C_SUMS, cs_scr,
                            lambda r_, k, rows: c_ref[r_ * T + rows.start:r_ * T + rows.stop, _tile(k)], False)
                    else:
                        assert act[0] == 'S' and all(('h', t[1], T // LP - 1) in did for p_ in _H_GROUPS[r] for t in p_[0])
                        items += h_sums(32 if span else 16, r)
                release(jobs, span, items)
        assert not jobs.side
    assert arrived == set(named) and all((k_, r) in did for k_ in 'KHQ' for r in range(nb))
    assert all((k_, r) in did for k_ in 'CS' for r in range(2)) and 'L' in did
    assert all(('F', r) in did for r in range(SB))

    def mixer_prep(g):
        sl = jnp.minimum(g, NSL - 1)
        rows = pl.ds(pl.multiple_of(sl * MS, MS), MS)

        def part(m, forms):
            def fn(dep):
                base = {}

                def get(i, k):
                    if (i, k) not in base:
                        rb, cb = (i, k) if m == 2 else (k, i)
                        r0 = mixw[m][2] + rb * MS
                        v = _after(st_in[r0:r0 + MS, _tile(cb)].astype(F32), _rows(dep, MS))
                        if m == 3 and (rb + 1) * T > Fd:
                            v = jnp.where(rb * T + sl * MS < Fd, v, 0.0)
                        base[i, k] = v
                    return base[i, k]

                for f in forms:
                    v = _form(f, get)
                    mw_scr[_MIXW[m, f], rows, :] = (0.5 * v if m % 2 else v).astype(BF16)
            return fn

        items = []
        for m in range(4):
            forms = [f for mm_, f in _MIXW if mm_ == m]
            cur, terms = [], set()
            for f in forms:
                new_terms = terms | {t[1:] for t in f}
                if cur and 3 * len(new_terms) + sum(2 * len(x) + 1 for x in cur + [f]) > MWOPS:
                    items.append(part(m, cur))
                    cur, terms = [], set()
                cur.append(f)
                terms |= {t[1:] for t in f}
            items.append(part(m, cur))
        return items

    def stage_wait():
        for cp in pcopies(0):
            cp.wait()
        pltpu.make_async_copy(st_in, st_in, wsem.at[7]).wait()

    def attn_body(g, carry):
        side = _gap_items(work, gap_scr) + _weight_form_items(work, gap_scr, wt_scr, wf_scr, (0, 1, 2))
        bufs = (q_scr, k_scr, v_scr, (pf_scr, vf_scr), wo_buf, acc_scr, flag_scr)
        _attention_step(*bufs, g >> 16, side)

        @pl.when(g + 1 < nattn)
        def _():
            copies = stage_in(g + 1) + [ocopy(g + 1)]
            for cp in copies:
                cp.start()
            bufs = (h_scr, hs_scr, c_ref, cs_scr, wf_scr, q_scr, k_scr, v_scr, (pf_scr, vf_scr))
            side = [(SD0 + int(i * SDS), fn) for i, fn in enumerate(mixer_prep(g))]
            _proj_step(*bufs, scale, gap_scr, side)
            for cp in prep_in(g + 1):
                cp.start()
            stage_wait()
            ocopy(g + 1).wait()

        return carry

    stage_wait()
    for cp in cp_late:
        cp.start()
    jax.lax.fori_loop(0, nattn, attn_body, 0)

    def safe_pair(g, carry):
        copies = pcopies(g) + [ocopy(g)]
        for cp in copies:
            cp.start()
        for cp in copies:
            cp.wait()
        for buf, j0, transpose in ((wk_buf, 0, False), (wv_buf, kc, True), (wq_buf, 2 * kc, False)):
            for (j, hd), w in _pair_tiles(buf, transpose).items():
                w_scr[hd, j0 + j] = w

        def tile(u, carry):
            r, hd = u // 2, u % 2
            rows = pl.ds(pl.multiple_of(r * T, T), T)
            ct = [c_ref[rows, _tile(j)] for j in range(kc)]
            k_scr[u] = sum(_dot(ct[j], _ld(w_scr, hd, j)) for j in range(kc)).astype(BF16)
            v_scr[u] = sum(_dot_nt(_ld(w_scr, hd, kc + j), ct[j]) for j in range(kc)).astype(BF16)
            q = sum(_dot(_ld(h_scr, r, j), _ld(w_scr, hd, 2 * kc + j)) for j in range(km))
            q_scr[u] = (q * scale).astype(BF16)
            return carry

        jax.lax.fori_loop(0, 2 * nb, tile, 0)
        _attention_safe(q_scr, k_scr, v_scr, wo_buf, acc_scr)
        return carry

    @pl.when(jnp.max(flag_scr[...]) > 0)
    def _():
        jax.lax.fori_loop(0, nb, zero, 0)
        jax.lax.fori_loop(0, nattn, safe_pair, 0)

    for cp in cp_late:
        cp.wait()
    mod = _dot(silu_cond(), wmb_ref[...])
    mod_scr[:, 2 * M:4 * M] = mod[:, 0:2 * M]
    mod_scr[:, 4 * M:5 * M] = 1.0 + mod[:, 2 * M:3 * M]
    mod_scr[:, 5 * M:6 * M] = mod[:, 3 * M:4 * M]
    OFF = x_ref.shape[0] - S
    CAR = t_scr.shape[0] - RB

    def p1(r0, l0, n, dep=None):
        ga = mod_scr[:, 2 * M:3 * M]
        if dep is not None:
            ga = jnp.concatenate([_after(ga[:, 0:T], dep), ga[:, T:]], axis=1)
        rows = pl.ds(r0, n)
        x1 = x_ref[rows, :].astype(F32) + _rows(ga, n) * acc_scr[rows, :]
        xh_scr[0, l0:l0 + n, :] = x1
        hb = _ln(x1) * _rows(mod_scr[:, 4 * M:5 * M], n) + _rows(mod_scr[:, 3 * M:4 * M], n)
        xh_scr[1, l0:l0 + n, :] = hb
        return _ln(hb)

    HT = T // 2

    def p1_store(r0, c, dep=None):
        v = p1(r0 + c * PC, OFF + c * PC, PC, dep)
        a1_scr[c * PC:(c + 1) * PC, :] = v
        return jnp.max(v[:, M - T:].reshape(PC // 8, 8, T), axis=0)

    t_scr[RB:RB + CAR - OFF, :] = jnp.zeros((CAR - OFF, M), F32)
    t_scr[RB + CAR - OFF:RB + CAR, :] = _gelu2(_dot(p1(0, 0, OFF).astype(BF16), w1_ref[...]))
    for c in range(RB // PC):
        p1_store(OFF, c)

    def out_copy(i):
        rows = pl.ds(i * T if isinstance(i, int) else pl.multiple_of(i * T, T), T)
        return pltpu.make_async_copy(out_buf.at[rows, :], out_hbm.at[rows, :], osem.at[i])

    def b_body(r, carry):
        gb = _rows(mod_scr[:, 5 * M:6 * M], T)
        r0 = pl.multiple_of(r * RB, RB)
        n0 = pl.multiple_of(jnp.minimum(r0 + RB, S - RB) + OFF, OFF)
        nh = RB // T
        now = [0]
        due = []
        pace = []

        def p1_item(c):
            def fn(dep):
                due.append((now[0] + PD, p1_store(n0, c, dep)))
                due.sort(key=lambda e: e[0])
            return fn

        pace += [(P0 + i * PSTEP, p1_item(i)) for i in range(RB // PC)]

        def mm(lhs, wts, dot=_dot):
            acc = None
            for x, w in zip(lhs, wts):
                if due and due[0][0] <= now[0]:
                    w = _tie(w, due.pop(0)[1])
                v = dot(x, w)
                now[0] += x.shape[0] // HT
                acc = v if acc is None else v + acc
                if pace and pace[0][0] <= now[0]:
                    pace.pop(0)[1](v[0:8, :])
            return acc

        def fast(m, base, finish, hook=None):
            prods = _MIX[m]
            dot = _dot_nt if m == 2 else _dot
            left, acc, done, cache = {}, {}, {}, {}
            for _, _, outs in prods:
                for _, i, h in outs:
                    left[i, h] = left.get((i, h), 0) + 1

            def act(form):
                sign, form = _canon(form)
                if form not in cache:
                    cache[form] = _form(form, lambda k, h: base(k)[h * HT:(h + 1) * HT]).astype(BF16)
                return sign, cache[form]

            for pi, (wf, af, outs) in enumerate(prods):
                w = _ld(mw_scr, _MIXW[m, wf])
                if af is None:
                    k = wf[0][2]
                    v = mm([jnp.concatenate([act(((1, k, h),))[1] for h in range(2)], axis=0)], [w], dot)
                    sign, parts = 1, [v[:HT], v[HT:]]
                else:
                    sign, x = act(af)
                    parts = [mm([x], [w], dot)] * len(outs)
                for (s_, i, h), v in zip(outs, parts):
                    s_ = s_ * sign
                    if (i, h) not in acc:
                        acc[i, h] = (s_, v)
                    else:
                        s0, u = acc[i, h]
                        acc[i, h] = (s0, u + v if s0 == s_ else u - v) if s0 > 0 or s_ < 0 else (1, v - u)
                    left[i, h] -= 1
                    if not left[i, h]:
                        s0, done[i, h] = acc.pop((i, h))
                        assert s0 > 0
                        if (i, 1 - h) in done:
                            finish(i, jnp.concatenate([done[i, 0], done[i, 1]], axis=0))
                if hook is not None:
                    hook(pi, act)

        t_scr[0:CAR, :] = t_scr[RB:RB + CAR, :]
        for hf in range(nh):
            def put_t(n, v):
                t = _gelu2(v)
                if hf == nh - 1:
                    t = jnp.concatenate([t[:T - OFF], jnp.where(r < nrb - 1, t[T - OFF:], 0.0)], axis=0)
                t_scr[CAR + hf * T:CAR + (hf + 1) * T, _tile(n)] = t

            fast(0, lambda k: a1_scr[_tile(hf), _tile(k)], put_t)
        cq = M // 4
        shifts = (-1, 1, -2, 2)
        lane = jax.lax.broadcasted_iota(jnp.int32, (T, T), 1)
        y1, z, a3 = [], [], []
        for hf in range(nh):
            base = CAR - OFF + hf * T
            sh = []
            for j in range(km):
                g_lo, g_hi = (j * T) // cq, ((j + 1) * T - 1) // cq
                assert g_hi - g_lo <= 1
                v = t_scr[base + shifts[g_lo]:base + shifts[g_lo] + T, _tile(j)]
                if g_hi != g_lo:
                    v2 = t_scr[base + shifts[g_hi]:base + shifts[g_hi] + T, _tile(j)]
                    v = jnp.where(lane < g_hi * cq - j * T, v, v2)
                else:
                    v = jnp.where(lane < T, v, 0.0)
                sh.append(v)
            hs = {}
            fast(1, lambda k: sh[k], hs.__setitem__)
            hs = jnp.concatenate([hs[n] for n in range(km)], axis=1)
            y1.append(hs + xh_scr[1, _tile(hf), :])
            z.append(xh_scr[0, _tile(hf), :] + gb * y1[hf])
            a3.append({})

            def ln_item(hf, c):
                def item(dep):
                    n = HT // NLN
                    for d in (0, HT):
                        v = y1[hf][d + c * n:d + (c + 1) * n]
                        if dep is not None:
                            v = jnp.concatenate([_after(v[:, :T], _rows(dep, n)), v[:, T:]], axis=1)
                        a3[hf][d + c * n] = _ln(v)
                return item

            ln_item(hf, 0)(None)
            pace += [(now[0] + LN0 + (c - 1) * LNS * (1 + hf), ln_item(hf, c)) for c in range(1, NLN)]
            pace.sort(key=lambda e: e[0])
        xh_scr[:, 0:OFF, :] = xh_scr[:, RB:RB + OFF, :]
        h3 = []
        for hf in range(nh):
            assert len(a3[hf]) == 2 * NLN
            af = jnp.concatenate([a3[hf][key] for key in sorted(a3[hf])], axis=0)
            row = {}
            narrow = []

            def hook(pi, act):
                j, rem = divmod(pi - NAR0, NARS)
                if rem == 0 and 0 <= j < km:
                    full = jnp.concatenate([act(((1, j, h),))[1] for h in range(2)], axis=0)
                    v = mm([w3_ref[:, _tile(j)]], [full], _dot_nt)
                    narrow[:] = [v + narrow[0] if narrow else v]

            def put_h(n, v):
                row[n] = _gelu2(v)
                if GD:
                    due.append((now[0] + GD, jnp.max(row[n].reshape(T // 8, 8, T), axis=0)))
                    due.sort(key=lambda e: e[0])

            fast(2, lambda k: af[:, _tile(k)], put_h, hook)
            fw = w3_ref.shape[0]
            row[Fd // T] = jnp.concatenate([_gelu2(narrow[0]), jnp.zeros((T - fw, T), F32)], axis=0).T
            h3.append(row)
        for hf in range(nh):
            rows = pl.ds(pl.multiple_of(r0 + hf * T, T), T)

            def finish(n, v):
                out_buf[rows, _tile(n)] = (z[hf][:, _tile(n)] + gb[:, _tile(n)] * v).astype(out_buf.dtype)

            fast(3, lambda k: h3[hf][k], finish)
            out_copy(r * nh + hf).start()
        assert not pace
        return carry

    jax.lax.fori_loop(0, nrb, b_body, 0)
    for i in range(nb):
        out_copy(i).wait()


@jax.jit
def pallas_adaLN_cond__compressed_kv_cla__mixer_s_mlp__prompt_kernel(
    A_x: jax.Array,
    A_c_kv: jax.Array,
    A_w_q: jax.Array,
    A_w_uk: jax.Array,
    A_w_uv: jax.Array,
    A_w_o: jax.Array,
    B_x: jax.Array,
    B_w1: jax.Array,
    B_w2: jax.Array,
    B_w3: jax.Array,
    B_w4: jax.Array,
    c: jax.Array,
    w_mod: jax.Array,
):
    _, S, M = A_x.shape
    Dc = A_c_kv.shape[2]
    H, D = A_w_q.shape[1], A_w_q.shape[2]
    Fd = B_w3.shape[1]
    assert D == T and A_c_kv.shape[1] == S and Dc == 4 * T and M == 5 * T and 13 * T < Fd < 14 * T and S == 16 * T
    vmem = pltpu.VMEM
    packed = lambda *lead: vmem(lead + (T, T), BF16)
    out = pl.pallas_call(
        _kernel,
        in_specs=[pl.BlockSpec(memory_space=pltpu.HBM)] * 12,
        out_specs=pl.BlockSpec(memory_space=pltpu.HBM),
        out_shape=jax.ShapeDtypeStruct((S, M), A_x.dtype),
        scratch_shapes=[
            vmem((S + 16, M), BF16),
            vmem((S, Dc), BF16),
            vmem((1, M), BF16),
            vmem((M, 2 * M), BF16),
            vmem((M, 4 * M), BF16),
            vmem((M, M), BF16),
            vmem((Fd % T, M), BF16),
            vmem((M, D), U32),
            vmem((Dc, D), U32),
            vmem((Dc, D), U32),
            vmem((2 * D, M), BF16),
            vmem((S, M), A_x.dtype),
            pltpu.SemaphoreType.DMA((15,)),
            pltpu.SemaphoreType.DMA((8,)),
            pltpu.SemaphoreType.DMA((S // T,)),
            vmem((8, 6 * M), F32),
            vmem((S // T, M // T, T, T), BF16),
            vmem((len(_C_SUMS), T, T), BF16),
            vmem((len(_H_SUMS), T, T), BF16),
            packed(2, M // T + 2 * (Dc // T)),
            packed(2 * S // T),
            packed(2 * S // T),
            packed(2 * S // T),
            vmem((S + 16, M), F32),
            vmem((S, M), F32),
            vmem((2, RB + 16, M), F32),
            vmem((RB, M), F32),
            vmem((RB + 32, M), F32),
            packed(len(_MIXW)),
            vmem((Dc // T, T, T), U32),
            vmem((len(_WF), T, T), BF16),
            vmem((3, 8, T), jnp.int32),
            vmem(((2 * (M // T) + Fd // T + -(-Fd // T)) * 16, M), BF16),
            vmem((_FENCE + 1, T, T), BF16),
            vmem((_FENCE + 1, T, T), BF16),
            vmem((8, T), F32),
        ],
        compiler_params=pltpu.CompilerParams(
            vmem_limit_bytes=100 * 1024 * 1024,
            disable_bounds_checks=True,
        ),
    )(
        A_x.reshape(S, M), A_c_kv.reshape(S, Dc),
        A_w_q, A_w_uk, A_w_uv,
        A_w_o.reshape(H // 2, 2 * D, M),
        B_w1, B_w2, B_w3.T, B_w4, c, w_mod,
    )
    return out.reshape(1, S, M)
```

```python
import functools
import math

import jax
import jax.numpy as jnp
import jax.experimental.pallas as pl
import jax.experimental.pallas.tpu as pltpu

F32 = jnp.float32
BF16 = jnp.bfloat16
U32 = jnp.uint32
NT = (((1,), (1,)), ((), ()))
T = 128
EPS = 1e-5
LOG2E = math.log2(math.e)

GRP = 4
LEAD = 10
PROW = 3
RES = 32
LAT_0 = 32
LAT_A = 16
LAT_B = 20
ALEAD = 32
QT = (4, 6)
ONV, OEND = 0.5, 24
FPOS, DPOS = 0, 0
SIDE0, SIDE1, SLAG, SDUE = 8, 60, 4, 8
SKIND = 'pvo'
HACKWO = 0
SG0, SG1 = 6, 4
SD0, SDS = 4, 1.5
WFN = (4, 4, 6)
VF0, VFS = 4, 1.7
L_LO, L_HI, L_RATIO = 2.0 ** -24, 2.0 ** 24, 4.0
RB = 256
PC = 32
P0, PSTEP, PD = 360, 27, 48
GD, NAR0, NARS = 36, 4, 8
PDUE = 20
MWOPS = 70
NLN, LN0, LNS = 4, 4, 5
LP = 16
SP0, SP1 = 76, 38
_prologue = lambda: ('|kva|Z; |b|; kva|wc|K0123; bw|xdn|C0@56 N0123@52 K4567; cx|mq|N4567@52 F0@56 K89ab; '
            'd|y|C1@56 F1@56 Kcdef; nmq|zo|M H01 H234567@30 F2@36 Q0123; y||H89ab@30 F3@36 Q4567; '
            'zo||L Hcdef@30 S0@%d Q89ab S1@%d Qcdef' % (SP0, SP1))


def _dot(a, b):
    return jnp.dot(a, b, preferred_element_type=F32)


def _dot_nt(a, b):
    return jax.lax.dot_general(a, b, NT, preferred_element_type=F32)


def _ln(x):
    m = jnp.mean(x, axis=-1, keepdims=True)
    xc = x - m
    v = jnp.mean(xc * xc, axis=-1, keepdims=True)
    return xc * jnp.exp2(jnp.log(v + EPS) * (-0.5 * LOG2E))


def _rows(v, n):
    return jnp.broadcast_to(v[None], (n // 8, 8, v.shape[1])).reshape(n, v.shape[1])


def _gelu2(x):
    c0 = math.sqrt(2.0 / math.pi)
    return x + x * jnp.tanh(x * (c0 + (c0 * 0.044715) * (x * x)))


def _after(x, dep):
    return jnp.where(dep > jnp.inf, dep, x)


def _tie(x, dep):
    xu = pltpu.bitcast(x, U32)
    first = jnp.where(dep > jnp.inf, jnp.uint32(0), xu[:8])
    return pltpu.bitcast(jnp.concatenate([first, xu[8:]], axis=0), BF16)


def _tile(j):
    return slice(j * T, (j + 1) * T)


def _ld(ref, *idx):
    return pltpu.bitcast(ref.bitcast(U32)[idx], BF16)


def _a_ops(a11, a12, a21, a22):
    return [a11 + a22, a21 + a22, a11, a22, a11 + a12, a21 - a11, a12 - a22]


def _b_ops(b11, b12, b21, b22):
    return [b11 + b22, b11, b12 - b22, b21 - b11, b22, b11 + b12, b21 + b22]


def _strassen(prod, col1=None, col2=None):
    m4 = prod(3)
    m2 = prod(1)
    c21 = m2 + m4
    if col1 is not None:
        e11, e21 = col1()
        m4, c21 = m4 + e11, c21 + e21
    m3 = prod(2)
    m5 = prod(4)
    c12 = m3 + m5
    if col2 is not None:
        e12, e22 = col2()
        c12, m3 = c12 + e12, m3 + e22
    m1 = prod(0)
    c11 = prod(6) + (m1 + (m4 - m5))
    c22 = prod(5) + (m1 + (m3 - m2))
    return c11, c12, c21, c22


def _group(rows, cols, pairs):
    xs, ys = dict.fromkeys(x for x, _ in pairs), dict.fromkeys(y for _, y in pairs)
    used = set(xs) | set(ys) | {(x[0], y[1]) for x, y in pairs} | {(y[0], x[1]) for x, y in pairs}
    prods = []
    for n, r in enumerate(rows):
        for i, k in [x for x in xs if x[0] == r]:
            mates = [y for x, y in pairs if x == (i, k)]
            prods.append((((1, i, k),) + tuple((1, i, k2) for _, k2 in mates), ((1, k, 0),),
                          ((1, i, 0), (-1, i, 1))))
            prods.append((((1, i, k),) + tuple((-1, i2, k) for i2, _ in mates), ((1, k, 0), (1, k, 1)),
                          ((1, i, 1),)))
        for i2, k2 in [y for y in ys if y[0] == r]:
            mates = [x for x, y in pairs if y == (i2, k2)]
            prods.append((((1, i2, k2),) + tuple((1, i2, k) for _, k in mates), ((1, k2, 1),),
                          ((1, i2, 1), (-1, i2, 0))))
            prods.append((((1, i2, k2),) + tuple((-1, i, k2) for i, _ in mates), ((1, k2, 0), (1, k2, 1)),
                          ((1, i2, 0),)))
        prods += [(((1, r, k),), ((1, k, h),), ((1, r, h),)) for k in cols if (r, k) not in used for h in (0, 1)]
        for (i, k), (i2, k2) in pairs:
            if r in (i, i2) and i + i2 - r in rows[n + 1:]:
                prods.append((((1, i, k2),), ((1, k2, 0), (-1, k, 0)), ((1, i2, 0), (1, i, 0))))
                prods.append((((1, i2, k), (1, i, k2)), ((1, k, 0), (1, k2, 1)), ((1, i2, 0), (1, i, 1))))
                prods.append((((1, i2, k),), ((1, k, 1), (-1, k2, 1)), ((1, i2, 1), (1, i, 1))))
    return prods


def _all_pairs(xrows, yrows):
    return [((x, a), (y, b)) for a, x in enumerate(xrows) for b, y in enumerate(yrows) if a != b]


_PAIRS65 = [((x[0] + 10, x[1]), (y[0] + 10, y[1])) for x, y in (
    ((0, 1), (1, 0)), ((0, 1), (5, 2)), ((2, 3), (1, 0)), ((2, 3), (3, 1)), ((2, 3), (5, 2)), ((3, 2), (1, 0)),
    ((4, 4), (0, 3)), ((4, 4), (1, 0)), ((4, 4), (3, 1)), ((4, 4), (5, 2)))]
_C_GROUPS = [_group(range(r, r + 8), range(4), _all_pairs(range(r, r + 4), range(r + 4, r + 8))) for r in (0, 8)]
_H_GROUPS = [_group(range(10), range(5), _all_pairs(range(5), range(5, 10))),
             _group(range(10, 16), range(5), _PAIRS65)]
_sum_index = lambda groups: {f: n for n, f in enumerate(
    dict.fromkeys(t[0] for g in groups for t in g if len(t[0]) > 1))}
_C_SUMS, _H_SUMS = _sum_index(_C_GROUPS), _sum_index(_H_GROUPS)


def _cells(rows, cols, pairs):
    xs = list(dict.fromkeys(p[0] for p in pairs))
    ys = list(dict.fromkeys(p[1] for p in pairs))
    used = set(xs + ys) | {(x[0], y[1]) for x, y in pairs} | {(y[0], x[1]) for x, y in pairs}

    def home_x(i, k):
        mates = [y for x, y in pairs if x == (i, k)]
        return [(((1, i, k),) + tuple((1, i, k2) for _, k2 in mates), ((1, k, 0),), ((1, i, 0), (-1, i, 1))),
                (((1, i, k),) + tuple((-1, i2, k) for i2, _ in mates), ((1, k, 0), (1, k, 1)), ((1, i, 1),))]

    def home_y(i2, k2):
        mates = [x for x, y in pairs if y == (i2, k2)]
        return [(((1, i2, k2),) + tuple((1, i2, k) for _, k in mates), ((1, k2, 1),), ((1, i2, 1), (-1, i2, 0))),
                (((1, i2, k2),) + tuple((-1, i, k2) for i, _ in mates), ((1, k2, 0), (1, k2, 1)), ((1, i2, 0),))]

    def cross(x, y):
        (i, k), (i2, k2) = x, y
        return [(((1, i, k2),), ((1, k2, 0), (-1, k, 0)), ((1, i2, 0), (1, i, 0))),
                (((1, i2, k), (1, i, k2)), ((1, k, 0), (1, k2, 1)), ((1, i2, 0), (1, i, 1))),
                (((1, i2, k),), ((1, k, 1), (-1, k2, 1)), ((1, i2, 1), (1, i, 1)))]

    direct = lambda i: [(((1, i, k),), None, ((1, i, 0), (1, i, 1))) for k in cols if (i, k) not in used]
    single = lambda i: ([t for x in xs if x[0] == i for t in home_x(*x)]
                        + [t for y in ys if y[0] == i for t in home_y(*y)] + direct(i))
    prods = []
    for n, i in enumerate(rows):
        prods += single(i)
        for i2 in rows[n + 1:]:
            for x, y in pairs:
                if {x[0], y[0]} == {i, i2}:
                    prods += cross(x, y)
    return prods


_square = lambda q: [((a, a), (q + b, b)) for a in range(q) for b in range(q) if a != b]
_shift = lambda pairs, r0: [((x[0] + r0, x[1]), (y[0] + r0, y[1])) for x, y in pairs]
_flip = lambda pairs: [(x[::-1], y[::-1]) for x, y in pairs]
_P35 = [((1, 2), (0, 4)), ((1, 2), (2, 1)), ((2, 3), (0, 4)), ((2, 3), (1, 0))]
_P45 = [((0, 2), (1, 1)), ((2, 4), (0, 3)), ((2, 4), (1, 1)), ((2, 4), (3, 2)), ((3, 0), (0, 3)), ((3, 0), (1, 1))]
_P55 = [((2, 1), (0, 4)), ((2, 1), (1, 0)), ((2, 1), (3, 2)), ((2, 1), (4, 3)), ((3, 3), (0, 4)), ((3, 3), (1, 0)),
        ((4, 2), (0, 4)), ((4, 2), (1, 0))]
_MIX = [_cells(range(5), range(5), _P55), _cells(range(5), range(5), _P55),
        _cells(range(13), range(5), _square(5) + _shift(_P35, 10)),
        _cells(range(5), range(14), _flip(_square(5) + _shift(_P45, 10)))]
_MIXW = {(m, f): n for n, (m, f) in enumerate(dict.fromkeys((m, t[0]) for m in range(4) for t in _MIX[m]))}
_MIX3 = min(n for (m, _), n in _MIXW.items() if m == 2)


def _form(form, get):
    acc = None
    for sign, i, j in form:
        v = get(i, j)
        acc = v if acc is None else (acc + v if sign > 0 else acc - v)
    return acc


def _gap_items(bufs, gap_scr):
    items = []
    for n, buf in enumerate(bufs):
        acc = []

        def part(r0, buf=buf, acc=acc):
            def fn(dep):
                wu = jnp.concatenate([buf[r:r + 8, :] for r in range(r0, r0 + T, 32)])
                mask = jnp.full((8, T), 0x7FFF0000, U32)
                if dep is not None:
                    mask = jnp.where(dep > jnp.inf, jnp.uint32(0), mask)
                mask = _rows(mask, 32)
                new = [jnp.sum(pltpu.bitcast(v & mask, F32).reshape(4, 8, T), axis=0) for v in (wu << 16, wu)]
                acc[:] = [u + v for u, v in zip(acc, new)] if acc else new
            return fn

        def last(_, n=n, acc=acc):
            bits = []
            for v in acc:
                l1 = jnp.sum(jnp.sum(v, axis=1, keepdims=True), axis=0, keepdims=True)
                bits.append(pltpu.bitcast(jnp.broadcast_to(l1, (8, T)), jnp.int32) >> 8)
            gap = jnp.clip((bits[0] - bits[1] + (1 << 14)) >> 15, -8, 8) << 23
            gap_scr[n] = gap
            return pltpu.bitcast(gap, F32)

        items += [part(r0) for r0 in range(0, buf.shape[0], T)] + [last]
    return items


def _pair_tiles(w_ref, transpose=False):
    tiles = {}
    for j in range(w_ref.shape[0] // T):
        wu = w_ref[_tile(j), :]
        if transpose:
            wu = wu.T
        tiles[j, 0] = pltpu.bitcast(wu << 16, F32).astype(BF16)
        tiles[j, 1] = pltpu.bitcast(wu & jnp.uint32(0xFFFF0000), F32).astype(BF16)
    return tiles


def _canon(form):
    if form[-1][0] < 0 and form[0][1:] > form[1][1:]:
        return -1, ((1,) + form[1][1:], (-1,) + form[0][1:])
    return 1, form


_w_forms = lambda groups: list(dict.fromkeys(_canon(t[1])[1] for g in groups for t in g))
_WF = {key: n for n, key in enumerate([(m, f) for m, groups in enumerate((_C_GROUPS, _C_GROUPS, _H_GROUPS))
                                       for f in _w_forms(groups)])}


def _weight_form_items(bufs, gap_scr, wt_scr, wf_scr, which):
    n = 16
    items = []

    def flip(j):
        def fn(dep):
            wu = bufs[1][_tile(j), :]
            wu = (wu if dep is None else jnp.where(_rows(dep, T) > jnp.inf, jnp.uint32(0), wu)).T
            wt_scr[j] = wu
            return pltpu.bitcast(wu[T - 8:], F32)
        return fn

    def part(m, r0, forms):
        def fn(dep):
            fac = pltpu.bitcast(0x3F800000 + gap_scr[m], F32)
            mask = jnp.full((8, T), 0xFFFF0000, U32)
            sh = jnp.full((8, T), 16, U32)
            if dep is not None:
                mask = jnp.where(dep > jnp.inf, jnp.uint32(0), mask)
                sh = jnp.where(dep > jnp.inf, jnp.uint32(0), sh)
            fac, mask, sh = _rows(fac, n), _rows(mask, n), _rows(sh, n)
            base = {}

            def get(k, h):
                if (k, h) not in base:
                    wu = wt_scr[k, r0:r0 + n, :] if m == 1 else bufs[m][k * T + r0:k * T + r0 + n, :]
                    base[k, h] = pltpu.bitcast(wu & mask, F32) * fac if h else pltpu.bitcast(wu << sh, F32)
                return base[k, h]

            for f in forms:
                wf_scr[_WF[m, f], r0:r0 + n, :] = _form(f, get).astype(BF16)
        return fn

    for m in which:
        forms = [f for mm, f in _WF if mm == m]
        if m == 1:
            items += [flip(j) for j in range(bufs[1].shape[0] // T)]
        per = -(-len(forms) // WFN[m])
        forms.sort(key=lambda f: sorted({t[1] for t in f}))
        items += [part(m, r0, forms[i:i + per]) for r0 in range(0, T, n) for i in range(0, len(forms), per)]
    return items


def _run_group(jobs, prods, a_get, w, transposed, finish):
    left = {}
    for _, _, outs in prods:
        for _, i, h in outs:
            left[i, h] = left.get((i, h), 0) + 1
    acc = {}
    for af, bf, outs in prods:
        sign, wt = w(bf)
        m = jobs.mm([wt], [a_get(af)], _dot_nt) if transposed else jobs.mm([a_get(af)], [wt], _dot)
        for s_, i, h in outs:
            if (i, h) not in acc:
                acc[i, h] = (s_ * sign, m)
            else:
                s0, v = acc[i, h]
                acc[i, h] = (s0, v + m if s0 == s_ * sign else v - m) if s0 > 0 or s_ * sign < 0 else (1, m - v)
            left[i, h] -= 1
            if not left[i, h]:
                s0, v = acc.pop((i, h))
                assert s0 > 0
                finish(2 * i + h, v)


class _Jobs:
    def __init__(self, side=()):
        self.res = []
        self.side = list(side)
        self.due = []

    def mm(self, lhs, wt, dot):
        acc = None
        for x, w in zip(lhs, wt):
            if self.due and self.due[0][0] <= len(self.res):
                x = _tie(x, self.due.pop(0)[1])
            v = dot(x, w)
            self.res.append(v)
            acc = v if acc is None else v + acc
            rel = 4 * (len(self.res) % 4)
            while self.side and self.side[0][0] <= len(self.res):
                out = self.side.pop(0)[1](v[8 * rel:8 * rel + 8, :])
                if out is not None:
                    self.due.append((len(self.res) + PDUE, out))
                rel = (rel + 2) % 16
        return acc


def _proj_step(h_scr, hs_scr, c_ref, cs_scr, wf_scr, q_scr, k_scr, v_scr, pf, scale, shifts, side):
    def weight(m):
        def get(form):
            sign, form = _canon(form)
            return sign, _ld(wf_scr, _WF[m, form])
        get.inv = pltpu.bitcast(0x3F800000 - shifts[m], F32)
        return get

    wk, wvT, wq = weight(0), weight(1), weight(2)
    c_get = lambda f: _ld(cs_scr, _C_SUMS[f]) if len(f) > 1 else c_ref[_tile(f[0][1]), _tile(f[0][2])]
    h_get = lambda f: _ld(hs_scr, _H_SUMS[f]) if len(f) > 1 else _ld(h_scr, f[0][1], f[0][2])

    def put(dst, w, mul=None):
        muls = [mul, _rows(w.inv if mul is None else w.inv * mul, T)]

        def fn(u, v):
            v = (v if muls[u % 2] is None else v * muls[u % 2]).astype(BF16)
            dst[u] = v.T if mul is not None and u in QT else v
        return fn

    jobs = _Jobs(side)
    put_v, stored = put(v_scr, wvT), set()
    nxt = [0]

    def fin_v(u, v):
        put_v(u, v)
        stored.add(u)
        for J in range(SB):
            if all(2 * (SB * J + k) + h in stored for k in range(SB) for h in range(2)) and ('J', J) not in stored:
                stored.add(('J', J))
                for fn in _v_form_items(v_scr, pf, J):
                    nxt[0] = max(nxt[0] + VFS, len(jobs.res) + VF0)
                    jobs.side.append((int(nxt[0]), fn))
                jobs.side.sort(key=lambda e: e[0])

    kk, vv, qq = ((c_get, wk, False, put(k_scr, wk)), (c_get, wvT, True, fin_v),
                  (h_get, wq, False, put(q_scr, wq, scale)))
    for prods, args in ((_C_GROUPS[0], kk), (_C_GROUPS[0], vv), (_C_GROUPS[1], vv), (_C_GROUPS[1], kk),
                        (_H_GROUPS[0], qq), (_H_GROUPS[1], qq)):
        _run_group(jobs, prods, *args)
    assert not jobs.side and not jobs.due


def _inner_group(rows, cols, pairs):
    xs, ys = dict.fromkeys(x for x, _ in pairs), dict.fromkeys(y for _, y in pairs)
    used = set(xs) | set(ys) | {(x[0], y[1]) for x, y in pairs} | {(y[0], x[1]) for x, y in pairs}
    prods = []
    for i, j in xs:
        mates = [y for x, y in pairs if x == (i, j)]
        prods.append((((1, i, 0),), ((1, 0, j), (-1, 1, j)), ((1, i, j),) + tuple((1, i2, j) for i2, _ in mates)))
        prods.append((((1, i, 0), (1, i, 1)), ((1, 1, j),), ((1, i, j),) + tuple((-1, i, j2) for _, j2 in mates)))
    for i2, j2 in ys:
        mates = [x for x, y in pairs if y == (i2, j2)]
        prods.append((((1, i2, 0), (1, i2, 1)), ((1, 0, j2),),
                      ((1, i2, j2),) + tuple((-1, i2, j) for _, j in mates)))
        prods.append((((1, i2, 1),), ((1, 0, j2), (-1, 1, j2)),
                      ((-1, i2, j2),) + tuple((-1, i, j2) for i, _ in mates)))
    prods += [(((1, i, h),), ((1, h, j),), ((1, i, j),))
              for i in rows for j in cols if (i, j) not in used for h in (0, 1)]
    for (i, j), (i2, j2) in pairs:
        lo, hi = min(j, j2), max(j, j2)
        prods.append((((1, i2, 0), (-1, i, 0)), ((1, 0, lo), (1, 0, hi)), ((1, i2, j),)))
        prods.append((((1, i, 0), (1, i2, 1)), ((1, 0, j2), (1, 1, j)), ((1, i, j2), (1, i2, j))))
        prods.append((((1, i, 1), (-1, i2, 1)), ((1, 1, lo), (1, 1, hi)), ((1, i, j2),)))
    return prods


def _o_jobs():
    prods = (_inner_group(range(10), range(5), _all_pairs(range(0, 10, 2), range(1, 10, 2)))
             + _inner_group(range(10, 16), range(5), _PAIRS65))
    row = lambda t: max(i for _, i, _ in t[0])
    unit = lambda t: max(2 * i + h for _, i, h in t[0])
    need = lambda t: unit(t) if row(t) == 15 else 2 * row(t) + 1
    return [(need(t), t) for t in sorted(prods, key=need)]


_O_JOBS = _o_jobs()


SB = 4


class _Star:
    def __init__(self, ts):
        self.ts, self.n = ts, len(ts)
        rn = range(self.n)
        self.pairs = [(i, j) for i in rn for j in rn if i < j]
        self.pf = {f: m for m, f in enumerate([('R', i) for i in rn] + [('C', i) for i in rn]
                                              + [('S', i, j) for i in rn for j in rn if i != j]
                                              + [('A', i, j) for i, j in self.pairs])}
        self.vf = {f: m for m, f in enumerate([('W', i) for i in rn]
                                              + [(q, i, j) for i, j in self.pairs for q in ('Q1', 'Q2', 'Q3')])}
        self.pv = {**{('W', i): ('R', i) for i in rn}, **{('B', i): ('C', i) for i in rn},
                   **{('Q1', i, j): ('S', i, j) for i, j in self.pairs},
                   **{('Q2', i, j): ('A', i, j) for i, j in self.pairs},
                   **{('Q3', i, j): ('S', j, i) for i, j in self.pairs}}

    def products(self, i):
        return [('W', i), ('B', i)] + [(q, i, j) for j in range(i + 1, self.n) for q in ('Q1', 'Q2', 'Q3')]


_FULL = _Star((-1.125, -0.375, 0.375, 1.125))
_HALF = _Star((-0.75, 0.75))
_DCELLS = [(0, 0), (1, 0), (1, 1), (2, 2), (3, 2), (3, 3)]
_HSLOT = (SB - 1) * len(_FULL.pf)
_DSLOT = _HSLOT + len(_HALF.pf)
_VSLOT = _DSLOT + len(_DCELLS)
_VHALF = (SB - 1) * len(_FULL.vf)
_FENCE = _VSLOT + (_VHALF + SB * len(_HALF.vf) + 1) // 2


def _v_slot(star, J, f):
    m = star.vf[f] + J * len(star.vf) + (0 if star is _FULL else _VHALF)
    return _VSLOT + m // 2, m % 2 * (T // 2)


def _v_form_items(v_scr, pf, J):
    n, HT = 16, T // 2

    def item(star, h, r0, pairs):
        def fn(dep):
            ts = [jnp.full((8, T), t, F32) for t in star.ts]
            ts = [_rows(t if dep is None else _after(t, dep), n) for t in ts]

            def get(k, a):
                r = (a * HT + r0) // 2
                return _ld(v_scr, 2 * (SB * J + k) + h, slice(r, r + n // 2)).astype(F32)

            def put(f, v):
                slot, r = _v_slot(star, J, f)
                pf[h][slot, r + r0:r + r0 + n, :] = v.astype(BF16)

            b = {(k, a): get(k, a) for k in sorted({k for pr in pairs or star.pairs for k in pr})
                 for a in range(2)}
            if pairs is None or star.n == 2:
                w = [b[k, 0] + ts[k] * b[k, 1] for k in range(star.n)]
                for k in range(star.n):
                    put(('W', k), w[k])
                for i, j in star.pairs:
                    put(('Q2', i, j), w[i] - w[j])
            for i, j in pairs or ():
                d0, d1 = b[j, 0] - b[i, 0], b[j, 1] - b[i, 1]
                put(('Q1', i, j), d0 + ts[i] * d1)
                put(('Q3', i, j), d0 + ts[j] * d1)
        return fn

    pr = _FULL.pairs
    parts = [(_HALF, _HALF.pairs)]
    if J < SB - 1:
        parts += [(_FULL, x) for x in (None, pr[:2], [pr[2], pr[4]], [pr[3], pr[5]])]
    return [item(star, h, r0, pairs) for h in range(2) for r0 in range(0, HT, n) for star, pairs in parts]


def _job_order(nsb):
    units = [(I, h) for I in range(nsb) for h in range(2)]
    qe, qv = [], []
    for I, h in units:
        es = [('e', I, h, J, p) for J in range(I) for p in range(SB)]
        ds = [('d', I, h) + c for c in _DCELLS]
        es.insert(max(len(es) - FPOS, 0), ('f', I, h))
        qe += es + ds if I or FPOS < 9 else ds[:DPOS] + es + ds[DPOS:]
        for i in range(SB):
            qv += [('p', I, h, f, J) for f in _FULL.products(i) for J in range(I)]
            if i >= 2:
                qv += [('p', I, h, f, None) for f in _HALF.products(i - 2)]
            qv += [('v', I, h) + c for c in _DCELLS if c[0] == i]
    qo = [('o', u, j) for j, (u, _) in enumerate(_O_JOBS)]
    cost = dict(e=8, f=8, d=2, p=1, v=2, o=2)
    order, done = [], {}
    now = [0]

    def emit(q):
        job = q.pop(0)
        order.append(job)
        now[0] += cost[job[0]]
        if job[0] == 'd':
            done[job] = now[0]
        elif job[0] == 'v' and job[4] == job[3]:
            done['u', 2 * (SB * job[1] + job[3]) + job[2]] = now[0]
        return cost[job[0]]

    def v_ready():
        if not qv:
            return False
        key = ('d', qv[0][1], qv[0][2], SB - 1, SB - 1)
        return key in done and done[key] + (LAT_0 if qv[0][1:3] == (0, 0) else LAT_A) <= now[0]

    def o_ready():
        return bool(qo) and ('u', qo[0][1]) in done and done['u', qo[0][1]] + LAT_B <= now[0]

    def fill(nv, no):
        n = 0
        while nv > 0 or no > 0 or n % 4:
            if no > 0 and n % 2 == 0 and o_ready() and no * ONV >= nv:
                no -= 2
                n += emit(qo)
            elif v_ready() and (nv > 0 or n % 4):
                c = emit(qv)
                nv -= c
                n += c
            elif o_ready() and n % 2 == 0 and (no > 0 or n % 4 or nv > 0) and len(qo) > RES:
                no -= 2
                n += emit(qo)
            else:
                break

    while qe:
        unit = qe[0][1:3]
        while qv and qv[0][2] == unit[1] and qv[0][1] < unit[0]:
            emit(qv)
        ne = 0
        while qe and ne < 8 and (ne == 0 or (qe[0][0] == 'd' and qe[0][1:3] == unit and ne + 2 <= 8)):
            ne += emit(qe)
        groups = lambda q: sum(cost[j[0]] for j in q) / 8
        old = [j for j in qv if j[1:3] != unit and ('d', j[1], j[2], SB - 1, SB - 1) in done]
        here = [j for j in qe if j[1:3] == unit]
        rest = sum(cost[j[0]] for j in old)
        nv = (rest - LAT_A) / (groups(here) + 1) if here else rest
        no = 2 * max(len(qo) - RES - OEND, 0) / (groups(qe) + 1)
        fill(int(nv + 0.5), int(no + 0.5))
    while qv or qo:
        if qv and v_ready():
            fill(6, 2)
            if not qv:
                continue
        elif o_ready():
            emit(qo)
        else:
            emit(qv or qo)
    return order


def _attention_safe(q_scr, k_scr, v_scr, wo_ref, acc_scr):
    causal = (jax.lax.broadcasted_iota(jnp.int32, (T, T), 0)
              <= jax.lax.broadcasted_iota(jnp.int32, (T, T), 1))

    def unit(u, carry):
        r, hd = u // 2, u % 2

        def block(c, mlo):
            m0, l, o = mlo
            s = _dot_nt(_ld(k_scr, 2 * c + hd), _ld(q_scr, u))
            s = jnp.where(jnp.logical_or(causal, c < r), s, -1e9 * LOG2E)
            m = jnp.maximum(m0, jnp.max(s, axis=0, keepdims=True))
            a = jnp.exp2(m0 - m)
            p = jnp.exp2(s - m)
            return (m, l * a + jnp.sum(p, axis=0, keepdims=True),
                    o * a + _dot(_ld(v_scr, 2 * c + hd), p.astype(BF16)))

        _, l, o = jax.lax.fori_loop(0, r + 1, block, (jnp.full((1, T), -jnp.inf, F32), jnp.zeros((1, T), F32),
                                                      jnp.zeros((T, T), F32)))
        rows = pl.ds(pl.multiple_of(r * T, T), T)
        acc_scr[rows, :] += _dot((o * (1.0 / l)).astype(BF16).T, wo_ref[pl.ds(pl.multiple_of(hd * T, T), T), :])
        return carry

    jax.lax.fori_loop(0, q_scr.shape[0], unit, 0)


def _attention_step(q_scr, k_scr, v_scr, pf, wo_ref, acc_scr, flag_scr, z, side):
    causal = (jax.lax.broadcasted_iota(jnp.int32, (T, T), 0)
              <= jax.lax.broadcasted_iota(jnp.int32, (T, T), 1))
    HT = T // 2
    lsum, lrow, acc, fg, dacc, of, lhs = {}, {}, {}, {}, {}, {}, {}
    res = []
    wo, terms = {}, {}
    left = {}
    done_side = [0, 0]
    chk = [jnp.zeros((8, T), F32), None]
    for _, t in _O_JOBS:
        for _, i, j in t[2]:
            left[i, j] = left.get((i, j), 0) + 1

    def add_l(u, v):
        lsum[u] = v if u not in lsum else lsum[u] + v

    csign = {}

    def p_forms(star, h, slot0, g, tiles, cell, when):
        n = star.n

        def put(f, v):
            pf[h][slot0 + star.pf[f], 16 * g:16 * g + 16, :] = v.astype(BF16)

        for i in range(n):
            row = [cell(i, k) for k in sorted(range(n), key=lambda k: when(i, k))]
            r = functools.reduce(lambda x, y: x + y, row)
            put(('R', i), r)
            add_l(tiles[i], r[:8] + r[8:])
            col = sorted(range(n), key=lambda i2: (when(i2, i), i2 != i))
            sign = csign[n, i] = 1 if col[0] == i else -1
            c = cell(col[0], i)
            for i2 in col[1:]:
                c = c + cell(i2, i) if (1 if i2 == i else -1) == sign else c - cell(i2, i)
            put(('C', i), c)
            for j in range(n):
                if j != i:
                    put(('S', i, j), cell(i, j))
        for i, j in star.pairs:
            put(('A', i, j), cell(i, j) + cell(j, i))

    due = []

    def scores(x, u):
        if due and due[0][0] <= done_side[1]:
            x = _tie(x, due.pop(0)[1])
        s = (_dot if u in QT else _dot_nt)(x, _ld(q_scr, u))
        res.append(s)
        return s

    def job_e(I, h, J, p):
        tiles = [2 * (SB * I + i) + h for i in range(SB)]
        ps = []
        for i, u in enumerate(tiles):
            x = jnp.concatenate([k_scr.bitcast(U32)[2 * (SB * J + (t - i) % SB) + h, 8 * g:8 * g + 8, :]
                                 for g in (2 * p, 2 * p + 1) for t in range(SB)], axis=0)
            ps.append(jnp.exp2(scores(pltpu.bitcast(x, BF16), u)))
        when = lambda i, k: (i + k) % SB
        for n, g in enumerate((2 * p, 2 * p + 1)):
            cell = lambda i, k: ps[i][16 * (SB * n + when(i, k)):16 * (SB * n + when(i, k)) + 16]
            p_forms(_FULL, h, J * len(_FULL.pf), g, tiles, cell, when)

    def job_f(I, h):
        tiles = [2 * (SB * I + 2 + i) + h for i in range(2)]
        ps = {(i, k): jnp.exp2(scores(_ld(k_scr, 2 * (SB * I + k) + h), u))
              for i, u in enumerate(tiles) for k in range(2)}
        for g in range(T // 16):
            p_forms(_HALF, h, _HSLOT, g, tiles, lambda i, k: ps[i, k][16 * g:16 * g + 16], lambda i, k: 0)

    def job_d(I, h, i, k):
        u = 2 * (SB * I + i) + h
        s = scores(_ld(k_scr, 2 * (SB * I + k) + h), u)
        if i == k:
            s = jnp.where(causal, s, -1e9 * LOG2E)
        p = jnp.exp2(s)
        add_l(u, jnp.sum(p.reshape(T // 8, 8, T), axis=0))
        pf[h][_DSLOT + _DCELLS.index((i, k))] = p.astype(BF16)
        if (i, k) == _DCELLS[-1]:
            pf[h][_FENCE + z, 0:16, :] = jnp.zeros((16, T), BF16)
            for u in [2 * (SB * I + a) + h for a in range(SB)]:
                lrow[u] = jnp.sum(lsum.pop(u), axis=0, keepdims=True)
            ls = [lrow[2 * (SB * I + a) + h] for a in range(SB)]
            lo = jnp.minimum(jnp.minimum(ls[0], ls[1]), jnp.minimum(ls[2], ls[3]))
            hi = jnp.maximum(jnp.maximum(ls[0], ls[1]), jnp.maximum(ls[2], ls[3]))
            ok = jnp.logical_and(lo >= L_LO, hi <= L_HI)
            ok = jnp.logical_and(ok, (hi if I else jnp.maximum(ls[2], ls[3]))
                                 <= L_RATIO * (lo if I else jnp.minimum(ls[2], ls[3])))
            bad = jnp.where(ok, 0.0, 1.0)
            chk[1] = bad if chk[1] is None else jnp.maximum(chk[1], bad)

    def job_p(I, h, f, J):
        star, last = (_HALF, True) if J is None else (_FULL, J == I - 1)
        blk = I if J is None else J
        if f[0] == 'B':
            x = _ld(v_scr, 2 * (SB * blk + f[1]) + h, slice(HT // 2, HT))
        else:
            slot, r = _v_slot(star, blk, f)
            x = _ld(pf[h], slot, slice(r // 2, (r + HT) // 2))
        v = _dot(x, _ld(pf[h], (_HSLOT if J is None else J * len(_FULL.pf)) + star.pf[star.pv[f]]))
        res.append(v)
        key = (star.n,) + f
        acc[key] = v if key not in acc else acc[key] + v
        if not last:
            return

        def add(which, i, v, sign=1):
            k_ = (star.n, which, i)
            if k_ not in fg:
                fg[k_] = v if sign > 0 else -v
            else:
                fg[k_] = fg[k_] + v if sign > 0 else fg[k_] - v

        if f[0] == 'W':
            add('F', f[1], acc.pop(key))
        elif f[0] == 'B':
            add('G', f[1], acc.pop(key), csign[star.n, f[1]])
        elif f[0] == 'Q3':
            _, i, j = f
            q1, q2, q3 = (acc.pop((star.n, q, i, j)) for q in ('Q1', 'Q2', 'Q3'))
            t = ((q1 + q2) + q3) * (1.0 / (star.ts[i] - star.ts[j]))
            add('G', i, t)
            add('G', j, t)
            add('F', i, q1)
            add('F', j, q3, -1)

    def job_v(I, h, i, k):
        u = 2 * (SB * I + i) + h
        v = _dot(_ld(v_scr, 2 * (SB * I + k) + h), _ld(pf[h], _DSLOT + _DCELLS.index((i, k))))
        res.append(v)
        dacc[u] = v if u not in dacc else dacc[u] + v
        if k == i:
            o = dacc.pop(u)
            for star, a in ([(_FULL, i)] if I else []) + ([(_HALF, i - 2)] if i >= 2 else []):
                f, g = fg.pop((star.n, 'F', a)), fg.pop((star.n, 'G', a))
                o = o + jnp.concatenate([f - star.ts[a] * g, g], axis=0)
            o = o * (1.0 / lrow[u])
            of[u] = o
            chk[0] = chk[0] + jnp.sum(o.reshape(T // 8, 8, T), axis=0)

    def job_o(_, n):
        af, bf, outs = _O_JOBS[n][1]
        if af not in lhs:
            v = _form(af, lambda i, h: of[2 * i + h])
            lhs[af] = _tie(v.astype(BF16).T, v[0:8, :])
        if bf not in wo:
            wo[bf] = (wo_ref[_tile(bf[0][1]), _tile(bf[0][2])] if len(bf) == 1 else
                      _form(bf, lambda h, j: wo_ref[_tile(h), _tile(j)].astype(F32)).astype(BF16))
            if HACKWO:
                wo[bf] = _ld(q_scr, len(wo) % 32)
        v = _dot(lhs[af], wo[bf])
        res.append(v)
        for sign, i, j in outs:
            terms.setdefault((i, j), []).append((sign, v))
            if len(terms[i, j]) == left[i, j]:
                tot = acc_scr[_tile(i), _tile(j)]
                for sg, m in terms.pop((i, j)):
                    tot = tot + m if sg > 0 else tot - m
                acc_scr[_tile(i), _tile(j)] = tot

    fns = dict(e=job_e, f=job_f, d=job_d, p=job_p, v=job_v, o=job_o)
    order = _job_order(q_scr.shape[0] // (2 * SB))
    for n, job in enumerate(order):
        assert job[0] not in 'efd' or not any(j[0] in 'pv' and j[2] == job[2] and j[1] < job[1] for j in order[n:])
    side = list(side)
    fences = [n for n, job in enumerate(order) if job[0] == 'd' and job[3:] == _DCELLS[-1]]
    step = (len(order) - SIDE0 - SIDE1 - 10) / len(side)
    for n, job in enumerate(order):
        done_side[1] = n
        fns[job[0]](*job[1:])
        last_chance = n >= len(order) - SIDE1
        near = any(-SG1 <= f - n <= SG0 for f in fences)
        if side and n >= SIDE0 + step * done_side[0] and ((job[0] in SKIND and not near) or last_chance):
            done_side[0] += 1
            v = side.pop(0)(res[-1 - SLAG][8 * (n % 4):8 * (n % 4) + 8, :])
            if v is not None:
                due.append((n + SDUE, v))
    assert not side and not due
    fine = jnp.abs(chk[0]) < jnp.inf
    flag_scr[...] = jnp.maximum(flag_scr[...], jnp.where(fine, chk[1], 1.0))


def _kernel(x_hbm, c_hbm, wq_hbm, wuk_hbm, wuv_hbm, wo_hbm, w1_hbm, w2_hbm, w3_hbm, w4_hbm,
            cond_hbm, wmod_hbm, out_hbm,
            x_ref, c_ref, cond_ref, wma_ref, wmb_ref, w1_ref, w3_ref,
            wq_buf, wk_buf, wv_buf, wo_buf, out_buf, sem, wsem, osem,
            mod_scr, h_scr, cs_scr, hs_scr, w_scr, q_scr, k_scr, v_scr, acc_scr, xn_scr, xh_scr, a1_scr, t_scr,
            mw_scr, m3_scr, wt_scr, wf_scr, gap_scr, st_in, pf_scr, vf_scr, flag_scr):
    S, M = x_hbm.shape
    D = wq_hbm.shape[2]
    nattn = wo_hbm.shape[0]
    Fd = w4_hbm.shape[0]
    scale = float(D) ** -0.5 * LOG2E
    nb, nrb = S // T, S // RB
    km, kc = M // T, c_hbm.shape[1] // T
    NX = 4
    XR = S // NX
    CB = XR // T

    work = (wk_buf, wv_buf, wq_buf)

    def pcopies(g, bufs=work, s0=0):
        return [pltpu.make_async_copy(src.bitcast(U32).at[:, g, :], dst, wsem.at[s0 + j])
                for j, (src, dst) in enumerate(zip((wuk_hbm, wuv_hbm, wq_hbm), bufs))]

    def ocopy(g):
        return pltpu.make_async_copy(wo_hbm.at[g], wo_buf, wsem.at[3])

    def chunk_copy(src, dst, i, s0):
        rows = slice(i * XR, (i + 1) * XR)
        return pltpu.make_async_copy(src.at[rows, :], dst.at[rows, :], sem.at[s0 + i])

    MS = 16
    NSL = T // MS
    assert nattn - 1 >= NSL
    mixw = ((w1_hbm, km, 0), (w2_hbm, km, km * MS), (w3_hbm, Fd // T, 2 * km * MS),
            (w4_hbm, -(-Fd // T), (2 * km + Fd // T) * MS))

    def prep_in(g):
        o = jnp.minimum(g, NSL - 1) * MS
        return [pltpu.make_async_copy(
            w.at[pl.ds(pl.multiple_of(jnp.minimum(b * T + o, w.shape[0] - MS), MS), MS), :],
            st_in.at[r0 + b * MS:r0 + (b + 1) * MS, :], wsem.at[7]) for w, nblk, r0 in mixw for b in range(nblk)]

    def stage_in(g):
        return pcopies(jnp.minimum(g + 1, nattn - 1))

    cp_cond = pltpu.make_async_copy(cond_hbm, cond_ref, sem.at[0])
    cp_wma = pltpu.make_async_copy(wmod_hbm.at[:, 0:2 * M], wma_ref, sem.at[1])
    cp_late = [pltpu.make_async_copy(src, dst, sem.at[2 + j]) for j, (src, dst) in enumerate((
        (wmod_hbm.at[:, 2 * M:6 * M], wmb_ref), (w1_hbm, w1_ref), (w3_hbm.at[Fd // T * T:, :], w3_ref)))]
    cp_x = [chunk_copy(x_hbm, x_ref, i, 7) for i in range(NX)]
    cp_c = [chunk_copy(c_hbm, c_ref, i, 7 + NX) for i in range(NX)]

    def silu_cond():
        cf = cond_ref[...].astype(F32)
        return jnp.broadcast_to((cf * jax.nn.sigmoid(cf)).astype(BF16), (8, M))

    cp_wk, cp_wv, cp_wq = pcopies(0)
    named = dict(k=cp_wk, v=cp_wv, q=cp_wq, o=ocopy(0), n=cp_cond, m=cp_wma)
    named.update(zip('abcd', cp_c))
    named.update(zip('wxyz', cp_x))
    started, arrived, did = set(), set(), set()

    def zero(r, carry):
        acc_scr[pl.ds(pl.multiple_of(r * T, T), T), :] = jnp.zeros((T, M), F32)
        return carry

    def x_rows(rows, dep):
        xf = x_ref[rows, :].astype(F32)
        if dep is None:
            return xf
        return jnp.concatenate([_after(xf[:, :T], _rows(dep, xf.shape[0])), xf[:, T:]], axis=1)

    def n_item(r, i):
        def fn(dep):
            rows = slice(r * T + i * LP, r * T + (i + 1) * LP)
            xn_scr[rows, :] = _ln(x_rows(rows, dep))
        return fn

    def h_item(r, i, normed):
        def fn(dep):
            rows = slice(i * LP, (i + 1) * LP)
            grows = slice(r * T + i * LP, r * T + (i + 1) * LP)
            sa = mod_scr[:, 0:M]
            if normed and dep is not None:
                sa = jnp.concatenate([_after(sa[:, _tile(j)], dep) for j in range(km)], axis=1)
            hf = ((xn_scr[grows, :] if normed else _ln(x_rows(grows, dep))) * _rows(mod_scr[:, M:2 * M], LP)
                  + _rows(sa, LP))
            for j in range(km):
                h_scr[r, j, rows, :] = hf[:, _tile(j)].astype(BF16)
            for f, n in _H_SUMS.items():
                if all(t[1] == r for t in f):
                    hs_scr[n, rows, :] = _form(f, lambda _, k: hf[:, _tile(k)]).astype(BF16)
            did.add(('h', r, i))
        return fn

    def release(jobs, span, items):
        if span and items:
            jobs.side += [(len(jobs.res) + 1 + i * span // len(items), fn) for i, fn in enumerate(items)]
            jobs.side.sort(key=lambda e: e[0])
        else:
            for fn in items:
                fn(None)

    def sum_items(n, group, index, dst, get, skip_rows):
        forms = [f for f in dict.fromkeys(t[0] for t in group)
                 if len(f) > 1 and not (skip_rows and len({t[1] for t in f}) == 1)]

        def item(f, rows):
            def fn(dep):
                def term(r, k):
                    v = get(r, k, rows).astype(F32)
                    return v if dep is None or (r, k) != f[0][1:] else _after(v, _rows(dep, v.shape[0]))
                dst[index[f], rows, :] = _form(f, term).astype(BF16)
            return fn

        return [item(f, slice(i, i + n)) for i in range(0, T, n) for f in forms]

    h_sums = lambda n, gi: sum_items(n, _H_GROUPS[gi], _H_SUMS, hs_scr,
                                     lambda r_, k, rows: h_scr[r_, k, rows, :], True)

    def stash(key, buf, j0, transpose=False):
        n = buf.shape[0] // T
        if key not in did:
            assert key in arrived
            did.add(key)
            for (j, hd), w in _pair_tiles(buf, transpose).items():
                w_scr[hd, j0 + j] = w
        return lambda hd: [_ld(w_scr, hd, j0 + j) for j in range(n)]

    def kv_tile(jobs, r):
        wk, wvT = stash('k', wk_buf, 0), stash('v', wv_buf, kc, True)
        ct = [c_ref[_tile(r), _tile(j)] for j in range(kc)]
        for hd in range(2):
            k_scr[2 * r + hd] = jobs.mm(ct, wk(hd), _dot).astype(BF16)
        for hd in range(2):
            v_scr[2 * r + hd] = jobs.mm(wvT(hd), ct, _dot_nt).astype(BF16)

    def q_tile(jobs, r):
        wq = stash('q', wq_buf, 2 * kc)
        ht = [_ld(h_scr, r, j) for j in range(km)]
        for hd in range(2):
            v = (jobs.mm(ht, wq(hd), _dot) * scale).astype(BF16)
            q_scr[2 * r + hd] = v.T if 2 * r + hd in QT else v

    for blk in _prologue().split(';'):
        waits, starts, acts = blk.split('|')
        for ch in waits.strip():
            assert ch in started and ch not in arrived
            arrived.add(ch)
            named[ch].wait()
        for ch in starts.strip():
            assert ch not in started
            started.add(ch)
            named[ch].start()
        jobs = _Jobs()
        for act in acts.split():
            if act == 'Z':
                jax.lax.fori_loop(0, nb, zero, 0)
                acc_scr[S:, :] = jnp.zeros((acc_scr.shape[0] - S, M), F32)
                x_ref[S:, :] = jnp.zeros((x_ref.shape[0] - S, M), BF16)
                flag_scr[...] = jnp.zeros(flag_scr.shape, F32)
            elif act == 'L':
                did.add('L')
                assert ('Q', 0) in did
                for cp in stage_in(0) + prep_in(0):
                    cp.start()
            elif act == 'M':
                assert arrived >= set('nm')
                mod = _dot(silu_cond(), wma_ref[...])
                mod_scr[:, 0:M] = mod[:, 0:M]
                mod_scr[:, M:2 * M] = 1.0 + mod[:, M:2 * M]
                did.add('M')
            else:
                act, _, span = act.partition('@')
                span = int(span or 0)
                items = []
                for r in [int(ch, 16) for ch in act[1:]]:
                    did.add((act[0], r))
                    if act[0] == 'K':
                        assert 'abcd'[r // CB] in arrived
                        kv_tile(jobs, r)
                    elif act[0] == 'H':
                        assert 'wxyz'[r // CB] in arrived and 'M' in did
                        items += [h_item(r, i, ('N', r) in did) for i in range(T // LP)]
                    elif act[0] == 'N':
                        assert 'wxyz'[r // CB] in arrived
                        items += [n_item(r, i) for i in range(T // LP)]
                    elif act[0] == 'Q':
                        assert all(('h', r, i) in did for i in range(T // LP))
                        q_tile(jobs, r)
                    elif act[0] == 'F':
                        assert all(('K', SB * r + k_) in did for k_ in range(SB))
                        items += _v_form_items(v_scr, (pf_scr, vf_scr), r)
                    elif act[0] == 'C':
                        assert all('abcd'[t[1] // CB] in arrived for p_ in _C_GROUPS[r] for t in p_[0])
                        items += sum_items(
                            32, _C_GROUPS[r], _C_SUMS, cs_scr,
                            lambda r_, k, rows: c_ref[r_ * T + rows.start:r_ * T + rows.stop, _tile(k)], False)
                    else:
                        assert act[0] == 'S' and all(('h', t[1], T // LP - 1) in did for p_ in _H_GROUPS[r] for t in p_[0])
                        items += h_sums(32 if span else 16, r)
                release(jobs, span, items)
        assert not jobs.side
    assert arrived == set(named) and all((k_, r) in did for k_ in 'KHQ' for r in range(nb))
    assert all((k_, r) in did for k_ in 'CS' for r in range(2)) and 'L' in did
    assert all(('F', r) in did for r in range(SB))

    def mixer_prep(g):
        sl = jnp.minimum(g, NSL - 1)
        rows = pl.ds(pl.multiple_of(sl * MS, MS), MS)

        def part(m, forms):
            def fn(dep):
                base = {}

                def get(i, k):
                    if (i, k) not in base:
                        rb, cb = (i, k) if m == 2 else (k, i)
                        r0 = mixw[m][2] + rb * MS
                        v = _after(st_in[r0:r0 + MS, _tile(cb)].astype(F32), _rows(dep, MS))
                        if m == 3 and (rb + 1) * T > Fd:
                            v = jnp.where(rb * T + sl * MS < Fd, v, 0.0)
                        base[i, k] = v
                    return base[i, k]

                for f in forms:
                    v = _form(f, get)
                    mw_scr[_MIXW[m, f], rows, :] = (0.5 * v if m % 2 else v).astype(BF16)
            return fn

        items = []
        for m in range(4):
            forms = [f for mm_, f in _MIXW if mm_ == m]
            cur, terms = [], set()
            for f in forms:
                new_terms = terms | {t[1:] for t in f}
                if cur and 3 * len(new_terms) + sum(2 * len(x) + 1 for x in cur + [f]) > MWOPS:
                    items.append(part(m, cur))
                    cur, terms = [], set()
                cur.append(f)
                terms |= {t[1:] for t in f}
            items.append(part(m, cur))

        n3 = sum(m == 2 for m, _ in _MIXW)
        first = min(n for (m, _), n in _MIXW.items() if m == 2)
        per = -(-n3 // (nattn - 1 - NSL))

        def turn(j):
            def fn(dep):
                n = jnp.minimum(jnp.maximum(g - NSL, 0) * per + j, n3 - 1)
                w = _tie(_ld(mw_scr, first + n), dep).T
                m3_scr[n] = w
                return pltpu.bitcast(pltpu.bitcast(w, U32)[T // 2 - 8:], F32)
            return fn

        return items + [turn(j) for j in range(per)]

    def stage_wait():
        for cp in pcopies(0):
            cp.wait()
        pltpu.make_async_copy(st_in, st_in, wsem.at[7]).wait()

    def attn_body(g, carry):
        side = _gap_items(work, gap_scr) + _weight_form_items(work, gap_scr, wt_scr, wf_scr, (0, 1, 2))
        bufs = (q_scr, k_scr, v_scr, (pf_scr, vf_scr), wo_buf, acc_scr, flag_scr)
        _attention_step(*bufs, g >> 16, side)

        @pl.when(g + 1 < nattn)
        def _():
            copies = stage_in(g + 1) + [ocopy(g + 1)]
            for cp in copies:
                cp.start()
            bufs = (h_scr, hs_scr, c_ref, cs_scr, wf_scr, q_scr, k_scr, v_scr, (pf_scr, vf_scr))
            side = [(SD0 + int(i * SDS), fn) for i, fn in enumerate(mixer_prep(g))]
            _proj_step(*bufs, scale, gap_scr, side)
            for cp in prep_in(g + 1):
                cp.start()
            stage_wait()
            ocopy(g + 1).wait()

        return carry

    stage_wait()
    for cp in cp_late:
        cp.start()
    jax.lax.fori_loop(0, nattn, attn_body, 0)

    def safe_pair(g, carry):
        copies = pcopies(g) + [ocopy(g)]
        for cp in copies:
            cp.start()
        for cp in copies:
            cp.wait()
        for buf, j0, transpose in ((wk_buf, 0, False), (wv_buf, kc, True), (wq_buf, 2 * kc, False)):
            for (j, hd), w in _pair_tiles(buf, transpose).items():
                w_scr[hd, j0 + j] = w

        def tile(u, carry):
            r, hd = u // 2, u % 2
            rows = pl.ds(pl.multiple_of(r * T, T), T)
            ct = [c_ref[rows, _tile(j)] for j in range(kc)]
            k_scr[u] = sum(_dot(ct[j], _ld(w_scr, hd, j)) for j in range(kc)).astype(BF16)
            v_scr[u] = sum(_dot_nt(_ld(w_scr, hd, kc + j), ct[j]) for j in range(kc)).astype(BF16)
            q = sum(_dot(_ld(h_scr, r, j), _ld(w_scr, hd, 2 * kc + j)) for j in range(km))
            q_scr[u] = (q * scale).astype(BF16)
            return carry

        jax.lax.fori_loop(0, 2 * nb, tile, 0)
        _attention_safe(q_scr, k_scr, v_scr, wo_buf, acc_scr)
        return carry

    @pl.when(jnp.max(flag_scr[...]) > 0)
    def _():
        jax.lax.fori_loop(0, nb, zero, 0)
        jax.lax.fori_loop(0, nattn, safe_pair, 0)

    for cp in cp_late:
        cp.wait()
    mod = _dot(silu_cond(), wmb_ref[...])
    mod_scr[:, 2 * M:4 * M] = mod[:, 0:2 * M]
    mod_scr[:, 4 * M:5 * M] = 1.0 + mod[:, 2 * M:3 * M]
    mod_scr[:, 5 * M:6 * M] = mod[:, 3 * M:4 * M]
    OFF = x_ref.shape[0] - S
    CAR = t_scr.shape[0] - RB

    def p1(r0, l0, n, dep=None):
        ga = mod_scr[:, 2 * M:3 * M]
        if dep is not None:
            ga = jnp.concatenate([_after(ga[:, 0:T], dep), ga[:, T:]], axis=1)
        rows = pl.ds(r0, n)
        x1 = x_ref[rows, :].astype(F32) + _rows(ga, n) * acc_scr[rows, :]
        xh_scr[0, l0:l0 + n, :] = x1
        hb = _ln(x1) * _rows(mod_scr[:, 4 * M:5 * M], n) + _rows(mod_scr[:, 3 * M:4 * M], n)
        xh_scr[1, l0:l0 + n, :] = hb
        return _ln(hb)

    HT = T // 2

    def p1_store(r0, c, dep=None):
        v = p1(r0 + c * PC, OFF + c * PC, PC, dep)
        a1_scr[c * PC:(c + 1) * PC, :] = v
        return jnp.max(v[:, M - T:].reshape(PC // 8, 8, T), axis=0)

    t_scr[RB:RB + CAR - OFF, :] = jnp.zeros((CAR - OFF, M), F32)
    t_scr[RB + CAR - OFF:RB + CAR, :] = _gelu2(_dot(p1(0, 0, OFF).astype(BF16), w1_ref[...]))
    for c in range(RB // PC):
        p1_store(OFF, c)

    def out_copy(i):
        rows = pl.ds(i * T if isinstance(i, int) else pl.multiple_of(i * T, T), T)
        return pltpu.make_async_copy(out_buf.at[rows, :], out_hbm.at[rows, :], osem.at[i])

    def b_body(r, carry):
        gb = _rows(mod_scr[:, 5 * M:6 * M], T)
        r0 = pl.multiple_of(r * RB, RB)
        n0 = pl.multiple_of(jnp.minimum(r0 + RB, S - RB) + OFF, OFF)
        nh = RB // T
        now = [0]
        due = []
        pace = []

        def p1_item(c):
            def fn(dep):
                due.append((now[0] + PD, p1_store(n0, c, dep)))
                due.sort(key=lambda e: e[0])
            return fn

        pace += [(P0 + i * PSTEP, p1_item(i)) for i in range(RB // PC)]

        def mm(lhs, wts, dot=_dot):
            acc = None
            for x, w in zip(lhs, wts):
                if due and due[0][0] <= now[0]:
                    w = _tie(w, due.pop(0)[1])
                v = dot(x, w)
                now[0] += x.shape[0] // HT
                acc = v if acc is None else v + acc
                if pace and pace[0][0] <= now[0]:
                    pace.pop(0)[1](v[0:8, :])
            return acc

        def fast(m, base, finish, hook=None):
            prods = _MIX[m]
            left, acc, done, cache = {}, {}, {}, {}
            for _, _, outs in prods:
                for _, i, h in outs:
                    left[i, h] = left.get((i, h), 0) + 1

            def act(form):
                sign, form = _canon(form)
                if form not in cache:
                    cache[form] = _form(form, lambda k, h: base(k)[h * HT:(h + 1) * HT]).astype(BF16)
                return sign, cache[form]

            for pi, (wf, af, outs) in enumerate(prods):
                w = _ld(m3_scr, _MIXW[m, wf] - _MIX3) if m == 2 else _ld(mw_scr, _MIXW[m, wf])
                if af is None:
                    k = wf[0][2]
                    v = mm([jnp.concatenate([act(((1, k, h),))[1] for h in range(2)], axis=0)], [w])
                    sign, parts = 1, [v[:HT], v[HT:]]
                else:
                    sign, x = act(af)
                    parts = [mm([x], [w])] * len(outs)
                for (s_, i, h), v in zip(outs, parts):
                    s_ = s_ * sign
                    if (i, h) not in acc:
                        acc[i, h] = (s_, v)
                    else:
                        s0, u = acc[i, h]
                        acc[i, h] = (s0, u + v if s0 == s_ else u - v) if s0 > 0 or s_ < 0 else (1, v - u)
                    left[i, h] -= 1
                    if not left[i, h]:
                        s0, done[i, h] = acc.pop((i, h))
                        assert s0 > 0
                        if (i, 1 - h) in done:
                            finish(i, jnp.concatenate([done[i, 0], done[i, 1]], axis=0))
                if hook is not None:
                    hook(pi, act)

        t_scr[0:CAR, :] = t_scr[RB:RB + CAR, :]
        for hf in range(nh):
            def put_t(n, v):
                t = _gelu2(v)
                if hf == nh - 1:
                    t = jnp.concatenate([t[:T - OFF], jnp.where(r < nrb - 1, t[T - OFF:], 0.0)], axis=0)
                t_scr[CAR + hf * T:CAR + (hf + 1) * T, _tile(n)] = t

            fast(0, lambda k: a1_scr[_tile(hf), _tile(k)], put_t)
        cq = M // 4
        shifts = (-1, 1, -2, 2)
        lane = jax.lax.broadcasted_iota(jnp.int32, (T, T), 1)
        y1, z, a3 = [], [], []
        for hf in range(nh):
            base = CAR - OFF + hf * T
            sh = []
            for j in range(km):
                g_lo, g_hi = (j * T) // cq, ((j + 1) * T - 1) // cq
                assert g_hi - g_lo <= 1
                v = t_scr[base + shifts[g_lo]:base + shifts[g_lo] + T, _tile(j)]
                if g_hi != g_lo:
                    v2 = t_scr[base + shifts[g_hi]:base + shifts[g_hi] + T, _tile(j)]
                    v = jnp.where(lane < g_hi * cq - j * T, v, v2)
                else:
                    v = jnp.where(lane < T, v, 0.0)
                sh.append(v)
            hs = {}
            fast(1, lambda k: sh[k], hs.__setitem__)
            hs = jnp.concatenate([hs[n] for n in range(km)], axis=1)
            y1.append(hs + xh_scr[1, _tile(hf), :])
            z.append(xh_scr[0, _tile(hf), :] + gb * y1[hf])
            a3.append({})

            def ln_item(hf, c):
                def item(dep):
                    n = HT // NLN
                    for d in (0, HT):
                        v = y1[hf][d + c * n:d + (c + 1) * n]
                        if dep is not None:
                            v = jnp.concatenate([_after(v[:, :T], _rows(dep, n)), v[:, T:]], axis=1)
                        a3[hf][d + c * n] = _ln(v)
                return item

            ln_item(hf, 0)(None)
            pace += [(now[0] + LN0 + (c - 1) * LNS * (1 + hf), ln_item(hf, c)) for c in range(1, NLN)]
            pace.sort(key=lambda e: e[0])
        xh_scr[:, 0:OFF, :] = xh_scr[:, RB:RB + OFF, :]
        h3 = []
        for hf in range(nh):
            assert len(a3[hf]) == 2 * NLN
            af = jnp.concatenate([a3[hf][key] for key in sorted(a3[hf])], axis=0)
            row = {}
            narrow = []

            def hook(pi, act):
                j, rem = divmod(pi - NAR0, NARS)
                if rem == 0 and 0 <= j < km:
                    full = jnp.concatenate([act(((1, j, h),))[1] for h in range(2)], axis=0)
                    v = mm([w3_ref[:, _tile(j)]], [full], _dot_nt)
                    narrow[:] = [v + narrow[0] if narrow else v]

            def put_h(n, v):
                row[n] = _gelu2(v)
                if GD:
                    due.append((now[0] + GD, jnp.max(row[n].reshape(T // 8, 8, T), axis=0)))
                    due.sort(key=lambda e: e[0])

            fast(2, lambda k: af[:, _tile(k)], put_h, hook)
            fw = w3_ref.shape[0]
            row[Fd // T] = jnp.concatenate([_gelu2(narrow[0]), jnp.zeros((T - fw, T), F32)], axis=0).T
            h3.append(row)
        for hf in range(nh):
            rows = pl.ds(pl.multiple_of(r0 + hf * T, T), T)

            def finish(n, v):
                out_buf[rows, _tile(n)] = (z[hf][:, _tile(n)] + gb[:, _tile(n)] * v).astype(out_buf.dtype)

            fast(3, lambda k: h3[hf][k], finish)
            out_copy(r * nh + hf).start()
        assert not pace
        return carry

    jax.lax.fori_loop(0, nrb, b_body, 0)
    for i in range(nb):
        out_copy(i).wait()


@jax.jit
def pallas_adaLN_cond__compressed_kv_cla__mixer_s_mlp__prompt_kernel(
    A_x: jax.Array,
    A_c_kv: jax.Array,
    A_w_q: jax.Array,
    A_w_uk: jax.Array,
    A_w_uv: jax.Array,
    A_w_o: jax.Array,
    B_x: jax.Array,
    B_w1: jax.Array,
    B_w2: jax.Array,
    B_w3: jax.Array,
    B_w4: jax.Array,
    c: jax.Array,
    w_mod: jax.Array,
):
    _, S, M = A_x.shape
    Dc = A_c_kv.shape[2]
    H, D = A_w_q.shape[1], A_w_q.shape[2]
    Fd = B_w3.shape[1]
    assert D == T and A_c_kv.shape[1] == S and Dc == 4 * T and M == 5 * T and 13 * T < Fd < 14 * T and S == 16 * T
    vmem = pltpu.VMEM
    packed = lambda *lead: vmem(lead + (T, T), BF16)
    out = pl.pallas_call(
        _kernel,
        in_specs=[pl.BlockSpec(memory_space=pltpu.HBM)] * 12,
        out_specs=pl.BlockSpec(memory_space=pltpu.HBM),
        out_shape=jax.ShapeDtypeStruct((S, M), A_x.dtype),
        scratch_shapes=[
            vmem((S + 16, M), BF16),
            vmem((S, Dc), BF16),
            vmem((1, M), BF16),
            vmem((M, 2 * M), BF16),
            vmem((M, 4 * M), BF16),
            vmem((M, M), BF16),
            vmem((Fd % T, M), BF16),
            vmem((M, D), U32),
            vmem((Dc, D), U32),
            vmem((Dc, D), U32),
            vmem((2 * D, M), BF16),
            vmem((S, M), A_x.dtype),
            pltpu.SemaphoreType.DMA((15,)),
            pltpu.SemaphoreType.DMA((8,)),
            pltpu.SemaphoreType.DMA((S // T,)),
            vmem((8, 6 * M), F32),
            vmem((S // T, M // T, T, T), BF16),
            vmem((len(_C_SUMS), T, T), BF16),
            vmem((len(_H_SUMS), T, T), BF16),
            packed(2, M // T + 2 * (Dc // T)),
            packed(2 * S // T),
            packed(2 * S // T),
            packed(2 * S // T),
            vmem((S + 16, M), F32),
            vmem((S, M), F32),
            vmem((2, RB + 16, M), F32),
            vmem((RB, M), F32),
            vmem((RB + 32, M), F32),
            packed(len(_MIXW)),
            packed(sum(m == 2 for m, _ in _MIXW)),
            vmem((Dc // T, T, T), U32),
            vmem((len(_WF), T, T), BF16),
            vmem((3, 8, T), jnp.int32),
            vmem(((2 * (M // T) + Fd // T + -(-Fd // T)) * 16, M), BF16),
            vmem((_FENCE + 1, T, T), BF16),
            vmem((_FENCE + 1, T, T), BF16),
            vmem((8, T), F32),
        ],
        compiler_params=pltpu.CompilerParams(
            vmem_limit_bytes=100 * 1024 * 1024,
            disable_bounds_checks=True,
        ),
    )(
        A_x.reshape(S, M), A_c_kv.reshape(S, Dc),
        A_w_q, A_w_uk, A_w_uv,
        A_w_o.reshape(H // 2, 2 * D, M),
        B_w1, B_w2, B_w3.T, B_w4, c, w_mod,
    )
    return out.reshape(1, S, M)
```

```python
import functools
import math

import jax
import jax.numpy as jnp
import jax.experimental.pallas as pl
import jax.experimental.pallas.tpu as pltpu

F32 = jnp.float32
BF16 = jnp.bfloat16
U32 = jnp.uint32
NT = (((1,), (1,)), ((), ()))
T = 128
EPS = 1e-5
LOG2E = math.log2(math.e)

GRP = 4
LEAD = 10
PROW = 3
RES = 32
LAT_0 = 32
LAT_A = 16
LAT_B = 20
ALEAD = 32
QT = (4, 6)
ONV, OEND = 0.5, 24
FPOS, DPOS = 0, 0
SIDE0, SIDE1, SLAG, SDUE = 8, 60, 4, 8
SKIND = 'pvo'
HACKWO = 0
SG0, SG1 = 6, 4
SD0, SDS = 4, 1.5
WFN = (4, 4, 6)
VF0, VFS = 4, 1.7
L_LO, L_HI, L_RATIO = 2.0 ** -24, 2.0 ** 24, 4.0
RB = 256
PC = 32
P0, PSTEP, PD = 390, 27, 56
GD, NAR0, NARS = 36, 4, 8
MSUB = (1, 1, 1, 1)
PDUE = 20
MWOPS = 70
NLN, LN0, LNS = 4, 4, 5
LP = 16
SP0, SP1 = 76, 38
_prologue = lambda: ('|kva|Z; |b|; kva|wc|K0123; bw|xdn|C0@56 N0123@52 K4567; cx|mq|N4567@52 F0@56 K89ab; '
            'd|y|C1@56 F1@56 Kcdef; nmq|zo|M H01 H234567@30 F2@36 Q0123; y||H89ab@30 F3@36 Q4567; '
            'zo||L Hcdef@30 S0@%d Q89ab S1@%d Qcdef' % (SP0, SP1))


def _dot(a, b):
    return jnp.dot(a, b, preferred_element_type=F32)


def _dot_nt(a, b):
    return jax.lax.dot_general(a, b, NT, preferred_element_type=F32)


def _ln(x):
    m = jnp.mean(x, axis=-1, keepdims=True)
    xc = x - m
    v = jnp.mean(xc * xc, axis=-1, keepdims=True)
    return xc * jnp.exp2(jnp.log(v + EPS) * (-0.5 * LOG2E))


def _rows(v, n):
    return jnp.broadcast_to(v[None], (n // 8, 8, v.shape[1])).reshape(n, v.shape[1])


def _gelu2(x):
    c0 = math.sqrt(2.0 / math.pi)
    return x + x * jnp.tanh(x * (c0 + (c0 * 0.044715) * (x * x)))


def _after(x, dep):
    return jnp.where(dep > jnp.inf, dep, x)


def _tie(x, dep):
    xu = pltpu.bitcast(x, U32)
    first = jnp.where(dep > jnp.inf, jnp.uint32(0), xu[:8])
    return pltpu.bitcast(jnp.concatenate([first, xu[8:]], axis=0), BF16)


def _tile(j):
    return slice(j * T, (j + 1) * T)


def _ld(ref, *idx):
    return pltpu.bitcast(ref.bitcast(U32)[idx], BF16)


def _a_ops(a11, a12, a21, a22):
    return [a11 + a22, a21 + a22, a11, a22, a11 + a12, a21 - a11, a12 - a22]


def _b_ops(b11, b12, b21, b22):
    return [b11 + b22, b11, b12 - b22, b21 - b11, b22, b11 + b12, b21 + b22]


def _strassen(prod, col1=None, col2=None):
    m4 = prod(3)
    m2 = prod(1)
    c21 = m2 + m4
    if col1 is not None:
        e11, e21 = col1()
        m4, c21 = m4 + e11, c21 + e21
    m3 = prod(2)
    m5 = prod(4)
    c12 = m3 + m5
    if col2 is not None:
        e12, e22 = col2()
        c12, m3 = c12 + e12, m3 + e22
    m1 = prod(0)
    c11 = prod(6) + (m1 + (m4 - m5))
    c22 = prod(5) + (m1 + (m3 - m2))
    return c11, c12, c21, c22


def _group(rows, cols, pairs):
    xs, ys = dict.fromkeys(x for x, _ in pairs), dict.fromkeys(y for _, y in pairs)
    used = set(xs) | set(ys) | {(x[0], y[1]) for x, y in pairs} | {(y[0], x[1]) for x, y in pairs}
    prods = []
    for n, r in enumerate(rows):
        for i, k in [x for x in xs if x[0] == r]:
            mates = [y for x, y in pairs if x == (i, k)]
            prods.append((((1, i, k),) + tuple((1, i, k2) for _, k2 in mates), ((1, k, 0),),
                          ((1, i, 0), (-1, i, 1))))
            prods.append((((1, i, k),) + tuple((-1, i2, k) for i2, _ in mates), ((1, k, 0), (1, k, 1)),
                          ((1, i, 1),)))
        for i2, k2 in [y for y in ys if y[0] == r]:
            mates = [x for x, y in pairs if y == (i2, k2)]
            prods.append((((1, i2, k2),) + tuple((1, i2, k) for _, k in mates), ((1, k2, 1),),
                          ((1, i2, 1), (-1, i2, 0))))
            prods.append((((1, i2, k2),) + tuple((-1, i, k2) for i, _ in mates), ((1, k2, 0), (1, k2, 1)),
                          ((1, i2, 0),)))
        prods += [(((1, r, k),), ((1, k, h),), ((1, r, h),)) for k in cols if (r, k) not in used for h in (0, 1)]
        for (i, k), (i2, k2) in pairs:
            if r in (i, i2) and i + i2 - r in rows[n + 1:]:
                prods.append((((1, i, k2),), ((1, k2, 0), (-1, k, 0)), ((1, i2, 0), (1, i, 0))))
                prods.append((((1, i2, k), (1, i, k2)), ((1, k, 0), (1, k2, 1)), ((1, i2, 0), (1, i, 1))))
                prods.append((((1, i2, k),), ((1, k, 1), (-1, k2, 1)), ((1, i2, 1), (1, i, 1))))
    return prods


def _all_pairs(xrows, yrows):
    return [((x, a), (y, b)) for a, x in enumerate(xrows) for b, y in enumerate(yrows) if a != b]


_PAIRS65 = [((x[0] + 10, x[1]), (y[0] + 10, y[1])) for x, y in (
    ((0, 1), (1, 0)), ((0, 1), (5, 2)), ((2, 3), (1, 0)), ((2, 3), (3, 1)), ((2, 3), (5, 2)), ((3, 2), (1, 0)),
    ((4, 4), (0, 3)), ((4, 4), (1, 0)), ((4, 4), (3, 1)), ((4, 4), (5, 2)))]
_C_GROUPS = [_group(range(r, r + 8), range(4), _all_pairs(range(r, r + 4), range(r + 4, r + 8))) for r in (0, 8)]
_H_GROUPS = [_group(range(10), range(5), _all_pairs(range(5), range(5, 10))),
             _group(range(10, 16), range(5), _PAIRS65)]
_sum_index = lambda groups: {f: n for n, f in enumerate(
    dict.fromkeys(t[0] for g in groups for t in g if len(t[0]) > 1))}
_C_SUMS, _H_SUMS = _sum_index(_C_GROUPS), _sum_index(_H_GROUPS)


def _cells(rows, cols, pairs):
    xs = list(dict.fromkeys(p[0] for p in pairs))
    ys = list(dict.fromkeys(p[1] for p in pairs))
    used = set(xs + ys) | {(x[0], y[1]) for x, y in pairs} | {(y[0], x[1]) for x, y in pairs}

    def home_x(i, k):
        mates = [y for x, y in pairs if x == (i, k)]
        return [(((1, i, k),) + tuple((1, i, k2) for _, k2 in mates), ((1, k, 0),), ((1, i, 0), (-1, i, 1))),
                (((1, i, k),) + tuple((-1, i2, k) for i2, _ in mates), ((1, k, 0), (1, k, 1)), ((1, i, 1),))]

    def home_y(i2, k2):
        mates = [x for x, y in pairs if y == (i2, k2)]
        return [(((1, i2, k2),) + tuple((1, i2, k) for _, k in mates), ((1, k2, 1),), ((1, i2, 1), (-1, i2, 0))),
                (((1, i2, k2),) + tuple((-1, i, k2) for i, _ in mates), ((1, k2, 0), (1, k2, 1)), ((1, i2, 0),))]

    def cross(x, y):
        (i, k), (i2, k2) = x, y
        return [(((1, i, k2),), ((1, k2, 0), (-1, k, 0)), ((1, i2, 0), (1, i, 0))),
                (((1, i2, k), (1, i, k2)), ((1, k, 0), (1, k2, 1)), ((1, i2, 0), (1, i, 1))),
                (((1, i2, k),), ((1, k, 1), (-1, k2, 1)), ((1, i2, 1), (1, i, 1)))]

    direct = lambda i: [(((1, i, k),), None, ((1, i, 0), (1, i, 1))) for k in cols if (i, k) not in used]
    single = lambda i: ([t for x in xs if x[0] == i for t in home_x(*x)]
                        + [t for y in ys if y[0] == i for t in home_y(*y)] + direct(i))
    prods = []
    for n, i in enumerate(rows):
        prods += single(i)
        for i2 in rows[n + 1:]:
            for x, y in pairs:
                if {x[0], y[0]} == {i, i2}:
                    prods += cross(x, y)
    return prods


_square = lambda q: [((a, a), (q + b, b)) for a in range(q) for b in range(q) if a != b]
_shift = lambda pairs, r0: [((x[0] + r0, x[1]), (y[0] + r0, y[1])) for x, y in pairs]
_flip = lambda pairs: [(x[::-1], y[::-1]) for x, y in pairs]
_P35 = [((1, 2), (0, 4)), ((1, 2), (2, 1)), ((2, 3), (0, 4)), ((2, 3), (1, 0))]
_P45 = [((0, 2), (1, 1)), ((2, 4), (0, 3)), ((2, 4), (1, 1)), ((2, 4), (3, 2)), ((3, 0), (0, 3)), ((3, 0), (1, 1))]
_P55 = [((2, 1), (0, 4)), ((2, 1), (1, 0)), ((2, 1), (3, 2)), ((2, 1), (4, 3)), ((3, 3), (0, 4)), ((3, 3), (1, 0)),
        ((4, 2), (0, 4)), ((4, 2), (1, 0))]
_MIX = [_cells(range(5), range(5), _P55), _cells(range(5), range(5), _P55),
        _cells(range(13), range(5), _square(5) + _shift(_P35, 10)),
        _cells(range(5), range(14), _flip(_square(5) + _shift(_P45, 10)))]
_MIXW = {(m, f): n for n, (m, f) in enumerate(dict.fromkeys((m, t[0]) for m in range(4) for t in _MIX[m]))}
_MIX3 = min(n for (m, _), n in _MIXW.items() if m == 2)


def _form(form, get):
    acc = None
    for sign, i, j in form:
        v = get(i, j)
        acc = v if acc is None else (acc + v if sign > 0 else acc - v)
    return acc


def _gap_items(bufs, gap_scr):
    items = []
    for n, buf in enumerate(bufs):
        acc = []

        def part(r0, buf=buf, acc=acc):
            def fn(dep):
                wu = jnp.concatenate([buf[r:r + 8, :] for r in range(r0, r0 + T, 32)])
                mask = jnp.full((8, T), 0x7FFF0000, U32)
                if dep is not None:
                    mask = jnp.where(dep > jnp.inf, jnp.uint32(0), mask)
                mask = _rows(mask, 32)
                new = [jnp.sum(pltpu.bitcast(v & mask, F32).reshape(4, 8, T), axis=0) for v in (wu << 16, wu)]
                acc[:] = [u + v for u, v in zip(acc, new)] if acc else new
            return fn

        def last(_, n=n, acc=acc):
            bits = []
            for v in acc:
                l1 = jnp.sum(jnp.sum(v, axis=1, keepdims=True), axis=0, keepdims=True)
                bits.append(pltpu.bitcast(jnp.broadcast_to(l1, (8, T)), jnp.int32) >> 8)
            gap = jnp.clip((bits[0] - bits[1] + (1 << 14)) >> 15, -8, 8) << 23
            gap_scr[n] = gap
            return pltpu.bitcast(gap, F32)

        items += [part(r0) for r0 in range(0, buf.shape[0], T)] + [last]
    return items


def _pair_tiles(w_ref, transpose=False):
    tiles = {}
    for j in range(w_ref.shape[0] // T):
        wu = w_ref[_tile(j), :]
        if transpose:
            wu = wu.T
        tiles[j, 0] = pltpu.bitcast(wu << 16, F32).astype(BF16)
        tiles[j, 1] = pltpu.bitcast(wu & jnp.uint32(0xFFFF0000), F32).astype(BF16)
    return tiles


def _canon(form):
    if form[-1][0] < 0 and form[0][1:] > form[1][1:]:
        return -1, ((1,) + form[1][1:], (-1,) + form[0][1:])
    return 1, form


_w_forms = lambda groups: list(dict.fromkeys(_canon(t[1])[1] for g in groups for t in g))
_WF = {key: n for n, key in enumerate([(m, f) for m, groups in enumerate((_C_GROUPS, _C_GROUPS, _H_GROUPS))
                                       for f in _w_forms(groups)])}


def _weight_form_items(bufs, gap_scr, wt_scr, wf_scr, which):
    n = 16
    items = []

    def flip(j):
        def fn(dep):
            wu = bufs[1][_tile(j), :]
            wu = (wu if dep is None else jnp.where(_rows(dep, T) > jnp.inf, jnp.uint32(0), wu)).T
            wt_scr[j] = wu
            return pltpu.bitcast(wu[T - 8:], F32)
        return fn

    def part(m, r0, forms):
        def fn(dep):
            fac = pltpu.bitcast(0x3F800000 + gap_scr[m], F32)
            mask = jnp.full((8, T), 0xFFFF0000, U32)
            sh = jnp.full((8, T), 16, U32)
            if dep is not None:
                mask = jnp.where(dep > jnp.inf, jnp.uint32(0), mask)
                sh = jnp.where(dep > jnp.inf, jnp.uint32(0), sh)
            fac, mask, sh = _rows(fac, n), _rows(mask, n), _rows(sh, n)
            base = {}

            def get(k, h):
                if (k, h) not in base:
                    wu = wt_scr[k, r0:r0 + n, :] if m == 1 else bufs[m][k * T + r0:k * T + r0 + n, :]
                    base[k, h] = pltpu.bitcast(wu & mask, F32) * fac if h else pltpu.bitcast(wu << sh, F32)
                return base[k, h]

            for f in forms:
                wf_scr[_WF[m, f], r0:r0 + n, :] = _form(f, get).astype(BF16)
        return fn

    for m in which:
        forms = [f for mm, f in _WF if mm == m]
        if m == 1:
            items += [flip(j) for j in range(bufs[1].shape[0] // T)]
        per = -(-len(forms) // WFN[m])
        forms.sort(key=lambda f: sorted({t[1] for t in f}))
        items += [part(m, r0, forms[i:i + per]) for r0 in range(0, T, n) for i in range(0, len(forms), per)]
    return items


def _run_group(jobs, prods, a_get, w, transposed, finish):
    left = {}
    for _, _, outs in prods:
        for _, i, h in outs:
            left[i, h] = left.get((i, h), 0) + 1
    acc = {}
    for af, bf, outs in prods:
        sign, wt = w(bf)
        m = jobs.mm([wt], [a_get(af)], _dot_nt) if transposed else jobs.mm([a_get(af)], [wt], _dot)
        for s_, i, h in outs:
            if (i, h) not in acc:
                acc[i, h] = (s_ * sign, m)
            else:
                s0, v = acc[i, h]
                acc[i, h] = (s0, v + m if s0 == s_ * sign else v - m) if s0 > 0 or s_ * sign < 0 else (1, m - v)
            left[i, h] -= 1
            if not left[i, h]:
                s0, v = acc.pop((i, h))
                assert s0 > 0
                finish(2 * i + h, v)


class _Jobs:
    def __init__(self, side=()):
        self.res = []
        self.side = list(side)
        self.due = []

    def mm(self, lhs, wt, dot):
        acc = None
        for x, w in zip(lhs, wt):
            if self.due and self.due[0][0] <= len(self.res):
                x = _tie(x, self.due.pop(0)[1])
            v = dot(x, w)
            self.res.append(v)
            acc = v if acc is None else v + acc
            rel = 4 * (len(self.res) % 4)
            while self.side and self.side[0][0] <= len(self.res):
                out = self.side.pop(0)[1](v[8 * rel:8 * rel + 8, :])
                if out is not None:
                    self.due.append((len(self.res) + PDUE, out))
                rel = (rel + 2) % 16
        return acc


def _proj_step(h_scr, hs_scr, c_ref, cs_scr, wf_scr, q_scr, k_scr, v_scr, pf, scale, shifts, side):
    def weight(m):
        def get(form):
            sign, form = _canon(form)
            return sign, _ld(wf_scr, _WF[m, form])
        get.inv = pltpu.bitcast(0x3F800000 - shifts[m], F32)
        return get

    wk, wvT, wq = weight(0), weight(1), weight(2)
    c_get = lambda f: _ld(cs_scr, _C_SUMS[f]) if len(f) > 1 else c_ref[_tile(f[0][1]), _tile(f[0][2])]
    h_get = lambda f: _ld(hs_scr, _H_SUMS[f]) if len(f) > 1 else _ld(h_scr, f[0][1], f[0][2])

    def put(dst, w, mul=None):
        muls = [mul, _rows(w.inv if mul is None else w.inv * mul, T)]

        def fn(u, v):
            v = (v if muls[u % 2] is None else v * muls[u % 2]).astype(BF16)
            dst[u] = v.T if mul is not None and u in QT else v
        return fn

    jobs = _Jobs(side)
    put_v, stored = put(v_scr, wvT), set()
    nxt = [0]

    def fin_v(u, v):
        put_v(u, v)
        stored.add(u)
        for J in range(SB):
            if all(2 * (SB * J + k) + h in stored for k in range(SB) for h in range(2)) and ('J', J) not in stored:
                stored.add(('J', J))
                for fn in _v_form_items(v_scr, pf, J):
                    nxt[0] = max(nxt[0] + VFS, len(jobs.res) + VF0)
                    jobs.side.append((int(nxt[0]), fn))
                jobs.side.sort(key=lambda e: e[0])

    kk, vv, qq = ((c_get, wk, False, put(k_scr, wk)), (c_get, wvT, True, fin_v),
                  (h_get, wq, False, put(q_scr, wq, scale)))
    for prods, args in ((_C_GROUPS[0], kk), (_C_GROUPS[0], vv), (_C_GROUPS[1], vv), (_C_GROUPS[1], kk),
                        (_H_GROUPS[0], qq), (_H_GROUPS[1], qq)):
        _run_group(jobs, prods, *args)
    assert not jobs.side and not jobs.due


def _inner_group(rows, cols, pairs):
    xs, ys = dict.fromkeys(x for x, _ in pairs), dict.fromkeys(y for _, y in pairs)
    used = set(xs) | set(ys) | {(x[0], y[1]) for x, y in pairs} | {(y[0], x[1]) for x, y in pairs}
    prods = []
    for i, j in xs:
        mates = [y for x, y in pairs if x == (i, j)]
        prods.append((((1, i, 0),), ((1, 0, j), (-1, 1, j)), ((1, i, j),) + tuple((1, i2, j) for i2, _ in mates)))
        prods.append((((1, i, 0), (1, i, 1)), ((1, 1, j),), ((1, i, j),) + tuple((-1, i, j2) for _, j2 in mates)))
    for i2, j2 in ys:
        mates = [x for x, y in pairs if y == (i2, j2)]
        prods.append((((1, i2, 0), (1, i2, 1)), ((1, 0, j2),),
                      ((1, i2, j2),) + tuple((-1, i2, j) for _, j in mates)))
        prods.append((((1, i2, 1),), ((1, 0, j2), (-1, 1, j2)),
                      ((-1, i2, j2),) + tuple((-1, i, j2) for i, _ in mates)))
    prods += [(((1, i, h),), ((1, h, j),), ((1, i, j),))
              for i in rows for j in cols if (i, j) not in used for h in (0, 1)]
    for (i, j), (i2, j2) in pairs:
        lo, hi = min(j, j2), max(j, j2)
        prods.append((((1, i2, 0), (-1, i, 0)), ((1, 0, lo), (1, 0, hi)), ((1, i2, j),)))
        prods.append((((1, i, 0), (1, i2, 1)), ((1, 0, j2), (1, 1, j)), ((1, i, j2), (1, i2, j))))
        prods.append((((1, i, 1), (-1, i2, 1)), ((1, 1, lo), (1, 1, hi)), ((1, i, j2),)))
    return prods


def _o_jobs():
    prods = (_inner_group(range(10), range(5), _all_pairs(range(0, 10, 2), range(1, 10, 2)))
             + _inner_group(range(10, 16), range(5), _PAIRS65))
    row = lambda t: max(i for _, i, _ in t[0])
    unit = lambda t: max(2 * i + h for _, i, h in t[0])
    need = lambda t: unit(t) if row(t) == 15 else 2 * row(t) + 1
    return [(need(t), t) for t in sorted(prods, key=need)]


_O_JOBS = _o_jobs()


SB = 4


class _Star:
    def __init__(self, ts):
        self.ts, self.n = ts, len(ts)
        rn = range(self.n)
        self.pairs = [(i, j) for i in rn for j in rn if i < j]
        self.pf = {f: m for m, f in enumerate([('R', i) for i in rn] + [('C', i) for i in rn]
                                              + [('S', i, j) for i in rn for j in rn if i != j]
                                              + [('A', i, j) for i, j in self.pairs])}
        self.vf = {f: m for m, f in enumerate([('W', i) for i in rn]
                                              + [(q, i, j) for i, j in self.pairs for q in ('Q1', 'Q2', 'Q3')])}
        self.pv = {**{('W', i): ('R', i) for i in rn}, **{('B', i): ('C', i) for i in rn},
                   **{('Q1', i, j): ('S', i, j) for i, j in self.pairs},
                   **{('Q2', i, j): ('A', i, j) for i, j in self.pairs},
                   **{('Q3', i, j): ('S', j, i) for i, j in self.pairs}}

    def products(self, i):
        return [('W', i), ('B', i)] + [(q, i, j) for j in range(i + 1, self.n) for q in ('Q1', 'Q2', 'Q3')]


_FULL = _Star((-1.125, -0.375, 0.375, 1.125))
_HALF = _Star((-0.75, 0.75))
_DCELLS = [(0, 0), (1, 0), (1, 1), (2, 2), (3, 2), (3, 3)]
_HSLOT = (SB - 1) * len(_FULL.pf)
_DSLOT = _HSLOT + len(_HALF.pf)
_VSLOT = _DSLOT + len(_DCELLS)
_VHALF = (SB - 1) * len(_FULL.vf)
_FENCE = _VSLOT + (_VHALF + SB * len(_HALF.vf) + 1) // 2


def _v_slot(star, J, f):
    m = star.vf[f] + J * len(star.vf) + (0 if star is _FULL else _VHALF)
    return _VSLOT + m // 2, m % 2 * (T // 2)


def _v_form_items(v_scr, pf, J):
    n, HT = 16, T // 2

    def item(star, h, r0, pairs):
        def fn(dep):
            ts = [jnp.full((8, T), t, F32) for t in star.ts]
            ts = [_rows(t if dep is None else _after(t, dep), n) for t in ts]

            def get(k, a):
                r = (a * HT + r0) // 2
                return _ld(v_scr, 2 * (SB * J + k) + h, slice(r, r + n // 2)).astype(F32)

            def put(f, v):
                slot, r = _v_slot(star, J, f)
                pf[h][slot, r + r0:r + r0 + n, :] = v.astype(BF16)

            b = {(k, a): get(k, a) for k in sorted({k for pr in pairs or star.pairs for k in pr})
                 for a in range(2)}
            if pairs is None or star.n == 2:
                w = [b[k, 0] + ts[k] * b[k, 1] for k in range(star.n)]
                for k in range(star.n):
                    put(('W', k), w[k])
                for i, j in star.pairs:
                    put(('Q2', i, j), w[i] - w[j])
            for i, j in pairs or ():
                d0, d1 = b[j, 0] - b[i, 0], b[j, 1] - b[i, 1]
                put(('Q1', i, j), d0 + ts[i] * d1)
                put(('Q3', i, j), d0 + ts[j] * d1)
        return fn

    pr = _FULL.pairs
    parts = [(_HALF, _HALF.pairs)]
    if J < SB - 1:
        parts += [(_FULL, x) for x in (None, pr[:2], [pr[2], pr[4]], [pr[3], pr[5]])]
    return [item(star, h, r0, pairs) for h in range(2) for r0 in range(0, HT, n) for star, pairs in parts]


def _job_order(nsb):
    units = [(I, h) for I in range(nsb) for h in range(2)]
    qe, qv = [], []
    for I, h in units:
        es = [('e', I, h, J, p) for J in range(I) for p in range(SB)]
        ds = [('d', I, h) + c for c in _DCELLS]
        es.insert(max(len(es) - FPOS, 0), ('f', I, h))
        qe += es + ds if I or FPOS < 9 else ds[:DPOS] + es + ds[DPOS:]
        for i in range(SB):
            qv += [('p', I, h, f, J) for f in _FULL.products(i) for J in range(I)]
            if i >= 2:
                qv += [('p', I, h, f, None) for f in _HALF.products(i - 2)]
            qv += [('v', I, h) + c for c in _DCELLS if c[0] == i]
    qo = [('o', u, j) for j, (u, _) in enumerate(_O_JOBS)]
    cost = dict(e=8, f=8, d=2, p=1, v=2, o=2)
    order, done = [], {}
    now = [0]

    def emit(q):
        job = q.pop(0)
        order.append(job)
        now[0] += cost[job[0]]
        if job[0] == 'd':
            done[job] = now[0]
        elif job[0] == 'v' and job[4] == job[3]:
            done['u', 2 * (SB * job[1] + job[3]) + job[2]] = now[0]
        return cost[job[0]]

    def v_ready():
        if not qv:
            return False
        key = ('d', qv[0][1], qv[0][2], SB - 1, SB - 1)
        return key in done and done[key] + (LAT_0 if qv[0][1:3] == (0, 0) else LAT_A) <= now[0]

    def o_ready():
        return bool(qo) and ('u', qo[0][1]) in done and done['u', qo[0][1]] + LAT_B <= now[0]

    def fill(nv, no):
        n = 0
        while nv > 0 or no > 0 or n % 4:
            if no > 0 and n % 2 == 0 and o_ready() and no * ONV >= nv:
                no -= 2
                n += emit(qo)
            elif v_ready() and (nv > 0 or n % 4):
                c = emit(qv)
                nv -= c
                n += c
            elif o_ready() and n % 2 == 0 and (no > 0 or n % 4 or nv > 0) and len(qo) > RES:
                no -= 2
                n += emit(qo)
            else:
                break

    while qe:
        unit = qe[0][1:3]
        while qv and qv[0][2] == unit[1] and qv[0][1] < unit[0]:
            emit(qv)
        ne = 0
        while qe and ne < 8 and (ne == 0 or (qe[0][0] == 'd' and qe[0][1:3] == unit and ne + 2 <= 8)):
            ne += emit(qe)
        groups = lambda q: sum(cost[j[0]] for j in q) / 8
        old = [j for j in qv if j[1:3] != unit and ('d', j[1], j[2], SB - 1, SB - 1) in done]
        here = [j for j in qe if j[1:3] == unit]
        rest = sum(cost[j[0]] for j in old)
        nv = (rest - LAT_A) / (groups(here) + 1) if here else rest
        no = 2 * max(len(qo) - RES - OEND, 0) / (groups(qe) + 1)
        fill(int(nv + 0.5), int(no + 0.5))
    while qv or qo:
        if qv and v_ready():
            fill(6, 2)
            if not qv:
                continue
        elif o_ready():
            emit(qo)
        else:
            emit(qv or qo)
    return order


def _attention_safe(q_scr, k_scr, v_scr, wo_ref, acc_scr):
    causal = (jax.lax.broadcasted_iota(jnp.int32, (T, T), 0)
              <= jax.lax.broadcasted_iota(jnp.int32, (T, T), 1))

    def unit(u, carry):
        r, hd = u // 2, u % 2

        def block(c, mlo):
            m0, l, o = mlo
            s = _dot_nt(_ld(k_scr, 2 * c + hd), _ld(q_scr, u))
            s = jnp.where(jnp.logical_or(causal, c < r), s, -1e9 * LOG2E)
            m = jnp.maximum(m0, jnp.max(s, axis=0, keepdims=True))
            a = jnp.exp2(m0 - m)
            p = jnp.exp2(s - m)
            return (m, l * a + jnp.sum(p, axis=0, keepdims=True),
                    o * a + _dot(_ld(v_scr, 2 * c + hd), p.astype(BF16)))

        _, l, o = jax.lax.fori_loop(0, r + 1, block, (jnp.full((1, T), -jnp.inf, F32), jnp.zeros((1, T), F32),
                                                      jnp.zeros((T, T), F32)))
        rows = pl.ds(pl.multiple_of(r * T, T), T)
        acc_scr[rows, :] += _dot((o * (1.0 / l)).astype(BF16).T, wo_ref[pl.ds(pl.multiple_of(hd * T, T), T), :])
        return carry

    jax.lax.fori_loop(0, q_scr.shape[0], unit, 0)


def _attention_step(q_scr, k_scr, v_scr, pf, wo_ref, acc_scr, flag_scr, z, side):
    causal = (jax.lax.broadcasted_iota(jnp.int32, (T, T), 0)
              <= jax.lax.broadcasted_iota(jnp.int32, (T, T), 1))
    HT = T // 2
    lsum, lrow, acc, fg, dacc, of, lhs = {}, {}, {}, {}, {}, {}, {}
    res = []
    wo, terms = {}, {}
    left = {}
    done_side = [0, 0]
    chk = [jnp.zeros((8, T), F32), None]
    for _, t in _O_JOBS:
        for _, i, j in t[2]:
            left[i, j] = left.get((i, j), 0) + 1

    def add_l(u, v):
        lsum[u] = v if u not in lsum else lsum[u] + v

    csign = {}

    def p_forms(star, h, slot0, g, tiles, cell, when):
        n = star.n

        def put(f, v):
            pf[h][slot0 + star.pf[f], 16 * g:16 * g + 16, :] = v.astype(BF16)

        for i in range(n):
            row = [cell(i, k) for k in sorted(range(n), key=lambda k: when(i, k))]
            r = functools.reduce(lambda x, y: x + y, row)
            put(('R', i), r)
            add_l(tiles[i], r[:8] + r[8:])
            col = sorted(range(n), key=lambda i2: (when(i2, i), i2 != i))
            sign = csign[n, i] = 1 if col[0] == i else -1
            c = cell(col[0], i)
            for i2 in col[1:]:
                c = c + cell(i2, i) if (1 if i2 == i else -1) == sign else c - cell(i2, i)
            put(('C', i), c)
            for j in range(n):
                if j != i:
                    put(('S', i, j), cell(i, j))
        for i, j in star.pairs:
            put(('A', i, j), cell(i, j) + cell(j, i))

    due = []

    def scores(x, u):
        if due and due[0][0] <= done_side[1]:
            x = _tie(x, due.pop(0)[1])
        s = (_dot if u in QT else _dot_nt)(x, _ld(q_scr, u))
        res.append(s)
        return s

    def job_e(I, h, J, p):
        tiles = [2 * (SB * I + i) + h for i in range(SB)]
        ps = []
        for i, u in enumerate(tiles):
            x = jnp.concatenate([k_scr.bitcast(U32)[2 * (SB * J + (t - i) % SB) + h, 8 * g:8 * g + 8, :]
                                 for g in (2 * p, 2 * p + 1) for t in range(SB)], axis=0)
            ps.append(jnp.exp2(scores(pltpu.bitcast(x, BF16), u)))
        when = lambda i, k: (i + k) % SB
        for n, g in enumerate((2 * p, 2 * p + 1)):
            cell = lambda i, k: ps[i][16 * (SB * n + when(i, k)):16 * (SB * n + when(i, k)) + 16]
            p_forms(_FULL, h, J * len(_FULL.pf), g, tiles, cell, when)

    def job_f(I, h):
        tiles = [2 * (SB * I + 2 + i) + h for i in range(2)]
        ps = {(i, k): jnp.exp2(scores(_ld(k_scr, 2 * (SB * I + k) + h), u))
              for i, u in enumerate(tiles) for k in range(2)}
        for g in range(T // 16):
            p_forms(_HALF, h, _HSLOT, g, tiles, lambda i, k: ps[i, k][16 * g:16 * g + 16], lambda i, k: 0)

    def job_d(I, h, i, k):
        u = 2 * (SB * I + i) + h
        s = scores(_ld(k_scr, 2 * (SB * I + k) + h), u)
        if i == k:
            s = jnp.where(causal, s, -1e9 * LOG2E)
        p = jnp.exp2(s)
        add_l(u, jnp.sum(p.reshape(T // 8, 8, T), axis=0))
        pf[h][_DSLOT + _DCELLS.index((i, k))] = p.astype(BF16)
        if (i, k) == _DCELLS[-1]:
            pf[h][_FENCE + z, 0:16, :] = jnp.zeros((16, T), BF16)
            for u in [2 * (SB * I + a) + h for a in range(SB)]:
                lrow[u] = jnp.sum(lsum.pop(u), axis=0, keepdims=True)
            ls = [lrow[2 * (SB * I + a) + h] for a in range(SB)]
            lo = jnp.minimum(jnp.minimum(ls[0], ls[1]), jnp.minimum(ls[2], ls[3]))
            hi = jnp.maximum(jnp.maximum(ls[0], ls[1]), jnp.maximum(ls[2], ls[3]))
            ok = jnp.logical_and(lo >= L_LO, hi <= L_HI)
            ok = jnp.logical_and(ok, (hi if I else jnp.maximum(ls[2], ls[3]))
                                 <= L_RATIO * (lo if I else jnp.minimum(ls[2], ls[3])))
            bad = jnp.where(ok, 0.0, 1.0)
            chk[1] = bad if chk[1] is None else jnp.maximum(chk[1], bad)

    def job_p(I, h, f, J):
        star, last = (_HALF, True) if J is None else (_FULL, J == I - 1)
        blk = I if J is None else J
        if f[0] == 'B':
            x = _ld(v_scr, 2 * (SB * blk + f[1]) + h, slice(HT // 2, HT))
        else:
            slot, r = _v_slot(star, blk, f)
            x = _ld(pf[h], slot, slice(r // 2, (r + HT) // 2))
        v = _dot(x, _ld(pf[h], (_HSLOT if J is None else J * len(_FULL.pf)) + star.pf[star.pv[f]]))
        res.append(v)
        key = (star.n,) + f
        acc[key] = v if key not in acc else acc[key] + v
        if not last:
            return

        def add(which, i, v, sign=1):
            k_ = (star.n, which, i)
            if k_ not in fg:
                fg[k_] = v if sign > 0 else -v
            else:
                fg[k_] = fg[k_] + v if sign > 0 else fg[k_] - v

        if f[0] == 'W':
            add('F', f[1], acc.pop(key))
        elif f[0] == 'B':
            add('G', f[1], acc.pop(key), csign[star.n, f[1]])
        elif f[0] == 'Q3':
            _, i, j = f
            q1, q2, q3 = (acc.pop((star.n, q, i, j)) for q in ('Q1', 'Q2', 'Q3'))
            t = ((q1 + q2) + q3) * (1.0 / (star.ts[i] - star.ts[j]))
            add('G', i, t)
            add('G', j, t)
            add('F', i, q1)
            add('F', j, q3, -1)

    def job_v(I, h, i, k):
        u = 2 * (SB * I + i) + h
        v = _dot(_ld(v_scr, 2 * (SB * I + k) + h), _ld(pf[h], _DSLOT + _DCELLS.index((i, k))))
        res.append(v)
        dacc[u] = v if u not in dacc else dacc[u] + v
        if k == i:
            o = dacc.pop(u)
            for star, a in ([(_FULL, i)] if I else []) + ([(_HALF, i - 2)] if i >= 2 else []):
                f, g = fg.pop((star.n, 'F', a)), fg.pop((star.n, 'G', a))
                o = o + jnp.concatenate([f - star.ts[a] * g, g], axis=0)
            o = o * (1.0 / lrow[u])
            of[u] = o
            chk[0] = chk[0] + jnp.sum(o.reshape(T // 8, 8, T), axis=0)

    def job_o(_, n):
        af, bf, outs = _O_JOBS[n][1]
        if af not in lhs:
            v = _form(af, lambda i, h: of[2 * i + h])
            lhs[af] = _tie(v.astype(BF16).T, v[0:8, :])
        if bf not in wo:
            wo[bf] = (wo_ref[_tile(bf[0][1]), _tile(bf[0][2])] if len(bf) == 1 else
                      _form(bf, lambda h, j: wo_ref[_tile(h), _tile(j)].astype(F32)).astype(BF16))
            if HACKWO:
                wo[bf] = _ld(q_scr, len(wo) % 32)
        v = _dot(lhs[af], wo[bf])
        res.append(v)
        for sign, i, j in outs:
            terms.setdefault((i, j), []).append((sign, v))
            if len(terms[i, j]) == left[i, j]:
                tot = acc_scr[_tile(i), _tile(j)]
                for sg, m in terms.pop((i, j)):
                    tot = tot + m if sg > 0 else tot - m
                acc_scr[_tile(i), _tile(j)] = tot

    fns = dict(e=job_e, f=job_f, d=job_d, p=job_p, v=job_v, o=job_o)
    order = _job_order(q_scr.shape[0] // (2 * SB))
    for n, job in enumerate(order):
        assert job[0] not in 'efd' or not any(j[0] in 'pv' and j[2] == job[2] and j[1] < job[1] for j in order[n:])
    side = list(side)
    fences = [n for n, job in enumerate(order) if job[0] == 'd' and job[3:] == _DCELLS[-1]]
    step = (len(order) - SIDE0 - SIDE1 - 10) / len(side)
    for n, job in enumerate(order):
        done_side[1] = n
        fns[job[0]](*job[1:])
        last_chance = n >= len(order) - SIDE1
        near = any(-SG1 <= f - n <= SG0 for f in fences)
        if side and n >= SIDE0 + step * done_side[0] and ((job[0] in SKIND and not near) or last_chance):
            done_side[0] += 1
            v = side.pop(0)(res[-1 - SLAG][8 * (n % 4):8 * (n % 4) + 8, :])
            if v is not None:
                due.append((n + SDUE, v))
    assert not side and not due
    fine = jnp.abs(chk[0]) < jnp.inf
    flag_scr[...] = jnp.maximum(flag_scr[...], jnp.where(fine, chk[1], 1.0))


def _kernel(x_hbm, c_hbm, wq_hbm, wuk_hbm, wuv_hbm, wo_hbm, w1_hbm, w2_hbm, w3_hbm, w4_hbm,
            cond_hbm, wmod_hbm, out_hbm,
            x_ref, c_ref, cond_ref, wma_ref, wmb_ref, w1_ref, w3_ref,
            wq_buf, wk_buf, wv_buf, wo_buf, out_buf, sem, wsem, osem,
            mod_scr, h_scr, cs_scr, hs_scr, w_scr, q_scr, k_scr, v_scr, acc_scr, xn_scr, xh_scr, a1_scr, t_scr,
            z_scr, mw_scr, m3_scr, wt_scr, wf_scr, gap_scr, st_in, pf_scr, vf_scr, flag_scr):
    S, M = x_hbm.shape
    D = wq_hbm.shape[2]
    nattn = wo_hbm.shape[0]
    Fd = w4_hbm.shape[0]
    scale = float(D) ** -0.5 * LOG2E
    nb, nrb = S // T, S // RB
    km, kc = M // T, c_hbm.shape[1] // T
    NX = 4
    XR = S // NX
    CB = XR // T

    work = (wk_buf, wv_buf, wq_buf)

    def pcopies(g, bufs=work, s0=0):
        return [pltpu.make_async_copy(src.bitcast(U32).at[:, g, :], dst, wsem.at[s0 + j])
                for j, (src, dst) in enumerate(zip((wuk_hbm, wuv_hbm, wq_hbm), bufs))]

    def ocopy(g):
        return pltpu.make_async_copy(wo_hbm.at[g], wo_buf, wsem.at[3])

    def chunk_copy(src, dst, i, s0):
        rows = slice(i * XR, (i + 1) * XR)
        return pltpu.make_async_copy(src.at[rows, :], dst.at[rows, :], sem.at[s0 + i])

    MS = 16
    NSL = T // MS
    assert nattn - 1 >= NSL
    mixw = ((w1_hbm, km, 0), (w2_hbm, km, km * MS), (w3_hbm, Fd // T, 2 * km * MS),
            (w4_hbm, -(-Fd // T), (2 * km + Fd // T) * MS))

    def prep_in(g):
        o = jnp.minimum(g, NSL - 1) * MS
        return [pltpu.make_async_copy(
            w.at[pl.ds(pl.multiple_of(jnp.minimum(b * T + o, w.shape[0] - MS), MS), MS), :],
            st_in.at[r0 + b * MS:r0 + (b + 1) * MS, :], wsem.at[7]) for w, nblk, r0 in mixw for b in range(nblk)]

    def stage_in(g):
        return pcopies(jnp.minimum(g + 1, nattn - 1))

    cp_cond = pltpu.make_async_copy(cond_hbm, cond_ref, sem.at[0])
    cp_wma = pltpu.make_async_copy(wmod_hbm.at[:, 0:2 * M], wma_ref, sem.at[1])
    cp_late = [pltpu.make_async_copy(src, dst, sem.at[2 + j]) for j, (src, dst) in enumerate((
        (wmod_hbm.at[:, 2 * M:6 * M], wmb_ref), (w1_hbm, w1_ref), (w3_hbm.at[Fd // T * T:, :], w3_ref)))]
    cp_x = [chunk_copy(x_hbm, x_ref, i, 7) for i in range(NX)]
    cp_c = [chunk_copy(c_hbm, c_ref, i, 7 + NX) for i in range(NX)]

    def silu_cond():
        cf = cond_ref[...].astype(F32)
        return jnp.broadcast_to((cf * jax.nn.sigmoid(cf)).astype(BF16), (8, M))

    cp_wk, cp_wv, cp_wq = pcopies(0)
    named = dict(k=cp_wk, v=cp_wv, q=cp_wq, o=ocopy(0), n=cp_cond, m=cp_wma)
    named.update(zip('abcd', cp_c))
    named.update(zip('wxyz', cp_x))
    started, arrived, did = set(), set(), set()

    def zero(r, carry):
        acc_scr[pl.ds(pl.multiple_of(r * T, T), T), :] = jnp.zeros((T, M), F32)
        return carry

    def x_rows(rows, dep):
        xf = x_ref[rows, :].astype(F32)
        if dep is None:
            return xf
        return jnp.concatenate([_after(xf[:, :T], _rows(dep, xf.shape[0])), xf[:, T:]], axis=1)

    def n_item(r, i):
        def fn(dep):
            rows = slice(r * T + i * LP, r * T + (i + 1) * LP)
            xn_scr[rows, :] = _ln(x_rows(rows, dep))
        return fn

    def h_item(r, i, normed):
        def fn(dep):
            rows = slice(i * LP, (i + 1) * LP)
            grows = slice(r * T + i * LP, r * T + (i + 1) * LP)
            sa = mod_scr[:, 0:M]
            if normed and dep is not None:
                sa = jnp.concatenate([_after(sa[:, _tile(j)], dep) for j in range(km)], axis=1)
            hf = ((xn_scr[grows, :] if normed else _ln(x_rows(grows, dep))) * _rows(mod_scr[:, M:2 * M], LP)
                  + _rows(sa, LP))
            for j in range(km):
                h_scr[r, j, rows, :] = hf[:, _tile(j)].astype(BF16)
            for f, n in _H_SUMS.items():
                if all(t[1] == r for t in f):
                    hs_scr[n, rows, :] = _form(f, lambda _, k: hf[:, _tile(k)]).astype(BF16)
            did.add(('h', r, i))
        return fn

    def release(jobs, span, items):
        if span and items:
            jobs.side += [(len(jobs.res) + 1 + i * span // len(items), fn) for i, fn in enumerate(items)]
            jobs.side.sort(key=lambda e: e[0])
        else:
            for fn in items:
                fn(None)

    def sum_items(n, group, index, dst, get, skip_rows):
        forms = [f for f in dict.fromkeys(t[0] for t in group)
                 if len(f) > 1 and not (skip_rows and len({t[1] for t in f}) == 1)]

        def item(f, rows):
            def fn(dep):
                def term(r, k):
                    v = get(r, k, rows).astype(F32)
                    return v if dep is None or (r, k) != f[0][1:] else _after(v, _rows(dep, v.shape[0]))
                dst[index[f], rows, :] = _form(f, term).astype(BF16)
            return fn

        return [item(f, slice(i, i + n)) for i in range(0, T, n) for f in forms]

    h_sums = lambda n, gi: sum_items(n, _H_GROUPS[gi], _H_SUMS, hs_scr,
                                     lambda r_, k, rows: h_scr[r_, k, rows, :], True)

    def stash(key, buf, j0, transpose=False):
        n = buf.shape[0] // T
        if key not in did:
            assert key in arrived
            did.add(key)
            for (j, hd), w in _pair_tiles(buf, transpose).items():
                w_scr[hd, j0 + j] = w
        return lambda hd: [_ld(w_scr, hd, j0 + j) for j in range(n)]

    def kv_tile(jobs, r):
        wk, wvT = stash('k', wk_buf, 0), stash('v', wv_buf, kc, True)
        ct = [c_ref[_tile(r), _tile(j)] for j in range(kc)]
        for hd in range(2):
            k_scr[2 * r + hd] = jobs.mm(ct, wk(hd), _dot).astype(BF16)
        for hd in range(2):
            v_scr[2 * r + hd] = jobs.mm(wvT(hd), ct, _dot_nt).astype(BF16)

    def q_tile(jobs, r):
        wq = stash('q', wq_buf, 2 * kc)
        ht = [_ld(h_scr, r, j) for j in range(km)]
        for hd in range(2):
            v = (jobs.mm(ht, wq(hd), _dot) * scale).astype(BF16)
            q_scr[2 * r + hd] = v.T if 2 * r + hd in QT else v

    for blk in _prologue().split(';'):
        waits, starts, acts = blk.split('|')
        for ch in waits.strip():
            assert ch in started and ch not in arrived
            arrived.add(ch)
            named[ch].wait()
        for ch in starts.strip():
            assert ch not in started
            started.add(ch)
            named[ch].start()
        jobs = _Jobs()
        for act in acts.split():
            if act == 'Z':
                jax.lax.fori_loop(0, nb, zero, 0)
                acc_scr[S:, :] = jnp.zeros((acc_scr.shape[0] - S, M), F32)
                x_ref[S:, :] = jnp.zeros((x_ref.shape[0] - S, M), BF16)
                flag_scr[...] = jnp.zeros(flag_scr.shape, F32)
            elif act == 'L':
                did.add('L')
                assert ('Q', 0) in did
                for cp in stage_in(0) + prep_in(0):
                    cp.start()
            elif act == 'M':
                assert arrived >= set('nm')
                mod = _dot(silu_cond(), wma_ref[...])
                mod_scr[:, 0:M] = mod[:, 0:M]
                mod_scr[:, M:2 * M] = 1.0 + mod[:, M:2 * M]
                did.add('M')
            else:
                act, _, span = act.partition('@')
                span = int(span or 0)
                items = []
                for r in [int(ch, 16) for ch in act[1:]]:
                    did.add((act[0], r))
                    if act[0] == 'K':
                        assert 'abcd'[r // CB] in arrived
                        kv_tile(jobs, r)
                    elif act[0] == 'H':
                        assert 'wxyz'[r // CB] in arrived and 'M' in did
                        items += [h_item(r, i, ('N', r) in did) for i in range(T // LP)]
                    elif act[0] == 'N':
                        assert 'wxyz'[r // CB] in arrived
                        items += [n_item(r, i) for i in range(T // LP)]
                    elif act[0] == 'Q':
                        assert all(('h', r, i) in did for i in range(T // LP))
                        q_tile(jobs, r)
                    elif act[0] == 'F':
                        assert all(('K', SB * r + k_) in did for k_ in range(SB))
                        items += _v_form_items(v_scr, (pf_scr, vf_scr), r)
                    elif act[0] == 'C':
                        assert all('abcd'[t[1] // CB] in arrived for p_ in _C_GROUPS[r] for t in p_[0])
                        items += sum_items(
                            32, _C_GROUPS[r], _C_SUMS, cs_scr,
                            lambda r_, k, rows: c_ref[r_ * T + rows.start:r_ * T + rows.stop, _tile(k)], False)
                    else:
                        assert act[0] == 'S' and all(('h', t[1], T // LP - 1) in did for p_ in _H_GROUPS[r] for t in p_[0])
                        items += h_sums(32 if span else 16, r)
                release(jobs, span, items)
        assert not jobs.side
    assert arrived == set(named) and all((k_, r) in did for k_ in 'KHQ' for r in range(nb))
    assert all((k_, r) in did for k_ in 'CS' for r in range(2)) and 'L' in did
    assert all(('F', r) in did for r in range(SB))

    def mixer_prep(g):
        sl = jnp.minimum(g, NSL - 1)
        rows = pl.ds(pl.multiple_of(sl * MS, MS), MS)

        def part(m, forms):
            def fn(dep):
                base = {}

                def get(i, k):
                    if (i, k) not in base:
                        rb, cb = (i, k) if m == 2 else (k, i)
                        r0 = mixw[m][2] + rb * MS
                        v = _after(st_in[r0:r0 + MS, _tile(cb)].astype(F32), _rows(dep, MS))
                        if m == 3 and (rb + 1) * T > Fd:
                            v = jnp.where(rb * T + sl * MS < Fd, v, 0.0)
                        base[i, k] = v
                    return base[i, k]

                for f in forms:
                    v = _form(f, get)
                    mw_scr[_MIXW[m, f], rows, :] = (0.5 * v if m % 2 else v).astype(BF16)
            return fn

        items = []
        for m in range(4):
            forms = [f for mm_, f in _MIXW if mm_ == m]
            cur, terms = [], set()
            for f in forms:
                new_terms = terms | {t[1:] for t in f}
                if cur and 3 * len(new_terms) + sum(2 * len(x) + 1 for x in cur + [f]) > MWOPS:
                    items.append(part(m, cur))
                    cur, terms = [], set()
                cur.append(f)
                terms |= {t[1:] for t in f}
            items.append(part(m, cur))

        n3 = sum(m == 2 for m, _ in _MIXW)
        first = min(n for (m, _), n in _MIXW.items() if m == 2)
        per = -(-n3 // (nattn - 1 - NSL))

        def turn(j):
            def fn(dep):
                n = jnp.minimum(jnp.maximum(g - NSL, 0) * per + j, n3 - 1)
                w = _tie(_ld(mw_scr, first + n), dep).T
                m3_scr[n] = w
                return pltpu.bitcast(pltpu.bitcast(w, U32)[T // 2 - 8:], F32)
            return fn

        return items + [turn(j) for j in range(per)]

    def stage_wait():
        for cp in pcopies(0):
            cp.wait()
        pltpu.make_async_copy(st_in, st_in, wsem.at[7]).wait()

    def attn_body(g, carry):
        side = _gap_items(work, gap_scr) + _weight_form_items(work, gap_scr, wt_scr, wf_scr, (0, 1, 2))
        bufs = (q_scr, k_scr, v_scr, (pf_scr, vf_scr), wo_buf, acc_scr, flag_scr)
        _attention_step(*bufs, g >> 16, side)

        @pl.when(g + 1 < nattn)
        def _():
            copies = stage_in(g + 1) + [ocopy(g + 1)]
            for cp in copies:
                cp.start()
            bufs = (h_scr, hs_scr, c_ref, cs_scr, wf_scr, q_scr, k_scr, v_scr, (pf_scr, vf_scr))
            side = [(SD0 + int(i * SDS), fn) for i, fn in enumerate(mixer_prep(g))]
            _proj_step(*bufs, scale, gap_scr, side)
            for cp in prep_in(g + 1):
                cp.start()
            stage_wait()
            ocopy(g + 1).wait()

        return carry

    stage_wait()
    for cp in cp_late:
        cp.start()
    jax.lax.fori_loop(0, nattn, attn_body, 0)

    def safe_pair(g, carry):
        copies = pcopies(g) + [ocopy(g)]
        for cp in copies:
            cp.start()
        for cp in copies:
            cp.wait()
        for buf, j0, transpose in ((wk_buf, 0, False), (wv_buf, kc, True), (wq_buf, 2 * kc, False)):
            for (j, hd), w in _pair_tiles(buf, transpose).items():
                w_scr[hd, j0 + j] = w

        def tile(u, carry):
            r, hd = u // 2, u % 2
            rows = pl.ds(pl.multiple_of(r * T, T), T)
            ct = [c_ref[rows, _tile(j)] for j in range(kc)]
            k_scr[u] = sum(_dot(ct[j], _ld(w_scr, hd, j)) for j in range(kc)).astype(BF16)
            v_scr[u] = sum(_dot_nt(_ld(w_scr, hd, kc + j), ct[j]) for j in range(kc)).astype(BF16)
            q = sum(_dot(_ld(h_scr, r, j), _ld(w_scr, hd, 2 * kc + j)) for j in range(km))
            q_scr[u] = (q * scale).astype(BF16)
            return carry

        jax.lax.fori_loop(0, 2 * nb, tile, 0)
        _attention_safe(q_scr, k_scr, v_scr, wo_buf, acc_scr)
        return carry

    @pl.when(jnp.max(flag_scr[...]) > 0)
    def _():
        jax.lax.fori_loop(0, nb, zero, 0)
        jax.lax.fori_loop(0, nattn, safe_pair, 0)

    for cp in cp_late:
        cp.wait()
    mod = _dot(silu_cond(), wmb_ref[...])
    mod_scr[:, 2 * M:4 * M] = mod[:, 0:2 * M]
    mod_scr[:, 4 * M:5 * M] = 1.0 + mod[:, 2 * M:3 * M]
    mod_scr[:, 5 * M:6 * M] = mod[:, 3 * M:4 * M]
    OFF = x_ref.shape[0] - S
    CAR = t_scr.shape[0] - RB

    def p1(r0, l0, n, dep=None):
        ga = mod_scr[:, 2 * M:3 * M]
        if dep is not None:
            ga = jnp.concatenate([_after(ga[:, 0:T], dep), ga[:, T:]], axis=1)
        rows = pl.ds(r0, n)
        x1 = x_ref[rows, :].astype(F32) + _rows(ga, n) * acc_scr[rows, :]
        xh_scr[0, l0:l0 + n, :] = x1
        hb = _ln(x1) * _rows(mod_scr[:, 4 * M:5 * M], n) + _rows(mod_scr[:, 3 * M:4 * M], n)
        xh_scr[1, l0:l0 + n, :] = hb
        return _ln(hb)

    HT = T // 2

    def p1_store(r0, c, dep=None):
        v = p1(r0 + c * PC, OFF + c * PC, PC, dep)
        a1_scr[c * PC:(c + 1) * PC, :] = v
        return jnp.max(v[:, M - T:].reshape(PC // 8, 8, T), axis=0)

    t_scr[RB:RB + CAR - OFF, :] = jnp.zeros((CAR - OFF, M), F32)
    t_scr[RB + CAR - OFF:RB + CAR, :] = _gelu2(_dot(p1(0, 0, OFF).astype(BF16), w1_ref[...]))
    for c in range(RB // PC):
        p1_store(OFF, c)

    def out_copy(i):
        rows = pl.ds(i * T if isinstance(i, int) else pl.multiple_of(i * T, T), T)
        return pltpu.make_async_copy(out_buf.at[rows, :], out_hbm.at[rows, :], osem.at[i])

    def b_body(r, carry):
        gb = _rows(mod_scr[:, 5 * M:6 * M], T)
        r0 = pl.multiple_of(r * RB, RB)
        n0 = pl.multiple_of(jnp.minimum(r0 + RB, S - RB) + OFF, OFF)
        nh = RB // T
        now = [0]
        due = []
        pace = []

        def p1_item(c):
            def fn(dep):
                due.append((now[0] + PD, p1_store(n0, c, dep)))
                due.sort(key=lambda e: e[0])
            return fn

        pace += [(P0 + i * PSTEP, p1_item(i)) for i in range(RB // PC)]

        def mm(lhs, wts, dot=_dot):
            acc = None
            for x, w in zip(lhs, wts):
                if due and due[0][0] <= now[0]:
                    w = _tie(w, due.pop(0)[1])
                v = dot(x, w)
                now[0] += x.shape[0] / HT
                acc = v if acc is None else v + acc
                if pace and pace[0][0] <= now[0]:
                    pace.pop(0)[1](v[0:8, :])
            return acc

        def fast(m, base, finish, hook=None):
            prods = _MIX[m]
            nsub = MSUB[m]
            n = HT // nsub
            done = {}
            for sub in range(nsub):
                left, acc, cache = {}, {}, {}
                for _, _, outs in prods:
                    for _, i, h in outs:
                        left[i, h] = left.get((i, h), 0) + 1

                def act(form):
                    sign, form = _canon(form)
                    if form not in cache:
                        cache[form] = _form(
                            form, lambda k, h: base(k)[h * HT + sub * n:h * HT + (sub + 1) * n]).astype(BF16)
                    return sign, cache[form]

                for pi, (wf, af, outs) in enumerate(prods):
                    w = _ld(m3_scr, _MIXW[m, wf] - _MIX3) if m == 2 else _ld(mw_scr, _MIXW[m, wf])
                    if af is None:
                        k = wf[0][2]
                        v = mm([jnp.concatenate([act(((1, k, h),))[1] for h in range(2)], axis=0)], [w])
                        sign, parts = 1, [v[:n], v[n:]]
                    else:
                        sign, x = act(af)
                        parts = [mm([x], [w])] * len(outs)
                    for (s_, i, h), v in zip(outs, parts):
                        s_ = s_ * sign
                        if (i, h) not in acc:
                            acc[i, h] = (s_, v)
                        else:
                            s0, u = acc[i, h]
                            acc[i, h] = (s0, u + v if s0 == s_ else u - v) if s0 > 0 or s_ < 0 else (1, v - u)
                        left[i, h] -= 1
                        if not left[i, h]:
                            s0, done[i, h, sub] = acc.pop((i, h))
                            assert s0 > 0
                            if all((i, hh, ss) in done for hh in range(2) for ss in range(nsub)):
                                finish(i, jnp.concatenate([done[i, hh, ss] for hh in range(2)
                                                           for ss in range(nsub)], axis=0))
                    if hook is not None and sub == nsub - 1:
                        hook(pi, act)

        t_scr[0:CAR, :] = t_scr[RB:RB + CAR, :]
        for hf in range(nh):
            def put_t(n, v):
                t = _gelu2(v)
                if hf == nh - 1:
                    t = jnp.concatenate([t[:T - OFF], jnp.where(r < nrb - 1, t[T - OFF:], 0.0)], axis=0)
                t_scr[CAR + hf * T:CAR + (hf + 1) * T, _tile(n)] = t

            fast(0, lambda k: a1_scr[_tile(hf), _tile(k)], put_t)
        cq = M // 4
        shifts = (-1, 1, -2, 2)
        lane = jax.lax.broadcasted_iota(jnp.int32, (T, T), 1)
        y1, a3 = [], []
        for hf in range(nh):
            base = CAR - OFF + hf * T
            sh = []
            for j in range(km):
                g_lo, g_hi = (j * T) // cq, ((j + 1) * T - 1) // cq
                assert g_hi - g_lo <= 1
                v = t_scr[base + shifts[g_lo]:base + shifts[g_lo] + T, _tile(j)]
                if g_hi != g_lo:
                    v2 = t_scr[base + shifts[g_hi]:base + shifts[g_hi] + T, _tile(j)]
                    v = jnp.where(lane < g_hi * cq - j * T, v, v2)
                else:
                    v = jnp.where(lane < T, v, 0.0)
                sh.append(v)
            hs = {}
            fast(1, lambda k: sh[k], hs.__setitem__)
            hs = jnp.concatenate([hs[n] for n in range(km)], axis=1)
            y1.append(hs + xh_scr[1, _tile(hf), :])
            z_scr[_tile(hf), :] = xh_scr[0, _tile(hf), :] + gb * y1[hf]
            a3.append({})

            def ln_item(hf, c):
                def item(dep):
                    n = HT // NLN
                    for d in (0, HT):
                        v = y1[hf][d + c * n:d + (c + 1) * n]
                        if dep is not None:
                            v = jnp.concatenate([_after(v[:, :T], _rows(dep, n)), v[:, T:]], axis=1)
                        a3[hf][d + c * n] = _ln(v)
                return item

            ln_item(hf, 0)(None)
            pace += [(now[0] + LN0 + (c - 1) * LNS * (1 + hf), ln_item(hf, c)) for c in range(1, NLN)]
            pace.sort(key=lambda e: e[0])
        xh_scr[:, 0:OFF, :] = xh_scr[:, RB:RB + OFF, :]
        z_scr[pl.ds(pl.multiple_of(RB + (r >> 16) * 8, 8), 8), :] = jnp.zeros((8, M), F32)
        h3 = []
        for hf in range(nh):
            assert len(a3[hf]) == 2 * NLN
            af = jnp.concatenate([a3[hf][key] for key in sorted(a3[hf])], axis=0)
            row = {}
            narrow = []

            def hook(pi, act):
                j, rem = divmod(pi - NAR0, NARS)
                if rem == 0 and 0 <= j < km:
                    full = jnp.concatenate([act(((1, j, h),))[1] for h in range(2)], axis=0)
                    v = mm([w3_ref[:, _tile(j)]], [full], _dot_nt)
                    narrow[:] = [v + narrow[0] if narrow else v]

            def put_h(n, v):
                row[n] = _gelu2(v)
                if GD:
                    due.append((now[0] + GD, jnp.max(row[n].reshape(T // 8, 8, T), axis=0)))
                    due.sort(key=lambda e: e[0])

            fast(2, lambda k: af[:, _tile(k)], put_h, hook)
            fw = w3_ref.shape[0]
            row[Fd // T] = jnp.concatenate([_gelu2(narrow[0]), jnp.zeros((T - fw, T), F32)], axis=0).T
            h3.append(row)
        for hf in range(nh):
            rows = pl.ds(pl.multiple_of(r0 + hf * T, T), T)

            def finish(n, v):
                out_buf[rows, _tile(n)] = (z_scr[_tile(hf), _tile(n)] + gb[:, _tile(n)] * v).astype(out_buf.dtype)

            fast(3, lambda k: h3[hf][k], finish)
            out_copy(r * nh + hf).start()
        assert not pace
        return carry

    jax.lax.fori_loop(0, nrb, b_body, 0)
    for i in range(nb):
        out_copy(i).wait()


@jax.jit
def pallas_adaLN_cond__compressed_kv_cla__mixer_s_mlp__prompt_kernel(
    A_x: jax.Array,
    A_c_kv: jax.Array,
    A_w_q: jax.Array,
    A_w_uk: jax.Array,
    A_w_uv: jax.Array,
    A_w_o: jax.Array,
    B_x: jax.Array,
    B_w1: jax.Array,
    B_w2: jax.Array,
    B_w3: jax.Array,
    B_w4: jax.Array,
    c: jax.Array,
    w_mod: jax.Array,
):
    _, S, M = A_x.shape
    Dc = A_c_kv.shape[2]
    H, D = A_w_q.shape[1], A_w_q.shape[2]
    Fd = B_w3.shape[1]
    assert D == T and A_c_kv.shape[1] == S and Dc == 4 * T and M == 5 * T and 13 * T < Fd < 14 * T and S == 16 * T
    vmem = pltpu.VMEM
    packed = lambda *lead: vmem(lead + (T, T), BF16)
    out = pl.pallas_call(
        _kernel,
        in_specs=[pl.BlockSpec(memory_space=pltpu.HBM)] * 12,
        out_specs=pl.BlockSpec(memory_space=pltpu.HBM),
        out_shape=jax.ShapeDtypeStruct((S, M), A_x.dtype),
        scratch_shapes=[
            vmem((S + 16, M), BF16),
            vmem((S, Dc), BF16),
            vmem((1, M), BF16),
            vmem((M, 2 * M), BF16),
            vmem((M, 4 * M), BF16),
            vmem((M, M), BF16),
            vmem((Fd % T, M), BF16),
            vmem((M, D), U32),
            vmem((Dc, D), U32),
            vmem((Dc, D), U32),
            vmem((2 * D, M), BF16),
            vmem((S, M), A_x.dtype),
            pltpu.SemaphoreType.DMA((15,)),
            pltpu.SemaphoreType.DMA((8,)),
            pltpu.SemaphoreType.DMA((S // T,)),
            vmem((8, 6 * M), F32),
            vmem((S // T, M // T, T, T), BF16),
            vmem((len(_C_SUMS), T, T), BF16),
            vmem((len(_H_SUMS), T, T), BF16),
            packed(2, M // T + 2 * (Dc // T)),
            packed(2 * S // T),
            packed(2 * S // T),
            packed(2 * S // T),
            vmem((S + 16, M), F32),
            vmem((S, M), F32),
            vmem((2, RB + 16, M), F32),
            vmem((RB, M), F32),
            vmem((RB + 32, M), F32),
            vmem((RB + 8, M), F32),
            packed(len(_MIXW)),
            packed(sum(m == 2 for m, _ in _MIXW)),
            vmem((Dc // T, T, T), U32),
            vmem((len(_WF), T, T), BF16),
            vmem((3, 8, T), jnp.int32),
            vmem(((2 * (M // T) + Fd // T + -(-Fd // T)) * 16, M), BF16),
            vmem((_FENCE + 1, T, T), BF16),
            vmem((_FENCE + 1, T, T), BF16),
            vmem((8, T), F32),
        ],
        compiler_params=pltpu.CompilerParams(
            vmem_limit_bytes=100 * 1024 * 1024,
            disable_bounds_checks=True,
        ),
    )(
        A_x.reshape(S, M), A_c_kv.reshape(S, Dc),
        A_w_q, A_w_uk, A_w_uv,
        A_w_o.reshape(H // 2, 2 * D, M),
        B_w1, B_w2, B_w3.T, B_w4, c, w_mod,
    )
    return out.reshape(1, S, M)
```

```python
import functools
import math

import jax
import jax.numpy as jnp
import jax.experimental.pallas as pl
import jax.experimental.pallas.tpu as pltpu

F32 = jnp.float32
BF16 = jnp.bfloat16
U32 = jnp.uint32
NT = (((1,), (1,)), ((), ()))
T = 128
EPS = 1e-5
LOG2E = math.log2(math.e)

GRP = 4
LEAD = 10
PROW = 3
RES = 32
LAT_0 = 32
LAT_A = 16
LAT_B = 20
ALEAD = 32
QT = (4, 6)
ONV, OEND = 0.5, 24
FPOS, DPOS = 0, 0
SIDE0, SIDE1, SLAG, SDUE = 8, 60, 4, 8
SKIND = 'pvo'
HACKWO = 0
SG0, SG1 = 6, 4
SD0, SDS = 4, 1.5
WFN = (4, 4, 6)
VF0, VFS = 4, 1.7
L_LO, L_HI, L_RATIO = 2.0 ** -24, 2.0 ** 24, 4.0
RB = 256
PC = 32
P0, PSTEP, PD = 300, 34, 36
GD, NAR0, NARS = 36, 4, 8
MSUB = (1, 1, 1, 1)
PSPLIT = 40
PDUE = 20
MWOPS = 70
NLN, LN0, LNS = 4, 4, 5
LP = 16
SP0, SP1 = 76, 38
_prologue = lambda: ('|kva|Z; |b|; kva|wc|K0123; bw|xdn|C0@56 N0123@52 K4567; cx|mq|N4567@52 F0@56 K89ab; '
            'd|y|C1@56 F1@56 Kcdef; nmq|zo|M H01 H234567@30 F2@36 Q0123; y||L H89ab@30 F3@36 Q4567; '
            'zo||Hcdef@30 S0@%d Q89ab S1@%d Qcdef' % (SP0, SP1))


def _dot(a, b):
    return jnp.dot(a, b, preferred_element_type=F32)


def _dot_nt(a, b):
    return jax.lax.dot_general(a, b, NT, preferred_element_type=F32)


def _ln(x):
    m = jnp.mean(x, axis=-1, keepdims=True)
    xc = x - m
    v = jnp.mean(xc * xc, axis=-1, keepdims=True)
    return xc * jnp.exp2(jnp.log(v + EPS) * (-0.5 * LOG2E))


def _rows(v, n):
    return jnp.broadcast_to(v[None], (n // 8, 8, v.shape[1])).reshape(n, v.shape[1])


def _gelu2(x):
    c0 = math.sqrt(2.0 / math.pi)
    return x + x * jnp.tanh(x * (c0 + (c0 * 0.044715) * (x * x)))


def _after(x, dep):
    return jnp.where(dep > jnp.inf, dep, x)


def _tie(x, dep):
    xu = pltpu.bitcast(x, U32)
    first = jnp.where(dep > jnp.inf, jnp.uint32(0), xu[:8])
    return pltpu.bitcast(jnp.concatenate([first, xu[8:]], axis=0), BF16)


def _tile(j):
    return slice(j * T, (j + 1) * T)


def _ld(ref, *idx):
    return pltpu.bitcast(ref.bitcast(U32)[idx], BF16)


def _a_ops(a11, a12, a21, a22):
    return [a11 + a22, a21 + a22, a11, a22, a11 + a12, a21 - a11, a12 - a22]


def _b_ops(b11, b12, b21, b22):
    return [b11 + b22, b11, b12 - b22, b21 - b11, b22, b11 + b12, b21 + b22]


def _strassen(prod, col1=None, col2=None):
    m4 = prod(3)
    m2 = prod(1)
    c21 = m2 + m4
    if col1 is not None:
        e11, e21 = col1()
        m4, c21 = m4 + e11, c21 + e21
    m3 = prod(2)
    m5 = prod(4)
    c12 = m3 + m5
    if col2 is not None:
        e12, e22 = col2()
        c12, m3 = c12 + e12, m3 + e22
    m1 = prod(0)
    c11 = prod(6) + (m1 + (m4 - m5))
    c22 = prod(5) + (m1 + (m3 - m2))
    return c11, c12, c21, c22


def _group(rows, cols, pairs):
    xs, ys = dict.fromkeys(x for x, _ in pairs), dict.fromkeys(y for _, y in pairs)
    used = set(xs) | set(ys) | {(x[0], y[1]) for x, y in pairs} | {(y[0], x[1]) for x, y in pairs}
    prods = []
    for n, r in enumerate(rows):
        for i, k in [x for x in xs if x[0] == r]:
            mates = [y for x, y in pairs if x == (i, k)]
            prods.append((((1, i, k),) + tuple((1, i, k2) for _, k2 in mates), ((1, k, 0),),
                          ((1, i, 0), (-1, i, 1))))
            prods.append((((1, i, k),) + tuple((-1, i2, k) for i2, _ in mates), ((1, k, 0), (1, k, 1)),
                          ((1, i, 1),)))
        for i2, k2 in [y for y in ys if y[0] == r]:
            mates = [x for x, y in pairs if y == (i2, k2)]
            prods.append((((1, i2, k2),) + tuple((1, i2, k) for _, k in mates), ((1, k2, 1),),
                          ((1, i2, 1), (-1, i2, 0))))
            prods.append((((1, i2, k2),) + tuple((-1, i, k2) for i, _ in mates), ((1, k2, 0), (1, k2, 1)),
                          ((1, i2, 0),)))
        prods += [(((1, r, k),), ((1, k, h),), ((1, r, h),)) for k in cols if (r, k) not in used for h in (0, 1)]
        for (i, k), (i2, k2) in pairs:
            if r in (i, i2) and i + i2 - r in rows[n + 1:]:
                prods.append((((1, i, k2),), ((1, k2, 0), (-1, k, 0)), ((1, i2, 0), (1, i, 0))))
                prods.append((((1, i2, k), (1, i, k2)), ((1, k, 0), (1, k2, 1)), ((1, i2, 0), (1, i, 1))))
                prods.append((((1, i2, k),), ((1, k, 1), (-1, k2, 1)), ((1, i2, 1), (1, i, 1))))
    return prods


def _all_pairs(xrows, yrows):
    return [((x, a), (y, b)) for a, x in enumerate(xrows) for b, y in enumerate(yrows) if a != b]


_PAIRS65 = [((x[0] + 10, x[1]), (y[0] + 10, y[1])) for x, y in (
    ((0, 1), (1, 0)), ((0, 1), (5, 2)), ((2, 3), (1, 0)), ((2, 3), (3, 1)), ((2, 3), (5, 2)), ((3, 2), (1, 0)),
    ((4, 4), (0, 3)), ((4, 4), (1, 0)), ((4, 4), (3, 1)), ((4, 4), (5, 2)))]
_C_GROUPS = [_group(range(r, r + 8), range(4), _all_pairs(range(r, r + 4), range(r + 4, r + 8))) for r in (0, 8)]
_H_GROUPS = [_group(range(10), range(5), _all_pairs(range(5), range(5, 10))),
             _group(range(10, 16), range(5), _PAIRS65)]
_sum_index = lambda groups: {f: n for n, f in enumerate(
    dict.fromkeys(t[0] for g in groups for t in g if len(t[0]) > 1))}
_C_SUMS, _H_SUMS = _sum_index(_C_GROUPS), _sum_index(_H_GROUPS)


def _cells(rows, cols, pairs):
    xs = list(dict.fromkeys(p[0] for p in pairs))
    ys = list(dict.fromkeys(p[1] for p in pairs))
    used = set(xs + ys) | {(x[0], y[1]) for x, y in pairs} | {(y[0], x[1]) for x, y in pairs}

    def home_x(i, k):
        mates = [y for x, y in pairs if x == (i, k)]
        return [(((1, i, k),) + tuple((1, i, k2) for _, k2 in mates), ((1, k, 0),), ((1, i, 0), (-1, i, 1))),
                (((1, i, k),) + tuple((-1, i2, k) for i2, _ in mates), ((1, k, 0), (1, k, 1)), ((1, i, 1),))]

    def home_y(i2, k2):
        mates = [x for x, y in pairs if y == (i2, k2)]
        return [(((1, i2, k2),) + tuple((1, i2, k) for _, k in mates), ((1, k2, 1),), ((1, i2, 1), (-1, i2, 0))),
                (((1, i2, k2),) + tuple((-1, i, k2) for i, _ in mates), ((1, k2, 0), (1, k2, 1)), ((1, i2, 0),))]

    def cross(x, y):
        (i, k), (i2, k2) = x, y
        return [(((1, i, k2),), ((1, k2, 0), (-1, k, 0)), ((1, i2, 0), (1, i, 0))),
                (((1, i2, k), (1, i, k2)), ((1, k, 0), (1, k2, 1)), ((1, i2, 0), (1, i, 1))),
                (((1, i2, k),), ((1, k, 1), (-1, k2, 1)), ((1, i2, 1), (1, i, 1)))]

    direct = lambda i: [(((1, i, k),), None, ((1, i, 0), (1, i, 1))) for k in cols if (i, k) not in used]
    single = lambda i: ([t for x in xs if x[0] == i for t in home_x(*x)]
                        + [t for y in ys if y[0] == i for t in home_y(*y)] + direct(i))
    prods = []
    for n, i in enumerate(rows):
        prods += single(i)
        for i2 in rows[n + 1:]:
            for x, y in pairs:
                if {x[0], y[0]} == {i, i2}:
                    prods += cross(x, y)
    return prods


_square = lambda q: [((a, a), (q + b, b)) for a in range(q) for b in range(q) if a != b]
_shift = lambda pairs, r0: [((x[0] + r0, x[1]), (y[0] + r0, y[1])) for x, y in pairs]
_flip = lambda pairs: [(x[::-1], y[::-1]) for x, y in pairs]
_P35 = [((1, 2), (0, 4)), ((1, 2), (2, 1)), ((2, 3), (0, 4)), ((2, 3), (1, 0))]
_P45 = [((0, 2), (1, 1)), ((2, 4), (0, 3)), ((2, 4), (1, 1)), ((2, 4), (3, 2)), ((3, 0), (0, 3)), ((3, 0), (1, 1))]
_P55 = [((2, 1), (0, 4)), ((2, 1), (1, 0)), ((2, 1), (3, 2)), ((2, 1), (4, 3)), ((3, 3), (0, 4)), ((3, 3), (1, 0)),
        ((4, 2), (0, 4)), ((4, 2), (1, 0))]
_MIX = [_cells(range(5), range(5), _P55), _cells(range(5), range(5), _P55),
        _cells(range(13), range(5), _square(5) + _shift(_P35, 10)),
        _cells(range(5), range(14), _flip(_square(5) + _shift(_P45, 10)))]
_MIXW = {(m, f): n for n, (m, f) in enumerate(dict.fromkeys((m, t[0]) for m in range(4) for t in _MIX[m]))}
_MIX3 = min(n for (m, _), n in _MIXW.items() if m == 2)


def _form(form, get):
    acc = None
    for sign, i, j in form:
        v = get(i, j)
        acc = v if acc is None else (acc + v if sign > 0 else acc - v)
    return acc


def _gap_items(bufs, gap_scr):
    items = []
    for n, buf in enumerate(bufs):
        acc = []

        def part(r0, buf=buf, acc=acc):
            def fn(dep):
                wu = jnp.concatenate([buf[r:r + 8, :] for r in range(r0, r0 + T, 32)])
                mask = jnp.full((8, T), 0x7FFF0000, U32)
                if dep is not None:
                    mask = jnp.where(dep > jnp.inf, jnp.uint32(0), mask)
                mask = _rows(mask, 32)
                new = [jnp.sum(pltpu.bitcast(v & mask, F32).reshape(4, 8, T), axis=0) for v in (wu << 16, wu)]
                acc[:] = [u + v for u, v in zip(acc, new)] if acc else new
            return fn

        def last(_, n=n, acc=acc):
            bits = []
            for v in acc:
                l1 = jnp.sum(jnp.sum(v, axis=1, keepdims=True), axis=0, keepdims=True)
                bits.append(pltpu.bitcast(jnp.broadcast_to(l1, (8, T)), jnp.int32) >> 8)
            gap = jnp.clip((bits[0] - bits[1] + (1 << 14)) >> 15, -8, 8) << 23
            gap_scr[n] = gap
            return pltpu.bitcast(gap, F32)

        items += [part(r0) for r0 in range(0, buf.shape[0], T)] + [last]
    return items


def _pair_tiles(w_ref, transpose=False):
    tiles = {}
    for j in range(w_ref.shape[0] // T):
        wu = w_ref[_tile(j), :]
        if transpose:
            wu = wu.T
        tiles[j, 0] = pltpu.bitcast(wu << 16, F32).astype(BF16)
        tiles[j, 1] = pltpu.bitcast(wu & jnp.uint32(0xFFFF0000), F32).astype(BF16)
    return tiles


def _canon(form):
    if form[-1][0] < 0 and form[0][1:] > form[1][1:]:
        return -1, ((1,) + form[1][1:], (-1,) + form[0][1:])
    return 1, form


_w_forms = lambda groups: list(dict.fromkeys(_canon(t[1])[1] for g in groups for t in g))
_WF = {key: n for n, key in enumerate([(m, f) for m, groups in enumerate((_C_GROUPS, _C_GROUPS, _H_GROUPS))
                                       for f in _w_forms(groups)])}


def _weight_form_items(bufs, gap_scr, wt_scr, wf_scr, which):
    n = 16
    items = []

    def flip(j):
        def fn(dep):
            wu = bufs[1][_tile(j), :]
            wu = (wu if dep is None else jnp.where(_rows(dep, T) > jnp.inf, jnp.uint32(0), wu)).T
            wt_scr[j] = wu
            return pltpu.bitcast(wu[T - 8:], F32)
        return fn

    def part(m, r0, forms):
        def fn(dep):
            fac = pltpu.bitcast(0x3F800000 + gap_scr[m], F32)
            mask = jnp.full((8, T), 0xFFFF0000, U32)
            sh = jnp.full((8, T), 16, U32)
            if dep is not None:
                mask = jnp.where(dep > jnp.inf, jnp.uint32(0), mask)
                sh = jnp.where(dep > jnp.inf, jnp.uint32(0), sh)
            fac, mask, sh = _rows(fac, n), _rows(mask, n), _rows(sh, n)
            base = {}

            def get(k, h):
                if (k, h) not in base:
                    wu = wt_scr[k, r0:r0 + n, :] if m == 1 else bufs[m][k * T + r0:k * T + r0 + n, :]
                    base[k, h] = pltpu.bitcast(wu & mask, F32) * fac if h else pltpu.bitcast(wu << sh, F32)
                return base[k, h]

            for f in forms:
                wf_scr[_WF[m, f], r0:r0 + n, :] = _form(f, get).astype(BF16)
        return fn

    for m in which:
        forms = [f for mm, f in _WF if mm == m]
        if m == 1:
            items += [flip(j) for j in range(bufs[1].shape[0] // T)]
        per = -(-len(forms) // WFN[m])
        forms.sort(key=lambda f: sorted({t[1] for t in f}))
        items += [part(m, r0, forms[i:i + per]) for r0 in range(0, T, n) for i in range(0, len(forms), per)]
    return items


def _run_group(jobs, prods, a_get, w, transposed, finish):
    left = {}
    for _, _, outs in prods:
        for _, i, h in outs:
            left[i, h] = left.get((i, h), 0) + 1
    acc = {}
    for af, bf, outs in prods:
        sign, wt = w(bf)
        m = jobs.mm([wt], [a_get(af)], _dot_nt) if transposed else jobs.mm([a_get(af)], [wt], _dot)
        for s_, i, h in outs:
            if (i, h) not in acc:
                acc[i, h] = (s_ * sign, m)
            else:
                s0, v = acc[i, h]
                acc[i, h] = (s0, v + m if s0 == s_ * sign else v - m) if s0 > 0 or s_ * sign < 0 else (1, m - v)
            left[i, h] -= 1
            if not left[i, h]:
                s0, v = acc.pop((i, h))
                assert s0 > 0
                finish(2 * i + h, v)


class _Jobs:
    def __init__(self, side=()):
        self.res = []
        self.side = list(side)
        self.due = []

    def mm(self, lhs, wt, dot):
        acc = None
        for x, w in zip(lhs, wt):
            if self.due and self.due[0][0] <= len(self.res):
                x = _tie(x, self.due.pop(0)[1])
            v = dot(x, w)
            self.res.append(v)
            acc = v if acc is None else v + acc
            rel = 4 * (len(self.res) % 4)
            while self.side and self.side[0][0] <= len(self.res):
                out = self.side.pop(0)[1](v[8 * rel:8 * rel + 8, :])
                if out is not None:
                    self.due.append((len(self.res) + PDUE, out))
                rel = (rel + 2) % 16
        return acc


def _proj_step(h_scr, hs_scr, c_ref, cs_scr, wf_scr, q_scr, k_scr, v_scr, pf, scale, shifts, side):
    def weight(m):
        def get(form):
            sign, form = _canon(form)
            return sign, _ld(wf_scr, _WF[m, form])
        get.inv = pltpu.bitcast(0x3F800000 - shifts[m], F32)
        return get

    wk, wvT, wq = weight(0), weight(1), weight(2)
    c_get = lambda f: _ld(cs_scr, _C_SUMS[f]) if len(f) > 1 else c_ref[_tile(f[0][1]), _tile(f[0][2])]
    h_get = lambda f: _ld(hs_scr, _H_SUMS[f]) if len(f) > 1 else _ld(h_scr, f[0][1], f[0][2])

    def put(dst, w, mul=None):
        muls = [mul, _rows(w.inv if mul is None else w.inv * mul, T)]

        def fn(u, v):
            v = (v if muls[u % 2] is None else v * muls[u % 2]).astype(BF16)
            dst[u] = v.T if mul is not None and u in QT else v
        return fn

    jobs = _Jobs(side)
    put_v, stored = put(v_scr, wvT), set()
    nxt = [0]

    def fin_v(u, v):
        put_v(u, v)
        stored.add(u)
        for J in range(SB):
            if all(2 * (SB * J + k) + h in stored for k in range(SB) for h in range(2)) and ('J', J) not in stored:
                stored.add(('J', J))
                for fn in _v_form_items(v_scr, pf, J):
                    nxt[0] = max(nxt[0] + VFS, len(jobs.res) + VF0)
                    jobs.side.append((int(nxt[0]), fn))
                jobs.side.sort(key=lambda e: e[0])

    kk, vv, qq = ((c_get, wk, False, put(k_scr, wk)), (c_get, wvT, True, fin_v),
                  (h_get, wq, False, put(q_scr, wq, scale)))
    for prods, args in ((_C_GROUPS[0], kk), (_C_GROUPS[0], vv), (_C_GROUPS[1], vv), (_C_GROUPS[1], kk),
                        (_H_GROUPS[0], qq), (_H_GROUPS[1], qq)):
        _run_group(jobs, prods, *args)
    assert not jobs.side and not jobs.due


def _inner_group(rows, cols, pairs):
    xs, ys = dict.fromkeys(x for x, _ in pairs), dict.fromkeys(y for _, y in pairs)
    used = set(xs) | set(ys) | {(x[0], y[1]) for x, y in pairs} | {(y[0], x[1]) for x, y in pairs}
    prods = []
    for i, j in xs:
        mates = [y for x, y in pairs if x == (i, j)]
        prods.append((((1, i, 0),), ((1, 0, j), (-1, 1, j)), ((1, i, j),) + tuple((1, i2, j) for i2, _ in mates)))
        prods.append((((1, i, 0), (1, i, 1)), ((1, 1, j),), ((1, i, j),) + tuple((-1, i, j2) for _, j2 in mates)))
    for i2, j2 in ys:
        mates = [x for x, y in pairs if y == (i2, j2)]
        prods.append((((1, i2, 0), (1, i2, 1)), ((1, 0, j2),),
                      ((1, i2, j2),) + tuple((-1, i2, j) for _, j in mates)))
        prods.append((((1, i2, 1),), ((1, 0, j2), (-1, 1, j2)),
                      ((-1, i2, j2),) + tuple((-1, i, j2) for i, _ in mates)))
    prods += [(((1, i, h),), ((1, h, j),), ((1, i, j),))
              for i in rows for j in cols if (i, j) not in used for h in (0, 1)]
    for (i, j), (i2, j2) in pairs:
        lo, hi = min(j, j2), max(j, j2)
        prods.append((((1, i2, 0), (-1, i, 0)), ((1, 0, lo), (1, 0, hi)), ((1, i2, j),)))
        prods.append((((1, i, 0), (1, i2, 1)), ((1, 0, j2), (1, 1, j)), ((1, i, j2), (1, i2, j))))
        prods.append((((1, i, 1), (-1, i2, 1)), ((1, 1, lo), (1, 1, hi)), ((1, i, j2),)))
    return prods


def _o_jobs():
    prods = (_inner_group(range(10), range(5), _all_pairs(range(0, 10, 2), range(1, 10, 2)))
             + _inner_group(range(10, 16), range(5), _PAIRS65))
    row = lambda t: max(i for _, i, _ in t[0])
    unit = lambda t: max(2 * i + h for _, i, h in t[0])
    need = lambda t: unit(t) if row(t) == 15 else 2 * row(t) + 1
    return [(need(t), t) for t in sorted(prods, key=need)]


_O_JOBS = _o_jobs()


SB = 4


class _Star:
    def __init__(self, ts):
        self.ts, self.n = ts, len(ts)
        rn = range(self.n)
        self.pairs = [(i, j) for i in rn for j in rn if i < j]
        self.pf = {f: m for m, f in enumerate([('R', i) for i in rn] + [('C', i) for i in rn]
                                              + [('S', i, j) for i in rn for j in rn if i != j]
                                              + [('A', i, j) for i, j in self.pairs])}
        self.vf = {f: m for m, f in enumerate([('W', i) for i in rn]
                                              + [(q, i, j) for i, j in self.pairs for q in ('Q1', 'Q2', 'Q3')])}
        self.pv = {**{('W', i): ('R', i) for i in rn}, **{('B', i): ('C', i) for i in rn},
                   **{('Q1', i, j): ('S', i, j) for i, j in self.pairs},
                   **{('Q2', i, j): ('A', i, j) for i, j in self.pairs},
                   **{('Q3', i, j): ('S', j, i) for i, j in self.pairs}}

    def products(self, i):
        return [('W', i), ('B', i)] + [(q, i, j) for j in range(i + 1, self.n) for q in ('Q1', 'Q2', 'Q3')]


_FULL = _Star((-1.125, -0.375, 0.375, 1.125))
_HALF = _Star((-0.75, 0.75))
_DCELLS = [(0, 0), (1, 0), (1, 1), (2, 2), (3, 2), (3, 3)]
_HSLOT = (SB - 1) * len(_FULL.pf)
_DSLOT = _HSLOT + len(_HALF.pf)
_VSLOT = _DSLOT + len(_DCELLS)
_VHALF = (SB - 1) * len(_FULL.vf)
_FENCE = _VSLOT + (_VHALF + SB * len(_HALF.vf) + 1) // 2


def _v_slot(star, J, f):
    m = star.vf[f] + J * len(star.vf) + (0 if star is _FULL else _VHALF)
    return _VSLOT + m // 2, m % 2 * (T // 2)


def _v_form_items(v_scr, pf, J):
    n, HT = 16, T // 2

    def item(star, h, r0, pairs):
        def fn(dep):
            ts = [jnp.full((8, T), t, F32) for t in star.ts]
            ts = [_rows(t if dep is None else _after(t, dep), n) for t in ts]

            def get(k, a):
                r = (a * HT + r0) // 2
                return _ld(v_scr, 2 * (SB * J + k) + h, slice(r, r + n // 2)).astype(F32)

            def put(f, v):
                slot, r = _v_slot(star, J, f)
                pf[h][slot, r + r0:r + r0 + n, :] = v.astype(BF16)

            b = {(k, a): get(k, a) for k in sorted({k for pr in pairs or star.pairs for k in pr})
                 for a in range(2)}
            if pairs is None or star.n == 2:
                w = [b[k, 0] + ts[k] * b[k, 1] for k in range(star.n)]
                for k in range(star.n):
                    put(('W', k), w[k])
                for i, j in star.pairs:
                    put(('Q2', i, j), w[i] - w[j])
            for i, j in pairs or ():
                d0, d1 = b[j, 0] - b[i, 0], b[j, 1] - b[i, 1]
                put(('Q1', i, j), d0 + ts[i] * d1)
                put(('Q3', i, j), d0 + ts[j] * d1)
        return fn

    pr = _FULL.pairs
    parts = [(_HALF, _HALF.pairs)]
    if J < SB - 1:
        parts += [(_FULL, x) for x in (None, pr[:2], [pr[2], pr[4]], [pr[3], pr[5]])]
    return [item(star, h, r0, pairs) for h in range(2) for r0 in range(0, HT, n) for star, pairs in parts]


def _job_order(nsb):
    units = [(I, h) for I in range(nsb) for h in range(2)]
    qe, qv = [], []
    for I, h in units:
        es = [('e', I, h, J, p) for J in range(I) for p in range(SB)]
        ds = [('d', I, h) + c for c in _DCELLS]
        es.insert(max(len(es) - FPOS, 0), ('f', I, h))
        qe += es + ds if I or FPOS < 9 else ds[:DPOS] + es + ds[DPOS:]
        for i in range(SB):
            qv += [('p', I, h, f, J) for f in _FULL.products(i) for J in range(I)]
            if i >= 2:
                qv += [('p', I, h, f, None) for f in _HALF.products(i - 2)]
            qv += [('v', I, h) + c for c in _DCELLS if c[0] == i]
    qo = [('o', u, j) for j, (u, _) in enumerate(_O_JOBS)]
    cost = dict(e=8, f=8, d=2, p=1, v=2, o=2)
    order, done = [], {}
    now = [0]

    def emit(q):
        job = q.pop(0)
        order.append(job)
        now[0] += cost[job[0]]
        if job[0] == 'd':
            done[job] = now[0]
        elif job[0] == 'v' and job[4] == job[3]:
            done['u', 2 * (SB * job[1] + job[3]) + job[2]] = now[0]
        return cost[job[0]]

    def v_ready():
        if not qv:
            return False
        key = ('d', qv[0][1], qv[0][2], SB - 1, SB - 1)
        return key in done and done[key] + (LAT_0 if qv[0][1:3] == (0, 0) else LAT_A) <= now[0]

    def o_ready():
        return bool(qo) and ('u', qo[0][1]) in done and done['u', qo[0][1]] + LAT_B <= now[0]

    def fill(nv, no):
        n = 0
        while nv > 0 or no > 0 or n % 4:
            if no > 0 and n % 2 == 0 and o_ready() and no * ONV >= nv:
                no -= 2
                n += emit(qo)
            elif v_ready() and (nv > 0 or n % 4):
                c = emit(qv)
                nv -= c
                n += c
            elif o_ready() and n % 2 == 0 and (no > 0 or n % 4 or nv > 0) and len(qo) > RES:
                no -= 2
                n += emit(qo)
            else:
                break

    while qe:
        unit = qe[0][1:3]
        while qv and qv[0][2] == unit[1] and qv[0][1] < unit[0]:
            emit(qv)
        ne = 0
        while qe and ne < 8 and (ne == 0 or (qe[0][0] == 'd' and qe[0][1:3] == unit and ne + 2 <= 8)):
            ne += emit(qe)
        groups = lambda q: sum(cost[j[0]] for j in q) / 8
        old = [j for j in qv if j[1:3] != unit and ('d', j[1], j[2], SB - 1, SB - 1) in done]
        here = [j for j in qe if j[1:3] == unit]
        rest = sum(cost[j[0]] for j in old)
        nv = (rest - LAT_A) / (groups(here) + 1) if here else rest
        no = 2 * max(len(qo) - RES - OEND, 0) / (groups(qe) + 1)
        fill(int(nv + 0.5), int(no + 0.5))
    while qv or qo:
        if qv and v_ready():
            fill(6, 2)
            if not qv:
                continue
        elif o_ready():
            emit(qo)
        else:
            emit(qv or qo)
    return order


def _attention_safe(q_scr, k_scr, v_scr, wo_ref, acc_scr):
    causal = (jax.lax.broadcasted_iota(jnp.int32, (T, T), 0)
              <= jax.lax.broadcasted_iota(jnp.int32, (T, T), 1))

    def unit(u, carry):
        r, hd = u // 2, u % 2

        def block(c, mlo):
            m0, l, o = mlo
            s = _dot_nt(_ld(k_scr, 2 * c + hd), _ld(q_scr, u))
            s = jnp.where(jnp.logical_or(causal, c < r), s, -1e9 * LOG2E)
            m = jnp.maximum(m0, jnp.max(s, axis=0, keepdims=True))
            a = jnp.exp2(m0 - m)
            p = jnp.exp2(s - m)
            return (m, l * a + jnp.sum(p, axis=0, keepdims=True),
                    o * a + _dot(_ld(v_scr, 2 * c + hd), p.astype(BF16)))

        _, l, o = jax.lax.fori_loop(0, r + 1, block, (jnp.full((1, T), -jnp.inf, F32), jnp.zeros((1, T), F32),
                                                      jnp.zeros((T, T), F32)))
        rows = pl.ds(pl.multiple_of(r * T, T), T)
        acc_scr[rows, :] += _dot((o * (1.0 / l)).astype(BF16).T, wo_ref[pl.ds(pl.multiple_of(hd * T, T), T), :])
        return carry

    jax.lax.fori_loop(0, q_scr.shape[0], unit, 0)


def _attention_step(q_scr, k_scr, v_scr, pf, wo_ref, acc_scr, flag_scr, z, side):
    causal = (jax.lax.broadcasted_iota(jnp.int32, (T, T), 0)
              <= jax.lax.broadcasted_iota(jnp.int32, (T, T), 1))
    HT = T // 2
    lsum, lrow, acc, fg, dacc, of, lhs = {}, {}, {}, {}, {}, {}, {}
    res = []
    wo, terms = {}, {}
    left = {}
    done_side = [0, 0]
    chk = [jnp.zeros((8, T), F32), None]
    for _, t in _O_JOBS:
        for _, i, j in t[2]:
            left[i, j] = left.get((i, j), 0) + 1

    def add_l(u, v):
        lsum[u] = v if u not in lsum else lsum[u] + v

    csign = {}

    def p_forms(star, h, slot0, g, tiles, cell, when):
        n = star.n

        def put(f, v):
            pf[h][slot0 + star.pf[f], 16 * g:16 * g + 16, :] = v.astype(BF16)

        for i in range(n):
            row = [cell(i, k) for k in sorted(range(n), key=lambda k: when(i, k))]
            r = functools.reduce(lambda x, y: x + y, row)
            put(('R', i), r)
            add_l(tiles[i], r[:8] + r[8:])
            col = sorted(range(n), key=lambda i2: (when(i2, i), i2 != i))
            sign = csign[n, i] = 1 if col[0] == i else -1
            c = cell(col[0], i)
            for i2 in col[1:]:
                c = c + cell(i2, i) if (1 if i2 == i else -1) == sign else c - cell(i2, i)
            put(('C', i), c)
            for j in range(n):
                if j != i:
                    put(('S', i, j), cell(i, j))
        for i, j in star.pairs:
            put(('A', i, j), cell(i, j) + cell(j, i))

    due = []

    def scores(x, u):
        if due and due[0][0] <= done_side[1]:
            x = _tie(x, due.pop(0)[1])
        s = (_dot if u in QT else _dot_nt)(x, _ld(q_scr, u))
        res.append(s)
        return s

    def job_e(I, h, J, p):
        tiles = [2 * (SB * I + i) + h for i in range(SB)]
        ps = []
        for i, u in enumerate(tiles):
            x = jnp.concatenate([k_scr.bitcast(U32)[2 * (SB * J + (t - i) % SB) + h, 8 * g:8 * g + 8, :]
                                 for g in (2 * p, 2 * p + 1) for t in range(SB)], axis=0)
            ps.append(jnp.exp2(scores(pltpu.bitcast(x, BF16), u)))
        when = lambda i, k: (i + k) % SB
        for n, g in enumerate((2 * p, 2 * p + 1)):
            cell = lambda i, k: ps[i][16 * (SB * n + when(i, k)):16 * (SB * n + when(i, k)) + 16]
            p_forms(_FULL, h, J * len(_FULL.pf), g, tiles, cell, when)

    def job_f(I, h):
        tiles = [2 * (SB * I + 2 + i) + h for i in range(2)]
        ps = {(i, k): jnp.exp2(scores(_ld(k_scr, 2 * (SB * I + k) + h), u))
              for i, u in enumerate(tiles) for k in range(2)}
        for g in range(T // 16):
            p_forms(_HALF, h, _HSLOT, g, tiles, lambda i, k: ps[i, k][16 * g:16 * g + 16], lambda i, k: 0)

    def job_d(I, h, i, k):
        u = 2 * (SB * I + i) + h
        s = scores(_ld(k_scr, 2 * (SB * I + k) + h), u)
        if i == k:
            s = jnp.where(causal, s, -1e9 * LOG2E)
        p = jnp.exp2(s)
        add_l(u, jnp.sum(p.reshape(T // 8, 8, T), axis=0))
        pf[h][_DSLOT + _DCELLS.index((i, k))] = p.astype(BF16)
        if (i, k) == _DCELLS[-1]:
            pf[h][_FENCE + z, 0:16, :] = jnp.zeros((16, T), BF16)
            for u in [2 * (SB * I + a) + h for a in range(SB)]:
                lrow[u] = jnp.sum(lsum.pop(u), axis=0, keepdims=True)
            ls = [lrow[2 * (SB * I + a) + h] for a in range(SB)]
            lo = jnp.minimum(jnp.minimum(ls[0], ls[1]), jnp.minimum(ls[2], ls[3]))
            hi = jnp.maximum(jnp.maximum(ls[0], ls[1]), jnp.maximum(ls[2], ls[3]))
            ok = jnp.logical_and(lo >= L_LO, hi <= L_HI)
            ok = jnp.logical_and(ok, (hi if I else jnp.maximum(ls[2], ls[3]))
                                 <= L_RATIO * (lo if I else jnp.minimum(ls[2], ls[3])))
            bad = jnp.where(ok, 0.0, 1.0)
            chk[1] = bad if chk[1] is None else jnp.maximum(chk[1], bad)

    def job_p(I, h, f, J):
        star, last = (_HALF, True) if J is None else (_FULL, J == I - 1)
        blk = I if J is None else J
        if f[0] == 'B':
            x = _ld(v_scr, 2 * (SB * blk + f[1]) + h, slice(HT // 2, HT))
        else:
            slot, r = _v_slot(star, blk, f)
            x = _ld(pf[h], slot, slice(r // 2, (r + HT) // 2))
        v = _dot(x, _ld(pf[h], (_HSLOT if J is None else J * len(_FULL.pf)) + star.pf[star.pv[f]]))
        res.append(v)
        key = (star.n,) + f
        acc[key] = v if key not in acc else acc[key] + v
        if not last:
            return

        def add(which, i, v, sign=1):
            k_ = (star.n, which, i)
            if k_ not in fg:
                fg[k_] = v if sign > 0 else -v
            else:
                fg[k_] = fg[k_] + v if sign > 0 else fg[k_] - v

        if f[0] == 'W':
            add('F', f[1], acc.pop(key))
        elif f[0] == 'B':
            add('G', f[1], acc.pop(key), csign[star.n, f[1]])
        elif f[0] == 'Q3':
            _, i, j = f
            q1, q2, q3 = (acc.pop((star.n, q, i, j)) for q in ('Q1', 'Q2', 'Q3'))
            t = ((q1 + q2) + q3) * (1.0 / (star.ts[i] - star.ts[j]))
            add('G', i, t)
            add('G', j, t)
            add('F', i, q1)
            add('F', j, q3, -1)

    def job_v(I, h, i, k):
        u = 2 * (SB * I + i) + h
        v = _dot(_ld(v_scr, 2 * (SB * I + k) + h), _ld(pf[h], _DSLOT + _DCELLS.index((i, k))))
        res.append(v)
        dacc[u] = v if u not in dacc else dacc[u] + v
        if k == i:
            o = dacc.pop(u)
            for star, a in ([(_FULL, i)] if I else []) + ([(_HALF, i - 2)] if i >= 2 else []):
                f, g = fg.pop((star.n, 'F', a)), fg.pop((star.n, 'G', a))
                o = o + jnp.concatenate([f - star.ts[a] * g, g], axis=0)
            o = o * (1.0 / lrow[u])
            of[u] = o
            chk[0] = chk[0] + jnp.sum(o.reshape(T // 8, 8, T), axis=0)

    def job_o(_, n):
        af, bf, outs = _O_JOBS[n][1]
        if af not in lhs:
            v = _form(af, lambda i, h: of[2 * i + h])
            lhs[af] = _tie(v.astype(BF16).T, v[0:8, :])
        if bf not in wo:
            wo[bf] = (wo_ref[_tile(bf[0][1]), _tile(bf[0][2])] if len(bf) == 1 else
                      _form(bf, lambda h, j: wo_ref[_tile(h), _tile(j)].astype(F32)).astype(BF16))
            if HACKWO:
                wo[bf] = _ld(q_scr, len(wo) % 32)
        v = _dot(lhs[af], wo[bf])
        res.append(v)
        for sign, i, j in outs:
            terms.setdefault((i, j), []).append((sign, v))
            if len(terms[i, j]) == left[i, j]:
                tot = acc_scr[_tile(i), _tile(j)]
                for sg, m in terms.pop((i, j)):
                    tot = tot + m if sg > 0 else tot - m
                acc_scr[_tile(i), _tile(j)] = tot

    fns = dict(e=job_e, f=job_f, d=job_d, p=job_p, v=job_v, o=job_o)
    order = _job_order(q_scr.shape[0] // (2 * SB))
    for n, job in enumerate(order):
        assert job[0] not in 'efd' or not any(j[0] in 'pv' and j[2] == job[2] and j[1] < job[1] for j in order[n:])
    side = list(side)
    fences = [n for n, job in enumerate(order) if job[0] == 'd' and job[3:] == _DCELLS[-1]]
    step = (len(order) - SIDE0 - SIDE1 - 10) / len(side)
    for n, job in enumerate(order):
        done_side[1] = n
        fns[job[0]](*job[1:])
        last_chance = n >= len(order) - SIDE1
        near = any(-SG1 <= f - n <= SG0 for f in fences)
        if side and n >= SIDE0 + step * done_side[0] and ((job[0] in SKIND and not near) or last_chance):
            done_side[0] += 1
            v = side.pop(0)(res[-1 - SLAG][8 * (n % 4):8 * (n % 4) + 8, :])
            if v is not None:
                due.append((n + SDUE, v))
    assert not side and not due
    fine = jnp.abs(chk[0]) < jnp.inf
    flag_scr[...] = jnp.maximum(flag_scr[...], jnp.where(fine, chk[1], 1.0))


def _kernel(x_hbm, c_hbm, wq_hbm, wuk_hbm, wuv_hbm, wo_hbm, w1_hbm, w2_hbm, w3_hbm, w4_hbm,
            cond_hbm, wmod_hbm, out_hbm,
            x_ref, c_ref, cond_ref, wma_ref, wmb_ref, w1_ref, w3_ref,
            wq_buf, wk_buf, wv_buf, wo_buf, out_buf, sem, wsem, osem,
            mod_scr, h_scr, cs_scr, hs_scr, w_scr, q_scr, k_scr, v_scr, acc_scr, xn_scr, xh_scr, a1_scr, t_scr,
            z_scr, mw_scr, m3_scr, wt_scr, wf_scr, gap_scr, st_in, pf_scr, vf_scr, flag_scr):
    S, M = x_hbm.shape
    D = wq_hbm.shape[2]
    nattn = wo_hbm.shape[0]
    Fd = w4_hbm.shape[0]
    scale = float(D) ** -0.5 * LOG2E
    nb, nrb = S // T, S // RB
    km, kc = M // T, c_hbm.shape[1] // T
    NX = 4
    XR = S // NX
    CB = XR // T

    work = (wk_buf, wv_buf, wq_buf)

    def pcopies(g, bufs=work, s0=0):
        return [pltpu.make_async_copy(src.bitcast(U32).at[:, g, :], dst, wsem.at[s0 + j])
                for j, (src, dst) in enumerate(zip((wuk_hbm, wuv_hbm, wq_hbm), bufs))]

    def ocopy(g):
        return pltpu.make_async_copy(wo_hbm.at[g], wo_buf, wsem.at[3])

    def chunk_copy(src, dst, i, s0):
        rows = slice(i * XR, (i + 1) * XR)
        return pltpu.make_async_copy(src.at[rows, :], dst.at[rows, :], sem.at[s0 + i])

    MS = 16
    NSL = T // MS
    assert nattn - 1 >= NSL
    mixw = ((w1_hbm, km, 0), (w2_hbm, km, km * MS), (w3_hbm, Fd // T, 2 * km * MS),
            (w4_hbm, -(-Fd // T), (2 * km + Fd // T) * MS))

    def prep_in(g):
        o = jnp.minimum(g, NSL - 1) * MS
        return [pltpu.make_async_copy(
            w.at[pl.ds(pl.multiple_of(jnp.minimum(b * T + o, w.shape[0] - MS), MS), MS), :],
            st_in.at[r0 + b * MS:r0 + (b + 1) * MS, :], wsem.at[7]) for w, nblk, r0 in mixw for b in range(nblk)]

    def stage_in(g):
        return pcopies(jnp.minimum(g + 1, nattn - 1))

    cp_cond = pltpu.make_async_copy(cond_hbm, cond_ref, sem.at[0])
    cp_wma = pltpu.make_async_copy(wmod_hbm.at[:, 0:2 * M], wma_ref, sem.at[1])
    cp_late = [pltpu.make_async_copy(src, dst, sem.at[2 + j]) for j, (src, dst) in enumerate((
        (wmod_hbm.at[:, 2 * M:6 * M], wmb_ref), (w1_hbm, w1_ref), (w3_hbm.at[Fd // T * T:, :], w3_ref)))]
    cp_x = [chunk_copy(x_hbm, x_ref, i, 7) for i in range(NX)]
    cp_c = [chunk_copy(c_hbm, c_ref, i, 7 + NX) for i in range(NX)]

    def silu_cond():
        cf = cond_ref[...].astype(F32)
        return jnp.broadcast_to((cf * jax.nn.sigmoid(cf)).astype(BF16), (8, M))

    cp_wk, cp_wv, cp_wq = pcopies(0)
    named = dict(k=cp_wk, v=cp_wv, q=cp_wq, o=ocopy(0), n=cp_cond, m=cp_wma)
    named.update(zip('abcd', cp_c))
    named.update(zip('wxyz', cp_x))
    started, arrived, did = set(), set(), set()

    def zero(r, carry):
        acc_scr[pl.ds(pl.multiple_of(r * T, T), T), :] = jnp.zeros((T, M), F32)
        return carry

    def x_rows(rows, dep):
        xf = x_ref[rows, :].astype(F32)
        if dep is None:
            return xf
        return jnp.concatenate([_after(xf[:, :T], _rows(dep, xf.shape[0])), xf[:, T:]], axis=1)

    def n_item(r, i):
        def fn(dep):
            rows = slice(r * T + i * LP, r * T + (i + 1) * LP)
            xn_scr[rows, :] = _ln(x_rows(rows, dep))
        return fn

    def h_item(r, i, normed):
        def fn(dep):
            rows = slice(i * LP, (i + 1) * LP)
            grows = slice(r * T + i * LP, r * T + (i + 1) * LP)
            sa = mod_scr[:, 0:M]
            if normed and dep is not None:
                sa = jnp.concatenate([_after(sa[:, _tile(j)], dep) for j in range(km)], axis=1)
            hf = ((xn_scr[grows, :] if normed else _ln(x_rows(grows, dep))) * _rows(mod_scr[:, M:2 * M], LP)
                  + _rows(sa, LP))
            for j in range(km):
                h_scr[r, j, rows, :] = hf[:, _tile(j)].astype(BF16)
            for f, n in _H_SUMS.items():
                if all(t[1] == r for t in f):
                    hs_scr[n, rows, :] = _form(f, lambda _, k: hf[:, _tile(k)]).astype(BF16)
            did.add(('h', r, i))
        return fn

    def release(jobs, span, items):
        if span and items:
            jobs.side += [(len(jobs.res) + 1 + i * span // len(items), fn) for i, fn in enumerate(items)]
            jobs.side.sort(key=lambda e: e[0])
        else:
            for fn in items:
                fn(None)

    def sum_items(n, group, index, dst, get, skip_rows):
        forms = [f for f in dict.fromkeys(t[0] for t in group)
                 if len(f) > 1 and not (skip_rows and len({t[1] for t in f}) == 1)]

        def item(f, rows):
            def fn(dep):
                def term(r, k):
                    v = get(r, k, rows).astype(F32)
                    return v if dep is None or (r, k) != f[0][1:] else _after(v, _rows(dep, v.shape[0]))
                dst[index[f], rows, :] = _form(f, term).astype(BF16)
            return fn

        return [item(f, slice(i, i + n)) for i in range(0, T, n) for f in forms]

    h_sums = lambda n, gi: sum_items(n, _H_GROUPS[gi], _H_SUMS, hs_scr,
                                     lambda r_, k, rows: h_scr[r_, k, rows, :], True)

    def stash(key, buf, j0, transpose=False):
        n = buf.shape[0] // T
        if key not in did:
            assert key in arrived
            did.add(key)
            for (j, hd), w in _pair_tiles(buf, transpose).items():
                w_scr[hd, j0 + j] = w
        return lambda hd: [_ld(w_scr, hd, j0 + j) for j in range(n)]

    def kv_tile(jobs, r):
        wk, wvT = stash('k', wk_buf, 0), stash('v', wv_buf, kc, True)
        ct = [c_ref[_tile(r), _tile(j)] for j in range(kc)]
        for hd in range(2):
            k_scr[2 * r + hd] = jobs.mm(ct, wk(hd), _dot).astype(BF16)
        for hd in range(2):
            v_scr[2 * r + hd] = jobs.mm(wvT(hd), ct, _dot_nt).astype(BF16)

    def q_tile(jobs, r):
        wq = stash('q', wq_buf, 2 * kc)
        ht = [_ld(h_scr, r, j) for j in range(km)]
        for hd in range(2):
            v = (jobs.mm(ht, wq(hd), _dot) * scale).astype(BF16)
            q_scr[2 * r + hd] = v.T if 2 * r + hd in QT else v

    for blk in _prologue().split(';'):
        waits, starts, acts = blk.split('|')
        for ch in waits.strip():
            assert ch in started and ch not in arrived
            arrived.add(ch)
            named[ch].wait()
        for ch in starts.strip():
            assert ch not in started
            started.add(ch)
            named[ch].start()
        jobs = _Jobs()
        for act in acts.split():
            if act == 'Z':
                jax.lax.fori_loop(0, nb, zero, 0)
                acc_scr[S:, :] = jnp.zeros((acc_scr.shape[0] - S, M), F32)
                x_ref[S:, :] = jnp.zeros((x_ref.shape[0] - S, M), BF16)
                flag_scr[...] = jnp.zeros(flag_scr.shape, F32)
            elif act == 'L':
                did.add('L')
                assert ('Q', 0) in did
                for cp in stage_in(0) + prep_in(0):
                    cp.start()
            elif act == 'M':
                assert arrived >= set('nm')
                mod = _dot(silu_cond(), wma_ref[...])
                mod_scr[:, 0:M] = mod[:, 0:M]
                mod_scr[:, M:2 * M] = 1.0 + mod[:, M:2 * M]
                did.add('M')
            else:
                act, _, span = act.partition('@')
                span = int(span or 0)
                items = []
                for r in [int(ch, 16) for ch in act[1:]]:
                    did.add((act[0], r))
                    if act[0] == 'K':
                        assert 'abcd'[r // CB] in arrived
                        kv_tile(jobs, r)
                    elif act[0] == 'H':
                        assert 'wxyz'[r // CB] in arrived and 'M' in did
                        items += [h_item(r, i, ('N', r) in did) for i in range(T // LP)]
                    elif act[0] == 'N':
                        assert 'wxyz'[r // CB] in arrived
                        items += [n_item(r, i) for i in range(T // LP)]
                    elif act[0] == 'Q':
                        assert all(('h', r, i) in did for i in range(T // LP))
                        q_tile(jobs, r)
                    elif act[0] == 'F':
                        assert all(('K', SB * r + k_) in did for k_ in range(SB))
                        items += _v_form_items(v_scr, (pf_scr, vf_scr), r)
                    elif act[0] == 'C':
                        assert all('abcd'[t[1] // CB] in arrived for p_ in _C_GROUPS[r] for t in p_[0])
                        items += sum_items(
                            32, _C_GROUPS[r], _C_SUMS, cs_scr,
                            lambda r_, k, rows: c_ref[r_ * T + rows.start:r_ * T + rows.stop, _tile(k)], False)
                    else:
                        assert act[0] == 'S' and all(('h', t[1], T // LP - 1) in did for p_ in _H_GROUPS[r] for t in p_[0])
                        items += h_sums(32 if span else 16, r)
                release(jobs, span, items)
        assert not jobs.side
    assert arrived == set(named) and all((k_, r) in did for k_ in 'KHQ' for r in range(nb))
    assert all((k_, r) in did for k_ in 'CS' for r in range(2)) and 'L' in did
    assert all(('F', r) in did for r in range(SB))

    def mixer_prep(g):
        sl = jnp.minimum(g, NSL - 1)
        rows = pl.ds(pl.multiple_of(sl * MS, MS), MS)

        def part(m, forms):
            def fn(dep):
                base = {}

                def get(i, k):
                    if (i, k) not in base:
                        rb, cb = (i, k) if m == 2 else (k, i)
                        r0 = mixw[m][2] + rb * MS
                        v = _after(st_in[r0:r0 + MS, _tile(cb)].astype(F32), _rows(dep, MS))
                        if m == 3 and (rb + 1) * T > Fd:
                            v = jnp.where(rb * T + sl * MS < Fd, v, 0.0)
                        base[i, k] = v
                    return base[i, k]

                for f in forms:
                    v = _form(f, get)
                    mw_scr[_MIXW[m, f], rows, :] = (0.5 * v if m % 2 else v).astype(BF16)
            return fn

        items = []
        for m in range(4):
            forms = [f for mm_, f in _MIXW if mm_ == m]
            cur, terms = [], set()
            for f in forms:
                new_terms = terms | {t[1:] for t in f}
                if cur and 3 * len(new_terms) + sum(2 * len(x) + 1 for x in cur + [f]) > MWOPS:
                    items.append(part(m, cur))
                    cur, terms = [], set()
                cur.append(f)
                terms |= {t[1:] for t in f}
            items.append(part(m, cur))

        n3 = sum(m == 2 for m, _ in _MIXW)
        first = min(n for (m, _), n in _MIXW.items() if m == 2)
        per = -(-n3 // (nattn - 1 - NSL))

        def turn(j):
            def fn(dep):
                n = jnp.minimum(jnp.maximum(g - NSL, 0) * per + j, n3 - 1)
                w = _tie(_ld(mw_scr, first + n), dep).T
                m3_scr[n] = w
                return pltpu.bitcast(pltpu.bitcast(w, U32)[T // 2 - 8:], F32)
            return fn

        return items + [turn(j) for j in range(per)]

    def stage_wait():
        for cp in pcopies(0):
            cp.wait()
        pltpu.make_async_copy(st_in, st_in, wsem.at[7]).wait()

    def attn_body(g, carry):
        side = _gap_items(work, gap_scr) + _weight_form_items(work, gap_scr, wt_scr, wf_scr, (0, 1, 2))
        bufs = (q_scr, k_scr, v_scr, (pf_scr, vf_scr), wo_buf, acc_scr, flag_scr)
        _attention_step(*bufs, g >> 16, side)

        @pl.when(g + 1 < nattn)
        def _():
            copies = stage_in(g + 1) + [ocopy(g + 1)]
            for cp in copies:
                cp.start()
            bufs = (h_scr, hs_scr, c_ref, cs_scr, wf_scr, q_scr, k_scr, v_scr, (pf_scr, vf_scr))
            side = [(SD0 + int(i * SDS), fn) for i, fn in enumerate(mixer_prep(g))]
            _proj_step(*bufs, scale, gap_scr, side)
            for cp in prep_in(g + 1):
                cp.start()
            stage_wait()
            ocopy(g + 1).wait()

        return carry

    stage_wait()
    for cp in cp_late:
        cp.start()
    jax.lax.fori_loop(0, nattn, attn_body, 0)

    def safe_pair(g, carry):
        copies = pcopies(g) + [ocopy(g)]
        for cp in copies:
            cp.start()
        for cp in copies:
            cp.wait()
        for buf, j0, transpose in ((wk_buf, 0, False), (wv_buf, kc, True), (wq_buf, 2 * kc, False)):
            for (j, hd), w in _pair_tiles(buf, transpose).items():
                w_scr[hd, j0 + j] = w

        def tile(u, carry):
            r, hd = u // 2, u % 2
            rows = pl.ds(pl.multiple_of(r * T, T), T)
            ct = [c_ref[rows, _tile(j)] for j in range(kc)]
            k_scr[u] = sum(_dot(ct[j], _ld(w_scr, hd, j)) for j in range(kc)).astype(BF16)
            v_scr[u] = sum(_dot_nt(_ld(w_scr, hd, kc + j), ct[j]) for j in range(kc)).astype(BF16)
            q = sum(_dot(_ld(h_scr, r, j), _ld(w_scr, hd, 2 * kc + j)) for j in range(km))
            q_scr[u] = (q * scale).astype(BF16)
            return carry

        jax.lax.fori_loop(0, 2 * nb, tile, 0)
        _attention_safe(q_scr, k_scr, v_scr, wo_buf, acc_scr)
        return carry

    @pl.when(jnp.max(flag_scr[...]) > 0)
    def _():
        jax.lax.fori_loop(0, nb, zero, 0)
        jax.lax.fori_loop(0, nattn, safe_pair, 0)

    for cp in cp_late:
        cp.wait()
    mod = _dot(silu_cond(), wmb_ref[...])
    mod_scr[:, 2 * M:4 * M] = mod[:, 0:2 * M]
    mod_scr[:, 4 * M:5 * M] = 1.0 + mod[:, 2 * M:3 * M]
    mod_scr[:, 5 * M:6 * M] = mod[:, 3 * M:4 * M]
    OFF = x_ref.shape[0] - S
    CAR = t_scr.shape[0] - RB

    def p1(r0, l0, n, dep=None):
        ga = mod_scr[:, 2 * M:3 * M]
        if dep is not None:
            ga = jnp.concatenate([_after(ga[:, 0:T], dep), ga[:, T:]], axis=1)
        rows = pl.ds(r0, n)
        x1 = x_ref[rows, :].astype(F32) + _rows(ga, n) * acc_scr[rows, :]
        xh_scr[0, l0:l0 + n, :] = x1
        hb = _ln(x1) * _rows(mod_scr[:, 4 * M:5 * M], n) + _rows(mod_scr[:, 3 * M:4 * M], n)
        xh_scr[1, l0:l0 + n, :] = hb
        return hb

    HT = T // 2
    last8 = lambda v: jnp.max(v[:, M - T:].reshape(PC // 8, 8, T), axis=0)

    def p1_store(r0, c, dep=None):
        v = _ln(p1(r0 + c * PC, OFF + c * PC, PC, dep))
        a1_scr[c * PC:(c + 1) * PC, :] = v
        return last8(v)

    def p1_first(r0, c, dep):
        return last8(p1(r0 + c * PC, OFF + c * PC, PC, dep))

    def p1_second(c, dep):
        hb = xh_scr[1, OFF + c * PC:OFF + (c + 1) * PC, :]
        v = _ln(jnp.concatenate([_after(hb[:, :T], _rows(dep, PC)), hb[:, T:]], axis=1))
        a1_scr[c * PC:(c + 1) * PC, :] = v
        return last8(v)

    t_scr[RB:RB + CAR - OFF, :] = jnp.zeros((CAR - OFF, M), F32)
    t_scr[RB + CAR - OFF:RB + CAR, :] = _gelu2(_dot(_ln(p1(0, 0, OFF)).astype(BF16), w1_ref[...]))
    for c in range(RB // PC):
        p1_store(OFF, c)

    def out_copy(i):
        rows = pl.ds(i * T if isinstance(i, int) else pl.multiple_of(i * T, T), T)
        return pltpu.make_async_copy(out_buf.at[rows, :], out_hbm.at[rows, :], osem.at[i])

    def b_body(r, carry):
        gb = _rows(mod_scr[:, 5 * M:6 * M], T)
        r0 = pl.multiple_of(r * RB, RB)
        n0 = pl.multiple_of(jnp.minimum(r0 + RB, S - RB) + OFF, OFF)
        nh = RB // T
        now = [0]
        due = []
        pace = []

        def p1_item(c, part):
            def fn(dep):
                v = (p1_store(n0, c, dep) if not PSPLIT else p1_first(n0, c, dep) if part == 0 else p1_second(c, dep))
                due.append((now[0] + PD, v))
                due.sort(key=lambda e: e[0])
            return fn

        pace += [(P0 + i * PSTEP + part * PSPLIT, p1_item(i, part)) for i in range(RB // PC)
                 for part in range(2 if PSPLIT else 1)]
        pace.sort(key=lambda e: e[0])

        def mm(lhs, wts, dot=_dot):
            acc = None
            for x, w in zip(lhs, wts):
                if due and due[0][0] <= now[0]:
                    w = _tie(w, due.pop(0)[1])
                v = dot(x, w)
                now[0] += x.shape[0] / HT
                acc = v if acc is None else v + acc
                if pace and pace[0][0] <= now[0]:
                    pace.pop(0)[1](v[0:8, :])
            return acc

        def fast(m, base, finish, hook=None):
            prods = _MIX[m]
            nsub = MSUB[m]
            n = HT // nsub
            done = {}
            for sub in range(nsub):
                left, acc, cache = {}, {}, {}
                for _, _, outs in prods:
                    for _, i, h in outs:
                        left[i, h] = left.get((i, h), 0) + 1

                def act(form):
                    sign, form = _canon(form)
                    if form not in cache:
                        cache[form] = _form(
                            form, lambda k, h: base(k)[h * HT + sub * n:h * HT + (sub + 1) * n]).astype(BF16)
                    return sign, cache[form]

                for pi, (wf, af, outs) in enumerate(prods):
                    w = _ld(m3_scr, _MIXW[m, wf] - _MIX3) if m == 2 else _ld(mw_scr, _MIXW[m, wf])
                    if af is None:
                        k = wf[0][2]
                        v = mm([jnp.concatenate([act(((1, k, h),))[1] for h in range(2)], axis=0)], [w])
                        sign, parts = 1, [v[:n], v[n:]]
                    else:
                        sign, x = act(af)
                        parts = [mm([x], [w])] * len(outs)
                    for (s_, i, h), v in zip(outs, parts):
                        s_ = s_ * sign
                        if (i, h) not in acc:
                            acc[i, h] = (s_, v)
                        else:
                            s0, u = acc[i, h]
                            acc[i, h] = (s0, u + v if s0 == s_ else u - v) if s0 > 0 or s_ < 0 else (1, v - u)
                        left[i, h] -= 1
                        if not left[i, h]:
                            s0, done[i, h, sub] = acc.pop((i, h))
                            assert s0 > 0
                            if all((i, hh, ss) in done for hh in range(2) for ss in range(nsub)):
                                finish(i, jnp.concatenate([done[i, hh, ss] for hh in range(2)
                                                           for ss in range(nsub)], axis=0))
                    if hook is not None and sub == nsub - 1:
                        hook(pi, act)

        t_scr[0:CAR, :] = t_scr[RB:RB + CAR, :]
        for hf in range(nh):
            def put_t(n, v):
                t = _gelu2(v)
                if hf == nh - 1:
                    t = jnp.concatenate([t[:T - OFF], jnp.where(r < nrb - 1, t[T - OFF:], 0.0)], axis=0)
                t_scr[CAR + hf * T:CAR + (hf + 1) * T, _tile(n)] = t

            fast(0, lambda k: a1_scr[_tile(hf), _tile(k)], put_t)
        cq = M // 4
        shifts = (-1, 1, -2, 2)
        lane = jax.lax.broadcasted_iota(jnp.int32, (T, T), 1)
        y1, a3 = [], []
        for hf in range(nh):
            base = CAR - OFF + hf * T
            sh = []
            for j in range(km):
                g_lo, g_hi = (j * T) // cq, ((j + 1) * T - 1) // cq
                assert g_hi - g_lo <= 1
                v = t_scr[base + shifts[g_lo]:base + shifts[g_lo] + T, _tile(j)]
                if g_hi != g_lo:
                    v2 = t_scr[base + shifts[g_hi]:base + shifts[g_hi] + T, _tile(j)]
                    v = jnp.where(lane < g_hi * cq - j * T, v, v2)
                else:
                    v = jnp.where(lane < T, v, 0.0)
                sh.append(v)
            hs = {}
            fast(1, lambda k: sh[k], hs.__setitem__)
            hs = jnp.concatenate([hs[n] for n in range(km)], axis=1)
            y1.append(hs + xh_scr[1, _tile(hf), :])
            z_scr[_tile(hf), :] = xh_scr[0, _tile(hf), :] + gb * y1[hf]
            a3.append({})

            def ln_item(hf, c):
                def item(dep):
                    n = HT // NLN
                    for d in (0, HT):
                        v = y1[hf][d + c * n:d + (c + 1) * n]
                        if dep is not None:
                            v = jnp.concatenate([_after(v[:, :T], _rows(dep, n)), v[:, T:]], axis=1)
                        a3[hf][d + c * n] = _ln(v)
                return item

            ln_item(hf, 0)(None)
            pace += [(now[0] + LN0 + (c - 1) * LNS * (1 + hf), ln_item(hf, c)) for c in range(1, NLN)]
            pace.sort(key=lambda e: e[0])
        xh_scr[:, 0:OFF, :] = xh_scr[:, RB:RB + OFF, :]
        z_scr[pl.ds(pl.multiple_of(RB + (r >> 16) * 8, 8), 8), :] = jnp.zeros((8, M), F32)
        h3 = []
        for hf in range(nh):
            assert len(a3[hf]) == 2 * NLN
            af = jnp.concatenate([a3[hf][key] for key in sorted(a3[hf])], axis=0)
            row = {}
            narrow = []

            def hook(pi, act):
                j, rem = divmod(pi - NAR0, NARS)
                if rem == 0 and 0 <= j < km:
                    full = jnp.concatenate([act(((1, j, h),))[1] for h in range(2)], axis=0)
                    v = mm([w3_ref[:, _tile(j)]], [full], _dot_nt)
                    narrow[:] = [v + narrow[0] if narrow else v]

            def put_h(n, v):
                row[n] = _gelu2(v)
                if GD:
                    due.append((now[0] + GD, jnp.max(row[n].reshape(T // 8, 8, T), axis=0)))
                    due.sort(key=lambda e: e[0])

            fast(2, lambda k: af[:, _tile(k)], put_h, hook)
            fw = w3_ref.shape[0]
            row[Fd // T] = jnp.concatenate([_gelu2(narrow[0]), jnp.zeros((T - fw, T), F32)], axis=0).T
            h3.append(row)
        for hf in range(nh):
            rows = pl.ds(pl.multiple_of(r0 + hf * T, T), T)

            def finish(n, v):
                out_buf[rows, _tile(n)] = (z_scr[_tile(hf), _tile(n)] + gb[:, _tile(n)] * v).astype(out_buf.dtype)

            fast(3, lambda k: h3[hf][k], finish)
            out_copy(r * nh + hf).start()
        assert not pace
        return carry

    jax.lax.fori_loop(0, nrb, b_body, 0)
    for i in range(nb):
        out_copy(i).wait()


@jax.jit
def pallas_adaLN_cond__compressed_kv_cla__mixer_s_mlp__prompt_kernel(
    A_x: jax.Array,
    A_c_kv: jax.Array,
    A_w_q: jax.Array,
    A_w_uk: jax.Array,
    A_w_uv: jax.Array,
    A_w_o: jax.Array,
    B_x: jax.Array,
    B_w1: jax.Array,
    B_w2: jax.Array,
    B_w3: jax.Array,
    B_w4: jax.Array,
    c: jax.Array,
    w_mod: jax.Array,
):
    _, S, M = A_x.shape
    Dc = A_c_kv.shape[2]
    H, D = A_w_q.shape[1], A_w_q.shape[2]
    Fd = B_w3.shape[1]
    assert D == T and A_c_kv.shape[1] == S and Dc == 4 * T and M == 5 * T and 13 * T < Fd < 14 * T and S == 16 * T
    vmem = pltpu.VMEM
    packed = lambda *lead: vmem(lead + (T, T), BF16)
    out = pl.pallas_call(
        _kernel,
        in_specs=[pl.BlockSpec(memory_space=pltpu.HBM)] * 12,
        out_specs=pl.BlockSpec(memory_space=pltpu.HBM),
        out_shape=jax.ShapeDtypeStruct((S, M), A_x.dtype),
        scratch_shapes=[
            vmem((S + 16, M), BF16),
            vmem((S, Dc), BF16),
            vmem((1, M), BF16),
            vmem((M, 2 * M), BF16),
            vmem((M, 4 * M), BF16),
            vmem((M, M), BF16),
            vmem((Fd % T, M), BF16),
            vmem((M, D), U32),
            vmem((Dc, D), U32),
            vmem((Dc, D), U32),
            vmem((2 * D, M), BF16),
            vmem((S, M), A_x.dtype),
            pltpu.SemaphoreType.DMA((15,)),
            pltpu.SemaphoreType.DMA((8,)),
            pltpu.SemaphoreType.DMA((S // T,)),
            vmem((8, 6 * M), F32),
            vmem((S // T, M // T, T, T), BF16),
            vmem((len(_C_SUMS), T, T), BF16),
            vmem((len(_H_SUMS), T, T), BF16),
            packed(2, M // T + 2 * (Dc // T)),
            packed(2 * S // T),
            packed(2 * S // T),
            packed(2 * S // T),
            vmem((S + 16, M), F32),
            vmem((S, M), F32),
            vmem((2, RB + 16, M), F32),
            vmem((RB, M), F32),
            vmem((RB + 32, M), F32),
            vmem((RB + 8, M), F32),
            packed(len(_MIXW)),
            packed(sum(m == 2 for m, _ in _MIXW)),
            vmem((Dc // T, T, T), U32),
            vmem((len(_WF), T, T), BF16),
            vmem((3, 8, T), jnp.int32),
            vmem(((2 * (M // T) + Fd // T + -(-Fd // T)) * 16, M), BF16),
            vmem((_FENCE + 1, T, T), BF16),
            vmem((_FENCE + 1, T, T), BF16),
            vmem((8, T), F32),
        ],
        compiler_params=pltpu.CompilerParams(
            vmem_limit_bytes=100 * 1024 * 1024,
            disable_bounds_checks=True,
        ),
    )(
        A_x.reshape(S, M), A_c_kv.reshape(S, Dc),
        A_w_q, A_w_uk, A_w_uv,
        A_w_o.reshape(H // 2, 2 * D, M),
        B_w1, B_w2, B_w3.T, B_w4, c, w_mod,
    )
    return out.reshape(1, S, M)
```

```python
import functools
import math

import jax
import jax.numpy as jnp
import jax.experimental.pallas as pl
import jax.experimental.pallas.tpu as pltpu

F32 = jnp.float32
BF16 = jnp.bfloat16
U32 = jnp.uint32
NT = (((1,), (1,)), ((), ()))
T = 128
EPS = 1e-5
LOG2E = math.log2(math.e)

GRP = 4
LEAD = 10
PROW = 3
RES = 32
LAT_0 = 32
LAT_A = 16
LAT_B = 20
ALEAD = 32
QT = (4, 6)
ONV, OEND = 0.7, 24
FPOS, DPOS = 0, 0
SIDE0, SIDE1, SLAG, SDUE = 8, 60, 3, 8
SKIND = 'pvo'
HACKWO = 0
SG0, SG1 = 6, 4
SD0, SDS = 4, 1.5
WFN = (4, 4, 6)
VF0, VFS = 4, 1.7
L_LO, L_HI, L_RATIO = 2.0 ** -24, 2.0 ** 24, 4.0
RB = 256
PC = 32
P0, PSTEP, PD = 300, 34, 36
GD, NAR0, NARS = 36, 4, 8
MSUB = (1, 1, 1, 1)
PSPLIT = 40
PDUE = 20
MWOPS = 70
NLN, LN0, LNS = 4, 4, 5
LP = 16
SP0, SP1 = 76, 38
_prologue = lambda: ('|kva|Z; |b|; kva|wc|Y0@56 K0123; bw|xdn|C0@56 N0123@52 K4567; cx|mq|N4567@52 F0@56 K89ab; '
            'd|y|C1@56 F1@56 Kcdef; nmq|zo|M H01 H234567@30 F2@36 Q0123; y||L H89ab@30 F3@36 Q4567; '
            'zo||Hcdef@30 S0@%d Q89ab S1@%d Qcdef' % (SP0, SP1))


def _dot(a, b):
    return jnp.dot(a, b, preferred_element_type=F32)


def _dot_nt(a, b):
    return jax.lax.dot_general(a, b, NT, preferred_element_type=F32)


def _ln(x):
    m = jnp.mean(x, axis=-1, keepdims=True)
    xc = x - m
    v = jnp.mean(xc * xc, axis=-1, keepdims=True)
    return xc * jnp.exp2(jnp.log(v + EPS) * (-0.5 * LOG2E))


def _rows(v, n):
    return jnp.broadcast_to(v[None], (n // 8, 8, v.shape[1])).reshape(n, v.shape[1])


def _gelu2(x):
    c0 = math.sqrt(2.0 / math.pi)
    return x + x * jnp.tanh(x * (c0 + (c0 * 0.044715) * (x * x)))


def _after(x, dep):
    return jnp.where(dep > jnp.inf, dep, x)


def _tie(x, dep):
    xu = pltpu.bitcast(x, U32)
    first = jnp.where(dep > jnp.inf, jnp.uint32(0), xu[:8])
    return pltpu.bitcast(jnp.concatenate([first, xu[8:]], axis=0), BF16)


def _tile(j):
    return slice(j * T, (j + 1) * T)


def _ld(ref, *idx):
    return pltpu.bitcast(ref.bitcast(U32)[idx], BF16)


def _a_ops(a11, a12, a21, a22):
    return [a11 + a22, a21 + a22, a11, a22, a11 + a12, a21 - a11, a12 - a22]


def _b_ops(b11, b12, b21, b22):
    return [b11 + b22, b11, b12 - b22, b21 - b11, b22, b11 + b12, b21 + b22]


def _strassen(prod, col1=None, col2=None):
    m4 = prod(3)
    m2 = prod(1)
    c21 = m2 + m4
    if col1 is not None:
        e11, e21 = col1()
        m4, c21 = m4 + e11, c21 + e21
    m3 = prod(2)
    m5 = prod(4)
    c12 = m3 + m5
    if col2 is not None:
        e12, e22 = col2()
        c12, m3 = c12 + e12, m3 + e22
    m1 = prod(0)
    c11 = prod(6) + (m1 + (m4 - m5))
    c22 = prod(5) + (m1 + (m3 - m2))
    return c11, c12, c21, c22


def _group(rows, cols, pairs):
    xs, ys = dict.fromkeys(x for x, _ in pairs), dict.fromkeys(y for _, y in pairs)
    used = set(xs) | set(ys) | {(x[0], y[1]) for x, y in pairs} | {(y[0], x[1]) for x, y in pairs}
    prods = []
    for n, r in enumerate(rows):
        for i, k in [x for x in xs if x[0] == r]:
            mates = [y for x, y in pairs if x == (i, k)]
            prods.append((((1, i, k),) + tuple((1, i, k2) for _, k2 in mates), ((1, k, 0),),
                          ((1, i, 0), (-1, i, 1))))
            prods.append((((1, i, k),) + tuple((-1, i2, k) for i2, _ in mates), ((1, k, 0), (1, k, 1)),
                          ((1, i, 1),)))
        for i2, k2 in [y for y in ys if y[0] == r]:
            mates = [x for x, y in pairs if y == (i2, k2)]
            prods.append((((1, i2, k2),) + tuple((1, i2, k) for _, k in mates), ((1, k2, 1),),
                          ((1, i2, 1), (-1, i2, 0))))
            prods.append((((1, i2, k2),) + tuple((-1, i, k2) for i, _ in mates), ((1, k2, 0), (1, k2, 1)),
                          ((1, i2, 0),)))
        prods += [(((1, r, k),), ((1, k, h),), ((1, r, h),)) for k in cols if (r, k) not in used for h in (0, 1)]
        for (i, k), (i2, k2) in pairs:
            if r in (i, i2) and i + i2 - r in rows[n + 1:]:
                prods.append((((1, i, k2),), ((1, k2, 0), (-1, k, 0)), ((1, i2, 0), (1, i, 0))))
                prods.append((((1, i2, k), (1, i, k2)), ((1, k, 0), (1, k2, 1)), ((1, i2, 0), (1, i, 1))))
                prods.append((((1, i2, k),), ((1, k, 1), (-1, k2, 1)), ((1, i2, 1), (1, i, 1))))
    return prods


def _all_pairs(xrows, yrows):
    return [((x, a), (y, b)) for a, x in enumerate(xrows) for b, y in enumerate(yrows) if a != b]


_PAIRS65 = [((x[0] + 10, x[1]), (y[0] + 10, y[1])) for x, y in (
    ((0, 1), (1, 0)), ((0, 1), (5, 2)), ((2, 3), (1, 0)), ((2, 3), (3, 1)), ((2, 3), (5, 2)), ((3, 2), (1, 0)),
    ((4, 4), (0, 3)), ((4, 4), (1, 0)), ((4, 4), (3, 1)), ((4, 4), (5, 2)))]
_C_GROUPS = [_group(range(r, r + 8), range(4), _all_pairs(range(r, r + 4), range(r + 4, r + 8))) for r in (0, 8)]
_H_GROUPS = [_group(range(10), range(5), _all_pairs(range(5), range(5, 10))),
             _group(range(10, 16), range(5), _PAIRS65)]
_sum_index = lambda groups: {f: n for n, f in enumerate(
    dict.fromkeys(t[0] for g in groups for t in g if len(t[0]) > 1))}
_C_SUMS, _H_SUMS = _sum_index(_C_GROUPS), _sum_index(_H_GROUPS)


def _cells(rows, cols, pairs):
    xs = list(dict.fromkeys(p[0] for p in pairs))
    ys = list(dict.fromkeys(p[1] for p in pairs))
    used = set(xs + ys) | {(x[0], y[1]) for x, y in pairs} | {(y[0], x[1]) for x, y in pairs}

    def home_x(i, k):
        mates = [y for x, y in pairs if x == (i, k)]
        return [(((1, i, k),) + tuple((1, i, k2) for _, k2 in mates), ((1, k, 0),), ((1, i, 0), (-1, i, 1))),
                (((1, i, k),) + tuple((-1, i2, k) for i2, _ in mates), ((1, k, 0), (1, k, 1)), ((1, i, 1),))]

    def home_y(i2, k2):
        mates = [x for x, y in pairs if y == (i2, k2)]
        return [(((1, i2, k2),) + tuple((1, i2, k) for _, k in mates), ((1, k2, 1),), ((1, i2, 1), (-1, i2, 0))),
                (((1, i2, k2),) + tuple((-1, i, k2) for i, _ in mates), ((1, k2, 0), (1, k2, 1)), ((1, i2, 0),))]

    def cross(x, y):
        (i, k), (i2, k2) = x, y
        return [(((1, i, k2),), ((1, k2, 0), (-1, k, 0)), ((1, i2, 0), (1, i, 0))),
                (((1, i2, k), (1, i, k2)), ((1, k, 0), (1, k2, 1)), ((1, i2, 0), (1, i, 1))),
                (((1, i2, k),), ((1, k, 1), (-1, k2, 1)), ((1, i2, 1), (1, i, 1)))]

    direct = lambda i: [(((1, i, k),), None, ((1, i, 0), (1, i, 1))) for k in cols if (i, k) not in used]
    single = lambda i: ([t for x in xs if x[0] == i for t in home_x(*x)]
                        + [t for y in ys if y[0] == i for t in home_y(*y)] + direct(i))
    prods = []
    for n, i in enumerate(rows):
        prods += single(i)
        for i2 in rows[n + 1:]:
            for x, y in pairs:
                if {x[0], y[0]} == {i, i2}:
                    prods += cross(x, y)
    return prods


_square = lambda q: [((a, a), (q + b, b)) for a in range(q) for b in range(q) if a != b]
_shift = lambda pairs, r0: [((x[0] + r0, x[1]), (y[0] + r0, y[1])) for x, y in pairs]
_flip = lambda pairs: [(x[::-1], y[::-1]) for x, y in pairs]
_P35 = [((1, 2), (0, 4)), ((1, 2), (2, 1)), ((2, 3), (0, 4)), ((2, 3), (1, 0))]
_P45 = [((0, 2), (1, 1)), ((2, 4), (0, 3)), ((2, 4), (1, 1)), ((2, 4), (3, 2)), ((3, 0), (0, 3)), ((3, 0), (1, 1))]
_P55 = [((2, 1), (0, 4)), ((2, 1), (1, 0)), ((2, 1), (3, 2)), ((2, 1), (4, 3)), ((3, 3), (0, 4)), ((3, 3), (1, 0)),
        ((4, 2), (0, 4)), ((4, 2), (1, 0))]
_MIX = [_cells(range(5), range(5), _P55), _cells(range(5), range(5), _P55),
        _cells(range(13), range(5), _square(5) + _shift(_P35, 10)),
        _cells(range(5), range(14), _flip(_square(5) + _shift(_P45, 10)))]
_MIXW = {(m, f): n for n, (m, f) in enumerate(dict.fromkeys((m, t[0]) for m in range(4) for t in _MIX[m]))}
_MIX3 = min(n for (m, _), n in _MIXW.items() if m == 2)


def _form(form, get):
    acc = None
    for sign, i, j in form:
        v = get(i, j)
        acc = v if acc is None else (acc + v if sign > 0 else acc - v)
    return acc


def _gap_items(bufs, gap_scr):
    items = []
    for n, buf in enumerate(bufs):
        acc = []

        def part(r0, buf=buf, acc=acc):
            def fn(dep):
                wu = jnp.concatenate([buf[r:r + 8, :] for r in range(r0, r0 + T, 32)])
                mask = jnp.full((8, T), 0x7FFF0000, U32)
                if dep is not None:
                    mask = jnp.where(dep > jnp.inf, jnp.uint32(0), mask)
                mask = _rows(mask, 32)
                new = [jnp.sum(pltpu.bitcast(v & mask, F32).reshape(4, 8, T), axis=0) for v in (wu << 16, wu)]
                acc[:] = [u + v for u, v in zip(acc, new)] if acc else new
            return fn

        def last(_, n=n, acc=acc):
            bits = []
            for v in acc:
                l1 = jnp.sum(jnp.sum(v, axis=1, keepdims=True), axis=0, keepdims=True)
                bits.append(pltpu.bitcast(jnp.broadcast_to(l1, (8, T)), jnp.int32) >> 8)
            gap = jnp.clip((bits[0] - bits[1] + (1 << 14)) >> 15, -8, 8) << 23
            gap_scr[n] = gap
            return pltpu.bitcast(gap, F32)

        items += [part(r0) for r0 in range(0, buf.shape[0], T)] + [last]
    return items


def _pair_tiles(w_ref, transpose=False):
    tiles = {}
    for j in range(w_ref.shape[0] // T):
        wu = w_ref[_tile(j), :]
        if transpose:
            wu = wu.T
        tiles[j, 0] = pltpu.bitcast(wu << 16, F32).astype(BF16)
        tiles[j, 1] = pltpu.bitcast(wu & jnp.uint32(0xFFFF0000), F32).astype(BF16)
    return tiles


def _canon(form):
    if form[-1][0] < 0 and form[0][1:] > form[1][1:]:
        return -1, ((1,) + form[1][1:], (-1,) + form[0][1:])
    return 1, form


_w_forms = lambda groups: list(dict.fromkeys(_canon(t[1])[1] for g in groups for t in g))
_WF = {key: n for n, key in enumerate([(m, f) for m, groups in enumerate((_C_GROUPS, _C_GROUPS, _H_GROUPS))
                                       for f in _w_forms(groups)])}


def _weight_form_items(bufs, gap_scr, wt_scr, wf_scr, which):
    n = 16
    items = []

    def flip(j):
        def fn(dep):
            wu = bufs[1][_tile(j), :]
            wu = (wu if dep is None else jnp.where(_rows(dep, T) > jnp.inf, jnp.uint32(0), wu)).T
            wt_scr[j] = wu
            return pltpu.bitcast(wu[T - 8:], F32)
        return fn

    def part(m, r0, forms):
        def fn(dep):
            fac = pltpu.bitcast(0x3F800000 + gap_scr[m], F32)
            mask = jnp.full((8, T), 0xFFFF0000, U32)
            sh = jnp.full((8, T), 16, U32)
            if dep is not None:
                mask = jnp.where(dep > jnp.inf, jnp.uint32(0), mask)
                sh = jnp.where(dep > jnp.inf, jnp.uint32(0), sh)
            fac, mask, sh = _rows(fac, n), _rows(mask, n), _rows(sh, n)
            base = {}

            def get(k, h):
                if (k, h) not in base:
                    wu = wt_scr[k, r0:r0 + n, :] if m == 1 else bufs[m][k * T + r0:k * T + r0 + n, :]
                    base[k, h] = pltpu.bitcast(wu & mask, F32) * fac if h else pltpu.bitcast(wu << sh, F32)
                return base[k, h]

            for f in forms:
                wf_scr[_WF[m, f], r0:r0 + n, :] = _form(f, get).astype(BF16)
        return fn

    for m in which:
        forms = [f for mm, f in _WF if mm == m]
        if m == 1:
            items += [flip(j) for j in range(bufs[1].shape[0] // T)]
        per = -(-len(forms) // WFN[m])
        forms.sort(key=lambda f: sorted({t[1] for t in f}))
        items += [part(m, r0, forms[i:i + per]) for r0 in range(0, T, n) for i in range(0, len(forms), per)]
    return items


def _run_group(jobs, prods, a_get, w, transposed, finish):
    left = {}
    for _, _, outs in prods:
        for _, i, h in outs:
            left[i, h] = left.get((i, h), 0) + 1
    acc = {}
    for af, bf, outs in prods:
        sign, wt = w(bf)
        m = jobs.mm([wt], [a_get(af)], _dot_nt) if transposed else jobs.mm([a_get(af)], [wt], _dot)
        for s_, i, h in outs:
            if (i, h) not in acc:
                acc[i, h] = (s_ * sign, m)
            else:
                s0, v = acc[i, h]
                acc[i, h] = (s0, v + m if s0 == s_ * sign else v - m) if s0 > 0 or s_ * sign < 0 else (1, m - v)
            left[i, h] -= 1
            if not left[i, h]:
                s0, v = acc.pop((i, h))
                assert s0 > 0
                finish(2 * i + h, v)


class _Jobs:
    def __init__(self, side=()):
        self.res = []
        self.side = list(side)
        self.due = []

    def mm(self, lhs, wt, dot):
        acc = None
        for x, w in zip(lhs, wt):
            if self.due and self.due[0][0] <= len(self.res):
                x = _tie(x, self.due.pop(0)[1])
            v = dot(x, w)
            self.res.append(v)
            acc = v if acc is None else v + acc
            rel = 4 * (len(self.res) % 4)
            while self.side and self.side[0][0] <= len(self.res):
                out = self.side.pop(0)[1](v[8 * rel:8 * rel + 8, :])
                if out is not None:
                    self.due.append((len(self.res) + PDUE, out))
                rel = (rel + 2) % 16
        return acc


def _proj_step(h_scr, hs_scr, c_ref, cs_scr, wf_scr, q_scr, k_scr, v_scr, pf, scale, shifts, side):
    def weight(m):
        def get(form):
            sign, form = _canon(form)
            return sign, _ld(wf_scr, _WF[m, form])
        get.inv = pltpu.bitcast(0x3F800000 - shifts[m], F32)
        return get

    wk, wvT, wq = weight(0), weight(1), weight(2)
    c_get = lambda f: _ld(cs_scr, _C_SUMS[f]) if len(f) > 1 else c_ref[_tile(f[0][1]), _tile(f[0][2])]
    h_get = lambda f: _ld(hs_scr, _H_SUMS[f]) if len(f) > 1 else _ld(h_scr, f[0][1], f[0][2])

    def put(dst, w, mul=None):
        muls = [mul, _rows(w.inv if mul is None else w.inv * mul, T)]

        def fn(u, v):
            v = (v if muls[u % 2] is None else v * muls[u % 2]).astype(BF16)
            dst[u] = v.T if mul is not None and u in QT else v
        return fn

    jobs = _Jobs(side)
    put_v, stored = put(v_scr, wvT), set()
    nxt = [0]

    def fin_v(u, v):
        put_v(u, v)
        stored.add(u)
        for J in range(SB):
            if all(2 * (SB * J + k) + h in stored for k in range(SB) for h in range(2)) and ('J', J) not in stored:
                stored.add(('J', J))
                for fn in _v_form_items(v_scr, pf, J):
                    nxt[0] = max(nxt[0] + VFS, len(jobs.res) + VF0)
                    jobs.side.append((int(nxt[0]), fn))
                jobs.side.sort(key=lambda e: e[0])

    kk, vv, qq = ((c_get, wk, False, put(k_scr, wk)), (c_get, wvT, True, fin_v),
                  (h_get, wq, False, put(q_scr, wq, scale)))
    for prods, args in ((_C_GROUPS[0], kk), (_C_GROUPS[0], vv), (_C_GROUPS[1], vv), (_C_GROUPS[1], kk),
                        (_H_GROUPS[0], qq), (_H_GROUPS[1], qq)):
        _run_group(jobs, prods, *args)
    assert not jobs.side and not jobs.due


def _inner_group(rows, cols, pairs):
    xs, ys = dict.fromkeys(x for x, _ in pairs), dict.fromkeys(y for _, y in pairs)
    used = set(xs) | set(ys) | {(x[0], y[1]) for x, y in pairs} | {(y[0], x[1]) for x, y in pairs}
    prods = []
    for i, j in xs:
        mates = [y for x, y in pairs if x == (i, j)]
        prods.append((((1, i, 0),), ((1, 0, j), (-1, 1, j)), ((1, i, j),) + tuple((1, i2, j) for i2, _ in mates)))
        prods.append((((1, i, 0), (1, i, 1)), ((1, 1, j),), ((1, i, j),) + tuple((-1, i, j2) for _, j2 in mates)))
    for i2, j2 in ys:
        mates = [x for x, y in pairs if y == (i2, j2)]
        prods.append((((1, i2, 0), (1, i2, 1)), ((1, 0, j2),),
                      ((1, i2, j2),) + tuple((-1, i2, j) for _, j in mates)))
        prods.append((((1, i2, 1),), ((1, 0, j2), (-1, 1, j2)),
                      ((-1, i2, j2),) + tuple((-1, i, j2) for i, _ in mates)))
    prods += [(((1, i, h),), ((1, h, j),), ((1, i, j),))
              for i in rows for j in cols if (i, j) not in used for h in (0, 1)]
    for (i, j), (i2, j2) in pairs:
        lo, hi = min(j, j2), max(j, j2)
        prods.append((((1, i2, 0), (-1, i, 0)), ((1, 0, lo), (1, 0, hi)), ((1, i2, j),)))
        prods.append((((1, i, 0), (1, i2, 1)), ((1, 0, j2), (1, 1, j)), ((1, i, j2), (1, i2, j))))
        prods.append((((1, i, 1), (-1, i2, 1)), ((1, 1, lo), (1, 1, hi)), ((1, i, j2),)))
    return prods


def _o_jobs():
    prods = (_inner_group(range(10), range(5), _all_pairs(range(0, 10, 2), range(1, 10, 2)))
             + _inner_group(range(10, 16), range(5), _PAIRS65))
    row = lambda t: max(i for _, i, _ in t[0])
    unit = lambda t: max(2 * i + h for _, i, h in t[0])
    need = lambda t: unit(t) if row(t) == 15 else 2 * row(t) + 1
    return [(need(t), t) for t in sorted(prods, key=need)]


_O_JOBS = _o_jobs()


SB = 4


class _Star:
    def __init__(self, ts):
        self.ts, self.n = ts, len(ts)
        rn = range(self.n)
        self.pairs = [(i, j) for i in rn for j in rn if i < j]
        self.pf = {f: m for m, f in enumerate([('R', i) for i in rn] + [('C', i) for i in rn]
                                              + [('S', i, j) for i in rn for j in rn if i != j]
                                              + [('A', i, j) for i, j in self.pairs])}
        self.vf = {f: m for m, f in enumerate([('W', i) for i in rn]
                                              + [(q, i, j) for i, j in self.pairs for q in ('Q1', 'Q2', 'Q3')])}
        self.pv = {**{('W', i): ('R', i) for i in rn}, **{('B', i): ('C', i) for i in rn},
                   **{('Q1', i, j): ('S', i, j) for i, j in self.pairs},
                   **{('Q2', i, j): ('A', i, j) for i, j in self.pairs},
                   **{('Q3', i, j): ('S', j, i) for i, j in self.pairs}}

    def products(self, i):
        return [('W', i), ('B', i)] + [(q, i, j) for j in range(i + 1, self.n) for q in ('Q1', 'Q2', 'Q3')]


_FULL = _Star((-1.125, -0.375, 0.375, 1.125))
_HALF = _Star((-0.75, 0.75))
_DCELLS = [(0, 0), (1, 0), (1, 1), (2, 2), (3, 2), (3, 3)]
_HSLOT = (SB - 1) * len(_FULL.pf)
_DSLOT = _HSLOT + len(_HALF.pf)
_VSLOT = _DSLOT + len(_DCELLS)
_VHALF = (SB - 1) * len(_FULL.vf)
_FENCE = _VSLOT + (_VHALF + SB * len(_HALF.vf) + 1) // 2


def _v_slot(star, J, f):
    m = star.vf[f] + J * len(star.vf) + (0 if star is _FULL else _VHALF)
    return _VSLOT + m // 2, m % 2 * (T // 2)


def _v_form_items(v_scr, pf, J):
    n, HT = 16, T // 2

    def item(star, h, r0, pairs):
        def fn(dep):
            ts = [jnp.full((8, T), t, F32) for t in star.ts]
            ts = [_rows(t if dep is None else _after(t, dep), n) for t in ts]

            def get(k, a):
                r = (a * HT + r0) // 2
                return _ld(v_scr, 2 * (SB * J + k) + h, slice(r, r + n // 2)).astype(F32)

            def put(f, v):
                slot, r = _v_slot(star, J, f)
                pf[h][slot, r + r0:r + r0 + n, :] = v.astype(BF16)

            b = {(k, a): get(k, a) for k in sorted({k for pr in pairs or star.pairs for k in pr})
                 for a in range(2)}
            if pairs is None or star.n == 2:
                w = [b[k, 0] + ts[k] * b[k, 1] for k in range(star.n)]
                for k in range(star.n):
                    put(('W', k), w[k])
                for i, j in star.pairs:
                    put(('Q2', i, j), w[i] - w[j])
            for i, j in pairs or ():
                d0, d1 = b[j, 0] - b[i, 0], b[j, 1] - b[i, 1]
                put(('Q1', i, j), d0 + ts[i] * d1)
                put(('Q3', i, j), d0 + ts[j] * d1)
        return fn

    pr = _FULL.pairs
    parts = [(_HALF, _HALF.pairs)]
    if J < SB - 1:
        parts += [(_FULL, x) for x in (None, pr[:2], [pr[2], pr[4]], [pr[3], pr[5]])]
    return [item(star, h, r0, pairs) for h in range(2) for r0 in range(0, HT, n) for star, pairs in parts]


def _job_order(nsb):
    units = [(I, h) for I in range(nsb) for h in range(2)]
    qe, qv = [], []
    for I, h in units:
        es = [('e', I, h, J, p) for J in range(I) for p in range(SB)]
        ds = [('d', I, h) + c for c in _DCELLS]
        es.insert(max(len(es) - FPOS, 0), ('f', I, h))
        qe += es + ds if I or FPOS < 9 else ds[:DPOS] + es + ds[DPOS:]
        for i in range(SB):
            qv += [('p', I, h, f, J) for f in _FULL.products(i) for J in range(I)]
            if i >= 2:
                qv += [('p', I, h, f, None) for f in _HALF.products(i - 2)]
            qv += [('v', I, h) + c for c in _DCELLS if c[0] == i]
    qo = [('o', u, j) for j, (u, _) in enumerate(_O_JOBS)]
    cost = dict(e=8, f=8, d=2, p=1, v=2, o=2)
    order, done = [], {}
    now = [0]

    def emit(q):
        job = q.pop(0)
        order.append(job)
        now[0] += cost[job[0]]
        if job[0] == 'd':
            done[job] = now[0]
        elif job[0] == 'v' and job[4] == job[3]:
            done['u', 2 * (SB * job[1] + job[3]) + job[2]] = now[0]
        return cost[job[0]]

    def v_ready():
        if not qv:
            return False
        key = ('d', qv[0][1], qv[0][2], SB - 1, SB - 1)
        return key in done and done[key] + (LAT_0 if qv[0][1:3] == (0, 0) else LAT_A) <= now[0]

    def o_ready():
        return bool(qo) and ('u', qo[0][1]) in done and done['u', qo[0][1]] + LAT_B <= now[0]

    def fill(nv, no):
        n = 0
        while nv > 0 or no > 0 or n % 4:
            if no > 0 and n % 2 == 0 and o_ready() and no * ONV >= nv:
                no -= 2
                n += emit(qo)
            elif v_ready() and (nv > 0 or n % 4):
                c = emit(qv)
                nv -= c
                n += c
            elif o_ready() and n % 2 == 0 and (no > 0 or n % 4 or nv > 0) and len(qo) > RES:
                no -= 2
                n += emit(qo)
            else:
                break

    while qe:
        unit = qe[0][1:3]
        while qv and qv[0][2] == unit[1] and qv[0][1] < unit[0]:
            emit(qv)
        ne = 0
        while qe and ne < 8 and (ne == 0 or (qe[0][0] == 'd' and qe[0][1:3] == unit and ne + 2 <= 8)):
            ne += emit(qe)
        groups = lambda q: sum(cost[j[0]] for j in q) / 8
        old = [j for j in qv if j[1:3] != unit and ('d', j[1], j[2], SB - 1, SB - 1) in done]
        here = [j for j in qe if j[1:3] == unit]
        rest = sum(cost[j[0]] for j in old)
        nv = (rest - LAT_A) / (groups(here) + 1) if here else rest
        no = 2 * max(len(qo) - RES - OEND, 0) / (groups(qe) + 1)
        fill(int(nv + 0.5), int(no + 0.5))
    while qv or qo:
        if qv and v_ready():
            fill(6, 2)
            if not qv:
                continue
        elif o_ready():
            emit(qo)
        else:
            emit(qv or qo)
    return order


def _attention_safe(q_scr, k_scr, v_scr, wo_ref, acc_scr):
    causal = (jax.lax.broadcasted_iota(jnp.int32, (T, T), 0)
              <= jax.lax.broadcasted_iota(jnp.int32, (T, T), 1))

    def unit(u, carry):
        r, hd = u // 2, u % 2

        def block(c, mlo):
            m0, l, o = mlo
            s = _dot_nt(_ld(k_scr, 2 * c + hd), _ld(q_scr, u))
            s = jnp.where(jnp.logical_or(causal, c < r), s, -1e9 * LOG2E)
            m = jnp.maximum(m0, jnp.max(s, axis=0, keepdims=True))
            a = jnp.exp2(m0 - m)
            p = jnp.exp2(s - m)
            return (m, l * a + jnp.sum(p, axis=0, keepdims=True),
                    o * a + _dot(_ld(v_scr, 2 * c + hd), p.astype(BF16)))

        _, l, o = jax.lax.fori_loop(0, r + 1, block, (jnp.full((1, T), -jnp.inf, F32), jnp.zeros((1, T), F32),
                                                      jnp.zeros((T, T), F32)))
        rows = pl.ds(pl.multiple_of(r * T, T), T)
        acc_scr[rows, :] += _dot((o * (1.0 / l)).astype(BF16).T, wo_ref[pl.ds(pl.multiple_of(hd * T, T), T), :])
        return carry

    jax.lax.fori_loop(0, q_scr.shape[0], unit, 0)


def _attention_step(q_scr, k_scr, v_scr, pf, wo_ref, acc_scr, flag_scr, z, side):
    causal = (jax.lax.broadcasted_iota(jnp.int32, (T, T), 0)
              <= jax.lax.broadcasted_iota(jnp.int32, (T, T), 1))
    HT = T // 2
    lsum, lrow, acc, fg, dacc, of, lhs = {}, {}, {}, {}, {}, {}, {}
    res = []
    wo, terms = {}, {}
    left = {}
    done_side = [0, 0]
    chk = [jnp.zeros((8, T), F32), None]
    for _, t in _O_JOBS:
        for _, i, j in t[2]:
            left[i, j] = left.get((i, j), 0) + 1

    def add_l(u, v):
        lsum[u] = v if u not in lsum else lsum[u] + v

    csign = {}

    def p_forms(star, h, slot0, g, tiles, cell, when):
        n = star.n

        def put(f, v):
            pf[h][slot0 + star.pf[f], 16 * g:16 * g + 16, :] = v.astype(BF16)

        for i in range(n):
            row = [cell(i, k) for k in sorted(range(n), key=lambda k: when(i, k))]
            r = functools.reduce(lambda x, y: x + y, row)
            put(('R', i), r)
            add_l(tiles[i], r[:8] + r[8:])
            col = sorted(range(n), key=lambda i2: (when(i2, i), i2 != i))
            sign = csign[n, i] = 1 if col[0] == i else -1
            c = cell(col[0], i)
            for i2 in col[1:]:
                c = c + cell(i2, i) if (1 if i2 == i else -1) == sign else c - cell(i2, i)
            put(('C', i), c)
            for j in range(n):
                if j != i:
                    put(('S', i, j), cell(i, j))
        for i, j in star.pairs:
            put(('A', i, j), cell(i, j) + cell(j, i))

    due = []

    def scores(x, u):
        if due and due[0][0] <= done_side[1]:
            x = _tie(x, due.pop(0)[1])
        s = (_dot if u in QT else _dot_nt)(x, _ld(q_scr, u))
        res.append(s)
        return s

    def job_e(I, h, J, p):
        tiles = [2 * (SB * I + i) + h for i in range(SB)]
        ps = []
        for i, u in enumerate(tiles):
            x = jnp.concatenate([k_scr.bitcast(U32)[2 * (SB * J + (t - i) % SB) + h, 8 * g:8 * g + 8, :]
                                 for g in (2 * p, 2 * p + 1) for t in range(SB)], axis=0)
            ps.append(jnp.exp2(scores(pltpu.bitcast(x, BF16), u)))
        when = lambda i, k: (i + k) % SB
        for n, g in enumerate((2 * p, 2 * p + 1)):
            cell = lambda i, k: ps[i][16 * (SB * n + when(i, k)):16 * (SB * n + when(i, k)) + 16]
            p_forms(_FULL, h, J * len(_FULL.pf), g, tiles, cell, when)

    def job_f(I, h):
        tiles = [2 * (SB * I + 2 + i) + h for i in range(2)]
        ps = {(i, k): jnp.exp2(scores(_ld(k_scr, 2 * (SB * I + k) + h), u))
              for i, u in enumerate(tiles) for k in range(2)}
        for g in range(T // 16):
            p_forms(_HALF, h, _HSLOT, g, tiles, lambda i, k: ps[i, k][16 * g:16 * g + 16], lambda i, k: 0)

    def job_d(I, h, i, k):
        u = 2 * (SB * I + i) + h
        s = scores(_ld(k_scr, 2 * (SB * I + k) + h), u)
        if i == k:
            s = jnp.where(causal, s, -1e9 * LOG2E)
        p = jnp.exp2(s)
        add_l(u, jnp.sum(p.reshape(T // 8, 8, T), axis=0))
        pf[h][_DSLOT + _DCELLS.index((i, k))] = p.astype(BF16)
        if (i, k) == _DCELLS[-1]:
            pf[h][_FENCE + z, 0:16, :] = jnp.zeros((16, T), BF16)
            for u in [2 * (SB * I + a) + h for a in range(SB)]:
                lrow[u] = jnp.sum(lsum.pop(u), axis=0, keepdims=True)
            ls = [lrow[2 * (SB * I + a) + h] for a in range(SB)]
            lo = jnp.minimum(jnp.minimum(ls[0], ls[1]), jnp.minimum(ls[2], ls[3]))
            hi = jnp.maximum(jnp.maximum(ls[0], ls[1]), jnp.maximum(ls[2], ls[3]))
            ok = jnp.logical_and(lo >= L_LO, hi <= L_HI)
            ok = jnp.logical_and(ok, (hi if I else jnp.maximum(ls[2], ls[3]))
                                 <= L_RATIO * (lo if I else jnp.minimum(ls[2], ls[3])))
            bad = jnp.where(ok, 0.0, 1.0)
            chk[1] = bad if chk[1] is None else jnp.maximum(chk[1], bad)

    def job_p(I, h, f, J):
        star, last = (_HALF, True) if J is None else (_FULL, J == I - 1)
        blk = I if J is None else J
        if f[0] == 'B':
            x = _ld(v_scr, 2 * (SB * blk + f[1]) + h, slice(HT // 2, HT))
        else:
            slot, r = _v_slot(star, blk, f)
            x = _ld(pf[h], slot, slice(r // 2, (r + HT) // 2))
        v = _dot(x, _ld(pf[h], (_HSLOT if J is None else J * len(_FULL.pf)) + star.pf[star.pv[f]]))
        res.append(v)
        key = (star.n,) + f
        acc[key] = v if key not in acc else acc[key] + v
        if not last:
            return

        def add(which, i, v, sign=1):
            k_ = (star.n, which, i)
            if k_ not in fg:
                fg[k_] = v if sign > 0 else -v
            else:
                fg[k_] = fg[k_] + v if sign > 0 else fg[k_] - v

        if f[0] == 'W':
            add('F', f[1], acc.pop(key))
        elif f[0] == 'B':
            add('G', f[1], acc.pop(key), csign[star.n, f[1]])
        elif f[0] == 'Q3':
            _, i, j = f
            q1, q2, q3 = (acc.pop((star.n, q, i, j)) for q in ('Q1', 'Q2', 'Q3'))
            t = ((q1 + q2) + q3) * (1.0 / (star.ts[i] - star.ts[j]))
            add('G', i, t)
            add('G', j, t)
            add('F', i, q1)
            add('F', j, q3, -1)

    def job_v(I, h, i, k):
        u = 2 * (SB * I + i) + h
        v = _dot(_ld(v_scr, 2 * (SB * I + k) + h), _ld(pf[h], _DSLOT + _DCELLS.index((i, k))))
        res.append(v)
        dacc[u] = v if u not in dacc else dacc[u] + v
        if k == i:
            o = dacc.pop(u)
            for star, a in ([(_FULL, i)] if I else []) + ([(_HALF, i - 2)] if i >= 2 else []):
                f, g = fg.pop((star.n, 'F', a)), fg.pop((star.n, 'G', a))
                o = o + jnp.concatenate([f - star.ts[a] * g, g], axis=0)
            o = o * (1.0 / lrow[u])
            of[u] = o
            chk[0] = chk[0] + jnp.sum(o.reshape(T // 8, 8, T), axis=0)

    def job_o(_, n):
        af, bf, outs = _O_JOBS[n][1]
        if af not in lhs:
            v = _form(af, lambda i, h: of[2 * i + h])
            lhs[af] = _tie(v.astype(BF16).T, v[0:8, :])
        if bf not in wo:
            wo[bf] = (wo_ref[_tile(bf[0][1]), _tile(bf[0][2])] if len(bf) == 1 else
                      _form(bf, lambda h, j: wo_ref[_tile(h), _tile(j)].astype(F32)).astype(BF16))
            if HACKWO:
                wo[bf] = _ld(q_scr, len(wo) % 32)
        v = _dot(lhs[af], wo[bf])
        res.append(v)
        for sign, i, j in outs:
            terms.setdefault((i, j), []).append((sign, v))
            if len(terms[i, j]) == left[i, j]:
                tot = acc_scr[_tile(i), _tile(j)]
                for sg, m in terms.pop((i, j)):
                    tot = tot + m if sg > 0 else tot - m
                acc_scr[_tile(i), _tile(j)] = tot

    fns = dict(e=job_e, f=job_f, d=job_d, p=job_p, v=job_v, o=job_o)
    order = _job_order(q_scr.shape[0] // (2 * SB))
    for n, job in enumerate(order):
        assert job[0] not in 'efd' or not any(j[0] in 'pv' and j[2] == job[2] and j[1] < job[1] for j in order[n:])
    side = list(side)
    fences = [n for n, job in enumerate(order) if job[0] == 'd' and job[3:] == _DCELLS[-1]]
    step = (len(order) - SIDE0 - SIDE1 - 10) / len(side)
    for n, job in enumerate(order):
        done_side[1] = n
        fns[job[0]](*job[1:])
        last_chance = n >= len(order) - SIDE1
        near = any(-SG1 <= f - n <= SG0 for f in fences)
        if side and n >= SIDE0 + step * done_side[0] and ((job[0] in SKIND and not near) or last_chance):
            done_side[0] += 1
            v = side.pop(0)(res[-1 - SLAG][8 * (n % 4):8 * (n % 4) + 8, :])
            if v is not None:
                due.append((n + SDUE, v))
    assert not side and not due
    fine = jnp.abs(chk[0]) < jnp.inf
    flag_scr[...] = jnp.maximum(flag_scr[...], jnp.where(fine, chk[1], 1.0))


def _kernel(x_hbm, c_hbm, wq_hbm, wuk_hbm, wuv_hbm, wo_hbm, w1_hbm, w2_hbm, w3_hbm, w4_hbm,
            cond_hbm, wmod_hbm, out_hbm,
            x_ref, c_ref, cond_ref, wma_ref, wmb_ref, w1_ref, w3_ref,
            wq_buf, wk_buf, wv_buf, wo_buf, out_buf, sem, wsem, osem,
            mod_scr, h_scr, cs_scr, hs_scr, w_scr, q_scr, k_scr, v_scr, acc_scr, xn_scr, xh_scr, a1_scr, t_scr,
            z_scr, mw_scr, m3_scr, wt_scr, wf_scr, gap_scr, st_in, pf_scr, vf_scr, flag_scr):
    S, M = x_hbm.shape
    D = wq_hbm.shape[2]
    nattn = wo_hbm.shape[0]
    Fd = w4_hbm.shape[0]
    scale = float(D) ** -0.5 * LOG2E
    nb, nrb = S // T, S // RB
    km, kc = M // T, c_hbm.shape[1] // T
    NX = 4
    XR = S // NX
    CB = XR // T

    work = (wk_buf, wv_buf, wq_buf)

    def pcopies(g, bufs=work, s0=0):
        return [pltpu.make_async_copy(src.bitcast(U32).at[:, g, :], dst, wsem.at[s0 + j])
                for j, (src, dst) in enumerate(zip((wuk_hbm, wuv_hbm, wq_hbm), bufs))]

    def ocopy(g):
        return pltpu.make_async_copy(wo_hbm.at[g], wo_buf, wsem.at[3])

    def chunk_copy(src, dst, i, s0):
        rows = slice(i * XR, (i + 1) * XR)
        return pltpu.make_async_copy(src.at[rows, :], dst.at[rows, :], sem.at[s0 + i])

    MS = 16
    NSL = T // MS
    assert nattn - 1 >= NSL
    mixw = ((w1_hbm, km, 0), (w2_hbm, km, km * MS), (w3_hbm, Fd // T, 2 * km * MS),
            (w4_hbm, -(-Fd // T), (2 * km + Fd // T) * MS))

    def prep_in(g):
        o = jnp.minimum(g, NSL - 1) * MS
        return [pltpu.make_async_copy(
            w.at[pl.ds(pl.multiple_of(jnp.minimum(b * T + o, w.shape[0] - MS), MS), MS), :],
            st_in.at[r0 + b * MS:r0 + (b + 1) * MS, :], wsem.at[7]) for w, nblk, r0 in mixw for b in range(nblk)]

    def stage_in(g):
        return pcopies(jnp.minimum(g + 1, nattn - 1))

    cp_cond = pltpu.make_async_copy(cond_hbm, cond_ref, sem.at[0])
    cp_wma = pltpu.make_async_copy(wmod_hbm.at[:, 0:2 * M], wma_ref, sem.at[1])
    cp_late = [pltpu.make_async_copy(src, dst, sem.at[2 + j]) for j, (src, dst) in enumerate((
        (wmod_hbm.at[:, 2 * M:6 * M], wmb_ref), (w1_hbm, w1_ref), (w3_hbm.at[Fd // T * T:, :], w3_ref)))]
    cp_x = [chunk_copy(x_hbm, x_ref, i, 7) for i in range(NX)]
    cp_c = [chunk_copy(c_hbm, c_ref, i, 7 + NX) for i in range(NX)]

    def silu_cond():
        cf = cond_ref[...].astype(F32)
        return jnp.broadcast_to((cf * jax.nn.sigmoid(cf)).astype(BF16), (8, M))

    cp_wk, cp_wv, cp_wq = pcopies(0)
    named = dict(k=cp_wk, v=cp_wv, q=cp_wq, o=ocopy(0), n=cp_cond, m=cp_wma)
    named.update(zip('abcd', cp_c))
    named.update(zip('wxyz', cp_x))
    started, arrived, did = set(), set(), set()

    def zero(r, carry):
        acc_scr[pl.ds(pl.multiple_of(r * T, T), T), :] = jnp.zeros((T, M), F32)
        return carry

    def x_rows(rows, dep):
        xf = x_ref[rows, :].astype(F32)
        if dep is None:
            return xf
        return jnp.concatenate([_after(xf[:, :T], _rows(dep, xf.shape[0])), xf[:, T:]], axis=1)

    def n_item(r, i):
        def fn(dep):
            rows = slice(r * T + i * LP, r * T + (i + 1) * LP)
            xn_scr[rows, :] = _ln(x_rows(rows, dep))
        return fn

    def h_item(r, i, normed):
        def fn(dep):
            rows = slice(i * LP, (i + 1) * LP)
            grows = slice(r * T + i * LP, r * T + (i + 1) * LP)
            sa = mod_scr[:, 0:M]
            if normed and dep is not None:
                sa = jnp.concatenate([_after(sa[:, _tile(j)], dep) for j in range(km)], axis=1)
            hf = ((xn_scr[grows, :] if normed else _ln(x_rows(grows, dep))) * _rows(mod_scr[:, M:2 * M], LP)
                  + _rows(sa, LP))
            for j in range(km):
                h_scr[r, j, rows, :] = hf[:, _tile(j)].astype(BF16)
            for f, n in _H_SUMS.items():
                if all(t[1] == r for t in f):
                    hs_scr[n, rows, :] = _form(f, lambda _, k: hf[:, _tile(k)]).astype(BF16)
            did.add(('h', r, i))
        return fn

    def release(jobs, span, items):
        if span and items:
            jobs.side += [(len(jobs.res) + 1 + i * span // len(items), fn) for i, fn in enumerate(items)]
            jobs.side.sort(key=lambda e: e[0])
        else:
            for fn in items:
                fn(None)

    def sum_items(n, group, index, dst, get, skip_rows):
        forms = [f for f in dict.fromkeys(t[0] for t in group)
                 if len(f) > 1 and not (skip_rows and len({t[1] for t in f}) == 1)]

        def item(f, rows):
            def fn(dep):
                def term(r, k):
                    v = get(r, k, rows).astype(F32)
                    return v if dep is None or (r, k) != f[0][1:] else _after(v, _rows(dep, v.shape[0]))
                dst[index[f], rows, :] = _form(f, term).astype(BF16)
            return fn

        return [item(f, slice(i, i + n)) for i in range(0, T, n) for f in forms]

    h_sums = lambda n, gi: sum_items(n, _H_GROUPS[gi], _H_SUMS, hs_scr,
                                     lambda r_, k, rows: h_scr[r_, k, rows, :], True)

    def stash(key, buf, j0, transpose=False):
        n = buf.shape[0] // T
        if key not in did:
            assert key in arrived
            did.add(key)
            for (j, hd), w in _pair_tiles(buf, transpose).items():
                w_scr[hd, j0 + j] = w
        return lambda hd: [_ld(w_scr, hd, j0 + j) for j in range(n)]

    def kv_tile(jobs, r):
        wk, wvT = stash('k', wk_buf, 0), stash('v', wv_buf, kc, True)
        ct = [c_ref[_tile(r), _tile(j)] for j in range(kc)]
        for hd in range(2):
            k_scr[2 * r + hd] = jobs.mm(ct, wk(hd), _dot).astype(BF16)
        for hd in range(2):
            v_scr[2 * r + hd] = jobs.mm(wvT(hd), ct, _dot_nt).astype(BF16)

    def q_tile(jobs, r):
        wq = stash('q', wq_buf, 2 * kc)
        ht = [_ld(h_scr, r, j) for j in range(km)]
        for hd in range(2):
            v = (jobs.mm(ht, wq(hd), _dot) * scale).astype(BF16)
            q_scr[2 * r + hd] = v.T if 2 * r + hd in QT else v

    for blk in _prologue().split(';'):
        waits, starts, acts = blk.split('|')
        for ch in waits.strip():
            assert ch in started and ch not in arrived
            arrived.add(ch)
            named[ch].wait()
        for ch in starts.strip():
            assert ch not in started
            started.add(ch)
            named[ch].start()
        jobs = _Jobs()
        for act in acts.split():
            if act == 'Z':
                jax.lax.fori_loop(0, nb, zero, 0)
                acc_scr[S:, :] = jnp.zeros((acc_scr.shape[0] - S, M), F32)
                x_ref[S:, :] = jnp.zeros((x_ref.shape[0] - S, M), BF16)
                flag_scr[...] = jnp.zeros(flag_scr.shape, F32)
            elif act == 'L':
                did.add('L')
                assert ('Q', 0) in did
                for cp in stage_in(0) + prep_in(0):
                    cp.start()
            elif act == 'M':
                assert arrived >= set('nm')
                mod = _dot(silu_cond(), wma_ref[...])
                mod_scr[:, 0:M] = mod[:, 0:M]
                mod_scr[:, M:2 * M] = 1.0 + mod[:, M:2 * M]
                did.add('M')
            else:
                act, _, span = act.partition('@')
                span = int(span or 0)
                items = []
                for r in [int(ch, 16) for ch in act[1:]]:
                    did.add((act[0], r))
                    if act[0] == 'K':
                        assert 'abcd'[r // CB] in arrived
                        kv_tile(jobs, r)
                    elif act[0] == 'H':
                        assert 'wxyz'[r // CB] in arrived and 'M' in did
                        items += [h_item(r, i, ('N', r) in did) for i in range(T // LP)]
                    elif act[0] == 'N':
                        assert 'wxyz'[r // CB] in arrived
                        items += [n_item(r, i) for i in range(T // LP)]
                    elif act[0] == 'Q':
                        assert all(('h', r, i) in did for i in range(T // LP))
                        q_tile(jobs, r)
                    elif act[0] == 'Y':
                        def zero_item(n0):
                            def fn(dep):
                                zero = jnp.where(dep > jnp.inf, jnp.uint32(1), jnp.uint32(0))
                                for n in range(n0, min(n0 + 4, _MIX3 + m3_scr.shape[0])):
                                    mw_scr.bitcast(U32)[n] = _rows(zero, T // 2)
                            return fn
                        items += [zero_item(n0) for n0 in range(_MIX3, _MIX3 + m3_scr.shape[0], 4)]
                    elif act[0] == 'F':
                        assert all(('K', SB * r + k_) in did for k_ in range(SB))
                        items += _v_form_items(v_scr, (pf_scr, vf_scr), r)
                    elif act[0] == 'C':
                        assert all('abcd'[t[1] // CB] in arrived for p_ in _C_GROUPS[r] for t in p_[0])
                        items += sum_items(
                            32, _C_GROUPS[r], _C_SUMS, cs_scr,
                            lambda r_, k, rows: c_ref[r_ * T + rows.start:r_ * T + rows.stop, _tile(k)], False)
                    else:
                        assert act[0] == 'S' and all(('h', t[1], T // LP - 1) in did for p_ in _H_GROUPS[r] for t in p_[0])
                        items += h_sums(32 if span else 16, r)
                release(jobs, span, items)
        assert not jobs.side
    assert arrived == set(named) and all((k_, r) in did for k_ in 'KHQ' for r in range(nb))
    assert all((k_, r) in did for k_ in 'CS' for r in range(2)) and 'L' in did
    assert all(('F', r) in did for r in range(SB))

    def mixer_prep(g):
        sl = jnp.minimum(g, NSL - 1)
        rows = pl.ds(pl.multiple_of(sl * MS, MS), MS)

        def part(m, forms):
            def fn(dep):
                base = {}

                def get(i, k):
                    if (i, k) not in base:
                        rb, cb = (i, k) if m == 2 else (k, i)
                        r0 = mixw[m][2] + rb * MS
                        v = _after(st_in[r0:r0 + MS, _tile(cb)].astype(F32), _rows(dep, MS))
                        if m == 3 and (rb + 1) * T > Fd:
                            v = jnp.where(rb * T + sl * MS < Fd, v, 0.0)
                        base[i, k] = v
                    return base[i, k]

                for f in forms:
                    v = _form(f, get)
                    mw_scr[_MIXW[m, f], rows, :] = (0.5 * v if m % 2 else v).astype(BF16)
            return fn

        items = []
        for m in range(4):
            forms = [f for mm_, f in _MIXW if mm_ == m]
            cur, terms = [], set()
            for f in forms:
                new_terms = terms | {t[1:] for t in f}
                if cur and 3 * len(new_terms) + sum(2 * len(x) + 1 for x in cur + [f]) > MWOPS:
                    items.append(part(m, cur))
                    cur, terms = [], set()
                cur.append(f)
                terms |= {t[1:] for t in f}
            items.append(part(m, cur))

        n3 = sum(m == 2 for m, _ in _MIXW)
        first = min(n for (m, _), n in _MIXW.items() if m == 2)
        per = -(-n3 // (nattn - 1 - NSL))

        def turn(j):
            def fn(dep):
                n = jnp.minimum(jnp.maximum(g - NSL, 0) * per + j, n3 - 1)
                w = _tie(_ld(mw_scr, first + n), dep).T
                m3_scr[n] = w
                return pltpu.bitcast(pltpu.bitcast(w, U32)[T // 2 - 8:], F32)
            return fn

        return items + [turn(j) for j in range(per)]

    def stage_wait():
        for cp in pcopies(0):
            cp.wait()
        pltpu.make_async_copy(st_in, st_in, wsem.at[7]).wait()

    def attn_body(g, carry):
        side = _gap_items(work, gap_scr) + _weight_form_items(work, gap_scr, wt_scr, wf_scr, (0, 1, 2))
        bufs = (q_scr, k_scr, v_scr, (pf_scr, vf_scr), wo_buf, acc_scr, flag_scr)
        _attention_step(*bufs, g >> 16, side)

        @pl.when(g + 1 < nattn)
        def _():
            copies = stage_in(g + 1) + [ocopy(g + 1)]
            for cp in copies:
                cp.start()
            bufs = (h_scr, hs_scr, c_ref, cs_scr, wf_scr, q_scr, k_scr, v_scr, (pf_scr, vf_scr))
            side = [(SD0 + int(i * SDS), fn) for i, fn in enumerate(mixer_prep(g))]
            _proj_step(*bufs, scale, gap_scr, side)
            for cp in prep_in(g + 1):
                cp.start()
            stage_wait()
            ocopy(g + 1).wait()

        return carry

    stage_wait()
    for cp in cp_late:
        cp.start()
    jax.lax.fori_loop(0, nattn, attn_body, 0)

    def safe_pair(g, carry):
        copies = pcopies(g) + [ocopy(g)]
        for cp in copies:
            cp.start()
        for cp in copies:
            cp.wait()
        for buf, j0, transpose in ((wk_buf, 0, False), (wv_buf, kc, True), (wq_buf, 2 * kc, False)):
            for (j, hd), w in _pair_tiles(buf, transpose).items():
                w_scr[hd, j0 + j] = w

        def tile(u, carry):
            r, hd = u // 2, u % 2
            rows = pl.ds(pl.multiple_of(r * T, T), T)
            ct = [c_ref[rows, _tile(j)] for j in range(kc)]
            k_scr[u] = sum(_dot(ct[j], _ld(w_scr, hd, j)) for j in range(kc)).astype(BF16)
            v_scr[u] = sum(_dot_nt(_ld(w_scr, hd, kc + j), ct[j]) for j in range(kc)).astype(BF16)
            q = sum(_dot(_ld(h_scr, r, j), _ld(w_scr, hd, 2 * kc + j)) for j in range(km))
            q_scr[u] = (q * scale).astype(BF16)
            return carry

        jax.lax.fori_loop(0, 2 * nb, tile, 0)
        _attention_safe(q_scr, k_scr, v_scr, wo_buf, acc_scr)
        return carry

    @pl.when(jnp.max(flag_scr[...]) > 0)
    def _():
        jax.lax.fori_loop(0, nb, zero, 0)
        jax.lax.fori_loop(0, nattn, safe_pair, 0)

    for cp in cp_late:
        cp.wait()
    mod = _dot(silu_cond(), wmb_ref[...])
    mod_scr[:, 2 * M:4 * M] = mod[:, 0:2 * M]
    mod_scr[:, 4 * M:5 * M] = 1.0 + mod[:, 2 * M:3 * M]
    mod_scr[:, 5 * M:6 * M] = mod[:, 3 * M:4 * M]
    OFF = x_ref.shape[0] - S
    CAR = t_scr.shape[0] - RB

    def p1(r0, l0, n, dep=None):
        ga = mod_scr[:, 2 * M:3 * M]
        if dep is not None:
            ga = jnp.concatenate([_after(ga[:, 0:T], dep), ga[:, T:]], axis=1)
        rows = pl.ds(r0, n)
        x1 = x_ref[rows, :].astype(F32) + _rows(ga, n) * acc_scr[rows, :]
        xh_scr[0, l0:l0 + n, :] = x1
        hb = _ln(x1) * _rows(mod_scr[:, 4 * M:5 * M], n) + _rows(mod_scr[:, 3 * M:4 * M], n)
        xh_scr[1, l0:l0 + n, :] = hb
        return hb

    HT = T // 2
    last8 = lambda v: jnp.max(v[:, M - T:].reshape(PC // 8, 8, T), axis=0)

    def p1_store(r0, c, dep=None):
        v = _ln(p1(r0 + c * PC, OFF + c * PC, PC, dep))
        a1_scr[c * PC:(c + 1) * PC, :] = v
        return last8(v)

    def p1_first(r0, c, dep):
        return last8(p1(r0 + c * PC, OFF + c * PC, PC, dep))

    def p1_second(c, dep):
        hb = xh_scr[1, OFF + c * PC:OFF + (c + 1) * PC, :]
        v = _ln(jnp.concatenate([_after(hb[:, :T], _rows(dep, PC)), hb[:, T:]], axis=1))
        a1_scr[c * PC:(c + 1) * PC, :] = v
        return last8(v)

    t_scr[RB:RB + CAR - OFF, :] = jnp.zeros((CAR - OFF, M), F32)
    t_scr[RB + CAR - OFF:RB + CAR, :] = _gelu2(_dot(_ln(p1(0, 0, OFF)).astype(BF16), w1_ref[...]))
    for c in range(RB // PC):
        p1_store(OFF, c)

    def out_copy(i):
        rows = pl.ds(i * T if isinstance(i, int) else pl.multiple_of(i * T, T), T)
        return pltpu.make_async_copy(out_buf.at[rows, :], out_hbm.at[rows, :], osem.at[i])

    def b_body(r, carry):
        gb = _rows(mod_scr[:, 5 * M:6 * M], T)
        r0 = pl.multiple_of(r * RB, RB)
        n0 = pl.multiple_of(jnp.minimum(r0 + RB, S - RB) + OFF, OFF)
        nh = RB // T
        now = [0]
        due = []
        pace = []

        def p1_item(c, part):
            def fn(dep):
                v = (p1_store(n0, c, dep) if not PSPLIT else p1_first(n0, c, dep) if part == 0 else p1_second(c, dep))
                due.append((now[0] + PD, v))
                due.sort(key=lambda e: e[0])
            return fn

        pace += [(P0 + i * PSTEP + part * PSPLIT, p1_item(i, part)) for i in range(RB // PC)
                 for part in range(2 if PSPLIT else 1)]
        pace.sort(key=lambda e: e[0])

        def mm(lhs, wts, dot=_dot):
            acc = None
            for x, w in zip(lhs, wts):
                if due and due[0][0] <= now[0]:
                    w = _tie(w, due.pop(0)[1])
                v = dot(x, w)
                now[0] += x.shape[0] / HT
                acc = v if acc is None else v + acc
                if pace and pace[0][0] <= now[0]:
                    pace.pop(0)[1](v[0:8, :])
            return acc

        def fast(m, base, finish, hook=None):
            prods = _MIX[m]
            nsub = MSUB[m]
            n = HT // nsub
            done = {}
            for sub in range(nsub):
                left, acc, cache = {}, {}, {}
                for _, _, outs in prods:
                    for _, i, h in outs:
                        left[i, h] = left.get((i, h), 0) + 1

                def act(form):
                    sign, form = _canon(form)
                    if form not in cache:
                        cache[form] = _form(
                            form, lambda k, h: base(k)[h * HT + sub * n:h * HT + (sub + 1) * n]).astype(BF16)
                    return sign, cache[form]

                for pi, (wf, af, outs) in enumerate(prods):
                    w = _ld(m3_scr, _MIXW[m, wf] - _MIX3) if m == 2 else _ld(mw_scr, _MIXW[m, wf])
                    if af is None:
                        k = wf[0][2]
                        v = mm([jnp.concatenate([act(((1, k, h),))[1] for h in range(2)], axis=0)], [w])
                        sign, parts = 1, [v[:n], v[n:]]
                    else:
                        sign, x = act(af)
                        parts = [mm([x], [w])] * len(outs)
                    for (s_, i, h), v in zip(outs, parts):
                        s_ = s_ * sign
                        if (i, h) not in acc:
                            acc[i, h] = (s_, v)
                        else:
                            s0, u = acc[i, h]
                            acc[i, h] = (s0, u + v if s0 == s_ else u - v) if s0 > 0 or s_ < 0 else (1, v - u)
                        left[i, h] -= 1
                        if not left[i, h]:
                            s0, done[i, h, sub] = acc.pop((i, h))
                            assert s0 > 0
                            if all((i, hh, ss) in done for hh in range(2) for ss in range(nsub)):
                                finish(i, jnp.concatenate([done[i, hh, ss] for hh in range(2)
                                                           for ss in range(nsub)], axis=0))
                    if hook is not None and sub == nsub - 1:
                        hook(pi, act)

        t_scr[0:CAR, :] = t_scr[RB:RB + CAR, :]
        for hf in range(nh):
            def put_t(n, v):
                t = _gelu2(v)
                if hf == nh - 1:
                    t = jnp.concatenate([t[:T - OFF], jnp.where(r < nrb - 1, t[T - OFF:], 0.0)], axis=0)
                t_scr[CAR + hf * T:CAR + (hf + 1) * T, _tile(n)] = t

            fast(0, lambda k: a1_scr[_tile(hf), _tile(k)], put_t)
        cq = M // 4
        shifts = (-1, 1, -2, 2)
        lane = jax.lax.broadcasted_iota(jnp.int32, (T, T), 1)
        y1, a3 = [], []
        for hf in range(nh):
            base = CAR - OFF + hf * T
            sh = []
            for j in range(km):
                g_lo, g_hi = (j * T) // cq, ((j + 1) * T - 1) // cq
                assert g_hi - g_lo <= 1
                v = t_scr[base + shifts[g_lo]:base + shifts[g_lo] + T, _tile(j)]
                if g_hi != g_lo:
                    v2 = t_scr[base + shifts[g_hi]:base + shifts[g_hi] + T, _tile(j)]
                    v = jnp.where(lane < g_hi * cq - j * T, v, v2)
                else:
                    v = jnp.where(lane < T, v, 0.0)
                sh.append(v)
            hs = {}
            fast(1, lambda k: sh[k], hs.__setitem__)
            hs = jnp.concatenate([hs[n] for n in range(km)], axis=1)
            y1.append(hs + xh_scr[1, _tile(hf), :])
            z_scr[_tile(hf), :] = xh_scr[0, _tile(hf), :] + gb * y1[hf]
            a3.append({})

            def ln_item(hf, c):
                def item(dep):
                    n = HT // NLN
                    for d in (0, HT):
                        v = y1[hf][d + c * n:d + (c + 1) * n]
                        if dep is not None:
                            v = jnp.concatenate([_after(v[:, :T], _rows(dep, n)), v[:, T:]], axis=1)
                        a3[hf][d + c * n] = _ln(v)
                return item

            ln_item(hf, 0)(None)
            pace += [(now[0] + LN0 + (c - 1) * LNS * (1 + hf), ln_item(hf, c)) for c in range(1, NLN)]
            pace.sort(key=lambda e: e[0])
        xh_scr[:, 0:OFF, :] = xh_scr[:, RB:RB + OFF, :]
        z_scr[pl.ds(pl.multiple_of(RB + (r >> 16) * 8, 8), 8), :] = jnp.zeros((8, M), F32)
        h3 = []
        for hf in range(nh):
            assert len(a3[hf]) == 2 * NLN
            af = jnp.concatenate([a3[hf][key] for key in sorted(a3[hf])], axis=0)
            row = {}
            narrow = []

            def hook(pi, act):
                j, rem = divmod(pi - NAR0, NARS)
                if rem == 0 and 0 <= j < km:
                    full = jnp.concatenate([act(((1, j, h),))[1] for h in range(2)], axis=0)
                    v = mm([w3_ref[:, _tile(j)]], [full], _dot_nt)
                    narrow[:] = [v + narrow[0] if narrow else v]

            def put_h(n, v):
                row[n] = _gelu2(v)
                if GD:
                    due.append((now[0] + GD, jnp.max(row[n].reshape(T // 8, 8, T), axis=0)))
                    due.sort(key=lambda e: e[0])

            fast(2, lambda k: af[:, _tile(k)], put_h, hook)
            fw = w3_ref.shape[0]
            row[Fd // T] = jnp.concatenate([_gelu2(narrow[0]), jnp.zeros((T - fw, T), F32)], axis=0).T
            h3.append(row)
        for hf in range(nh):
            rows = pl.ds(pl.multiple_of(r0 + hf * T, T), T)

            def finish(n, v):
                out_buf[rows, _tile(n)] = (z_scr[_tile(hf), _tile(n)] + gb[:, _tile(n)] * v).astype(out_buf.dtype)

            fast(3, lambda k: h3[hf][k], finish)
            out_copy(r * nh + hf).start()
        assert not pace
        return carry

    jax.lax.fori_loop(0, nrb, b_body, 0)
    for i in range(nb):
        out_copy(i).wait()


@jax.jit
def pallas_adaLN_cond__compressed_kv_cla__mixer_s_mlp__prompt_kernel(
    A_x: jax.Array,
    A_c_kv: jax.Array,
    A_w_q: jax.Array,
    A_w_uk: jax.Array,
    A_w_uv: jax.Array,
    A_w_o: jax.Array,
    B_x: jax.Array,
    B_w1: jax.Array,
    B_w2: jax.Array,
    B_w3: jax.Array,
    B_w4: jax.Array,
    c: jax.Array,
    w_mod: jax.Array,
):
    _, S, M = A_x.shape
    Dc = A_c_kv.shape[2]
    H, D = A_w_q.shape[1], A_w_q.shape[2]
    Fd = B_w3.shape[1]
    assert D == T and A_c_kv.shape[1] == S and Dc == 4 * T and M == 5 * T and 13 * T < Fd < 14 * T and S == 16 * T
    vmem = pltpu.VMEM
    packed = lambda *lead: vmem(lead + (T, T), BF16)
    out = pl.pallas_call(
        _kernel,
        in_specs=[pl.BlockSpec(memory_space=pltpu.HBM)] * 12,
        out_specs=pl.BlockSpec(memory_space=pltpu.HBM),
        out_shape=jax.ShapeDtypeStruct((S, M), A_x.dtype),
        scratch_shapes=[
            vmem((S + 16, M), BF16),
            vmem((S, Dc), BF16),
            vmem((1, M), BF16),
            vmem((M, 2 * M), BF16),
            vmem((M, 4 * M), BF16),
            vmem((M, M), BF16),
            vmem((Fd % T, M), BF16),
            vmem((M, D), U32),
            vmem((Dc, D), U32),
            vmem((Dc, D), U32),
            vmem((2 * D, M), BF16),
            vmem((S, M), A_x.dtype),
            pltpu.SemaphoreType.DMA((15,)),
            pltpu.SemaphoreType.DMA((8,)),
            pltpu.SemaphoreType.DMA((S // T,)),
            vmem((8, 6 * M), F32),
            vmem((S // T, M // T, T, T), BF16),
            vmem((len(_C_SUMS), T, T), BF16),
            vmem((len(_H_SUMS), T, T), BF16),
            packed(2, M // T + 2 * (Dc // T)),
            packed(2 * S // T),
            packed(2 * S // T),
            packed(2 * S // T),
            vmem((S + 16, M), F32),
            vmem((S, M), F32),
            vmem((2, RB + 16, M), F32),
            vmem((RB, M), F32),
            vmem((RB + 32, M), F32),
            vmem((RB + 8, M), F32),
            packed(len(_MIXW)),
            packed(sum(m == 2 for m, _ in _MIXW)),
            vmem((Dc // T, T, T), U32),
            vmem((len(_WF), T, T), BF16),
            vmem((3, 8, T), jnp.int32),
            vmem(((2 * (M // T) + Fd // T + -(-Fd // T)) * 16, M), BF16),
            vmem((_FENCE + 1, T, T), BF16),
            vmem((_FENCE + 1, T, T), BF16),
            vmem((8, T), F32),
        ],
        compiler_params=pltpu.CompilerParams(
            vmem_limit_bytes=100 * 1024 * 1024,
            disable_bounds_checks=True,
        ),
    )(
        A_x.reshape(S, M), A_c_kv.reshape(S, Dc),
        A_w_q, A_w_uk, A_w_uv,
        A_w_o.reshape(H // 2, 2 * D, M),
        B_w1, B_w2, B_w3.T, B_w4, c, w_mod,
    )
    return out.reshape(1, S, M)
```

```python
import functools
import math

import jax
import jax.numpy as jnp
import jax.experimental.pallas as pl
import jax.experimental.pallas.tpu as pltpu

F32 = jnp.float32
BF16 = jnp.bfloat16
U32 = jnp.uint32
NT = (((1,), (1,)), ((), ()))
T = 128
EPS = 1e-5
LOG2E = math.log2(math.e)

L_LO, L_HI, L_RATIO = 2.0 ** -24, 2.0 ** 24, 4.0

LAT_0, LAT_A = 32, 16
LAT_B = 20
RES, OEND = 32, 24
ONV = 0.7
QT = (4, 6)
SIDE0, SIDE1 = 8, 60
SLAG, SDUE = 3, 8
SG0, SG1 = 6, 4
WFN = (4, 4, 6)
SD0, SDS = 4, 1.5
VF0, VFS = 4, 1.6
PDUE = 20
MWOPS = 70
RB = 256
PC = 32
P0, PSTEP, PSPLIT, PD = 300, 34, 40, 36
NLN, LN0, LNS = 4, 4, 5
GD = 36
NAR0, NARS = 10, 10
LP = 16
SP0, SP1 = 76, 38
_prologue = lambda: ('|kva|Z; |b|; kva|wc|Y0@56 K0123; bw|xdn|C0@56 N0123@52 K4567; cx|mq|N4567@52 F0@56 K89ab; '
            'd|y|C1@56 F1@56 Kcdef; nmq|zo|M H01 H234567@30 F2@36 Q0123; y||L H89ab@30 F3@36 Q4567; '
            'zo||Hcdef@30 S0@%d Q89ab S1@%d Qcdef' % (SP0, SP1))


def _dot(a, b):
    return jnp.dot(a, b, preferred_element_type=F32)


def _dot_nt(a, b):
    return jax.lax.dot_general(a, b, NT, preferred_element_type=F32)


def _ln(x):
    m = jnp.mean(x, axis=-1, keepdims=True)
    xc = x - m
    v = jnp.mean(xc * xc, axis=-1, keepdims=True)
    return xc * jnp.exp2(jnp.log(v + EPS) * (-0.5 * LOG2E))


def _rows(v, n):
    return jnp.broadcast_to(v[None], (n // 8, 8, v.shape[1])).reshape(n, v.shape[1])


def _gelu2(x):
    c0 = math.sqrt(2.0 / math.pi)
    return x + x * jnp.tanh(x * (c0 + (c0 * 0.044715) * (x * x)))


def _after(x, dep):
    return jnp.where(dep > jnp.inf, dep, x)


def _tie(x, dep):
    xu = pltpu.bitcast(x, U32)
    first = jnp.where(dep > jnp.inf, jnp.uint32(0), xu[:8])
    return pltpu.bitcast(jnp.concatenate([first, xu[8:]], axis=0), BF16)


def _tile(j):
    return slice(j * T, (j + 1) * T)


def _ld(ref, *idx):
    return pltpu.bitcast(ref.bitcast(U32)[idx], BF16)


def _group(rows, cols, pairs):
    xs, ys = dict.fromkeys(x for x, _ in pairs), dict.fromkeys(y for _, y in pairs)
    used = set(xs) | set(ys) | {(x[0], y[1]) for x, y in pairs} | {(y[0], x[1]) for x, y in pairs}
    prods = []
    for n, r in enumerate(rows):
        for i, k in [x for x in xs if x[0] == r]:
            mates = [y for x, y in pairs if x == (i, k)]
            prods.append((((1, i, k),) + tuple((1, i, k2) for _, k2 in mates), ((1, k, 0),),
                          ((1, i, 0), (-1, i, 1))))
            prods.append((((1, i, k),) + tuple((-1, i2, k) for i2, _ in mates), ((1, k, 0), (1, k, 1)),
                          ((1, i, 1),)))
        for i2, k2 in [y for y in ys if y[0] == r]:
            mates = [x for x, y in pairs if y == (i2, k2)]
            prods.append((((1, i2, k2),) + tuple((1, i2, k) for _, k in mates), ((1, k2, 1),),
                          ((1, i2, 1), (-1, i2, 0))))
            prods.append((((1, i2, k2),) + tuple((-1, i, k2) for i, _ in mates), ((1, k2, 0), (1, k2, 1)),
                          ((1, i2, 0),)))
        prods += [(((1, r, k),), ((1, k, h),), ((1, r, h),)) for k in cols if (r, k) not in used for h in (0, 1)]
        for (i, k), (i2, k2) in pairs:
            if r in (i, i2) and i + i2 - r in rows[n + 1:]:
                prods.append((((1, i, k2),), ((1, k2, 0), (-1, k, 0)), ((1, i2, 0), (1, i, 0))))
                prods.append((((1, i2, k), (1, i, k2)), ((1, k, 0), (1, k2, 1)), ((1, i2, 0), (1, i, 1))))
                prods.append((((1, i2, k),), ((1, k, 1), (-1, k2, 1)), ((1, i2, 1), (1, i, 1))))
    return prods


def _all_pairs(xrows, yrows):
    return [((x, a), (y, b)) for a, x in enumerate(xrows) for b, y in enumerate(yrows) if a != b]


_PAIRS65 = [((x[0] + 10, x[1]), (y[0] + 10, y[1])) for x, y in (
    ((0, 1), (1, 0)), ((0, 1), (5, 2)), ((2, 3), (1, 0)), ((2, 3), (3, 1)), ((2, 3), (5, 2)), ((3, 2), (1, 0)),
    ((4, 4), (0, 3)), ((4, 4), (1, 0)), ((4, 4), (3, 1)), ((4, 4), (5, 2)))]
_C_GROUPS = [_group(range(r, r + 8), range(4), _all_pairs(range(r, r + 4), range(r + 4, r + 8))) for r in (0, 8)]
_H_GROUPS = [_group(range(10), range(5), _all_pairs(range(5), range(5, 10))),
             _group(range(10, 16), range(5), _PAIRS65)]
_sum_index = lambda groups: {f: n for n, f in enumerate(
    dict.fromkeys(t[0] for g in groups for t in g if len(t[0]) > 1))}
_C_SUMS, _H_SUMS = _sum_index(_C_GROUPS), _sum_index(_H_GROUPS)


def _cells(rows, cols, pairs):
    xs = list(dict.fromkeys(p[0] for p in pairs))
    ys = list(dict.fromkeys(p[1] for p in pairs))
    used = set(xs + ys) | {(x[0], y[1]) for x, y in pairs} | {(y[0], x[1]) for x, y in pairs}

    def home_x(i, k):
        mates = [y for x, y in pairs if x == (i, k)]
        return [(((1, i, k),) + tuple((1, i, k2) for _, k2 in mates), ((1, k, 0),), ((1, i, 0), (-1, i, 1))),
                (((1, i, k),) + tuple((-1, i2, k) for i2, _ in mates), ((1, k, 0), (1, k, 1)), ((1, i, 1),))]

    def home_y(i2, k2):
        mates = [x for x, y in pairs if y == (i2, k2)]
        return [(((1, i2, k2),) + tuple((1, i2, k) for _, k in mates), ((1, k2, 1),), ((1, i2, 1), (-1, i2, 0))),
                (((1, i2, k2),) + tuple((-1, i, k2) for i, _ in mates), ((1, k2, 0), (1, k2, 1)), ((1, i2, 0),))]

    def cross(x, y):
        (i, k), (i2, k2) = x, y
        return [(((1, i, k2),), ((1, k2, 0), (-1, k, 0)), ((1, i2, 0), (1, i, 0))),
                (((1, i2, k), (1, i, k2)), ((1, k, 0), (1, k2, 1)), ((1, i2, 0), (1, i, 1))),
                (((1, i2, k),), ((1, k, 1), (-1, k2, 1)), ((1, i2, 1), (1, i, 1)))]

    direct = lambda i: [(((1, i, k),), None, ((1, i, 0), (1, i, 1))) for k in cols if (i, k) not in used]
    single = lambda i: ([t for x in xs if x[0] == i for t in home_x(*x)]
                        + [t for y in ys if y[0] == i for t in home_y(*y)] + direct(i))
    prods = []
    for n, i in enumerate(rows):
        prods += single(i)
        for i2 in rows[n + 1:]:
            for x, y in pairs:
                if {x[0], y[0]} == {i, i2}:
                    prods += cross(x, y)
    return prods


_square = lambda q: [((a, a), (q + b, b)) for a in range(q) for b in range(q) if a != b]
_shift = lambda pairs, r0: [((x[0] + r0, x[1]), (y[0] + r0, y[1])) for x, y in pairs]
_flip = lambda pairs: [(x[::-1], y[::-1]) for x, y in pairs]
_P35 = [((1, 2), (0, 4)), ((1, 2), (2, 1)), ((2, 3), (0, 4)), ((2, 3), (1, 0))]
_P45 = [((0, 2), (1, 1)), ((2, 4), (0, 3)), ((2, 4), (1, 1)), ((2, 4), (3, 2)), ((3, 0), (0, 3)), ((3, 0), (1, 1))]
_P55 = [((2, 1), (0, 4)), ((2, 1), (1, 0)), ((2, 1), (3, 2)), ((2, 1), (4, 3)), ((3, 3), (0, 4)), ((3, 3), (1, 0)),
        ((4, 2), (0, 4)), ((4, 2), (1, 0))]
_MIX = [_cells(range(5), range(5), _P55), _cells(range(5), range(5), _P55),
        _cells(range(13), range(5), _square(5) + _shift(_P35, 10)),
        _cells(range(5), range(14), _flip(_square(5) + _shift(_P45, 10)))]
_MIXW = {(m, f): n for n, (m, f) in enumerate(dict.fromkeys((m, t[0]) for m in range(4) for t in _MIX[m]))}
_MIX3 = min(n for (m, _), n in _MIXW.items() if m == 2)


def _form(form, get):
    acc = None
    for sign, i, j in form:
        v = get(i, j)
        acc = v if acc is None else (acc + v if sign > 0 else acc - v)
    return acc


def _gap_items(bufs, gap_scr):
    items = []
    for n, buf in enumerate(bufs):
        acc = []

        def part(r0, buf=buf, acc=acc):
            def fn(dep):
                wu = jnp.concatenate([buf[r:r + 8, :] for r in range(r0, r0 + T, 32)])
                mask = jnp.full((8, T), 0x7FFF0000, U32)
                if dep is not None:
                    mask = jnp.where(dep > jnp.inf, jnp.uint32(0), mask)
                mask = _rows(mask, 32)
                new = [jnp.sum(pltpu.bitcast(v & mask, F32).reshape(4, 8, T), axis=0) for v in (wu << 16, wu)]
                acc[:] = [u + v for u, v in zip(acc, new)] if acc else new
            return fn

        def last(_, n=n, acc=acc):
            bits = []
            for v in acc:
                l1 = jnp.sum(jnp.sum(v, axis=1, keepdims=True), axis=0, keepdims=True)
                bits.append(pltpu.bitcast(jnp.broadcast_to(l1, (8, T)), jnp.int32) >> 8)
            gap = jnp.clip((bits[0] - bits[1] + (1 << 14)) >> 15, -8, 8) << 23
            gap_scr[n] = gap
            return pltpu.bitcast(gap, F32)

        items += [part(r0) for r0 in range(0, buf.shape[0], T)] + [last]
    return items


def _pair_tiles(w_ref, transpose=False):
    tiles = {}
    for j in range(w_ref.shape[0] // T):
        wu = w_ref[_tile(j), :]
        if transpose:
            wu = wu.T
        tiles[j, 0] = pltpu.bitcast(wu << 16, F32).astype(BF16)
        tiles[j, 1] = pltpu.bitcast(wu & jnp.uint32(0xFFFF0000), F32).astype(BF16)
    return tiles


def _canon(form):
    if form[-1][0] < 0 and form[0][1:] > form[1][1:]:
        return -1, ((1,) + form[1][1:], (-1,) + form[0][1:])
    return 1, form


_w_forms = lambda groups: list(dict.fromkeys(_canon(t[1])[1] for g in groups for t in g))
_WF = {key: n for n, key in enumerate([(m, f) for m, groups in enumerate((_C_GROUPS, _C_GROUPS, _H_GROUPS))
                                       for f in _w_forms(groups)])}


def _weight_form_items(bufs, gap_scr, wt_scr, wf_scr):
    n = 16
    items = []

    def flip(j):
        def fn(dep):
            wu = bufs[1][_tile(j), :]
            wu = (wu if dep is None else jnp.where(_rows(dep, T) > jnp.inf, jnp.uint32(0), wu)).T
            wt_scr[j] = wu
            return pltpu.bitcast(wu[T - 8:], F32)
        return fn

    def part(m, r0, forms):
        def fn(dep):
            fac = pltpu.bitcast(0x3F800000 + gap_scr[m], F32)
            mask = jnp.full((8, T), 0xFFFF0000, U32)
            sh = jnp.full((8, T), 16, U32)
            if dep is not None:
                mask = jnp.where(dep > jnp.inf, jnp.uint32(0), mask)
                sh = jnp.where(dep > jnp.inf, jnp.uint32(0), sh)
            fac, mask, sh = _rows(fac, n), _rows(mask, n), _rows(sh, n)
            base = {}

            def get(k, h):
                if (k, h) not in base:
                    wu = wt_scr[k, r0:r0 + n, :] if m == 1 else bufs[m][k * T + r0:k * T + r0 + n, :]
                    base[k, h] = pltpu.bitcast(wu & mask, F32) * fac if h else pltpu.bitcast(wu << sh, F32)
                return base[k, h]

            for f in forms:
                wf_scr[_WF[m, f], r0:r0 + n, :] = _form(f, get).astype(BF16)
        return fn

    for m in range(3):
        forms = [f for mm, f in _WF if mm == m]
        if m == 1:
            items += [flip(j) for j in range(bufs[1].shape[0] // T)]
        per = -(-len(forms) // WFN[m])
        forms.sort(key=lambda f: sorted({t[1] for t in f}))
        items += [part(m, r0, forms[i:i + per]) for r0 in range(0, T, n) for i in range(0, len(forms), per)]
    return items


def _run_group(jobs, prods, a_get, w, transposed, finish):
    left = {}
    for _, _, outs in prods:
        for _, i, h in outs:
            left[i, h] = left.get((i, h), 0) + 1
    acc = {}
    for af, bf, outs in prods:
        sign, wt = w(bf)
        m = jobs.mm([wt], [a_get(af)], _dot_nt) if transposed else jobs.mm([a_get(af)], [wt], _dot)
        for s_, i, h in outs:
            if (i, h) not in acc:
                acc[i, h] = (s_ * sign, m)
            else:
                s0, v = acc[i, h]
                acc[i, h] = (s0, v + m if s0 == s_ * sign else v - m) if s0 > 0 or s_ * sign < 0 else (1, m - v)
            left[i, h] -= 1
            if not left[i, h]:
                s0, v = acc.pop((i, h))
                assert s0 > 0
                finish(2 * i + h, v)


class _Jobs:
    def __init__(self, side=()):
        self.res = []
        self.side = list(side)
        self.due = []

    def mm(self, lhs, wt, dot):
        acc = None
        for x, w in zip(lhs, wt):
            if self.due and self.due[0][0] <= len(self.res):
                x = _tie(x, self.due.pop(0)[1])
            v = dot(x, w)
            self.res.append(v)
            acc = v if acc is None else v + acc
            rel = 4 * (len(self.res) % 4)
            while self.side and self.side[0][0] <= len(self.res):
                out = self.side.pop(0)[1](v[8 * rel:8 * rel + 8, :])
                if out is not None:
                    self.due.append((len(self.res) + PDUE, out))
                rel = (rel + 2) % 16
        return acc


def _proj_step(h_scr, hs_scr, c_ref, cs_scr, wf_scr, q_scr, k_scr, v_scr, pf, scale, shifts, side):
    def weight(m):
        def get(form):
            sign, form = _canon(form)
            return sign, _ld(wf_scr, _WF[m, form])
        get.inv = pltpu.bitcast(0x3F800000 - shifts[m], F32)
        return get

    wk, wvT, wq = weight(0), weight(1), weight(2)
    c_get = lambda f: _ld(cs_scr, _C_SUMS[f]) if len(f) > 1 else c_ref[_tile(f[0][1]), _tile(f[0][2])]
    h_get = lambda f: _ld(hs_scr, _H_SUMS[f]) if len(f) > 1 else _ld(h_scr, f[0][1], f[0][2])

    def put(dst, w, mul=None):
        muls = [mul, _rows(w.inv if mul is None else w.inv * mul, T)]

        def fn(u, v):
            v = (v if muls[u % 2] is None else v * muls[u % 2]).astype(BF16)
            dst[u] = v.T if mul is not None and u in QT else v
        return fn

    jobs = _Jobs(side)
    put_v, stored = put(v_scr, wvT), set()
    nxt = [0]

    def fin_v(u, v):
        put_v(u, v)
        stored.add(u)
        for J in range(SB):
            if all(2 * (SB * J + k) + h in stored for k in range(SB) for h in range(2)) and ('J', J) not in stored:
                stored.add(('J', J))
                for fn in _v_form_items(v_scr, pf, J):
                    nxt[0] = max(nxt[0] + VFS, len(jobs.res) + VF0)
                    jobs.side.append((int(nxt[0]), fn))
                jobs.side.sort(key=lambda e: e[0])

    kk, vv, qq = ((c_get, wk, False, put(k_scr, wk)), (c_get, wvT, True, fin_v),
                  (h_get, wq, False, put(q_scr, wq, scale)))
    for prods, args in ((_C_GROUPS[0], kk), (_C_GROUPS[0], vv), (_C_GROUPS[1], vv), (_C_GROUPS[1], kk),
                        (_H_GROUPS[0], qq), (_H_GROUPS[1], qq)):
        _run_group(jobs, prods, *args)
    assert not jobs.side and not jobs.due


def _inner_group(rows, cols, pairs):
    xs, ys = dict.fromkeys(x for x, _ in pairs), dict.fromkeys(y for _, y in pairs)
    used = set(xs) | set(ys) | {(x[0], y[1]) for x, y in pairs} | {(y[0], x[1]) for x, y in pairs}
    prods = []
    for i, j in xs:
        mates = [y for x, y in pairs if x == (i, j)]
        prods.append((((1, i, 0),), ((1, 0, j), (-1, 1, j)), ((1, i, j),) + tuple((1, i2, j) for i2, _ in mates)))
        prods.append((((1, i, 0), (1, i, 1)), ((1, 1, j),), ((1, i, j),) + tuple((-1, i, j2) for _, j2 in mates)))
    for i2, j2 in ys:
        mates = [x for x, y in pairs if y == (i2, j2)]
        prods.append((((1, i2, 0), (1, i2, 1)), ((1, 0, j2),),
                      ((1, i2, j2),) + tuple((-1, i2, j) for _, j in mates)))
        prods.append((((1, i2, 1),), ((1, 0, j2), (-1, 1, j2)),
                      ((-1, i2, j2),) + tuple((-1, i, j2) for i, _ in mates)))
    prods += [(((1, i, h),), ((1, h, j),), ((1, i, j),))
              for i in rows for j in cols if (i, j) not in used for h in (0, 1)]
    for (i, j), (i2, j2) in pairs:
        lo, hi = min(j, j2), max(j, j2)
        prods.append((((1, i2, 0), (-1, i, 0)), ((1, 0, lo), (1, 0, hi)), ((1, i2, j),)))
        prods.append((((1, i, 0), (1, i2, 1)), ((1, 0, j2), (1, 1, j)), ((1, i, j2), (1, i2, j))))
        prods.append((((1, i, 1), (-1, i2, 1)), ((1, 1, lo), (1, 1, hi)), ((1, i, j2),)))
    return prods


def _o_jobs():
    prods = (_inner_group(range(10), range(5), _all_pairs(range(0, 10, 2), range(1, 10, 2)))
             + _inner_group(range(10, 16), range(5), _PAIRS65))
    row = lambda t: max(i for _, i, _ in t[0])
    unit = lambda t: max(2 * i + h for _, i, h in t[0])
    need = lambda t: unit(t) if row(t) == 15 else 2 * row(t) + 1
    return [(need(t), t) for t in sorted(prods, key=need)]


_O_JOBS = _o_jobs()


SB = 4


class _Star:
    def __init__(self, ts):
        self.ts, self.n = ts, len(ts)
        rn = range(self.n)
        self.pairs = [(i, j) for i in rn for j in rn if i < j]
        self.pf = {f: m for m, f in enumerate([('R', i) for i in rn] + [('C', i) for i in rn]
                                              + [('S', i, j) for i in rn for j in rn if i != j]
                                              + [('A', i, j) for i, j in self.pairs])}
        self.vf = {f: m for m, f in enumerate([('W', i) for i in rn]
                                              + [(q, i, j) for i, j in self.pairs for q in ('Q1', 'Q2', 'Q3')])}
        self.pv = {**{('W', i): ('R', i) for i in rn}, **{('B', i): ('C', i) for i in rn},
                   **{('Q1', i, j): ('S', i, j) for i, j in self.pairs},
                   **{('Q2', i, j): ('A', i, j) for i, j in self.pairs},
                   **{('Q3', i, j): ('S', j, i) for i, j in self.pairs}}

    def products(self, i):
        return [('W', i), ('B', i)] + [(q, i, j) for j in range(i + 1, self.n) for q in ('Q1', 'Q2', 'Q3')]


_FULL = _Star((-1.125, -0.375, 0.375, 1.125))
_HALF = _Star((-0.75, 0.75))
_DCELLS = [(0, 0), (1, 0), (1, 1), (2, 2), (3, 2), (3, 3)]
_HSLOT = (SB - 1) * len(_FULL.pf)
_DSLOT = _HSLOT + len(_HALF.pf)
_VSLOT = _DSLOT + len(_DCELLS)
_VHALF = (SB - 1) * len(_FULL.vf)
_FENCE = _VSLOT + (_VHALF + SB * len(_HALF.vf) + 1) // 2


def _v_slot(star, J, f):
    m = star.vf[f] + J * len(star.vf) + (0 if star is _FULL else _VHALF)
    return _VSLOT + m // 2, m % 2 * (T // 2)


def _v_form_items(v_scr, pf, J):
    n, HT = 16, T // 2

    def item(star, h, r0, pairs):
        def fn(dep):
            ts = [jnp.full((8, T), t, F32) for t in star.ts]
            ts = [_rows(t if dep is None else _after(t, dep), n) for t in ts]

            def get(k, a):
                r = (a * HT + r0) // 2
                return _ld(v_scr, 2 * (SB * J + k) + h, slice(r, r + n // 2)).astype(F32)

            def put(f, v):
                slot, r = _v_slot(star, J, f)
                pf[h][slot, r + r0:r + r0 + n, :] = v.astype(BF16)

            b = {(k, a): get(k, a) for k in sorted({k for pr in pairs or star.pairs for k in pr})
                 for a in range(2)}
            if pairs is None or star.n == 2:
                w = [b[k, 0] + ts[k] * b[k, 1] for k in range(star.n)]
                for k in range(star.n):
                    put(('W', k), w[k])
                for i, j in star.pairs:
                    put(('Q2', i, j), w[i] - w[j])
            for i, j in pairs or ():
                d0, d1 = b[j, 0] - b[i, 0], b[j, 1] - b[i, 1]
                put(('Q1', i, j), d0 + ts[i] * d1)
                put(('Q3', i, j), d0 + ts[j] * d1)
        return fn

    pr = _FULL.pairs
    parts = [(_HALF, _HALF.pairs)]
    if J < SB - 1:
        parts += [(_FULL, x) for x in (None, pr[:2], [pr[2], pr[4]], [pr[3], pr[5]])]
    return [item(star, h, r0, pairs) for h in range(2) for r0 in range(0, HT, n) for star, pairs in parts]


def _job_order(nsb):
    units = [(I, h) for I in range(nsb) for h in range(2)]
    qe, qv = [], []
    for I, h in units:
        qe += [('e', I, h, J, p) for J in range(I) for p in range(SB)] + [('f', I, h)]
        qe += [('d', I, h) + c for c in _DCELLS]
        for i in range(SB):
            qv += [('p', I, h, f, J) for f in _FULL.products(i) for J in range(I)]
            if i >= 2:
                qv += [('p', I, h, f, None) for f in _HALF.products(i - 2)]
            qv += [('v', I, h) + c for c in _DCELLS if c[0] == i]
    qo = [('o', u, j) for j, (u, _) in enumerate(_O_JOBS)]
    cost = dict(e=8, f=8, d=2, p=1, v=2, o=2)
    order, done = [], {}
    now = [0]

    def emit(q):
        job = q.pop(0)
        order.append(job)
        now[0] += cost[job[0]]
        if job[0] == 'd':
            done[job] = now[0]
        elif job[0] == 'v' and job[4] == job[3]:
            done['u', 2 * (SB * job[1] + job[3]) + job[2]] = now[0]
        return cost[job[0]]

    def v_ready():
        if not qv:
            return False
        key = ('d', qv[0][1], qv[0][2], SB - 1, SB - 1)
        return key in done and done[key] + (LAT_0 if qv[0][1:3] == (0, 0) else LAT_A) <= now[0]

    def o_ready():
        return bool(qo) and ('u', qo[0][1]) in done and done['u', qo[0][1]] + LAT_B <= now[0]

    def fill(nv, no):
        n = 0
        while nv > 0 or no > 0 or n % 4:
            if no > 0 and n % 2 == 0 and o_ready() and no * ONV >= nv:
                no -= 2
                n += emit(qo)
            elif v_ready() and (nv > 0 or n % 4):
                c = emit(qv)
                nv -= c
                n += c
            elif o_ready() and n % 2 == 0 and (no > 0 or n % 4 or nv > 0) and len(qo) > RES:
                no -= 2
                n += emit(qo)
            else:
                break

    while qe:
        unit = qe[0][1:3]
        while qv and qv[0][2] == unit[1] and qv[0][1] < unit[0]:
            emit(qv)
        ne = 0
        while qe and ne < 8 and (ne == 0 or (qe[0][0] == 'd' and qe[0][1:3] == unit and ne + 2 <= 8)):
            ne += emit(qe)
        groups = lambda q: sum(cost[j[0]] for j in q) / 8
        old = [j for j in qv if j[1:3] != unit and ('d', j[1], j[2], SB - 1, SB - 1) in done]
        here = [j for j in qe if j[1:3] == unit]
        rest = sum(cost[j[0]] for j in old)
        nv = (rest - LAT_A) / (groups(here) + 1) if here else rest
        no = 2 * max(len(qo) - RES - OEND, 0) / (groups(qe) + 1)
        fill(int(nv + 0.5), int(no + 0.5))
    while qv or qo:
        if qv and v_ready():
            fill(6, 2)
            if not qv:
                continue
        elif o_ready():
            emit(qo)
        else:
            emit(qv or qo)
    return order


def _attention_safe(q_scr, k_scr, v_scr, wo_ref, acc_scr):
    causal = (jax.lax.broadcasted_iota(jnp.int32, (T, T), 0)
              <= jax.lax.broadcasted_iota(jnp.int32, (T, T), 1))

    def unit(u, carry):
        r, hd = u // 2, u % 2

        def block(c, mlo):
            m0, l, o = mlo
            s = _dot_nt(_ld(k_scr, 2 * c + hd), _ld(q_scr, u))
            s = jnp.where(jnp.logical_or(causal, c < r), s, -1e9 * LOG2E)
            m = jnp.maximum(m0, jnp.max(s, axis=0, keepdims=True))
            a = jnp.exp2(m0 - m)
            p = jnp.exp2(s - m)
            return (m, l * a + jnp.sum(p, axis=0, keepdims=True),
                    o * a + _dot(_ld(v_scr, 2 * c + hd), p.astype(BF16)))

        _, l, o = jax.lax.fori_loop(0, r + 1, block, (jnp.full((1, T), -jnp.inf, F32), jnp.zeros((1, T), F32),
                                                      jnp.zeros((T, T), F32)))
        rows = pl.ds(pl.multiple_of(r * T, T), T)
        acc_scr[rows, :] += _dot((o * (1.0 / l)).astype(BF16).T, wo_ref[pl.ds(pl.multiple_of(hd * T, T), T), :])
        return carry

    jax.lax.fori_loop(0, q_scr.shape[0], unit, 0)


def _attention_step(q_scr, k_scr, v_scr, pf, wo_ref, acc_scr, flag_scr, z, side):
    causal = (jax.lax.broadcasted_iota(jnp.int32, (T, T), 0)
              <= jax.lax.broadcasted_iota(jnp.int32, (T, T), 1))
    HT = T // 2
    lsum, lrow, acc, fg, dacc, of, lhs = {}, {}, {}, {}, {}, {}, {}
    res = []
    wo, terms = {}, {}
    left = {}
    done_side = [0, 0]
    chk = [jnp.zeros((8, T), F32), None]
    for _, t in _O_JOBS:
        for _, i, j in t[2]:
            left[i, j] = left.get((i, j), 0) + 1

    def add_l(u, v):
        lsum[u] = v if u not in lsum else lsum[u] + v

    csign = {}

    def p_forms(star, h, slot0, g, tiles, cell, when):
        n = star.n

        def put(f, v):
            pf[h][slot0 + star.pf[f], 16 * g:16 * g + 16, :] = v.astype(BF16)

        for i in range(n):
            row = [cell(i, k) for k in sorted(range(n), key=lambda k: when(i, k))]
            r = functools.reduce(lambda x, y: x + y, row)
            put(('R', i), r)
            add_l(tiles[i], r[:8] + r[8:])
            col = sorted(range(n), key=lambda i2: (when(i2, i), i2 != i))
            sign = csign[n, i] = 1 if col[0] == i else -1
            c = cell(col[0], i)
            for i2 in col[1:]:
                c = c + cell(i2, i) if (1 if i2 == i else -1) == sign else c - cell(i2, i)
            put(('C', i), c)
            for j in range(n):
                if j != i:
                    put(('S', i, j), cell(i, j))
        for i, j in star.pairs:
            put(('A', i, j), cell(i, j) + cell(j, i))

    due = []

    def scores(x, u):
        if due and due[0][0] <= done_side[1]:
            x = _tie(x, due.pop(0)[1])
        s = (_dot if u in QT else _dot_nt)(x, _ld(q_scr, u))
        res.append(s)
        return s

    def job_e(I, h, J, p):
        tiles = [2 * (SB * I + i) + h for i in range(SB)]
        ps = []
        for i, u in enumerate(tiles):
            x = jnp.concatenate([k_scr.bitcast(U32)[2 * (SB * J + (t - i) % SB) + h, 8 * g:8 * g + 8, :]
                                 for g in (2 * p, 2 * p + 1) for t in range(SB)], axis=0)
            ps.append(jnp.exp2(scores(pltpu.bitcast(x, BF16), u)))
        when = lambda i, k: (i + k) % SB
        for n, g in enumerate((2 * p, 2 * p + 1)):
            cell = lambda i, k: ps[i][16 * (SB * n + when(i, k)):16 * (SB * n + when(i, k)) + 16]
            p_forms(_FULL, h, J * len(_FULL.pf), g, tiles, cell, when)

    def job_f(I, h):
        tiles = [2 * (SB * I + 2 + i) + h for i in range(2)]
        ps = {(i, k): jnp.exp2(scores(_ld(k_scr, 2 * (SB * I + k) + h), u))
              for i, u in enumerate(tiles) for k in range(2)}
        for g in range(T // 16):
            p_forms(_HALF, h, _HSLOT, g, tiles, lambda i, k: ps[i, k][16 * g:16 * g + 16], lambda i, k: 0)

    def job_d(I, h, i, k):
        u = 2 * (SB * I + i) + h
        s = scores(_ld(k_scr, 2 * (SB * I + k) + h), u)
        if i == k:
            s = jnp.where(causal, s, -1e9 * LOG2E)
        p = jnp.exp2(s)
        add_l(u, jnp.sum(p.reshape(T // 8, 8, T), axis=0))
        pf[h][_DSLOT + _DCELLS.index((i, k))] = p.astype(BF16)
        if (i, k) == _DCELLS[-1]:
            pf[h][_FENCE + z, 0:16, :] = jnp.zeros((16, T), BF16)
            for u in [2 * (SB * I + a) + h for a in range(SB)]:
                lrow[u] = jnp.sum(lsum.pop(u), axis=0, keepdims=True)
            ls = [lrow[2 * (SB * I + a) + h] for a in range(SB)]
            lo = jnp.minimum(jnp.minimum(ls[0], ls[1]), jnp.minimum(ls[2], ls[3]))
            hi = jnp.maximum(jnp.maximum(ls[0], ls[1]), jnp.maximum(ls[2], ls[3]))
            ok = jnp.logical_and(lo >= L_LO, hi <= L_HI)
            ok = jnp.logical_and(ok, (hi if I else jnp.maximum(ls[2], ls[3]))
                                 <= L_RATIO * (lo if I else jnp.minimum(ls[2], ls[3])))
            bad = jnp.where(ok, 0.0, 1.0)
            chk[1] = bad if chk[1] is None else jnp.maximum(chk[1], bad)

    def job_p(I, h, f, J):
        star, last = (_HALF, True) if J is None else (_FULL, J == I - 1)
        blk = I if J is None else J
        if f[0] == 'B':
            x = _ld(v_scr, 2 * (SB * blk + f[1]) + h, slice(HT // 2, HT))
        else:
            slot, r = _v_slot(star, blk, f)
            x = _ld(pf[h], slot, slice(r // 2, (r + HT) // 2))
        v = _dot(x, _ld(pf[h], (_HSLOT if J is None else J * len(_FULL.pf)) + star.pf[star.pv[f]]))
        res.append(v)
        key = (star.n,) + f
        acc[key] = v if key not in acc else acc[key] + v
        if not last:
            return

        def add(which, i, v, sign=1):
            k_ = (star.n, which, i)
            if k_ not in fg:
                fg[k_] = v if sign > 0 else -v
            else:
                fg[k_] = fg[k_] + v if sign > 0 else fg[k_] - v

        if f[0] == 'W':
            add('F', f[1], acc.pop(key))
        elif f[0] == 'B':
            add('G', f[1], acc.pop(key), csign[star.n, f[1]])
        elif f[0] == 'Q3':
            _, i, j = f
            q1, q2, q3 = (acc.pop((star.n, q, i, j)) for q in ('Q1', 'Q2', 'Q3'))
            t = ((q1 + q2) + q3) * (1.0 / (star.ts[i] - star.ts[j]))
            add('G', i, t)
            add('G', j, t)
            add('F', i, q1)
            add('F', j, q3, -1)

    def job_v(I, h, i, k):
        u = 2 * (SB * I + i) + h
        v = _dot(_ld(v_scr, 2 * (SB * I + k) + h), _ld(pf[h], _DSLOT + _DCELLS.index((i, k))))
        res.append(v)
        dacc[u] = v if u not in dacc else dacc[u] + v
        if k == i:
            o = dacc.pop(u)
            for star, a in ([(_FULL, i)] if I else []) + ([(_HALF, i - 2)] if i >= 2 else []):
                f, g = fg.pop((star.n, 'F', a)), fg.pop((star.n, 'G', a))
                o = o + jnp.concatenate([f - star.ts[a] * g, g], axis=0)
            o = o * (1.0 / lrow[u])
            of[u] = o
            chk[0] = chk[0] + jnp.sum(o.reshape(T // 8, 8, T), axis=0)

    def job_o(_, n):
        af, bf, outs = _O_JOBS[n][1]
        if af not in lhs:
            v = _form(af, lambda i, h: of[2 * i + h])
            lhs[af] = _tie(v.astype(BF16).T, v[0:8, :])
        if bf not in wo:
            wo[bf] = (wo_ref[_tile(bf[0][1]), _tile(bf[0][2])] if len(bf) == 1 else
                      _form(bf, lambda h, j: wo_ref[_tile(h), _tile(j)].astype(F32)).astype(BF16))
        v = _dot(lhs[af], wo[bf])
        res.append(v)
        for sign, i, j in outs:
            terms.setdefault((i, j), []).append((sign, v))
            if len(terms[i, j]) == left[i, j]:
                tot = acc_scr[_tile(i), _tile(j)]
                for sg, m in terms.pop((i, j)):
                    tot = tot + m if sg > 0 else tot - m
                acc_scr[_tile(i), _tile(j)] = tot

    fns = dict(e=job_e, f=job_f, d=job_d, p=job_p, v=job_v, o=job_o)
    order = _job_order(q_scr.shape[0] // (2 * SB))
    for n, job in enumerate(order):
        assert job[0] not in 'efd' or not any(j[0] in 'pv' and j[2] == job[2] and j[1] < job[1] for j in order[n:])
    side = list(side)
    fences = [n for n, job in enumerate(order) if job[0] == 'd' and job[3:] == _DCELLS[-1]]
    step = (len(order) - SIDE0 - SIDE1 - 10) / len(side)
    for n, job in enumerate(order):
        done_side[1] = n
        fns[job[0]](*job[1:])
        last_chance = n >= len(order) - SIDE1
        near = any(-SG1 <= f - n <= SG0 for f in fences)
        if side and n >= SIDE0 + step * done_side[0] and ((job[0] in 'pvo' and not near) or last_chance):
            done_side[0] += 1
            v = side.pop(0)(res[-1 - SLAG][8 * (n % 4):8 * (n % 4) + 8, :])
            if v is not None:
                due.append((n + SDUE, v))
    assert not side and not due
    fine = jnp.abs(chk[0]) < jnp.inf
    flag_scr[...] = jnp.maximum(flag_scr[...], jnp.where(fine, chk[1], 1.0))


def _kernel(x_hbm, c_hbm, wq_hbm, wuk_hbm, wuv_hbm, wo_hbm, w1_hbm, w2_hbm, w3_hbm, w4_hbm,
            cond_hbm, wmod_hbm, out_hbm,
            x_ref, c_ref, cond_ref, wma_ref, wmb_ref, w1_ref, w3_ref,
            wq_buf, wk_buf, wv_buf, wo_buf, out_buf, sem, wsem, osem,
            mod_scr, h_scr, cs_scr, hs_scr, w_scr, q_scr, k_scr, v_scr, acc_scr, xn_scr, xh_scr, a1_scr, t_scr,
            z_scr, mw_scr, m3_scr, wt_scr, wf_scr, gap_scr, st_in, pf_scr, vf_scr, flag_scr):
    S, M = x_hbm.shape
    D = wq_hbm.shape[2]
    nattn = wo_hbm.shape[0]
    Fd = w4_hbm.shape[0]
    scale = float(D) ** -0.5 * LOG2E
    nb, nrb = S // T, S // RB
    km, kc = M // T, c_hbm.shape[1] // T
    NX = 4
    XR = S // NX
    CB = XR // T

    work = (wk_buf, wv_buf, wq_buf)

    def pcopies(g, bufs=work, s0=0):
        return [pltpu.make_async_copy(src.bitcast(U32).at[:, g, :], dst, wsem.at[s0 + j])
                for j, (src, dst) in enumerate(zip((wuk_hbm, wuv_hbm, wq_hbm), bufs))]

    def ocopy(g):
        return pltpu.make_async_copy(wo_hbm.at[g], wo_buf, wsem.at[3])

    def chunk_copy(src, dst, i, s0):
        rows = slice(i * XR, (i + 1) * XR)
        return pltpu.make_async_copy(src.at[rows, :], dst.at[rows, :], sem.at[s0 + i])

    MS = 16
    NSL = T // MS
    assert nattn - 1 >= NSL
    mixw = ((w1_hbm, km, 0), (w2_hbm, km, km * MS), (w3_hbm, Fd // T, 2 * km * MS),
            (w4_hbm, -(-Fd // T), (2 * km + Fd // T) * MS))

    def prep_in(g):
        o = jnp.minimum(g, NSL - 1) * MS
        return [pltpu.make_async_copy(
            w.at[pl.ds(pl.multiple_of(jnp.minimum(b * T + o, w.shape[0] - MS), MS), MS), :],
            st_in.at[r0 + b * MS:r0 + (b + 1) * MS, :], wsem.at[7]) for w, nblk, r0 in mixw for b in range(nblk)]

    def stage_in(g):
        return pcopies(jnp.minimum(g + 1, nattn - 1))

    cp_cond = pltpu.make_async_copy(cond_hbm, cond_ref, sem.at[0])
    cp_wma = pltpu.make_async_copy(wmod_hbm.at[:, 0:2 * M], wma_ref, sem.at[1])
    cp_late = [pltpu.make_async_copy(src, dst, sem.at[2 + j]) for j, (src, dst) in enumerate((
        (wmod_hbm.at[:, 2 * M:6 * M], wmb_ref), (w1_hbm, w1_ref), (w3_hbm.at[Fd // T * T:, :], w3_ref)))]
    cp_x = [chunk_copy(x_hbm, x_ref, i, 7) for i in range(NX)]
    cp_c = [chunk_copy(c_hbm, c_ref, i, 7 + NX) for i in range(NX)]

    def silu_cond():
        cf = cond_ref[...].astype(F32)
        return jnp.broadcast_to((cf * jax.nn.sigmoid(cf)).astype(BF16), (8, M))

    cp_wk, cp_wv, cp_wq = pcopies(0)
    named = dict(k=cp_wk, v=cp_wv, q=cp_wq, o=ocopy(0), n=cp_cond, m=cp_wma)
    named.update(zip('abcd', cp_c))
    named.update(zip('wxyz', cp_x))
    started, arrived, did = set(), set(), set()

    def zero(r, carry):
        acc_scr[pl.ds(pl.multiple_of(r * T, T), T), :] = jnp.zeros((T, M), F32)
        return carry

    def x_rows(rows, dep):
        xf = x_ref[rows, :].astype(F32)
        if dep is None:
            return xf
        return jnp.concatenate([_after(xf[:, :T], _rows(dep, xf.shape[0])), xf[:, T:]], axis=1)

    def n_item(r, i):
        def fn(dep):
            rows = slice(r * T + i * LP, r * T + (i + 1) * LP)
            xn_scr[rows, :] = _ln(x_rows(rows, dep))
        return fn

    def h_item(r, i, normed):
        def fn(dep):
            rows = slice(i * LP, (i + 1) * LP)
            grows = slice(r * T + i * LP, r * T + (i + 1) * LP)
            sa = mod_scr[:, 0:M]
            if normed and dep is not None:
                sa = jnp.concatenate([_after(sa[:, _tile(j)], dep) for j in range(km)], axis=1)
            hf = ((xn_scr[grows, :] if normed else _ln(x_rows(grows, dep))) * _rows(mod_scr[:, M:2 * M], LP)
                  + _rows(sa, LP))
            for j in range(km):
                h_scr[r, j, rows, :] = hf[:, _tile(j)].astype(BF16)
            for f, n in _H_SUMS.items():
                if all(t[1] == r for t in f):
                    hs_scr[n, rows, :] = _form(f, lambda _, k: hf[:, _tile(k)]).astype(BF16)
            did.add(('h', r, i))
        return fn

    def release(jobs, span, items):
        if span and items:
            jobs.side += [(len(jobs.res) + 1 + i * span // len(items), fn) for i, fn in enumerate(items)]
            jobs.side.sort(key=lambda e: e[0])
        else:
            for fn in items:
                fn(None)

    def sum_items(n, group, index, dst, get, skip_rows):
        forms = [f for f in dict.fromkeys(t[0] for t in group)
                 if len(f) > 1 and not (skip_rows and len({t[1] for t in f}) == 1)]

        def item(f, rows):
            def fn(dep):
                def term(r, k):
                    v = get(r, k, rows).astype(F32)
                    return v if dep is None or (r, k) != f[0][1:] else _after(v, _rows(dep, v.shape[0]))
                dst[index[f], rows, :] = _form(f, term).astype(BF16)
            return fn

        return [item(f, slice(i, i + n)) for i in range(0, T, n) for f in forms]

    h_sums = lambda n, gi: sum_items(n, _H_GROUPS[gi], _H_SUMS, hs_scr,
                                     lambda r_, k, rows: h_scr[r_, k, rows, :], True)

    def stash(key, buf, j0, transpose=False):
        n = buf.shape[0] // T
        if key not in did:
            assert key in arrived
            did.add(key)
            for (j, hd), w in _pair_tiles(buf, transpose).items():
                w_scr[hd, j0 + j] = w
        return lambda hd: [_ld(w_scr, hd, j0 + j) for j in range(n)]

    def kv_tile(jobs, r):
        wk, wvT = stash('k', wk_buf, 0), stash('v', wv_buf, kc, True)
        ct = [c_ref[_tile(r), _tile(j)] for j in range(kc)]
        for hd in range(2):
            k_scr[2 * r + hd] = jobs.mm(ct, wk(hd), _dot).astype(BF16)
        for hd in range(2):
            v_scr[2 * r + hd] = jobs.mm(wvT(hd), ct, _dot_nt).astype(BF16)

    def q_tile(jobs, r):
        wq = stash('q', wq_buf, 2 * kc)
        ht = [_ld(h_scr, r, j) for j in range(km)]
        for hd in range(2):
            v = (jobs.mm(ht, wq(hd), _dot) * scale).astype(BF16)
            q_scr[2 * r + hd] = v.T if 2 * r + hd in QT else v

    for blk in _prologue().split(';'):
        waits, starts, acts = blk.split('|')
        for ch in waits.strip():
            assert ch in started and ch not in arrived
            arrived.add(ch)
            named[ch].wait()
        for ch in starts.strip():
            assert ch not in started
            started.add(ch)
            named[ch].start()
        jobs = _Jobs()
        for act in acts.split():
            if act == 'Z':
                jax.lax.fori_loop(0, nb, zero, 0)
                acc_scr[S:, :] = jnp.zeros((acc_scr.shape[0] - S, M), F32)
                x_ref[S:, :] = jnp.zeros((x_ref.shape[0] - S, M), BF16)
                flag_scr[...] = jnp.zeros(flag_scr.shape, F32)
            elif act == 'L':
                did.add('L')
                assert ('Q', 0) in did
                for cp in stage_in(0) + prep_in(0):
                    cp.start()
            elif act == 'M':
                assert arrived >= set('nm')
                mod = _dot(silu_cond(), wma_ref[...])
                mod_scr[:, 0:M] = mod[:, 0:M]
                mod_scr[:, M:2 * M] = 1.0 + mod[:, M:2 * M]
                did.add('M')
            else:
                act, _, span = act.partition('@')
                span = int(span or 0)
                items = []
                for r in [int(ch, 16) for ch in act[1:]]:
                    did.add((act[0], r))
                    if act[0] == 'K':
                        assert 'abcd'[r // CB] in arrived
                        kv_tile(jobs, r)
                    elif act[0] == 'H':
                        assert 'wxyz'[r // CB] in arrived and 'M' in did
                        items += [h_item(r, i, ('N', r) in did) for i in range(T // LP)]
                    elif act[0] == 'N':
                        assert 'wxyz'[r // CB] in arrived
                        items += [n_item(r, i) for i in range(T // LP)]
                    elif act[0] == 'Q':
                        assert all(('h', r, i) in did for i in range(T // LP))
                        q_tile(jobs, r)
                    elif act[0] == 'Y':
                        def zero_item(n0):
                            def fn(dep):
                                zero = jnp.where(dep > jnp.inf, jnp.uint32(1), jnp.uint32(0))
                                for n in range(n0, min(n0 + 4, _MIX3 + m3_scr.shape[0])):
                                    mw_scr.bitcast(U32)[n] = _rows(zero, T // 2)
                            return fn
                        items += [zero_item(n0) for n0 in range(_MIX3, _MIX3 + m3_scr.shape[0], 4)]
                    elif act[0] == 'F':
                        assert all(('K', SB * r + k_) in did for k_ in range(SB))
                        items += _v_form_items(v_scr, (pf_scr, vf_scr), r)
                    elif act[0] == 'C':
                        assert all('abcd'[t[1] // CB] in arrived for p_ in _C_GROUPS[r] for t in p_[0])
                        items += sum_items(
                            32, _C_GROUPS[r], _C_SUMS, cs_scr,
                            lambda r_, k, rows: c_ref[r_ * T + rows.start:r_ * T + rows.stop, _tile(k)], False)
                    else:
                        assert act[0] == 'S' and all(('h', t[1], T // LP - 1) in did for p_ in _H_GROUPS[r] for t in p_[0])
                        items += h_sums(32 if span else 16, r)
                release(jobs, span, items)
        assert not jobs.side
    assert arrived == set(named) and all((k_, r) in did for k_ in 'KHQ' for r in range(nb))
    assert all((k_, r) in did for k_ in 'CS' for r in range(2)) and 'L' in did
    assert all(('F', r) in did for r in range(SB))

    def mixer_prep(g):
        sl = jnp.minimum(g, NSL - 1)
        rows = pl.ds(pl.multiple_of(sl * MS, MS), MS)

        def part(m, forms):
            def fn(dep):
                base = {}

                def get(i, k):
                    if (i, k) not in base:
                        rb, cb = (i, k) if m == 2 else (k, i)
                        r0 = mixw[m][2] + rb * MS
                        v = _after(st_in[r0:r0 + MS, _tile(cb)].astype(F32), _rows(dep, MS))
                        if m == 3 and (rb + 1) * T > Fd:
                            v = jnp.where(rb * T + sl * MS < Fd, v, 0.0)
                        base[i, k] = v
                    return base[i, k]

                for f in forms:
                    v = _form(f, get)
                    mw_scr[_MIXW[m, f], rows, :] = (0.5 * v if m % 2 else v).astype(BF16)
            return fn

        items = []
        for m in range(4):
            forms = [f for mm_, f in _MIXW if mm_ == m]
            cur, terms = [], set()
            for f in forms:
                new_terms = terms | {t[1:] for t in f}
                if cur and 3 * len(new_terms) + sum(2 * len(x) + 1 for x in cur + [f]) > MWOPS:
                    items.append(part(m, cur))
                    cur, terms = [], set()
                cur.append(f)
                terms |= {t[1:] for t in f}
            items.append(part(m, cur))

        n3 = sum(m == 2 for m, _ in _MIXW)
        first = min(n for (m, _), n in _MIXW.items() if m == 2)
        per = -(-n3 // (nattn - 1 - NSL))

        def turn(j):
            def fn(dep):
                n = jnp.minimum(jnp.maximum(g - NSL, 0) * per + j, n3 - 1)
                w = _tie(_ld(mw_scr, first + n), dep).T
                m3_scr[n] = w
                return pltpu.bitcast(pltpu.bitcast(w, U32)[T // 2 - 8:], F32)
            return fn

        return items + [turn(j) for j in range(per)]

    def stage_wait():
        for cp in pcopies(0):
            cp.wait()
        pltpu.make_async_copy(st_in, st_in, wsem.at[7]).wait()

    def attn_body(g, carry):
        side = _gap_items(work, gap_scr) + _weight_form_items(work, gap_scr, wt_scr, wf_scr)
        bufs = (q_scr, k_scr, v_scr, (pf_scr, vf_scr), wo_buf, acc_scr, flag_scr)
        _attention_step(*bufs, g >> 16, side)

        @pl.when(g + 1 < nattn)
        def _():
            copies = stage_in(g + 1) + [ocopy(g + 1)]
            for cp in copies:
                cp.start()
            bufs = (h_scr, hs_scr, c_ref, cs_scr, wf_scr, q_scr, k_scr, v_scr, (pf_scr, vf_scr))
            side = [(SD0 + int(i * SDS), fn) for i, fn in enumerate(mixer_prep(g))]
            _proj_step(*bufs, scale, gap_scr, side)
            for cp in prep_in(g + 1):
                cp.start()
            stage_wait()
            ocopy(g + 1).wait()

        return carry

    stage_wait()
    for cp in cp_late:
        cp.start()
    jax.lax.fori_loop(0, nattn, attn_body, 0)

    def safe_pair(g, carry):
        copies = pcopies(g) + [ocopy(g)]
        for cp in copies:
            cp.start()
        for cp in copies:
            cp.wait()
        for buf, j0, transpose in ((wk_buf, 0, False), (wv_buf, kc, True), (wq_buf, 2 * kc, False)):
            for (j, hd), w in _pair_tiles(buf, transpose).items():
                w_scr[hd, j0 + j] = w

        def tile(u, carry):
            r, hd = u // 2, u % 2
            rows = pl.ds(pl.multiple_of(r * T, T), T)
            ct = [c_ref[rows, _tile(j)] for j in range(kc)]
            k_scr[u] = sum(_dot(ct[j], _ld(w_scr, hd, j)) for j in range(kc)).astype(BF16)
            v_scr[u] = sum(_dot_nt(_ld(w_scr, hd, kc + j), ct[j]) for j in range(kc)).astype(BF16)
            q = sum(_dot(_ld(h_scr, r, j), _ld(w_scr, hd, 2 * kc + j)) for j in range(km))
            q_scr[u] = (q * scale).astype(BF16)
            return carry

        jax.lax.fori_loop(0, 2 * nb, tile, 0)
        _attention_safe(q_scr, k_scr, v_scr, wo_buf, acc_scr)
        return carry

    @pl.when(jnp.max(flag_scr[...]) > 0)
    def _():
        jax.lax.fori_loop(0, nb, zero, 0)
        jax.lax.fori_loop(0, nattn, safe_pair, 0)

    for cp in cp_late:
        cp.wait()
    mod = _dot(silu_cond(), wmb_ref[...])
    mod_scr[:, 2 * M:4 * M] = mod[:, 0:2 * M]
    mod_scr[:, 4 * M:5 * M] = 1.0 + mod[:, 2 * M:3 * M]
    mod_scr[:, 5 * M:6 * M] = mod[:, 3 * M:4 * M]
    OFF = x_ref.shape[0] - S
    CAR = t_scr.shape[0] - RB

    def p1(r0, l0, n, dep=None):
        ga = mod_scr[:, 2 * M:3 * M]
        if dep is not None:
            ga = jnp.concatenate([_after(ga[:, 0:T], dep), ga[:, T:]], axis=1)
        rows = pl.ds(r0, n)
        x1 = x_ref[rows, :].astype(F32) + _rows(ga, n) * acc_scr[rows, :]
        xh_scr[0, l0:l0 + n, :] = x1
        hb = _ln(x1) * _rows(mod_scr[:, 4 * M:5 * M], n) + _rows(mod_scr[:, 3 * M:4 * M], n)
        xh_scr[1, l0:l0 + n, :] = hb
        return hb

    HT = T // 2
    last8 = lambda v: jnp.max(v[:, M - T:].reshape(PC // 8, 8, T), axis=0)

    def p1_store(r0, c, dep=None):
        v = _ln(p1(r0 + c * PC, OFF + c * PC, PC, dep))
        a1_scr[c * PC:(c + 1) * PC, :] = v
        return last8(v)

    def p1_first(r0, c, dep):
        return last8(p1(r0 + c * PC, OFF + c * PC, PC, dep))

    def p1_second(c, dep):
        hb = xh_scr[1, OFF + c * PC:OFF + (c + 1) * PC, :]
        v = _ln(jnp.concatenate([_after(hb[:, :T], _rows(dep, PC)), hb[:, T:]], axis=1))
        a1_scr[c * PC:(c + 1) * PC, :] = v
        return last8(v)

    t_scr[RB:RB + CAR - OFF, :] = jnp.zeros((CAR - OFF, M), F32)
    t_scr[RB + CAR - OFF:RB + CAR, :] = _gelu2(_dot(_ln(p1(0, 0, OFF)).astype(BF16), w1_ref[...]))
    for c in range(RB // PC):
        p1_store(OFF, c)

    def out_copy(i):
        rows = pl.ds(i * T if isinstance(i, int) else pl.multiple_of(i * T, T), T)
        return pltpu.make_async_copy(out_buf.at[rows, :], out_hbm.at[rows, :], osem.at[i])

    def b_body(r, carry):
        gb = _rows(mod_scr[:, 5 * M:6 * M], T)
        r0 = pl.multiple_of(r * RB, RB)
        n0 = pl.multiple_of(jnp.minimum(r0 + RB, S - RB) + OFF, OFF)
        nh = RB // T
        now = [0]
        due = []
        pace = []

        def p1_item(c, part):
            def fn(dep):
                v = p1_first(n0, c, dep) if part == 0 else p1_second(c, dep)
                due.append((now[0] + PD, v))
                due.sort(key=lambda e: e[0])
            return fn

        pace += [(P0 + i * PSTEP + part * PSPLIT, p1_item(i, part)) for i in range(RB // PC)
                 for part in range(2)]
        pace.sort(key=lambda e: e[0])

        def mm(lhs, wts, dot=_dot):
            acc = None
            for x, w in zip(lhs, wts):
                if due and due[0][0] <= now[0]:
                    w = _tie(w, due.pop(0)[1])
                v = dot(x, w)
                now[0] += x.shape[0] // HT
                acc = v if acc is None else v + acc
                if pace and pace[0][0] <= now[0]:
                    pace.pop(0)[1](v[0:8, :])
            return acc

        def fast(m, base, finish, hook=None):
            prods = _MIX[m]
            left, acc, done, cache = {}, {}, {}, {}
            for _, _, outs in prods:
                for _, i, h in outs:
                    left[i, h] = left.get((i, h), 0) + 1

            def act(form):
                sign, form = _canon(form)
                if form not in cache:
                    cache[form] = _form(form, lambda k, h: base(k)[h * HT:(h + 1) * HT]).astype(BF16)
                return sign, cache[form]

            for pi, (wf, af, outs) in enumerate(prods):
                w = _ld(m3_scr, _MIXW[m, wf] - _MIX3) if m == 2 else _ld(mw_scr, _MIXW[m, wf])
                if af is None:
                    k = wf[0][2]
                    v = mm([jnp.concatenate([act(((1, k, h),))[1] for h in range(2)], axis=0)], [w])
                    sign, parts = 1, [v[:HT], v[HT:]]
                else:
                    sign, x = act(af)
                    parts = [mm([x], [w])] * len(outs)
                for (s_, i, h), v in zip(outs, parts):
                    s_ = s_ * sign
                    if (i, h) not in acc:
                        acc[i, h] = (s_, v)
                    else:
                        s0, u = acc[i, h]
                        acc[i, h] = (s0, u + v if s0 == s_ else u - v) if s0 > 0 or s_ < 0 else (1, v - u)
                    left[i, h] -= 1
                    if not left[i, h]:
                        s0, done[i, h] = acc.pop((i, h))
                        assert s0 > 0
                        if (i, 1 - h) in done:
                            finish(i, jnp.concatenate([done[i, 0], done[i, 1]], axis=0))
                if hook is not None:
                    hook(pi, act)

        t_scr[0:CAR, :] = t_scr[RB:RB + CAR, :]
        for hf in range(nh):
            def put_t(n, v):
                t = _gelu2(v)
                if hf == nh - 1:
                    t = jnp.concatenate([t[:T - OFF], jnp.where(r < nrb - 1, t[T - OFF:], 0.0)], axis=0)
                t_scr[CAR + hf * T:CAR + (hf + 1) * T, _tile(n)] = t

            fast(0, lambda k: a1_scr[_tile(hf), _tile(k)], put_t)
        cq = M // 4
        shifts = (-1, 1, -2, 2)
        lane = jax.lax.broadcasted_iota(jnp.int32, (T, T), 1)
        y1, a3 = [], []
        for hf in range(nh):
            base = CAR - OFF + hf * T
            sh = []
            for j in range(km):
                g_lo, g_hi = (j * T) // cq, ((j + 1) * T - 1) // cq
                assert g_hi - g_lo <= 1
                v = t_scr[base + shifts[g_lo]:base + shifts[g_lo] + T, _tile(j)]
                if g_hi != g_lo:
                    v2 = t_scr[base + shifts[g_hi]:base + shifts[g_hi] + T, _tile(j)]
                    v = jnp.where(lane < g_hi * cq - j * T, v, v2)
                else:
                    v = jnp.where(lane < T, v, 0.0)
                sh.append(v)
            hs = {}
            fast(1, lambda k: sh[k], hs.__setitem__)
            hs = jnp.concatenate([hs[n] for n in range(km)], axis=1)
            y1.append(hs + xh_scr[1, _tile(hf), :])
            z_scr[_tile(hf), :] = xh_scr[0, _tile(hf), :] + gb * y1[hf]
            a3.append({})

            def ln_item(hf, c):
                def item(dep):
                    n = HT // NLN
                    for d in (0, HT):
                        v = y1[hf][d + c * n:d + (c + 1) * n]
                        if dep is not None:
                            v = jnp.concatenate([_after(v[:, :T], _rows(dep, n)), v[:, T:]], axis=1)
                        a3[hf][d + c * n] = _ln(v)
                return item

            ln_item(hf, 0)(None)
            pace += [(now[0] + LN0 + (c - 1) * LNS * (1 + hf), ln_item(hf, c)) for c in range(1, NLN)]
            pace.sort(key=lambda e: e[0])
        xh_scr[:, 0:OFF, :] = xh_scr[:, RB:RB + OFF, :]
        z_scr[pl.ds(pl.multiple_of(RB + (r >> 16) * 8, 8), 8), :] = jnp.zeros((8, M), F32)
        h3 = []
        for hf in range(nh):
            assert len(a3[hf]) == 2 * NLN
            af = jnp.concatenate([a3[hf][key] for key in sorted(a3[hf])], axis=0)
            row = {}
            narrow = []

            def hook(pi, act):
                j, rem = divmod(pi - NAR0, NARS)
                if rem == 0 and 0 <= j < km:
                    full = jnp.concatenate([act(((1, j, h),))[1] for h in range(2)], axis=0)
                    v = mm([w3_ref[:, _tile(j)]], [full], _dot_nt)
                    narrow[:] = [v + narrow[0] if narrow else v]

            def put_h(n, v):
                row[n] = _gelu2(v)
                if GD:
                    due.append((now[0] + GD, jnp.max(row[n].reshape(T // 8, 8, T), axis=0)))
                    due.sort(key=lambda e: e[0])

            fast(2, lambda k: af[:, _tile(k)], put_h, hook)
            fw = w3_ref.shape[0]
            row[Fd // T] = jnp.concatenate([_gelu2(narrow[0]), jnp.zeros((T - fw, T), F32)], axis=0).T
            h3.append(row)
        for hf in range(nh):
            rows = pl.ds(pl.multiple_of(r0 + hf * T, T), T)

            def finish(n, v):
                out_buf[rows, _tile(n)] = (z_scr[_tile(hf), _tile(n)] + gb[:, _tile(n)] * v).astype(out_buf.dtype)
                pltpu.make_async_copy(out_buf.at[rows, _tile(n)], out_hbm.at[rows, _tile(n)],
                                      osem.at[r * nh + hf]).start()

            fast(3, lambda k: h3[hf][k], finish)
        assert not pace
        return carry

    jax.lax.fori_loop(0, nrb, b_body, 0)
    for i in range(nb):
        out_copy(i).wait()


@jax.jit
def pallas_adaLN_cond__compressed_kv_cla__mixer_s_mlp__prompt_kernel(
    A_x: jax.Array,
    A_c_kv: jax.Array,
    A_w_q: jax.Array,
    A_w_uk: jax.Array,
    A_w_uv: jax.Array,
    A_w_o: jax.Array,
    B_x: jax.Array,
    B_w1: jax.Array,
    B_w2: jax.Array,
    B_w3: jax.Array,
    B_w4: jax.Array,
    c: jax.Array,
    w_mod: jax.Array,
):
    _, S, M = A_x.shape
    Dc = A_c_kv.shape[2]
    H, D = A_w_q.shape[1], A_w_q.shape[2]
    Fd = B_w3.shape[1]
    assert D == T and A_c_kv.shape[1] == S and Dc == 4 * T and M == 5 * T and 13 * T < Fd < 14 * T and S == 16 * T
    vmem = pltpu.VMEM
    packed = lambda *lead: vmem(lead + (T, T), BF16)
    out = pl.pallas_call(
        _kernel,
        in_specs=[pl.BlockSpec(memory_space=pltpu.HBM)] * 12,
        out_specs=pl.BlockSpec(memory_space=pltpu.HBM),
        out_shape=jax.ShapeDtypeStruct((S, M), A_x.dtype),
        scratch_shapes=[
            vmem((S + 16, M), BF16),
            vmem((S, Dc), BF16),
            vmem((1, M), BF16),
            vmem((M, 2 * M), BF16),
            vmem((M, 4 * M), BF16),
            vmem((M, M), BF16),
            vmem((Fd % T, M), BF16),
            vmem((M, D), U32),
            vmem((Dc, D), U32),
            vmem((Dc, D), U32),
            vmem((2 * D, M), BF16),
            vmem((S, M), A_x.dtype),
            pltpu.SemaphoreType.DMA((15,)),
            pltpu.SemaphoreType.DMA((8,)),
            pltpu.SemaphoreType.DMA((S // T,)),
            vmem((8, 6 * M), F32),
            vmem((S // T, M // T, T, T), BF16),
            vmem((len(_C_SUMS), T, T), BF16),
            vmem((len(_H_SUMS), T, T), BF16),
            packed(2, M // T + 2 * (Dc // T)),
            packed(2 * S // T),
            packed(2 * S // T),
            packed(2 * S // T),
            vmem((S + 16, M), F32),
            vmem((S, M), F32),
            vmem((2, RB + 16, M), F32),
            vmem((RB, M), F32),
            vmem((RB + 32, M), F32),
            vmem((RB + 8, M), F32),
            packed(len(_MIXW)),
            packed(sum(m == 2 for m, _ in _MIXW)),
            vmem((Dc // T, T, T), U32),
            vmem((len(_WF), T, T), BF16),
            vmem((3, 8, T), jnp.int32),
            vmem(((2 * (M // T) + Fd // T + -(-Fd // T)) * 16, M), BF16),
            vmem((_FENCE + 1, T, T), BF16),
            vmem((_FENCE + 1, T, T), BF16),
            vmem((8, T), F32),
        ],
        compiler_params=pltpu.CompilerParams(
            vmem_limit_bytes=100 * 1024 * 1024,
            disable_bounds_checks=True,
        ),
    )(
        A_x.reshape(S, M), A_c_kv.reshape(S, Dc),
        A_w_q, A_w_uk, A_w_uv,
        A_w_o.reshape(H // 2, 2 * D, M),
        B_w1, B_w2, B_w3.T, B_w4, c, w_mod,
    )
    return out.reshape(1, S, M)
```

```python
import functools
import math

import jax
import jax.numpy as jnp
import jax.experimental.pallas as pl
import jax.experimental.pallas.tpu as pltpu

F32 = jnp.float32
BF16 = jnp.bfloat16
U32 = jnp.uint32
NT = (((1,), (1,)), ((), ()))
T = 128
EPS = 1e-5
LOG2E = math.log2(math.e)

L_LO, L_HI, L_RATIO = 2.0 ** -24, 2.0 ** 24, 4.0

LAT_0, LAT_A = 32, 16
LAT_B = 20
RES, OEND = 32, 24
ONV = 0.7
QT = (4, 6)
SIDE0, SIDE1 = 8, 60
SLAG, SDUE = 3, 8
SG0, SG1 = 6, 4
WFN = (4, 4, 6)
SD0, SDS = 4, 1.5
VF0, VFS = 4, 1.6
PDUE = 20
MWOPS = 70
RB = 256
PC = 32
P0, PSTEP, PSPLIT, PD = 300, 34, 40, 36
NLN, LN0, LNS = 4, 4, 5
GD = 36
NAR0, NARS = 10, 10
LP = 16
SP0, SP1 = 76, 38
_prologue = lambda: ('|kva|Z; |b|; kva|wc|Y0@56 K0123; bw|xdn|C0@56 N0123@52 K4567; cx|mq|N4567@52 F0@56 K89ab; '
            'd|y|C1@56 F1@56 Kcdef; nmq|zo|M H01 H234567@30 F2@36 Q0123; y||L H89ab@30 F3@36 Q4567; '
            'zo||Hcdef@30 S0@%d Q89ab S1@%d Qcdef' % (SP0, SP1))


def _dot(a, b):
    return jnp.dot(a, b, preferred_element_type=F32)


def _dot_nt(a, b):
    return jax.lax.dot_general(a, b, NT, preferred_element_type=F32)


def _ln(x):
    m = jnp.mean(x, axis=-1, keepdims=True)
    xc = x - m
    v = jnp.mean(xc * xc, axis=-1, keepdims=True)
    return xc * jnp.exp2(jnp.log(v + EPS) * (-0.5 * LOG2E))


def _rows(v, n):
    return jnp.broadcast_to(v[None], (n // 8, 8, v.shape[1])).reshape(n, v.shape[1])


def _gelu2(x):
    c0 = math.sqrt(2.0 / math.pi)
    return x + x * jnp.tanh(x * (c0 + (c0 * 0.044715) * (x * x)))


def _after(x, dep):
    return jnp.where(dep > jnp.inf, dep, x)


def _tie(x, dep):
    xu = pltpu.bitcast(x, U32)
    first = jnp.where(dep > jnp.inf, jnp.uint32(0), xu[:8])
    return pltpu.bitcast(jnp.concatenate([first, xu[8:]], axis=0), BF16)


def _tile(j):
    return slice(j * T, (j + 1) * T)


def _ld(ref, *idx):
    return pltpu.bitcast(ref.bitcast(U32)[idx], BF16)


def _group(rows, cols, pairs):
    xs, ys = dict.fromkeys(x for x, _ in pairs), dict.fromkeys(y for _, y in pairs)
    used = set(xs) | set(ys) | {(x[0], y[1]) for x, y in pairs} | {(y[0], x[1]) for x, y in pairs}
    prods = []
    for n, r in enumerate(rows):
        for i, k in [x for x in xs if x[0] == r]:
            mates = [y for x, y in pairs if x == (i, k)]
            prods.append((((1, i, k),) + tuple((1, i, k2) for _, k2 in mates), ((1, k, 0),),
                          ((1, i, 0), (-1, i, 1))))
            prods.append((((1, i, k),) + tuple((-1, i2, k) for i2, _ in mates), ((1, k, 0), (1, k, 1)),
                          ((1, i, 1),)))
        for i2, k2 in [y for y in ys if y[0] == r]:
            mates = [x for x, y in pairs if y == (i2, k2)]
            prods.append((((1, i2, k2),) + tuple((1, i2, k) for _, k in mates), ((1, k2, 1),),
                          ((1, i2, 1), (-1, i2, 0))))
            prods.append((((1, i2, k2),) + tuple((-1, i, k2) for i, _ in mates), ((1, k2, 0), (1, k2, 1)),
                          ((1, i2, 0),)))
        prods += [(((1, r, k),), ((1, k, h),), ((1, r, h),)) for k in cols if (r, k) not in used for h in (0, 1)]
        for (i, k), (i2, k2) in pairs:
            if r in (i, i2) and i + i2 - r in rows[n + 1:]:
                prods.append((((1, i, k2),), ((1, k2, 0), (-1, k, 0)), ((1, i2, 0), (1, i, 0))))
                prods.append((((1, i2, k), (1, i, k2)), ((1, k, 0), (1, k2, 1)), ((1, i2, 0), (1, i, 1))))
                prods.append((((1, i2, k),), ((1, k, 1), (-1, k2, 1)), ((1, i2, 1), (1, i, 1))))
    return prods


def _all_pairs(xrows, yrows):
    return [((x, a), (y, b)) for a, x in enumerate(xrows) for b, y in enumerate(yrows) if a != b]


_PAIRS65 = [((x[0] + 10, x[1]), (y[0] + 10, y[1])) for x, y in (
    ((0, 1), (1, 0)), ((0, 1), (5, 2)), ((2, 3), (1, 0)), ((2, 3), (3, 1)), ((2, 3), (5, 2)), ((3, 2), (1, 0)),
    ((4, 4), (0, 3)), ((4, 4), (1, 0)), ((4, 4), (3, 1)), ((4, 4), (5, 2)))]
_C_GROUPS = [_group(range(r, r + 8), range(4), _all_pairs(range(r, r + 4), range(r + 4, r + 8))) for r in (0, 8)]
_H_GROUPS = [_group(range(10), range(5), _all_pairs(range(5), range(5, 10))),
             _group(range(10, 16), range(5), _PAIRS65)]
_sum_index = lambda groups: {f: n for n, f in enumerate(
    dict.fromkeys(t[0] for g in groups for t in g if len(t[0]) > 1))}
_C_SUMS, _H_SUMS = _sum_index(_C_GROUPS), _sum_index(_H_GROUPS)


def _cells(rows, cols, pairs):
    xs = list(dict.fromkeys(p[0] for p in pairs))
    ys = list(dict.fromkeys(p[1] for p in pairs))
    used = set(xs + ys) | {(x[0], y[1]) for x, y in pairs} | {(y[0], x[1]) for x, y in pairs}

    def home_x(i, k):
        mates = [y for x, y in pairs if x == (i, k)]
        return [(((1, i, k),) + tuple((1, i, k2) for _, k2 in mates), ((1, k, 0),), ((1, i, 0), (-1, i, 1))),
                (((1, i, k),) + tuple((-1, i2, k) for i2, _ in mates), ((1, k, 0), (1, k, 1)), ((1, i, 1),))]

    def home_y(i2, k2):
        mates = [x for x, y in pairs if y == (i2, k2)]
        return [(((1, i2, k2),) + tuple((1, i2, k) for _, k in mates), ((1, k2, 1),), ((1, i2, 1), (-1, i2, 0))),
                (((1, i2, k2),) + tuple((-1, i, k2) for i, _ in mates), ((1, k2, 0), (1, k2, 1)), ((1, i2, 0),))]

    def cross(x, y):
        (i, k), (i2, k2) = x, y
        return [(((1, i, k2),), ((1, k2, 0), (-1, k, 0)), ((1, i2, 0), (1, i, 0))),
                (((1, i2, k), (1, i, k2)), ((1, k, 0), (1, k2, 1)), ((1, i2, 0), (1, i, 1))),
                (((1, i2, k),), ((1, k, 1), (-1, k2, 1)), ((1, i2, 1), (1, i, 1)))]

    direct = lambda i: [(((1, i, k),), None, ((1, i, 0), (1, i, 1))) for k in cols if (i, k) not in used]
    single = lambda i: ([t for x in xs if x[0] == i for t in home_x(*x)]
                        + [t for y in ys if y[0] == i for t in home_y(*y)] + direct(i))
    prods = []
    for n, i in enumerate(rows):
        prods += single(i)
        for i2 in rows[n + 1:]:
            for x, y in pairs:
                if {x[0], y[0]} == {i, i2}:
                    prods += cross(x, y)
    return prods


_square = lambda q: [((a, a), (q + b, b)) for a in range(q) for b in range(q) if a != b]
_shift = lambda pairs, r0: [((x[0] + r0, x[1]), (y[0] + r0, y[1])) for x, y in pairs]
_flip = lambda pairs: [(x[::-1], y[::-1]) for x, y in pairs]
_P35 = [((1, 2), (0, 4)), ((1, 2), (2, 1)), ((2, 3), (0, 4)), ((2, 3), (1, 0))]
_P45 = [((0, 2), (1, 1)), ((2, 4), (0, 3)), ((2, 4), (1, 1)), ((2, 4), (3, 2)), ((3, 0), (0, 3)), ((3, 0), (1, 1))]
_P55 = [((2, 1), (0, 4)), ((2, 1), (1, 0)), ((2, 1), (3, 2)), ((2, 1), (4, 3)), ((3, 3), (0, 4)), ((3, 3), (1, 0)),
        ((4, 2), (0, 4)), ((4, 2), (1, 0))]
_MIX = [_cells(range(5), range(5), _P55), _cells(range(5), range(5), _P55),
        _cells(range(13), range(5), _square(5) + _shift(_P35, 10)),
        _cells(range(5), range(14), _flip(_square(5) + _shift(_P45, 10)))]
_MIXW = {(m, f): n for n, (m, f) in enumerate(dict.fromkeys((m, t[0]) for m in range(4) for t in _MIX[m]))}
_MIX3 = min(n for (m, _), n in _MIXW.items() if m == 2)


def _form(form, get):
    acc = None
    for sign, i, j in form:
        v = get(i, j)
        acc = v if acc is None else (acc + v if sign > 0 else acc - v)
    return acc


def _gap_items(bufs, gap_scr):
    items = []
    for n, buf in enumerate(bufs):
        acc = []

        def part(r0, buf=buf, acc=acc):
            def fn(dep):
                wu = jnp.concatenate([buf[r:r + 8, :] for r in range(r0, r0 + T, 32)])
                mask = jnp.full((8, T), 0x7FFF0000, U32)
                if dep is not None:
                    mask = jnp.where(dep > jnp.inf, jnp.uint32(0), mask)
                mask = _rows(mask, 32)
                new = [jnp.sum(pltpu.bitcast(v & mask, F32).reshape(4, 8, T), axis=0) for v in (wu << 16, wu)]
                acc[:] = [u + v for u, v in zip(acc, new)] if acc else new
            return fn

        def last(_, n=n, acc=acc):
            bits = []
            for v in acc:
                l1 = jnp.sum(jnp.sum(v, axis=1, keepdims=True), axis=0, keepdims=True)
                bits.append(pltpu.bitcast(jnp.broadcast_to(l1, (8, T)), jnp.int32) >> 8)
            gap = jnp.clip((bits[0] - bits[1] + (1 << 14)) >> 15, -8, 8) << 23
            gap_scr[n] = gap
            return pltpu.bitcast(gap, F32)

        items += [part(r0) for r0 in range(0, buf.shape[0], T)] + [last]
    return items


def _pair_tiles(w_ref, transpose=False):
    tiles = {}
    for j in range(w_ref.shape[0] // T):
        wu = w_ref[_tile(j), :]
        if transpose:
            wu = wu.T
        tiles[j, 0] = pltpu.bitcast(wu << 16, F32).astype(BF16)
        tiles[j, 1] = pltpu.bitcast(wu & jnp.uint32(0xFFFF0000), F32).astype(BF16)
    return tiles


def _canon(form):
    if form[-1][0] < 0 and form[0][1:] > form[1][1:]:
        return -1, ((1,) + form[1][1:], (-1,) + form[0][1:])
    return 1, form


_w_forms = lambda groups: list(dict.fromkeys(_canon(t[1])[1] for g in groups for t in g))
_WF = {key: n for n, key in enumerate([(m, f) for m, groups in enumerate((_C_GROUPS, _C_GROUPS, _H_GROUPS))
                                       for f in _w_forms(groups)])}


def _weight_form_items(bufs, gap_scr, wt_scr, wf_scr):
    n = 16
    items = []

    def flip(j):
        def fn(dep):
            wu = bufs[1][_tile(j), :]
            wu = (wu if dep is None else jnp.where(_rows(dep, T) > jnp.inf, jnp.uint32(0), wu)).T
            wt_scr[j] = wu
            return pltpu.bitcast(wu[T - 8:], F32)
        return fn

    def part(m, r0, forms):
        def fn(dep):
            fac = pltpu.bitcast(0x3F800000 + gap_scr[m], F32)
            mask = jnp.full((8, T), 0xFFFF0000, U32)
            sh = jnp.full((8, T), 16, U32)
            if dep is not None:
                mask = jnp.where(dep > jnp.inf, jnp.uint32(0), mask)
                sh = jnp.where(dep > jnp.inf, jnp.uint32(0), sh)
            fac, mask, sh = _rows(fac, n), _rows(mask, n), _rows(sh, n)
            base = {}

            def get(k, h):
                if (k, h) not in base:
                    wu = wt_scr[k, r0:r0 + n, :] if m == 1 else bufs[m][k * T + r0:k * T + r0 + n, :]
                    base[k, h] = pltpu.bitcast(wu & mask, F32) * fac if h else pltpu.bitcast(wu << sh, F32)
                return base[k, h]

            for f in forms:
                wf_scr[_WF[m, f], r0:r0 + n, :] = _form(f, get).astype(BF16)
        return fn

    for m in range(3):
        forms = [f for mm, f in _WF if mm == m]
        if m == 1:
            items += [flip(j) for j in range(bufs[1].shape[0] // T)]
        per = -(-len(forms) // WFN[m])
        forms.sort(key=lambda f: sorted({t[1] for t in f}))
        items += [part(m, r0, forms[i:i + per]) for r0 in range(0, T, n) for i in range(0, len(forms), per)]
    return items


def _run_group(jobs, prods, a_get, w, transposed, finish):
    left = {}
    for _, _, outs in prods:
        for _, i, h in outs:
            left[i, h] = left.get((i, h), 0) + 1
    acc = {}
    for af, bf, outs in prods:
        sign, wt = w(bf)
        m = jobs.mm([wt], [a_get(af)], _dot_nt) if transposed else jobs.mm([a_get(af)], [wt], _dot)
        for s_, i, h in outs:
            if (i, h) not in acc:
                acc[i, h] = (s_ * sign, m)
            else:
                s0, v = acc[i, h]
                acc[i, h] = (s0, v + m if s0 == s_ * sign else v - m) if s0 > 0 or s_ * sign < 0 else (1, m - v)
            left[i, h] -= 1
            if not left[i, h]:
                s0, v = acc.pop((i, h))
                assert s0 > 0
                finish(2 * i + h, v)


class _Jobs:
    def __init__(self, side=()):
        self.res = []
        self.side = list(side)
        self.due = []

    def mm(self, lhs, wt, dot):
        acc = None
        for x, w in zip(lhs, wt):
            if self.due and self.due[0][0] <= len(self.res):
                x = _tie(x, self.due.pop(0)[1])
            v = dot(x, w)
            self.res.append(v)
            acc = v if acc is None else v + acc
            rel = 4 * (len(self.res) % 4)
            while self.side and self.side[0][0] <= len(self.res):
                out = self.side.pop(0)[1](v[8 * rel:8 * rel + 8, :])
                if out is not None:
                    self.due.append((len(self.res) + PDUE, out))
                rel = (rel + 2) % 16
        return acc


def _proj_step(h_scr, hs_scr, c_ref, cs_scr, wf_scr, q_scr, k_scr, v_scr, pf, scale, shifts, side):
    def weight(m):
        def get(form):
            sign, form = _canon(form)
            return sign, _ld(wf_scr, _WF[m, form])
        get.inv = pltpu.bitcast(0x3F800000 - shifts[m], F32)
        return get

    wk, wvT, wq = weight(0), weight(1), weight(2)
    c_get = lambda f: _ld(cs_scr, _C_SUMS[f]) if len(f) > 1 else c_ref[_tile(f[0][1]), _tile(f[0][2])]
    h_get = lambda f: _ld(hs_scr, _H_SUMS[f]) if len(f) > 1 else _ld(h_scr, f[0][1], f[0][2])

    def put(dst, w, mul=None):
        muls = [mul, _rows(w.inv if mul is None else w.inv * mul, T)]

        def fn(u, v):
            v = (v if muls[u % 2] is None else v * muls[u % 2]).astype(BF16)
            dst[u] = v.T if mul is not None and u in QT else v
        return fn

    jobs = _Jobs(side)
    put_v, stored = put(v_scr, wvT), set()
    nxt = [0]

    def fin_v(u, v):
        put_v(u, v)
        stored.add(u)
        for J in range(SB):
            if all(2 * (SB * J + k) + h in stored for k in range(SB) for h in range(2)) and ('J', J) not in stored:
                stored.add(('J', J))
                for fn in _v_form_items(v_scr, pf, J):
                    nxt[0] = max(nxt[0] + VFS, len(jobs.res) + VF0)
                    jobs.side.append((int(nxt[0]), fn))
                jobs.side.sort(key=lambda e: e[0])

    kk, vv, qq = ((c_get, wk, False, put(k_scr, wk)), (c_get, wvT, True, fin_v),
                  (h_get, wq, False, put(q_scr, wq, scale)))
    for prods, args in ((_C_GROUPS[0], kk), (_C_GROUPS[0], vv), (_C_GROUPS[1], vv), (_C_GROUPS[1], kk),
                        (_H_GROUPS[0], qq), (_H_GROUPS[1], qq)):
        _run_group(jobs, prods, *args)
    assert not jobs.side and not jobs.due


def _inner_group(rows, cols, pairs):
    xs, ys = dict.fromkeys(x for x, _ in pairs), dict.fromkeys(y for _, y in pairs)
    used = set(xs) | set(ys) | {(x[0], y[1]) for x, y in pairs} | {(y[0], x[1]) for x, y in pairs}
    prods = []
    for i, j in xs:
        mates = [y for x, y in pairs if x == (i, j)]
        prods.append((((1, i, 0),), ((1, 0, j), (-1, 1, j)), ((1, i, j),) + tuple((1, i2, j) for i2, _ in mates)))
        prods.append((((1, i, 0), (1, i, 1)), ((1, 1, j),), ((1, i, j),) + tuple((-1, i, j2) for _, j2 in mates)))
    for i2, j2 in ys:
        mates = [x for x, y in pairs if y == (i2, j2)]
        prods.append((((1, i2, 0), (1, i2, 1)), ((1, 0, j2),),
                      ((1, i2, j2),) + tuple((-1, i2, j) for _, j in mates)))
        prods.append((((1, i2, 1),), ((1, 0, j2), (-1, 1, j2)),
                      ((-1, i2, j2),) + tuple((-1, i, j2) for i, _ in mates)))
    prods += [(((1, i, h),), ((1, h, j),), ((1, i, j),))
              for i in rows for j in cols if (i, j) not in used for h in (0, 1)]
    for (i, j), (i2, j2) in pairs:
        lo, hi = min(j, j2), max(j, j2)
        prods.append((((1, i2, 0), (-1, i, 0)), ((1, 0, lo), (1, 0, hi)), ((1, i2, j),)))
        prods.append((((1, i, 0), (1, i2, 1)), ((1, 0, j2), (1, 1, j)), ((1, i, j2), (1, i2, j))))
        prods.append((((1, i, 1), (-1, i2, 1)), ((1, 1, lo), (1, 1, hi)), ((1, i, j2),)))
    return prods


def _o_jobs():
    prods = (_inner_group(range(10), range(5), _all_pairs(range(0, 10, 2), range(1, 10, 2)))
             + _inner_group(range(10, 16), range(5), _PAIRS65))
    row = lambda t: max(i for _, i, _ in t[0])
    unit = lambda t: max(2 * i + h for _, i, h in t[0])
    need = lambda t: unit(t) if row(t) == 15 else 2 * row(t) + 1
    return [(need(t), t) for t in sorted(prods, key=need)]


_O_JOBS = _o_jobs()


SB = 4


class _Star:
    def __init__(self, ts):
        self.ts, self.n = ts, len(ts)
        rn = range(self.n)
        self.pairs = [(i, j) for i in rn for j in rn if i < j]
        self.pf = {f: m for m, f in enumerate([('R', i) for i in rn] + [('C', i) for i in rn]
                                              + [('S', i, j) for i in rn for j in rn if i != j]
                                              + [('A', i, j) for i, j in self.pairs])}
        self.vf = {f: m for m, f in enumerate([('W', i) for i in rn]
                                              + [(q, i, j) for i, j in self.pairs for q in ('Q1', 'Q2', 'Q3')])}
        self.pv = {**{('W', i): ('R', i) for i in rn}, **{('B', i): ('C', i) for i in rn},
                   **{('Q1', i, j): ('S', i, j) for i, j in self.pairs},
                   **{('Q2', i, j): ('A', i, j) for i, j in self.pairs},
                   **{('Q3', i, j): ('S', j, i) for i, j in self.pairs}}

    def products(self, i):
        return [('W', i), ('B', i)] + [(q, i, j) for j in range(i + 1, self.n) for q in ('Q1', 'Q2', 'Q3')]


_FULL = _Star((-1.125, -0.375, 0.375, 1.125))
_HALF = _Star((-0.75, 0.75))
_DCELLS = [(0, 0), (1, 0), (1, 1), (2, 2), (3, 2), (3, 3)]
_HSLOT = (SB - 1) * len(_FULL.pf)
_DSLOT = _HSLOT + len(_HALF.pf)
_VSLOT = _DSLOT + len(_DCELLS)
_VHALF = (SB - 1) * len(_FULL.vf)
_FENCE = _VSLOT + (_VHALF + SB * len(_HALF.vf) + 1) // 2


def _v_slot(star, J, f):
    m = star.vf[f] + J * len(star.vf) + (0 if star is _FULL else _VHALF)
    return _VSLOT + m // 2, m % 2 * (T // 2)


def _v_form_items(v_scr, pf, J):
    n, HT = 16, T // 2

    def item(star, h, r0, pairs):
        def fn(dep):
            ts = [jnp.full((8, T), t, F32) for t in star.ts]
            ts = [_rows(t if dep is None else _after(t, dep), n) for t in ts]

            def get(k, a):
                r = (a * HT + r0) // 2
                return _ld(v_scr, 2 * (SB * J + k) + h, slice(r, r + n // 2)).astype(F32)

            def put(f, v):
                slot, r = _v_slot(star, J, f)
                pf[h][slot, r + r0:r + r0 + n, :] = v.astype(BF16)

            b = {(k, a): get(k, a) for k in sorted({k for pr in pairs or star.pairs for k in pr})
                 for a in range(2)}
            if pairs is None or star.n == 2:
                w = [b[k, 0] + ts[k] * b[k, 1] for k in range(star.n)]
                for k in range(star.n):
                    put(('W', k), w[k])
                for i, j in star.pairs:
                    put(('Q2', i, j), w[i] - w[j])
            for i, j in pairs or ():
                d0, d1 = b[j, 0] - b[i, 0], b[j, 1] - b[i, 1]
                put(('Q1', i, j), d0 + ts[i] * d1)
                put(('Q3', i, j), d0 + ts[j] * d1)
        return fn

    pr = _FULL.pairs
    parts = [(_HALF, _HALF.pairs)]
    if J < SB - 1:
        parts += [(_FULL, x) for x in (None, pr[:2], [pr[2], pr[4]], [pr[3], pr[5]])]
    return [item(star, h, r0, pairs) for h in range(2) for r0 in range(0, HT, n) for star, pairs in parts]


def _job_order(nsb):
    units = [(I, h) for I in range(nsb) for h in range(2)]
    qe, qv = [], []
    for I, h in units:
        qe += [('e', I, h, J, p) for J in range(I) for p in range(SB)] + [('f', I, h)]
        qe += [('d', I, h) + c for c in _DCELLS]
        for i in range(SB):
            qv += [('p', I, h, f, J) for f in _FULL.products(i) for J in range(I)]
            if i >= 2:
                qv += [('p', I, h, f, None) for f in _HALF.products(i - 2)]
            qv += [('v', I, h) + c for c in _DCELLS if c[0] == i]
    qo = [('o', u, j) for j, (u, _) in enumerate(_O_JOBS)]
    cost = dict(e=8, f=8, d=2, p=1, v=2, o=2)
    order, done = [], {}
    now = [0]

    def emit(q):
        job = q.pop(0)
        order.append(job)
        now[0] += cost[job[0]]
        if job[0] == 'd':
            done[job] = now[0]
        elif job[0] == 'v' and job[4] == job[3]:
            done['u', 2 * (SB * job[1] + job[3]) + job[2]] = now[0]
        return cost[job[0]]

    def v_ready():
        if not qv:
            return False
        key = ('d', qv[0][1], qv[0][2], SB - 1, SB - 1)
        return key in done and done[key] + (LAT_0 if qv[0][1:3] == (0, 0) else LAT_A) <= now[0]

    def o_ready():
        return bool(qo) and ('u', qo[0][1]) in done and done['u', qo[0][1]] + LAT_B <= now[0]

    def fill(nv, no):
        n = 0
        while nv > 0 or no > 0 or n % 4:
            if no > 0 and n % 2 == 0 and o_ready() and no * ONV >= nv:
                no -= 2
                n += emit(qo)
            elif v_ready() and (nv > 0 or n % 4):
                c = emit(qv)
                nv -= c
                n += c
            elif o_ready() and n % 2 == 0 and (no > 0 or n % 4 or nv > 0) and len(qo) > RES:
                no -= 2
                n += emit(qo)
            else:
                break

    while qe:
        unit = qe[0][1:3]
        while qv and qv[0][2] == unit[1] and qv[0][1] < unit[0]:
            emit(qv)
        ne = 0
        while qe and ne < 8 and (ne == 0 or (qe[0][0] == 'd' and qe[0][1:3] == unit and ne + 2 <= 8)):
            ne += emit(qe)
        groups = lambda q: sum(cost[j[0]] for j in q) / 8
        old = [j for j in qv if j[1:3] != unit and ('d', j[1], j[2], SB - 1, SB - 1) in done]
        here = [j for j in qe if j[1:3] == unit]
        rest = sum(cost[j[0]] for j in old)
        nv = (rest - LAT_A) / (groups(here) + 1) if here else rest
        no = 2 * max(len(qo) - RES - OEND, 0) / (groups(qe) + 1)
        fill(int(nv + 0.5), int(no + 0.5))
    while qv or qo:
        if qv and v_ready():
            fill(6, 2)
            if not qv:
                continue
        elif o_ready():
            emit(qo)
        else:
            emit(qv or qo)
    return order


def _attention_safe(q_scr, k_scr, v_scr, wo_ref, acc_scr):
    causal = (jax.lax.broadcasted_iota(jnp.int32, (T, T), 0)
              <= jax.lax.broadcasted_iota(jnp.int32, (T, T), 1))

    def unit(u, carry):
        r, hd = u // 2, u % 2

        def block(c, mlo):
            m0, l, o = mlo
            s = _dot_nt(_ld(k_scr, 2 * c + hd), _ld(q_scr, u))
            s = jnp.where(jnp.logical_or(causal, c < r), s, -1e9 * LOG2E)
            m = jnp.maximum(m0, jnp.max(s, axis=0, keepdims=True))
            a = jnp.exp2(m0 - m)
            p = jnp.exp2(s - m)
            return (m, l * a + jnp.sum(p, axis=0, keepdims=True),
                    o * a + _dot(_ld(v_scr, 2 * c + hd), p.astype(BF16)))

        _, l, o = jax.lax.fori_loop(0, r + 1, block, (jnp.full((1, T), -jnp.inf, F32), jnp.zeros((1, T), F32),
                                                      jnp.zeros((T, T), F32)))
        rows = pl.ds(pl.multiple_of(r * T, T), T)
        acc_scr[rows, :] += _dot((o * (1.0 / l)).astype(BF16).T, wo_ref[pl.ds(pl.multiple_of(hd * T, T), T), :])
        return carry

    jax.lax.fori_loop(0, q_scr.shape[0], unit, 0)


def _attention_step(q_scr, k_scr, v_scr, pf, wo_ref, acc_scr, flag_scr, z, side):
    causal = (jax.lax.broadcasted_iota(jnp.int32, (T, T), 0)
              <= jax.lax.broadcasted_iota(jnp.int32, (T, T), 1))
    HT = T // 2
    lsum, lrow, acc, fg, dacc, of, lhs = {}, {}, {}, {}, {}, {}, {}
    res = []
    wo, terms = {}, {}
    left = {}
    done_side = [0, 0]
    chk = [jnp.zeros((8, T), F32), None]
    for _, t in _O_JOBS:
        for _, i, j in t[2]:
            left[i, j] = left.get((i, j), 0) + 1

    def add_l(u, v):
        lsum[u] = v if u not in lsum else lsum[u] + v

    csign = {}

    def p_forms(star, h, slot0, g, tiles, cell, when):
        n = star.n

        def put(f, v):
            pf[h][slot0 + star.pf[f], 16 * g:16 * g + 16, :] = v.astype(BF16)

        for i in range(n):
            row = [cell(i, k) for k in sorted(range(n), key=lambda k: when(i, k))]
            r = functools.reduce(lambda x, y: x + y, row)
            put(('R', i), r)
            add_l(tiles[i], r[:8] + r[8:])
            col = sorted(range(n), key=lambda i2: (when(i2, i), i2 != i))
            sign = csign[n, i] = 1 if col[0] == i else -1
            c = cell(col[0], i)
            for i2 in col[1:]:
                c = c + cell(i2, i) if (1 if i2 == i else -1) == sign else c - cell(i2, i)
            put(('C', i), c)
            for j in range(n):
                if j != i:
                    put(('S', i, j), cell(i, j))
        for i, j in star.pairs:
            put(('A', i, j), cell(i, j) + cell(j, i))

    due = []

    def scores(x, u):
        if due and due[0][0] <= done_side[1]:
            x = _tie(x, due.pop(0)[1])
        s = (_dot if u in QT else _dot_nt)(x, _ld(q_scr, u))
        res.append(s)
        return s

    def job_e(I, h, J, p):
        tiles = [2 * (SB * I + i) + h for i in range(SB)]
        ps = []
        for i, u in enumerate(tiles):
            x = jnp.concatenate([k_scr.bitcast(U32)[2 * (SB * J + (t - i) % SB) + h, 8 * g:8 * g + 8, :]
                                 for g in (2 * p, 2 * p + 1) for t in range(SB)], axis=0)
            ps.append(jnp.exp2(scores(pltpu.bitcast(x, BF16), u)))
        when = lambda i, k: (i + k) % SB
        for n, g in enumerate((2 * p, 2 * p + 1)):
            cell = lambda i, k: ps[i][16 * (SB * n + when(i, k)):16 * (SB * n + when(i, k)) + 16]
            p_forms(_FULL, h, J * len(_FULL.pf), g, tiles, cell, when)

    def job_f(I, h):
        tiles = [2 * (SB * I + 2 + i) + h for i in range(2)]
        ps = {(i, k): jnp.exp2(scores(_ld(k_scr, 2 * (SB * I + k) + h), u))
              for i, u in enumerate(tiles) for k in range(2)}
        for g in range(T // 16):
            p_forms(_HALF, h, _HSLOT, g, tiles, lambda i, k: ps[i, k][16 * g:16 * g + 16], lambda i, k: 0)

    def job_d(I, h, i, k):
        u = 2 * (SB * I + i) + h
        s = scores(_ld(k_scr, 2 * (SB * I + k) + h), u)
        if i == k:
            s = jnp.where(causal, s, -1e9 * LOG2E)
        p = jnp.exp2(s)
        add_l(u, jnp.sum(p.reshape(T // 8, 8, T), axis=0))
        pf[h][_DSLOT + _DCELLS.index((i, k))] = p.astype(BF16)
        if (i, k) == _DCELLS[-1]:
            pf[h][_FENCE + z, 0:16, :] = jnp.zeros((16, T), BF16)
            for u in [2 * (SB * I + a) + h for a in range(SB)]:
                lrow[u] = jnp.sum(lsum.pop(u), axis=0, keepdims=True)
            ls = [lrow[2 * (SB * I + a) + h] for a in range(SB)]
            lo = jnp.minimum(jnp.minimum(ls[0], ls[1]), jnp.minimum(ls[2], ls[3]))
            hi = jnp.maximum(jnp.maximum(ls[0], ls[1]), jnp.maximum(ls[2], ls[3]))
            ok = jnp.logical_and(lo >= L_LO, hi <= L_HI)
            ok = jnp.logical_and(ok, (hi if I else jnp.maximum(ls[2], ls[3]))
                                 <= L_RATIO * (lo if I else jnp.minimum(ls[2], ls[3])))
            bad = jnp.where(ok, 0.0, 1.0)
            chk[1] = bad if chk[1] is None else jnp.maximum(chk[1], bad)

    def job_p(I, h, f, J):
        star, last = (_HALF, True) if J is None else (_FULL, J == I - 1)
        blk = I if J is None else J
        if f[0] == 'B':
            x = _ld(v_scr, 2 * (SB * blk + f[1]) + h, slice(HT // 2, HT))
        else:
            slot, r = _v_slot(star, blk, f)
            x = _ld(pf[h], slot, slice(r // 2, (r + HT) // 2))
        v = _dot(x, _ld(pf[h], (_HSLOT if J is None else J * len(_FULL.pf)) + star.pf[star.pv[f]]))
        res.append(v)
        key = (star.n,) + f
        acc[key] = v if key not in acc else acc[key] + v
        if not last:
            return

        def add(which, i, v, sign=1):
            k_ = (star.n, which, i)
            if k_ not in fg:
                fg[k_] = v if sign > 0 else -v
            else:
                fg[k_] = fg[k_] + v if sign > 0 else fg[k_] - v

        if f[0] == 'W':
            add('F', f[1], acc.pop(key))
        elif f[0] == 'B':
            add('G', f[1], acc.pop(key), csign[star.n, f[1]])
        elif f[0] == 'Q3':
            _, i, j = f
            q1, q2, q3 = (acc.pop((star.n, q, i, j)) for q in ('Q1', 'Q2', 'Q3'))
            t = ((q1 + q2) + q3) * (1.0 / (star.ts[i] - star.ts[j]))
            add('G', i, t)
            add('G', j, t)
            add('F', i, q1)
            add('F', j, q3, -1)

    def job_v(I, h, i, k):
        u = 2 * (SB * I + i) + h
        v = _dot(_ld(v_scr, 2 * (SB * I + k) + h), _ld(pf[h], _DSLOT + _DCELLS.index((i, k))))
        res.append(v)
        dacc[u] = v if u not in dacc else dacc[u] + v
        if k == i:
            o = dacc.pop(u)
            for star, a in ([(_FULL, i)] if I else []) + ([(_HALF, i - 2)] if i >= 2 else []):
                f, g = fg.pop((star.n, 'F', a)), fg.pop((star.n, 'G', a))
                o = o + jnp.concatenate([f - star.ts[a] * g, g], axis=0)
            o = o * (1.0 / lrow[u])
            of[u] = o
            chk[0] = chk[0] + jnp.sum(o.reshape(T // 8, 8, T), axis=0)

    def job_o(_, n):
        af, bf, outs = _O_JOBS[n][1]
        if af not in lhs:
            v = _form(af, lambda i, h: of[2 * i + h])
            lhs[af] = _tie(v.astype(BF16).T, v[0:8, :])
        if bf not in wo:
            wo[bf] = (wo_ref[_tile(bf[0][1]), _tile(bf[0][2])] if len(bf) == 1 else
                      _form(bf, lambda h, j: wo_ref[_tile(h), _tile(j)].astype(F32)).astype(BF16))
        v = _dot(lhs[af], wo[bf])
        res.append(v)
        for sign, i, j in outs:
            terms.setdefault((i, j), []).append((sign, v))
            if len(terms[i, j]) == left[i, j]:
                tot = acc_scr[_tile(i), _tile(j)]
                for sg, m in terms.pop((i, j)):
                    tot = tot + m if sg > 0 else tot - m
                acc_scr[_tile(i), _tile(j)] = tot

    fns = dict(e=job_e, f=job_f, d=job_d, p=job_p, v=job_v, o=job_o)
    order = _job_order(q_scr.shape[0] // (2 * SB))
    for n, job in enumerate(order):
        assert job[0] not in 'efd' or not any(j[0] in 'pv' and j[2] == job[2] and j[1] < job[1] for j in order[n:])
    side = list(side)
    fences = [n for n, job in enumerate(order) if job[0] == 'd' and job[3:] == _DCELLS[-1]]
    step = (len(order) - SIDE0 - SIDE1 - 10) / len(side)
    for n, job in enumerate(order):
        done_side[1] = n
        fns[job[0]](*job[1:])
        last_chance = n >= len(order) - SIDE1
        near = any(-SG1 <= f - n <= SG0 for f in fences)
        if side and n >= SIDE0 + step * done_side[0] and ((job[0] in 'pvo' and not near) or last_chance):
            done_side[0] += 1
            v = side.pop(0)(res[-1 - SLAG][8 * (n % 4):8 * (n % 4) + 8, :])
            if v is not None:
                due.append((n + SDUE, v))
    assert not side and not due
    fine = jnp.abs(chk[0]) < jnp.inf
    flag_scr[...] = jnp.maximum(flag_scr[...], jnp.where(fine, chk[1], 1.0))


def _kernel(x_hbm, c_hbm, wq_hbm, wuk_hbm, wuv_hbm, wo_hbm, w1_hbm, w2_hbm, w3_hbm, w4_hbm,
            cond_hbm, wmod_hbm, out_hbm,
            x_ref, c_ref, cond_ref, wma_ref, wmb_ref, w1_ref, w3_ref,
            wq_buf, wk_buf, wv_buf, wo_buf, out_buf, sem, wsem, osem,
            mod_scr, h_scr, cs_scr, hs_scr, w_scr, q_scr, k_scr, v_scr, acc_scr, xn_scr, xh_scr, a1_scr, t_scr,
            z_scr, mw_scr, m3_scr, wt_scr, wf_scr, gap_scr, st_in, pf_scr, vf_scr, flag_scr):
    S, M = x_hbm.shape
    D = wq_hbm.shape[2]
    nattn = wo_hbm.shape[0]
    Fd = w4_hbm.shape[0]
    scale = float(D) ** -0.5 * LOG2E
    nb, nrb = S // T, S // RB
    km, kc = M // T, c_hbm.shape[1] // T
    NX = 4
    XR = S // NX
    CB = XR // T

    work = (wk_buf, wv_buf, wq_buf)

    def pcopies(g, bufs=work, s0=0):
        return [pltpu.make_async_copy(src.bitcast(U32).at[:, g, :], dst, wsem.at[s0 + j])
                for j, (src, dst) in enumerate(zip((wuk_hbm, wuv_hbm, wq_hbm), bufs))]

    def ocopy(g):
        return pltpu.make_async_copy(wo_hbm.at[g], wo_buf, wsem.at[3])

    def chunk_copy(src, dst, i, s0):
        rows = slice(i * XR, (i + 1) * XR)
        return pltpu.make_async_copy(src.at[rows, :], dst.at[rows, :], sem.at[s0 + i])

    MS = 16
    NSL = T // MS
    assert nattn - 1 >= NSL
    mixw = ((w1_hbm, km, 0), (w2_hbm, km, km * MS), (w3_hbm, Fd // T, 2 * km * MS),
            (w4_hbm, -(-Fd // T), (2 * km + Fd // T) * MS))

    def prep_in(g):
        o = jnp.minimum(g, NSL - 1) * MS
        return [pltpu.make_async_copy(
            w.at[pl.ds(pl.multiple_of(jnp.minimum(b * T + o, w.shape[0] - MS), MS), MS), :],
            st_in.at[r0 + b * MS:r0 + (b + 1) * MS, :], wsem.at[7]) for w, nblk, r0 in mixw for b in range(nblk)]

    def stage_in(g):
        return pcopies(jnp.minimum(g + 1, nattn - 1))

    cp_cond = pltpu.make_async_copy(cond_hbm, cond_ref, sem.at[0])
    cp_wma = pltpu.make_async_copy(wmod_hbm.at[:, 0:2 * M], wma_ref, sem.at[1])
    cp_late = [pltpu.make_async_copy(src, dst, sem.at[2 + j]) for j, (src, dst) in enumerate((
        (wmod_hbm.at[:, 2 * M:6 * M], wmb_ref), (w1_hbm, w1_ref), (w3_hbm.at[Fd // T * T:, :], w3_ref)))]
    cp_x = [chunk_copy(x_hbm, x_ref, i, 7) for i in range(NX)]
    cp_c = [chunk_copy(c_hbm, c_ref, i, 7 + NX) for i in range(NX)]

    def silu_cond():
        cf = cond_ref[...].astype(F32)
        return jnp.broadcast_to((cf * jax.nn.sigmoid(cf)).astype(BF16), (8, M))

    cp_wk, cp_wv, cp_wq = pcopies(0)
    named = dict(k=cp_wk, v=cp_wv, q=cp_wq, o=ocopy(0), n=cp_cond, m=cp_wma)
    named.update(zip('abcd', cp_c))
    named.update(zip('wxyz', cp_x))
    started, arrived, did = set(), set(), set()

    def zero(r, carry):
        acc_scr[pl.ds(pl.multiple_of(r * T, T), T), :] = jnp.zeros((T, M), F32)
        return carry

    def x_rows(rows, dep):
        xf = x_ref[rows, :].astype(F32)
        if dep is None:
            return xf
        return jnp.concatenate([_after(xf[:, :T], _rows(dep, xf.shape[0])), xf[:, T:]], axis=1)

    def n_item(r, i):
        def fn(dep):
            rows = slice(r * T + i * LP, r * T + (i + 1) * LP)
            xn_scr[rows, :] = _ln(x_rows(rows, dep))
        return fn

    def h_item(r, i, normed):
        def fn(dep):
            rows = slice(i * LP, (i + 1) * LP)
            grows = slice(r * T + i * LP, r * T + (i + 1) * LP)
            sa = mod_scr[:, 0:M]
            if normed and dep is not None:
                sa = jnp.concatenate([_after(sa[:, _tile(j)], dep) for j in range(km)], axis=1)
            hf = ((xn_scr[grows, :] if normed else _ln(x_rows(grows, dep))) * _rows(mod_scr[:, M:2 * M], LP)
                  + _rows(sa, LP))
            for j in range(km):
                h_scr[r, j, rows, :] = hf[:, _tile(j)].astype(BF16)
            for f, n in _H_SUMS.items():
                if all(t[1] == r for t in f):
                    hs_scr[n, rows, :] = _form(f, lambda _, k: hf[:, _tile(k)]).astype(BF16)
            did.add(('h', r, i))
        return fn

    def release(jobs, span, items):
        if span and items:
            jobs.side += [(len(jobs.res) + 1 + i * span // len(items), fn) for i, fn in enumerate(items)]
            jobs.side.sort(key=lambda e: e[0])
        else:
            for fn in items:
                fn(None)

    def sum_items(n, group, index, dst, get, skip_rows):
        forms = [f for f in dict.fromkeys(t[0] for t in group)
                 if len(f) > 1 and not (skip_rows and len({t[1] for t in f}) == 1)]

        def item(f, rows):
            def fn(dep):
                def term(r, k):
                    v = get(r, k, rows).astype(F32)
                    return v if dep is None or (r, k) != f[0][1:] else _after(v, _rows(dep, v.shape[0]))
                dst[index[f], rows, :] = _form(f, term).astype(BF16)
            return fn

        return [item(f, slice(i, i + n)) for i in range(0, T, n) for f in forms]

    h_sums = lambda n, gi: sum_items(n, _H_GROUPS[gi], _H_SUMS, hs_scr,
                                     lambda r_, k, rows: h_scr[r_, k, rows, :], True)

    def stash(key, buf, j0, transpose=False):
        n = buf.shape[0] // T
        if key not in did:
            assert key in arrived
            did.add(key)
            for (j, hd), w in _pair_tiles(buf, transpose).items():
                w_scr[hd, j0 + j] = w
        return lambda hd: [_ld(w_scr, hd, j0 + j) for j in range(n)]

    def kv_tile(jobs, r):
        wk, wvT = stash('k', wk_buf, 0), stash('v', wv_buf, kc, True)
        ct = [c_ref[_tile(r), _tile(j)] for j in range(kc)]
        for hd in range(2):
            k_scr[2 * r + hd] = jobs.mm(ct, wk(hd), _dot).astype(BF16)
        for hd in range(2):
            v_scr[2 * r + hd] = jobs.mm(wvT(hd), ct, _dot_nt).astype(BF16)

    def q_tile(jobs, r):
        wq = stash('q', wq_buf, 2 * kc)
        ht = [_ld(h_scr, r, j) for j in range(km)]
        for hd in range(2):
            v = (jobs.mm(ht, wq(hd), _dot) * scale).astype(BF16)
            q_scr[2 * r + hd] = v.T if 2 * r + hd in QT else v

    for blk in _prologue().split(';'):
        waits, starts, acts = blk.split('|')
        for ch in waits.strip():
            assert ch in started and ch not in arrived
            arrived.add(ch)
            named[ch].wait()
        for ch in starts.strip():
            assert ch not in started
            started.add(ch)
            named[ch].start()
        jobs = _Jobs()
        for act in acts.split():
            if act == 'Z':
                jax.lax.fori_loop(0, nb, zero, 0)
                acc_scr[S:, :] = jnp.zeros((acc_scr.shape[0] - S, M), F32)
                x_ref[S:, :] = jnp.zeros((x_ref.shape[0] - S, M), BF16)
                flag_scr[...] = jnp.zeros(flag_scr.shape, F32)
            elif act == 'L':
                did.add('L')
                assert ('Q', 0) in did
                for cp in stage_in(0) + prep_in(0):
                    cp.start()
            elif act == 'M':
                assert arrived >= set('nm')
                mod = _dot(silu_cond(), wma_ref[...])
                mod_scr[:, 0:M] = mod[:, 0:M]
                mod_scr[:, M:2 * M] = 1.0 + mod[:, M:2 * M]
                did.add('M')
            else:
                act, _, span = act.partition('@')
                span = int(span or 0)
                items = []
                for r in [int(ch, 16) for ch in act[1:]]:
                    did.add((act[0], r))
                    if act[0] == 'K':
                        assert 'abcd'[r // CB] in arrived
                        kv_tile(jobs, r)
                    elif act[0] == 'H':
                        assert 'wxyz'[r // CB] in arrived and 'M' in did
                        items += [h_item(r, i, ('N', r) in did) for i in range(T // LP)]
                    elif act[0] == 'N':
                        assert 'wxyz'[r // CB] in arrived
                        items += [n_item(r, i) for i in range(T // LP)]
                    elif act[0] == 'Q':
                        assert all(('h', r, i) in did for i in range(T // LP))
                        q_tile(jobs, r)
                    elif act[0] == 'Y':
                        def zero_item(n0):
                            def fn(dep):
                                zero = jnp.where(dep > jnp.inf, jnp.uint32(1), jnp.uint32(0))
                                for n in range(n0, min(n0 + 4, _MIX3 + m3_scr.shape[0])):
                                    mw_scr.bitcast(U32)[n] = _rows(zero, T // 2)
                            return fn
                        items += [zero_item(n0) for n0 in range(_MIX3, _MIX3 + m3_scr.shape[0], 4)]
                    elif act[0] == 'F':
                        assert all(('K', SB * r + k_) in did for k_ in range(SB))
                        items += _v_form_items(v_scr, (pf_scr, vf_scr), r)
                    elif act[0] == 'C':
                        assert all('abcd'[t[1] // CB] in arrived for p_ in _C_GROUPS[r] for t in p_[0])
                        items += sum_items(
                            32, _C_GROUPS[r], _C_SUMS, cs_scr,
                            lambda r_, k, rows: c_ref[r_ * T + rows.start:r_ * T + rows.stop, _tile(k)], False)
                    else:
                        assert act[0] == 'S' and all(('h', t[1], T // LP - 1) in did for p_ in _H_GROUPS[r] for t in p_[0])
                        items += h_sums(32 if span else 16, r)
                release(jobs, span, items)
        assert not jobs.side
    assert arrived == set(named) and all((k_, r) in did for k_ in 'KHQ' for r in range(nb))
    assert all((k_, r) in did for k_ in 'CS' for r in range(2)) and 'L' in did
    assert all(('F', r) in did for r in range(SB))

    def mixer_prep(g):
        sl = jnp.minimum(g, NSL - 1)
        rows = pl.ds(pl.multiple_of(sl * MS, MS), MS)

        def part(m, forms):
            def fn(dep):
                base = {}

                def get(i, k):
                    if (i, k) not in base:
                        rb, cb = (i, k) if m == 2 else (k, i)
                        r0 = mixw[m][2] + rb * MS
                        v = _after(st_in[r0:r0 + MS, _tile(cb)].astype(F32), _rows(dep, MS))
                        if m == 3 and (rb + 1) * T > Fd:
                            v = jnp.where(rb * T + sl * MS < Fd, v, 0.0)
                        base[i, k] = v
                    return base[i, k]

                for f in forms:
                    v = _form(f, get)
                    mw_scr[_MIXW[m, f], rows, :] = (0.5 * v if m % 2 else v).astype(BF16)
            return fn

        items = []
        for m in range(4):
            forms = [f for mm_, f in _MIXW if mm_ == m]
            cur, terms = [], set()
            for f in forms:
                new_terms = terms | {t[1:] for t in f}
                if cur and 3 * len(new_terms) + sum(2 * len(x) + 1 for x in cur + [f]) > MWOPS:
                    items.append(part(m, cur))
                    cur, terms = [], set()
                cur.append(f)
                terms |= {t[1:] for t in f}
            items.append(part(m, cur))

        n3 = sum(m == 2 for m, _ in _MIXW)
        first = min(n for (m, _), n in _MIXW.items() if m == 2)
        per = -(-n3 // (nattn - 1 - NSL))

        def turn(j):
            def fn(dep):
                n = jnp.minimum(jnp.maximum(g - NSL, 0) * per + j, n3 - 1)
                w = _tie(_ld(mw_scr, first + n), dep).T
                m3_scr[n] = w
                return pltpu.bitcast(pltpu.bitcast(w, U32)[T // 2 - 8:], F32)
            return fn

        return items + [turn(j) for j in range(per)]

    def stage_wait():
        for cp in pcopies(0):
            cp.wait()
        pltpu.make_async_copy(st_in, st_in, wsem.at[7]).wait()

    def attn_body(g, carry):
        side = _gap_items(work, gap_scr) + _weight_form_items(work, gap_scr, wt_scr, wf_scr)
        bufs = (q_scr, k_scr, v_scr, (pf_scr, vf_scr), wo_buf, acc_scr, flag_scr)
        _attention_step(*bufs, g >> 16, side)

        @pl.when(g + 1 < nattn)
        def _():
            copies = stage_in(g + 1) + [ocopy(g + 1)]
            for cp in copies:
                cp.start()
            bufs = (h_scr, hs_scr, c_ref, cs_scr, wf_scr, q_scr, k_scr, v_scr, (pf_scr, vf_scr))
            side = [(SD0 + int(i * SDS), fn) for i, fn in enumerate(mixer_prep(g))]
            _proj_step(*bufs, scale, gap_scr, side)
            for cp in prep_in(g + 1):
                cp.start()
            stage_wait()
            ocopy(g + 1).wait()

        return carry

    stage_wait()
    for cp in cp_late:
        cp.start()
    jax.lax.fori_loop(0, nattn, attn_body, 0)

    def safe_pair(g, carry):
        copies = pcopies(g) + [ocopy(g)]
        for cp in copies:
            cp.start()
        for cp in copies:
            cp.wait()
        for buf, j0, transpose in ((wk_buf, 0, False), (wv_buf, kc, True), (wq_buf, 2 * kc, False)):
            for (j, hd), w in _pair_tiles(buf, transpose).items():
                w_scr[hd, j0 + j] = w

        def tile(u, carry):
            r, hd = u // 2, u % 2
            rows = pl.ds(pl.multiple_of(r * T, T), T)
            ct = [c_ref[rows, _tile(j)] for j in range(kc)]
            k_scr[u] = sum(_dot(ct[j], _ld(w_scr, hd, j)) for j in range(kc)).astype(BF16)
            v_scr[u] = sum(_dot_nt(_ld(w_scr, hd, kc + j), ct[j]) for j in range(kc)).astype(BF16)
            q = sum(_dot(_ld(h_scr, r, j), _ld(w_scr, hd, 2 * kc + j)) for j in range(km))
            q_scr[u] = (q * scale).astype(BF16)
            return carry

        jax.lax.fori_loop(0, 2 * nb, tile, 0)
        _attention_safe(q_scr, k_scr, v_scr, wo_buf, acc_scr)
        return carry

    @pl.when(jnp.max(flag_scr[...]) > 0)
    def _():
        jax.lax.fori_loop(0, nb, zero, 0)
        jax.lax.fori_loop(0, nattn, safe_pair, 0)

    for cp in cp_late:
        cp.wait()
    mod = _dot(silu_cond(), wmb_ref[...])
    mod_scr[:, 2 * M:4 * M] = mod[:, 0:2 * M]
    mod_scr[:, 4 * M:5 * M] = 1.0 + mod[:, 2 * M:3 * M]
    mod_scr[:, 5 * M:6 * M] = mod[:, 3 * M:4 * M]
    OFF = x_ref.shape[0] - S
    CAR = t_scr.shape[0] - RB

    def p1(r0, l0, n, dep=None):
        ga = mod_scr[:, 2 * M:3 * M]
        if dep is not None:
            ga = jnp.concatenate([_after(ga[:, 0:T], dep), ga[:, T:]], axis=1)
        rows = pl.ds(r0, n)
        x1 = x_ref[rows, :].astype(F32) + _rows(ga, n) * acc_scr[rows, :]
        xh_scr[0, l0:l0 + n, :] = x1
        hb = _ln(x1) * _rows(mod_scr[:, 4 * M:5 * M], n) + _rows(mod_scr[:, 3 * M:4 * M], n)
        xh_scr[1, l0:l0 + n, :] = hb
        return hb

    HT = T // 2
    last8 = lambda v: jnp.max(v[:, M - T:].reshape(PC // 8, 8, T), axis=0)

    def p1_store(r0, c, dep=None):
        v = _ln(p1(r0 + c * PC, OFF + c * PC, PC, dep))
        a1_scr[c * PC:(c + 1) * PC, :] = v
        return last8(v)

    def p1_first(r0, c, dep):
        return last8(p1(r0 + c * PC, OFF + c * PC, PC, dep))

    def p1_second(c, dep):
        hb = xh_scr[1, OFF + c * PC:OFF + (c + 1) * PC, :]
        v = _ln(jnp.concatenate([_after(hb[:, :T], _rows(dep, PC)), hb[:, T:]], axis=1))
        a1_scr[c * PC:(c + 1) * PC, :] = v
        return last8(v)

    t_scr[RB:RB + CAR - OFF, :] = jnp.zeros((CAR - OFF, M), F32)
    t_scr[RB + CAR - OFF:RB + CAR, :] = _gelu2(_dot(_ln(p1(0, 0, OFF)).astype(BF16), w1_ref[...]))
    for c in range(RB // PC):
        p1_store(OFF, c)

    def out_copy(i):
        rows = pl.ds(i * T if isinstance(i, int) else pl.multiple_of(i * T, T), T)
        return pltpu.make_async_copy(out_buf.at[rows, :], out_hbm.at[rows, :], osem.at[i])

    def b_body(r, carry):
        gb = _rows(mod_scr[:, 5 * M:6 * M], T)
        r0 = pl.multiple_of(r * RB, RB)
        n0 = pl.multiple_of(jnp.minimum(r0 + RB, S - RB) + OFF, OFF)
        nh = RB // T
        now = [0]
        due = []
        pace = []

        def p1_item(c, part):
            def fn(dep):
                v = p1_first(n0, c, dep) if part == 0 else p1_second(c, dep)
                due.append((now[0] + PD, v))
                due.sort(key=lambda e: e[0])
            return fn

        pace += [(P0 + i * PSTEP + part * PSPLIT, p1_item(i, part)) for i in range(RB // PC)
                 for part in range(2)]
        pace.sort(key=lambda e: e[0])

        def mm(lhs, wts, dot=_dot):
            acc = None
            for x, w in zip(lhs, wts):
                if due and due[0][0] <= now[0]:
                    w = _tie(w, due.pop(0)[1])
                v = dot(x, w)
                now[0] += x.shape[0] // HT
                acc = v if acc is None else v + acc
                if pace and pace[0][0] <= now[0]:
                    pace.pop(0)[1](v[0:8, :])
            return acc

        def fast(m, base, finish, hook=None):
            prods = _MIX[m]
            left, acc, done, cache = {}, {}, {}, {}
            for _, _, outs in prods:
                for _, i, h in outs:
                    left[i, h] = left.get((i, h), 0) + 1

            def act(form):
                sign, form = _canon(form)
                if form not in cache:
                    cache[form] = _form(form, lambda k, h: base(k)[h * HT:(h + 1) * HT]).astype(BF16)
                return sign, cache[form]

            for pi, (wf, af, outs) in enumerate(prods):
                w = _ld(m3_scr, _MIXW[m, wf] - _MIX3) if m == 2 else _ld(mw_scr, _MIXW[m, wf])
                if af is None:
                    k = wf[0][2]
                    v = mm([jnp.concatenate([act(((1, k, h),))[1] for h in range(2)], axis=0)], [w])
                    sign, parts = 1, [v[:HT], v[HT:]]
                else:
                    sign, x = act(af)
                    parts = [mm([x], [w])] * len(outs)
                for (s_, i, h), v in zip(outs, parts):
                    s_ = s_ * sign
                    if (i, h) not in acc:
                        acc[i, h] = (s_, v)
                    else:
                        s0, u = acc[i, h]
                        acc[i, h] = (s0, u + v if s0 == s_ else u - v) if s0 > 0 or s_ < 0 else (1, v - u)
                    left[i, h] -= 1
                    if not left[i, h]:
                        s0, done[i, h] = acc.pop((i, h))
                        assert s0 > 0
                        if (i, 1 - h) in done:
                            finish(i, jnp.concatenate([done[i, 0], done[i, 1]], axis=0))
                if hook is not None:
                    hook(pi, act)

        t_scr[0:CAR, :] = t_scr[RB:RB + CAR, :]
        for hf in range(nh):
            def put_t(n, v):
                t = _gelu2(v)
                if hf == nh - 1:
                    t = jnp.concatenate([t[:T - OFF], jnp.where(r < nrb - 1, t[T - OFF:], 0.0)], axis=0)
                t_scr[CAR + hf * T:CAR + (hf + 1) * T, _tile(n)] = t

            fast(0, lambda k: a1_scr[_tile(hf), _tile(k)], put_t)
        cq = M // 4
        shifts = (-1, 1, -2, 2)
        lane = jax.lax.broadcasted_iota(jnp.int32, (T, T), 1)
        y1, a3 = [], []
        for hf in range(nh):
            base = CAR - OFF + hf * T
            sh = []
            for j in range(km):
                g_lo, g_hi = (j * T) // cq, ((j + 1) * T - 1) // cq
                assert g_hi - g_lo <= 1

                def shifted(d):
                    v = t_scr[base - 8:base + T + 8, _tile(j)]
                    return pltpu.roll(v, (-d) % (T + 16), 0)[8:8 + T]

                v = shifted(shifts[g_lo])
                if g_hi != g_lo:
                    v = jnp.where(lane < g_hi * cq - j * T, v, shifted(shifts[g_hi]))
                sh.append(v)
            hs = {}
            fast(1, lambda k: sh[k], hs.__setitem__)
            hs = jnp.concatenate([hs[n] for n in range(km)], axis=1)
            y1.append(hs + xh_scr[1, _tile(hf), :])
            z_scr[_tile(hf), :] = xh_scr[0, _tile(hf), :] + gb * y1[hf]
            a3.append({})

            def ln_item(hf, c):
                def item(dep):
                    n = HT // NLN
                    for d in (0, HT):
                        v = y1[hf][d + c * n:d + (c + 1) * n]
                        if dep is not None:
                            v = jnp.concatenate([_after(v[:, :T], _rows(dep, n)), v[:, T:]], axis=1)
                        a3[hf][d + c * n] = _ln(v)
                return item

            ln_item(hf, 0)(None)
            pace += [(now[0] + LN0 + (c - 1) * LNS * (1 + hf), ln_item(hf, c)) for c in range(1, NLN)]
            pace.sort(key=lambda e: e[0])
        xh_scr[:, 0:OFF, :] = xh_scr[:, RB:RB + OFF, :]
        z_scr[pl.ds(pl.multiple_of(RB + (r >> 16) * 8, 8), 8), :] = jnp.zeros((8, M), F32)
        h3 = []
        for hf in range(nh):
            assert len(a3[hf]) == 2 * NLN
            af = jnp.concatenate([a3[hf][key] for key in sorted(a3[hf])], axis=0)
            row = {}
            narrow = []

            def hook(pi, act):
                j, rem = divmod(pi - NAR0, NARS)
                if rem == 0 and 0 <= j < km:
                    full = jnp.concatenate([act(((1, j, h),))[1] for h in range(2)], axis=0)
                    v = mm([w3_ref[:, _tile(j)]], [full], _dot_nt)
                    narrow[:] = [v + narrow[0] if narrow else v]

            def put_h(n, v):
                row[n] = _gelu2(v)
                if GD:
                    due.append((now[0] + GD, jnp.max(row[n].reshape(T // 8, 8, T), axis=0)))
                    due.sort(key=lambda e: e[0])

            fast(2, lambda k: af[:, _tile(k)], put_h, hook)
            fw = w3_ref.shape[0]
            row[Fd // T] = jnp.concatenate([_gelu2(narrow[0]), jnp.zeros((T - fw, T), F32)], axis=0).T
            h3.append(row)
        for hf in range(nh):
            rows = pl.ds(pl.multiple_of(r0 + hf * T, T), T)

            def finish(n, v):
                out_buf[rows, _tile(n)] = (z_scr[_tile(hf), _tile(n)] + gb[:, _tile(n)] * v).astype(out_buf.dtype)
                pltpu.make_async_copy(out_buf.at[rows, _tile(n)], out_hbm.at[rows, _tile(n)],
                                      osem.at[r * nh + hf]).start()

            fast(3, lambda k: h3[hf][k], finish)
        assert not pace
        return carry

    jax.lax.fori_loop(0, nrb, b_body, 0)
    for i in range(nb):
        out_copy(i).wait()


@jax.jit
def pallas_adaLN_cond__compressed_kv_cla__mixer_s_mlp__prompt_kernel(
    A_x: jax.Array,
    A_c_kv: jax.Array,
    A_w_q: jax.Array,
    A_w_uk: jax.Array,
    A_w_uv: jax.Array,
    A_w_o: jax.Array,
    B_x: jax.Array,
    B_w1: jax.Array,
    B_w2: jax.Array,
    B_w3: jax.Array,
    B_w4: jax.Array,
    c: jax.Array,
    w_mod: jax.Array,
):
    _, S, M = A_x.shape
    Dc = A_c_kv.shape[2]
    H, D = A_w_q.shape[1], A_w_q.shape[2]
    Fd = B_w3.shape[1]
    assert D == T and A_c_kv.shape[1] == S and Dc == 4 * T and M == 5 * T and 13 * T < Fd < 14 * T and S == 16 * T
    vmem = pltpu.VMEM
    packed = lambda *lead: vmem(lead + (T, T), BF16)
    out = pl.pallas_call(
        _kernel,
        in_specs=[pl.BlockSpec(memory_space=pltpu.HBM)] * 12,
        out_specs=pl.BlockSpec(memory_space=pltpu.HBM),
        out_shape=jax.ShapeDtypeStruct((S, M), A_x.dtype),
        scratch_shapes=[
            vmem((S + 16, M), BF16),
            vmem((S, Dc), BF16),
            vmem((1, M), BF16),
            vmem((M, 2 * M), BF16),
            vmem((M, 4 * M), BF16),
            vmem((M, M), BF16),
            vmem((Fd % T, M), BF16),
            vmem((M, D), U32),
            vmem((Dc, D), U32),
            vmem((Dc, D), U32),
            vmem((2 * D, M), BF16),
            vmem((S, M), A_x.dtype),
            pltpu.SemaphoreType.DMA((15,)),
            pltpu.SemaphoreType.DMA((8,)),
            pltpu.SemaphoreType.DMA((S // T,)),
            vmem((8, 6 * M), F32),
            vmem((S // T, M // T, T, T), BF16),
            vmem((len(_C_SUMS), T, T), BF16),
            vmem((len(_H_SUMS), T, T), BF16),
            packed(2, M // T + 2 * (Dc // T)),
            packed(2 * S // T),
            packed(2 * S // T),
            packed(2 * S // T),
            vmem((S + 16, M), F32),
            vmem((S, M), F32),
            vmem((2, RB + 16, M), F32),
            vmem((RB, M), F32),
            vmem((RB + 32, M), F32),
            vmem((RB + 8, M), F32),
            packed(len(_MIXW)),
            packed(sum(m == 2 for m, _ in _MIXW)),
            vmem((Dc // T, T, T), U32),
            vmem((len(_WF), T, T), BF16),
            vmem((3, 8, T), jnp.int32),
            vmem(((2 * (M // T) + Fd // T + -(-Fd // T)) * 16, M), BF16),
            vmem((_FENCE + 1, T, T), BF16),
            vmem((_FENCE + 1, T, T), BF16),
            vmem((8, T), F32),
        ],
        compiler_params=pltpu.CompilerParams(
            vmem_limit_bytes=100 * 1024 * 1024,
            disable_bounds_checks=True,
        ),
    )(
        A_x.reshape(S, M), A_c_kv.reshape(S, Dc),
        A_w_q, A_w_uk, A_w_uv,
        A_w_o.reshape(H // 2, 2 * D, M),
        B_w1, B_w2, B_w3.T, B_w4, c, w_mod,
    )
    return out.reshape(1, S, M)
```

```python
import functools
import math

import jax
import jax.numpy as jnp
import jax.experimental.pallas as pl
import jax.experimental.pallas.tpu as pltpu

F32 = jnp.float32
BF16 = jnp.bfloat16
U32 = jnp.uint32
NT = (((1,), (1,)), ((), ()))
T = 128
EPS = 1e-5
LOG2E = math.log2(math.e)

L_LO, L_HI, L_RATIO = 2.0 ** -24, 2.0 ** 24, 4.0

LAT_0, LAT_A = 24, 17
LAT_B = 20
RES, OEND = 32, 24
ONV = 0.7
TV, TO = 6, 2
QT = (4, 6)
SIDE0, SIDE1 = 8, 60
SLAG, SDUE = 3, 8
SG0, SG1 = 4, 0
WFK, WFQ = 4, 6
SD0, SDS = 4, 1.7
VF0, VFS = 4, 1.6
PDUE = 19
MWOPS = 74
RB = 256
PC = 32
P0, PSTEP, PSPLIT, PD = 305, 35, 44, 36
NLN, LN0, LNS = 4, 2, 6
GD = 36
NAR0, NARS = 10, 10
LP = 16
SP0, SP1 = 76, 38
_prologue = lambda: ('|kva|Z; |b|; kva|wc|Y0@56 K0123; bw|xdn|C0@56 N0123@52 K4567; cx|mq|N4567@52 F0@56 K89ab; '
            'd|y|C1@56 F1@56 Kcdef; nmq|zo|M H01 H234567@30 F2@36 Q0123; y||L H89ab@30 F3@36 Q4567; '
            'zo||Hcdef@30 S0@%d Q89ab S1@%d Qcdef' % (SP0, SP1))


def _dot(a, b):
    return jnp.dot(a, b, preferred_element_type=F32)


def _dot_nt(a, b):
    return jax.lax.dot_general(a, b, NT, preferred_element_type=F32)


def _ln(x):
    m = jnp.mean(x, axis=-1, keepdims=True)
    xc = x - m
    v = jnp.mean(xc * xc, axis=-1, keepdims=True)
    return xc * jnp.exp2(jnp.log(v + EPS) * (-0.5 * LOG2E))


def _rows(v, n):
    return jnp.broadcast_to(v[None], (n // 8, 8, v.shape[1])).reshape(n, v.shape[1])


def _gelu2(x):
    c0 = math.sqrt(2.0 / math.pi)
    return x + x * jnp.tanh(x * (c0 + (c0 * 0.044715) * (x * x)))


def _after(x, dep):
    return jnp.where(dep > jnp.inf, dep, x)


def _tie(x, dep):
    xu = pltpu.bitcast(x, U32)
    first = jnp.where(dep > jnp.inf, jnp.uint32(0), xu[:8])
    return pltpu.bitcast(jnp.concatenate([first, xu[8:]], axis=0), BF16)


def _tile(j):
    return slice(j * T, (j + 1) * T)


def _ld(ref, *idx):
    return pltpu.bitcast(ref.bitcast(U32)[idx], BF16)


def _group(rows, cols, pairs):
    xs, ys = dict.fromkeys(x for x, _ in pairs), dict.fromkeys(y for _, y in pairs)
    used = set(xs) | set(ys) | {(x[0], y[1]) for x, y in pairs} | {(y[0], x[1]) for x, y in pairs}
    prods = []
    for n, r in enumerate(rows):
        for i, k in [x for x in xs if x[0] == r]:
            mates = [y for x, y in pairs if x == (i, k)]
            prods.append((((1, i, k),) + tuple((1, i, k2) for _, k2 in mates), ((1, k, 0),),
                          ((1, i, 0), (-1, i, 1))))
            prods.append((((1, i, k),) + tuple((-1, i2, k) for i2, _ in mates), ((1, k, 0), (1, k, 1)),
                          ((1, i, 1),)))
        for i2, k2 in [y for y in ys if y[0] == r]:
            mates = [x for x, y in pairs if y == (i2, k2)]
            prods.append((((1, i2, k2),) + tuple((1, i2, k) for _, k in mates), ((1, k2, 1),),
                          ((1, i2, 1), (-1, i2, 0))))
            prods.append((((1, i2, k2),) + tuple((-1, i, k2) for i, _ in mates), ((1, k2, 0), (1, k2, 1)),
                          ((1, i2, 0),)))
        prods += [(((1, r, k),), ((1, k, h),), ((1, r, h),)) for k in cols if (r, k) not in used for h in (0, 1)]
        for (i, k), (i2, k2) in pairs:
            if r in (i, i2) and i + i2 - r in rows[n + 1:]:
                prods.append((((1, i, k2),), ((1, k2, 0), (-1, k, 0)), ((1, i2, 0), (1, i, 0))))
                prods.append((((1, i2, k), (1, i, k2)), ((1, k, 0), (1, k2, 1)), ((1, i2, 0), (1, i, 1))))
                prods.append((((1, i2, k),), ((1, k, 1), (-1, k2, 1)), ((1, i2, 1), (1, i, 1))))
    return prods


def _all_pairs(xrows, yrows):
    return [((x, a), (y, b)) for a, x in enumerate(xrows) for b, y in enumerate(yrows) if a != b]


_PAIRS65 = [((x[0] + 10, x[1]), (y[0] + 10, y[1])) for x, y in (
    ((0, 1), (1, 0)), ((0, 1), (5, 2)), ((2, 3), (1, 0)), ((2, 3), (3, 1)), ((2, 3), (5, 2)), ((3, 2), (1, 0)),
    ((4, 4), (0, 3)), ((4, 4), (1, 0)), ((4, 4), (3, 1)), ((4, 4), (5, 2)))]
_C_GROUPS = [_group(range(r, r + 8), range(4), _all_pairs(range(r, r + 4), range(r + 4, r + 8))) for r in (0, 8)]
_H_GROUPS = [_group(range(10), range(5), _all_pairs(range(5), range(5, 10))),
             _group(range(10, 16), range(5), _PAIRS65)]
_sum_index = lambda groups: {f: n for n, f in enumerate(
    dict.fromkeys(t[0] for g in groups for t in g if len(t[0]) > 1))}
_C_SUMS, _H_SUMS = _sum_index(_C_GROUPS), _sum_index(_H_GROUPS)


def _cells(rows, cols, pairs):
    xs = list(dict.fromkeys(p[0] for p in pairs))
    ys = list(dict.fromkeys(p[1] for p in pairs))
    used = set(xs + ys) | {(x[0], y[1]) for x, y in pairs} | {(y[0], x[1]) for x, y in pairs}

    def home_x(i, k):
        mates = [y for x, y in pairs if x == (i, k)]
        return [(((1, i, k),) + tuple((1, i, k2) for _, k2 in mates), ((1, k, 0),), ((1, i, 0), (-1, i, 1))),
                (((1, i, k),) + tuple((-1, i2, k) for i2, _ in mates), ((1, k, 0), (1, k, 1)), ((1, i, 1),))]

    def home_y(i2, k2):
        mates = [x for x, y in pairs if y == (i2, k2)]
        return [(((1, i2, k2),) + tuple((1, i2, k) for _, k in mates), ((1, k2, 1),), ((1, i2, 1), (-1, i2, 0))),
                (((1, i2, k2),) + tuple((-1, i, k2) for i, _ in mates), ((1, k2, 0), (1, k2, 1)), ((1, i2, 0),))]

    def cross(x, y):
        (i, k), (i2, k2) = x, y
        return [(((1, i, k2),), ((1, k2, 0), (-1, k, 0)), ((1, i2, 0), (1, i, 0))),
                (((1, i2, k), (1, i, k2)), ((1, k, 0), (1, k2, 1)), ((1, i2, 0), (1, i, 1))),
                (((1, i2, k),), ((1, k, 1), (-1, k2, 1)), ((1, i2, 1), (1, i, 1)))]

    direct = lambda i: [(((1, i, k),), None, ((1, i, 0), (1, i, 1))) for k in cols if (i, k) not in used]
    single = lambda i: ([t for x in xs if x[0] == i for t in home_x(*x)]
                        + [t for y in ys if y[0] == i for t in home_y(*y)] + direct(i))
    prods = []
    for n, i in enumerate(rows):
        prods += single(i)
        for i2 in rows[n + 1:]:
            for x, y in pairs:
                if {x[0], y[0]} == {i, i2}:
                    prods += cross(x, y)
    return prods


_square = lambda q: [((a, a), (q + b, b)) for a in range(q) for b in range(q) if a != b]
_shift = lambda pairs, r0: [((x[0] + r0, x[1]), (y[0] + r0, y[1])) for x, y in pairs]
_flip = lambda pairs: [(x[::-1], y[::-1]) for x, y in pairs]
_P35 = [((1, 2), (0, 4)), ((1, 2), (2, 1)), ((2, 3), (0, 4)), ((2, 3), (1, 0))]
_P45 = [((0, 2), (1, 1)), ((2, 4), (0, 3)), ((2, 4), (1, 1)), ((2, 4), (3, 2)), ((3, 0), (0, 3)), ((3, 0), (1, 1))]
_P55 = [((2, 1), (0, 4)), ((2, 1), (1, 0)), ((2, 1), (3, 2)), ((2, 1), (4, 3)), ((3, 3), (0, 4)), ((3, 3), (1, 0)),
        ((4, 2), (0, 4)), ((4, 2), (1, 0))]
_MIX = [_cells(range(5), range(5), _P55), _cells(range(5), range(5), _P55),
        _cells(range(13), range(5), _square(5) + _shift(_P35, 10)),
        _cells(range(5), range(14), _flip(_square(5) + _shift(_P45, 10)))]
_MIXW = {(m, f): n for n, (m, f) in enumerate(dict.fromkeys((m, t[0]) for m in range(4) for t in _MIX[m]))}
_MIX3 = min(n for (m, _), n in _MIXW.items() if m == 2)


def _form(form, get):
    acc = None
    for sign, i, j in form:
        v = get(i, j)
        acc = v if acc is None else (acc + v if sign > 0 else acc - v)
    return acc


def _gap_items(bufs, gap_scr):
    items = []
    for n, buf in enumerate(bufs):
        acc = []

        def part(r0, buf=buf, acc=acc):
            def fn(dep):
                wu = jnp.concatenate([buf[r:r + 8, :] for r in range(r0, r0 + T, 32)])
                mask = jnp.full((8, T), 0x7FFF0000, U32)
                if dep is not None:
                    mask = jnp.where(dep > jnp.inf, jnp.uint32(0), mask)
                mask = _rows(mask, 32)
                new = [jnp.sum(pltpu.bitcast(v & mask, F32).reshape(4, 8, T), axis=0) for v in (wu << 16, wu)]
                acc[:] = [u + v for u, v in zip(acc, new)] if acc else new
            return fn

        def last(_, n=n, acc=acc):
            bits = []
            for v in acc:
                l1 = jnp.sum(jnp.sum(v, axis=1, keepdims=True), axis=0, keepdims=True)
                bits.append(pltpu.bitcast(jnp.broadcast_to(l1, (8, T)), jnp.int32) >> 8)
            gap = jnp.clip((bits[0] - bits[1] + (1 << 14)) >> 15, -8, 8) << 23
            gap_scr[n] = gap
            return pltpu.bitcast(gap, F32)

        items += [part(r0) for r0 in range(0, buf.shape[0], T)] + [last]
    return items


def _pair_tiles(w_ref, transpose=False):
    tiles = {}
    for j in range(w_ref.shape[0] // T):
        wu = w_ref[_tile(j), :]
        if transpose:
            wu = wu.T
        tiles[j, 0] = pltpu.bitcast(wu << 16, F32).astype(BF16)
        tiles[j, 1] = pltpu.bitcast(wu & jnp.uint32(0xFFFF0000), F32).astype(BF16)
    return tiles


def _canon(form):
    if form[-1][0] < 0 and form[0][1:] > form[1][1:]:
        return -1, ((1,) + form[1][1:], (-1,) + form[0][1:])
    return 1, form


_w_forms = lambda groups: list(dict.fromkeys(_canon(t[1])[1] for g in groups for t in g))
_WF = {key: n for n, key in enumerate([(m, f) for m, groups in enumerate((_C_GROUPS, _C_GROUPS, _H_GROUPS))
                                       for f in _w_forms(groups)])}


def _weight_form_items(bufs, gap_scr, wt_scr, wf_scr):
    n = 16
    items = []

    def flip(j):
        def fn(dep):
            wu = bufs[1][_tile(j), :]
            wu = (wu if dep is None else jnp.where(_rows(dep, T) > jnp.inf, jnp.uint32(0), wu)).T
            wt_scr[j] = wu
            return pltpu.bitcast(wu[T - 8:], F32)
        return fn

    def part(m, r0, forms):
        def fn(dep):
            fac = pltpu.bitcast(0x3F800000 + gap_scr[m], F32)
            mask = jnp.full((8, T), 0xFFFF0000, U32)
            sh = jnp.full((8, T), 16, U32)
            if dep is not None:
                mask = jnp.where(dep > jnp.inf, jnp.uint32(0), mask)
                sh = jnp.where(dep > jnp.inf, jnp.uint32(0), sh)
            fac, mask, sh = _rows(fac, n), _rows(mask, n), _rows(sh, n)
            base = {}

            def get(k, h):
                if (k, h) not in base:
                    wu = wt_scr[k, r0:r0 + n, :] if m == 1 else bufs[m][k * T + r0:k * T + r0 + n, :]
                    base[k, h] = pltpu.bitcast(wu & mask, F32) * fac if h else pltpu.bitcast(wu << sh, F32)
                return base[k, h]

            for f in forms:
                wf_scr[_WF[m, f], r0:r0 + n, :] = _form(f, get).astype(BF16)
        return fn

    for m in range(3):
        forms = [f for mm, f in _WF if mm == m]
        if m == 1:
            items += [flip(j) for j in range(bufs[1].shape[0] // T)]
        per = -(-len(forms) // (WFQ if m == 2 else WFK))
        forms.sort(key=lambda f: sorted({t[1] for t in f}))
        items += [part(m, r0, forms[i:i + per]) for r0 in range(0, T, n) for i in range(0, len(forms), per)]
    return items


def _run_group(jobs, prods, a_get, w, transposed, finish):
    left = {}
    for _, _, outs in prods:
        for _, i, h in outs:
            left[i, h] = left.get((i, h), 0) + 1
    acc = {}
    for af, bf, outs in prods:
        sign, wt = w(bf)
        m = jobs.mm([wt], [a_get(af)], _dot_nt) if transposed else jobs.mm([a_get(af)], [wt], _dot)
        for s_, i, h in outs:
            if (i, h) not in acc:
                acc[i, h] = (s_ * sign, m)
            else:
                s0, v = acc[i, h]
                acc[i, h] = (s0, v + m if s0 == s_ * sign else v - m) if s0 > 0 or s_ * sign < 0 else (1, m - v)
            left[i, h] -= 1
            if not left[i, h]:
                s0, v = acc.pop((i, h))
                assert s0 > 0
                finish(2 * i + h, v)


class _Jobs:
    def __init__(self, side=()):
        self.res = []
        self.side = list(side)
        self.due = []

    def mm(self, lhs, wt, dot):
        acc = None
        for x, w in zip(lhs, wt):
            if self.due and self.due[0][0] <= len(self.res):
                x = _tie(x, self.due.pop(0)[1])
            v = dot(x, w)
            self.res.append(v)
            acc = v if acc is None else v + acc
            rel = 4 * (len(self.res) % 4)
            while self.side and self.side[0][0] <= len(self.res):
                out = self.side.pop(0)[1](v[8 * rel:8 * rel + 8, :])
                if out is not None:
                    self.due.append((len(self.res) + PDUE, out))
                rel = (rel + 2) % 16
        return acc


def _proj_step(h_scr, hs_scr, c_ref, cs_scr, wf_scr, q_scr, k_scr, v_scr, pf, scale, shifts, side):
    def weight(m):
        def get(form):
            sign, form = _canon(form)
            return sign, _ld(wf_scr, _WF[m, form])
        get.inv = pltpu.bitcast(0x3F800000 - shifts[m], F32)
        return get

    wk, wvT, wq = weight(0), weight(1), weight(2)
    c_get = lambda f: _ld(cs_scr, _C_SUMS[f]) if len(f) > 1 else c_ref[_tile(f[0][1]), _tile(f[0][2])]
    h_get = lambda f: _ld(hs_scr, _H_SUMS[f]) if len(f) > 1 else _ld(h_scr, f[0][1], f[0][2])

    def put(dst, w, mul=None):
        muls = [mul, _rows(w.inv if mul is None else w.inv * mul, T)]

        def fn(u, v):
            v = (v if muls[u % 2] is None else v * muls[u % 2]).astype(BF16)
            dst[u] = v.T if mul is not None and u in QT else v
        return fn

    jobs = _Jobs(side)
    put_v, stored = put(v_scr, wvT), set()
    nxt = [0]

    def fin_v(u, v):
        put_v(u, v)
        stored.add(u)
        for J in range(SB):
            if all(2 * (SB * J + k) + h in stored for k in range(SB) for h in range(2)) and ('J', J) not in stored:
                stored.add(('J', J))
                for fn in _v_form_items(v_scr, pf, J):
                    nxt[0] = max(nxt[0] + VFS, len(jobs.res) + VF0)
                    jobs.side.append((int(nxt[0]), fn))
                jobs.side.sort(key=lambda e: e[0])

    kk, vv, qq = ((c_get, wk, False, put(k_scr, wk)), (c_get, wvT, True, fin_v),
                  (h_get, wq, False, put(q_scr, wq, scale)))
    for prods, args in ((_C_GROUPS[0], kk), (_C_GROUPS[0], vv), (_C_GROUPS[1], vv), (_C_GROUPS[1], kk),
                        (_H_GROUPS[0], qq), (_H_GROUPS[1], qq)):
        _run_group(jobs, prods, *args)
    assert not jobs.side and not jobs.due


def _inner_group(rows, cols, pairs):
    xs, ys = dict.fromkeys(x for x, _ in pairs), dict.fromkeys(y for _, y in pairs)
    used = set(xs) | set(ys) | {(x[0], y[1]) for x, y in pairs} | {(y[0], x[1]) for x, y in pairs}
    prods = []
    for i, j in xs:
        mates = [y for x, y in pairs if x == (i, j)]
        prods.append((((1, i, 0),), ((1, 0, j), (-1, 1, j)), ((1, i, j),) + tuple((1, i2, j) for i2, _ in mates)))
        prods.append((((1, i, 0), (1, i, 1)), ((1, 1, j),), ((1, i, j),) + tuple((-1, i, j2) for _, j2 in mates)))
    for i2, j2 in ys:
        mates = [x for x, y in pairs if y == (i2, j2)]
        prods.append((((1, i2, 0), (1, i2, 1)), ((1, 0, j2),),
                      ((1, i2, j2),) + tuple((-1, i2, j) for _, j in mates)))
        prods.append((((1, i2, 1),), ((1, 0, j2), (-1, 1, j2)),
                      ((-1, i2, j2),) + tuple((-1, i, j2) for i, _ in mates)))
    prods += [(((1, i, h),), ((1, h, j),), ((1, i, j),))
              for i in rows for j in cols if (i, j) not in used for h in (0, 1)]
    for (i, j), (i2, j2) in pairs:
        lo, hi = min(j, j2), max(j, j2)
        prods.append((((1, i2, 0), (-1, i, 0)), ((1, 0, lo), (1, 0, hi)), ((1, i2, j),)))
        prods.append((((1, i, 0), (1, i2, 1)), ((1, 0, j2), (1, 1, j)), ((1, i, j2), (1, i2, j))))
        prods.append((((1, i, 1), (-1, i2, 1)), ((1, 1, lo), (1, 1, hi)), ((1, i, j2),)))
    return prods


def _o_jobs():
    prods = (_inner_group(range(10), range(5), _all_pairs(range(0, 10, 2), range(1, 10, 2)))
             + _inner_group(range(10, 16), range(5), _PAIRS65))
    row = lambda t: max(i for _, i, _ in t[0])
    unit = lambda t: max(2 * i + h for _, i, h in t[0])
    need = lambda t: unit(t) if row(t) == 15 else 2 * row(t) + 1
    return [(need(t), t) for t in sorted(prods, key=need)]


_O_JOBS = _o_jobs()


SB = 4


class _Star:
    def __init__(self, ts):
        self.ts, self.n = ts, len(ts)
        rn = range(self.n)
        self.pairs = [(i, j) for i in rn for j in rn if i < j]
        self.pf = {f: m for m, f in enumerate([('R', i) for i in rn] + [('C', i) for i in rn]
                                              + [('S', i, j) for i in rn for j in rn if i != j]
                                              + [('A', i, j) for i, j in self.pairs])}
        self.vf = {f: m for m, f in enumerate([('W', i) for i in rn]
                                              + [(q, i, j) for i, j in self.pairs for q in ('Q1', 'Q2', 'Q3')])}
        self.pv = {**{('W', i): ('R', i) for i in rn}, **{('B', i): ('C', i) for i in rn},
                   **{('Q1', i, j): ('S', i, j) for i, j in self.pairs},
                   **{('Q2', i, j): ('A', i, j) for i, j in self.pairs},
                   **{('Q3', i, j): ('S', j, i) for i, j in self.pairs}}

    def products(self, i):
        return [('W', i), ('B', i)] + [(q, i, j) for j in range(i + 1, self.n) for q in ('Q1', 'Q2', 'Q3')]


_FULL = _Star((-1.125, -0.375, 0.375, 1.125))
_HALF = _Star((-0.75, 0.75))
_DCELLS = [(0, 0), (1, 0), (1, 1), (2, 2), (3, 2), (3, 3)]
_HSLOT = (SB - 1) * len(_FULL.pf)
_DSLOT = _HSLOT + len(_HALF.pf)
_VSLOT = _DSLOT + len(_DCELLS)
_VHALF = (SB - 1) * len(_FULL.vf)
_FENCE = _VSLOT + (_VHALF + SB * len(_HALF.vf) + 1) // 2


def _v_slot(star, J, f):
    m = star.vf[f] + J * len(star.vf) + (0 if star is _FULL else _VHALF)
    return _VSLOT + m // 2, m % 2 * (T // 2)


def _v_form_items(v_scr, pf, J):
    n, HT = 16, T // 2

    def item(star, h, r0, pairs):
        def fn(dep):
            ts = [jnp.full((8, T), t, F32) for t in star.ts]
            ts = [_rows(t if dep is None else _after(t, dep), n) for t in ts]

            def get(k, a):
                r = (a * HT + r0) // 2
                return _ld(v_scr, 2 * (SB * J + k) + h, slice(r, r + n // 2)).astype(F32)

            def put(f, v):
                slot, r = _v_slot(star, J, f)
                pf[h][slot, r + r0:r + r0 + n, :] = v.astype(BF16)

            b = {(k, a): get(k, a) for k in sorted({k for pr in pairs or star.pairs for k in pr})
                 for a in range(2)}
            if pairs is None or star.n == 2:
                w = [b[k, 0] + ts[k] * b[k, 1] for k in range(star.n)]
                for k in range(star.n):
                    put(('W', k), w[k])
                for i, j in star.pairs:
                    put(('Q2', i, j), w[i] - w[j])
            for i, j in pairs or ():
                d0, d1 = b[j, 0] - b[i, 0], b[j, 1] - b[i, 1]
                put(('Q1', i, j), d0 + ts[i] * d1)
                put(('Q3', i, j), d0 + ts[j] * d1)
        return fn

    pr = _FULL.pairs
    parts = [(_HALF, _HALF.pairs)]
    if J < SB - 1:
        parts += [(_FULL, x) for x in (None, pr[:2], [pr[2], pr[4]], [pr[3], pr[5]])]
    return [item(star, h, r0, pairs) for h in range(2) for r0 in range(0, HT, n) for star, pairs in parts]


def _job_order(nsb):
    units = [(I, h) for I in range(nsb) for h in range(2)]
    qe, qv = [], []
    for I, h in units:
        qe += [('e', I, h, J, p) for J in range(I) for p in range(SB)] + [('f', I, h)]
        qe += [('d', I, h) + c for c in _DCELLS]
        for i in range(SB):
            qv += [('p', I, h, f, J) for f in _FULL.products(i) for J in range(I)]
            if i >= 2:
                qv += [('p', I, h, f, None) for f in _HALF.products(i - 2)]
            qv += [('v', I, h) + c for c in _DCELLS if c[0] == i]
    qo = [('o', u, j) for j, (u, _) in enumerate(_O_JOBS)]
    cost = dict(e=8, f=8, d=2, p=1, v=2, o=2)
    order, done = [], {}
    now = [0]

    def emit(q):
        job = q.pop(0)
        order.append(job)
        now[0] += cost[job[0]]
        if job[0] == 'd':
            done[job] = now[0]
        elif job[0] == 'v' and job[4] == job[3]:
            done['u', 2 * (SB * job[1] + job[3]) + job[2]] = now[0]
        return cost[job[0]]

    def v_ready():
        if not qv:
            return False
        key = ('d', qv[0][1], qv[0][2], SB - 1, SB - 1)
        return key in done and done[key] + (LAT_0 if qv[0][1:3] == (0, 0) else LAT_A) <= now[0]

    def o_ready():
        return bool(qo) and ('u', qo[0][1]) in done and done['u', qo[0][1]] + LAT_B <= now[0]

    def fill(nv, no):
        n = 0
        while nv > 0 or no > 0 or n % 4:
            if no > 0 and n % 2 == 0 and o_ready() and no * ONV >= nv:
                no -= 2
                n += emit(qo)
            elif v_ready() and (nv > 0 or n % 4):
                c = emit(qv)
                nv -= c
                n += c
            elif o_ready() and n % 2 == 0 and (no > 0 or n % 4 or nv > 0) and len(qo) > RES:
                no -= 2
                n += emit(qo)
            else:
                break

    while qe:
        unit = qe[0][1:3]
        while qv and qv[0][2] == unit[1] and qv[0][1] < unit[0]:
            emit(qv)
        ne = 0
        while qe and ne < 8 and (ne == 0 or (qe[0][0] == 'd' and qe[0][1:3] == unit and ne + 2 <= 8)):
            ne += emit(qe)
        groups = lambda q: sum(cost[j[0]] for j in q) / 8
        old = [j for j in qv if j[1:3] != unit and ('d', j[1], j[2], SB - 1, SB - 1) in done]
        here = [j for j in qe if j[1:3] == unit]
        rest = sum(cost[j[0]] for j in old)
        nv = (rest - LAT_A) / (groups(here) + 1) if here else rest
        no = 2 * max(len(qo) - RES - OEND, 0) / (groups(qe) + 1)
        fill(int(nv + 0.5), int(no + 0.5))
    while qv or qo:
        if qv and v_ready():
            fill(TV, TO)
            if not qv:
                continue
        elif o_ready():
            emit(qo)
        else:
            emit(qv or qo)
    return order


def _attention_safe(q_scr, k_scr, v_scr, wo_ref, acc_scr):
    causal = (jax.lax.broadcasted_iota(jnp.int32, (T, T), 0)
              <= jax.lax.broadcasted_iota(jnp.int32, (T, T), 1))

    def unit(u, carry):
        r, hd = u // 2, u % 2

        def block(c, mlo):
            m0, l, o = mlo
            s = _dot_nt(_ld(k_scr, 2 * c + hd), _ld(q_scr, u))
            s = jnp.where(jnp.logical_or(causal, c < r), s, -1e9 * LOG2E)
            m = jnp.maximum(m0, jnp.max(s, axis=0, keepdims=True))
            a = jnp.exp2(m0 - m)
            p = jnp.exp2(s - m)
            return (m, l * a + jnp.sum(p, axis=0, keepdims=True),
                    o * a + _dot(_ld(v_scr, 2 * c + hd), p.astype(BF16)))

        _, l, o = jax.lax.fori_loop(0, r + 1, block, (jnp.full((1, T), -jnp.inf, F32), jnp.zeros((1, T), F32),
                                                      jnp.zeros((T, T), F32)))
        rows = pl.ds(pl.multiple_of(r * T, T), T)
        acc_scr[rows, :] += _dot((o * (1.0 / l)).astype(BF16).T, wo_ref[pl.ds(pl.multiple_of(hd * T, T), T), :])
        return carry

    jax.lax.fori_loop(0, q_scr.shape[0], unit, 0)


def _attention_step(q_scr, k_scr, v_scr, pf, wo_ref, acc_scr, flag_scr, z, side):
    causal = (jax.lax.broadcasted_iota(jnp.int32, (T, T), 0)
              <= jax.lax.broadcasted_iota(jnp.int32, (T, T), 1))
    HT = T // 2
    lsum, lrow, acc, fg, dacc, of, lhs = {}, {}, {}, {}, {}, {}, {}
    res = []
    wo, terms = {}, {}
    left = {}
    done_side = [0, 0]
    chk = [jnp.zeros((8, T), F32), None]
    for _, t in _O_JOBS:
        for _, i, j in t[2]:
            left[i, j] = left.get((i, j), 0) + 1

    def add_l(u, v):
        lsum[u] = v if u not in lsum else lsum[u] + v

    csign = {}

    def p_forms(star, h, slot0, g, tiles, cell, when):
        n = star.n

        def put(f, v):
            pf[h][slot0 + star.pf[f], 16 * g:16 * g + 16, :] = v.astype(BF16)

        for i in range(n):
            row = [cell(i, k) for k in sorted(range(n), key=lambda k: when(i, k))]
            r = functools.reduce(lambda x, y: x + y, row)
            put(('R', i), r)
            add_l(tiles[i], r[:8] + r[8:])
            col = sorted(range(n), key=lambda i2: (when(i2, i), i2 != i))
            sign = csign[n, i] = 1 if col[0] == i else -1
            c = cell(col[0], i)
            for i2 in col[1:]:
                c = c + cell(i2, i) if (1 if i2 == i else -1) == sign else c - cell(i2, i)
            put(('C', i), c)
            for j in range(n):
                if j != i:
                    put(('S', i, j), cell(i, j))
        for i, j in star.pairs:
            put(('A', i, j), cell(i, j) + cell(j, i))

    due = []

    def scores(x, u):
        if due and due[0][0] <= done_side[1]:
            x = _tie(x, due.pop(0)[1])
        s = (_dot if u in QT else _dot_nt)(x, _ld(q_scr, u))
        res.append(s)
        return s

    def job_e(I, h, J, p):
        tiles = [2 * (SB * I + i) + h for i in range(SB)]
        ps = []
        for i, u in enumerate(tiles):
            x = jnp.concatenate([k_scr.bitcast(U32)[2 * (SB * J + (t - i) % SB) + h, 8 * g:8 * g + 8, :]
                                 for g in (2 * p, 2 * p + 1) for t in range(SB)], axis=0)
            ps.append(jnp.exp2(scores(pltpu.bitcast(x, BF16), u)))
        when = lambda i, k: (i + k) % SB
        for n, g in enumerate((2 * p, 2 * p + 1)):
            cell = lambda i, k: ps[i][16 * (SB * n + when(i, k)):16 * (SB * n + when(i, k)) + 16]
            p_forms(_FULL, h, J * len(_FULL.pf), g, tiles, cell, when)

    def job_f(I, h):
        tiles = [2 * (SB * I + 2 + i) + h for i in range(2)]
        ps = {(i, k): jnp.exp2(scores(_ld(k_scr, 2 * (SB * I + k) + h), u))
              for i, u in enumerate(tiles) for k in range(2)}
        for g in range(T // 16):
            p_forms(_HALF, h, _HSLOT, g, tiles, lambda i, k: ps[i, k][16 * g:16 * g + 16], lambda i, k: 0)

    def job_d(I, h, i, k):
        u = 2 * (SB * I + i) + h
        s = scores(_ld(k_scr, 2 * (SB * I + k) + h), u)
        if i == k:
            s = jnp.where(causal, s, -1e9 * LOG2E)
        p = jnp.exp2(s)
        add_l(u, jnp.sum(p.reshape(T // 8, 8, T), axis=0))
        pf[h][_DSLOT + _DCELLS.index((i, k))] = p.astype(BF16)
        if (i, k) == _DCELLS[-1]:
            pf[h][_FENCE + z, 0:16, :] = jnp.zeros((16, T), BF16)
            for u in [2 * (SB * I + a) + h for a in range(SB)]:
                lrow[u] = jnp.sum(lsum.pop(u), axis=0, keepdims=True)
            ls = [lrow[2 * (SB * I + a) + h] for a in range(SB)]
            lo = jnp.minimum(jnp.minimum(ls[0], ls[1]), jnp.minimum(ls[2], ls[3]))
            hi = jnp.maximum(jnp.maximum(ls[0], ls[1]), jnp.maximum(ls[2], ls[3]))
            ok = jnp.logical_and(lo >= L_LO, hi <= L_HI)
            ok = jnp.logical_and(ok, (hi if I else jnp.maximum(ls[2], ls[3]))
                                 <= L_RATIO * (lo if I else jnp.minimum(ls[2], ls[3])))
            bad = jnp.where(ok, 0.0, 1.0)
            chk[1] = bad if chk[1] is None else jnp.maximum(chk[1], bad)

    def job_p(I, h, f, J):
        star, last = (_HALF, True) if J is None else (_FULL, J == I - 1)
        blk = I if J is None else J
        if f[0] == 'B':
            x = _ld(v_scr, 2 * (SB * blk + f[1]) + h, slice(HT // 2, HT))
        else:
            slot, r = _v_slot(star, blk, f)
            x = _ld(pf[h], slot, slice(r // 2, (r + HT) // 2))
        v = _dot(x, _ld(pf[h], (_HSLOT if J is None else J * len(_FULL.pf)) + star.pf[star.pv[f]]))
        res.append(v)
        key = (star.n,) + f
        acc[key] = v if key not in acc else acc[key] + v
        if not last:
            return

        def add(which, i, v, sign=1):
            k_ = (star.n, which, i)
            if k_ not in fg:
                fg[k_] = v if sign > 0 else -v
            else:
                fg[k_] = fg[k_] + v if sign > 0 else fg[k_] - v

        if f[0] == 'W':
            add('F', f[1], acc.pop(key))
        elif f[0] == 'B':
            add('G', f[1], acc.pop(key), csign[star.n, f[1]])
        elif f[0] == 'Q3':
            _, i, j = f
            q1, q2, q3 = (acc.pop((star.n, q, i, j)) for q in ('Q1', 'Q2', 'Q3'))
            t = ((q1 + q2) + q3) * (1.0 / (star.ts[i] - star.ts[j]))
            add('G', i, t)
            add('G', j, t)
            add('F', i, q1)
            add('F', j, q3, -1)

    def job_v(I, h, i, k):
        u = 2 * (SB * I + i) + h
        v = _dot(_ld(v_scr, 2 * (SB * I + k) + h), _ld(pf[h], _DSLOT + _DCELLS.index((i, k))))
        res.append(v)
        dacc[u] = v if u not in dacc else dacc[u] + v
        if k == i:
            o = dacc.pop(u)
            for star, a in ([(_FULL, i)] if I else []) + ([(_HALF, i - 2)] if i >= 2 else []):
                f, g = fg.pop((star.n, 'F', a)), fg.pop((star.n, 'G', a))
                o = o + jnp.concatenate([f - star.ts[a] * g, g], axis=0)
            o = o * (1.0 / lrow[u])
            of[u] = o
            chk[0] = chk[0] + jnp.sum(o.reshape(T // 8, 8, T), axis=0)

    def job_o(_, n):
        af, bf, outs = _O_JOBS[n][1]
        if af not in lhs:
            v = _form(af, lambda i, h: of[2 * i + h])
            lhs[af] = _tie(v.astype(BF16).T, v[0:8, :])
        if bf not in wo:
            wo[bf] = (wo_ref[_tile(bf[0][1]), _tile(bf[0][2])] if len(bf) == 1 else
                      _form(bf, lambda h, j: wo_ref[_tile(h), _tile(j)].astype(F32)).astype(BF16))
        v = _dot(lhs[af], wo[bf])
        res.append(v)
        for sign, i, j in outs:
            terms.setdefault((i, j), []).append((sign, v))
            if len(terms[i, j]) == left[i, j]:
                tot = acc_scr[_tile(i), _tile(j)]
                for sg, m in terms.pop((i, j)):
                    tot = tot + m if sg > 0 else tot - m
                acc_scr[_tile(i), _tile(j)] = tot

    fns = dict(e=job_e, f=job_f, d=job_d, p=job_p, v=job_v, o=job_o)
    order = _job_order(q_scr.shape[0] // (2 * SB))
    for n, job in enumerate(order):
        assert job[0] not in 'efd' or not any(j[0] in 'pv' and j[2] == job[2] and j[1] < job[1] for j in order[n:])
    side = list(side)
    fences = [n for n, job in enumerate(order) if job[0] == 'd' and job[3:] == _DCELLS[-1]]
    step = (len(order) - SIDE0 - SIDE1 - 10) / len(side)
    for n, job in enumerate(order):
        done_side[1] = n
        fns[job[0]](*job[1:])
        last_chance = n >= len(order) - SIDE1
        near = any(-SG1 <= f - n <= SG0 for f in fences)
        if side and n >= SIDE0 + step * done_side[0] and ((job[0] in 'pvo' and not near) or last_chance):
            done_side[0] += 1
            v = side.pop(0)(res[-1 - SLAG][8 * (n % 4):8 * (n % 4) + 8, :])
            if v is not None:
                due.append((n + SDUE, v))
    assert not side and not due
    fine = jnp.abs(chk[0]) < jnp.inf
    flag_scr[...] = jnp.maximum(flag_scr[...], jnp.where(fine, chk[1], 1.0))


def _kernel(x_hbm, c_hbm, wq_hbm, wuk_hbm, wuv_hbm, wo_hbm, w1_hbm, w2_hbm, w3_hbm, w4_hbm,
            cond_hbm, wmod_hbm, out_hbm,
            x_ref, c_ref, cond_ref, wma_ref, wmb_ref, w1_ref, w3_ref,
            wq_buf, wk_buf, wv_buf, wo_buf, out_buf, sem, wsem, osem,
            mod_scr, h_scr, cs_scr, hs_scr, w_scr, q_scr, k_scr, v_scr, acc_scr, xn_scr, xh_scr, a1_scr, t_scr,
            z_scr, mw_scr, m3_scr, wt_scr, wf_scr, gap_scr, st_in, pf_scr, vf_scr, flag_scr):
    S, M = x_hbm.shape
    D = wq_hbm.shape[2]
    nattn = wo_hbm.shape[0]
    Fd = w4_hbm.shape[0]
    scale = float(D) ** -0.5 * LOG2E
    nb, nrb = S // T, S // RB
    km, kc = M // T, c_hbm.shape[1] // T
    NX = 4
    XR = S // NX
    CB = XR // T

    work = (wk_buf, wv_buf, wq_buf)

    def pcopies(g, bufs=work, s0=0):
        return [pltpu.make_async_copy(src.bitcast(U32).at[:, g, :], dst, wsem.at[s0 + j])
                for j, (src, dst) in enumerate(zip((wuk_hbm, wuv_hbm, wq_hbm), bufs))]

    def ocopy(g):
        return pltpu.make_async_copy(wo_hbm.at[g], wo_buf, wsem.at[3])

    def chunk_copy(src, dst, i, s0):
        rows = slice(i * XR, (i + 1) * XR)
        return pltpu.make_async_copy(src.at[rows, :], dst.at[rows, :], sem.at[s0 + i])

    MS = 16
    NSL = T // MS
    assert nattn - 1 >= NSL
    mixw = ((w1_hbm, km, 0), (w2_hbm, km, km * MS), (w3_hbm, Fd // T, 2 * km * MS),
            (w4_hbm, -(-Fd // T), (2 * km + Fd // T) * MS))

    def prep_in(g):
        o = jnp.minimum(g, NSL - 1) * MS
        return [pltpu.make_async_copy(
            w.at[pl.ds(pl.multiple_of(jnp.minimum(b * T + o, w.shape[0] - MS), MS), MS), :],
            st_in.at[r0 + b * MS:r0 + (b + 1) * MS, :], wsem.at[7]) for w, nblk, r0 in mixw for b in range(nblk)]

    def stage_in(g):
        return pcopies(jnp.minimum(g + 1, nattn - 1))

    cp_cond = pltpu.make_async_copy(cond_hbm, cond_ref, sem.at[0])
    cp_wma = pltpu.make_async_copy(wmod_hbm.at[:, 0:2 * M], wma_ref, sem.at[1])
    cp_late = [pltpu.make_async_copy(src, dst, sem.at[2 + j]) for j, (src, dst) in enumerate((
        (wmod_hbm.at[:, 2 * M:6 * M], wmb_ref), (w1_hbm, w1_ref), (w3_hbm.at[Fd // T * T:, :], w3_ref)))]
    cp_x = [chunk_copy(x_hbm, x_ref, i, 7) for i in range(NX)]
    cp_c = [chunk_copy(c_hbm, c_ref, i, 7 + NX) for i in range(NX)]

    def silu_cond():
        cf = cond_ref[...].astype(F32)
        return jnp.broadcast_to((cf * jax.nn.sigmoid(cf)).astype(BF16), (8, M))

    cp_wk, cp_wv, cp_wq = pcopies(0)
    named = dict(k=cp_wk, v=cp_wv, q=cp_wq, o=ocopy(0), n=cp_cond, m=cp_wma)
    named.update(zip('abcd', cp_c))
    named.update(zip('wxyz', cp_x))
    started, arrived, did = set(), set(), set()

    def zero(r, carry):
        acc_scr[pl.ds(pl.multiple_of(r * T, T), T), :] = jnp.zeros((T, M), F32)
        return carry

    def x_rows(rows, dep):
        xf = x_ref[rows, :].astype(F32)
        if dep is None:
            return xf
        return jnp.concatenate([_after(xf[:, :T], _rows(dep, xf.shape[0])), xf[:, T:]], axis=1)

    def n_item(r, i):
        def fn(dep):
            rows = slice(r * T + i * LP, r * T + (i + 1) * LP)
            xn_scr[rows, :] = _ln(x_rows(rows, dep))
        return fn

    def h_item(r, i, normed):
        def fn(dep):
            rows = slice(i * LP, (i + 1) * LP)
            grows = slice(r * T + i * LP, r * T + (i + 1) * LP)
            sa = mod_scr[:, 0:M]
            if normed and dep is not None:
                sa = jnp.concatenate([_after(sa[:, _tile(j)], dep) for j in range(km)], axis=1)
            hf = ((xn_scr[grows, :] if normed else _ln(x_rows(grows, dep))) * _rows(mod_scr[:, M:2 * M], LP)
                  + _rows(sa, LP))
            for j in range(km):
                h_scr[r, j, rows, :] = hf[:, _tile(j)].astype(BF16)
            for f, n in _H_SUMS.items():
                if all(t[1] == r for t in f):
                    hs_scr[n, rows, :] = _form(f, lambda _, k: hf[:, _tile(k)]).astype(BF16)
            did.add(('h', r, i))
        return fn

    def release(jobs, span, items):
        if span and items:
            jobs.side += [(len(jobs.res) + 1 + i * span // len(items), fn) for i, fn in enumerate(items)]
            jobs.side.sort(key=lambda e: e[0])
        else:
            for fn in items:
                fn(None)

    def sum_items(n, group, index, dst, get, skip_rows):
        forms = [f for f in dict.fromkeys(t[0] for t in group)
                 if len(f) > 1 and not (skip_rows and len({t[1] for t in f}) == 1)]

        def item(f, rows):
            def fn(dep):
                def term(r, k):
                    v = get(r, k, rows).astype(F32)
                    return v if dep is None or (r, k) != f[0][1:] else _after(v, _rows(dep, v.shape[0]))
                dst[index[f], rows, :] = _form(f, term).astype(BF16)
            return fn

        return [item(f, slice(i, i + n)) for i in range(0, T, n) for f in forms]

    h_sums = lambda n, gi: sum_items(n, _H_GROUPS[gi], _H_SUMS, hs_scr,
                                     lambda r_, k, rows: h_scr[r_, k, rows, :], True)

    def stash(key, buf, j0, transpose=False):
        n = buf.shape[0] // T
        if key not in did:
            assert key in arrived
            did.add(key)
            for (j, hd), w in _pair_tiles(buf, transpose).items():
                w_scr[hd, j0 + j] = w
        return lambda hd: [_ld(w_scr, hd, j0 + j) for j in range(n)]

    def kv_tile(jobs, r):
        wk, wvT = stash('k', wk_buf, 0), stash('v', wv_buf, kc, True)
        ct = [c_ref[_tile(r), _tile(j)] for j in range(kc)]
        for hd in range(2):
            k_scr[2 * r + hd] = jobs.mm(ct, wk(hd), _dot).astype(BF16)
        for hd in range(2):
            v_scr[2 * r + hd] = jobs.mm(wvT(hd), ct, _dot_nt).astype(BF16)

    def q_tile(jobs, r):
        wq = stash('q', wq_buf, 2 * kc)
        ht = [_ld(h_scr, r, j) for j in range(km)]
        for hd in range(2):
            v = (jobs.mm(ht, wq(hd), _dot) * scale).astype(BF16)
            q_scr[2 * r + hd] = v.T if 2 * r + hd in QT else v

    for blk in _prologue().split(';'):
        waits, starts, acts = blk.split('|')
        for ch in waits.strip():
            assert ch in started and ch not in arrived
            arrived.add(ch)
            named[ch].wait()
        for ch in starts.strip():
            assert ch not in started
            started.add(ch)
            named[ch].start()
        jobs = _Jobs()
        for act in acts.split():
            if act == 'Z':
                jax.lax.fori_loop(0, nb, zero, 0)
                acc_scr[S:, :] = jnp.zeros((acc_scr.shape[0] - S, M), F32)
                x_ref[S:, :] = jnp.zeros((x_ref.shape[0] - S, M), BF16)
                flag_scr[...] = jnp.zeros(flag_scr.shape, F32)
            elif act == 'L':
                did.add('L')
                assert ('Q', 0) in did
                for cp in stage_in(0) + prep_in(0):
                    cp.start()
            elif act == 'M':
                assert arrived >= set('nm')
                mod = _dot(silu_cond(), wma_ref[...])
                mod_scr[:, 0:M] = mod[:, 0:M]
                mod_scr[:, M:2 * M] = 1.0 + mod[:, M:2 * M]
                did.add('M')
            else:
                act, _, span = act.partition('@')
                span = int(span or 0)
                items = []
                for r in [int(ch, 16) for ch in act[1:]]:
                    did.add((act[0], r))
                    if act[0] == 'K':
                        assert 'abcd'[r // CB] in arrived
                        kv_tile(jobs, r)
                    elif act[0] == 'H':
                        assert 'wxyz'[r // CB] in arrived and 'M' in did
                        items += [h_item(r, i, ('N', r) in did) for i in range(T // LP)]
                    elif act[0] == 'N':
                        assert 'wxyz'[r // CB] in arrived
                        items += [n_item(r, i) for i in range(T // LP)]
                    elif act[0] == 'Q':
                        assert all(('h', r, i) in did for i in range(T // LP))
                        q_tile(jobs, r)
                    elif act[0] == 'Y':
                        def zero_item(n0):
                            def fn(dep):
                                zero = jnp.where(dep > jnp.inf, jnp.uint32(1), jnp.uint32(0))
                                for n in range(n0, min(n0 + 4, _MIX3 + m3_scr.shape[0])):
                                    mw_scr.bitcast(U32)[n] = _rows(zero, T // 2)
                            return fn
                        items += [zero_item(n0) for n0 in range(_MIX3, _MIX3 + m3_scr.shape[0], 4)]
                    elif act[0] == 'F':
                        assert all(('K', SB * r + k_) in did for k_ in range(SB))
                        items += _v_form_items(v_scr, (pf_scr, vf_scr), r)
                    elif act[0] == 'C':
                        assert all('abcd'[t[1] // CB] in arrived for p_ in _C_GROUPS[r] for t in p_[0])
                        items += sum_items(
                            32, _C_GROUPS[r], _C_SUMS, cs_scr,
                            lambda r_, k, rows: c_ref[r_ * T + rows.start:r_ * T + rows.stop, _tile(k)], False)
                    else:
                        assert act[0] == 'S' and all(('h', t[1], T // LP - 1) in did for p_ in _H_GROUPS[r] for t in p_[0])
                        items += h_sums(32 if span else 16, r)
                release(jobs, span, items)
        assert not jobs.side
    assert arrived == set(named) and all((k_, r) in did for k_ in 'KHQ' for r in range(nb))
    assert all((k_, r) in did for k_ in 'CS' for r in range(2)) and 'L' in did
    assert all(('F', r) in did for r in range(SB))

    def mixer_prep(g):
        sl = jnp.minimum(g, NSL - 1)
        rows = pl.ds(pl.multiple_of(sl * MS, MS), MS)

        def part(m, forms):
            def fn(dep):
                base = {}

                def get(i, k):
                    if (i, k) not in base:
                        rb, cb = (i, k) if m == 2 else (k, i)
                        r0 = mixw[m][2] + rb * MS
                        v = _after(st_in[r0:r0 + MS, _tile(cb)].astype(F32), _rows(dep, MS))
                        if m == 3 and (rb + 1) * T > Fd:
                            v = jnp.where(rb * T + sl * MS < Fd, v, 0.0)
                        base[i, k] = v
                    return base[i, k]

                for f in forms:
                    v = _form(f, get)
                    mw_scr[_MIXW[m, f], rows, :] = (0.5 * v if m % 2 else v).astype(BF16)
            return fn

        items = []
        for m in range(4):
            forms = [f for mm_, f in _MIXW if mm_ == m]
            cur, terms = [], set()
            for f in forms:
                new_terms = terms | {t[1:] for t in f}
                if cur and 3 * len(new_terms) + sum(2 * len(x) + 1 for x in cur + [f]) > MWOPS:
                    items.append(part(m, cur))
                    cur, terms = [], set()
                cur.append(f)
                terms |= {t[1:] for t in f}
            items.append(part(m, cur))

        n3 = sum(m == 2 for m, _ in _MIXW)
        first = min(n for (m, _), n in _MIXW.items() if m == 2)
        per = -(-n3 // (nattn - 1 - NSL))

        def turn(j):
            def fn(dep):
                n = jnp.minimum(jnp.maximum(g - NSL, 0) * per + j, n3 - 1)
                w = _tie(_ld(mw_scr, first + n), dep).T
                m3_scr[n] = w
                return pltpu.bitcast(pltpu.bitcast(w, U32)[T // 2 - 8:], F32)
            return fn

        return items + [turn(j) for j in range(per)]

    def stage_wait():
        for cp in pcopies(0):
            cp.wait()
        pltpu.make_async_copy(st_in, st_in, wsem.at[7]).wait()

    def attn_body(g, carry):
        side = _gap_items(work, gap_scr) + _weight_form_items(work, gap_scr, wt_scr, wf_scr)
        bufs = (q_scr, k_scr, v_scr, (pf_scr, vf_scr), wo_buf, acc_scr, flag_scr)
        _attention_step(*bufs, g >> 16, side)

        @pl.when(g + 1 < nattn)
        def _():
            copies = stage_in(g + 1) + [ocopy(g + 1)]
            for cp in copies:
                cp.start()
            bufs = (h_scr, hs_scr, c_ref, cs_scr, wf_scr, q_scr, k_scr, v_scr, (pf_scr, vf_scr))
            side = [(SD0 + int(i * SDS), fn) for i, fn in enumerate(mixer_prep(g))]
            _proj_step(*bufs, scale, gap_scr, side)
            for cp in prep_in(g + 1):
                cp.start()
            stage_wait()
            ocopy(g + 1).wait()

        return carry

    stage_wait()
    for cp in cp_late:
        cp.start()
    jax.lax.fori_loop(0, nattn, attn_body, 0)

    def safe_pair(g, carry):
        copies = pcopies(g) + [ocopy(g)]
        for cp in copies:
            cp.start()
        for cp in copies:
            cp.wait()
        for buf, j0, transpose in ((wk_buf, 0, False), (wv_buf, kc, True), (wq_buf, 2 * kc, False)):
            for (j, hd), w in _pair_tiles(buf, transpose).items():
                w_scr[hd, j0 + j] = w

        def tile(u, carry):
            r, hd = u // 2, u % 2
            rows = pl.ds(pl.multiple_of(r * T, T), T)
            ct = [c_ref[rows, _tile(j)] for j in range(kc)]
            k_scr[u] = sum(_dot(ct[j], _ld(w_scr, hd, j)) for j in range(kc)).astype(BF16)
            v_scr[u] = sum(_dot_nt(_ld(w_scr, hd, kc + j), ct[j]) for j in range(kc)).astype(BF16)
            q = sum(_dot(_ld(h_scr, r, j), _ld(w_scr, hd, 2 * kc + j)) for j in range(km))
            q_scr[u] = (q * scale).astype(BF16)
            return carry

        jax.lax.fori_loop(0, 2 * nb, tile, 0)
        _attention_safe(q_scr, k_scr, v_scr, wo_buf, acc_scr)
        return carry

    @pl.when(jnp.max(flag_scr[...]) > 0)
    def _():
        jax.lax.fori_loop(0, nb, zero, 0)
        jax.lax.fori_loop(0, nattn, safe_pair, 0)

    for cp in cp_late:
        cp.wait()
    mod = _dot(silu_cond(), wmb_ref[...])
    mod_scr[:, 2 * M:4 * M] = mod[:, 0:2 * M]
    mod_scr[:, 4 * M:5 * M] = 1.0 + mod[:, 2 * M:3 * M]
    mod_scr[:, 5 * M:6 * M] = mod[:, 3 * M:4 * M]
    OFF = x_ref.shape[0] - S
    CAR = t_scr.shape[0] - RB

    def p1(r0, l0, n, dep=None):
        ga = mod_scr[:, 2 * M:3 * M]
        if dep is not None:
            ga = jnp.concatenate([_after(ga[:, 0:T], dep), ga[:, T:]], axis=1)
        rows = pl.ds(r0, n)
        x1 = x_ref[rows, :].astype(F32) + _rows(ga, n) * acc_scr[rows, :]
        xh_scr[0, l0:l0 + n, :] = x1
        hb = _ln(x1) * _rows(mod_scr[:, 4 * M:5 * M], n) + _rows(mod_scr[:, 3 * M:4 * M], n)
        xh_scr[1, l0:l0 + n, :] = hb
        return hb

    HT = T // 2
    last8 = lambda v: jnp.max(v[:, M - T:].reshape(PC // 8, 8, T), axis=0)

    def p1_store(r0, c, dep=None):
        v = _ln(p1(r0 + c * PC, OFF + c * PC, PC, dep))
        a1_scr[c * PC:(c + 1) * PC, :] = v
        return last8(v)

    def p1_first(r0, c, dep):
        return last8(p1(r0 + c * PC, OFF + c * PC, PC, dep))

    def p1_second(c, dep):
        hb = xh_scr[1, OFF + c * PC:OFF + (c + 1) * PC, :]
        v = _ln(jnp.concatenate([_after(hb[:, :T], _rows(dep, PC)), hb[:, T:]], axis=1))
        a1_scr[c * PC:(c + 1) * PC, :] = v
        return last8(v)

    t_scr[RB:RB + CAR - OFF, :] = jnp.zeros((CAR - OFF, M), F32)
    t_scr[RB + CAR - OFF:RB + CAR, :] = _gelu2(_dot(_ln(p1(0, 0, OFF)).astype(BF16), w1_ref[...]))
    for c in range(RB // PC):
        p1_store(OFF, c)

    def out_copy(i):
        rows = pl.ds(i * T if isinstance(i, int) else pl.multiple_of(i * T, T), T)
        return pltpu.make_async_copy(out_buf.at[rows, :], out_hbm.at[rows, :], osem.at[i])

    def b_body(r, carry):
        gb = _rows(mod_scr[:, 5 * M:6 * M], T)
        r0 = pl.multiple_of(r * RB, RB)
        n0 = pl.multiple_of(jnp.minimum(r0 + RB, S - RB) + OFF, OFF)
        nh = RB // T
        now = [0]
        due = []
        pace = []

        def p1_item(c, part):
            def fn(dep):
                v = p1_first(n0, c, dep) if part == 0 else p1_second(c, dep)
                due.append((now[0] + PD, v))
                due.sort(key=lambda e: e[0])
            return fn

        pace += [(P0 + i * PSTEP + part * PSPLIT, p1_item(i, part)) for i in range(RB // PC)
                 for part in range(2)]
        pace.sort(key=lambda e: e[0])

        def mm(lhs, wts, dot=_dot):
            acc = None
            for x, w in zip(lhs, wts):
                if due and due[0][0] <= now[0]:
                    w = _tie(w, due.pop(0)[1])
                v = dot(x, w)
                now[0] += x.shape[0] // HT
                acc = v if acc is None else v + acc
                if pace and pace[0][0] <= now[0]:
                    pace.pop(0)[1](v[0:8, :])
            return acc

        def fast(m, base, finish, hook=None):
            prods = _MIX[m]
            left, acc, done, cache = {}, {}, {}, {}
            for _, _, outs in prods:
                for _, i, h in outs:
                    left[i, h] = left.get((i, h), 0) + 1

            def act(form):
                sign, form = _canon(form)
                if form not in cache:
                    cache[form] = _form(form, lambda k, h: base(k)[h * HT:(h + 1) * HT]).astype(BF16)
                return sign, cache[form]

            for pi, (wf, af, outs) in enumerate(prods):
                w = _ld(m3_scr, _MIXW[m, wf] - _MIX3) if m == 2 else _ld(mw_scr, _MIXW[m, wf])
                if af is None:
                    k = wf[0][2]
                    v = mm([jnp.concatenate([act(((1, k, h),))[1] for h in range(2)], axis=0)], [w])
                    sign, parts = 1, [v[:HT], v[HT:]]
                else:
                    sign, x = act(af)
                    parts = [mm([x], [w])] * len(outs)
                for (s_, i, h), v in zip(outs, parts):
                    s_ = s_ * sign
                    if (i, h) not in acc:
                        acc[i, h] = (s_, v)
                    else:
                        s0, u = acc[i, h]
                        acc[i, h] = (s0, u + v if s0 == s_ else u - v) if s0 > 0 or s_ < 0 else (1, v - u)
                    left[i, h] -= 1
                    if not left[i, h]:
                        s0, done[i, h] = acc.pop((i, h))
                        assert s0 > 0
                        if (i, 1 - h) in done:
                            finish(i, jnp.concatenate([done[i, 0], done[i, 1]], axis=0))
                if hook is not None:
                    hook(pi, act)

        t_scr[0:CAR, :] = t_scr[RB:RB + CAR, :]
        for hf in range(nh):
            def put_t(n, v):
                t = _gelu2(v)
                if hf == nh - 1:
                    t = jnp.concatenate([t[:T - OFF], jnp.where(r < nrb - 1, t[T - OFF:], 0.0)], axis=0)
                t_scr[CAR + hf * T:CAR + (hf + 1) * T, _tile(n)] = t

            fast(0, lambda k: a1_scr[_tile(hf), _tile(k)], put_t)
        cq = M // 4
        shifts = (-1, 1, -2, 2)
        lane = jax.lax.broadcasted_iota(jnp.int32, (T, T), 1)
        y1, a3 = [], []
        for hf in range(nh):
            base = CAR - OFF + hf * T
            sh = []
            for j in range(km):
                g_lo, g_hi = (j * T) // cq, ((j + 1) * T - 1) // cq
                assert g_hi - g_lo <= 1

                def shifted(d):
                    v = t_scr[base - 8:base + T + 8, _tile(j)]
                    return pltpu.roll(v, (-d) % (T + 16), 0)[8:8 + T]

                v = shifted(shifts[g_lo])
                if g_hi != g_lo:
                    v = jnp.where(lane < g_hi * cq - j * T, v, shifted(shifts[g_hi]))
                sh.append(v)
            hs = {}
            fast(1, lambda k: sh[k], hs.__setitem__)
            hs = jnp.concatenate([hs[n] for n in range(km)], axis=1)
            y1.append(hs + xh_scr[1, _tile(hf), :])
            z_scr[_tile(hf), :] = xh_scr[0, _tile(hf), :] + gb * y1[hf]
            a3.append({})

            def ln_item(hf, c):
                def item(dep):
                    n = HT // NLN
                    for d in (0, HT):
                        v = y1[hf][d + c * n:d + (c + 1) * n]
                        if dep is not None:
                            v = jnp.concatenate([_after(v[:, :T], _rows(dep, n)), v[:, T:]], axis=1)
                        a3[hf][d + c * n] = _ln(v)
                return item

            ln_item(hf, 0)(None)
            pace += [(now[0] + LN0 + (c - 1) * LNS * (1 + hf), ln_item(hf, c)) for c in range(1, NLN)]
            pace.sort(key=lambda e: e[0])
        xh_scr[:, 0:OFF, :] = xh_scr[:, RB:RB + OFF, :]
        z_scr[pl.ds(pl.multiple_of(RB + (r >> 16) * 8, 8), 8), :] = jnp.zeros((8, M), F32)
        h3 = []
        for hf in range(nh):
            assert len(a3[hf]) == 2 * NLN
            af = jnp.concatenate([a3[hf][key] for key in sorted(a3[hf])], axis=0)
            row = {}
            narrow = []

            def hook(pi, act):
                j, rem = divmod(pi - NAR0, NARS)
                if rem == 0 and 0 <= j < km:
                    full = jnp.concatenate([act(((1, j, h),))[1] for h in range(2)], axis=0)
                    v = mm([w3_ref[:, _tile(j)]], [full], _dot_nt)
                    narrow[:] = [v + narrow[0] if narrow else v]

            def put_h(n, v):
                row[n] = _gelu2(v)
                if GD:
                    due.append((now[0] + GD, jnp.max(row[n].reshape(T // 8, 8, T), axis=0)))
                    due.sort(key=lambda e: e[0])

            fast(2, lambda k: af[:, _tile(k)], put_h, hook)
            fw = w3_ref.shape[0]
            row[Fd // T] = jnp.concatenate([_gelu2(narrow[0]), jnp.zeros((T - fw, T), F32)], axis=0).T
            h3.append(row)
        for hf in range(nh):
            rows = pl.ds(pl.multiple_of(r0 + hf * T, T), T)

            def finish(n, v):
                out_buf[rows, _tile(n)] = (z_scr[_tile(hf), _tile(n)] + gb[:, _tile(n)] * v).astype(out_buf.dtype)
                pltpu.make_async_copy(out_buf.at[rows, _tile(n)], out_hbm.at[rows, _tile(n)],
                                      osem.at[r * nh + hf]).start()

            fast(3, lambda k: h3[hf][k], finish)
        assert not pace
        return carry

    jax.lax.fori_loop(0, nrb, b_body, 0)
    for i in range(nb):
        out_copy(i).wait()


@jax.jit
def pallas_adaLN_cond__compressed_kv_cla__mixer_s_mlp__prompt_kernel(
    A_x: jax.Array,
    A_c_kv: jax.Array,
    A_w_q: jax.Array,
    A_w_uk: jax.Array,
    A_w_uv: jax.Array,
    A_w_o: jax.Array,
    B_x: jax.Array,
    B_w1: jax.Array,
    B_w2: jax.Array,
    B_w3: jax.Array,
    B_w4: jax.Array,
    c: jax.Array,
    w_mod: jax.Array,
):
    _, S, M = A_x.shape
    Dc = A_c_kv.shape[2]
    H, D = A_w_q.shape[1], A_w_q.shape[2]
    Fd = B_w3.shape[1]
    assert D == T and A_c_kv.shape[1] == S and Dc == 4 * T and M == 5 * T and 13 * T < Fd < 14 * T and S == 16 * T
    vmem = pltpu.VMEM
    packed = lambda *lead: vmem(lead + (T, T), BF16)
    out = pl.pallas_call(
        _kernel,
        in_specs=[pl.BlockSpec(memory_space=pltpu.HBM)] * 12,
        out_specs=pl.BlockSpec(memory_space=pltpu.HBM),
        out_shape=jax.ShapeDtypeStruct((S, M), A_x.dtype),
        scratch_shapes=[
            vmem((S + 16, M), BF16),
            vmem((S, Dc), BF16),
            vmem((1, M), BF16),
            vmem((M, 2 * M), BF16),
            vmem((M, 4 * M), BF16),
            vmem((M, M), BF16),
            vmem((Fd % T, M), BF16),
            vmem((M, D), U32),
            vmem((Dc, D), U32),
            vmem((Dc, D), U32),
            vmem((2 * D, M), BF16),
            vmem((S, M), A_x.dtype),
            pltpu.SemaphoreType.DMA((15,)),
            pltpu.SemaphoreType.DMA((8,)),
            pltpu.SemaphoreType.DMA((S // T,)),
            vmem((8, 6 * M), F32),
            vmem((S // T, M // T, T, T), BF16),
            vmem((len(_C_SUMS), T, T), BF16),
            vmem((len(_H_SUMS), T, T), BF16),
            packed(2, M // T + 2 * (Dc // T)),
            packed(2 * S // T),
            packed(2 * S // T),
            packed(2 * S // T),
            vmem((S + 16, M), F32),
            vmem((S, M), F32),
            vmem((2, RB + 16, M), F32),
            vmem((RB, M), F32),
            vmem((RB + 32, M), F32),
            vmem((RB + 8, M), F32),
            packed(len(_MIXW)),
            packed(sum(m == 2 for m, _ in _MIXW)),
            vmem((Dc // T, T, T), U32),
            vmem((len(_WF), T, T), BF16),
            vmem((3, 8, T), jnp.int32),
            vmem(((2 * (M // T) + Fd // T + -(-Fd // T)) * 16, M), BF16),
            vmem((_FENCE + 1, T, T), BF16),
            vmem((_FENCE + 1, T, T), BF16),
            vmem((8, T), F32),
        ],
        compiler_params=pltpu.CompilerParams(
            vmem_limit_bytes=100 * 1024 * 1024,
            disable_bounds_checks=True,
        ),
    )(
        A_x.reshape(S, M), A_c_kv.reshape(S, Dc),
        A_w_q, A_w_uk, A_w_uv,
        A_w_o.reshape(H // 2, 2 * D, M),
        B_w1, B_w2, B_w3.T, B_w4, c, w_mod,
    )
    return out.reshape(1, S, M)
```

```python
import functools
import math

import jax
import jax.numpy as jnp
import jax.experimental.pallas as pl
import jax.experimental.pallas.tpu as pltpu

F32 = jnp.float32
BF16 = jnp.bfloat16
U32 = jnp.uint32
NT = (((1,), (1,)), ((), ()))
T = 128
EPS = 1e-5
LOG2E = math.log2(math.e)

L_LO, L_HI, L_RATIO = 2.0 ** -24, 2.0 ** 24, 4.0

LAT_0, LAT_A = 24, 17
LAT_B = 20
RES, OEND = 32, 24
ONV = 0.7
TV, TO = 6, 2
QT = (4, 6)
SIDE0, SIDE1 = 8, 60
SLAG, SDUE = 3, 8
SG0, SG1 = 4, 0
WFK, WFQ = 4, 6
SD0, SDS = 4, 1.7
VF0, VFS = 4, 1.6
PDUE = 19
MWOPS = 74
RB = 256
PC = 32
P0, PSTEP, PSPLIT, PD = 305, 33, 44, 42
NLN, LN0, LNS = 4, 2, 3
GD = 36
NAR0, NARS = 16, 10
LP = 16
HNOW, SH1, SF2, SH2, SF3, SH3, SP0, SP1 = 3, 39, 40, 32, 30, 36, 76, 38
_prologue = lambda: (
    '|kva|Z; |b|; kva|wc|Y0@56 K0123; bw|xdn|C0@56 N0123@52 K4567; cx|mq|N4567@52 F0@56 K89ab; '
    f'd|y|C1@56 F1@56 Kcdef; nmq|zo|M H{"01234567"[:HNOW]} H{"01234567"[HNOW:]}@{SH1} F2@{SF2} Q0123; '
    f'y||L H89ab@{SH2} F3@{SF3} Q4567; zo||Hcdef@{SH3} S0@{SP0} Q89ab S1@{SP1} Qcdef')


def _dot(a, b):
    return jnp.dot(a, b, preferred_element_type=F32)


def _dot_nt(a, b):
    return jax.lax.dot_general(a, b, NT, preferred_element_type=F32)


def _ln(x):
    m = jnp.mean(x, axis=-1, keepdims=True)
    xc = x - m
    v = jnp.mean(xc * xc, axis=-1, keepdims=True)
    return xc * jnp.exp2(jnp.log(v + EPS) * (-0.5 * LOG2E))


def _rows(v, n):
    return jnp.broadcast_to(v[None], (n // 8, 8, v.shape[1])).reshape(n, v.shape[1])


def _gelu2(x):
    c0 = math.sqrt(2.0 / math.pi)
    return x + x * jnp.tanh(x * (c0 + (c0 * 0.044715) * (x * x)))


def _after(x, dep):
    return jnp.where(dep > jnp.inf, dep, x)


def _tie(x, dep):
    xu = pltpu.bitcast(x, U32)
    first = jnp.where(dep > jnp.inf, jnp.uint32(0), xu[:8])
    return pltpu.bitcast(jnp.concatenate([first, xu[8:]], axis=0), BF16)


def _tile(j):
    return slice(j * T, (j + 1) * T)


def _ld(ref, *idx):
    return pltpu.bitcast(ref.bitcast(U32)[idx], BF16)


def _group(rows, cols, pairs):
    xs, ys = dict.fromkeys(x for x, _ in pairs), dict.fromkeys(y for _, y in pairs)
    used = set(xs) | set(ys) | {(x[0], y[1]) for x, y in pairs} | {(y[0], x[1]) for x, y in pairs}
    prods = []
    for n, r in enumerate(rows):
        for i, k in [x for x in xs if x[0] == r]:
            mates = [y for x, y in pairs if x == (i, k)]
            prods.append((((1, i, k),) + tuple((1, i, k2) for _, k2 in mates), ((1, k, 0),),
                          ((1, i, 0), (-1, i, 1))))
            prods.append((((1, i, k),) + tuple((-1, i2, k) for i2, _ in mates), ((1, k, 0), (1, k, 1)),
                          ((1, i, 1),)))
        for i2, k2 in [y for y in ys if y[0] == r]:
            mates = [x for x, y in pairs if y == (i2, k2)]
            prods.append((((1, i2, k2),) + tuple((1, i2, k) for _, k in mates), ((1, k2, 1),),
                          ((1, i2, 1), (-1, i2, 0))))
            prods.append((((1, i2, k2),) + tuple((-1, i, k2) for i, _ in mates), ((1, k2, 0), (1, k2, 1)),
                          ((1, i2, 0),)))
        prods += [(((1, r, k),), ((1, k, h),), ((1, r, h),)) for k in cols if (r, k) not in used for h in (0, 1)]
        for (i, k), (i2, k2) in pairs:
            if r in (i, i2) and i + i2 - r in rows[n + 1:]:
                prods.append((((1, i, k2),), ((1, k2, 0), (-1, k, 0)), ((1, i2, 0), (1, i, 0))))
                prods.append((((1, i2, k), (1, i, k2)), ((1, k, 0), (1, k2, 1)), ((1, i2, 0), (1, i, 1))))
                prods.append((((1, i2, k),), ((1, k, 1), (-1, k2, 1)), ((1, i2, 1), (1, i, 1))))
    return prods


def _all_pairs(xrows, yrows):
    return [((x, a), (y, b)) for a, x in enumerate(xrows) for b, y in enumerate(yrows) if a != b]


_PAIRS65 = [((x[0] + 10, x[1]), (y[0] + 10, y[1])) for x, y in (
    ((0, 1), (1, 0)), ((0, 1), (5, 2)), ((2, 3), (1, 0)), ((2, 3), (3, 1)), ((2, 3), (5, 2)), ((3, 2), (1, 0)),
    ((4, 4), (0, 3)), ((4, 4), (1, 0)), ((4, 4), (3, 1)), ((4, 4), (5, 2)))]
_C_GROUPS = [_group(range(r, r + 8), range(4), _all_pairs(range(r, r + 4), range(r + 4, r + 8))) for r in (0, 8)]
_H_GROUPS = [_group(range(10), range(5), _all_pairs(range(5), range(5, 10))),
             _group(range(10, 16), range(5), _PAIRS65)]
_sum_index = lambda groups: {f: n for n, f in enumerate(
    dict.fromkeys(t[0] for g in groups for t in g if len(t[0]) > 1))}
_C_SUMS, _H_SUMS = _sum_index(_C_GROUPS), _sum_index(_H_GROUPS)


def _cells(rows, cols, pairs):
    xs = list(dict.fromkeys(p[0] for p in pairs))
    ys = list(dict.fromkeys(p[1] for p in pairs))
    used = set(xs + ys) | {(x[0], y[1]) for x, y in pairs} | {(y[0], x[1]) for x, y in pairs}

    def home_x(i, k):
        mates = [y for x, y in pairs if x == (i, k)]
        return [(((1, i, k),) + tuple((1, i, k2) for _, k2 in mates), ((1, k, 0),), ((1, i, 0), (-1, i, 1))),
                (((1, i, k),) + tuple((-1, i2, k) for i2, _ in mates), ((1, k, 0), (1, k, 1)), ((1, i, 1),))]

    def home_y(i2, k2):
        mates = [x for x, y in pairs if y == (i2, k2)]
        return [(((1, i2, k2),) + tuple((1, i2, k) for _, k in mates), ((1, k2, 1),), ((1, i2, 1), (-1, i2, 0))),
                (((1, i2, k2),) + tuple((-1, i, k2) for i, _ in mates), ((1, k2, 0), (1, k2, 1)), ((1, i2, 0),))]

    def cross(x, y):
        (i, k), (i2, k2) = x, y
        return [(((1, i, k2),), ((1, k2, 0), (-1, k, 0)), ((1, i2, 0), (1, i, 0))),
                (((1, i2, k), (1, i, k2)), ((1, k, 0), (1, k2, 1)), ((1, i2, 0), (1, i, 1))),
                (((1, i2, k),), ((1, k, 1), (-1, k2, 1)), ((1, i2, 1), (1, i, 1)))]

    direct = lambda i: [(((1, i, k),), None, ((1, i, 0), (1, i, 1))) for k in cols if (i, k) not in used]
    single = lambda i: ([t for x in xs if x[0] == i for t in home_x(*x)]
                        + [t for y in ys if y[0] == i for t in home_y(*y)] + direct(i))
    prods = []
    for n, i in enumerate(rows):
        prods += single(i)
        for i2 in rows[n + 1:]:
            for x, y in pairs:
                if {x[0], y[0]} == {i, i2}:
                    prods += cross(x, y)
    return prods


_square = lambda q: [((a, a), (q + b, b)) for a in range(q) for b in range(q) if a != b]
_shift = lambda pairs, r0: [((x[0] + r0, x[1]), (y[0] + r0, y[1])) for x, y in pairs]
_flip = lambda pairs: [(x[::-1], y[::-1]) for x, y in pairs]
_P35 = [((1, 2), (0, 4)), ((1, 2), (2, 1)), ((2, 3), (0, 4)), ((2, 3), (1, 0))]
_P45 = [((0, 2), (1, 1)), ((2, 4), (0, 3)), ((2, 4), (1, 1)), ((2, 4), (3, 2)), ((3, 0), (0, 3)), ((3, 0), (1, 1))]
_P55 = [((2, 1), (0, 4)), ((2, 1), (1, 0)), ((2, 1), (3, 2)), ((2, 1), (4, 3)), ((3, 3), (0, 4)), ((3, 3), (1, 0)),
        ((4, 2), (0, 4)), ((4, 2), (1, 0))]
_MIX = [_cells(range(5), range(5), _P55), _cells(range(5), range(5), _P55),
        _cells(range(13), range(5), _square(5) + _shift(_P35, 10)),
        _cells(range(5), range(14), _flip(_square(5) + _shift(_P45, 10)))]
_MIXW = {(m, f): n for n, (m, f) in enumerate(dict.fromkeys((m, t[0]) for m in range(4) for t in _MIX[m]))}
_MIX3 = min(n for (m, _), n in _MIXW.items() if m == 2)


def _form(form, get):
    acc = None
    for sign, i, j in form:
        v = get(i, j)
        acc = v if acc is None else (acc + v if sign > 0 else acc - v)
    return acc


def _gap_items(bufs, gap_scr):
    items = []
    for n, buf in enumerate(bufs):
        acc = []

        def part(r0, buf=buf, acc=acc):
            def fn(dep):
                wu = jnp.concatenate([buf[r:r + 8, :] for r in range(r0, r0 + T, 32)])
                mask = jnp.full((8, T), 0x7FFF0000, U32)
                if dep is not None:
                    mask = jnp.where(dep > jnp.inf, jnp.uint32(0), mask)
                mask = _rows(mask, 32)
                new = [jnp.sum(pltpu.bitcast(v & mask, F32).reshape(4, 8, T), axis=0) for v in (wu << 16, wu)]
                acc[:] = [u + v for u, v in zip(acc, new)] if acc else new
            return fn

        def last(_, n=n, acc=acc):
            bits = []
            for v in acc:
                l1 = jnp.sum(jnp.sum(v, axis=1, keepdims=True), axis=0, keepdims=True)
                bits.append(pltpu.bitcast(jnp.broadcast_to(l1, (8, T)), jnp.int32) >> 8)
            gap = jnp.clip((bits[0] - bits[1] + (1 << 14)) >> 15, -8, 8) << 23
            gap_scr[n] = gap
            return pltpu.bitcast(gap, F32)

        items += [part(r0) for r0 in range(0, buf.shape[0], T)] + [last]
    return items


def _pair_tiles(w_ref, transpose=False):
    tiles = {}
    for j in range(w_ref.shape[0] // T):
        wu = w_ref[_tile(j), :]
        if transpose:
            wu = wu.T
        tiles[j, 0] = pltpu.bitcast(wu << 16, F32).astype(BF16)
        tiles[j, 1] = pltpu.bitcast(wu & jnp.uint32(0xFFFF0000), F32).astype(BF16)
    return tiles


def _canon(form):
    if form[-1][0] < 0 and form[0][1:] > form[1][1:]:
        return -1, ((1,) + form[1][1:], (-1,) + form[0][1:])
    return 1, form


_w_forms = lambda groups: list(dict.fromkeys(_canon(t[1])[1] for g in groups for t in g))
_WF = {key: n for n, key in enumerate([(m, f) for m, groups in enumerate((_C_GROUPS, _C_GROUPS, _H_GROUPS))
                                       for f in _w_forms(groups)])}


def _weight_form_items(bufs, gap_scr, wt_scr, wf_scr):
    n = 16
    items = []

    def flip(j):
        def fn(dep):
            wu = bufs[1][_tile(j), :]
            wu = (wu if dep is None else jnp.where(_rows(dep, T) > jnp.inf, jnp.uint32(0), wu)).T
            wt_scr[j] = wu
            return pltpu.bitcast(wu[T - 8:], F32)
        return fn

    def part(m, r0, forms):
        def fn(dep):
            fac = pltpu.bitcast(0x3F800000 + gap_scr[m], F32)
            mask = jnp.full((8, T), 0xFFFF0000, U32)
            sh = jnp.full((8, T), 16, U32)
            if dep is not None:
                mask = jnp.where(dep > jnp.inf, jnp.uint32(0), mask)
                sh = jnp.where(dep > jnp.inf, jnp.uint32(0), sh)
            fac, mask, sh = _rows(fac, n), _rows(mask, n), _rows(sh, n)
            base = {}

            def get(k, h):
                if (k, h) not in base:
                    wu = wt_scr[k, r0:r0 + n, :] if m == 1 else bufs[m][k * T + r0:k * T + r0 + n, :]
                    base[k, h] = pltpu.bitcast(wu & mask, F32) * fac if h else pltpu.bitcast(wu << sh, F32)
                return base[k, h]

            for f in forms:
                wf_scr[_WF[m, f], r0:r0 + n, :] = _form(f, get).astype(BF16)
        return fn

    for m in range(3):
        forms = [f for mm, f in _WF if mm == m]
        if m == 1:
            items += [flip(j) for j in range(bufs[1].shape[0] // T)]
        per = -(-len(forms) // (WFQ if m == 2 else WFK))
        forms.sort(key=lambda f: sorted({t[1] for t in f}))
        items += [part(m, r0, forms[i:i + per]) for r0 in range(0, T, n) for i in range(0, len(forms), per)]
    return items


def _run_group(jobs, prods, a_get, w, transposed, finish):
    left = {}
    for _, _, outs in prods:
        for _, i, h in outs:
            left[i, h] = left.get((i, h), 0) + 1
    acc = {}
    for af, bf, outs in prods:
        sign, wt = w(bf)
        m = jobs.mm([wt], [a_get(af)], _dot_nt) if transposed else jobs.mm([a_get(af)], [wt], _dot)
        for s_, i, h in outs:
            if (i, h) not in acc:
                acc[i, h] = (s_ * sign, m)
            else:
                s0, v = acc[i, h]
                acc[i, h] = (s0, v + m if s0 == s_ * sign else v - m) if s0 > 0 or s_ * sign < 0 else (1, m - v)
            left[i, h] -= 1
            if not left[i, h]:
                s0, v = acc.pop((i, h))
                assert s0 > 0
                finish(2 * i + h, v)


class _Jobs:
    def __init__(self, side=()):
        self.res = []
        self.side = list(side)
        self.due = []

    def mm(self, lhs, wt, dot):
        acc = None
        for x, w in zip(lhs, wt):
            if self.due and self.due[0][0] <= len(self.res):
                x = _tie(x, self.due.pop(0)[1])
            v = dot(x, w)
            self.res.append(v)
            acc = v if acc is None else v + acc
            rel = 4 * (len(self.res) % 4)
            while self.side and self.side[0][0] <= len(self.res):
                out = self.side.pop(0)[1](v[8 * rel:8 * rel + 8, :])
                if out is not None:
                    self.due.append((len(self.res) + PDUE, out))
                rel = (rel + 2) % 16
        return acc


def _proj_step(h_scr, hs_scr, c_ref, cs_scr, wf_scr, q_scr, k_scr, v_scr, pf, scale, shifts, side):
    def weight(m):
        def get(form):
            sign, form = _canon(form)
            return sign, _ld(wf_scr, _WF[m, form])
        get.inv = pltpu.bitcast(0x3F800000 - shifts[m], F32)
        return get

    wk, wvT, wq = weight(0), weight(1), weight(2)
    c_get = lambda f: _ld(cs_scr, _C_SUMS[f]) if len(f) > 1 else c_ref[_tile(f[0][1]), _tile(f[0][2])]
    h_get = lambda f: _ld(hs_scr, _H_SUMS[f]) if len(f) > 1 else _ld(h_scr, f[0][1], f[0][2])

    def put(dst, w, mul=None):
        muls = [mul, _rows(w.inv if mul is None else w.inv * mul, T)]

        def fn(u, v):
            v = (v if muls[u % 2] is None else v * muls[u % 2]).astype(BF16)
            dst[u] = v.T if mul is not None and u in QT else v
        return fn

    jobs = _Jobs(side)
    put_v, stored = put(v_scr, wvT), set()
    nxt = [0]

    def fin_v(u, v):
        put_v(u, v)
        stored.add(u)
        for J in range(SB):
            if all(2 * (SB * J + k) + h in stored for k in range(SB) for h in range(2)) and ('J', J) not in stored:
                stored.add(('J', J))
                for fn in _v_form_items(v_scr, pf, J):
                    nxt[0] = max(nxt[0] + VFS, len(jobs.res) + VF0)
                    jobs.side.append((int(nxt[0]), fn))
                jobs.side.sort(key=lambda e: e[0])

    kk, vv, qq = ((c_get, wk, False, put(k_scr, wk)), (c_get, wvT, True, fin_v),
                  (h_get, wq, False, put(q_scr, wq, scale)))
    for prods, args in ((_C_GROUPS[0], kk), (_C_GROUPS[0], vv), (_C_GROUPS[1], vv), (_C_GROUPS[1], kk),
                        (_H_GROUPS[0], qq), (_H_GROUPS[1], qq)):
        _run_group(jobs, prods, *args)
    assert not jobs.side and not jobs.due


def _inner_group(rows, cols, pairs):
    xs, ys = dict.fromkeys(x for x, _ in pairs), dict.fromkeys(y for _, y in pairs)
    used = set(xs) | set(ys) | {(x[0], y[1]) for x, y in pairs} | {(y[0], x[1]) for x, y in pairs}
    prods = []
    for i, j in xs:
        mates = [y for x, y in pairs if x == (i, j)]
        prods.append((((1, i, 0),), ((1, 0, j), (-1, 1, j)), ((1, i, j),) + tuple((1, i2, j) for i2, _ in mates)))
        prods.append((((1, i, 0), (1, i, 1)), ((1, 1, j),), ((1, i, j),) + tuple((-1, i, j2) for _, j2 in mates)))
    for i2, j2 in ys:
        mates = [x for x, y in pairs if y == (i2, j2)]
        prods.append((((1, i2, 0), (1, i2, 1)), ((1, 0, j2),),
                      ((1, i2, j2),) + tuple((-1, i2, j) for _, j in mates)))
        prods.append((((1, i2, 1),), ((1, 0, j2), (-1, 1, j2)),
                      ((-1, i2, j2),) + tuple((-1, i, j2) for i, _ in mates)))
    prods += [(((1, i, h),), ((1, h, j),), ((1, i, j),))
              for i in rows for j in cols if (i, j) not in used for h in (0, 1)]
    for (i, j), (i2, j2) in pairs:
        lo, hi = min(j, j2), max(j, j2)
        prods.append((((1, i2, 0), (-1, i, 0)), ((1, 0, lo), (1, 0, hi)), ((1, i2, j),)))
        prods.append((((1, i, 0), (1, i2, 1)), ((1, 0, j2), (1, 1, j)), ((1, i, j2), (1, i2, j))))
        prods.append((((1, i, 1), (-1, i2, 1)), ((1, 1, lo), (1, 1, hi)), ((1, i, j2),)))
    return prods


def _o_jobs():
    prods = (_inner_group(range(10), range(5), _all_pairs(range(0, 10, 2), range(1, 10, 2)))
             + _inner_group(range(10, 16), range(5), _PAIRS65))
    row = lambda t: max(i for _, i, _ in t[0])
    unit = lambda t: max(2 * i + h for _, i, h in t[0])
    need = lambda t: unit(t) if row(t) == 15 else 2 * row(t) + 1
    return [(need(t), t) for t in sorted(prods, key=need)]


_O_JOBS = _o_jobs()


SB = 4


class _Star:
    def __init__(self, ts):
        self.ts, self.n = ts, len(ts)
        rn = range(self.n)
        self.pairs = [(i, j) for i in rn for j in rn if i < j]
        self.pf = {f: m for m, f in enumerate([('R', i) for i in rn] + [('C', i) for i in rn]
                                              + [('S', i, j) for i in rn for j in rn if i != j]
                                              + [('A', i, j) for i, j in self.pairs])}
        self.vf = {f: m for m, f in enumerate([('W', i) for i in rn]
                                              + [(q, i, j) for i, j in self.pairs for q in ('Q1', 'Q2', 'Q3')])}
        self.pv = {**{('W', i): ('R', i) for i in rn}, **{('B', i): ('C', i) for i in rn},
                   **{('Q1', i, j): ('S', i, j) for i, j in self.pairs},
                   **{('Q2', i, j): ('A', i, j) for i, j in self.pairs},
                   **{('Q3', i, j): ('S', j, i) for i, j in self.pairs}}

    def products(self, i):
        return [('W', i), ('B', i)] + [(q, i, j) for j in range(i + 1, self.n) for q in ('Q1', 'Q2', 'Q3')]


_FULL = _Star((-1.125, -0.375, 0.375, 1.125))
_HALF = _Star((-0.75, 0.75))
_DCELLS = [(0, 0), (1, 0), (1, 1), (2, 2), (3, 2), (3, 3)]
_HSLOT = (SB - 1) * len(_FULL.pf)
_DSLOT = _HSLOT + len(_HALF.pf)
_VSLOT = _DSLOT + len(_DCELLS)
_VHALF = (SB - 1) * len(_FULL.vf)
_FENCE = _VSLOT + (_VHALF + SB * len(_HALF.vf) + 1) // 2


def _v_slot(star, J, f):
    m = star.vf[f] + J * len(star.vf) + (0 if star is _FULL else _VHALF)
    return _VSLOT + m // 2, m % 2 * (T // 2)


def _v_form_items(v_scr, pf, J):
    n, HT = 16, T // 2

    def item(star, h, r0, pairs):
        def fn(dep):
            ts = [jnp.full((8, T), t, F32) for t in star.ts]
            ts = [_rows(t if dep is None else _after(t, dep), n) for t in ts]

            def get(k, a):
                r = (a * HT + r0) // 2
                return _ld(v_scr, 2 * (SB * J + k) + h, slice(r, r + n // 2)).astype(F32)

            def put(f, v):
                slot, r = _v_slot(star, J, f)
                pf[h][slot, r + r0:r + r0 + n, :] = v.astype(BF16)

            b = {(k, a): get(k, a) for k in sorted({k for pr in pairs or star.pairs for k in pr})
                 for a in range(2)}
            if pairs is None or star.n == 2:
                w = [b[k, 0] + ts[k] * b[k, 1] for k in range(star.n)]
                for k in range(star.n):
                    put(('W', k), w[k])
                for i, j in star.pairs:
                    put(('Q2', i, j), w[i] - w[j])
            for i, j in pairs or ():
                d0, d1 = b[j, 0] - b[i, 0], b[j, 1] - b[i, 1]
                put(('Q1', i, j), d0 + ts[i] * d1)
                put(('Q3', i, j), d0 + ts[j] * d1)
        return fn

    pr = _FULL.pairs
    parts = [(_HALF, _HALF.pairs)]
    if J < SB - 1:
        parts += [(_FULL, x) for x in (None, pr[:2], [pr[2], pr[4]], [pr[3], pr[5]])]
    return [item(star, h, r0, pairs) for h in range(2) for r0 in range(0, HT, n) for star, pairs in parts]


def _job_order(nsb):
    units = [(I, h) for I in range(nsb) for h in range(2)]
    qe, qv = [], []
    for I, h in units:
        qe += [('e', I, h, J, p) for J in range(I) for p in range(SB)] + [('f', I, h)]
        qe += [('d', I, h) + c for c in _DCELLS]
        for i in range(SB):
            qv += [('p', I, h, f, J) for f in _FULL.products(i) for J in range(I)]
            if i >= 2:
                qv += [('p', I, h, f, None) for f in _HALF.products(i - 2)]
            qv += [('v', I, h) + c for c in _DCELLS if c[0] == i]
    qo = [('o', u, j) for j, (u, _) in enumerate(_O_JOBS)]
    cost = dict(e=8, f=8, d=2, p=1, v=2, o=2)
    order, done = [], {}
    now = [0]

    def emit(q):
        job = q.pop(0)
        order.append(job)
        now[0] += cost[job[0]]
        if job[0] == 'd':
            done[job] = now[0]
        elif job[0] == 'v' and job[4] == job[3]:
            done['u', 2 * (SB * job[1] + job[3]) + job[2]] = now[0]
        return cost[job[0]]

    def v_ready():
        if not qv:
            return False
        key = ('d', qv[0][1], qv[0][2], SB - 1, SB - 1)
        return key in done and done[key] + (LAT_0 if qv[0][1:3] == (0, 0) else LAT_A) <= now[0]

    def o_ready():
        return bool(qo) and ('u', qo[0][1]) in done and done['u', qo[0][1]] + LAT_B <= now[0]

    def fill(nv, no):
        n = 0
        while nv > 0 or no > 0 or n % 4:
            if no > 0 and n % 2 == 0 and o_ready() and no * ONV >= nv:
                no -= 2
                n += emit(qo)
            elif v_ready() and (nv > 0 or n % 4):
                c = emit(qv)
                nv -= c
                n += c
            elif o_ready() and n % 2 == 0 and (no > 0 or n % 4 or nv > 0) and len(qo) > RES:
                no -= 2
                n += emit(qo)
            else:
                break

    while qe:
        unit = qe[0][1:3]
        while qv and qv[0][2] == unit[1] and qv[0][1] < unit[0]:
            emit(qv)
        ne = 0
        while qe and ne < 8 and (ne == 0 or (qe[0][0] == 'd' and qe[0][1:3] == unit and ne + 2 <= 8)):
            ne += emit(qe)
        groups = lambda q: sum(cost[j[0]] for j in q) / 8
        old = [j for j in qv if j[1:3] != unit and ('d', j[1], j[2], SB - 1, SB - 1) in done]
        here = [j for j in qe if j[1:3] == unit]
        rest = sum(cost[j[0]] for j in old)
        nv = (rest - LAT_A) / (groups(here) + 1) if here else rest
        no = 2 * max(len(qo) - RES - OEND, 0) / (groups(qe) + 1)
        fill(int(nv + 0.5), int(no + 0.5))
    while qv or qo:
        if qv and v_ready():
            fill(TV, TO)
            if not qv:
                continue
        elif o_ready():
            emit(qo)
        else:
            emit(qv or qo)
    return order


def _attention_safe(q_scr, k_scr, v_scr, wo_ref, acc_scr):
    causal = (jax.lax.broadcasted_iota(jnp.int32, (T, T), 0)
              <= jax.lax.broadcasted_iota(jnp.int32, (T, T), 1))

    def unit(u, carry):
        r, hd = u // 2, u % 2

        def block(c, mlo):
            m0, l, o = mlo
            s = _dot_nt(_ld(k_scr, 2 * c + hd), _ld(q_scr, u))
            s = jnp.where(jnp.logical_or(causal, c < r), s, -1e9 * LOG2E)
            m = jnp.maximum(m0, jnp.max(s, axis=0, keepdims=True))
            a = jnp.exp2(m0 - m)
            p = jnp.exp2(s - m)
            return (m, l * a + jnp.sum(p, axis=0, keepdims=True),
                    o * a + _dot(_ld(v_scr, 2 * c + hd), p.astype(BF16)))

        _, l, o = jax.lax.fori_loop(0, r + 1, block, (jnp.full((1, T), -jnp.inf, F32), jnp.zeros((1, T), F32),
                                                      jnp.zeros((T, T), F32)))
        rows = pl.ds(pl.multiple_of(r * T, T), T)
        acc_scr[rows, :] += _dot((o * (1.0 / l)).astype(BF16).T, wo_ref[pl.ds(pl.multiple_of(hd * T, T), T), :])
        return carry

    jax.lax.fori_loop(0, q_scr.shape[0], unit, 0)


def _attention_step(q_scr, k_scr, v_scr, pf, wo_ref, acc_scr, flag_scr, z, side):
    causal = (jax.lax.broadcasted_iota(jnp.int32, (T, T), 0)
              <= jax.lax.broadcasted_iota(jnp.int32, (T, T), 1))
    HT = T // 2
    lsum, lrow, acc, fg, dacc, of, lhs = {}, {}, {}, {}, {}, {}, {}
    res = []
    wo, terms = {}, {}
    left = {}
    done_side = [0, 0]
    chk = [jnp.zeros((8, T), F32), None]
    for _, t in _O_JOBS:
        for _, i, j in t[2]:
            left[i, j] = left.get((i, j), 0) + 1

    def add_l(u, v):
        lsum[u] = v if u not in lsum else lsum[u] + v

    csign = {}

    def p_forms(star, h, slot0, g, tiles, cell, when):
        n = star.n

        def put(f, v):
            pf[h][slot0 + star.pf[f], 16 * g:16 * g + 16, :] = v.astype(BF16)

        for i in range(n):
            row = [cell(i, k) for k in sorted(range(n), key=lambda k: when(i, k))]
            r = functools.reduce(lambda x, y: x + y, row)
            put(('R', i), r)
            add_l(tiles[i], r[:8] + r[8:])
            col = sorted(range(n), key=lambda i2: (when(i2, i), i2 != i))
            sign = csign[n, i] = 1 if col[0] == i else -1
            c = cell(col[0], i)
            for i2 in col[1:]:
                c = c + cell(i2, i) if (1 if i2 == i else -1) == sign else c - cell(i2, i)
            put(('C', i), c)
            for j in range(n):
                if j != i:
                    put(('S', i, j), cell(i, j))
        for i, j in star.pairs:
            put(('A', i, j), cell(i, j) + cell(j, i))

    due = []

    def scores(x, u):
        if due and due[0][0] <= done_side[1]:
            x = _tie(x, due.pop(0)[1])
        s = (_dot if u in QT else _dot_nt)(x, _ld(q_scr, u))
        res.append(s)
        return s

    def job_e(I, h, J, p):
        tiles = [2 * (SB * I + i) + h for i in range(SB)]
        ps = []
        for i, u in enumerate(tiles):
            x = jnp.concatenate([k_scr.bitcast(U32)[2 * (SB * J + (t - i) % SB) + h, 8 * g:8 * g + 8, :]
                                 for g in (2 * p, 2 * p + 1) for t in range(SB)], axis=0)
            ps.append(jnp.exp2(scores(pltpu.bitcast(x, BF16), u)))
        when = lambda i, k: (i + k) % SB
        for n, g in enumerate((2 * p, 2 * p + 1)):
            cell = lambda i, k: ps[i][16 * (SB * n + when(i, k)):16 * (SB * n + when(i, k)) + 16]
            p_forms(_FULL, h, J * len(_FULL.pf), g, tiles, cell, when)

    def job_f(I, h):
        tiles = [2 * (SB * I + 2 + i) + h for i in range(2)]
        ps = {(i, k): jnp.exp2(scores(_ld(k_scr, 2 * (SB * I + k) + h), u))
              for i, u in enumerate(tiles) for k in range(2)}
        for g in range(T // 16):
            p_forms(_HALF, h, _HSLOT, g, tiles, lambda i, k: ps[i, k][16 * g:16 * g + 16], lambda i, k: 0)

    def job_d(I, h, i, k):
        u = 2 * (SB * I + i) + h
        s = scores(_ld(k_scr, 2 * (SB * I + k) + h), u)
        if i == k:
            s = jnp.where(causal, s, -1e9 * LOG2E)
        p = jnp.exp2(s)
        add_l(u, jnp.sum(p.reshape(T // 8, 8, T), axis=0))
        pf[h][_DSLOT + _DCELLS.index((i, k))] = p.astype(BF16)
        if (i, k) == _DCELLS[-1]:
            pf[h][_FENCE + z, 0:16, :] = jnp.zeros((16, T), BF16)
            for u in [2 * (SB * I + a) + h for a in range(SB)]:
                lrow[u] = jnp.sum(lsum.pop(u), axis=0, keepdims=True)
            ls = [lrow[2 * (SB * I + a) + h] for a in range(SB)]
            lo = jnp.minimum(jnp.minimum(ls[0], ls[1]), jnp.minimum(ls[2], ls[3]))
            hi = jnp.maximum(jnp.maximum(ls[0], ls[1]), jnp.maximum(ls[2], ls[3]))
            ok = jnp.logical_and(lo >= L_LO, hi <= L_HI)
            ok = jnp.logical_and(ok, (hi if I else jnp.maximum(ls[2], ls[3]))
                                 <= L_RATIO * (lo if I else jnp.minimum(ls[2], ls[3])))
            bad = jnp.where(ok, 0.0, 1.0)
            chk[1] = bad if chk[1] is None else jnp.maximum(chk[1], bad)

    def job_p(I, h, f, J):
        star, last = (_HALF, True) if J is None else (_FULL, J == I - 1)
        blk = I if J is None else J
        if f[0] == 'B':
            x = _ld(v_scr, 2 * (SB * blk + f[1]) + h, slice(HT // 2, HT))
        else:
            slot, r = _v_slot(star, blk, f)
            x = _ld(pf[h], slot, slice(r // 2, (r + HT) // 2))
        v = _dot(x, _ld(pf[h], (_HSLOT if J is None else J * len(_FULL.pf)) + star.pf[star.pv[f]]))
        res.append(v)
        key = (star.n,) + f
        acc[key] = v if key not in acc else acc[key] + v
        if not last:
            return

        def add(which, i, v, sign=1):
            k_ = (star.n, which, i)
            if k_ not in fg:
                fg[k_] = v if sign > 0 else -v
            else:
                fg[k_] = fg[k_] + v if sign > 0 else fg[k_] - v

        if f[0] == 'W':
            add('F', f[1], acc.pop(key))
        elif f[0] == 'B':
            add('G', f[1], acc.pop(key), csign[star.n, f[1]])
        elif f[0] == 'Q3':
            _, i, j = f
            q1, q2, q3 = (acc.pop((star.n, q, i, j)) for q in ('Q1', 'Q2', 'Q3'))
            t = ((q1 + q2) + q3) * (1.0 / (star.ts[i] - star.ts[j]))
            add('G', i, t)
            add('G', j, t)
            add('F', i, q1)
            add('F', j, q3, -1)

    def job_v(I, h, i, k):
        u = 2 * (SB * I + i) + h
        v = _dot(_ld(v_scr, 2 * (SB * I + k) + h), _ld(pf[h], _DSLOT + _DCELLS.index((i, k))))
        res.append(v)
        dacc[u] = v if u not in dacc else dacc[u] + v
        if k == i:
            o = dacc.pop(u)
            for star, a in ([(_FULL, i)] if I else []) + ([(_HALF, i - 2)] if i >= 2 else []):
                f, g = fg.pop((star.n, 'F', a)), fg.pop((star.n, 'G', a))
                o = o + jnp.concatenate([f - star.ts[a] * g, g], axis=0)
            o = o * (1.0 / lrow[u])
            of[u] = o
            chk[0] = chk[0] + jnp.sum(o.reshape(T // 8, 8, T), axis=0)

    def job_o(_, n):
        af, bf, outs = _O_JOBS[n][1]
        if af not in lhs:
            v = _form(af, lambda i, h: of[2 * i + h])
            lhs[af] = _tie(v.astype(BF16).T, v[0:8, :])
        if bf not in wo:
            wo[bf] = (wo_ref[_tile(bf[0][1]), _tile(bf[0][2])] if len(bf) == 1 else
                      _form(bf, lambda h, j: wo_ref[_tile(h), _tile(j)].astype(F32)).astype(BF16))
        v = _dot(lhs[af], wo[bf])
        res.append(v)
        for sign, i, j in outs:
            terms.setdefault((i, j), []).append((sign, v))
            if len(terms[i, j]) == left[i, j]:
                tot = acc_scr[_tile(i), _tile(j)]
                for sg, m in terms.pop((i, j)):
                    tot = tot + m if sg > 0 else tot - m
                acc_scr[_tile(i), _tile(j)] = tot

    fns = dict(e=job_e, f=job_f, d=job_d, p=job_p, v=job_v, o=job_o)
    order = _job_order(q_scr.shape[0] // (2 * SB))
    for n, job in enumerate(order):
        assert job[0] not in 'efd' or not any(j[0] in 'pv' and j[2] == job[2] and j[1] < job[1] for j in order[n:])
    side = list(side)
    fences = [n for n, job in enumerate(order) if job[0] == 'd' and job[3:] == _DCELLS[-1]]
    step = (len(order) - SIDE0 - SIDE1 - 10) / len(side)
    for n, job in enumerate(order):
        done_side[1] = n
        fns[job[0]](*job[1:])
        last_chance = n >= len(order) - SIDE1
        near = any(-SG1 <= f - n <= SG0 for f in fences)
        if side and n >= SIDE0 + step * done_side[0] and ((job[0] in 'pvo' and not near) or last_chance):
            done_side[0] += 1
            v = side.pop(0)(res[-1 - SLAG][8 * (n % 4):8 * (n % 4) + 8, :])
            if v is not None:
                due.append((n + SDUE, v))
    assert not side and not due
    fine = jnp.abs(chk[0]) < jnp.inf
    flag_scr[...] = jnp.maximum(flag_scr[...], jnp.where(fine, chk[1], 1.0))


def _kernel(x_hbm, c_hbm, wq_hbm, wuk_hbm, wuv_hbm, wo_hbm, w1_hbm, w2_hbm, w3_hbm, w4_hbm,
            cond_hbm, wmod_hbm, out_hbm,
            x_ref, c_ref, cond_ref, wma_ref, wmb_ref, w1_ref, w3_ref,
            wq_buf, wk_buf, wv_buf, wo_buf, out_buf, sem, wsem, osem,
            mod_scr, h_scr, cs_scr, hs_scr, w_scr, q_scr, k_scr, v_scr, acc_scr, xn_scr, xh_scr, a1_scr, t_scr,
            z_scr, mw_scr, m3_scr, wt_scr, wf_scr, gap_scr, st_in, pf_scr, vf_scr, flag_scr):
    S, M = x_hbm.shape
    D = wq_hbm.shape[2]
    nattn = wo_hbm.shape[0]
    Fd = w4_hbm.shape[0]
    scale = float(D) ** -0.5 * LOG2E
    nb, nrb = S // T, S // RB
    km, kc = M // T, c_hbm.shape[1] // T
    NX = 4
    XR = S // NX
    CB = XR // T

    work = (wk_buf, wv_buf, wq_buf)

    def pcopies(g, bufs=work, s0=0):
        return [pltpu.make_async_copy(src.bitcast(U32).at[:, g, :], dst, wsem.at[s0 + j])
                for j, (src, dst) in enumerate(zip((wuk_hbm, wuv_hbm, wq_hbm), bufs))]

    def ocopy(g):
        return pltpu.make_async_copy(wo_hbm.at[g], wo_buf, wsem.at[3])

    def chunk_copy(src, dst, i, s0):
        rows = slice(i * XR, (i + 1) * XR)
        return pltpu.make_async_copy(src.at[rows, :], dst.at[rows, :], sem.at[s0 + i])

    MS = 16
    NSL = T // MS
    assert nattn - 1 >= NSL
    mixw = ((w1_hbm, km, 0), (w2_hbm, km, km * MS), (w3_hbm, Fd // T, 2 * km * MS),
            (w4_hbm, -(-Fd // T), (2 * km + Fd // T) * MS))

    def prep_in(g):
        o = jnp.minimum(g, NSL - 1) * MS
        return [pltpu.make_async_copy(
            w.at[pl.ds(pl.multiple_of(jnp.minimum(b * T + o, w.shape[0] - MS), MS), MS), :],
            st_in.at[r0 + b * MS:r0 + (b + 1) * MS, :], wsem.at[7]) for w, nblk, r0 in mixw for b in range(nblk)]

    def stage_in(g):
        return pcopies(jnp.minimum(g + 1, nattn - 1))

    cp_cond = pltpu.make_async_copy(cond_hbm, cond_ref, sem.at[0])
    cp_wma = pltpu.make_async_copy(wmod_hbm.at[:, 0:2 * M], wma_ref, sem.at[1])
    cp_late = [pltpu.make_async_copy(src, dst, sem.at[2 + j]) for j, (src, dst) in enumerate((
        (wmod_hbm.at[:, 2 * M:6 * M], wmb_ref), (w1_hbm, w1_ref), (w3_hbm.at[Fd // T * T:, :], w3_ref)))]
    cp_x = [chunk_copy(x_hbm, x_ref, i, 7) for i in range(NX)]
    cp_c = [chunk_copy(c_hbm, c_ref, i, 7 + NX) for i in range(NX)]

    def silu_cond():
        cf = cond_ref[...].astype(F32)
        return jnp.broadcast_to((cf * jax.nn.sigmoid(cf)).astype(BF16), (8, M))

    cp_wk, cp_wv, cp_wq = pcopies(0)
    named = dict(k=cp_wk, v=cp_wv, q=cp_wq, o=ocopy(0), n=cp_cond, m=cp_wma)
    named.update(zip('abcd', cp_c))
    named.update(zip('wxyz', cp_x))
    started, arrived, did = set(), set(), set()

    def zero(r, carry):
        acc_scr[pl.ds(pl.multiple_of(r * T, T), T), :] = jnp.zeros((T, M), F32)
        return carry

    def x_rows(rows, dep):
        xf = x_ref[rows, :].astype(F32)
        if dep is None:
            return xf
        return jnp.concatenate([_after(xf[:, :T], _rows(dep, xf.shape[0])), xf[:, T:]], axis=1)

    def n_item(r, i):
        def fn(dep):
            rows = slice(r * T + i * LP, r * T + (i + 1) * LP)
            xn_scr[rows, :] = _ln(x_rows(rows, dep))
        return fn

    def h_item(r, i, normed):
        def fn(dep):
            rows = slice(i * LP, (i + 1) * LP)
            grows = slice(r * T + i * LP, r * T + (i + 1) * LP)
            sa = mod_scr[:, 0:M]
            if normed and dep is not None:
                sa = jnp.concatenate([_after(sa[:, _tile(j)], dep) for j in range(km)], axis=1)
            hf = ((xn_scr[grows, :] if normed else _ln(x_rows(grows, dep))) * _rows(mod_scr[:, M:2 * M], LP)
                  + _rows(sa, LP))
            for j in range(km):
                h_scr[r, j, rows, :] = hf[:, _tile(j)].astype(BF16)
            for f, n in _H_SUMS.items():
                if all(t[1] == r for t in f):
                    hs_scr[n, rows, :] = _form(f, lambda _, k: hf[:, _tile(k)]).astype(BF16)
            did.add(('h', r, i))
        return fn

    def release(jobs, span, items):
        if span and items:
            jobs.side += [(len(jobs.res) + 1 + i * span // len(items), fn) for i, fn in enumerate(items)]
            jobs.side.sort(key=lambda e: e[0])
        else:
            for fn in items:
                fn(None)

    def sum_items(n, group, index, dst, get, skip_rows):
        forms = [f for f in dict.fromkeys(t[0] for t in group)
                 if len(f) > 1 and not (skip_rows and len({t[1] for t in f}) == 1)]

        def item(f, rows):
            def fn(dep):
                def term(r, k):
                    v = get(r, k, rows).astype(F32)
                    return v if dep is None or (r, k) != f[0][1:] else _after(v, _rows(dep, v.shape[0]))
                dst[index[f], rows, :] = _form(f, term).astype(BF16)
            return fn

        return [item(f, slice(i, i + n)) for i in range(0, T, n) for f in forms]

    h_sums = lambda n, gi: sum_items(n, _H_GROUPS[gi], _H_SUMS, hs_scr,
                                     lambda r_, k, rows: h_scr[r_, k, rows, :], True)

    def stash(key, buf, j0, transpose=False):
        n = buf.shape[0] // T
        if key not in did:
            assert key in arrived
            did.add(key)
            for (j, hd), w in _pair_tiles(buf, transpose).items():
                w_scr[hd, j0 + j] = w
        return lambda hd: [_ld(w_scr, hd, j0 + j) for j in range(n)]

    def kv_tile(jobs, r):
        wk, wvT = stash('k', wk_buf, 0), stash('v', wv_buf, kc, True)
        ct = [c_ref[_tile(r), _tile(j)] for j in range(kc)]
        for hd in range(2):
            k_scr[2 * r + hd] = jobs.mm(ct, wk(hd), _dot).astype(BF16)
        for hd in range(2):
            v_scr[2 * r + hd] = jobs.mm(wvT(hd), ct, _dot_nt).astype(BF16)

    def q_tile(jobs, r):
        wq = stash('q', wq_buf, 2 * kc)
        ht = [_ld(h_scr, r, j) for j in range(km)]
        for hd in range(2):
            v = (jobs.mm(ht, wq(hd), _dot) * scale).astype(BF16)
            q_scr[2 * r + hd] = v.T if 2 * r + hd in QT else v

    for blk in _prologue().split(';'):
        waits, starts, acts = blk.split('|')
        for ch in waits.strip():
            assert ch in started and ch not in arrived
            arrived.add(ch)
            named[ch].wait()
        for ch in starts.strip():
            assert ch not in started
            started.add(ch)
            named[ch].start()
        jobs = _Jobs()
        for act in acts.split():
            if act == 'Z':
                jax.lax.fori_loop(0, nb, zero, 0)
                acc_scr[S:, :] = jnp.zeros((acc_scr.shape[0] - S, M), F32)
                x_ref[S:, :] = jnp.zeros((x_ref.shape[0] - S, M), BF16)
                flag_scr[...] = jnp.zeros(flag_scr.shape, F32)
            elif act == 'L':
                did.add('L')
                assert ('Q', 0) in did
                for cp in stage_in(0) + prep_in(0):
                    cp.start()
            elif act == 'M':
                assert arrived >= set('nm')
                mod = _dot(silu_cond(), wma_ref[...])
                mod_scr[:, 0:M] = mod[:, 0:M]
                mod_scr[:, M:2 * M] = 1.0 + mod[:, M:2 * M]
                did.add('M')
            else:
                act, _, span = act.partition('@')
                span = int(span or 0)
                items = []
                for r in [int(ch, 16) for ch in act[1:]]:
                    did.add((act[0], r))
                    if act[0] == 'K':
                        assert 'abcd'[r // CB] in arrived
                        kv_tile(jobs, r)
                    elif act[0] == 'H':
                        assert 'wxyz'[r // CB] in arrived and 'M' in did
                        items += [h_item(r, i, ('N', r) in did) for i in range(T // LP)]
                    elif act[0] == 'N':
                        assert 'wxyz'[r // CB] in arrived
                        items += [n_item(r, i) for i in range(T // LP)]
                    elif act[0] == 'Q':
                        assert all(('h', r, i) in did for i in range(T // LP))
                        q_tile(jobs, r)
                    elif act[0] == 'Y':
                        def zero_item(n0):
                            def fn(dep):
                                zero = jnp.where(dep > jnp.inf, jnp.uint32(1), jnp.uint32(0))
                                for n in range(n0, min(n0 + 4, _MIX3 + m3_scr.shape[0])):
                                    mw_scr.bitcast(U32)[n] = _rows(zero, T // 2)
                            return fn
                        items += [zero_item(n0) for n0 in range(_MIX3, _MIX3 + m3_scr.shape[0], 4)]
                    elif act[0] == 'F':
                        assert all(('K', SB * r + k_) in did for k_ in range(SB))
                        items += _v_form_items(v_scr, (pf_scr, vf_scr), r)
                    elif act[0] == 'C':
                        assert all('abcd'[t[1] // CB] in arrived for p_ in _C_GROUPS[r] for t in p_[0])
                        items += sum_items(
                            32, _C_GROUPS[r], _C_SUMS, cs_scr,
                            lambda r_, k, rows: c_ref[r_ * T + rows.start:r_ * T + rows.stop, _tile(k)], False)
                    else:
                        assert act[0] == 'S' and all(('h', t[1], T // LP - 1) in did for p_ in _H_GROUPS[r] for t in p_[0])
                        items += h_sums(32 if span else 16, r)
                release(jobs, span, items)
        assert not jobs.side
    assert arrived == set(named) and all((k_, r) in did for k_ in 'KHQ' for r in range(nb))
    assert all((k_, r) in did for k_ in 'CS' for r in range(2)) and 'L' in did
    assert all(('F', r) in did for r in range(SB))

    def mixer_prep(g):
        sl = jnp.minimum(g, NSL - 1)
        rows = pl.ds(pl.multiple_of(sl * MS, MS), MS)

        def part(m, forms):
            def fn(dep):
                base = {}

                def get(i, k):
                    if (i, k) not in base:
                        rb, cb = (i, k) if m == 2 else (k, i)
                        r0 = mixw[m][2] + rb * MS
                        v = _after(st_in[r0:r0 + MS, _tile(cb)].astype(F32), _rows(dep, MS))
                        if m == 3 and (rb + 1) * T > Fd:
                            v = jnp.where(rb * T + sl * MS < Fd, v, 0.0)
                        base[i, k] = v
                    return base[i, k]

                for f in forms:
                    v = _form(f, get)
                    mw_scr[_MIXW[m, f], rows, :] = (0.5 * v if m % 2 else v).astype(BF16)
            return fn

        items = []
        for m in range(4):
            forms = [f for mm_, f in _MIXW if mm_ == m]
            cur, terms = [], set()
            for f in forms:
                new_terms = terms | {t[1:] for t in f}
                if cur and 3 * len(new_terms) + sum(2 * len(x) + 1 for x in cur + [f]) > MWOPS:
                    items.append(part(m, cur))
                    cur, terms = [], set()
                cur.append(f)
                terms |= {t[1:] for t in f}
            items.append(part(m, cur))

        n3 = sum(m == 2 for m, _ in _MIXW)
        first = min(n for (m, _), n in _MIXW.items() if m == 2)
        per = -(-n3 // (nattn - 1 - NSL))

        def turn(j):
            def fn(dep):
                n = jnp.minimum(jnp.maximum(g - NSL, 0) * per + j, n3 - 1)
                w = _tie(_ld(mw_scr, first + n), dep).T
                m3_scr[n] = w
                return pltpu.bitcast(pltpu.bitcast(w, U32)[T // 2 - 8:], F32)
            return fn

        return items + [turn(j) for j in range(per)]

    def stage_wait():
        for cp in pcopies(0):
            cp.wait()
        pltpu.make_async_copy(st_in, st_in, wsem.at[7]).wait()

    def attn_body(g, carry):
        side = _gap_items(work, gap_scr) + _weight_form_items(work, gap_scr, wt_scr, wf_scr)
        bufs = (q_scr, k_scr, v_scr, (pf_scr, vf_scr), wo_buf, acc_scr, flag_scr)
        _attention_step(*bufs, g >> 16, side)

        @pl.when(g + 1 < nattn)
        def _():
            copies = stage_in(g + 1) + [ocopy(g + 1)]
            for cp in copies:
                cp.start()
            bufs = (h_scr, hs_scr, c_ref, cs_scr, wf_scr, q_scr, k_scr, v_scr, (pf_scr, vf_scr))
            side = [(SD0 + int(i * SDS), fn) for i, fn in enumerate(mixer_prep(g))]
            _proj_step(*bufs, scale, gap_scr, side)
            for cp in prep_in(g + 1):
                cp.start()
            stage_wait()
            ocopy(g + 1).wait()

        return carry

    stage_wait()
    for cp in cp_late:
        cp.start()
    jax.lax.fori_loop(0, nattn, attn_body, 0)

    def safe_pair(g, carry):
        copies = pcopies(g) + [ocopy(g)]
        for cp in copies:
            cp.start()
        for cp in copies:
            cp.wait()
        for buf, j0, transpose in ((wk_buf, 0, False), (wv_buf, kc, True), (wq_buf, 2 * kc, False)):
            for (j, hd), w in _pair_tiles(buf, transpose).items():
                w_scr[hd, j0 + j] = w

        def tile(u, carry):
            r, hd = u // 2, u % 2
            rows = pl.ds(pl.multiple_of(r * T, T), T)
            ct = [c_ref[rows, _tile(j)] for j in range(kc)]
            k_scr[u] = sum(_dot(ct[j], _ld(w_scr, hd, j)) for j in range(kc)).astype(BF16)
            v_scr[u] = sum(_dot_nt(_ld(w_scr, hd, kc + j), ct[j]) for j in range(kc)).astype(BF16)
            q = sum(_dot(_ld(h_scr, r, j), _ld(w_scr, hd, 2 * kc + j)) for j in range(km))
            q_scr[u] = (q * scale).astype(BF16)
            return carry

        jax.lax.fori_loop(0, 2 * nb, tile, 0)
        _attention_safe(q_scr, k_scr, v_scr, wo_buf, acc_scr)
        return carry

    @pl.when(jnp.max(flag_scr[...]) > 0)
    def _():
        jax.lax.fori_loop(0, nb, zero, 0)
        jax.lax.fori_loop(0, nattn, safe_pair, 0)

    for cp in cp_late:
        cp.wait()
    mod = _dot(silu_cond(), wmb_ref[...])
    mod_scr[:, 2 * M:4 * M] = mod[:, 0:2 * M]
    mod_scr[:, 4 * M:5 * M] = 1.0 + mod[:, 2 * M:3 * M]
    mod_scr[:, 5 * M:6 * M] = mod[:, 3 * M:4 * M]
    OFF = x_ref.shape[0] - S
    CAR = t_scr.shape[0] - RB

    def p1(r0, l0, n, dep=None):
        ga = mod_scr[:, 2 * M:3 * M]
        if dep is not None:
            ga = jnp.concatenate([_after(ga[:, 0:T], dep), ga[:, T:]], axis=1)
        rows = pl.ds(r0, n)
        x1 = x_ref[rows, :].astype(F32) + _rows(ga, n) * acc_scr[rows, :]
        xh_scr[0, l0:l0 + n, :] = x1
        hb = _ln(x1) * _rows(mod_scr[:, 4 * M:5 * M], n) + _rows(mod_scr[:, 3 * M:4 * M], n)
        xh_scr[1, l0:l0 + n, :] = hb
        return hb

    HT = T // 2
    last8 = lambda v: jnp.max(v[:, M - T:].reshape(PC // 8, 8, T), axis=0)

    def p1_store(r0, c, dep=None):
        v = _ln(p1(r0 + c * PC, OFF + c * PC, PC, dep))
        a1_scr[c * PC:(c + 1) * PC, :] = v
        return last8(v)

    def p1_first(r0, c, dep):
        return last8(p1(r0 + c * PC, OFF + c * PC, PC, dep))

    def p1_second(c, dep):
        hb = xh_scr[1, OFF + c * PC:OFF + (c + 1) * PC, :]
        v = _ln(jnp.concatenate([_after(hb[:, :T], _rows(dep, PC)), hb[:, T:]], axis=1))
        a1_scr[c * PC:(c + 1) * PC, :] = v
        return last8(v)

    t_scr[RB:RB + CAR - OFF, :] = jnp.zeros((CAR - OFF, M), F32)
    t_scr[RB + CAR - OFF:RB + CAR, :] = _gelu2(_dot(_ln(p1(0, 0, OFF)).astype(BF16), w1_ref[...]))
    for c in range(RB // PC):
        p1_store(OFF, c)

    def out_copy(i):
        rows = pl.ds(i * T if isinstance(i, int) else pl.multiple_of(i * T, T), T)
        return pltpu.make_async_copy(out_buf.at[rows, :], out_hbm.at[rows, :], osem.at[i])

    def b_body(r, carry):
        gb = _rows(mod_scr[:, 5 * M:6 * M], T)
        r0 = pl.multiple_of(r * RB, RB)
        n0 = pl.multiple_of(jnp.minimum(r0 + RB, S - RB) + OFF, OFF)
        nh = RB // T
        now = [0]
        due = []
        pace = []

        def p1_item(c, part):
            def fn(dep):
                v = p1_first(n0, c, dep) if part == 0 else p1_second(c, dep)
                due.append((now[0] + PD, v))
                due.sort(key=lambda e: e[0])
            return fn

        pace += [(P0 + i * PSTEP + part * PSPLIT, p1_item(i, part)) for i in range(RB // PC)
                 for part in range(2)]
        pace.sort(key=lambda e: e[0])

        def mm(lhs, wts, dot=_dot):
            acc = None
            for x, w in zip(lhs, wts):
                if due and due[0][0] <= now[0]:
                    w = _tie(w, due.pop(0)[1])
                v = dot(x, w)
                now[0] += x.shape[0] // HT
                acc = v if acc is None else v + acc
                if pace and pace[0][0] <= now[0]:
                    pace.pop(0)[1](v[0:8, :])
            return acc

        def fast(m, base, finish, hook=None):
            prods = _MIX[m]
            left, acc, done, cache = {}, {}, {}, {}
            for _, _, outs in prods:
                for _, i, h in outs:
                    left[i, h] = left.get((i, h), 0) + 1

            def act(form):
                sign, form = _canon(form)
                if form not in cache:
                    cache[form] = _form(form, lambda k, h: base(k)[h * HT:(h + 1) * HT]).astype(BF16)
                return sign, cache[form]

            for pi, (wf, af, outs) in enumerate(prods):
                w = _ld(m3_scr, _MIXW[m, wf] - _MIX3) if m == 2 else _ld(mw_scr, _MIXW[m, wf])
                if af is None:
                    k = wf[0][2]
                    v = mm([jnp.concatenate([act(((1, k, h),))[1] for h in range(2)], axis=0)], [w])
                    sign, parts = 1, [v[:HT], v[HT:]]
                else:
                    sign, x = act(af)
                    parts = [mm([x], [w])] * len(outs)
                for (s_, i, h), v in zip(outs, parts):
                    s_ = s_ * sign
                    if (i, h) not in acc:
                        acc[i, h] = (s_, v)
                    else:
                        s0, u = acc[i, h]
                        acc[i, h] = (s0, u + v if s0 == s_ else u - v) if s0 > 0 or s_ < 0 else (1, v - u)
                    left[i, h] -= 1
                    if not left[i, h]:
                        s0, done[i, h] = acc.pop((i, h))
                        assert s0 > 0
                        if (i, 1 - h) in done:
                            finish(i, jnp.concatenate([done[i, 0], done[i, 1]], axis=0))
                if hook is not None:
                    hook(pi, act)

        t_scr[0:CAR, :] = t_scr[RB:RB + CAR, :]
        for hf in range(nh):
            def put_t(n, v):
                t = _gelu2(v)
                if hf == nh - 1:
                    t = jnp.concatenate([t[:T - OFF], jnp.where(r < nrb - 1, t[T - OFF:], 0.0)], axis=0)
                t_scr[CAR + hf * T:CAR + (hf + 1) * T, _tile(n)] = t

            fast(0, lambda k: a1_scr[_tile(hf), _tile(k)], put_t)
        cq = M // 4
        shifts = (-1, 1, -2, 2)
        lane = jax.lax.broadcasted_iota(jnp.int32, (T, T), 1)
        y1, a3 = [], []
        for hf in range(nh):
            base = CAR - OFF + hf * T
            sh = []
            for j in range(km):
                g_lo, g_hi = (j * T) // cq, ((j + 1) * T - 1) // cq
                assert g_hi - g_lo <= 1

                def shifted(d):
                    v = t_scr[base - 8:base + T + 8, _tile(j)]
                    return pltpu.roll(v, (-d) % (T + 16), 0)[8:8 + T]

                v = shifted(shifts[g_lo])
                if g_hi != g_lo:
                    v = jnp.where(lane < g_hi * cq - j * T, v, shifted(shifts[g_hi]))
                sh.append(v)
            hs = {}
            fast(1, lambda k: sh[k], hs.__setitem__)
            hs = jnp.concatenate([hs[n] for n in range(km)], axis=1)
            y1.append(hs + xh_scr[1, _tile(hf), :])
            z_scr[_tile(hf), :] = xh_scr[0, _tile(hf), :] + gb * y1[hf]
            a3.append({})

            def ln_item(hf, c):
                def item(dep):
                    n = HT // NLN
                    for d in (0, HT):
                        v = y1[hf][d + c * n:d + (c + 1) * n]
                        if dep is not None:
                            v = jnp.concatenate([_after(v[:, :T], _rows(dep, n)), v[:, T:]], axis=1)
                        a3[hf][d + c * n] = _ln(v)
                return item

            ln_item(hf, 0)(None)
            pace += [(now[0] + LN0 + (c - 1) * LNS * (1 + hf), ln_item(hf, c)) for c in range(1, NLN)]
            pace.sort(key=lambda e: e[0])
        xh_scr[:, 0:OFF, :] = xh_scr[:, RB:RB + OFF, :]
        z_scr[pl.ds(pl.multiple_of(RB + (r >> 16) * 8, 8), 8), :] = jnp.zeros((8, M), F32)
        h3 = []
        for hf in range(nh):
            assert len(a3[hf]) == 2 * NLN
            af = jnp.concatenate([a3[hf][key] for key in sorted(a3[hf])], axis=0)
            row = {}
            narrow = []

            def hook(pi, act):
                j, rem = divmod(pi - NAR0, NARS)
                if rem == 0 and 0 <= j < km:
                    full = jnp.concatenate([act(((1, j, h),))[1] for h in range(2)], axis=0)
                    v = mm([w3_ref[:, _tile(j)]], [full], _dot_nt)
                    narrow[:] = [v + narrow[0] if narrow else v]

            def put_h(n, v):
                row[n] = _gelu2(v)
                if GD:
                    due.append((now[0] + GD, jnp.max(row[n].reshape(T // 8, 8, T), axis=0)))
                    due.sort(key=lambda e: e[0])

            fast(2, lambda k: af[:, _tile(k)], put_h, hook)
            fw = w3_ref.shape[0]
            row[Fd // T] = jnp.concatenate([_gelu2(narrow[0]), jnp.zeros((T - fw, T), F32)], axis=0).T
            h3.append(row)
        for hf in range(nh):
            rows = pl.ds(pl.multiple_of(r0 + hf * T, T), T)

            def finish(n, v):
                out_buf[rows, _tile(n)] = (z_scr[_tile(hf), _tile(n)] + gb[:, _tile(n)] * v).astype(out_buf.dtype)
                pltpu.make_async_copy(out_buf.at[rows, _tile(n)], out_hbm.at[rows, _tile(n)],
                                      osem.at[r * nh + hf]).start()

            fast(3, lambda k: h3[hf][k], finish)
        assert not pace
        return carry

    jax.lax.fori_loop(0, nrb, b_body, 0)
    for i in range(nb):
        out_copy(i).wait()


@jax.jit
def pallas_adaLN_cond__compressed_kv_cla__mixer_s_mlp__prompt_kernel(
    A_x: jax.Array,
    A_c_kv: jax.Array,
    A_w_q: jax.Array,
    A_w_uk: jax.Array,
    A_w_uv: jax.Array,
    A_w_o: jax.Array,
    B_x: jax.Array,
    B_w1: jax.Array,
    B_w2: jax.Array,
    B_w3: jax.Array,
    B_w4: jax.Array,
    c: jax.Array,
    w_mod: jax.Array,
):
    _, S, M = A_x.shape
    Dc = A_c_kv.shape[2]
    H, D = A_w_q.shape[1], A_w_q.shape[2]
    Fd = B_w3.shape[1]
    assert D == T and A_c_kv.shape[1] == S and Dc == 4 * T and M == 5 * T and 13 * T < Fd < 14 * T and S == 16 * T
    vmem = pltpu.VMEM
    packed = lambda *lead: vmem(lead + (T, T), BF16)
    out = pl.pallas_call(
        _kernel,
        in_specs=[pl.BlockSpec(memory_space=pltpu.HBM)] * 12,
        out_specs=pl.BlockSpec(memory_space=pltpu.HBM),
        out_shape=jax.ShapeDtypeStruct((S, M), A_x.dtype),
        scratch_shapes=[
            vmem((S + 16, M), BF16),
            vmem((S, Dc), BF16),
            vmem((1, M), BF16),
            vmem((M, 2 * M), BF16),
            vmem((M, 4 * M), BF16),
            vmem((M, M), BF16),
            vmem((Fd % T, M), BF16),
            vmem((M, D), U32),
            vmem((Dc, D), U32),
            vmem((Dc, D), U32),
            vmem((2 * D, M), BF16),
            vmem((S, M), A_x.dtype),
            pltpu.SemaphoreType.DMA((15,)),
            pltpu.SemaphoreType.DMA((8,)),
            pltpu.SemaphoreType.DMA((S // T,)),
            vmem((8, 6 * M), F32),
            vmem((S // T, M // T, T, T), BF16),
            vmem((len(_C_SUMS), T, T), BF16),
            vmem((len(_H_SUMS), T, T), BF16),
            packed(2, M // T + 2 * (Dc // T)),
            packed(2 * S // T),
            packed(2 * S // T),
            packed(2 * S // T),
            vmem((S + 16, M), F32),
            vmem((S, M), F32),
            vmem((2, RB + 16, M), F32),
            vmem((RB, M), F32),
            vmem((RB + 32, M), F32),
            vmem((RB + 8, M), F32),
            packed(len(_MIXW)),
            packed(sum(m == 2 for m, _ in _MIXW)),
            vmem((Dc // T, T, T), U32),
            vmem((len(_WF), T, T), BF16),
            vmem((3, 8, T), jnp.int32),
            vmem(((2 * (M // T) + Fd // T + -(-Fd // T)) * 16, M), BF16),
            vmem((_FENCE + 1, T, T), BF16),
            vmem((_FENCE + 1, T, T), BF16),
            vmem((8, T), F32),
        ],
        compiler_params=pltpu.CompilerParams(
            vmem_limit_bytes=100 * 1024 * 1024,
            disable_bounds_checks=True,
        ),
    )(
        A_x.reshape(S, M), A_c_kv.reshape(S, Dc),
        A_w_q, A_w_uk, A_w_uv,
        A_w_o.reshape(H // 2, 2 * D, M),
        B_w1, B_w2, B_w3.T, B_w4, c, w_mod,
    )
    return out.reshape(1, S, M)
```
